```python
import jax
import jax.numpy as jnp

def _softmax(x, axis=-1):
    return jax.nn.softmax(x, axis=axis)
def _gelu(x):
    return jax.nn.gelu(x, approximate=True)
def _silu(x):
    return jax.nn.silu(x)
def _sigmoid(x):
    return jax.nn.sigmoid(x)
def _layernorm(x, axis=-1, eps=1e-5):
    m = jnp.mean(x, axis=axis, keepdims=True)
    v = jnp.var(x, axis=axis, keepdims=True)
    return (x - m) / jnp.sqrt(v + eps)
def _scatter_add(tgt, idx, src, axis=0):
    return tgt.at[idx].add(src)
def _segment_sum(src, seg, n):
    return jax.ops.segment_sum(src, seg, n)
class _Rng:
    def __init__(self, key):
        self._k = key
    def _next(self):
        self._k, sub = jax.random.split(self._k)
        return sub
    def normal(self, shape):
        return jax.random.normal(self._next(), shape, dtype=jnp.bfloat16)
    def randint(self, lo, hi, shape):
        return jax.random.randint(self._next(), shape, lo, hi, dtype=jnp.int32)
    def uniform(self, shape, lo=0.0, hi=1.0):
        return jax.random.uniform(self._next(), shape, jnp.bfloat16, lo, hi)
    def permutation(self, n):
        return jax.random.permutation(self._next(), n)


kernel_name = 'standalone__dcn_v2_cross__recsys'

def setup_inputs():
    _rng = _Rng(jax.random.key(int.from_bytes(__import__("os").urandom(4), "little")))
    _w = (lambda a: (lambda t: t.astype(jnp.bfloat16) if jnp.issubdtype(t.dtype, jnp.floating) else t)(jnp.asarray(a)))
    B, F, D, L = 16384, 26, 128, 6
    Din = min(F * D, 1024)
    return {
        "x0": _w((lambda *s: _rng.normal(s) * 0.05)(B, Din)),
        "ws": _w((lambda *s: _rng.normal(s) * 0.05)(L, Din, Din)),
        "bs": _w((lambda *s: _rng.normal(s) * 0.05)(L, Din)),
    }

def reference(x0, ws, bs):
    x = x0
    for l in range(ws.shape[0]):
        x = x0 * (x @ ws[l] + bs[l]) + x
    return x
```

```python
import functools
import jax
import jax.numpy as jnp
import jax.experimental.pallas as pl
import jax.experimental.pallas.tpu as pltpu

f32 = jnp.float32
bf16 = jnp.bfloat16

def _dot(a, b):
    return jnp.dot(a, b, preferred_element_type=f32)

LA = {1: [((0, 0), 1), ((1, 1), 1)], 2: [((1, 0), 1), ((1, 1), 1)], 3: [((0, 0), 1)],
      4: [((1, 1), 1)], 5: [((0, 0), 1), ((0, 1), 1)], 6: [((1, 0), 1), ((0, 0), -1)],
      7: [((0, 1), 1), ((1, 1), -1)]}
LB = {1: [((0, 0), 1), ((1, 1), 1)], 2: [((0, 0), 1)], 3: [((0, 1), 1), ((1, 1), -1)],
      4: [((1, 0), 1), ((0, 0), -1)], 5: [((1, 1), 1)], 6: [((0, 0), 1), ((0, 1), 1)],
      7: [((1, 0), 1), ((1, 1), 1)]}

SCHED_X = [
    (3, [('m3', [(1, 'm')])], []),
    (5, [('m5', [(1, 'm')])], [((0, 1), [(1, 'm'), (1, 'm3')])]),
    (2, [('m2', [(1, 'm')])], []),
    (4, [('u', [(1, 'm'), (-1, 'm5')])], [((1, 0), [(1, 'm'), (1, 'm2')])]),
    (1, [('m1', [(1, 'm')])], []),
    (6, [], [((1, 1), [(1, 'm'), (1, 'm1'), (-1, 'm2'), (1, 'm3')])]),
    (7, [], [((0, 0), [(1, 'm'), (1, 'm1'), (1, 'u')])]),
]
SCHED_Y = [
    (4, [('m4', [(1, 'm')])], []),
    (2, [('m2', [(1, 'm')])], [((1, 0), [(1, 'm'), (1, 'm4')])]),
    (5, [('m5', [(1, 'm')])], []),
    (3, [('u', [(1, 'm'), (-1, 'm2')])], [((0, 1), [(1, 'm'), (1, 'm5')])]),
    (1, [('m1', [(1, 'm')])], []),
    (7, [], [((0, 0), [(1, 'm'), (1, 'm1'), (-1, 'm5'), (1, 'm4')])]),
    (6, [], [((1, 1), [(1, 'm'), (1, 'm1'), (1, 'u')])]),
]
SLOTS = {'m3': 0, 'm4': 0, 'm5': 1, 'm2': 2, 'u': 3, 'm1': 4}

def lincomb(terms):
    terms = sorted(terms, key=lambda t: -t[0])
    assert terms[0][0] == 1
    acc = terms[0][1]
    for s, v in terms[1:]:
        acc = acc + v if s == 1 else acc - v
    return acc

NX = 3 * 16
NI = 2 * 5
NO = 5 * 4

def _kernel(x0_ref, w_ref, b_ref, o_ref, t_ref, z_ref, *bufs, L, TM, D, RC, LA_AHEAD, NZ):
    H = D // 4
    Mh = TM // 4
    xb = bufs[:NX]
    ib = bufs[NX:NX + NI]
    ob = bufs[NX + NI:NX + NI + NO]

    @pl.when(pl.program_id(0) == 0)
    def _():
        for k in range(NZ):
            z_ref[k] = 0
        def prep(l, c):
            blk = lambda r, cc: w_ref[l, r * H:(r + 1) * H, cc * H:(cc + 1) * H].astype(f32)
            for p in range(1, 8):
                sub = {(i, j): lincomb([(s, blk(2 * I + i, 2 * J + j)) for (I, J), s in LB[p]])
                       for i in range(2) for j in range(2)}
                for q in range(1, 8):
                    v = lincomb([(s, sub[ij]) for ij, s in LB[q]])
                    t_ref[l, (p - 1) * 7 + q - 1] = pltpu.bitcast(v.astype(bf16), jnp.uint32)
            return c
        jax.lax.fori_loop(0, L, prep, 0)

    zs = z_ref[0]
    zls = [z_ref[k] for k in range(1, NZ)]
    cnt = [0]
    def newzl():
        cnt[0] += 1
        return zls[cnt[0] % len(zls)]

    def ld(buf, r, zl):
        return buf[zl, r:r + RC, :]

    def st(buf, r, v):
        buf[zs, r:r + RC, :] = v

    def X(b, R, C):
        return xb[b * 16 + R * 4 + C]

    def t_load(l, k):
        return pltpu.bitcast(t_ref[l, k], bf16)

    def xbuf(l):
        return 0 if l == 0 else 1 + (l - 1) % 2

    x0_done = set()
    def ensure_x0(R, C):
        if (R, C) in x0_done:
            return
        x0_done.add((R, C))
        for r in range(0, Mh, RC):
            st(X(0, R, C), r, x0_ref[R * Mh + r:R * Mh + r + RC, C * H:(C + 1) * H].astype(f32))

    def make_lhs(l, p, q):
        src = xbuf(l)
        blocks = [(s1 * s2, 2 * I + i, 2 * J + j) for (I, J), s1 in LA[p] for (i, j), s2 in LA[q]]
        if l == 0:
            if len(blocks) == 1:
                _, R, C = blocks[0]
                return x0_ref[R * Mh:(R + 1) * Mh, C * H:(C + 1) * H]
            for _, R, C in blocks:
                ensure_x0(R, C)
        zl = newzl()
        chunks = []
        for r in range(0, Mh, RC):
            chunks.append(lincomb([(s, ld(X(src, R, C), r, zl)) for s, R, C in blocks]))
        v = jnp.concatenate(chunks, axis=0) if len(chunks) > 1 else chunks[0]
        return v.astype(bf16)

    def consume(n, l, po, qi, m):
        p, ostores, ofinals = po
        q, istores, ifinals = qi
        par = (n // 7) % 2
        zl = newzl()
        bias = {}
        for (i, j), _ in ifinals:
            if p in (3, 4):
                J = 1 if p == 3 else 0
                c0 = (2 * J + j) * H
                bias[j] = b_ref[l, :, c0:c0 + H].astype(f32)
            for (I, J), _ in ofinals:
                if l == 0:
                    ensure_x0(2 * I + i, 2 * J + j)
        for r in range(0, Mh, RC):
            mv = m[r:r + RC, :]
            val = lambda src: mv if src == 'm' else ld(ib[par * 5 + SLOTS[src]], r, zl)
            fin = [(ij, lincomb([(s, val(src)) for s, src in terms])) for ij, terms in ifinals]
            stl = [(name, lincomb([(s, val(src)) for s, src in terms])) for name, terms in istores]
            for name, v in stl:
                st(ib[par * 5 + SLOTS[name]], r, v)
            for (i, j), d in fin:
                if p in (3, 4):
                    d = d + bias[j]
                oval = lambda src: d if src == 'm' else ld(ob[SLOTS[src] * 4 + i * 2 + j], r, zl)
                ofin = [(IJ, lincomb([(s, oval(src)) for s, src in terms])) for IJ, terms in ofinals]
                ost = [(name, lincomb([(s, oval(src)) for s, src in terms])) for name, terms in ostores]
                for name, v in ost:
                    st(ob[SLOTS[name] * 4 + i * 2 + j], r, v)
                for (I, J), y in ofin:
                    R = 2 * I + i
                    C = 2 * J + j
                    x0v = ld(X(0, R, C), r, zl)
                    xv = x0v if l == 0 else ld(X(xbuf(l), R, C), r, zl)
                    xn = x0v * y + xv
                    if l == L - 1:
                        o_ref[R * Mh + r:R * Mh + r + RC, C * H:(C + 1) * H] = xn.astype(o_ref.dtype)
                    else:
                        st(X(xbuf(l + 1), R, C), r, xn)

    seq = []
    for l in range(L):
        so = SCHED_X if l % 2 == 0 else SCHED_Y
        for po in so:
            si = SCHED_X if l % 2 == 0 else SCHED_Y
            for qi in si:
                seq.append((l, po, qi))

    if LA_AHEAD == 0:
        for n, (l, po, qi) in enumerate(seq):
            lhs = make_lhs(l, po[0], qi[0])
            m = _dot(lhs, t_load(l, (po[0] - 1) * 7 + qi[0] - 1))
            consume(n, l, po, qi, m)
    else:
        prev = None
        for n, (l, po, qi) in enumerate(seq):
            lhs = make_lhs(l, po[0], qi[0])
            m = _dot(lhs, t_load(l, (po[0] - 1) * 7 + qi[0] - 1))
            if prev is not None:
                consume(*prev)
            prev = (n, l, po, qi, m)
        consume(*prev)

@jax.jit
def pallas_standalone__dcn_v2_cross__recsys_kernel(x0, ws, bs):
    TM, RC, LA_AHEAD, NZ = 512, 128, 0, 2
    B, D = x0.shape
    L = ws.shape[0]
    H = D // 4
    bs3 = bs.reshape(L, 1, D)
    tsh = pltpu.VMEM((L, 49, H // 2, H), jnp.uint32)
    leaf = pltpu.VMEM((1, TM // 4, H), f32)
    return pl.pallas_call(
        functools.partial(_kernel, L=L, TM=TM, D=D, RC=RC, LA_AHEAD=LA_AHEAD, NZ=NZ),
        grid=(B // TM,),
        in_specs=[
            pl.BlockSpec((TM, D), lambda i: (i, 0)),
            pl.BlockSpec((L, D, D), lambda i: (0, 0, 0)),
            pl.BlockSpec((L, 1, D), lambda i: (0, 0, 0)),
        ],
        out_specs=pl.BlockSpec((TM, D), lambda i: (i, 0)),
        out_shape=jax.ShapeDtypeStruct((B, D), x0.dtype),
        scratch_shapes=[tsh, pltpu.SMEM((NZ,), jnp.int32)] + [leaf] * (NX + NI + NO),
        compiler_params=pltpu.CompilerParams(
            dimension_semantics=("arbitrary",),
            vmem_limit_bytes=110 * 1024 * 1024,
        ),
    )(x0, ws, bs3)
```

```python
import functools

import jax
import jax.numpy as jnp
import numpy as np
import jax.experimental.pallas as pl
import jax.experimental.pallas.tpu as pltpu

f32 = jnp.float32
bf16 = jnp.bfloat16
u32 = jnp.uint32
i32 = jnp.int32


def _dot(a, b):
    return jnp.dot(a, b, preferred_element_type=f32)


LA = {1: [((0, 0), 1), ((1, 1), 1)],
      2: [((0, 0), 1), ((0, 1), 1), ((1, 0), 1), ((1, 1), 1)],
      3: [((0, 0), 1), ((0, 1), -1)],
      4: [((0, 1), 1), ((1, 1), 1)],
      5: [((0, 0), 1), ((0, 1), 1)],
      6: [((0, 1), 1), ((0, 0), -1), ((1, 0), 1), ((1, 1), -1)],
      7: [((0, 1), 1), ((1, 1), -1)]}
D2 = (1.0, 2.0)
BF = {1: 1.0, 2: 0.5, 3: 0.5, 4: 0.5, 5: 0.5, 6: 0.5, 7: 0.5}


def leaf_scale(R, C):
    d = lambda r: D2[r // 2] * D2[r % 2]
    return d(R) / d(C)


def a_ops(a11, a12, a21, a22):
    l1 = a11 + a22
    g = a12 + a21
    return {1: l1, 2: g + l1, 3: a11 - a12, 4: a12 + a22, 5: a11 + a12, 6: g - l1, 7: a12 - a22}


def b_ops(b11, b12, b21, b22):
    r1 = b11 + b22
    g = b12 + b21
    return {1: r1, 2: b11 - b12, 3: b12 - b22, 4: g - r1, 5: b12 + b22, 6: b11 + b12, 7: g + r1}


def lincomb(terms):
    assert terms[0][0] == 1
    acc = terms[0][1]
    for s, v in terms[1:]:
        acc = acc + v if s == 1 else acc - v
    return acc


OUTER = [3, 5, 1, 4, 7, 2, 6]
ROUNDS = [('1', None), ('35', 0), ('35', 1), ('47', 0), ('47', 1), ('26', 0), ('26', 1)]
OACT = {
    3: ([(1, (0, 1))], [('M3', [(1, 'd')])], []),
    5: ([], [('M5', [(1, 'd')])], [((0, 1), [(1, 'd'), (1, 'M3')])]),
    1: ([(1, (1, 1)), (-1, (0, 1))], [('S', [(1, 'd'), (1, 'M3'), (-1, 'M5')])], []),
    4: ([(1, (0, 0)), (-1, (1, 1))], [('A11', [(1, 'd'), (1, 'S')]), ('W', [(1, 'd'), (1, 'M3'), (1, 'M5')])], []),
    7: ([], [('U', [(1, 'W'), (-1, 'd')])], [((0, 0), [(1, 'd'), (1, 'A11')])]),
    2: ([], [('A22', [(1, 'S'), (-1, 'd')]), ('A21', [(1, 'd'), (1, 'U'), (1, 'bias21')])], []),
    6: ([], [], [((1, 1), [(1, 'd'), (1, 'A22')]), ((1, 0), [(1, 'd'), (1, 'A21')])]),
}
BIAS21 = [(1, (1, 0)), (1, (1, 1)), (-1, (0, 1)), (-1, (0, 0))]
OSL = {'M3': 0, 'M5': 1, 'S': 2, 'A11': 3, 'W': 4, 'U': 5, 'A22': 6, 'A21': 7}
ISL = {'m1': 0, 's': 1, 'v': 2, 'u': 3}
PREP_ORDER = (2, 6, 3, 5, 1, 4, 7)
X0_COPY = {1: (0, 1), 2: (0, 0), 3: (1, 1), 6: (1, 0)}
CONV_SLOTS = (0, 1, 2, 3)
NX0, NX, NI, NO, NS = 32, 4, 16, 64, 2


def spread(n, base, lo, hi, width):
    load = list(base)
    out = []
    for _ in range(n):
        t = min(range(lo, hi), key=lambda t: (sum(2 * load[u] + 1 for u in range(t, t + width)), t))
        for u in range(t, t + width):
            load[u] += 1
        out.append(t)
    return sorted(out)


def round_weights(unit):
    outer = {3: 1, 5: 3, 1: 3, 4: 4, 7: 4, 2: 3, 6: 6}
    inner = [(2, 0), (5, 1), (5, 1), (6, 1), (6, 1), (6, 2), (6, 2)]
    return {p: tuple(2 * (a + n * outer[p]) / unit for a, n in inner) for p in outer}


def _kernel(x_hbm, w_hbm, b_hbm, o_hbm, *scratch, L, TM, R0, NMAIN, D, cfg):
    H = D // 4
    Mh = TM // 4
    NT = H // 128
    NC = Mh // 16
    MP = cfg['MP']
    STG = cfg['STG']
    assert NT == 2 and L % 2 == 0
    bufs = scratch[:-9]
    bf_ref, xn2_ref, o2_ref, t_ref, w_ref, xr_ref, xp_ref, b_ref, sem = scratch[-9:]
    x0b = bufs[:NX0]
    xb = bufs[NX0:NX0 + NX]
    o = NX0 + NX
    ib = bufs[o:o + NI]
    ob = bufs[o + NI:o + NI + NO]
    sb = bufs[o + NI + NO:]
    GROW = 16 * MP

    def xloc(l, R, C, k):
        off = 8 * ((2 * (C // 2) + 2 * (R // 2) + (l % 2 if STG > 1 else 0)) % 4) if STG else 0
        return xb[(l % 2) * 2 + R // 2], (((R % 2) * 4 + C) * 2 + k) * MP + off

    def x0loc(R, C, k):
        return x0b[(R * 4 + C) * 2 + k], (8 * ((2 * (C // 2) + 2 * (R // 2) + 1) % 4) if STG else 0)

    def iloc(g, name, n):
        return ib[((g % 2) * 4 + ISL[name]) * 2 + n], (8 * (ISL[name] % 4) if STG else 0)

    def oloc(name, i, j, n):
        return ob[(OSL[name] * 4 + i * 2 + j) * 2 + n], (8 * ((OSL[name] + 2 * j) % 4) if STG else 0)

    def const_after(anchor, s, reps):
        sv = jax.lax.bitcast_convert_type(anchor | int(np.float32(s).view(np.int32)), f32)
        return jnp.tile(sv, (reps, 1))

    def conv(src, zs, R, C, r, nr, anchor=None):
        v = src[R * Mh + r:R * Mh + r + nr, C * H:(C + 1) * H].astype(f32)
        s = leaf_scale(R, C)
        sv = None if anchor is None else const_after(anchor, s, nr // 8)
        for k in range(NT):
            vk = v[:, k * 128:(k + 1) * 128]
            if sv is not None:
                vk = vk * sv
            elif s != 1.0:
                vk = vk * s
            buf, r0 = xloc(0, R, C, k)
            buf[zs, r0 + r:r0 + r + nr, :] = vk

    def a_chunk(g, l, p, c, k, zs, za, anchor=None):
        r = 16 * c
        def leaf(R, C):
            buf, r0 = xloc(l, R, C, k)
            gated = (R // 2, C // 2) == LA[p][0][0]
            v = buf[za if gated else 0, r0 + r:r0 + r + 16, :]
            if X0_COPY.get(g) == (R // 2, C // 2):
                dst, d0 = x0loc(R, C, k)
                dst[zs, d0 + r:d0 + r + 16, :] = v * const_after(anchor, 1.0 / leaf_scale(R, C), 2)
            return v
        a = {}
        for i in range(2):
            for j in range(2):
                terms = [(s, leaf(2 * I + i, 2 * J + j)) for (I, J), s in LA[p]]
                if anchor is not None and (i, j) == (0, 1):
                    v = terms[0][1]
                    top = jax.lax.bitcast_convert_type(jax.lax.bitcast_convert_type(v[0:8], i32) | anchor, f32)
                    terms[0] = (1, jnp.concatenate([top, v[8:16]], axis=0))
                a[(i, j)] = lincomb(terms)
        ops = a_ops(a[(0, 0)], a[(0, 1)], a[(1, 0)], a[(1, 1)])
        v = jnp.concatenate([ops[q] for q in range(1, 8)], axis=0)
        so = 16 * k if STG else 0
        sb[g % 2][zs, k, c, so:so + 112, :] = v.astype(bf16)

    def prep(l, r, anchors):
        wide = {(R, C): w_ref[l, pl.ds(R * H + r, 16), C * H:(C + 1) * H] for R in range(4) for C in range(4)}
        for n in range(NT):
            def blk(R, C):
                v = wide[(R, C)].astype(f32)[:, n * 128:(n + 1) * 128]
                s = D2[R // 2] / D2[C // 2]
                return v if s == 1.0 else v * s
            B = {(R, C): blk(R, C) for R in range(4) for C in range(4)}
            O = {(i, j): b_ops(B[(i, j)], B[(i, 2 + j)], B[(2 + i, j)], B[(2 + i, 2 + j)])
                 for i in range(2) for j in range(2)}
            for p in PREP_ORDER:
                anchor = next(anchors)
                def sc(i, j):
                    s = D2[i] / D2[j] * BF[p] * 0.5
                    return O[(i, j)][p] * (s if anchor is None else const_after(anchor, s, 2))
                T = b_ops(sc(0, 0), sc(0, 1), sc(1, 0), sc(1, 1))
                T[1] = T[1] + T[1]
                for q in range(1, 8):
                    t_ref[l, (p - 1) * 7 + q - 1, n, pl.ds(r, 16), :] = T[q].astype(bf16)

    def w_copy(l):
        return pltpu.make_async_copy(w_hbm.at[l], w_ref.at[l], sem.at[l])

    def in_copy(t, slot):
        return pltpu.make_async_copy(x_hbm.at[pl.ds(pl.multiple_of(t * TM, 32), TM)], xn2_ref.at[slot], sem.at[L + slot])

    def out_copy(t, slot, h):
        hm = TM // 2
        return pltpu.make_async_copy(o2_ref.at[slot, pl.ds(h * hm, hm)],
                                     o_hbm.at[pl.ds(pl.multiple_of(t * TM + h * hm, 32), hm)],
                                     sem.at[L + 4 + 2 * slot + h])

    xr_in = pltpu.make_async_copy(x_hbm.at[pl.ds(NMAIN * TM, R0)], xr_ref, sem.at[L + 2])
    xr_out = pltpu.make_async_copy(xr_ref, o_hbm.at[pl.ds(NMAIN * TM, R0)], sem.at[L + 2])
    b_in = pltpu.make_async_copy(b_hbm, b_ref, sem.at[L + 3])

    def prologue():
        b_in.start()
        xr_in.start()
        for l in range(L):
            w_copy(l).start()
        in_copy(0, 0).start()
        in_copy(min(1, NMAIN - 1), 1).start()
        b_in.wait()
        for l in range(L):
            bf_ref[l] = b_ref[l:l + 1, :].astype(f32)
        xr_in.wait()
        xp_ref[...] = xr_ref[...].astype(f32)
        NSUB = cfg['NSUB']
        RB = R0 // NSUB
        PR = H // NSUB
        def sub(it, c):
            l = it // NSUB
            j = it % NSUB
            @pl.when(j == 0)
            def _():
                w_copy(l).wait()
            zero = jax.lax.shift_right_logical(it, 12)
            rows = pl.ds(pl.multiple_of(j * RB, RB), RB)
            x = xp_ref[rows, :]
            xbf = x.astype(bf16)
            KH = D // 2
            passes, ys = [], []
            for jt in range(D // 128):
                cols = slice(jt * 128, (jt + 1) * 128)
                ya = _dot(xbf[:, :KH], w_ref[l, 0:KH, cols]) + bf_ref[l, :, cols]
                yb = _dot(xbf[:, KH:], w_ref[l, KH:D, cols]) + ya
                passes += [ya, yb]
                ys.append(yb)
            xp_ref[rows, :] = xr_ref[rows, :].astype(f32) * jnp.concatenate(ys, axis=1) + x
            na = (PR // 16) * NT * 7
            def gen():
                tot = len(passes) * (RB // 8)
                for u in range(na):
                    if u < cfg['AFREE']:
                        yield None
                        continue
                    f = int((u - cfg['AFREE']) * cfg['ANC'] * tot / (na - cfg['AFREE']))
                    ps, rr = divmod(f, RB // 8)
                    yield jax.lax.bitcast_convert_type(passes[ps][rr * 8:rr * 8 + 8, :], i32) & zero
            anchors = gen()
            for u in range(PR // 16):
                prep(l, pl.multiple_of(j * PR + u * 16, 16), anchors)
            return c
        jax.lax.fori_loop(0, L * NSUB, sub, 0)
        xr_ref[...] = xp_ref[...].astype(bf16)
        xr_out.start()
        in_copy(0, 0).wait()
        for R in range(4):
            for C in range(4):
                conv(xn2_ref.at[0], 0, R, C, 0, Mh)
        for c in range(NC):
            for k in range(NT):
                a_chunk(0, 0, OUTER[0], c, k, 0, 0)

    def main(tile, carry):
        zs, za = jax.lax.shift_right_logical(tile, 12), jax.lax.shift_right_logical(tile, 13)
        slot = tile % 2
        in_copy(jnp.minimum(tile + 2, NMAIN - 1), slot).start()
        in_copy(0, 1 - slot).wait()
        @pl.when(tile > 1)
        def _():
            out_copy(0, slot, 0).wait()
            out_copy(0, slot, 1).wait()
        xn_ref = xn2_ref.at[1 - slot]
        o_ref = o2_ref.at[slot]

        def ld(loc):
            return loc[0][0, loc[1]:loc[1] + Mh, :]

        def st(loc, v):
            loc[0][zs, loc[1]:loc[1] + Mh, :] = v

        def lhs_load(g, q):
            ref = sb[g % 2].bitcast(u32)
            cols = []
            for k in range(NT):
                r0 = (q - 1 + (k if STG else 0)) * 8
                cols.append(ref[0, k, :, r0:r0 + 8, :].reshape(Mh // 2, 128))
            return pltpu.bitcast(jnp.concatenate(cols, axis=1), bf16)

        def wload(l, p, q, n):
            return pltpu.bitcast(t_ref.bitcast(u32)[l, (p - 1) * 7 + q - 1, n], bf16)

        def outer_act(l, p, i, j, n, d):
            def bias(terms):
                def one(I, J):
                    R, C = 2 * I + i, 2 * J + j
                    bv = bf_ref[l, :, C * H + n * 128:C * H + (n + 1) * 128]
                    if l == 0:
                        bv = bv + 1.0
                    s = leaf_scale(R, C)
                    return bv if s == 1.0 else bv * s
                return lincomb([(s, one(*IJ)) for s, IJ in terms])
            bt, stores, finals = OACT[p]
            if bt:
                d = d + bias(bt)
            cache = {'d': d}
            def val(src):
                if src not in cache:
                    cache[src] = bias(BIAS21) if src == 'bias21' else ld(oloc(src, i, j, n))
                return cache[src]
            fin = [(IJ, lincomb([(s, val(src)) for s, src in terms])) for IJ, terms in finals]
            stl = [(name, lincomb([(s, val(src)) for s, src in terms])) for name, terms in stores]
            for name, v in stl:
                st(oloc(name, i, j, n), v)
            for (I, J), y in fin:
                R, C = 2 * I + i, 2 * J + j
                xn = ld(x0loc(R, C, n)) * y
                if l > 0:
                    xn = xn + ld(xloc(l, R, C, n))
                if l == L - 1:
                    s = leaf_scale(R, C)
                    if s != 1.0:
                        xn = xn * (1.0 / s)
                    o_ref[R * Mh:(R + 1) * Mh, C * H + n * 128:C * H + (n + 1) * 128] = xn.astype(o_ref.dtype)
                else:
                    st(xloc(l + 1, R, C, n), xn)

        def issue(g, l, p, rd):
            kind, n = rd
            if kind == '1':
                lhs = lhs_load(g, 1)
                return (_dot(lhs, wload(l, p, 1, 0)), _dot(lhs, wload(l, p, 1, 1)))
            qa, qb = int(kind[0]), int(kind[1])
            return (_dot(lhs_load(g, qa), wload(l, p, qa, n)), _dot(lhs_load(g, qb), wload(l, p, qb, n)))

        def consume(g, l, p, rd, res):
            kind, n = rd
            a, b = res
            if kind == '1':
                st(iloc(g, 'm1', 0), a)
                st(iloc(g, 'm1', 1), b)
            elif kind == '35':
                v = a + b
                st(iloc(g, 's', n), (a - b) + ld(iloc(g, 'm1', n)))
                st(iloc(g, 'v', n), v)
                outer_act(l, p, 0, 1, n, v)
            elif kind == '47':
                st(iloc(g, 'u', n), (a - b) + ld(iloc(g, 'v', n)))
                outer_act(l, p, 0, 0, n, (a + b) + ld(iloc(g, 's', n)))
            else:
                outer_act(l, p, 1, 1, n, (b - a) + ld(iloc(g, 's', n)))
                outer_act(l, p, 1, 0, n, (b + a) + ld(iloc(g, 'u', n)))

        WT = round_weights(cfg['UNIT'])
        outs = [(l, p) for l in range(L) for p in OUTER]
        G = len(outs)
        outs.append((0, OUTER[0]))
        prev = None
        for g in range(G):
            l, p = outs[g]
            l2, p2 = outs[g + 1]
            if g == G - 1:
                out_copy(tile, slot, 0).start()
            wts = [WT[outs[g - 1][1]][6] if g else 0] + list(WT[p])
            base = [wts[t // NC] for t in range(8 * NC)]
            chunks = [(c, k) for c in range(NC) for k in range(NT)]
            times = spread(len(chunks), base, NC if g == 0 else cfg['LO'], 7 * NC - cfg['HI'] - cfg['WID'], cfg['WID'])
            units = []
            if l == L - 1 and g % 7 in CONV_SLOTS:
                R = CONV_SLOTS.index(g % 7)
                units = [(R, C, 16 * c) for C in range(4) for c in range(NC)]
            per = len(units) // len(chunks)
            for ri, rd in enumerate(ROUNDS):
                res = issue(g, l, p, rd)
                for t, (c, k) in zip(times, chunks):
                    if t // NC != ri:
                        continue
                    gr = 16 * (t % NC)
                    gate = prev[0][gr:gr + 8, :]
                    xb[(l2 % 2) * 2][0, GROW:GROW + 8, :] = gate
                    a_chunk(g + 1, l2, p2, c, k, zs, za, jax.lax.bitcast_convert_type(gate, i32) & zs)
                    if per:
                        anchor = jax.lax.bitcast_convert_type(prev[1][gr + 8:gr + 16, :], i32) & zs
                    for _ in range(per):
                        R, C, rr = units.pop()
                        conv(xn_ref, zs, R, C, rr, 16, anchor)
                consume(g, l, p, rd, res)
                prev = res
            assert not units
        out_copy(tile, slot, 1).start()
        return carry

    prologue()
    jax.lax.fori_loop(0, NMAIN, main, 0)
    xr_out.wait()
    in_copy(0, (NMAIN - 1) % 2).wait()
    for t in range(max(NMAIN - 2, 0), NMAIN):
        out_copy(0, t % 2, 0).wait()
        out_copy(0, t % 2, 1).wait()


DEFAULT = dict(UNIT=30, LO=2, HI=0, WID=3, NSUB=1, ANC=0.98, AFREE=4, STG=1, GW=None, DBC=True)


def build(TM=512, **kw):
    def f(x0, ws, bs):
        B, D = x0.shape
        L = ws.shape[0]
        H = D // 4
        Mh = TM // 4
        nmain = (B - 1) // TM
        R0 = B - nmain * TM
        cfg = dict(DEFAULT, **kw)
        MP = cfg['MP'] = (Mh + 24 + 31) // 32 * 32
        half = pltpu.VMEM((1, MP, 128), f32)
        xhalf = pltpu.VMEM((1, 16 * MP + 32, 128), f32)
        sop = pltpu.VMEM((1, H // 128, Mh // 16, 128, 128), bf16)
        tsh = pltpu.VMEM((L, 49, H // 128, H, 128), bf16)
        if cfg['GW'] is None:
            cfg['GW'] = 7 * (L - 1)
        anyspec = pl.BlockSpec(memory_space=pl.ANY)
        return pl.pallas_call(
            functools.partial(_kernel, L=L, TM=TM, R0=R0, NMAIN=nmain, D=D, cfg=cfg),
            in_specs=[anyspec, anyspec, anyspec],
            out_specs=anyspec,
            out_shape=jax.ShapeDtypeStruct((B, D), x0.dtype),
            scratch_shapes=[half] * NX0 + [xhalf] * NX + [half] * (NI + NO) + [sop] * NS
                           + [pltpu.VMEM((8, 1, D), f32), pltpu.VMEM((2, TM, D), bf16), pltpu.VMEM((2, TM, D), bf16), tsh,
                              pltpu.VMEM((L, D, D), bf16), pltpu.VMEM((R0, D), bf16), pltpu.VMEM((R0, D), f32),
                              pltpu.VMEM((L, D), bf16), pltpu.SemaphoreType.DMA((L + 8,))],
            compiler_params=pltpu.CompilerParams(
                vmem_limit_bytes=110 * 1024 * 1024,
                internal_scratch_in_bytes=65536,
                disable_bounds_checks=cfg['DBC'],
            ),
        )(x0, ws, bs)
    return f


@jax.jit
def pallas_standalone__dcn_v2_cross__recsys_kernel(x0, ws, bs):
    return build(TM=576)(x0, ws, bs)
```

```python
import functools

import jax
import jax.numpy as jnp
import numpy as np
import jax.experimental.pallas as pl
import jax.experimental.pallas.tpu as pltpu

f32 = jnp.float32
bf16 = jnp.bfloat16
u32 = jnp.uint32
i32 = jnp.int32


def _dot(a, b):
    return jnp.dot(a, b, preferred_element_type=f32)


LA = {1: [((0, 0), 1), ((1, 1), 1)],
      2: [((0, 0), 1), ((0, 1), 1), ((1, 0), 1), ((1, 1), 1)],
      3: [((0, 0), 1), ((0, 1), -1)],
      4: [((0, 1), 1), ((1, 1), 1)],
      5: [((0, 0), 1), ((0, 1), 1)],
      6: [((0, 1), 1), ((0, 0), -1), ((1, 0), 1), ((1, 1), -1)],
      7: [((0, 1), 1), ((1, 1), -1)]}
D2 = (1.0, 2.0)
BF = {1: 1.0, 2: 0.5, 3: 0.5, 4: 0.5, 5: 0.5, 6: 0.5, 7: 0.5}


def leaf_scale(R, C):
    d = lambda r: D2[r // 2] * D2[r % 2]
    return d(R) / d(C)


def a_ops(a11, a12, a21, a22):
    l1 = a11 + a22
    g = a12 + a21
    return {1: l1, 2: g + l1, 3: a11 - a12, 4: a12 + a22, 5: a11 + a12, 6: g - l1, 7: a12 - a22}


def b_ops(b11, b12, b21, b22):
    r1 = b11 + b22
    g = b12 + b21
    return {1: r1, 2: b11 - b12, 3: b12 - b22, 4: g - r1, 5: b12 + b22, 6: b11 + b12, 7: g + r1}


def lincomb(terms):
    assert terms[0][0] == 1
    acc = terms[0][1]
    for s, v in terms[1:]:
        acc = acc + v if s == 1 else acc - v
    return acc


OUTER = [3, 5, 1, 4, 7, 2, 6]
ROUNDS = [('1', None), ('35', 0), ('35', 1), ('47', 0), ('47', 1), ('26', 0), ('26', 1)]
B11, B12, B21, B22 = (0, 0), (0, 1), (1, 0), (1, 1)
OACTS = {
  'bal': {
    3: ([(1, B12)], [('M3', [(1, 'd')])], []),
    5: ([], [('M5', [(1, 'd')])], [(B12, [(1, 'd'), (1, 'M3')])]),
    1: ([(1, B22), (-1, B12)], [('S', [(1, 'd'), (1, 'M3'), (-1, 'M5')])], []),
    4: ([(1, B11), (-1, B22)], [('A11', [(1, 'd'), (1, 'S')]), ('W', [(1, 'd'), (1, 'M3'), (1, 'M5')])], []),
    7: ([], [('U', [(1, 'W'), (-1, 'd')])], [(B11, [(1, 'd'), (1, 'A11')])]),
    2: ([], [('A22', [(1, 'S'), (-1, 'd')]), ('A21', [(1, 'd'), (1, 'U'), (1, ((1, B21), (1, B22), (-1, B12), (-1, B11)))])], []),
    6: ([], [], [(B22, [(1, 'd'), (1, 'A22')]), (B21, [(1, 'd'), (1, 'A21')])]),
  },
  'raw': {
    3: ([(1, B21), (-1, B11), (1, B22)], [('M3', [(1, 'd')])], []),
    5: ([], [('M5', [(1, 'd')])], [(B12, [(1, 'd'), (1, 'M3'), (1, ((1, B12), (-1, B21), (1, B11), (-1, B22)))])]),
    1: ([(1, B11), (-1, B21)], [('S', [(1, 'd'), (1, 'M3'), (-1, 'M5')])], []),
    4: ([(1, B11), (-1, B22)], [('A11', [(1, 'd')])], []),
    7: ([], [('U', [(1, 'A11'), (-1, 'd'), (1, 'M3'), (1, 'M5')])], [(B11, [(1, 'd'), (1, 'S'), (1, 'A11')])]),
    2: ([], [('A22', [(1, 'd')])], []),
    6: ([], [], [(B22, [(1, 'd'), (1, 'S'), (-1, 'A22')]), (B21, [(1, 'd'), (1, 'U'), (1, 'A22')])]),
  },
  'raw2': {
    3: ([(1, B21), (-1, B11), (1, B22)], [('M3', [(1, 'd')])], []),
    5: ([], [('M5', [(1, 'd')])], [(B12, [(1, 'd'), (1, 'M3'), (1, ((1, B12), (-1, B21), (1, B11), (-1, B22)))])]),
    1: ([(1, B11), (-1, B21)], [('S', [(1, 'd'), (1, 'M3'), (-1, 'M5')])], []),
    4: ([(1, B11), (-1, B22)], [('A11', [(1, 'd')]), ('W', [(1, 'd'), (1, 'M3'), (1, 'M5')])], []),
    7: ([], [('U', [(1, 'W'), (-1, 'd')])], [(B11, [(1, 'd'), (1, 'S'), (1, 'A11')])]),
    2: ([], [('A22', [(1, 'd')])], []),
    6: ([], [], [(B22, [(1, 'd'), (1, 'S'), (-1, 'A22')]), (B21, [(1, 'd'), (1, 'U'), (1, 'A22')])]),
  },
  'raw3': {
    3: ([(1, B21), (-1, B11), (1, B22)], [('M3', [(1, 'd')])], []),
    5: ([], [('M5', [(1, 'd')])], [(B12, [(1, 'd'), (1, 'M3'), (1, ((1, B12), (-1, B21), (1, B11), (-1, B22)))])]),
    1: ([(1, B11), (-1, B21)], [('S', [(1, 'd'), (1, 'M3'), (-1, 'M5')])], []),
    4: ([(1, B11), (-1, B22)], [('A11', [(1, 'd')])], []),
    7: ([], [('U', [(1, 'A11'), (-1, 'd')])], [(B11, [(1, 'd'), (1, 'S'), (1, 'A11')])]),
    2: ([], [('A22', [(1, 'd')]), ('A21', [(1, 'd'), (1, 'U'), (1, 'M3'), (1, 'M5')])], []),
    6: ([], [], [(B22, [(1, 'd'), (1, 'S'), (-1, 'A22')]), (B21, [(1, 'd'), (1, 'A21')])]),
  },
}
OSL = {'M3': 0, 'M5': 1, 'S': 2, 'A11': 3, 'W': 4, 'U': 5, 'A22': 6, 'A21': 7}
ISL = {'m1': 0, 's': 1, 'v': 2, 'u': 3}
PREP_ORDER = (2, 6, 3, 5, 1, 4, 7)
X0_COPY = {1: (0, 1), 2: (0, 0), 3: (1, 1), 6: (1, 0)}
CONV_SLOTS = (0, 1, 2, 3)
NX0, NX, NI, NO, NS = 32, 4, 16, 64, 2


def spread(n, base, lo, hi, width):
    load = list(base)
    out = []
    for _ in range(n):
        t = min(range(lo, hi), key=lambda t: (sum(2 * load[u] + 1 for u in range(t, t + width)), t))
        for u in range(t, t + width):
            load[u] += 1
        out.append(t)
    return sorted(out)


def raw_slot(act):
    for name, terms in act[1]:
        if terms == [(1, 'd')]:
            return name
    return None


def round_weights(oact, unit, vw, reuse):
    wt = {}
    for p, (bt, stores, finals) in oact.items():
        alu = bool(bt) + sum(len(t) - 1 for _, t in stores) + sum(len(t) + 1 for _, t in finals)
        nst = len(stores) + len(finals)
        vs = 1 if (reuse and raw_slot(oact[p])) else 2
        inner = [(2, 2, 0), (5, vs, 1), (5, vs, 1), (6, 1, 1), (6, 1, 1), (6, 0, 2), (6, 0, 2)]
        wt[p] = tuple(2 * (a + n * alu + vw * (st + n * nst)) / unit for a, st, n in inner)
    return wt


def _kernel(x_hbm, w_hbm, b_hbm, o_hbm, *scratch, L, TM, R0, NMAIN, D, cfg):
    H = D // 4
    Mh = TM // 4
    NT = H // 128
    NC = Mh // 16
    MP = cfg['MP']
    STG = cfg['STG']
    assert NT == 2 and L % 2 == 0
    bufs = scratch[:-9]
    bf_ref, xn2_ref, o2_ref, t_ref, w_ref, xr_ref, xp_ref, b_ref, sem = scratch[-9:]
    x0b = bufs[:NX0]
    xb = bufs[NX0:NX0 + NX]
    o = NX0 + NX
    ib = bufs[o:o + NI]
    ob = bufs[o + NI:o + NI + NO]
    sb = bufs[o + NI + NO:]
    GROW = 16 * MP

    def xloc(l, R, C, k):
        off = 8 * ((2 * (C // 2) + 2 * (R // 2) + (l % 2 if STG > 1 else 0)) % 4) if STG else 0
        return xb[(l % 2) * 2 + R // 2], (((R % 2) * 4 + C) * 2 + k) * MP + off

    def x0loc(R, C, k):
        return x0b[(R * 4 + C) * 2 + k], (8 * ((2 * (C // 2) + 2 * (R // 2) + 1) % 4) if STG else 0)

    def iloc(g, name, n):
        return ib[((g % 2) * 4 + ISL[name]) * 2 + n], (8 * (ISL[name] % 4) if STG else 0)

    def oloc(name, i, j, n):
        return ob[(OSL[name] * 4 + i * 2 + j) * 2 + n], (8 * ((OSL[name] + 2 * j) % 4) if STG else 0)

    def const_after(anchor, s, reps):
        sv = jax.lax.bitcast_convert_type(anchor | int(np.float32(s).view(np.int32)), f32)
        return jnp.tile(sv, (reps, 1))

    def conv(src, zs, R, C, r, nr, anchor=None):
        v = src[R * Mh + r:R * Mh + r + nr, C * H:(C + 1) * H].astype(f32)
        s = leaf_scale(R, C)
        sv = None if anchor is None else const_after(anchor, s, nr // 8)
        for k in range(NT):
            vk = v[:, k * 128:(k + 1) * 128]
            if sv is not None:
                vk = vk * sv
            elif s != 1.0:
                vk = vk * s
            buf, r0 = xloc(0, R, C, k)
            buf[zs, r0 + r:r0 + r + nr, :] = vk

    def a_chunk(g, l, p, c, k, zs, za, anchor=None):
        r = 16 * c
        def leaf(R, C):
            buf, r0 = xloc(l, R, C, k)
            gated = (R // 2, C // 2) == LA[p][0][0]
            v = buf[za if gated else 0, r0 + r:r0 + r + 16, :]
            if dict(zip((B12, B11, B22, B21), cfg['XC']))[(R // 2, C // 2)] == g:
                dst, d0 = x0loc(R, C, k)
                dst[zs, d0 + r:d0 + r + 16, :] = v * const_after(anchor, 1.0 / leaf_scale(R, C), 2)
            return v
        a = {}
        for i in range(2):
            for j in range(2):
                terms = [(s, leaf(2 * I + i, 2 * J + j)) for (I, J), s in LA[p]]
                if anchor is not None and (i, j) == (0, 1):
                    v = terms[0][1]
                    top = jax.lax.bitcast_convert_type(jax.lax.bitcast_convert_type(v[0:8], i32) | anchor, f32)
                    terms[0] = (1, jnp.concatenate([top, v[8:16]], axis=0))
                a[(i, j)] = lincomb(terms)
        ops = a_ops(a[(0, 0)], a[(0, 1)], a[(1, 0)], a[(1, 1)])
        v = jnp.concatenate([ops[q] for q in range(1, 8)], axis=0)
        so = 16 * k if STG else 0
        sb[g % 2][zs, k, c, so:so + 112, :] = v.astype(bf16)

    def prep(l, r, anchors):
        wide = {(R, C): w_ref[l, pl.ds(R * H + r, 16), C * H:(C + 1) * H] for R in range(4) for C in range(4)}
        for n in range(NT):
            def blk(R, C):
                v = wide[(R, C)].astype(f32)[:, n * 128:(n + 1) * 128]
                s = D2[R // 2] / D2[C // 2]
                return v if s == 1.0 else v * s
            B = {(R, C): blk(R, C) for R in range(4) for C in range(4)}
            O = {(i, j): b_ops(B[(i, j)], B[(i, 2 + j)], B[(2 + i, j)], B[(2 + i, 2 + j)])
                 for i in range(2) for j in range(2)}
            for p in PREP_ORDER:
                anchor = next(anchors)
                def sc(i, j):
                    s = D2[i] / D2[j] * BF[p] * 0.5
                    return O[(i, j)][p] * (s if anchor is None else const_after(anchor, s, 2))
                T = b_ops(sc(0, 0), sc(0, 1), sc(1, 0), sc(1, 1))
                T[1] = T[1] + T[1]
                for q in range(1, 8):
                    t_ref[l, (p - 1) * 7 + q - 1, n, pl.ds(r, 16), :] = T[q].astype(bf16)

    def w_copy(l):
        return pltpu.make_async_copy(w_hbm.at[l], w_ref.at[l], sem.at[l])

    def in_copy(t, slot):
        return pltpu.make_async_copy(x_hbm.at[pl.ds(pl.multiple_of(t * TM, 32), TM)], xn2_ref.at[slot], sem.at[L + slot])

    def out_copy(t, slot, h):
        hm = TM // 2
        return pltpu.make_async_copy(o2_ref.at[slot, pl.ds(h * hm, hm)],
                                     o_hbm.at[pl.ds(pl.multiple_of(t * TM + h * hm, 32), hm)],
                                     sem.at[L + 4 + 2 * slot + h])

    xr_in = pltpu.make_async_copy(x_hbm.at[pl.ds(NMAIN * TM, R0)], xr_ref, sem.at[L + 2])
    xr_out = pltpu.make_async_copy(xr_ref, o_hbm.at[pl.ds(NMAIN * TM, R0)], sem.at[L + 2])
    b_in = pltpu.make_async_copy(b_hbm, b_ref, sem.at[L + 3])

    def prologue():
        b_in.start()
        xr_in.start()
        for l in range(L):
            w_copy(l).start()
        in_copy(0, 0).start()
        in_copy(min(1, NMAIN - 1), 1).start()
        b_in.wait()
        for l in range(L):
            bf_ref[l] = b_ref[l:l + 1, :].astype(f32)
        xr_in.wait()
        xp_ref[...] = xr_ref[...].astype(f32)
        NSUB = cfg['NSUB']
        RB = R0 // NSUB
        PR = H // NSUB
        def sub(it, c):
            l = it // NSUB
            j = it % NSUB
            @pl.when(j == 0)
            def _():
                w_copy(l).wait()
            zero = jax.lax.shift_right_logical(it, 12)
            rows = pl.ds(pl.multiple_of(j * RB, RB), RB)
            x = xp_ref[rows, :]
            xbf = x.astype(bf16)
            KH = D // 2
            passes, ys = [], []
            for jt in range(D // 128):
                cols = slice(jt * 128, (jt + 1) * 128)
                ya = _dot(xbf[:, :KH], w_ref[l, 0:KH, cols]) + bf_ref[l, :, cols]
                yb = _dot(xbf[:, KH:], w_ref[l, KH:D, cols]) + ya
                passes += [ya, yb]
                ys.append(yb)
            xp_ref[rows, :] = xr_ref[rows, :].astype(f32) * jnp.concatenate(ys, axis=1) + x
            na = (PR // 16) * NT * 7
            def gen():
                tot = len(passes) * (RB // 8)
                for u in range(na):
                    if u < cfg['AFREE']:
                        yield None
                        continue
                    f = int((u - cfg['AFREE']) * cfg['ANC'] * tot / (na - cfg['AFREE']))
                    ps, rr = divmod(f, RB // 8)
                    yield jax.lax.bitcast_convert_type(passes[ps][rr * 8:rr * 8 + 8, :], i32) & zero
            anchors = gen()
            for u in range(PR // 16):
                prep(l, pl.multiple_of(j * PR + u * 16, 16), anchors)
            return c
        jax.lax.fori_loop(0, L * NSUB, sub, 0)
        xr_ref[...] = xp_ref[...].astype(bf16)
        xr_out.start()
        in_copy(0, 0).wait()
        for R in range(4):
            for C in range(4):
                conv(xn2_ref.at[0], 0, R, C, 0, Mh)
        for c in range(NC):
            for k in range(NT):
                a_chunk(0, 0, OUTER[0], c, k, 0, 0)

    def main(tile, carry):
        zs, za = jax.lax.shift_right_logical(tile, 12), jax.lax.shift_right_logical(tile, 13)
        slot = tile % 2
        in_copy(jnp.minimum(tile + 2, NMAIN - 1), slot).start()
        in_copy(0, 1 - slot).wait()
        @pl.when(tile > 1)
        def _():
            out_copy(0, slot, 0).wait()
            out_copy(0, slot, 1).wait()
        xn_ref = xn2_ref.at[1 - slot]
        o_ref = o2_ref.at[slot]

        def ld(loc):
            return loc[0][0, loc[1]:loc[1] + Mh, :]

        def st(loc, v):
            loc[0][zs, loc[1]:loc[1] + Mh, :] = v

        def lhs_load(g, q):
            if cfg['NOBC'] & 1:
                cols = []
                for k in range(NT):
                    r0 = (q - 1 + (k if STG else 0)) * 16
                    cols.append(sb[g % 2][0, k, :, r0:r0 + 16, :].reshape(Mh, 128))
                return jnp.concatenate(cols, axis=1)
            ref = sb[g % 2].bitcast(u32)
            cols = []
            for k in range(NT):
                r0 = (q - 1 + (k if STG else 0)) * 8
                cols.append(ref[0, k, :, r0:r0 + 8, :].reshape(Mh // 2, 128))
            return pltpu.bitcast(jnp.concatenate(cols, axis=1), bf16)

        def wload(l, p, q, n):
            if cfg['NOBC'] & 2:
                return t_ref[l, (p - 1) * 7 + q - 1, n]
            return pltpu.bitcast(t_ref.bitcast(u32)[l, (p - 1) * 7 + q - 1, n], bf16)

        OACT = OACTS[cfg['OA']]

        def bias(l, terms, i, j, n, minus=None):
            coef = {}
            for sg, (ii, jj) in ((1, (i, j)),) + (((-1, minus),) if minus else ()):
                for cf, (I, J) in terms:
                    R, C = 2 * I + ii, 2 * J + jj
                    coef[C] = coef.get(C, 0.0) + sg * cf * leaf_scale(R, C)
            acc = None
            for C, cf in sorted(coef.items()):
                if cf == 0.0:
                    continue
                bv = bf_ref[l, :, C * H + n * 128:C * H + (n + 1) * 128]
                if l == 0:
                    bv = bv + 1.0
                bv = bv if cf == 1.0 else bv * cf
                acc = bv if acc is None else acc + bv
            return acc

        def outer_act(l, p, i, j, n, d):
            bt, stores, finals = OACT[p]
            if bt:
                reused = cfg['REUSE'] and raw_slot(OACT[p]) and (i, j) == (1, 0)
                d = d + bias(l, bt, i, j, n, (0, 1) if reused else None)
            cache = {'d': d}
            def val(src):
                if src not in cache:
                    cache[src] = ld(oloc(src, i, j, n)) if isinstance(src, str) else bias(l, src, i, j, n)
                return cache[src]
            fin = [(IJ, lincomb([(s, val(src)) for s, src in terms])) for IJ, terms in finals]
            stl = [(name, lincomb([(s, val(src)) for s, src in terms])) for name, terms in stores]
            for name, v in stl:
                st(oloc(name, i, j, n), v)
            for (I, J), y in fin:
                R, C = 2 * I + i, 2 * J + j
                xn = ld(x0loc(R, C, n)) * y
                if l > 0:
                    xn = xn + ld(xloc(l, R, C, n))
                if l == L - 1:
                    s = leaf_scale(R, C)
                    if s != 1.0:
                        xn = xn * (1.0 / s)
                    o_ref[R * Mh:(R + 1) * Mh, C * H + n * 128:C * H + (n + 1) * 128] = xn.astype(o_ref.dtype)
                else:
                    st(xloc(l + 1, R, C, n), xn)

        def issue(g, l, p, rd):
            kind, n = rd
            if kind == '1':
                lhs = lhs_load(g, 1)
                return (_dot(lhs, wload(l, p, 1, 0)), _dot(lhs, wload(l, p, 1, 1)))
            qa, qb = int(kind[0]), int(kind[1])
            return (_dot(lhs_load(g, qa), wload(l, p, qa, n)), _dot(lhs_load(g, qb), wload(l, p, qb, n)))

        def consume(g, l, p, rd, res):
            kind, n = rd
            a, b = res
            rs = raw_slot(OACT[p]) if cfg['REUSE'] else None
            if kind == '1':
                st(iloc(g, 'm1', 0), a)
                st(iloc(g, 'm1', 1), b)
            elif kind == '35':
                v = a + b
                st(iloc(g, 's', n), (a - b) + ld(iloc(g, 'm1', n)))
                if not rs:
                    st(iloc(g, 'v', n), v)
                outer_act(l, p, 0, 1, n, v)
            elif kind == '47':
                st(iloc(g, 'u', n), (a - b) + ld(oloc(rs, 0, 1, n) if rs else iloc(g, 'v', n)))
                outer_act(l, p, 0, 0, n, (a + b) + ld(iloc(g, 's', n)))
            else:
                outer_act(l, p, 1, 1, n, (b - a) + ld(iloc(g, 's', n)))
                outer_act(l, p, 1, 0, n, (b + a) + ld(iloc(g, 'u', n)))

        WT = round_weights(OACT, cfg['UNIT'], cfg['VW'], cfg['REUSE'])
        outs = [(l, p) for l in range(L) for p in OUTER]
        G = len(outs)
        outs.append((0, OUTER[0]))
        prev = None
        for g in range(G):
            l, p = outs[g]
            l2, p2 = outs[g + 1]
            if g == G - 1:
                out_copy(tile, slot, 0).start()
            wts = [WT[outs[g - 1][1]][6] if g else 0] + list(WT[p])
            base = [wts[t // NC] for t in range(8 * NC)]
            chunks = [(c, k) for c in range(NC) for k in range(NT)]
            times = spread(len(chunks), base, NC if g == 0 else cfg['LO'], 7 * NC - cfg['HI'] - cfg['WID'], cfg['WID'])
            units = []
            if l == L - 1 and g % 7 in cfg['CS']:
                R = cfg['CS'].index(g % 7)
                units = [(R, C, 16 * c) for C in range(4) for c in range(NC)]
            per = len(units) // len(chunks)
            for ri, rd in enumerate(ROUNDS):
                res = issue(g, l, p, rd)
                for t, (c, k) in zip(times, chunks):
                    if t // NC != ri:
                        continue
                    gr = 16 * (t % NC)
                    gate = prev[0][gr:gr + 8, :]
                    xb[(l2 % 2) * 2][0, GROW:GROW + 8, :] = gate
                    a_chunk(g + 1, l2, p2, c, k, zs, za, jax.lax.bitcast_convert_type(gate, i32) & zs)
                    if per:
                        anchor = jax.lax.bitcast_convert_type(prev[1][gr + 8:gr + 16, :], i32) & zs
                    for _ in range(per):
                        R, C, rr = units.pop()
                        conv(xn_ref, zs, R, C, rr, 16, anchor)
                consume(g, l, p, rd, res)
                prev = res
            assert not units
        out_copy(tile, slot, 1).start()
        return carry

    prologue()
    jax.lax.fori_loop(0, NMAIN, main, 0)
    xr_out.wait()
    in_copy(0, (NMAIN - 1) % 2).wait()
    for t in range(max(NMAIN - 2, 0), NMAIN):
        out_copy(0, t % 2, 0).wait()
        out_copy(0, t % 2, 1).wait()


DEFAULT = dict(UNIT=60, LO=0, HI=0, WID=3, NSUB=1, ANC=0.98, AFREE=4, STG=1, GW=None, DBC=True, NOBC=0, OA='raw', REUSE=1, VW=3, CS=(0, 2, 3, 5), XC=(1, 2, 4, 6))


def build(TM=512, **kw):
    def f(x0, ws, bs):
        B, D = x0.shape
        L = ws.shape[0]
        H = D // 4
        Mh = TM // 4
        nmain = (B - 1) // TM
        R0 = B - nmain * TM
        cfg = dict(DEFAULT, **kw)
        MP = cfg['MP'] = (Mh + 24 + 31) // 32 * 32
        half = pltpu.VMEM((1, MP, 128), f32)
        xhalf = pltpu.VMEM((1, 16 * MP + 32, 128), f32)
        sop = pltpu.VMEM((1, H // 128, Mh // 16, 128, 128), bf16)
        tsh = pltpu.VMEM((L, 49, H // 128, H, 128), bf16)
        if cfg['GW'] is None:
            cfg['GW'] = 7 * (L - 1)
        anyspec = pl.BlockSpec(memory_space=pl.ANY)
        return pl.pallas_call(
            functools.partial(_kernel, L=L, TM=TM, R0=R0, NMAIN=nmain, D=D, cfg=cfg),
            in_specs=[anyspec, anyspec, anyspec],
            out_specs=anyspec,
            out_shape=jax.ShapeDtypeStruct((B, D), x0.dtype),
            scratch_shapes=[half] * NX0 + [xhalf] * NX + [half] * (NI + NO) + [sop] * NS
                           + [pltpu.VMEM((8, 1, D), f32), pltpu.VMEM((2, TM, D), bf16), pltpu.VMEM((2, TM, D), bf16), tsh,
                              pltpu.VMEM((L, D, D), bf16), pltpu.VMEM((R0, D), bf16), pltpu.VMEM((R0, D), f32),
                              pltpu.VMEM((L, D), bf16), pltpu.SemaphoreType.DMA((L + 8,))],
            compiler_params=pltpu.CompilerParams(
                vmem_limit_bytes=110 * 1024 * 1024,
                internal_scratch_in_bytes=65536,
                disable_bounds_checks=cfg['DBC'],
            ),
        )(x0, ws, bs)
    return f


@jax.jit
def pallas_standalone__dcn_v2_cross__recsys_kernel(x0, ws, bs):
    return build(TM=576)(x0, ws, bs)
```

```python
import functools

import jax
import jax.numpy as jnp
import numpy as np
import jax.experimental.pallas as pl
import jax.experimental.pallas.tpu as pltpu

f32 = jnp.float32
bf16 = jnp.bfloat16
u32 = jnp.uint32
i32 = jnp.int32


def _dot(a, b):
    return jnp.dot(a, b, preferred_element_type=f32)


LA = {1: [((0, 0), 1), ((1, 1), 1)],
      2: [((0, 0), 1), ((0, 1), 1), ((1, 0), 1), ((1, 1), 1)],
      3: [((0, 0), 1), ((0, 1), -1)],
      4: [((0, 1), 1), ((1, 1), 1)],
      5: [((0, 0), 1), ((0, 1), 1)],
      6: [((0, 1), 1), ((0, 0), -1), ((1, 0), 1), ((1, 1), -1)],
      7: [((0, 1), 1), ((1, 1), -1)]}
D2 = (1.0, 2.0)
BF = {1: 1.0, 2: 0.5, 3: 0.5, 4: 0.5, 5: 0.5, 6: 0.5, 7: 0.5}


def leaf_scale(R, C):
    d = lambda r: D2[r // 2] * D2[r % 2]
    return d(R) / d(C)


def a_ops(a11, a12, a21, a22):
    l1 = a11 + a22
    g = a12 + a21
    return {1: l1, 2: g + l1, 3: a11 - a12, 4: a12 + a22, 5: a11 + a12, 6: g - l1, 7: a12 - a22}


def b_ops(b11, b12, b21, b22):
    r1 = b11 + b22
    g = b12 + b21
    return {1: r1, 2: b11 - b12, 3: b12 - b22, 4: g - r1, 5: b12 + b22, 6: b11 + b12, 7: g + r1}


def lincomb(terms):
    assert terms[0][0] == 1
    acc = terms[0][1]
    for s, v in terms[1:]:
        acc = acc + v if s == 1 else acc - v
    return acc


OUTER = [3, 5, 1, 4, 7, 2, 6]
ROUNDS = [('1', None), ('35', 0), ('35', 1), ('47', 0), ('47', 1), ('26', 0), ('26', 1)]
B11, B12, B21, B22 = (0, 0), (0, 1), (1, 0), (1, 1)
OACTS = {
  'bal': {
    3: ([(1, B12)], [('M3', [(1, 'd')])], []),
    5: ([], [('M5', [(1, 'd')])], [(B12, [(1, 'd'), (1, 'M3')])]),
    1: ([(1, B22), (-1, B12)], [('S', [(1, 'd'), (1, 'M3'), (-1, 'M5')])], []),
    4: ([(1, B11), (-1, B22)], [('A11', [(1, 'd'), (1, 'S')]), ('W', [(1, 'd'), (1, 'M3'), (1, 'M5')])], []),
    7: ([], [('U', [(1, 'W'), (-1, 'd')])], [(B11, [(1, 'd'), (1, 'A11')])]),
    2: ([], [('A22', [(1, 'S'), (-1, 'd')]), ('A21', [(1, 'd'), (1, 'U'), (1, ((1, B21), (1, B22), (-1, B12), (-1, B11)))])], []),
    6: ([], [], [(B22, [(1, 'd'), (1, 'A22')]), (B21, [(1, 'd'), (1, 'A21')])]),
  },
  'raw': {
    3: ([(1, B21), (-1, B11), (1, B22)], [('M3', [(1, 'd')])], []),
    5: ([], [('M5', [(1, 'd')])], [(B12, [(1, 'd'), (1, 'M3'), (1, ((1, B12), (-1, B21), (1, B11), (-1, B22)))])]),
    1: ([(1, B11), (-1, B21)], [('S', [(1, 'd'), (1, 'M3'), (-1, 'M5')])], []),
    4: ([(1, B11), (-1, B22)], [('A11', [(1, 'd')])], []),
    7: ([], [('U', [(1, 'A11'), (-1, 'd'), (1, 'M3'), (1, 'M5')])], [(B11, [(1, 'd'), (1, 'S'), (1, 'A11')])]),
    2: ([], [('A22', [(1, 'd')])], []),
    6: ([], [], [(B22, [(1, 'd'), (1, 'S'), (-1, 'A22')]), (B21, [(1, 'd'), (1, 'U'), (1, 'A22')])]),
  },
  'rawB': {
    3: ([(1, B21), (-1, B11), (1, B22)], [('M3', [(1, 'd')])], []),
    5: ([], [('M5', [(1, 'd')])], [(B12, [(1, 'd'), (1, 'M3'), (1, ((1, B12), (-1, B21), (1, B11), (-1, B22)))])]),
    1: ([(2, B11), (-1, B21), (-1, B22)], [('S', [(1, 'd'), (1, 'M3'), (-1, 'M5')])], []),
    4: ([], [('A11', [(1, 'd')])], []),
    7: ([], [('U', [(1, 'A11'), (-1, 'd'), (1, 'M3'), (1, 'M5')])], [(B11, [(1, 'd'), (1, 'S'), (1, 'A11')])]),
    2: ([(1, B11), (-1, B22)], [('A22', [(1, 'd')])], []),
    6: ([], [], [(B22, [(1, 'd'), (1, 'S'), (-1, 'A22')]), (B21, [(1, 'd'), (1, 'U'), (1, 'A22')])]),
  },
  'raw4': {
    3: ([(1, B21), (-1, B11), (1, B22)], [('M3', [(1, 'd')])], []),
    5: ([], [('M5', [(1, 'd')])], [(B12, [(1, 'd'), (1, 'M3'), (1, ((1, B12), (-1, B21), (1, B11), (-1, B22)))])]),
    1: ([(1, B11), (-1, B21)], [('S', [(1, 'd'), (1, 'M3'), (-1, 'M5')])], []),
    4: ([(1, B11), (-1, B22)], [('A11', [(1, 'd')])], []),
    7: ([], [('U', [(1, 'd')])], [(B11, [(1, 'd'), (1, 'S'), (1, 'A11')])]),
    2: ([], [('A22', [(1, 'd')]), ('A21', [(1, 'd'), (1, 'A11'), (-1, 'U'), (1, 'M3'), (1, 'M5')])], []),
    6: ([], [], [(B22, [(1, 'd'), (1, 'S'), (-1, 'A22')]), (B21, [(1, 'd'), (1, 'A21')])]),
  },
  'raw5': {
    3: ([(1, B12)], [('M3', [(1, 'd')])], []),
    5: ([], [('M5', [(1, 'd')])], [(B12, [(1, 'd'), (1, 'M3')])]),
    1: ([(1, B11), (-1, B12)], [('S', [(1, 'd'), (1, 'M3'), (-1, 'M5')])], []),
    4: ([], [('A11', [(1, 'd')])], []),
    7: ([], [('U', [(1, 'd')])], [(B11, [(1, 'd'), (1, 'S'), (1, 'A11')])]),
    2: ([(1, B11), (-1, B22)], [('A22', [(1, 'd')]),
        ('A21', [(1, 'd'), (1, 'A11'), (-1, 'U'), (1, 'M3'), (1, 'M5'), (1, ((1, B21), (-1, B12), (-1, B11), (1, B22)))])], []),
    6: ([], [], [(B22, [(1, 'd'), (1, 'S'), (-1, 'A22')]), (B21, [(1, 'd'), (1, 'A21')])]),
  },
  'raw2': {
    3: ([(1, B21), (-1, B11), (1, B22)], [('M3', [(1, 'd')])], []),
    5: ([], [('M5', [(1, 'd')])], [(B12, [(1, 'd'), (1, 'M3'), (1, ((1, B12), (-1, B21), (1, B11), (-1, B22)))])]),
    1: ([(1, B11), (-1, B21)], [('S', [(1, 'd'), (1, 'M3'), (-1, 'M5')])], []),
    4: ([(1, B11), (-1, B22)], [('A11', [(1, 'd')]), ('W', [(1, 'd'), (1, 'M3'), (1, 'M5')])], []),
    7: ([], [('U', [(1, 'W'), (-1, 'd')])], [(B11, [(1, 'd'), (1, 'S'), (1, 'A11')])]),
    2: ([], [('A22', [(1, 'd')])], []),
    6: ([], [], [(B22, [(1, 'd'), (1, 'S'), (-1, 'A22')]), (B21, [(1, 'd'), (1, 'U'), (1, 'A22')])]),
  },
  'raw3': {
    3: ([(1, B21), (-1, B11), (1, B22)], [('M3', [(1, 'd')])], []),
    5: ([], [('M5', [(1, 'd')])], [(B12, [(1, 'd'), (1, 'M3'), (1, ((1, B12), (-1, B21), (1, B11), (-1, B22)))])]),
    1: ([(1, B11), (-1, B21)], [('S', [(1, 'd'), (1, 'M3'), (-1, 'M5')])], []),
    4: ([(1, B11), (-1, B22)], [('A11', [(1, 'd')])], []),
    7: ([], [('U', [(1, 'A11'), (-1, 'd')])], [(B11, [(1, 'd'), (1, 'S'), (1, 'A11')])]),
    2: ([], [('A22', [(1, 'd')]), ('A21', [(1, 'd'), (1, 'U'), (1, 'M3'), (1, 'M5')])], []),
    6: ([], [], [(B22, [(1, 'd'), (1, 'S'), (-1, 'A22')]), (B21, [(1, 'd'), (1, 'A21')])]),
  },
}
OSL = {'M3': 0, 'M5': 1, 'S': 2, 'A11': 3, 'W': 4, 'U': 5, 'A22': 6, 'A21': 7}
ISL = {'m1': 0, 's': 1, 'v': 2, 'u': 3}
PREP_ORDER = (2, 6, 3, 5, 1, 4, 7)
X0_COPY = {1: (0, 1), 2: (0, 0), 3: (1, 1), 6: (1, 0)}
CONV_SLOTS = (0, 1, 2, 3)
NX0, NX, NI, NO, NS, N3 = 32, 6, 16, 64, 7, 16
Q3 = (3, 5, 4, 7)
LAG = 8


def place(shapes, base, lo, hi):
    load = list(base) + [0.0] * 8
    out = []
    for sh in shapes:
        t = min(range(lo, hi + 1), key=lambda t: (round(sum((2 * load[t + u] + w) * w for u, w in enumerate(sh)), 6), t))
        for u, w in enumerate(sh):
            load[t + u] += w
        out.append(t)
    return out


def raw_slot(act):
    for name, terms in act[1]:
        if terms == [(1, 'd')]:
            return name
    return None


def rounds_of(p, sel):
    if p in sel:
        return ([('1', None), ('x', '1')] + [(qp, r) for qp in ('35', '47') for r in ('35', '47', '26')]
                + [('26', 0), ('26', 1)])
    return ROUNDS


def round_usage(act, rd, first, last):
    bt, stores, finals = act
    alu = bool(bt) + sum(len(t) - 1 for _, t in stores) + sum(len(t) + (0 if first else 1) + (2 if last else 0) for _, t in finals)
    nst = len(stores) + len(finals)
    nld = len({x for _, t in stores + finals for _, x in t if isinstance(x, str) and x != 'd'}) + len(finals) * (1 if first else 2)
    kind, n = rd
    rs = bool(raw_slot(act))
    if isinstance(n, str):
        e = kind == '47'
        a, st, ld, m = {'1': (4, 4, 0, 0), '35': (11 + e, 3 + (not rs), 3 + e, 1), '47': (14 + 2 * e, 3 + (not rs and not e), 6 + 2 * e, 1),
                        '26': (14 + 2 * e, 2 + 2 * (not rs and not e), 6 + 2 * e, 2)}[n]
        ld += 5
    else:
        a, st, ld, m = {'1': (2, 2, 0, 0), '35': (5, 2 - rs, 1, 1), '47': (6, 1, 2, 1), '26': (6, 0, 2, 2)}[kind]
        ld += 4
    return a + m * alu, st + m * nst, ld + m * nld


def yds(groups, cap):
    n = len(cap)
    speed = [0.0] * n
    cls, gcls = [-1] * n, {}
    free = [True] * n
    todo = list(groups)
    while todo:
        pre = [0.0]
        for t in range(n):
            pre.append(pre[-1] + (cap[t] if free[t] else 0.0))
        best = None
        for a in sorted({g[0] for g in todo}):
            for b in sorted({g[1] for g in todo}):
                if b < a:
                    continue
                w = sum(g[2] for g in todo if g[0] >= a and g[1] <= b)
                if w > 0:
                    d = w / max(pre[b + 1] - pre[a], 1e-9)
                    if best is None or d > best[0]:
                        best = (d, a, b)
        d, a, b = best
        for t in range(a, b + 1):
            if free[t]:
                speed[t], free[t], cls[t] = d, False, len(gcls)
        gcls.update({g[:2]: len(gcls) for g in todo if g[0] >= a and g[1] <= b})
        todo = [g for g in todo if not (g[0] >= a and g[1] <= b)]
    return speed, cls, gcls


def _kernel(x_hbm, w_hbm, b_hbm, o_hbm, *scratch, L, TM, R0, NMAIN, D, cfg):
    H = D // 4
    Mh = TM // 4
    Mq = Mh // 2
    NT = H // 128
    NC = Mh // 16
    MP = cfg['MP']
    SEL = cfg['SEL']
    D3 = D2 if SEL else (1.0, 1.0)
    assert NT == 2 and L % 2 == 0 and (not SEL or Mq % 16 == 0)
    bufs = scratch[:-10]
    bf_ref, xn2_ref, o2_ref, t_ref, t3_ref, w_ref, xr_ref, xp_ref, b_ref, sem = scratch[-10:]
    x0b = bufs[:NX0]
    xb = bufs[NX0:NX0 + NX]
    o = NX0 + NX
    ib = bufs[o:o + NI]
    ob = bufs[o + NI:o + NI + NO]
    o += NI + NO
    jb = bufs[o:o + N3]
    sb = bufs[o + N3:o + N3 + NS]
    s3b = bufs[o + N3 + NS:]
    GROW = 16 * MP
    OACT = OACTS[cfg['OA']]

    def scale(R, C, h, k):
        return leaf_scale(R, C) * D3[h] / D3[k]

    def xset(l):
        return 4 if l == 0 else (l % 2) * 2

    def xloc(l, R, C, k):
        off = 8 * ((2 * (C // 2) + 2 * (R // 2)) % 4)
        return xb[xset(l) + R // 2], (((R % 2) * 4 + C) * 2 + k) * MP + off

    def x0loc(R, C, k):
        return x0b[(R * 4 + C) * 2 + k], 8 * ((2 * (C // 2) + 2 * (R // 2) + 1) % 4)

    def iloc(g, name, n):
        return ib[((g % 2) * 4 + ISL[name]) * 2 + n], 8 * (ISL[name] % 4)

    def oloc(name, i, j, n):
        return ob[(OSL[name] * 4 + i * 2 + j) * 2 + n], 8 * ((OSL[name] + 2 * j) % 4)

    def jloc(qp, name, al):
        i = ((qp == '47') * 4 + ('1', 's', 'u', 'v').index(name)) * 2 + al
        return jb[i], 8 * ((i + i // 2) % 4)

    def const_after(anchor, s, reps):
        sv = jax.lax.bitcast_convert_type(anchor | int(np.float32(s).view(np.int32)), f32)
        return jnp.tile(sv, (reps, 1))

    def conv(src, zs, R, C, r, nr, anchor=None):
        v = src[R * Mh + r:R * Mh + r + nr, C * H:(C + 1) * H].astype(f32)
        for k in range(NT):
            vk = v[:, k * 128:(k + 1) * 128]
            s = scale(R, C, r // Mq, k)
            if anchor is not None:
                vk = vk * const_after(anchor, s, nr // 8)
            elif s != 1.0:
                vk = vk * s
            buf, r0 = xloc(0, R, C, k)
            buf[zs, r0 + r:r0 + r + nr, :] = vk

    ORD = (3, 5, 4, 7, 1, 2, 6)
    SPOS = {q: u for u, q in enumerate(ORD)}

    STAGES = {1: [((0, 0), (0, 1), (1, 1), (1, 0))], 2: [((0, 0), (0, 1)), ((1, 1), (1, 0))],
              3: [((0, 0), (0, 1)), ((1, 1),), ((1, 0),)]}

    def a_unit(E, F, outs_, l, save, st8, group, zs, za, anchor):
        tie = group[1] if len(group) > 1 and group[0] == (0, 0) else group[0]
        def total(plist, ij, first):
            terms = []
            for u, (s, (R, C, k, r)) in enumerate(plist):
                buf, r0 = xloc(l, R, C, k)
                v = buf[za if (u == 0 and R < 2) else 0, r0 + r:r0 + r + 16, :]
                if (R // 2, C // 2) in save:
                    d, d0 = x0loc(R, C, k)
                    s0 = 1.0 / scale(R, C, r // Mq, k)
                    d[zs, d0 + r:d0 + r + 16, :] = v * (s0 if anchor is None else const_after(anchor, s0, 2))
                if anchor is not None and u == 0 and first and ij == tie:
                    top = jax.lax.bitcast_convert_type(jax.lax.bitcast_convert_type(v[0:8], i32) | anchor, f32)
                    v = jnp.concatenate([top, v[8:16]], axis=0)
                terms.append((s, v))
            return lincomb(terms)
        for ij in group:
            e = total(E[ij], ij, True)
            f = total(F[ij], ij, False) if F else None
            for sg, _, _ in outs_:
                st8[(sg, ij)] = e if not F else (e + f if sg == 1 else e - f)
        for sg, qs, (ref, idx, off) in outs_:
            a = lambda i, j: st8[(sg, (i, j))]
            ops = {}
            if (0, 1) in group:
                ops[3], ops[5] = (lambda: a(0, 0) - a(0, 1)), (lambda: a(0, 0) + a(0, 1))
            if (1, 1) in group:
                st8[(sg, 'l1')] = a(0, 0) + a(1, 1)
                ops[4], ops[7], ops[1] = (lambda: a(0, 1) + a(1, 1)), (lambda: a(0, 1) - a(1, 1)), (lambda: st8[(sg, 'l1')])
            if (1, 0) in group:
                gg = a(0, 1) + a(1, 0)
                ops[2], ops[6] = (lambda: gg + st8[(sg, 'l1')]), (lambda: gg - st8[(sg, 'l1')])
            now = [q for q in qs if q in ops]
            if now:
                r0 = 16 * (off + SPOS[now[0]])
                v = jnp.concatenate([ops[q]() for q in now], axis=0)
                ref[(zs,) + idx + (slice(r0, r0 + 16 * len(now)), slice(None))] = v.astype(bf16)

    PAIR = {(5, 3): ([B11], [B12]), (4, 7): ([B12], [B22]), (2, 6): ([B12, B21], [B11, B22])}

    def a_chunk(gs, l, ps, c, k):
        blk = lambda bl: {(i, j): [(s, (2 * I + i, 2 * J + j, k, 16 * c)) for (I, J), s in bl]
                          for i in range(2) for j in range(2)}
        if len(ps) == 1:
            E, F = blk(LA[ps[0]]), None
        else:
            E, F = (blk([(b, 1) for b in bl]) for bl in PAIR[ps])
        save = [b for b, gg in zip((B12, B11, B22, B21), cfg['XC']) if gg in gs and l == 0]
        outs_ = [(sg, ORD[4:] if p in SEL else ORD, (sb[p - 1], (k, c), k)) for sg, p in zip((1, -1), ps)]
        return functools.partial(a_unit, E, F, outs_, l, save)

    def a_chunk3(l, p, qs, c):
        blk = lambda i, j: {(h, k): [(s, (2 * I + i, 2 * J + j, k, h * Mq + 16 * c)) for (I, J), s in LA[p]]
                            for h in range(2) for k in range(2)}
        E, F = (blk(*bl[0]) for bl in PAIR[qs])
        outs_ = [(sg, ORD, (s3b[SEL.index(p)], (Q3.index(q), c), Q3.index(q) % 2)) for sg, q in zip((1, -1), qs)]
        return functools.partial(a_unit, E, F, outs_, l, [])

    def prep(l, r, anchors):
        keep = {}
        for k in range(NT):
            wide = {(R, C): w_ref[l, pl.ds(R * H + k * 128 + r, 16), C * H:(C + 1) * H] for R in range(4) for C in range(4)}
            for n in range(NT):
                def blk(R, C):
                    v = wide[(R, C)].astype(f32)[:, n * 128:(n + 1) * 128]
                    s = D2[R // 2] / D2[C // 2]
                    return v if s == 1.0 else v * s
                B = {(R, C): blk(R, C) for R in range(4) for C in range(4)}
                O = {(i, j): b_ops(B[(i, j)], B[(i, 2 + j)], B[(2 + i, j)], B[(2 + i, 2 + j)])
                     for i in range(2) for j in range(2)}
                for p in PREP_ORDER:
                    anchor = next(anchors)
                    def sc(i, j):
                        s = D2[i] / D2[j] * BF[p] * 0.5 * D3[k] / D3[n]
                        return O[(i, j)][p] * (s if anchor is None else const_after(anchor, s, 2))
                    T = b_ops(sc(0, 0), sc(0, 1), sc(1, 0), sc(1, 1))
                    T[1] = T[1] + T[1]
                    for q in range(1, 8):
                        if p in SEL and q in Q3:
                            keep[(p, q, k, n)] = T[q]
                        else:
                            t_ref[l, (p - 1) * 7 + q - 1, n, pl.ds(k * 128 + r, 16), :] = T[q].astype(bf16)
        for p in SEL:
            for q in Q3:
                half = const_after(next(anchors), 0.5, 2)
                T = b_ops(*[keep[(p, q, k, n)] * half for k in range(2) for n in range(2)])
                T[1] = T[1] + T[1]
                for u in range(1, 8):
                    t3_ref[l, (SEL.index(p) * 4 + Q3.index(q)) * 7 + u - 1, pl.ds(r, 16), :] = T[u].astype(bf16)

    outs = [(l, p) for l in range(L) for p in OUTER]
    G = len(outs)
    sched, start, wts = [], [], []
    for g in range(G):
        start.append(len(wts))
        for rd in rounds_of(outs[g][1], SEL):
            n = NC // 2 if isinstance(rd[1], str) else NC
            sched.append((g, rd, len(wts), n))
            wts += [round_usage(OACT[outs[g][1]], rd, outs[g][0] == 0, outs[g][0] == L - 1)] * n
    start.append(len(wts))
    T = start[G]
    jobs = []
    conv_end = start[G - 7 + cfg['CE']]
    st_ = lambda g: start[g] if g >= 0 else start[g + G] - T
    cost = lambda alu, st, ld: cfg['CA'] * alu / 64 + cfg['CS_'] * st / 16 + cfg['CL'] * ld / 48
    for g in range(G):
        l2, p2 = outs[g]
        top_only = all(I == 0 for (I, J), _ in LA[p2])
        ready = 7 * (g // 7) - (2 if top_only else 0)
        lo = max(st_(ready), conv_end - T)
        hi = max(start[g] - LAG - 3 - cfg['HI'], lo)
        nt = len(LA[p2])
        pr = [ps for ps in PAIR if p2 in ps and ps in cfg['OPAIR']]
        a = []
        if not pr or outs[g + 1 if g + 1 < G else 0][1] in pr[0]:
            ps = pr[0] if pr else (p2,)
            gs = (g, g + 1) if pr else (g,)
            sv = 8 * sum(gg in gs for gg in cfg['XC'])
            nq = sum(3 if p in SEL else 7 for p in ps)
            alu = (8 * nt if pr else 8 * (nt - 1)) + sum(8 if p in SEL else 16 for p in ps) + nq
            ns = cfg['NST'][0] if nq <= 3 else cfg['NST'][1] if nq <= 7 else cfg['NST'][2]
            a = [(lo, hi, cost(alu + sv, nq + ns + sv, 8 * nt), ns, l2, a_chunk(gs, l2, ps, c, k))
                 for c in range(NC) for k in range(NT)]
        if p2 in SEL:
            hi3 = hi + (NC if g else 0)
            b = [(lo, hi3, cost(16 * nt + 46, 17, 16 * nt), 3, l2, a_chunk3(l2, p2, qs, c))
                 for c in range(NC // 2) for qs in ((5, 3), (4, 7))]
            a += b
        jobs += a
    for R in range(4):
        hi = conv_end - 2
        jobs += [(start[6], hi, cost(18, 8, 4), 'conv', 0, (R, C, c)) for C in range(4) for c in range(0, NC, 2)]
    use = [max(cfg['UA'] * a / 32, st / 8, cfg['UL'] * ld / 24) for a, st, ld in wts]
    cap = [max(cfg['CAP'] - max(use[t], use[(t + 1) % T]), 0.0) ** cfg['GAM'] for t in range(T)]
    for t in range(T - cfg['TAIL'], T):
        cap[t] = 0.0
    cap3 = cap * 3
    all3 = [(lo + k * T, hi + k * T, w, ji, k) for k in range(3) for ji, (lo, hi, w, _, _, _) in enumerate(jobs)
            if lo + k * T >= 0]
    grp = {}
    for lo, hi, w, _, _ in all3:
        grp[(lo, hi)] = grp.get((lo, hi), 0.0) + w
    speed, cls, gcls = yds([(lo, hi, w) for (lo, hi), w in grp.items()], cap3)
    when = [[] for _ in jobs]
    pend = {}
    for j in sorted(all3, key=lambda j: (j[1], j[4], j[3])):
        pend.setdefault(j[:2], []).append(j)
    debt = 0.0
    cur, left = None, 0
    FR = {1: (1.0,), 2: cfg['FR2'], 3: cfg['FR3']}
    for t in range(3 * T):
        while True:
            if cur is None:
                rdy = [q[0] for w, q in pend.items() if q and w[0] <= t and (gcls[w] == cls[t] or w[1] <= t)]
                if not rdy:
                    debt = max(debt, 0.0)
                    break
                j = rdy[0]
                nst = 1 if jobs[j[3]][3] == 'conv' else jobs[j[3]][3]
                if nst > 1 and j[1] > t and (t + cfg['TAIL'] + 2 * nst) // T != t // T:
                    break
            else:
                j = cur
            must = j[1] <= t or (cur is not None and (t + cfg['TAIL'] + 1) // T != t // T)
            if not must and (cap3[t] == 0.0 or debt > 0.5 * speed[t] * cap3[t]):
                break
            if cur is None:
                pend[j[:2]].pop(0)
                cur, left = j, nst
            debt += j[2] * FR[nst][nst - left]
            if j[4] == 1:
                when[j[3]].append(t - T)
            left -= 1
            if left == 0:
                cur = None
        debt -= speed[t] * cap3[t]
    if cfg.get('SHOW'):
        for g in range(G):
            print(g, 'speed %.2f' % speed[T + start[g] + 5])
            print('  ', ''.join('%2d' % round(10 * use[t]) for t in range(start[g], start[g + 1])))
            print('  ', ''.join('%2s' % ''.join((str(j[3])[0] if u == 0 else '.') for j, w in zip(jobs, when) for u, x in enumerate(w) if x % T == t) for t in range(start[g], start[g + 1])))
    plan_events = {}
    carried = []
    for ts, (lo, hi, sh, kind, l2, job) in sorted(zip(when, jobs), key=lambda e: e[0][0] % T):
        assert (ts[0] < 0) == (ts[-1] < 0)
        if ts[0] < 0:
            carried.append(job)
        for t, group in zip(ts, [None] if kind == 'conv' else STAGES[kind]):
            plan_events.setdefault(t % T, []).append((kind, l2, job, id(job), group))

    def w_copy(l):
        return pltpu.make_async_copy(w_hbm.at[l], w_ref.at[l], sem.at[l])

    def in_copy(t, slot):
        return pltpu.make_async_copy(x_hbm.at[pl.ds(pl.multiple_of(t * TM, 32), TM)], xn2_ref.at[slot], sem.at[L + slot])

    def out_copy(t, slot, h):
        hm = TM // 2
        return pltpu.make_async_copy(o2_ref.at[slot, pl.ds(h * hm, hm)],
                                     o_hbm.at[pl.ds(pl.multiple_of(t * TM + h * hm, 32), hm)],
                                     sem.at[L + 4 + 2 * slot + h])

    xr_in = pltpu.make_async_copy(x_hbm.at[pl.ds(NMAIN * TM, R0)], xr_ref, sem.at[L + 2])
    xr_out = pltpu.make_async_copy(xr_ref, o_hbm.at[pl.ds(NMAIN * TM, R0)], sem.at[L + 2])
    b_in = pltpu.make_async_copy(b_hbm, b_ref, sem.at[L + 3])

    def prologue():
        b_in.start()
        xr_in.start()
        for l in range(L):
            w_copy(l).start()
        in_copy(0, 0).start()
        in_copy(min(1, NMAIN - 1), 1).start()
        b_in.wait()
        for l in range(L):
            bf_ref[l] = b_ref[l:l + 1, :].astype(f32)
        xr_in.wait()
        xp_ref[...] = xr_ref[...].astype(f32)
        NSUB = cfg['NSUB']
        RB = R0 // NSUB
        PR = 128 // NSUB
        def sub(it, c):
            l = it // NSUB
            j = it % NSUB
            @pl.when(j == 0)
            def _():
                w_copy(l).wait()
            zero = jax.lax.shift_right_logical(it, 12)
            rows = pl.ds(pl.multiple_of(j * RB, RB), RB)
            x = xp_ref[rows, :]
            xbf = x.astype(bf16)
            KH = D // 2
            passes, ys = [], []
            for jt in range(D // 128):
                cols = slice(jt * 128, (jt + 1) * 128)
                ya = _dot(xbf[:, :KH], w_ref[l, 0:KH, cols]) + bf_ref[l, :, cols]
                yb = _dot(xbf[:, KH:], w_ref[l, KH:D, cols]) + ya
                passes += [ya, yb]
                ys.append(yb)
            xp_ref[rows, :] = xr_ref[rows, :].astype(f32) * jnp.concatenate(ys, axis=1) + x
            na = (PR // 16) * (NT * NT * 7 + 4 * len(SEL))
            def gen():
                tot = len(passes) * (RB // 8)
                for u in range(na):
                    if u < cfg['AFREE']:
                        yield None
                        continue
                    f = int((u - cfg['AFREE']) * cfg['ANC'] * tot / (na - cfg['AFREE']))
                    ps, rr = divmod(f, RB // 8)
                    yield jax.lax.bitcast_convert_type(passes[ps][rr * 8:rr * 8 + 8, :], i32) & zero
            anchors = gen()
            for u in range(PR // 16):
                prep(l, pl.multiple_of(j * PR + u * 16, 16), anchors)
            return c
        jax.lax.fori_loop(0, L * NSUB, sub, 0)
        xr_ref[...] = xp_ref[...].astype(bf16)
        xr_out.start()
        in_copy(0, 0).wait()
        for R in range(4):
            for C in range(4):
                for h in range(2):
                    conv(xn2_ref.at[0], 0, R, C, h * Mq, Mq)
        for job in carried:
            job({}, STAGES[1][0], 0, 0, None)

    def main(tile, carry):
        zs, za = jax.lax.shift_right_logical(tile, 12), jax.lax.shift_right_logical(tile, 13)
        slot = tile % 2
        in_copy(jnp.minimum(tile + 2, NMAIN - 1), slot).start()
        in_copy(0, 1 - slot).wait()
        @pl.when(tile > 1)
        def _():
            out_copy(0, slot, 0).wait()
            out_copy(0, slot, 1).wait()
        xn_ref = xn2_ref.at[1 - slot]
        o_ref = o2_ref.at[slot]

        def rows(h):
            return (0, Mh) if h is None else (h * Mq, Mq)

        def ld(loc, h=None):
            r0, nr = rows(h)
            return loc[0][0, loc[1] + r0:loc[1] + r0 + nr, :]

        def st(loc, v, h=None):
            r0, nr = rows(h)
            loc[0][zs, loc[1] + r0:loc[1] + r0 + nr, :] = v

        def by_half(v, h, fn):
            if h is not None:
                return fn(v, h)
            if not SEL:
                return fn(v, 0)
            return jnp.concatenate([fn(v[:Mq], 0), fn(v[Mq:], 1)], axis=0)

        def gather(ref, idx, slot_):
            if cfg['NOBC']:
                v = ref[idx + (slice(None), slice(slot_ * 16, slot_ * 16 + 16), slice(None))]
                return v.reshape(v.shape[0] * 16, 128)
            v = ref.bitcast(u32)[idx + (slice(None), slice(slot_ * 8, slot_ * 8 + 8), slice(None))]
            return v.reshape(v.shape[0] * 8, 128)

        def as_bf16(v):
            return v if cfg['NOBC'] else pltpu.bitcast(v, bf16)

        def lhs_load(p, q):
            return as_bf16(jnp.concatenate([gather(sb[p - 1], (0, k), SPOS[q] + k) for k in range(NT)], axis=1))

        def wload(l, p, q, n):
            return as_bf16((t_ref if cfg['NOBC'] else t_ref.bitcast(u32))[l, (p - 1) * 7 + q - 1, n])

        def tile_dot(l, p, q, r):
            u = Q3.index(q)
            lhs = as_bf16(gather(s3b[SEL.index(p)], (0, u), SPOS[r] + u % 2))
            w = as_bf16((t3_ref if cfg['NOBC'] else t3_ref.bitcast(u32))[l, (SEL.index(p) * 4 + u) * 7 + r - 1])
            return _dot(lhs, w)

        def bias(l, terms, where):
            coef = {}
            for sg, i, j, n, h in where:
                for cf, (I, J) in terms:
                    R, C = 2 * I + i, 2 * J + j
                    coef[(C, n)] = coef.get((C, n), 0.0) + sg * cf * scale(R, C, h, n)
            acc = None
            for (C, n), cf in sorted(coef.items()):
                if cf == 0.0:
                    continue
                bv = bf_ref[l, :, C * H + n * 128:C * H + (n + 1) * 128]
                if l == 0:
                    bv = bv + 1.0
                bv = bv if cf == 1.0 else bv * cf
                acc = bv if acc is None else acc + bv
            return acc

        def add_bias(v, l, terms, where, h):
            if h is not None:
                return v + bias(l, terms, where(h))
            bv = bias(l, terms, where(0))
            return by_half(v, h, lambda x, hh: x + (bv if D3[hh] == 1.0 else bv * D3[hh]))

        def outer_act(l, p, i, j, n, d, h=None):
            bt, stores, finals = OACT[p]
            if bt:
                def where(hh):
                    w = [(1, i, j, n, hh)]
                    if raw_slot(OACT[p]) and (i, j) == (1, 0):
                        w.append((-1, 0, 1, n, hh))
                    if raw_slot(OACT[p]) and (h, n) == (1, 0):
                        w.append((-1, i, j, 1, 0))
                    return w
                d = add_bias(d, l, bt, where, h)
            cache = {'d': d}
            def comb(terms):
                for _, src in terms:
                    if isinstance(src, str) and src not in cache:
                        cache[src] = ld(oloc(src, i, j, n), h)
                v = lincomb([(s, cache[src]) for s, src in terms if isinstance(src, str)])
                for _, src in terms:
                    if not isinstance(src, str):
                        v = add_bias(v, l, src, lambda hh: [(1, i, j, n, hh)], h)
                return v
            fin = [(IJ, comb(terms)) for IJ, terms in finals]
            stl = [(name, comb(terms)) for name, terms in stores]
            for name, v in stl:
                st(oloc(name, i, j, n), v, h)
            for (I, J), y in fin:
                R, C = 2 * I + i, 2 * J + j
                xn = ld(x0loc(R, C, n), h) * y
                if l > 0:
                    xn = xn + ld(xloc(l, R, C, n), h)
                if l == L - 1:
                    xn = by_half(xn, h, lambda x, hh: x if scale(R, C, hh, n) == 1.0 else x * (1.0 / scale(R, C, hh, n)))
                    r0, nr = rows(h)
                    o_ref[R * Mh + r0:R * Mh + r0 + nr, C * H + n * 128:C * H + (n + 1) * 128] = xn.astype(o_ref.dtype)
                else:
                    st(xloc(l + 1, R, C, n), xn, h)

        def issue(g, l, p, rd):
            kind, n = rd
            if n == '1':
                return tuple(tile_dot(l, p, q, 1) for q in Q3)
            if isinstance(n, str):
                return tuple(tile_dot(l, p, int(q), int(r)) for r in n for q in kind)
            if kind == '1':
                lhs = lhs_load(p, 1)
                return (_dot(lhs, wload(l, p, 1, 0)), _dot(lhs, wload(l, p, 1, 1)))
            qa, qb = int(kind[0]), int(kind[1])
            return (_dot(lhs_load(p, qa), wload(l, p, qa, n)), _dot(lhs_load(p, qb), wload(l, p, qb, n)))

        def inner_act(g, l, p, kind, n, h, P, Q):
            rs = raw_slot(OACT[p])
            if kind == '35':
                st(iloc(g, 's', n), Q + ld(iloc(g, 'm1', n), h), h)
                if not rs:
                    st(iloc(g, 'v', n), P, h)
                outer_act(l, p, 0, 1, n, P, h)
            elif kind == '47':
                st(iloc(g, 'u', n), Q + ld(oloc(rs, 0, 1, n) if rs else iloc(g, 'v', n), h), h)
                outer_act(l, p, 0, 0, n, P + ld(iloc(g, 's', n), h), h)
            else:
                outer_act(l, p, 1, 1, n, ld(iloc(g, 's', n), h) - Q, h)
                outer_act(l, p, 1, 0, n, P + ld(iloc(g, 'u', n), h), h)

        def consume(g, l, p, rd, res):
            kind, n = rd
            if n == '1':
                for qp, a, b in (('35', res[0], res[1]), ('47', res[2], res[3])):
                    st(jloc(qp, '1', 0), a + b, 0)
                    st(jloc(qp, '1', 1), a - b, 0)
            elif isinstance(n, str):
                x, z, y, w = res
                aa, bb = (x + z, x - z), (y + w, y - w)
                sm = [aa[al] + bb[al] for al in range(2)]
                df = [aa[al] - bb[al] for al in range(2)]
                J = lambda name, al: ld(jloc(kind, name, al), 0)
                if n == '35':
                    for al in range(2):
                        st(jloc(kind, 's', al), df[al] + J('1', al), 0)
                    if kind == '47' and not raw_slot(OACT[p]):
                        st(jloc(kind, 'v', 0), sm[0], 0)
                    inner_act(g, l, p, kind, 1, 0, sm[0], sm[1])
                elif n == '47':
                    rs = raw_slot(OACT[p])
                    vin = oloc(rs, 0, 1, 1) if rs else iloc(g, 'v', 1)
                    if kind == '35':
                        v = [[(1, vin)], [(1, iloc(g, 's', 1)), (-1, iloc(g, 'm1', 1))]]
                    else:
                        v = [[(1, oloc(rs, 0, 0, 1)), (-1, iloc(g, 's', 1))] if rs else [(1, jloc(kind, 'v', 0))],
                             [(1, iloc(g, 'u', 1)), (-1, vin)]]
                    for al in range(2):
                        st(jloc(kind, 'u', al), lincomb([(1, df[al])] + [(s, ld(loc, 0)) for s, loc in v[al]]), 0)
                    inner_act(g, l, p, kind, 0, 0, sm[0] + J('s', 0), sm[1] + J('s', 1))
                else:
                    inner_act(g, l, p, kind, 1, 1, J('s', 0) - df[0], J('s', 1) - df[1])
                    inner_act(g, l, p, kind, 0, 1, sm[0] + J('u', 0), sm[1] + J('u', 1))
            elif kind == '1':
                st(iloc(g, 'm1', 0), res[0])
                st(iloc(g, 'm1', 1), res[1])
            else:
                inner_act(g, l, p, kind, n, None, res[0] + res[1], res[0] - res[1])

        events = {t: list(v) for t, v in plan_events.items()}
        state = {}
        for g, rd, t0, n in sched:
            l, p = outs[g]
            if g == G - 1 and t0 == start[g]:
                out_copy(tile, slot, 0).start()
            res = issue(g, l, p, rd)
            for t in range(t0, t0 + n):
                for kind, l2, job, key, stage in events.pop(t, []):
                    gr = 16 * (t - t0)
                    gate = res[cfg['GSRC']][gr + cfg['GPH']:gr + cfg['GPH'] + 8, :]
                    anchor = jax.lax.bitcast_convert_type(gate, i32) & zs
                    if kind != 'conv':
                        xb[xset(l2)][0, GROW:GROW + 8, :] = gate
                        job(state.setdefault(key, {}), stage, zs, za, anchor)
                    else:
                        R, C, c = job
                        for cc in range(c, min(c + 2, NC)):
                            conv(xn_ref, zs, R, C, 16 * cc, 16, anchor)
            consume(g, l, p, rd, res)
        assert not events
        out_copy(tile, slot, 1).start()
        return carry

    prologue()
    jax.lax.fori_loop(0, NMAIN, main, 0)
    xr_out.wait()
    in_copy(0, (NMAIN - 1) % 2).wait()
    for t in range(max(NMAIN - 2, 0), NMAIN):
        out_copy(0, t % 2, 0).wait()
        out_copy(0, t % 2, 1).wait()


DEFAULT = dict(UNIT=60, LO=0, HI=0, NSUB=1, ANC=0.98, AFREE=4, DBC=True, NOBC=0, OA='raw5', VW=3, CS=(0, 2, 3, 5), XC=(1, 2, 4, 6),
               SEL=(3, 5, 4, 7), AHEAD=7, CE=5, TAIL=6, GPH=8, GSRC=0, CA=1.0, CS_=0.5, CL=0.3, UA=1.0, UL=0.8, CAP=0.85, OPAIR=((2, 6),), FR2=(.4, .6), FR3=(.35, .37, .28), NST=(1, 2, 3), GAM=1.0, MIX=0, SPLIT=('big4', 'big'), SGAP=1, F4=1.0, BIG=(1, 1, .4), SMALL=(.5, .2), CONVW=(.6, .2))


def build(TM=512, **kw):
    def f(x0, ws, bs):
        B, D = x0.shape
        L = ws.shape[0]
        H = D // 4
        Mh = TM // 4
        nmain = (B - 1) // TM
        R0 = B - nmain * TM
        cfg = dict(DEFAULT, **kw)
        MP = cfg['MP'] = (Mh + 24 + 31) // 32 * 32
        half = pltpu.VMEM((1, MP, 128), f32)
        xhalf = pltpu.VMEM((1, 16 * MP + 32, 128), f32)
        sop = pltpu.VMEM((1, H // 128, Mh // 16, 128, 128), bf16)
        s3op = pltpu.VMEM((1, 4, max(Mh // 32, 1), 128, 128), bf16)
        t3sh = pltpu.VMEM((L, max(len(cfg['SEL']), 1) * 28, 128, 128), bf16)
        tsh = pltpu.VMEM((L, 49, H // 128, H, 128), bf16)
        anyspec = pl.BlockSpec(memory_space=pl.ANY)
        return pl.pallas_call(
            functools.partial(_kernel, L=L, TM=TM, R0=R0, NMAIN=nmain, D=D, cfg=cfg),
            in_specs=[anyspec, anyspec, anyspec],
            out_specs=anyspec,
            out_shape=jax.ShapeDtypeStruct((B, D), x0.dtype),
            scratch_shapes=[half] * NX0 + [xhalf] * NX + [half] * (NI + NO + N3) + [sop] * NS + [s3op] * len(cfg['SEL'])
                           + [pltpu.VMEM((8, 1, D), f32), pltpu.VMEM((2, TM, D), bf16), pltpu.VMEM((2, TM, D), bf16), tsh, t3sh,
                              pltpu.VMEM((L, D, D), bf16), pltpu.VMEM((R0, D), bf16), pltpu.VMEM((R0, D), f32),
                              pltpu.VMEM((L, D), bf16), pltpu.SemaphoreType.DMA((L + 8,))],
            compiler_params=pltpu.CompilerParams(
                vmem_limit_bytes=110 * 1024 * 1024,
                internal_scratch_in_bytes=65536,
                disable_bounds_checks=cfg['DBC'],
            ),
        )(x0, ws, bs)
    return f


@jax.jit
def pallas_standalone__dcn_v2_cross__recsys_kernel(x0, ws, bs):
    return build(TM=640)(x0, ws, bs)
```

```python
import functools

import jax
import jax.numpy as jnp
import numpy as np
import jax.experimental.pallas as pl
import jax.experimental.pallas.tpu as pltpu

f32 = jnp.float32
bf16 = jnp.bfloat16
u32 = jnp.uint32
i32 = jnp.int32


def _dot(a, b):
    return jnp.dot(a, b, preferred_element_type=f32)


LA = {1: [((0, 0), 1), ((1, 1), 1)],
      2: [((0, 0), 1), ((0, 1), 1), ((1, 0), 1), ((1, 1), 1)],
      3: [((0, 0), 1), ((0, 1), -1)],
      4: [((0, 1), 1), ((1, 1), 1)],
      5: [((0, 0), 1), ((0, 1), 1)],
      6: [((0, 1), 1), ((0, 0), -1), ((1, 0), 1), ((1, 1), -1)],
      7: [((0, 1), 1), ((1, 1), -1)]}
D2 = (1.0, 2.0)
BF = {1: 1.0, 2: 0.5, 3: 0.5, 4: 0.5, 5: 0.5, 6: 0.5, 7: 0.5}


def leaf_scale(R, C):
    d = lambda r: D2[r // 2] * D2[r % 2]
    return d(R) / d(C)


def a_ops(a11, a12, a21, a22):
    l1 = a11 + a22
    g = a12 + a21
    return {1: l1, 2: g + l1, 3: a11 - a12, 4: a12 + a22, 5: a11 + a12, 6: g - l1, 7: a12 - a22}


def b_ops(b11, b12, b21, b22):
    r1 = b11 + b22
    g = b12 + b21
    return {1: r1, 2: b11 - b12, 3: b12 - b22, 4: g - r1, 5: b12 + b22, 6: b11 + b12, 7: g + r1}


def lincomb(terms):
    assert terms[0][0] == 1
    acc = terms[0][1]
    for s, v in terms[1:]:
        acc = acc + v if s == 1 else acc - v
    return acc


OUTER = [3, 5, 1, 4, 7, 2, 6]
ROUNDS = [('1', None), ('35', 0), ('35', 1), ('47', 0), ('47', 1), ('26', 0), ('26', 1)]
B11, B12, B21, B22 = (0, 0), (0, 1), (1, 0), (1, 1)
OACTS = {
  'bal': {
    3: ([(1, B12)], [('M3', [(1, 'd')])], []),
    5: ([], [('M5', [(1, 'd')])], [(B12, [(1, 'd'), (1, 'M3')])]),
    1: ([(1, B22), (-1, B12)], [('S', [(1, 'd'), (1, 'M3'), (-1, 'M5')])], []),
    4: ([(1, B11), (-1, B22)], [('A11', [(1, 'd'), (1, 'S')]), ('W', [(1, 'd'), (1, 'M3'), (1, 'M5')])], []),
    7: ([], [('U', [(1, 'W'), (-1, 'd')])], [(B11, [(1, 'd'), (1, 'A11')])]),
    2: ([], [('A22', [(1, 'S'), (-1, 'd')]), ('A21', [(1, 'd'), (1, 'U'), (1, ((1, B21), (1, B22), (-1, B12), (-1, B11)))])], []),
    6: ([], [], [(B22, [(1, 'd'), (1, 'A22')]), (B21, [(1, 'd'), (1, 'A21')])]),
  },
  'raw': {
    3: ([(1, B21), (-1, B11), (1, B22)], [('M3', [(1, 'd')])], []),
    5: ([], [('M5', [(1, 'd')])], [(B12, [(1, 'd'), (1, 'M3'), (1, ((1, B12), (-1, B21), (1, B11), (-1, B22)))])]),
    1: ([(1, B11), (-1, B21)], [('S', [(1, 'd'), (1, 'M3'), (-1, 'M5')])], []),
    4: ([(1, B11), (-1, B22)], [('A11', [(1, 'd')])], []),
    7: ([], [('U', [(1, 'A11'), (-1, 'd'), (1, 'M3'), (1, 'M5')])], [(B11, [(1, 'd'), (1, 'S'), (1, 'A11')])]),
    2: ([], [('A22', [(1, 'd')])], []),
    6: ([], [], [(B22, [(1, 'd'), (1, 'S'), (-1, 'A22')]), (B21, [(1, 'd'), (1, 'U'), (1, 'A22')])]),
  },
  'rawB': {
    3: ([(1, B21), (-1, B11), (1, B22)], [('M3', [(1, 'd')])], []),
    5: ([], [('M5', [(1, 'd')])], [(B12, [(1, 'd'), (1, 'M3'), (1, ((1, B12), (-1, B21), (1, B11), (-1, B22)))])]),
    1: ([(2, B11), (-1, B21), (-1, B22)], [('S', [(1, 'd'), (1, 'M3'), (-1, 'M5')])], []),
    4: ([], [('A11', [(1, 'd')])], []),
    7: ([], [('U', [(1, 'A11'), (-1, 'd'), (1, 'M3'), (1, 'M5')])], [(B11, [(1, 'd'), (1, 'S'), (1, 'A11')])]),
    2: ([(1, B11), (-1, B22)], [('A22', [(1, 'd')])], []),
    6: ([], [], [(B22, [(1, 'd'), (1, 'S'), (-1, 'A22')]), (B21, [(1, 'd'), (1, 'U'), (1, 'A22')])]),
  },
  'raw4': {
    3: ([(1, B21), (-1, B11), (1, B22)], [('M3', [(1, 'd')])], []),
    5: ([], [('M5', [(1, 'd')])], [(B12, [(1, 'd'), (1, 'M3'), (1, ((1, B12), (-1, B21), (1, B11), (-1, B22)))])]),
    1: ([(1, B11), (-1, B21)], [('S', [(1, 'd'), (1, 'M3'), (-1, 'M5')])], []),
    4: ([(1, B11), (-1, B22)], [('A11', [(1, 'd')])], []),
    7: ([], [('U', [(1, 'd')])], [(B11, [(1, 'd'), (1, 'S'), (1, 'A11')])]),
    2: ([], [('A22', [(1, 'd')]), ('A21', [(1, 'd'), (1, 'A11'), (-1, 'U'), (1, 'M3'), (1, 'M5')])], []),
    6: ([], [], [(B22, [(1, 'd'), (1, 'S'), (-1, 'A22')]), (B21, [(1, 'd'), (1, 'A21')])]),
  },
  'raw5': {
    3: ([(1, B12)], [('M3', [(1, 'd')])], []),
    5: ([], [('M5', [(1, 'd')])], [(B12, [(1, 'd'), (1, 'M3')])]),
    1: ([(1, B11), (-1, B12)], [('S', [(1, 'd'), (1, 'M3'), (-1, 'M5')])], []),
    4: ([], [('A11', [(1, 'd')])], []),
    7: ([], [('U', [(1, 'd')])], [(B11, [(1, 'd'), (1, 'S'), (1, 'A11')])]),
    2: ([(1, B11), (-1, B22)], [('A22', [(1, 'd')]),
        ('A21', [(1, 'd'), (1, 'A11'), (-1, 'U'), (1, 'M3'), (1, 'M5'), (1, ((1, B21), (-1, B12), (-1, B11), (1, B22)))])], []),
    6: ([], [], [(B22, [(1, 'd'), (1, 'S'), (-1, 'A22')]), (B21, [(1, 'd'), (1, 'A21')])]),
  },
  'raw2': {
    3: ([(1, B21), (-1, B11), (1, B22)], [('M3', [(1, 'd')])], []),
    5: ([], [('M5', [(1, 'd')])], [(B12, [(1, 'd'), (1, 'M3'), (1, ((1, B12), (-1, B21), (1, B11), (-1, B22)))])]),
    1: ([(1, B11), (-1, B21)], [('S', [(1, 'd'), (1, 'M3'), (-1, 'M5')])], []),
    4: ([(1, B11), (-1, B22)], [('A11', [(1, 'd')]), ('W', [(1, 'd'), (1, 'M3'), (1, 'M5')])], []),
    7: ([], [('U', [(1, 'W'), (-1, 'd')])], [(B11, [(1, 'd'), (1, 'S'), (1, 'A11')])]),
    2: ([], [('A22', [(1, 'd')])], []),
    6: ([], [], [(B22, [(1, 'd'), (1, 'S'), (-1, 'A22')]), (B21, [(1, 'd'), (1, 'U'), (1, 'A22')])]),
  },
  'raw3': {
    3: ([(1, B21), (-1, B11), (1, B22)], [('M3', [(1, 'd')])], []),
    5: ([], [('M5', [(1, 'd')])], [(B12, [(1, 'd'), (1, 'M3'), (1, ((1, B12), (-1, B21), (1, B11), (-1, B22)))])]),
    1: ([(1, B11), (-1, B21)], [('S', [(1, 'd'), (1, 'M3'), (-1, 'M5')])], []),
    4: ([(1, B11), (-1, B22)], [('A11', [(1, 'd')])], []),
    7: ([], [('U', [(1, 'A11'), (-1, 'd')])], [(B11, [(1, 'd'), (1, 'S'), (1, 'A11')])]),
    2: ([], [('A22', [(1, 'd')]), ('A21', [(1, 'd'), (1, 'U'), (1, 'M3'), (1, 'M5')])], []),
    6: ([], [], [(B22, [(1, 'd'), (1, 'S'), (-1, 'A22')]), (B21, [(1, 'd'), (1, 'A21')])]),
  },
}
OSL = {'M3': 0, 'M5': 1, 'S': 2, 'A11': 3, 'W': 4, 'U': 5, 'A22': 6, 'A21': 7}
ISL = {'m1': 0, 's': 1, 'v': 2, 'u': 3}
PREP_ORDER = (2, 6, 3, 5, 1, 4, 7)
X0_COPY = {1: (0, 1), 2: (0, 0), 3: (1, 1), 6: (1, 0)}
CONV_SLOTS = (0, 1, 2, 3)
NX0, NX, NI, NO, NS, N3 = 32, 6, 16, 64, 7, 26
Q3 = (3, 5, 4, 7)
Q6 = (3, 5, 4, 7, 2, 6)
LAG = 8


def place(shapes, base, lo, hi):
    load = list(base) + [0.0] * 8
    out = []
    for sh in shapes:
        t = min(range(lo, hi + 1), key=lambda t: (round(sum((2 * load[t + u] + w) * w for u, w in enumerate(sh)), 6), t))
        for u, w in enumerate(sh):
            load[t + u] += w
        out.append(t)
    return out


def raw_slot(act):
    for name, terms in act[1]:
        if terms == [(1, 'd')]:
            return name
    return None


def rounds_of(p, sel, sel3):
    if p in sel:
        tail = [('26', 0), ('26', 1)]
        if p in sel3:
            tail = [('y', '1')] * (sel3.index(p) % 2 == 0) + [('26', r) for r in ('35', '47', '26')]
        return [('1', None), ('x', '1')] + [(qp, r) for qp in ('35', '47') for r in ('35', '47', '26')] + tail
    return ROUNDS


def round_usage(act, rd, first, last):
    bt, stores, finals = act
    alu = bool(bt) + sum(len(t) - 1 for _, t in stores) + sum(len(t) + (0 if first else 1) + (2 if last else 0) for _, t in finals)
    nst = len(stores) + len(finals)
    nld = len({x for _, t in stores + finals for _, x in t if isinstance(x, str) and x != 'd'}) + len(finals) * (1 if first else 2)
    kind, n = rd
    rs = bool(raw_slot(act))
    if isinstance(n, str):
        e = kind == '47'
        if kind == '26':
            a, st, ld, m = {'35': (12, 2, 4, 2), '47': (18, 2, 8, 2), '26': (16, 0, 8, 4)}[n]
            return a + m * alu, st + m * nst, ld + 5 + m * nld
        a, st, ld, m = {'1': (4, 4, 0, 0), '35': (11 + e, 3 + (not rs), 3 + e, 1), '47': (14 + 2 * e, 3 + (not rs and not e), 6 + 2 * e, 1),
                        '26': (14 + 2 * e, 2 + 2 * (not rs and not e), 6 + 2 * e, 2)}[n]
        ld += 5
    else:
        a, st, ld, m = {'1': (2, 2, 0, 0), '35': (5, 2 - rs, 1, 1), '47': (6, 1, 2, 1), '26': (6, 0, 2, 2)}[kind]
        ld += 4
    return a + m * alu, st + m * nst, ld + m * nld


def yds(groups, cap):
    n = len(cap)
    speed = [0.0] * n
    cls, gcls = [-1] * n, {}
    free = [True] * n
    todo = list(groups)
    while todo:
        pre = [0.0]
        for t in range(n):
            pre.append(pre[-1] + (cap[t] if free[t] else 0.0))
        best = None
        for a in sorted({g[0] for g in todo}):
            for b in sorted({g[1] for g in todo}):
                if b < a:
                    continue
                w = sum(g[2] for g in todo if g[0] >= a and g[1] <= b)
                if w > 0:
                    d = w / max(pre[b + 1] - pre[a], 1e-9)
                    if best is None or d > best[0]:
                        best = (d, a, b)
        d, a, b = best
        for t in range(a, b + 1):
            if free[t]:
                speed[t], free[t], cls[t] = d, False, len(gcls)
        gcls.update({g[:2]: len(gcls) for g in todo if g[0] >= a and g[1] <= b})
        todo = [g for g in todo if not (g[0] >= a and g[1] <= b)]
    return speed, cls, gcls


def _kernel(x_hbm, w_hbm, b_hbm, o_hbm, *scratch, L, TM, R0, NMAIN, D, cfg):
    H = D // 4
    Mh = TM // 4
    Mq = Mh // 2
    NT = H // 128
    NC = Mh // 16
    MP = cfg['MP']
    SEL = cfg['SEL']
    SEL3 = cfg['SEL3']
    q3of = lambda p: Q6 if p in SEL3 else Q3 if p in SEL else ()
    TIDX = {pq: u for u, pq in enumerate((p, q) for p in range(1, 8) for q in range(1, 8) if q not in q3of(p))}
    T3OFF = {p: sum(len(q3of(x)) for x in SEL[:u]) for u, p in enumerate(SEL)}
    D3 = D2 if SEL else (1.0, 1.0)
    assert NT == 2 and L % 2 == 0 and (not SEL or Mq % 16 == 0)
    bufs = scratch[:-10]
    bf_ref, xn2_ref, o2_ref, t_ref, t3_ref, w_ref, xr_ref, xp_ref, b_ref, sem = scratch[-10:]
    x0b = bufs[:NX0]
    xb = bufs[NX0:NX0 + NX]
    o = NX0 + NX
    ib = bufs[o:o + NI]
    ob = bufs[o + NI:o + NI + NO]
    o += NI + NO
    jb = bufs[o:o + N3]
    sb = bufs[o + N3:o + N3 + NS]
    s3b = bufs[o + N3 + NS:]
    GROW = 16 * MP
    kb = xb[0:2]
    OACT = OACTS[cfg['OA']]

    def scale(R, C, h, k):
        return leaf_scale(R, C) * D3[h] / D3[k]

    def xset(l):
        return 4 if l == 0 else (l % 2) * 2

    def xloc(l, R, C, k):
        off = 8 * ((2 * (C // 2) + 2 * (R // 2)) % 4)
        return xb[xset(l) + R // 2], (((R % 2) * 4 + C) * 2 + k) * MP + off

    def x0loc(R, C, k):
        return x0b[(R * 4 + C) * 2 + k], 8 * ((2 * (C // 2) + 2 * (R // 2) + 1) % 4)

    def iloc(g, name, n):
        return ib[((g % 2) * 4 + ISL[name]) * 2 + n], 8 * (ISL[name] % 4)

    def oloc(name, i, j, n):
        return ob[(OSL[name] * 4 + i * 2 + j) * 2 + n], 8 * ((OSL[name] + 2 * j) % 4)

    def jloc(qp, name, al, second=False):
        i = (('35', '47', '26').index(qp) * 4 + ('1', 's', 'u', 'v').index(name)) * 2 + al
        if second:
            i = 24 + al
        return jb[i], 8 * ((i + i // 2) % 4)

    def const_after(anchor, s, reps):
        sv = jax.lax.bitcast_convert_type(anchor | int(np.float32(s).view(np.int32)), f32)
        return jnp.tile(sv, (reps, 1))

    def conv(src, zs, R, C, r, nr, anchor=None):
        v = src[R * Mh + r:R * Mh + r + nr, C * H:(C + 1) * H].astype(f32)
        for k in range(NT):
            vk = v[:, k * 128:(k + 1) * 128]
            s = scale(R, C, r // Mq, k)
            if anchor is not None:
                vk = vk * const_after(anchor, s, nr // 8)
            elif s != 1.0:
                vk = vk * s
            buf, r0 = xloc(0, R, C, k)
            buf[zs, r0 + r:r0 + r + nr, :] = vk

    ORD = (3, 5, 4, 7, 1, 2, 6)
    SPOS = {q: u for u, q in enumerate(ORD)}

    STAGES = {1: [((0, 0), (0, 1), (1, 1), (1, 0))], 2: [((0, 0), (0, 1)), ((1, 1), (1, 0))],
              3: [((0, 0), (0, 1)), ((1, 1),), ((1, 0),)], 4: [((0, 0),), ((0, 1),), ((1, 1),), ((1, 0),)]}

    def a_unit(E, F, outs_, l, save, fdst, st8, group, zs, za, anchor):
        tie = group[1] if len(group) > 1 and group[0] == (0, 0) else group[0]
        def total(plist, ij, first):
            terms = []
            for u, (s, (R, C, k, r)) in enumerate(plist):
                buf, r0 = xloc(l, R, C, k)
                v = buf[za if (u == 0 and R < 2) else 0, r0 + r:r0 + r + 16, :]
                if (R // 2, C // 2) in save:
                    d, d0 = x0loc(R, C, k)
                    s0 = 1.0 / scale(R, C, r // Mq, k)
                    d[zs, d0 + r:d0 + r + 16, :] = v * (s0 if anchor is None else const_after(anchor, s0, 2))
                if anchor is not None and u == 0 and first and ij == tie:
                    top = jax.lax.bitcast_convert_type(jax.lax.bitcast_convert_type(v[0:8], i32) | anchor, f32)
                    v = jnp.concatenate([top, v[8:16]], axis=0)
                terms.append((s, v))
            return lincomb(terms)
        for ij in group:
            e = total(E[ij], ij, True)
            f = total(F[ij], ij, False) if F else None
            if fdst:
                ref, idx, off = fdst(*ij)
                ref[(zs,) + idx + (slice(16 * off, 16 * off + 16), slice(None))] = f.astype(bf16)
            for sg, _, _ in outs_:
                st8[(sg, ij)] = e if not F else (e + f if sg == 1 else e - f)
        for sg, qs, (ref, idx, off) in outs_:
            a = lambda i, j: st8[(sg, (i, j))]
            ops = {}
            if (0, 1) in group:
                ops[3], ops[5] = (lambda: a(0, 0) - a(0, 1)), (lambda: a(0, 0) + a(0, 1))
            if (1, 1) in group:
                st8[(sg, 'l1')] = a(0, 0) + a(1, 1)
                ops[4], ops[7], ops[1] = (lambda: a(0, 1) + a(1, 1)), (lambda: a(0, 1) - a(1, 1)), (lambda: st8[(sg, 'l1')])
            if (1, 0) in group:
                gg = a(0, 1) + a(1, 0)
                ops[2], ops[6] = (lambda: gg + st8[(sg, 'l1')]), (lambda: gg - st8[(sg, 'l1')])
            now = [q for q in qs if q in ops]
            if now:
                r0 = 16 * (off + SPOS[now[0]])
                v = jnp.concatenate([ops[q]() for q in now], axis=0)
                ref[(zs,) + idx + (slice(r0, r0 + 16 * len(now)), slice(None))] = v.astype(bf16)

    PAIR = {(5, 3): ([B11], [B12]), (4, 7): ([B12], [B22]), (2, 6): ([B12, B21], [B11, B22])}

    def a_chunk(gs, l, ps, c, k):
        blk = lambda bl: {(i, j): [(s, (2 * I + i, 2 * J + j, k, 16 * c)) for (I, J), s in bl]
                          for i in range(2) for j in range(2)}
        if len(ps) == 1:
            E, F = blk(LA[ps[0]]), None
        else:
            E, F = (blk([(b, 1) for b in bl]) for bl in PAIR[ps])
        save = [b for b, gg in zip((B12, B11, B22, B21), cfg['XC']) if gg in gs and l == 0]
        outs_ = [(sg, ORD[4:] if p in SEL else ORD, (sb[p - 1], (k, c), k)) for sg, p in zip((1, -1), ps)]
        return functools.partial(a_unit, E, F, outs_, l, save, None)

    def a_chunk3(g, l, p, qs, c):
        blk = lambda bl: {(h, k): [(s, (2 * I + i, 2 * J + j, k, h * Mq + 16 * c)) for i, j in bl for (I, J), s in LA[p]]
                          for h in range(2) for k in range(2)}
        E, F = (blk(bl) for bl in PAIR[qs])
        outs_ = [(sg, ORD, (s3b[SEL.index(p)], (Q6.index(q), c), Q6.index(q) % 2)) for sg, q in zip((1, -1), qs)]
        if qs != (2, 6):
            return functools.partial(a_unit, E, F, outs_, l, [], None)
        save = [b for b, gg in zip((B12, B11, B22, B21), cfg['XC']) if gg == g and l == 0]
        fdst = lambda h, k: (sb[p - 1], (k, h * (NC // 2) + c), k + SPOS[1])
        return functools.partial(a_unit, E, F, outs_, l, save, fdst)

    def prep(l, r, anchors, zero, par):
        keep = {}
        for k in range(NT):
            wide = {(R, C): w_ref[l, pl.ds(R * H + k * 128 + r, 16), C * H:(C + 1) * H] for R in range(4) for C in range(4)}
            for n in range(NT):
                def blk(R, C):
                    v = wide[(R, C)].astype(f32)[:, n * 128:(n + 1) * 128]
                    s = D2[R // 2] / D2[C // 2]
                    return v if s == 1.0 else v * s
                B = {(R, C): blk(R, C) for R in range(4) for C in range(4)}
                O = {(i, j): b_ops(B[(i, j)], B[(i, 2 + j)], B[(2 + i, j)], B[(2 + i, 2 + j)])
                     for i in range(2) for j in range(2)}
                for p in PREP_ORDER:
                    anchor = next(anchors)
                    def sc(i, j):
                        s = D2[i] / D2[j] * BF[p] * 0.5 * D3[k] / D3[n] * (0.5 if cfg['FOLD'] and p in SEL else 1.0)
                        return O[(i, j)][p] * (s if anchor is None else const_after(anchor, s, 2))
                    T = b_ops(sc(0, 0), sc(0, 1), sc(1, 0), sc(1, 1))
                    for q in range(1, 8):
                        if q in q3of(p):
                            if cfg['STAGE']:
                                u = ((T3OFF[p] + Q6.index(q)) * 4 + k * 2 + n) * 16
                                kb[par][zero, u:u + 16, :] = T[q]
                            else:
                                keep[(p, q, k, n)] = T[q]
                        else:
                            sq = BF[q] * 2.0 * (2.0 if cfg['FOLD'] and p in SEL else 1.0)
                            v = T[q] if sq == 1.0 else T[q] * sq
                            t_ref[l, TIDX[(p, q)], n, pl.ds(k * 128 + r, 16), :] = v.astype(bf16)
        for p in SEL:
            for q in q3of(p):
                if cfg['STAGE']:
                    u = (T3OFF[p] + Q6.index(q)) * 64
                    kv = [kb[par][0, u + 16 * e:u + 16 * e + 16, :] for e in range(4)]
                else:
                    kv = [keep[(p, q, k, n)] for k in range(2) for n in range(2)]
                anchor = next(anchors)
                if cfg['FOLD']:
                    b = jax.lax.bitcast_convert_type(kv[1], i32) | jnp.tile(anchor, (2, 1))
                    kv[1] = jax.lax.bitcast_convert_type(b, f32)
                else:
                    kv = [v * const_after(anchor, 0.5, 2) for v in kv]
                T = b_ops(*kv)
                T[1] = T[1] + T[1]
                for u in range(1, 8):
                    t3_ref[l, (T3OFF[p] + Q6.index(q)) * 7 + u - 1, pl.ds(r, 16), :] = T[u].astype(bf16)

    outs = [(l, p) for l in range(L) for p in OUTER]
    G = len(outs)
    sched, start, wts = [], [], []
    for g in range(G):
        start.append(len(wts))
        for rd in rounds_of(outs[g][1], SEL, SEL3):
            n = NC // 2 if isinstance(rd[1], str) else NC
            sched.append((g, rd, len(wts), n))
            wts += [round_usage(OACT[outs[g][1]], rd, outs[g][0] == 0, outs[g][0] == L - 1)] * n
    start.append(len(wts))
    T = start[G]
    jobs = []
    conv_end = start[G - 7 + cfg['CE']]
    st_ = lambda g: start[g] if g >= 0 else start[g + G] - T
    cost = lambda alu, st, ld: cfg['CA'] * alu / 64 + cfg['CS_'] * st / 16 + cfg['CL'] * ld / 48
    for g in range(G):
        l2, p2 = outs[g]
        top_only = all(I == 0 for (I, J), _ in LA[p2])
        ready = 7 * (g // 7) - (2 if top_only else 0)
        lo = max(st_(ready), conv_end - T)
        hi = max(start[g] - LAG - 3 - cfg['HI'], lo)
        nt = len(LA[p2])
        pr = [ps for ps in PAIR if p2 in ps and ps in cfg['OPAIR']]
        a = []
        if p2 in SEL3:
            assert not pr
            hy = hi
            if SEL3.index(p2) % 2:
                host = 7 * (g // 7) + OUTER.index(SEL3[SEL3.index(p2) - 1])
                hy = max([t0 for gg, rd, t0, _ in sched if gg == host and rd[0] == 'y'][0] - LAG - 3 - cfg['HI'], lo)
            sv = 32 * sum(gg == g for gg in cfg['XC'])
            a = [(lo, hy, cost(32 * nt + 50 + sv, 21 + sv, 32 * nt), cfg['NS26'], l2, a_chunk3(g, l2, p2, (2, 6), c)) for c in range(NC // 2)]
        elif not pr or outs[g + 1 if g + 1 < G else 0][1] in pr[0]:
            ps = pr[0] if pr else (p2,)
            gs = (g, g + 1) if pr else (g,)
            sv = 8 * sum(gg in gs for gg in cfg['XC'])
            nq = sum(3 if p in SEL else 7 for p in ps)
            alu = (8 * nt if pr else 8 * (nt - 1)) + sum(8 if p in SEL else 16 for p in ps) + nq
            ns = cfg['NST'][0] if nq <= 3 else cfg['NST'][1] if nq <= 7 else cfg['NST'][2]
            a = [(lo, hi, cost(alu + sv, nq + ns + sv, 8 * nt), ns, l2, a_chunk(gs, l2, ps, c, k))
                 for c in range(NC) for k in range(NT)]
        if p2 in SEL:
            hi3 = hi + (NC if g else 0)
            b = [(lo, hi3, cost(16 * nt + 46, 17, 16 * nt), 3, l2, a_chunk3(g, l2, p2, qs, c))
                 for c in range(NC // 2) for qs in ((5, 3), (4, 7))]
            a += b
        jobs += a
    for R in range(4):
        hi = conv_end - 2
        jobs += [(start[6], hi, cost(18, 8, 4), 'conv', 0, (R, C, c)) for C in range(4) for c in range(0, NC, 2)]
    use = [max(cfg['UA'] * a / 32, st / 8, cfg['UL'] * ld / 24) for a, st, ld in wts]
    cap = [max(cfg['CAP'] - max(use[t], use[(t + 1) % T]), 0.0) ** cfg['GAM'] for t in range(T)]
    for t in range(T - cfg['TAIL'], T):
        cap[t] = 0.0
    cap3 = cap * 3
    all3 = [(lo + k * T, hi + k * T, w, ji, k) for k in range(3) for ji, (lo, hi, w, _, _, _) in enumerate(jobs)
            if lo + k * T >= 0]
    grp = {}
    for lo, hi, w, _, _ in all3:
        grp[(lo, hi)] = grp.get((lo, hi), 0.0) + w
    speed, cls, gcls = yds([(lo, hi, w) for (lo, hi), w in grp.items()], cap3)
    when = [[] for _ in jobs]
    pend = {}
    for j in sorted(all3, key=lambda j: (j[1], j[4], j[3])):
        pend.setdefault(j[:2], []).append(j)
    debt = 0.0
    cur, left = None, 0
    FR = {1: (1.0,), 2: cfg['FR2'], 3: cfg['FR3'], 4: cfg['FR4']}
    for t in range(3 * T):
        while True:
            if cur is None:
                rdy = [q[0] for w, q in pend.items() if q and w[0] <= t and (gcls[w] == cls[t] or w[1] <= t)]
                if not rdy:
                    debt = max(debt, 0.0)
                    break
                j = rdy[0]
                nst = 1 if jobs[j[3]][3] == 'conv' else jobs[j[3]][3]
                if nst > 1 and j[1] > t and (t + cfg['TAIL'] + 2 * nst) // T != t // T:
                    break
            else:
                j = cur
            must = j[1] <= t or (cur is not None and (t + cfg['TAIL'] + 1) // T != t // T)
            if not must and (cap3[t] == 0.0 or debt > 0.5 * speed[t] * cap3[t]):
                break
            if cur is None:
                pend[j[:2]].pop(0)
                cur, left = j, nst
            debt += j[2] * FR[nst][nst - left]
            if j[4] == 1:
                when[j[3]].append(t - T)
            left -= 1
            if left == 0:
                cur = None
        debt -= speed[t] * cap3[t]
    if cfg.get('SHOW'):
        for g in range(G):
            print(g, 'speed %.2f' % speed[T + start[g] + 5])
            print('  ', ''.join('%2d' % round(10 * use[t]) for t in range(start[g], start[g + 1])))
            print('  ', ''.join('%2s' % ''.join((str(j[3])[0] if u == 0 else '.') for j, w in zip(jobs, when) for u, x in enumerate(w) if x % T == t) for t in range(start[g], start[g + 1])))
    plan_events = {}
    carried = []
    for ts, (lo, hi, sh, kind, l2, job) in sorted(zip(when, jobs), key=lambda e: e[0][0] % T):
        assert (ts[0] < 0) == (ts[-1] < 0)
        if ts[0] < 0:
            carried.append(job)
        for t, group in zip(ts, [None] if kind == 'conv' else STAGES[kind]):
            plan_events.setdefault(t % T, []).append((kind, l2, job, id(job), group))

    def w_copy(l):
        return pltpu.make_async_copy(w_hbm.at[l], w_ref.at[l], sem.at[l])

    def in_copy(t, slot):
        return pltpu.make_async_copy(x_hbm.at[pl.ds(pl.multiple_of(t * TM, 32), TM)], xn2_ref.at[slot], sem.at[L + slot])

    def out_copy(t, slot, h):
        hm = TM // 2
        return pltpu.make_async_copy(o2_ref.at[slot, pl.ds(h * hm, hm)],
                                     o_hbm.at[pl.ds(pl.multiple_of(t * TM + h * hm, 32), hm)],
                                     sem.at[L + 4 + 2 * slot + h])

    xr_in = pltpu.make_async_copy(x_hbm.at[pl.ds(NMAIN * TM, R0)], xr_ref, sem.at[L + 2])
    xr_out = pltpu.make_async_copy(xr_ref, o_hbm.at[pl.ds(NMAIN * TM, R0)], sem.at[L + 2])
    b_in = pltpu.make_async_copy(b_hbm, b_ref, sem.at[L + 3])

    def prologue():
        b_in.start()
        xr_in.start()
        for l in range(L):
            w_copy(l).start()
        in_copy(0, 0).start()
        in_copy(min(1, NMAIN - 1), 1).start()
        b_in.wait()
        for l in range(L):
            bf_ref[l] = b_ref[l:l + 1, :].astype(f32)
        xr_in.wait()
        xp_ref[0] = xr_ref[...].astype(f32)
        xp_ref[1] = xr_ref[...].astype(f32)
        NSUB = cfg['NSUB']
        RB = R0 // NSUB
        PR = 128 // NSUB
        def sub(it, c):
            l = it // NSUB
            j = it % NSUB
            @pl.when(j == 0)
            def _():
                w_copy(l).wait()
            zero = jax.lax.shift_right_logical(it, 12)
            rows = pl.ds(pl.multiple_of(j * RB, RB), RB)
            x = xp_ref[0, rows, :]
            xbf = x.astype(bf16)
            KH = D // 2
            passes, ys = [], []
            for jt in range(D // 128):
                cols = slice(jt * 128, (jt + 1) * 128)
                ya = _dot(xbf[:, :KH], w_ref[l, 0:KH, cols]) + bf_ref[l, :, cols]
                yb = _dot(xbf[:, KH:], w_ref[l, KH:D, cols]) + ya
                passes += [ya, yb]
                ys.append(yb)
            xp_ref[0, rows, :] = xp_ref[1, rows, :] * jnp.concatenate(ys, axis=1) + x
            na = (PR // 16) * (NT * NT * 7 + 4 * len(SEL) + 2 * len(SEL3))
            def gen():
                tot = len(passes) * (RB // 8)
                for u in range(na):
                    if u < cfg['AFREE']:
                        yield None
                        continue
                    f = int((u - cfg['AFREE']) * cfg['ANC'] * tot / (na - cfg['AFREE']))
                    ps, rr = divmod(f, RB // 8)
                    yield jax.lax.bitcast_convert_type(passes[ps][rr * 8:rr * 8 + 8, :], i32) & zero
            anchors = gen()
            for u in range(PR // 16):
                prep(l, pl.multiple_of(j * PR + u * 16, 16), anchors, zero, u % 2)
            return c
        jax.lax.fori_loop(0, L * NSUB, sub, 0)
        xr_ref[...] = xp_ref[0].astype(bf16)
        xr_out.start()
        in_copy(0, 0).wait()
        for R in range(4):
            for C in range(4):
                for h in range(2):
                    conv(xn2_ref.at[0], 0, R, C, h * Mq, Mq)
        for job in carried:
            job({}, STAGES[1][0], 0, 0, None)

    def main(tile, carry):
        zs, za = jax.lax.shift_right_logical(tile, 12), jax.lax.shift_right_logical(tile, 13)
        slot = tile % 2
        in_copy(jnp.minimum(tile + 2, NMAIN - 1), slot).start()
        in_copy(0, 1 - slot).wait()
        @pl.when(tile > 1)
        def _():
            out_copy(0, slot, 0).wait()
            out_copy(0, slot, 1).wait()
        xn_ref = xn2_ref.at[1 - slot]
        o_ref = o2_ref.at[slot]

        def rows(h):
            return (0, Mh) if h is None else (h * Mq, Mq)

        def ld(loc, h=None):
            r0, nr = rows(h)
            return loc[0][0, loc[1] + r0:loc[1] + r0 + nr, :]

        def st(loc, v, h=None):
            r0, nr = rows(h)
            loc[0][zs, loc[1] + r0:loc[1] + r0 + nr, :] = v

        def by_half(v, h, fn):
            if h is not None:
                return fn(v, h)
            if not SEL:
                return fn(v, 0)
            return jnp.concatenate([fn(v[:Mq], 0), fn(v[Mq:], 1)], axis=0)

        def gather(ref, idx, slot_):
            if cfg['NOBC']:
                v = ref[idx + (slice(None), slice(slot_ * 16, slot_ * 16 + 16), slice(None))]
                return v.reshape(v.shape[0] * 16, 128)
            v = ref.bitcast(u32)[idx + (slice(None), slice(slot_ * 8, slot_ * 8 + 8), slice(None))]
            return v.reshape(v.shape[0] * 8, 128)

        def as_bf16(v):
            return v if cfg['NOBC'] else pltpu.bitcast(v, bf16)

        def lhs_load(p, q):
            return as_bf16(jnp.concatenate([gather(sb[p - 1], (0, k), SPOS[q] + k) for k in range(NT)], axis=1))

        def wload(l, p, q, n):
            return as_bf16((t_ref if cfg['NOBC'] else t_ref.bitcast(u32))[l, TIDX[(p, q)], n])

        def tile_dot(l, p, q, r):
            u = Q6.index(q)
            lhs = as_bf16(gather(s3b[SEL.index(p)], (0, u), SPOS[r] + u % 2))
            w = as_bf16((t3_ref if cfg['NOBC'] else t3_ref.bitcast(u32))[l, (T3OFF[p] + u) * 7 + r - 1])
            return _dot(lhs, w)

        def bias(l, terms, where):
            coef = {}
            for sg, i, j, n, h in where:
                for cf, (I, J) in terms:
                    R, C = 2 * I + i, 2 * J + j
                    coef[(C, n)] = coef.get((C, n), 0.0) + sg * cf * scale(R, C, h, n)
            acc = None
            for (C, n), cf in sorted(coef.items()):
                if cf == 0.0:
                    continue
                bv = bf_ref[l, :, C * H + n * 128:C * H + (n + 1) * 128]
                if l == 0:
                    bv = bv + 1.0
                bv = bv if cf == 1.0 else bv * cf
                acc = bv if acc is None else acc + bv
            return acc

        def add_bias(v, l, terms, where, h):
            if h is not None:
                return v + bias(l, terms, where(h))
            bv = bias(l, terms, where(0))
            return by_half(v, h, lambda x, hh: x + (bv if D3[hh] == 1.0 else bv * D3[hh]))

        def outer_act(l, p, i, j, n, d, h=None):
            bt, stores, finals = OACT[p]
            if bt:
                def where(hh):
                    w = [(1, i, j)]
                    if raw_slot(OACT[p]) and (i, j) == (1, 0):
                        w.append((-1, 0, 1))
                    res_ = [x + (n, hh) for x in w]
                    if raw_slot(OACT[p]) and (h, n) == (1, 0):
                        res_ += [(-sg, ii, jj, 1, 0) for sg, ii, jj in w]
                    return res_
                d = add_bias(d, l, bt, where, h)
            cache = {'d': d}
            def comb(terms):
                for _, src in terms:
                    if isinstance(src, str) and src not in cache:
                        cache[src] = ld(oloc(src, i, j, n), h)
                v = lincomb([(s, cache[src]) for s, src in terms if isinstance(src, str)])
                for _, src in terms:
                    if not isinstance(src, str):
                        v = add_bias(v, l, src, lambda hh: [(1, i, j, n, hh)], h)
                return v
            fin = [(IJ, comb(terms)) for IJ, terms in finals]
            stl = [(name, comb(terms)) for name, terms in stores]
            for name, v in stl:
                st(oloc(name, i, j, n), v, h)
            for (I, J), y in fin:
                R, C = 2 * I + i, 2 * J + j
                xn = ld(x0loc(R, C, n), h) * y
                if l > 0:
                    xn = xn + ld(xloc(l, R, C, n), h)
                if l == L - 1:
                    xn = by_half(xn, h, lambda x, hh: x if scale(R, C, hh, n) == 1.0 else x * (1.0 / scale(R, C, hh, n)))
                    r0, nr = rows(h)
                    o_ref[R * Mh + r0:R * Mh + r0 + nr, C * H + n * 128:C * H + (n + 1) * 128] = xn.astype(o_ref.dtype)
                else:
                    st(xloc(l + 1, R, C, n), xn, h)

        def issue(g, l, p, rd):
            kind, n = rd
            if kind == 'y':
                return tuple(tile_dot(l, pp, q, 1) for pp in (p, SEL3[SEL3.index(p) + 1]) for q in (2, 6))
            if n == '1':
                return tuple(tile_dot(l, p, q, 1) for q in Q3)
            if isinstance(n, str):
                return tuple(tile_dot(l, p, int(q), int(r)) for r in n for q in kind)
            if kind == '1':
                lhs = lhs_load(p, 1)
                return (_dot(lhs, wload(l, p, 1, 0)), _dot(lhs, wload(l, p, 1, 1)))
            qa, qb = int(kind[0]), int(kind[1])
            return (_dot(lhs_load(p, qa), wload(l, p, qa, n)), _dot(lhs_load(p, qb), wload(l, p, qb, n)))

        def inner_act(g, l, p, kind, n, h, P, Q):
            rs = raw_slot(OACT[p])
            if kind == '35':
                st(iloc(g, 's', n), Q + ld(iloc(g, 'm1', n), h), h)
                if not rs:
                    st(iloc(g, 'v', n), P, h)
                outer_act(l, p, 0, 1, n, P, h)
            elif kind == '47':
                st(iloc(g, 'u', n), Q + ld(oloc(rs, 0, 1, n) if rs else iloc(g, 'v', n), h), h)
                outer_act(l, p, 0, 0, n, P + ld(iloc(g, 's', n), h), h)
            else:
                outer_act(l, p, 1, 1, n, ld(iloc(g, 's', n), h) - Q, h)
                outer_act(l, p, 1, 0, n, P + ld(iloc(g, 'u', n), h), h)

        def consume(g, l, p, rd, res):
            kind, n = rd
            if kind == 'y':
                for sec, a, b in ((False, res[0], res[1]), (True, res[2], res[3])):
                    st(jloc('26', '1', 0, sec), a + b, 0)
                    st(jloc('26', '1', 1, sec), a - b, 0)
            elif n == '1':
                for qp, a, b in (('35', res[0], res[1]), ('47', res[2], res[3])):
                    st(jloc(qp, '1', 0), a + b, 0)
                    st(jloc(qp, '1', 1), a - b, 0)
            elif isinstance(n, str):
                x, z, y, w = res
                aa, bb = (x + z, x - z), (y + w, y - w)
                sm = [aa[al] + bb[al] for al in range(2)]
                df = [aa[al] - bb[al] for al in range(2)]
                sec = kind == '26' and SEL3.index(p) % 2 == 1
                J = lambda name, al: ld(jloc(kind, name, al, sec and name == '1'), 0)
                if n == '35':
                    for al in range(2):
                        st(jloc(kind, 's', al), df[al] + J('1', al), 0)
                    if kind == '47' and not raw_slot(OACT[p]):
                        st(jloc(kind, 'v', 0), sm[0], 0)
                    inner_act(g, l, p, kind, 1, 0, sm[0], sm[1])
                elif n == '47':
                    rs = raw_slot(OACT[p])
                    vin = oloc(rs, 0, 1, 1) if rs else iloc(g, 'v', 1)
                    if kind == '26':
                        v = [[(1, oloc(rs, 1, 0, 1)), (-1, iloc(g, 'u', 1))], [(1, iloc(g, 's', 1)), (-1, oloc(rs, 1, 1, 1))]]
                    elif kind == '35':
                        v = [[(1, vin)], [(1, iloc(g, 's', 1)), (-1, iloc(g, 'm1', 1))]]
                    else:
                        v = [[(1, oloc(rs, 0, 0, 1)), (-1, iloc(g, 's', 1))] if rs else [(1, jloc(kind, 'v', 0))],
                             [(1, iloc(g, 'u', 1)), (-1, vin)]]
                    for al in range(2):
                        st(jloc(kind, 'u', al), lincomb([(1, df[al])] + [(s, ld(loc, 0)) for s, loc in v[al]]), 0)
                    inner_act(g, l, p, kind, 0, 0, sm[0] + J('s', 0), sm[1] + J('s', 1))
                else:
                    inner_act(g, l, p, kind, 1, 1, J('s', 0) - df[0], J('s', 1) - df[1])
                    inner_act(g, l, p, kind, 0, 1, sm[0] + J('u', 0), sm[1] + J('u', 1))
            elif kind == '1':
                st(iloc(g, 'm1', 0), res[0])
                st(iloc(g, 'm1', 1), res[1])
            else:
                inner_act(g, l, p, kind, n, None, res[0] + res[1], res[0] - res[1])

        events = {t: list(v) for t, v in plan_events.items()}
        state = {}
        for g, rd, t0, n in sched:
            l, p = outs[g]
            if g == G - 1 and t0 == start[g]:
                out_copy(tile, slot, 0).start()
            res = issue(g, l, p, rd)
            for t in range(t0, t0 + n):
                nev, nth = len(events.get(t, [])), 0
                for kind, l2, job, key, stage in events.pop(t, []):
                    gr = 16 * (t - t0)
                    mini = isinstance(rd[1], str)
                    ph = cfg['GPHM'] if mini else cfg['GPH']
                    if cfg['DBL'] and nth == 0 and nev > 1:
                        ph = 0
                    nth += 1
                    gate = res[cfg['GSRCM'] if mini else cfg['GSRC']][gr + ph:gr + ph + 8, :]
                    if mini and cfg['GADD']:
                        gate = gate + res[1][gr + ph:gr + ph + 8, :]
                    anchor = jax.lax.bitcast_convert_type(gate, i32) & zs
                    if kind != 'conv':
                        xb[xset(l2)][0, GROW:GROW + 8, :] = gate
                        job(state.setdefault(key, {}), stage, zs, za, anchor)
                    else:
                        R, C, c = job
                        for cc in range(c, min(c + 2, NC)):
                            conv(xn_ref, zs, R, C, 16 * cc, 16, anchor)
            consume(g, l, p, rd, res)
        assert not events
        out_copy(tile, slot, 1).start()
        return carry

    prologue()
    jax.lax.fori_loop(0, NMAIN, main, 0)
    xr_out.wait()
    in_copy(0, (NMAIN - 1) % 2).wait()
    for t in range(max(NMAIN - 2, 0), NMAIN):
        out_copy(0, t % 2, 0).wait()
        out_copy(0, t % 2, 1).wait()


DEFAULT = dict(UNIT=60, LO=0, HI=0, NSUB=1, ANC=1.0, AFREE=4, DBC=True, NOBC=0, OA='raw5', VW=3, CS=(0, 2, 3, 5), XC=(1, 2, 4, 6),
               SEL=(3, 5, 4, 7), AHEAD=7, CE=5, TAIL=6, SEL3=(3, 4), NS26=4, FR4=(.16, .26, .31, .27), FOLD=0, STAGE=1, GPH=8, GSRC=0, GPHM=8, GSRCM=0, GADD=1, DBL=1, CA=1.0, CS_=0.5, CL=0.3, UA=1.0, UL=0.8, CAP=0.85, OPAIR=((2, 6),), FR2=(.4, .6), FR3=(.35, .37, .28), NST=(1, 2, 3), GAM=1.0, MIX=0, SPLIT=('big4', 'big'), SGAP=1, F4=1.0, BIG=(1, 1, .4), SMALL=(.5, .2), CONVW=(.6, .2))


def build(TM=512, **kw):
    def f(x0, ws, bs):
        B, D = x0.shape
        L = ws.shape[0]
        H = D // 4
        Mh = TM // 4
        nmain = (B - 1) // TM
        R0 = B - nmain * TM
        cfg = dict(DEFAULT, **kw)
        MP = cfg['MP'] = (Mh + 24 + 31) // 32 * 32
        half = pltpu.VMEM((1, MP, 128), f32)
        xhalf = pltpu.VMEM((1, 16 * MP + 32, 128), f32)
        sop = pltpu.VMEM((1, H // 128, Mh // 16, 128, 128), bf16)
        s3op = pltpu.VMEM((1, 6, max(Mh // 32, 1), 128, 128), bf16)
        t3sh = pltpu.VMEM((L, max(len(cfg['SEL']), 1) * 28 + len(cfg['SEL3']) * 14, 128, 128), bf16)
        tsh = pltpu.VMEM((L, 49 - 4 * len(cfg['SEL']) - 2 * len(cfg['SEL3']), H // 128, H, 128), bf16)
        anyspec = pl.BlockSpec(memory_space=pl.ANY)
        return pl.pallas_call(
            functools.partial(_kernel, L=L, TM=TM, R0=R0, NMAIN=nmain, D=D, cfg=cfg),
            in_specs=[anyspec, anyspec, anyspec],
            out_specs=anyspec,
            out_shape=jax.ShapeDtypeStruct((B, D), x0.dtype),
            scratch_shapes=[half] * NX0 + [xhalf] * NX + [half] * (NI + NO + N3) + [sop] * NS + [s3op] * len(cfg['SEL'])
                           + [pltpu.VMEM((8, 1, D), f32), pltpu.VMEM((2, TM, D), bf16), pltpu.VMEM((2, TM, D), bf16), tsh, t3sh,
                              pltpu.VMEM((L, D, D), bf16), pltpu.VMEM((R0, D), bf16), pltpu.VMEM((2, R0, D), f32),
                              pltpu.VMEM((L, D), bf16), pltpu.SemaphoreType.DMA((L + 8,))],
            compiler_params=pltpu.CompilerParams(
                vmem_limit_bytes=110 * 1024 * 1024,
                internal_scratch_in_bytes=65536,
                disable_bounds_checks=cfg['DBC'],
            ),
        )(x0, ws, bs)
    return f


@jax.jit
def pallas_standalone__dcn_v2_cross__recsys_kernel(x0, ws, bs):
    return build(TM=640)(x0, ws, bs)
```

```python
import functools

import jax
import jax.numpy as jnp
import jax.experimental.pallas as pl
import jax.experimental.pallas.tpu as pltpu

f32 = jnp.float32
bf16 = jnp.bfloat16
u32 = jnp.uint32

B11, B12, B21, B22 = (0, 0), (0, 1), (1, 0), (1, 1)
LA = {1: [(B11, 1), (B22, 1)], 2: [(B11, 1), (B12, 1), (B21, 1), (B22, 1)], 3: [(B11, 1), (B12, -1)],
      4: [(B12, 1), (B22, 1)], 5: [(B11, 1), (B12, 1)], 6: [(B12, 1), (B11, -1), (B21, 1), (B22, -1)],
      7: [(B12, 1), (B22, -1)]}
PAIRS = ((5, 3), (4, 7), (2, 6))
ORD = (3, 5, 4, 7, 1, 2, 6)
D2 = (1.0, 2.0)
BF = {1: 1.0, 2: 0.5, 3: 0.5, 4: 0.5, 5: 0.5, 6: 0.5, 7: 0.5}
OUTER = (3, 5, 1, 4, 7, 2, 6)
OACT = {
    3: ([(1, B12)], [('M3', [(1, 'd')])], []),
    5: ([], [('M5', [(1, 'd')])], [(B12, [(1, 'd'), (1, 'M3')])]),
    1: ([(1, B11), (-1, B12)], [('S', [(1, 'd'), (1, 'M3'), (-1, 'M5')])], []),
    4: ([], [('M4', [(1, 'd')])], []),
    7: ([], [('M7', [(1, 'd')])], [(B11, [(1, 'd'), (1, 'S'), (1, 'M4')])]),
    2: ([(1, B11), (-1, B22)], [('M2', [(1, 'd')]),
        ('U', [(1, 'd'), (1, 'M4'), (-1, 'M7'), (1, 'M3'), (1, 'M5'), (1, ((1, B21), (-1, B12), (-1, B11), (1, B22)))])], []),
    6: ([], [], [(B22, [(1, 'd'), (1, 'S'), (-1, 'M2')]), (B21, [(1, 'd'), (1, 'U')])]),
}
OSL = {'M3': 0, 'M5': 1, 'S': 2, 'M4': 3, 'M7': 4, 'M2': 6, 'U': 5}
ISL = {'m1': 0, 's': 1, 'v': 2, 'u': 3}
STAGES = {1: [(B11, B12, B21, B22)], 2: [(B11, B12), (B21, B22)], 3: [(B11, B12), (B22,), (B21,)],
          4: [(B11,), (B12,), (B22,), (B21,)]}
PREP_ORDER = (2, 6, 3, 5, 1, 4, 7)
LAG = 8


def _dot(a, b):
    return jnp.dot(a, b, preferred_element_type=f32)


def scale(R, C, h, k):
    return D2[R // 2] * D2[R % 2] * D2[h] / (D2[C // 2] * D2[C % 2] * D2[k])


def b_ops(b11, b12, b21, b22):
    r1 = b11 + b22
    g = b12 + b21
    return {1: r1, 2: b11 - b12, 3: b12 - b22, 4: g - r1, 5: b12 + b22, 6: b11 + b12, 7: g + r1}


def lincomb(terms):
    assert terms[0][0] == 1
    acc = terms[0][1]
    for s, v in terms[1:]:
        acc = acc + v if s == 1 else acc - v
    return acc


def raw_slot(p):
    return next((name for name, terms in OACT[p][1] if terms == [(1, 'd')]), None)


def round_usage(p, rd, first, last):
    bt, stores, finals = OACT[p]
    alu = bool(bt) + sum(len(t) - 1 for _, t in stores) + sum(len(t) + (not first) + 2 * last for _, t in finals)
    nst = len(stores) + len(finals)
    nld = len({x for _, t in stores + finals for _, x in t if isinstance(x, str) and x != 'd'}) + len(finals) * (2 - first)
    kind, n = rd
    if isinstance(n, str):
        e = kind == '47'
        if kind == '26':
            a, st, ld, m = {'35': (12, 2, 9, 2), '47': (18, 2, 13, 2), '26': (16, 0, 13, 4)}[n]
        else:
            a, st, ld, m = {'1': (4, 4, 5, 0), '35': (11 + e, 3, 8 + e, 1), '47': (14 + 2 * e, 3, 11 + 2 * e, 1),
                            '26': (14 + 2 * e, 2, 11 + 2 * e, 2)}[n]
    else:
        a, st, ld, m = {'1': (2, 2, 4, 0), '35': (5, 2 - bool(raw_slot(p)), 5, 1), '47': (6, 1, 6, 1),
                        '26': (6, 0, 6, 2)}[kind]
    return a + m * alu, st + m * nst, ld + m * nld


def yds(groups, cap):
    n = len(cap)
    speed, cls, gcls = [0.0] * n, [-1] * n, {}
    todo = list(groups)
    while todo:
        pre = [0.0]
        for t in range(n):
            pre.append(pre[-1] + (cap[t] if cls[t] < 0 else 0.0))
        best = None
        for a in sorted({g[0] for g in todo}):
            w = 0.0
            for g in sorted((g for g in todo if g[0] >= a), key=lambda g: g[1]):
                w += g[2]
                d = w / max(pre[g[1] + 1] - pre[a], 1e-9)
                if best is None or d > best[0]:
                    best = (d, a, g[1])
        d, a, b = best
        for t in range(a, b + 1):
            if cls[t] < 0:
                speed[t], cls[t] = d, len(gcls)
        gcls.update({g[:2]: len(gcls) for g in todo if g[0] >= a and g[1] <= b})
        todo = [g for g in todo if not (g[0] >= a and g[1] <= b)]
    return speed, cls, gcls


def spread_jobs(jobs, cap, tail):
    T = len(cap)
    cap3 = cap * 3
    all3 = [(lo + k * T, hi + k * T, ji, k) for k in range(3) for ji, (lo, hi, _) in enumerate(jobs) if lo + k * T >= 0]
    pend = {}
    for j in sorted(all3, key=lambda j: (j[1], j[3], j[2])):
        pend.setdefault(j[:2], []).append(j)
    speed, cls, gcls = yds([w + (sum(sum(jobs[j[2]][2]) for j in q),) for w, q in pend.items()], cap3)
    when = [[] for _ in jobs]
    debt, cur, done = 0.0, None, 0
    for t in range(3 * T):
        while True:
            j = cur
            if j is None:
                rdy = [q[0] for w, q in pend.items() if q and w[0] <= t and (gcls[w] == cls[t] or w[1] <= t)]
                if not rdy:
                    debt = max(debt, 0.0)
                    break
                j = rdy[0]
                nst = len(jobs[j[2]][2])
                if nst > 1 and j[1] > t and (t + tail + 2 * nst) // T != t // T:
                    break
            must = j[1] <= t or (cur is not None and (t + tail + 1) // T != t // T)
            if not must and (cap3[t] == 0.0 or debt > 0.5 * speed[t] * cap3[t]):
                break
            if cur is None:
                pend[j[:2]].pop(0)
                cur, done = j, 0
            debt += jobs[j[2]][2][done]
            if j[3] == 1:
                when[j[2]].append(t - T)
            done += 1
            if done == len(jobs[j[2]][2]):
                cur = None
        debt -= speed[t] * cap3[t]
    return when


def layout(cfg):
    sel, sel3 = cfg['SEL'], cfg['SEL3']
    pairs3 = {p: [qs for qs in PAIRS if p in sel3 or (p in sel and qs != (2, 6))] for p in range(1, 8)}
    q2 = {p: [q for q in ORD if not any(q in qs for qs in pairs3[p])] for p in range(1, 8)}
    return pairs3, q2


def _kernel(x_hbm, w_hbm, b_hbm, o_hbm, *scratch, L, TM, R0, NMAIN, D, cfg):
    H, Mh, Mq = D // 4, TM // 4, TM // 8
    NC, NQ = Mh // 16, Mq // 16
    MP = Mh + 32
    SEL, SEL3 = cfg['SEL'], cfg['SEL3']
    pairs3, q2 = layout(cfg)
    prods3 = [(p, q) for p in SEL for qs in pairs3[p] for q in qs]
    assert H == 256 and L % 2 == 0 and Mq % 16 == 0 and all(raw_slot(p) for p in SEL)
    it = iter(scratch)
    take = lambda n: [next(it) for _ in range(n)]
    x0b, xb, ib, ob, jb = take(4), take(6), take(16), take(56), take(20)
    s2 = dict(zip((1, 3, 4, 5, 7, 2), take(6)))
    s3 = {(p, qs): next(it) for p in SEL for qs in pairs3[p]}
    t2 = dict(zip(range(1, 8), take(7)))
    t3_ref, kb0, kb1, bf_ref, xn2_ref, o2_ref, w_ref, xr_ref, xp_ref, b_ref, sem = it

    xset = lambda l: 4 if l == 0 else (l % 2) * 2
    xoff = lambda I, J: 16 * ((I + J) % 2)
    xloc = lambda l, R, C, k: (xb[xset(l) + R // 2], (R % 2, C, k), xoff(R // 2, C // 2))
    x0loc = lambda R, C, k: (x0b[(R // 2) * 2 + C // 2], (R % 2, C % 2, k), 8 + xoff(R // 2, C // 2))
    iloc = lambda g, name, n: (ib[((g % 2) * 4 + ISL[name]) * 2 + n], (), 8 * ISL[name])
    oloc = lambda name, i, j, n: (ob[(OSL[name] * 4 + i * 2 + j) * 2 + n], (), 8 * ((OSL[name] + 2 * j) % 4))

    def jloc(kind, name, al, second=False):
        i = 18 + al if second else (('35', '47', '26').index(kind) * 3 + ('1', 's', 'u').index(name)) * 2 + al
        return jb[i], (), 8 * ((i + i // 2) % 4)

    def s2loc(p):
        return (s2[2], (2, 6).index(p)) if p in (2, 6) else (s2[p], 0)

    def tie(v, anchor, r=0):
        if anchor is None:
            return v
        return jnp.concatenate([v[:r]] * (r > 0) + [jax.lax.select(anchor[0], anchor[1], v[r:r + 8])] + [v[r + 8:]] * (r + 8 < v.shape[0]), axis=0)

    def consts(anchor, ss, reps):
        one = {s: jnp.full((8, 128), s, f32) for s in set(ss)}
        if anchor is not None:
            one = {s: jax.lax.select(anchor[0], anchor[1], v) for s, v in one.items()}
        return jnp.concatenate([one[s] for s in ss for _ in range(reps)], axis=0)

    def conv(src, zs, R, C, r, nr, anchor=None):
        v = src[R * Mh + r:R * Mh + r + nr, C * H:(C + 1) * H].astype(f32)
        for k in range(2):
            buf, idx, off = xloc(0, R, C, k)
            sv = consts(anchor, [scale(R, C, (r + u) // Mq, k) for u in range(0, nr, 16)], 2)
            buf[(zs,) + idx + (slice(off + r, off + r + nr),)] = v[:, k * 128:(k + 1) * 128] * sv

    def block_sum(l, terms, ii, jj, kk, r, save, zs, za, anchor, at=None):
        rng = lambda t: slice(t[0], t[-1] + 1)
        vals = []
        for u, ((I, J), s) in enumerate(terms):
            r0 = xoff(I, J) + r
            v = xb[xset(l) + I][za if u == 0 else 0, rng(ii), slice(2 * J + jj[0], 2 * J + jj[-1] + 1), rng(kk), r0:r0 + 16, :]
            if (I, J) in save:
                sv = consts(anchor, [1.0 / scale(2 * I + i, 2 * J + j, r // Mq, k) for i in ii for j in jj for k in kk], 2)
                x0b[I * 2 + J][zs, rng(ii), rng(jj), rng(kk), r0 + 8:r0 + 24, :] = v * sv.reshape(v.shape)
            if u == 0 and at is not None and cfg['TIEL'] in (1, 2) and anchor is not None:
                v = tie(v.reshape(v.size // 128, 128), anchor, at + cfg['T8']).reshape(v.shape)
            vals.append((s, v))
        v = lincomb(vals)
        v = v.reshape(v.size // 128, 128)
        if cfg['TIEL'] == 3 and at is not None:
            v = tie(v, anchor, at)
        return v

    def finish(e, f, group, qs, store, st8, anchor):
        if not cfg['TIEL']:
            e = tie(e, anchor)
        a = e[None] if f is None else jnp.concatenate([e + f, e - f], axis=0).reshape(2, e.shape[0], 128)
        for u, b in enumerate(group):
            st8[b] = a if len(group) == 1 else a[:, 16 * u:16 * u + 16]
        ops = {}
        if B12 in group and 3 in qs:
            ops[3], ops[5] = st8[B11] - st8[B12], st8[B11] + st8[B12]
        if B22 in group:
            if 4 in qs:
                ops[4], ops[7] = st8[B12] + st8[B22], st8[B12] - st8[B22]
            ops[1] = st8['l1'] = st8[B11] + st8[B22]
        if B21 in group:
            g = st8[B12] + st8[B21]
            ops[2], ops[6] = g + st8['l1'], g - st8['l1']
        now = [q for q in qs if q in ops]
        if now:
            r0 = 16 * qs.index(now[0])
            store(slice(r0, r0 + 16 * len(now)), jnp.concatenate([ops[q] for q in now], axis=1).astype(bf16))

    def unit2(l, ps, c, k, save, st8, group, zs, za, anchor):
        ii, jj = sorted({b[0] for b in group}), sorted({b[1] for b in group})
        bs = lambda terms, at: block_sum(l, terms, ii, jj, [k], 16 * c, save, zs, za, anchor, at)
        at = 16 * (len(group) > 1)
        e, f = (bs(LA[ps[0]], at), None) if len(ps) == 1 else (bs([(B12, 1), (B21, 1)], at), bs([(B11, 1), (B22, 1)], None))
        def store(rows, v):
            s2[ps[0]][zs, :, k, c, rows, :] = v
        finish(e, f, group, q2[ps[0]], store, st8, anchor)

    def unit3(l, p, qs, c, save, st8, group, zs, za, anchor):
        for h in sorted({b[0] for b in group}):
            grp = tuple(b for b in group if b[0] == h)
            kk = [b[1] for b in grp]
            ii, jj = {(5, 3): ([0], [0, 1]), (4, 7): ([0, 1], [1]), (2, 6): ([0, 1], [0, 1])}[qs]
            v = block_sum(l, LA[p], ii, jj, sorted(kk), h * Mq + 16 * c, save, zs, za, anchor,
                          16 * (len(kk) > 1 or (qs == (2, 6) and not cfg['TF'])))
            n = 16 * len(kk)
            piece = lambda u: v[u * n:(u + 1) * n]
            if qs == (2, 6):
                e, f = piece(1) + piece(2), piece(0) + piece(3)
                r0 = 16 * q2[p].index(1)
                s2[p][zs, 0, min(kk):max(kk) + 1, h * NQ + c, r0:r0 + 16, :] = f.reshape(len(kk), 16, 128).astype(bf16)
            else:
                e, f = piece(0), piece(1)
            def store(rows, w):
                s3[(p, qs)][zs, :, c, rows, :] = w
            finish(e, f, tuple(sorted(grp)), ORD, store, st8, anchor)

    def prep(l, u, anchors, zero):
        kb = (kb0, kb1)[u % 2]
        for k in range(2):
            wide = [w_ref[l, R * H + k * 128 + 16 * u:R * H + k * 128 + 16 * u + 16, :].astype(f32) for R in range(4)]
            for n in range(2):
                def blk(R, C):
                    v = wide[R][:, C * H + n * 128:C * H + (n + 1) * 128]
                    s = D2[R // 2] / D2[C // 2]
                    return v if s == 1.0 else v * s
                O = {(i, j): b_ops(blk(i, j), blk(i, 2 + j), blk(2 + i, j), blk(2 + i, 2 + j)) for i, j in (B11, B12, B21, B22)}
                for p in PREP_ORDER:
                    anchor = next(anchors)
                    s = BF[p] * 0.5 * D2[k] / D2[n]
                    cs = {f: consts(anchor, [s * f], 2) for f in (0.5, 1.0, 2.0)}
                    T = b_ops(*[O[(i, j)][p] * cs[D2[i] / D2[j]] for i, j in (B11, B12, B21, B22)])
                    T[1] = T[1] + T[1]
                    t2[p][l, n, k * 8 + u] = jnp.concatenate([T[q] for q in q2[p]], axis=0).astype(bf16)
                    mine = [e for e, pq in enumerate(prods3) if pq[0] == p]
                    if mine:
                        kb[zero, k * 2 + n, 16 * mine[0]:16 * mine[-1] + 16, :] = jnp.concatenate(
                            [T[prods3[e][1]] for e in mine], axis=0)
        for e in range(len(prods3)):
            v = kb[0, :, 16 * e:16 * e + 16, :] * consts(next(anchors), [0.5], 2)
            T = b_ops(v[0], v[1], v[2], v[3])
            T[1] = T[1] + T[1]
            t3_ref[l, e, u] = jnp.concatenate([T[q] for q in ORD], axis=0).astype(bf16)

    def rounds_of(p):
        rs = [('1', None)] + [('x', '1')] * (p in SEL)
        for kind, qs in zip(('35', '47', '26'), PAIRS):
            if kind == '26' and p in SEL3[::2]:
                rs.append(('y', '1'))
            rs += [(kind, r) for r in (('35', '47', '26') if qs in pairs3[p] else (0, 1))]
        return rs

    outs = [(l, p) for l in range(L) for p in OUTER]
    G = len(outs)
    sched, start, use = [], [], []
    for g, (l, p) in enumerate(outs):
        start.append(len(use))
        for rd in rounds_of(p):
            n = NQ if isinstance(rd[1], str) else NC
            sched.append((g, rd, len(use), n))
            a, st_, ld_ = round_usage(p, rd, l == 0, l == L - 1)
            use += [max(a / 32, st_ / 8, cfg['UL'] * ld_ / 24)] * n
    T = len(use)
    cap = [max(cfg['CAP'] - max(use[t], use[(t + 1) % T]), 0.0) * (t < T - cfg['TAIL']) for t in range(T)]
    jobs = []
    def add(lo, hi, alu, st_, ld_, nst, l, fn):
        w = alu / 64 + cfg['CS'] * (st_ + nst) / 16 + cfg['CL'] * ld_ / 48
        jobs.append((lo, max(hi, lo), [w * f for f in cfg['FR'][nst - 1]], l, fn))
    for g, (l, p) in enumerate(outs):
        ready = 7 * l - 2 * all(I == 0 for (I, J), _ in LA[p])
        lo = start[ready] - (T if ready < 0 else 0)
        hi = start[g] - LAG - 3
        nt = len(LA[p])
        save = [b for b, pp in cfg['XC'].items() if pp == p and l == 0]
        if p in SEL3:
            if p in SEL3[1::2]:
                host = 7 * l + OUTER.index(SEL3[SEL3.index(p) - 1])
                hi = [t0 for gg, rd, t0, _ in sched if gg == host and rd[0] == 'y'][0] - LAG - 3
            for c in range(NQ):
                add(lo, hi, 32 * nt + 50 + 32 * len(save), 18 + 32 * len(save), 32 * nt, 4, l,
                    functools.partial(unit3, l, p, (2, 6), c, save))
        elif p != 6:
            ps = (2, 6) if p == 2 else (p,)
            nq = len(q2[p]) * len(ps)
            alu = 8 * (nt - 2 + len(ps)) + (8 if p in SEL else 16) * len(ps) + nq
            for c in range(NC):
                for k in range(2):
                    add(lo, hi, alu + 8 * len(save), nq + 8 * len(save), 8 * nt, 1 if nq <= 3 else 2 if nq <= 7 else 3, l,
                        functools.partial(unit2, l, ps, c, k, save))
        if p in SEL:
            for c in range(NQ):
                for qs in PAIRS[:2]:
                    add(lo, start[g] - LAG - 3 + (NC if g else 0), 16 * nt + 46, 14, 16 * nt, 3, l,
                        functools.partial(unit3, l, p, qs, c, []))
    for R in range(4):
        for C in range(4):
            for c in range(0, NC, 2):
                add(start[6], start[G - 2] - 2, 18, 7, 4, 1, None, (R, C, 16 * c))
    plan, carried = {}, []
    for ts, job in sorted(zip(spread_jobs([j[:3] for j in jobs], cap, cfg['TAIL']), jobs), key=lambda e: e[0][0] % T):
        assert (ts[0] < 0) == (ts[-1] < 0)
        if ts[0] < 0:
            carried.append(job[4])
        for t, group in zip(ts, STAGES[len(ts)]):
            plan.setdefault(t % T, []).append((job[3], job[4], group))

    def w_copy(l):
        return pltpu.make_async_copy(w_hbm.at[l], w_ref.at[l], sem.at[l])

    def in_copy(t, slot):
        return pltpu.make_async_copy(x_hbm.at[pl.ds(pl.multiple_of(t * TM, 32), TM)], xn2_ref.at[slot], sem.at[L + slot])

    def out_copy(t, slot, h):
        hm = TM // 2
        return pltpu.make_async_copy(o2_ref.at[slot, pl.ds(h * hm, hm)],
                                     o_hbm.at[pl.ds(pl.multiple_of(t * TM + h * hm, 32), hm)],
                                     sem.at[L + 4 + 2 * slot + h])

    xr_in = pltpu.make_async_copy(x_hbm.at[pl.ds(NMAIN * TM, R0)], xr_ref, sem.at[L + 2])
    xr_out = pltpu.make_async_copy(xr_ref, o_hbm.at[pl.ds(NMAIN * TM, R0)], sem.at[L + 2])
    b_in = pltpu.make_async_copy(b_hbm, b_ref, sem.at[L + 3])

    def prologue():
        b_in.start()
        xr_in.start()
        for l in range(L):
            w_copy(l).start()
        in_copy(0, 0).start()
        in_copy(min(1, NMAIN - 1), 1).start()
        b_in.wait()
        for l in range(L):
            bf_ref[l] = b_ref[l:l + 1, :].astype(f32)
        xr_in.wait()
        xp_ref[0] = xr_ref[...].astype(f32)
        xp_ref[1] = xr_ref[...].astype(f32)

        def layer(l, carry):
            w_copy(l).wait()
            zero = jax.lax.shift_right_logical(l, 12)
            never = jnp.broadcast_to(zero, (8, 128)) != 0
            x = xp_ref[0]
            xbf = x.astype(bf16)
            passes = []
            for jt in range(D // 128):
                cols = slice(jt * 128, (jt + 1) * 128)
                ya = _dot(xbf[:, :D // 2], w_ref[l, 0:D // 2, cols]) + bf_ref[l, :, cols]
                passes += [ya, _dot(xbf[:, D // 2:], w_ref[l, D // 2:D, cols]) + ya]
            xp_ref[0] = xp_ref[1] * jnp.concatenate(passes[1::2], axis=1) + x
            na, free = 8 * (28 + len(prods3)), cfg['AFREE']
            def gen():
                for u in range(na):
                    ps, rr = divmod((u - free) * len(passes) * (R0 // 8) // (na - free), R0 // 8)
                    yield None if u < free else (never, passes[ps][rr * 8:rr * 8 + 8, :])
            anchors = gen()
            for u in range(8):
                prep(l, u, anchors, zero)
            return carry

        jax.lax.fori_loop(0, L, layer, 0)
        xr_ref[...] = xp_ref[0].astype(bf16)
        xr_out.start()
        in_copy(0, 0).wait()
        for R in range(4):
            for C in range(4):
                conv(xn2_ref.at[0], 0, R, C, 0, Mh)
        for fn in carried:
            fn({}, STAGES[1][0], 0, 0, None)

    def main(tile, carry):
        zs, za = jax.lax.shift_right_logical(tile, 12), jax.lax.shift_right_logical(tile, 13)
        never = jnp.broadcast_to(zs, (8, 128)) != 0
        slot = tile % 2
        in_copy(jnp.minimum(tile + 2, NMAIN - 1), slot).start()
        in_copy(jnp.minimum(tile + 1, NMAIN - 1), 1 - slot).wait()

        @pl.when(tile > 1)
        def _():
            out_copy(tile - 2, slot, 0).wait()
            out_copy(tile - 2, slot, 1).wait()

        xn_ref = xn2_ref.at[1 - slot]
        o_ref = o2_ref.at[slot]
        rows = lambda h, r0: slice(r0, r0 + Mh) if h is None else slice(r0 + h * Mq, r0 + (h + 1) * Mq)

        def ld(loc, h=None):
            return loc[0][(0,) + loc[1] + (rows(h, loc[2]),)]

        def st(loc, v, h=None):
            loc[0][(zs,) + loc[1] + (rows(h, loc[2]),)] = v

        def by_half(v, h, fn):
            return fn(v, h) if h is not None else jnp.concatenate([fn(v[:Mq], 0), fn(v[Mq:], 1)], axis=0)

        def gather(ref, idx, n, pos):
            if cfg['NOBC']:
                return ref[idx + (slice(0, n), slice(16 * pos, 16 * pos + 16))].reshape(16 * n, 128)
            return ref.bitcast(u32)[idx + (slice(0, n), slice(8 * pos, 8 * pos + 8))].reshape(8 * n, 128)

        as_bf16 = lambda v: v if cfg['NOBC'] else pltpu.bitcast(v, bf16)

        def lhs2(p, q):
            ref, u = s2loc(p)
            return as_bf16(jnp.concatenate([gather(ref, (0, u, k), NC, q2[p].index(q)) for k in range(2)], axis=1))

        def rhs2(l, p, q, n):
            return as_bf16(gather(t2[p], (l, n), 16, q2[p].index(q)))

        def dot3(l, p, q, r):
            qs = next(qs for qs in PAIRS if q in qs)
            return _dot(as_bf16(gather(s3[(p, qs)], (0, qs.index(q)), NQ, ORD.index(r))),
                        as_bf16(gather(t3_ref, (l, prods3.index((p, q))), 8, ORD.index(r))))

        def add_bias(v, l, terms, where, h):
            coef = {}
            for sg, i, j, n, hh in where(h or 0):
                for cf, (I, J) in terms:
                    key = (2 * J + j) * 2 + n
                    coef[key] = coef.get(key, 0.0) + sg * cf * scale(2 * I + i, 2 * J + j, hh, n)
            bv = None
            for key, cf in sorted(coef.items()):
                if cf != 0.0:
                    b = bf_ref[l, :, key * 128:(key + 1) * 128]
                    b = (b + 1.0 if l == 0 else b) * cf
                    bv = b if bv is None else bv + b
            return v + bv if h is not None else by_half(v, h, lambda x, hh: x + bv * D2[hh])

        def outer_act(l, p, i, j, n, d, h):
            bt, stores, finals = OACT[p]
            if bt:
                def where(hh):
                    w = [(1, i, j)] + [(-1, 0, 1)] * bool(raw_slot(p) and (i, j) == B21)
                    again = [(-sg, ii, jj, 1, 0) for sg, ii, jj in w] if (h, n) == (1, 0) else []
                    return [x + (n, hh) for x in w] + again
                d = add_bias(d, l, bt, where, h)
            cache = {'d': d}
            def comb(terms):
                for _, src in terms:
                    if isinstance(src, str) and src not in cache:
                        cache[src] = ld(oloc(src, i, j, n), h)
                v = lincomb([(s, cache[src]) for s, src in terms if isinstance(src, str)])
                for _, src in terms:
                    if not isinstance(src, str):
                        v = add_bias(v, l, src, lambda hh: [(1, i, j, n, hh)], h)
                return v
            fin = [(IJ, comb(terms)) for IJ, terms in finals]
            for name, v in [(name, comb(terms)) for name, terms in stores]:
                st(oloc(name, i, j, n), v, h)
            for (I, J), y in fin:
                R, C = 2 * I + i, 2 * J + j
                xn = ld(x0loc(R, C, n), h) * y
                if l > 0:
                    xn = xn + ld(xloc(l, R, C, n), h)
                if l < L - 1:
                    st(xloc(l + 1, R, C, n), xn, h)
                else:
                    xn = by_half(xn, h, lambda x, hh: x if scale(R, C, hh, n) == 1.0 else x * (1.0 / scale(R, C, hh, n)))
                    o_ref[rows(h, R * Mh), C * H + n * 128:C * H + (n + 1) * 128] = xn.astype(bf16)

        def inner_act(g, l, p, kind, n, h, P, Q):
            vloc = oloc(raw_slot(p), 0, 1, n) if raw_slot(p) else iloc(g, 'v', n)
            if kind == '35':
                st(iloc(g, 's', n), Q + ld(iloc(g, 'm1', n), h), h)
                if not raw_slot(p):
                    st(vloc, P, h)
                outer_act(l, p, 0, 1, n, P, h)
            elif kind == '47':
                st(iloc(g, 'u', n), Q + ld(vloc, h), h)
                outer_act(l, p, 0, 0, n, P + ld(iloc(g, 's', n), h), h)
            else:
                outer_act(l, p, 1, 1, n, ld(iloc(g, 's', n), h) - Q, h)
                outer_act(l, p, 1, 0, n, P + ld(iloc(g, 'u', n), h), h)

        def issue(l, p, rd):
            kind, n = rd
            if kind == 'x':
                return [dot3(l, p, q, 1) for q in (3, 5, 4, 7)]
            if kind == 'y':
                return [dot3(l, pp, q, 1) for pp in (p, SEL3[SEL3.index(p) + 1]) for q in (2, 6)]
            if isinstance(n, str):
                return [dot3(l, p, int(q), int(r)) for r in n for q in kind]
            if kind == '1':
                lhs = lhs2(p, 1)
                return [_dot(lhs, rhs2(l, p, 1, 0)), _dot(lhs, rhs2(l, p, 1, 1))]
            return [_dot(lhs2(p, int(q)), rhs2(l, p, int(q), n)) for q in kind]

        def consume(g, l, p, rd, res):
            kind, n = rd
            if n == '1':
                for u, where in enumerate((('35', False), ('47', False)) if kind == 'x' else (('26', False), ('26', True))):
                    st(jloc(where[0], '1', 0, where[1]), res[2 * u] + res[2 * u + 1], 0)
                    st(jloc(where[0], '1', 1, where[1]), res[2 * u] - res[2 * u + 1], 0)
            elif isinstance(n, str):
                aa, bb = (res[0] + res[1], res[0] - res[1]), (res[2] + res[3], res[2] - res[3])
                sm = [aa[al] + bb[al] for al in range(2)]
                df = [aa[al] - bb[al] for al in range(2)]
                J = lambda name, al: ld(jloc(kind, name, al, name == '1' and kind == '26' and p in SEL3[1::2]), 0)
                if n == '35':
                    for al in range(2):
                        st(jloc(kind, 's', al), df[al] + J('1', al), 0)
                    inner_act(g, l, p, kind, 1, 0, sm[0], sm[1])
                elif n == '47':
                    O, I = (lambda i, j: oloc(raw_slot(p), i, j, 1)), (lambda name: iloc(g, name, 1))
                    v = {'35': [[(1, O(0, 1))], [(1, I('s')), (-1, I('m1'))]],
                         '47': [[(1, O(0, 0)), (-1, I('s'))], [(1, I('u')), (-1, O(0, 1))]],
                         '26': [[(1, O(1, 0)), (-1, I('u'))], [(1, I('s')), (-1, O(1, 1))]]}[kind]
                    for al in range(2):
                        st(jloc(kind, 'u', al), lincomb([(1, df[al])] + [(s, ld(loc, 0)) for s, loc in v[al]]), 0)
                    inner_act(g, l, p, kind, 0, 0, sm[0] + J('s', 0), sm[1] + J('s', 1))
                else:
                    inner_act(g, l, p, kind, 1, 1, J('s', 0) - df[0], J('s', 1) - df[1])
                    inner_act(g, l, p, kind, 0, 1, sm[0] + J('u', 0), sm[1] + J('u', 1))
            elif kind == '1':
                st(iloc(g, 'm1', 0), res[0])
                st(iloc(g, 'm1', 1), res[1])
            else:
                inner_act(g, l, p, kind, n, None, res[0] + res[1], res[0] - res[1])

        state = {}
        for g, rd, t0, n in sched:
            l, p = outs[g]
            if t0 == start[G - 1]:
                out_copy(tile, slot, 0).start()
            res = issue(l, p, rd)
            for t in range(t0, t0 + n):
                ev = plan.get(t, [])
                for u, (l2, fn, group) in enumerate(ev):
                    gr = 16 * (t - t0) + (0 if u == 0 and len(ev) > 1 else 8)
                    gate = res[0][gr:gr + 8, :]
                    if cfg['GADD'] and isinstance(rd[1], str):
                        gate = gate + res[1][gr:gr + 8, :]
                    if l2 is None:
                        conv(xn_ref, zs, *fn, min(32, Mh - fn[2]), (never, gate))
                    else:
                        xb[xset(l2)][0, 0, 0, 0, MP - 8:MP, :] = gate
                        fn(state.setdefault(id(fn), {}), group, zs, za, (never, gate))
            consume(g, l, p, rd, res)
        out_copy(tile, slot, 1).start()
        return carry

    prologue()
    jax.lax.fori_loop(0, NMAIN, main, 0)
    xr_out.wait()
    in_copy(NMAIN - 1, (NMAIN - 1) % 2).wait()
    for t in range(max(NMAIN - 2, 0), NMAIN):
        out_copy(t, t % 2, 0).wait()
        out_copy(t, t % 2, 1).wait()


DEFAULT = dict(SEL=(3, 5, 4, 7), SEL3=(3, 4), XC={B12: 5, B11: 1, B22: 7, B21: 2}, AFREE=4, NOBC=0, TIEL=3, GADD=1, TF=0, T8=0, TAIL=6,
               CS=0.5, CL=0.3, UL=0.8, CAP=0.85, FR=((1.,), (.4, .6), (.35, .37, .28), (.16, .26, .31, .27)))


def build(TM=640, **kw):
    def f(x0, ws, bs):
        B, D = x0.shape
        L = ws.shape[0]
        cfg = dict(DEFAULT, **kw)
        Mh = TM // 4
        MP = Mh + 32
        nmain = (B - 1) // TM
        R0 = B - nmain * TM
        pairs3, q2 = layout(cfg)
        n3 = sum(2 * len(v) for v in pairs3.values())
        pad = lambda n: n + (2 - n) % 4
        V = pltpu.VMEM
        half = V((1, MP, 128), f32)
        scratch = ([V((1, 2, 2, 2, MP, 128), f32)] * 4 + [V((1, 2, 4, 2, MP, 128), f32)] * 6 + [half] * (16 + 56 + 20)
                   + [V((1, 1 + (p == 2), 2, pad(Mh // 16), 16 * len(q2[p]), 128), bf16) for p in (1, 3, 4, 5, 7, 2)]
                   + [V((1, 2, pad(Mh // 32), 112, 128), bf16)] * (n3 // 2)
                   + [V((L, 2, 16, 16 * len(q2[p]), 128), bf16) for p in range(1, 8)]
                   + [V((L, n3, 8, 112, 128), bf16), V((1, 4, 16 * n3, 128), f32), V((1, 4, 16 * n3, 128), f32),
                      V((8, 1, D), f32), V((2, TM, D), bf16), V((2, TM, D), bf16), V((L, D, D), bf16),
                      V((R0, D), bf16), V((2, R0, D), f32), V((L, D), bf16), pltpu.SemaphoreType.DMA((L + 8,))])
        anyspec = pl.BlockSpec(memory_space=pl.ANY)
        return pl.pallas_call(
            functools.partial(_kernel, L=L, TM=TM, R0=R0, NMAIN=nmain, D=D, cfg=cfg),
            in_specs=[anyspec, anyspec, anyspec],
            out_specs=anyspec,
            out_shape=jax.ShapeDtypeStruct((B, D), x0.dtype),
            scratch_shapes=scratch,
            compiler_params=pltpu.CompilerParams(
                vmem_limit_bytes=110 * 1024 * 1024,
                internal_scratch_in_bytes=65536,
                disable_bounds_checks=True,
            ),
        )(x0, ws, bs)
    return f


@jax.jit
def pallas_standalone__dcn_v2_cross__recsys_kernel(x0, ws, bs):
    return build(TM=640)(x0, ws, bs)
```

```python
import functools

import jax
import jax.numpy as jnp
import jax.experimental.pallas as pl
import jax.experimental.pallas.tpu as pltpu

f32 = jnp.float32
bf16 = jnp.bfloat16
u32 = jnp.uint32

B11, B12, B21, B22 = (0, 0), (0, 1), (1, 0), (1, 1)
LA = {1: [(B11, 1), (B22, 1)], 2: [(B11, 1), (B12, 1), (B21, 1), (B22, 1)], 3: [(B11, 1), (B12, -1)],
      4: [(B12, 1), (B22, 1)], 5: [(B11, 1), (B12, 1)], 6: [(B12, 1), (B11, -1), (B21, 1), (B22, -1)],
      7: [(B12, 1), (B22, -1)]}
PAIRS = ((5, 3), (4, 7), (2, 6))
ORD = (3, 5, 4, 7, 1, 2, 6)
D2 = (1.0, 2.0)
BF = {1: 1.0, 2: 0.5, 3: 0.5, 4: 0.5, 5: 0.5, 6: 0.5, 7: 0.5}
OUTER = (3, 5, 1, 4, 7, 2, 6)
OACT = {
    3: ([(1, B12)], [('M3', [(1, 'd')])], []),
    5: ([], [('M5', [(1, 'd')])], [(B12, [(1, 'd'), (1, 'M3')])]),
    1: ([(1, B11), (-1, B12)], [('S', [(1, 'd'), (1, 'M3'), (-1, 'M5')])], []),
    4: ([], [('M4', [(1, 'd')])], []),
    7: ([], [('M7', [(1, 'd')])], [(B11, [(1, 'd'), (1, 'S'), (1, 'M4')])]),
    2: ([(1, B11), (-1, B22)], [('M2', [(1, 'd')]),
        ('U', [(1, 'd'), (1, 'M4'), (-1, 'M7'), (1, 'M3'), (1, 'M5'), (1, ((1, B21), (-1, B12), (-1, B11), (1, B22)))])], []),
    6: ([], [], [(B22, [(1, 'd'), (1, 'S'), (-1, 'M2')]), (B21, [(1, 'd'), (1, 'U')])]),
}
OSL = {'M3': 0, 'M5': 1, 'S': 2, 'M4': 3, 'M7': 4, 'M2': 6, 'U': 5}
ISL = {'m1': 0, 's': 1, 'v': 2, 'u': 3}
STAGES = {1: [(B11, B12, B21, B22)], 2: [(B11, B12), (B21, B22)], 3: [(B11, B12), (B22,), (B21,)],
          4: [(B11,), (B12,), (B22,), (B21,)]}
BIAS = [(p, extra, i, j, n, h) for p in OUTER for extra in (False, True)
        if (any(not isinstance(x, str) for _, t in OACT[p][1] + OACT[p][2] for _, x in t) if extra else OACT[p][0])
        for i in range(2) for j in range(2) for n in range(2) for h in range(2)]
PREP_ORDER = (2, 6, 3, 5, 1, 4, 7)
LAG = 8


def _dot(a, b):
    return jnp.dot(a, b, preferred_element_type=f32)


def scale(R, C, h, k):
    return D2[R // 2] * D2[R % 2] * D2[h] / (D2[C // 2] * D2[C % 2] * D2[k])


def b_ops(b11, b12, b21, b22):
    r1 = b11 + b22
    g = b12 + b21
    return {1: r1, 2: b11 - b12, 3: b12 - b22, 4: g - r1, 5: b12 + b22, 6: b11 + b12, 7: g + r1}


def lincomb(terms):
    assert terms[0][0] == 1
    acc = terms[0][1]
    for s, v in terms[1:]:
        acc = acc + v if s == 1 else acc - v
    return acc


def raw_slot(p):
    return next((name for name, terms in OACT[p][1] if terms == [(1, 'd')]), None)


def round_usage(p, rd, first, last, defer):
    bt, stores, finals = OACT[p]
    alu = bool(bt) + sum(len(t) - 1 for _, t in stores) + sum(len(t) + (not first) + 2 * last for _, t in finals)
    nst = len(stores) + len(finals)
    nld = len({x for _, t in stores + finals for _, x in t if isinstance(x, str) and x != 'd'}) + len(finals) * (2 - first)
    kind, n = rd
    if isinstance(n, str):
        e = kind == '47'
        if kind == '26':
            a, st, ld, m = {'35': (12, 2, 9, 2), '47': (18, 2, 13, 2), '26': (16, 0, 13, 4)}[n]
            if n in defer and finals:
                alu, nst, nld = 0, 1, 0
        else:
            a, st, ld, m = {'1': (4, 4, 5, 0), '35': (11 + e, 3, 8 + e, 1), '47': (14 + 2 * e, 3, 11 + 2 * e, 1),
                            '26': (14 + 2 * e, 2, 11 + 2 * e, 2)}[n]
    else:
        a, st, ld, m = {'1': (2, 2, 4, 0), '35': (5, 2 - bool(raw_slot(p)), 5, 1), '47': (6, 1, 6, 1),
                        '26': (6, 0, 6, 2)}[kind]
    return a + m * alu, st + m * nst, ld + m * nld


def yds(groups, cap):
    n = len(cap)
    speed, cls, gcls = [0.0] * n, [-1] * n, {}
    todo = list(groups)
    while todo:
        pre = [0.0]
        for t in range(n):
            pre.append(pre[-1] + (cap[t] if cls[t] < 0 else 0.0))
        best = None
        for a in sorted({g[0] for g in todo}):
            w = 0.0
            for g in sorted((g for g in todo if g[0] >= a), key=lambda g: g[1]):
                w += g[2]
                d = w / max(pre[g[1] + 1] - pre[a], 1e-9)
                if best is None or d > best[0]:
                    best = (d, a, g[1])
        d, a, b = best
        for t in range(a, b + 1):
            if cls[t] < 0:
                speed[t], cls[t] = d, len(gcls)
        gcls.update({g[:2]: len(gcls) for g in todo if g[0] >= a and g[1] <= b})
        todo = [g for g in todo if not (g[0] >= a and g[1] <= b)]
    return speed, cls, gcls


def spread_jobs(jobs, cap, tail):
    T = len(cap)
    cap3 = cap * 3
    all3 = [(lo + k * T, hi + k * T, ji, k) for k in range(3) for ji, (lo, hi, _) in enumerate(jobs) if lo + k * T >= 0]
    pend = {}
    for j in sorted(all3, key=lambda j: (j[1], j[3], j[2])):
        pend.setdefault(j[:2], []).append(j)
    speed, cls, gcls = yds([w + (sum(sum(jobs[j[2]][2]) for j in q),) for w, q in pend.items()], cap3)
    when = [[] for _ in jobs]
    debt, cur, done = 0.0, None, 0
    for t in range(3 * T):
        while True:
            j = cur
            if j is None:
                rdy = [q[0] for w, q in pend.items() if q and w[0] <= t and (gcls[w] == cls[t] or w[1] <= t)]
                if not rdy:
                    debt = max(debt, 0.0)
                    break
                j = rdy[0]
                nst = len(jobs[j[2]][2])
                if nst > 1 and j[1] > t and (t + tail + 2 * nst) // T != t // T:
                    break
            must = j[1] <= t or (cur is not None and (t + tail + 1) // T != t // T)
            if not must and (cap3[t] == 0.0 or debt > 0.5 * speed[t] * cap3[t]):
                break
            if cur is None:
                pend[j[:2]].pop(0)
                cur, done = j, 0
            debt += jobs[j[2]][2][done]
            if j[3] == 1:
                when[j[2]].append(t - T)
            done += 1
            if done == len(jobs[j[2]][2]):
                cur = None
        debt -= speed[t] * cap3[t]
    return when


def layout(cfg):
    sel, sel3 = cfg['SEL'], cfg['SEL3']
    pairs3 = {p: [qs for qs in PAIRS if p in sel3 or (p in sel and qs != (2, 6))] for p in range(1, 8)}
    q2 = {p: [q for q in ORD if not any(q in qs for qs in pairs3[p])] for p in range(1, 8)}
    return pairs3, q2


def _kernel(x_hbm, w_hbm, b_hbm, o_hbm, *scratch, L, TM, R0, NMAIN, D, cfg):
    H, Mh, Mq = D // 4, TM // 4, TM // 8
    NC, NQ = Mh // 16, Mq // 16
    MP = Mh + 32
    SEL, SEL3 = cfg['SEL'], cfg['SEL3']
    pairs3, q2 = layout(cfg)
    prods3 = [(p, q) for p in SEL for qs in pairs3[p] for q in qs]
    assert H == 256 and L % 2 == 0 and Mq % 16 == 0 and all(raw_slot(p) for p in SEL)
    it = iter(scratch)
    take = lambda n: [next(it) for _ in range(n)]
    x0b, xb, ib, ob, jb = take(4), take(6), take(16), take(56), take(20)
    s2 = dict(zip((1, 3, 4, 5, 7, 2), take(6)))
    s3 = {(p, qs): next(it) for p in SEL for qs in pairs3[p]}
    t2 = dict(zip(range(1, 8), take(7)))
    t3_ref, kb0, kb1, bt_ref, bf_ref, xn2_ref, o2_ref, w_ref, xr_ref, xp_ref, b_ref, sem = it

    xset = lambda l: 4 if l == 0 else (l % 2) * 2
    xoff = lambda I, J: cfg['XO'] * ((I + J) % 2)
    xloc = lambda l, R, C, k: (xb[xset(l) + R // 2], (R % 2, C, k), xoff(R // 2, C // 2))
    x0loc = lambda R, C, k: (x0b[(R // 2) * 2 + C // 2], (R % 2, C % 2, k), 8 + xoff(R // 2, C // 2))
    iloc = lambda g, name, n: (ib[((g % 2) * 4 + ISL[name]) * 2 + n], (), 8 * ISL[name])
    oloc = lambda name, i, j, n: (ob[(OSL[name] * 4 + i * 2 + j) * 2 + n], (), 8 * ((OSL[name] + 2 * j) % 4))

    def jloc(kind, name, al, second=False):
        i = 18 + al if second else (('35', '47', '26').index(kind) * 3 + ('1', 's', 'u').index(name)) * 2 + al
        return jb[i], (), 8 * ((i + i // 2) % 4)

    def s2loc(p):
        return (s2[2], (2, 6).index(p)) if p in (2, 6) else (s2[p], 0)

    def bias_coefs(p, extra, i, j, n, h):
        where = [(1, i, j, n, h)]
        if extra:
            terms = next(x for _, t in OACT[p][1] + OACT[p][2] for _, x in t if not isinstance(x, str))
        else:
            terms = OACT[p][0]
            w = [(1, i, j)] + [(-1, 0, 1)] * bool(raw_slot(p) and (i, j) == B21)
            where = [x + (n, h) for x in w]
            if (h, n) == (1, 0) and PAIRS[{B12: 0, B11: 1}.get((i, j), 2)] in pairs3[p]:
                where += [(-sg, ii, jj, 1, 0) for sg, ii, jj in w]
        coef = {}
        for sg, ii, jj, nn, hh in where:
            for cf, (I, J) in terms:
                key = (2 * J + jj) * 2 + nn
                coef[key] = coef.get(key, 0.0) + sg * cf * scale(2 * I + ii, 2 * J + jj, hh, nn)
        return coef

    def tie(v, anchor, r=0):
        if anchor is None:
            return v
        return jnp.concatenate([v[:r]] * (r > 0) + [jax.lax.select(anchor[0], anchor[1], v[r:r + 8])] + [v[r + 8:]] * (r + 8 < v.shape[0]), axis=0)

    def consts(anchor, ss, reps):
        one = {s: jnp.full((8, 128), s, f32) for s in set(ss)}
        if anchor is not None:
            one = {s: jax.lax.select(anchor[0], anchor[1], v) for s, v in one.items()}
        return jnp.concatenate([one[s] for s in ss for _ in range(reps)], axis=0)

    def conv(src, zs, R, C, r, nr, anchor=None):
        v = src[R * Mh + r:R * Mh + r + nr, C * H:(C + 1) * H].astype(f32)
        for k in range(2):
            buf, idx, off = xloc(0, R, C, k)
            sv = consts(anchor, [scale(R, C, (r + u) // Mq, k) for u in range(0, nr, 16)], 2)
            buf[(zs,) + idx + (slice(off + r, off + r + nr),)] = v[:, k * 128:(k + 1) * 128] * sv

    def block_sum(l, terms, ii, jj, kk, r, save, zs, za, anchor, at=None):
        rng = lambda t: slice(t[0], t[-1] + 1)
        vals = []
        for u, ((I, J), s) in enumerate(terms):
            r0 = xoff(I, J) + r
            v = xb[xset(l) + I][za if u == 0 else 0, rng(ii), slice(2 * J + jj[0], 2 * J + jj[-1] + 1), rng(kk), r0:r0 + 16, :]
            if (I, J) in save:
                sv = consts(anchor, [1.0 / scale(2 * I + i, 2 * J + j, r // Mq, k) for i in ii for j in jj for k in kk], 2)
                x0b[I * 2 + J][zs, rng(ii), rng(jj), rng(kk), r0 + 8:r0 + 24, :] = v * sv.reshape(v.shape)
            if u == 0 and at is not None and cfg['TIEL'] in (1, 2) and anchor is not None:
                v = tie(v.reshape(v.size // 128, 128), anchor, at + cfg['T8']).reshape(v.shape)
            vals.append((s, v))
        v = lincomb(vals)
        v = v.reshape(v.size // 128, 128)
        if cfg['TIEL'] == 3 and at is not None:
            v = tie(v, anchor, at)
        return v

    def finish(e, f, group, qs, store, st8, anchor):
        if not cfg['TIEL']:
            e = tie(e, anchor)
        a = e[None] if f is None else jnp.concatenate([e + f, e - f], axis=0).reshape(2, e.shape[0], 128)
        for u, b in enumerate(group):
            st8[b] = a if len(group) == 1 else a[:, 16 * u:16 * u + 16]
        ops = {}
        if B12 in group and 3 in qs:
            ops[3], ops[5] = st8[B11] - st8[B12], st8[B11] + st8[B12]
        if B22 in group:
            if 4 in qs:
                ops[4], ops[7] = st8[B12] + st8[B22], st8[B12] - st8[B22]
            ops[1] = st8['l1'] = st8[B11] + st8[B22]
        if B21 in group:
            g = st8[B12] + st8[B21]
            ops[2], ops[6] = g + st8['l1'], g - st8['l1']
        now = [q for q in qs if q in ops]
        if now:
            r0 = 16 * qs.index(now[0])
            store(slice(r0, r0 + 16 * len(now)), jnp.concatenate([ops[q] for q in now], axis=1).astype(bf16))

    def unit2(l, ps, c, k, save, st8, group, zs, za, anchor):
        ii, jj = sorted({b[0] for b in group}), sorted({b[1] for b in group})
        bs = lambda terms, at: block_sum(l, terms, ii, jj, [k], 16 * c, save, zs, za, anchor, at)
        at = 16 * (len(group) > 1)
        e, f = (bs(LA[ps[0]], at), None) if len(ps) == 1 else (bs([(B12, 1), (B21, 1)], at), bs([(B11, 1), (B22, 1)], None))
        def store(rows, v):
            s2[ps[0]][zs, :, k, c, rows, :] = v
        finish(e, f, group, q2[ps[0]], store, st8, anchor)

    def unit3(l, p, qs, c, save, st8, group, zs, za, anchor):
        for h in sorted({b[0] for b in group}):
            grp = tuple(b for b in group if b[0] == h)
            kk = [b[1] for b in grp]
            ii, jj = {(5, 3): ([0], [0, 1]), (4, 7): ([0, 1], [1]), (2, 6): ([0, 1], [0, 1])}[qs]
            v = block_sum(l, LA[p], ii, jj, sorted(kk), h * Mq + 16 * c, save, zs, za, anchor,
                          16 * (len(kk) > 1 or (qs == (2, 6) and not cfg['TF'])))
            n = 16 * len(kk)
            piece = lambda u: v[u * n:(u + 1) * n]
            if qs == (2, 6):
                e, f = piece(1) + piece(2), piece(0) + piece(3)
                r0 = 16 * q2[p].index(1)
                s2[p][zs, 0, min(kk):max(kk) + 1, h * NQ + c, r0:r0 + 16, :] = f.reshape(len(kk), 16, 128).astype(bf16)
            else:
                e, f = piece(0), piece(1)
            def store(rows, w):
                s3[(p, qs)][zs, :, c, rows, :] = w
            finish(e, f, tuple(sorted(grp)), ORD, store, st8, anchor)

    def prep(l, u, anchors, zero, kb):
        for k in range(2):
            wide = [w_ref[l, R * 2 + k, u].astype(f32) for R in range(4)]
            for n in range(2):
                def blk(R, C):
                    v = wide[R][:, C * H + n * 128:C * H + (n + 1) * 128]
                    s = D2[R // 2] / D2[C // 2]
                    return v if s == 1.0 else v * s
                O = {(i, j): b_ops(blk(i, j), blk(i, 2 + j), blk(2 + i, j), blk(2 + i, 2 + j)) for i, j in (B11, B12, B21, B22)}
                for p in PREP_ORDER:
                    anchor = next(anchors)
                    s = BF[p] * 0.5 * D2[k] / D2[n]
                    cs = {f: consts(anchor, [s * f], 2) for f in (0.5, 1.0, 2.0)}
                    T = b_ops(*[O[(i, j)][p] * cs[D2[i] / D2[j]] for i, j in (B11, B12, B21, B22)])
                    T[1] = T[1] + T[1]
                    t2[p][l, n, k * 8 + u] = jnp.concatenate([T[q] for q in q2[p]], axis=0).astype(bf16)
                    mine = [e for e, pq in enumerate(prods3) if pq[0] == p]
                    if mine:
                        kb[zero, k * 2 + n, 16 * mine[0]:16 * mine[-1] + 16, :] = jnp.concatenate(
                            [T[prods3[e][1]] for e in mine], axis=0)
        for e in range(len(prods3)):
            v = kb[0, :, 16 * e:16 * e + 16, :] * consts(next(anchors), [0.5], 2)
            T = b_ops(v[0], v[1], v[2], v[3])
            T[1] = T[1] + T[1]
            t3_ref[l, e, u] = jnp.concatenate([T[q] for q in ORD], axis=0).astype(bf16)

    def rounds_of(p):
        rs = [('1', None)] + [('x', '1')] * (p in SEL)
        for kind, qs in zip(('35', '47', '26'), PAIRS):
            if kind == '26' and p in SEL3[::2]:
                rs.append(('y', '1'))
            rs += [(kind, r) for r in (('35', '47', '26') if qs in pairs3[p] else (0, 1))]
        return rs

    outs = [(l, p) for l in range(L) for p in OUTER]
    G = len(outs)
    sched, start, use = [], [], []
    for g, (l, p) in enumerate(outs):
        start.append(len(use))
        for rd in rounds_of(p):
            n = NQ if isinstance(rd[1], str) else NC
            sched.append((g, rd, len(use), n))
            a, st_, ld_ = round_usage(p, rd, l == 0, l == L - 1, cfg['DEFER'])
            use += [max(a / 32, st_ / 8, cfg['UL'] * ld_ / 24)] * n
    T = len(use)
    cap = [max(cfg['CAP'] - max(use[t], use[(t + 1) % T]), 0.0) * (t < T - cfg['TAIL']) for t in range(T)]
    for g in range(G):
        for t in range(start[g], (start + [T])[g + 1]):
            cap[t] *= cfg['CM'][g % 7]
    jobs = []
    def add(lo, hi, alu, st_, ld_, nst, l, fn):
        w = alu / 64 + cfg['CS'] * (st_ + nst) / 16 + cfg['CL'] * ld_ / 48
        w *= cfg['KW'][0 if l in (None, 'fin') else nst]
        jobs.append((lo, max(hi, lo), [w * f for f in cfg['FR'][nst - 1]], l, fn))
    for g, (l, p) in enumerate(outs):
        ready = 7 * l - 2 * all(I == 0 for (I, J), _ in LA[p])
        lo = start[ready] - (T if ready < 0 else 0)
        if 7 in SEL3 and cfg['DEFER'] and ready % 7 == 5 and l > 0:
            lo += cfg['EW'] + 1
        if p in SEL3 and OACT[p][2]:
            for h, n in [(0, 1)] * ('35' in cfg['DEFER']) + [(0, 0)] * ('47' in cfg['DEFER']) + [(1, 1), (1, 0)] * ('26' in cfg['DEFER']):
                for c in range(0, NQ):
                    e0 = start[g + 1]
                    add(e0, e0 + cfg['EW'] if p == 7 else start[7 * l + 5] - 1, 20 + 8 * (l == L - 1), 3, 20, 1, 'fin',
                        (l, p, n, h * Mq + 16 * c))
        hi = start[g] - LAG - 3
        nt = len(LA[p])
        save = [b for b, pp in cfg['XC'].items() if pp == p and l == 0]
        if p in SEL3:
            if p in SEL3[1::2]:
                host = 7 * l + OUTER.index(SEL3[SEL3.index(p) - 1])
                hi = [t0 for gg, rd, t0, _ in sched if gg == host and rd[0] == 'y'][0] - LAG - 3
            for c in range(NQ):
                add(lo, hi, 32 * nt + 50 + 32 * len(save), 18 + 32 * len(save), 32 * nt, 4, l,
                    functools.partial(unit3, l, p, (2, 6), c, save))
        elif p != 6:
            ps = (2, 6) if p == 2 else (p,)
            nq = len(q2[p]) * len(ps)
            alu = 8 * (nt - 2 + len(ps)) + (8 if p in SEL else 16) * len(ps) + nq
            for c in range(NC):
                for k in range(2):
                    add(lo, hi, alu + 8 * len(save), nq + 8 * len(save), 8 * nt, 1 if nq <= 3 else 2 if nq <= 7 else 3, l,
                        functools.partial(unit2, l, ps, c, k, save))
        if p in SEL:
            for qs, c in ([(qs, c) for qs in PAIRS[:2] for c in range(NQ)] if cfg['QO'] else
                          [(qs, c) for c in range(NQ) for qs in PAIRS[:2]]):
                if True:
                    add(lo, start[g] - LAG - 3 + (NC if g else 0), 16 * nt + 46, 14, 16 * nt, 3, l,
                        functools.partial(unit3, l, p, qs, c, []))
    for R in range(4):
        for C in range(4):
            for c in range(0, NC, 2):
                add(start[6], start[G - 2] - 2, 18, 7, 4, 1, None, (R, C, 16 * c))
    when = spread_jobs([j[:3] for j in jobs], cap, cfg['TAIL'])
    evs = [e[:1] + e[2:] for e in sorted((t % T, ts[0] % T, ji, u) for ji, ts in enumerate(when) for u, t in enumerate(ts))]
    half = {}
    for e, (t, ji, u) in enumerate(evs):
        half[(ji, u)] = 2 * t + (0 if e + 1 < len(evs) and evs[e + 1][0] == t and (e == 0 or evs[e - 1][0] != t) else 1)
    SEG = cfg['SEG']
    for sg, seeds in enumerate(cfg['SEEDS']):
        mine = [e for e, ev in enumerate(evs) if ev[0] // SEG == sg]
        for seed in seeds:
            for e in mine:
                _, ji, u = evs[e]
                r = (e * 2654435761 + seed * 97531 + 12345) * 2246822519 % 4294967296 >> 8
                if r % 100 >= cfg['PJ']:
                    continue
                h = half[(ji, u)] + (2, -2, 1, -1, 2, -2)[r // 100 % 6]
                off = when[ji][u] - when[ji][u] % T
                lo_ = max(2 * (jobs[ji][0] - off), 2 * sg * SEG, half[evs[e - 1][1:]] + 1 if e else 0)
                hi_ = min(2 * (jobs[ji][1] - off) + 1, 2 * (sg + 1) * SEG - 1,
                          half[evs[e + 1][1:]] - 1 if e + 1 < len(evs) else 2 * (T - cfg['TAIL']))
                if lo_ <= h <= hi_:
                    half[(ji, u)] = h
    if cfg.get('SHOW'):
        for g in range(7, 14):
            rg = range(start[g], start[g + 1])
            print('  ', ''.join('%2d' % round(10 * use[t]) for t in rg))
            print('  ', ''.join('%2s' % ''.join((str(len(w)) if u == 0 else '.') for w in when for u, x in enumerate(w) if x % T == t) for t in rg))
    plan = {}
    for _, ji, u in evs:
        plan.setdefault(half[(ji, u)] // 2, []).append((half[(ji, u)] % 2, jobs[ji][3], jobs[ji][4], STAGES[len(when[ji])][u]))
    assert all((ts[0] < 0) == (ts[-1] < 0) for ts in when)
    carried = [(job[4], len(ts)) for ts, job in zip(when, jobs) if ts[0] < 0]

    def w_copy(l):
        return pltpu.make_async_copy(w_hbm.at[l], w_ref.at[l], sem.at[l])

    def w0_copy(u):
        return pltpu.make_async_copy(w_hbm.at[0, :, u], w_ref.at[0, :, u], sem.at[L + 10 + u])

    def in_copy(t, slot):
        return pltpu.make_async_copy(x_hbm.at[pl.ds(pl.multiple_of(t * TM, 32), TM)], xn2_ref.at[slot], sem.at[L + slot])

    def out_copy(t, slot, part):
        r0, nr = ((0, 2 * Mh), (2 * Mh, Mh), (3 * Mh, Mh))[part]
        return pltpu.make_async_copy(o2_ref.at[slot, pl.ds(r0, nr)],
                                     o_hbm.at[pl.ds(pl.multiple_of(t * TM + r0, 32), nr)],
                                     sem.at[L + 4 + 3 * slot + part])

    xr_in = pltpu.make_async_copy(x_hbm.at[pl.ds(NMAIN * TM, R0)], xr_ref, sem.at[L + 2])
    xr_out = pltpu.make_async_copy(xr_ref, o_hbm.at[pl.ds(NMAIN * TM, R0)], sem.at[L + 2])
    b_in = pltpu.make_async_copy(b_hbm, b_ref, sem.at[L + 3])

    def prologue():
        b_in.start()
        for u in range(8):
            w0_copy(u).start()
        xr_in.start()
        in_copy(0, 0).start()
        for l in range(1, L):
            w_copy(l).start()
        in_copy(min(1, NMAIN - 1), 1).start()
        b_in.wait()
        for l in range(L):
            bf_ref[l] = b_ref[l:l + 1, :].astype(f32)

        def bias_tiles(l, carry):
            b = jnp.broadcast_to(bf_ref[l] + (l == 0).astype(f32), (8, D))
            for u, site in enumerate(BIAS):
                terms = [b[:, key * 128:(key + 1) * 128] * cf for key, cf in sorted(bias_coefs(*site).items()) if cf != 0.0]
                bt_ref[l, u] = functools.reduce(lambda x, y: x + y, terms)
            return carry
        jax.lax.fori_loop(0, L, bias_tiles, 0)
        if cfg.get('FAST'):
            return

        def slab(u, carry):
            w0_copy(u).wait()
            zero = jax.lax.shift_right_logical(u, 12)
            prep(0, u, iter(lambda: None, 0), zero, kb0)
            return zero
        zero = jax.lax.fori_loop(0, cfg['NSLAB'], slab, 0)

        def plain(l, xbf, x0f, x, na, free, never, j0=0, j1=D // 128):
            passes = []
            for jt in range(j0, j1):
                cols = slice(jt * 128, (jt + 1) * 128)
                ya = _dot(xbf[:, :D // 2], w_ref[l, 0:4, :, :, cols].reshape(D // 2, 128)) + bf_ref[l, :, cols]
                passes += [ya, _dot(xbf[:, D // 2:], w_ref[l, 4:8, :, :, cols].reshape(D // 2, 128)) + ya]
            xp_ref[0, :, j0 * 128:j1 * 128] = x0f * jnp.concatenate(passes[1::2], axis=1) + x
            for u in range(na):
                ps, rr = divmod((u - free) * len(passes) * (R0 // 8) // (na - free), R0 // 8)
                yield None if u < free else (never, passes[ps][rr * 8:rr * 8 + 8, :])

        for u in range(cfg['NSLAB'], 8):
            w0_copy(u).wait()
        xr_in.wait()
        never = jnp.broadcast_to(zero, (8, 128)) != 0
        jm = cfg['JM']
        x0f = xr_ref[:, :jm * 128].astype(f32)
        xp_ref[1, :, :jm * 128] = x0f
        anchors = plain(0, xr_ref[...], x0f, x0f, (8 - cfg['NSLAB']) * (28 + len(prods3)), cfg['AFREE'], never, 0, jm)
        for u in range(cfg['NSLAB'], 8):
            prep(0, u, anchors, zero, (kb0, kb1)[u % 2])
        in_copy(0, 0).wait()
        x0f = xr_ref[:, jm * 128:].astype(f32)
        xp_ref[1, :, jm * 128:] = x0f
        units = [(R, C, r) for R in range(4) for C in range(4) for r in range(0, Mh, 32)]
        anchors = plain(0, xr_ref[...], x0f, x0f, len(units) + sum(n for _, n in carried) + 2, 4, never, jm)
        for R, C, r in units[:len(units) // 2]:
            conv(xn2_ref.at[0], zero, R, C, r, min(32, Mh - r), next(anchors))
        for fn, n in carried:
            st8 = {}
            for group in STAGES[n]:
                anchor = next(anchors)
                xb[xset(0)][0, 0, 0, 0, Mh + 24:Mh + 32, :] = anchor[1]
                fn(st8, group, zero, jax.lax.shift_right_logical(zero, 1), anchor)
        for R, C, r in units[len(units) // 2:]:
            conv(xn2_ref.at[0], zero, R, C, r, min(32, Mh - r), next(anchors))

        def layer(l, carry):
            w_copy(l).wait()
            zero = jax.lax.shift_right_logical(l, 12)
            x = xp_ref[0]
            anchors = plain(l, x.astype(bf16), xp_ref[1], x, 8 * (28 + len(prods3)), cfg['AFREE'],
                            jnp.broadcast_to(zero, (8, 128)) != 0)
            for u in range(8):
                prep(l, u, anchors, zero, (kb0, kb1)[u % 2])
            return carry

        jax.lax.fori_loop(1, L, layer, 0)
        xr_ref[...] = xp_ref[0].astype(bf16)
        xr_out.start()

    def main(tile, carry):
        zs, za = jax.lax.shift_right_logical(tile, 12), jax.lax.shift_right_logical(tile, 13)
        never = jnp.broadcast_to(zs, (8, 128)) != 0
        slot = tile % 2
        in_copy(jnp.minimum(tile + 2, NMAIN - 1), slot).start()
        in_copy(jnp.minimum(tile + 1, NMAIN - 1), 1 - slot).wait()

        @pl.when(tile > 1)
        def _():
            for part in range(3):
                out_copy(tile - 2, slot, part).wait()

        xn_ref = xn2_ref.at[1 - slot]
        o_ref = o2_ref.at[slot]
        def rows(h, r0):
            if isinstance(h, tuple):
                return slice(r0 + h[0], r0 + h[0] + h[1])
            return slice(r0, r0 + Mh) if h is None else slice(r0 + h * Mq, r0 + (h + 1) * Mq)

        def ld(loc, h=None):
            return loc[0][(0,) + loc[1] + (rows(h, loc[2]),)]

        def st(loc, v, h=None):
            loc[0][(zs,) + loc[1] + (rows(h, loc[2]),)] = v

        def by_half(v, h, fn):
            if isinstance(h, tuple):
                h = h[0] // Mq
            return fn(v, h) if h is not None else jnp.concatenate([fn(v[:Mq], 0), fn(v[Mq:], 1)], axis=0)

        def gather(ref, idx, n, pos):
            if cfg['NOBC']:
                return ref[idx + (slice(0, n), slice(16 * pos, 16 * pos + 16))].reshape(16 * n, 128)
            return ref.bitcast(u32)[idx + (slice(0, n), slice(8 * pos, 8 * pos + 8))].reshape(8 * n, 128)

        as_bf16 = lambda v: v if cfg['NOBC'] else pltpu.bitcast(v, bf16)

        def lhs2(p, q):
            ref, u = s2loc(p)
            return as_bf16(jnp.concatenate([gather(ref, (0, u, k), NC, q2[p].index(q)) for k in range(2)], axis=1))

        def rhs2(l, p, q, n):
            return as_bf16(gather(t2[p], (l, n), 16, q2[p].index(q)))

        def dot3(l, p, q, r):
            qs = next(qs for qs in PAIRS if q in qs)
            return _dot(as_bf16(gather(s3[(p, qs)], (0, qs.index(q)), NQ, ORD.index(r))),
                        as_bf16(gather(t3_ref, (l, prods3.index((p, q))), 8, ORD.index(r))))

        def add_bias(v, l, site, h):
            def one(x, hh):
                b = bt_ref[l, BIAS.index(site + (hh,))]
                return (x.reshape(Mq // 8, 8, 128) + b).reshape(Mq, 128)
            return by_half(v, h, one)

        def outer_act(l, p, i, j, n, d, h, part=None):
            bt, stores, finals = OACT[p]
            if part == 'stores':
                finals = []
            if part == 'finals':
                bt, stores = [], []
            if bt:
                d = add_bias(d, l, (p, False, i, j, n), h)
            cache = {'d': d}
            def comb(terms):
                for _, src in terms:
                    if isinstance(src, str) and src not in cache:
                        cache[src] = ld(oloc(src, i, j, n), h)
                v = lincomb([(s, cache[src]) for s, src in terms if isinstance(src, str)])
                for _, src in terms:
                    if not isinstance(src, str):
                        v = add_bias(v, l, (p, True, i, j, n), h)
                return v
            fin = [(IJ, comb(terms)) for IJ, terms in finals]
            for name, v in [(name, comb(terms)) for name, terms in stores]:
                st(oloc(name, i, j, n), v, h)
            for (I, J), y in fin:
                R, C = 2 * I + i, 2 * J + j
                xn = ld(x0loc(R, C, n), h) * y
                if l > 0:
                    xn = xn + ld(xloc(l, R, C, n), h)
                if l < L - 1:
                    st(xloc(l + 1, R, C, n), xn, h)
                else:
                    xn = by_half(xn, h, lambda x, hh: x if scale(R, C, hh, n) == 1.0 else x * (1.0 / scale(R, C, hh, n)))
                    o_ref[rows(h, R * Mh), C * H + n * 128:C * H + (n + 1) * 128] = xn.astype(bf16)

        def inner_act(g, l, p, kind, n, h, P, Q, part=None):
            vloc = oloc(raw_slot(p), 0, 1, n) if raw_slot(p) else iloc(g, 'v', n)
            if kind == '35':
                st(iloc(g, 's', n), Q + ld(iloc(g, 'm1', n), h), h)
                if not raw_slot(p):
                    st(vloc, P, h)
                outer_act(l, p, 0, 1, n, P, h)
            elif kind == '47':
                st(iloc(g, 'u', n), Q + ld(vloc, h), h)
                outer_act(l, p, 0, 0, n, P + ld(iloc(g, 's', n), h), h)
            else:
                outer_act(l, p, 1, 1, n, ld(iloc(g, 's', n), h) - Q, h, part)
                outer_act(l, p, 1, 0, n, P + ld(iloc(g, 'u', n), h), h, part)

        def issue(l, p, rd):
            kind, n = rd
            if kind == 'x':
                return [dot3(l, p, q, 1) for q in (3, 5, 4, 7)]
            if kind == 'y':
                return [dot3(l, pp, q, 1) for pp in (p, SEL3[SEL3.index(p) + 1]) for q in (2, 6)]
            if isinstance(n, str):
                return [dot3(l, p, int(q), int(r)) for r in n for q in kind]
            if kind == '1':
                lhs = lhs2(p, 1)
                return [_dot(lhs, rhs2(l, p, 1, 0)), _dot(lhs, rhs2(l, p, 1, 1))]
            return [_dot(lhs2(p, int(q)), rhs2(l, p, int(q), n)) for q in kind]

        def consume(g, l, p, rd, res):
            kind, n = rd
            if n == '1':
                for u, where in enumerate((('35', False), ('47', False)) if kind == 'x' else (('26', False), ('26', True))):
                    st(jloc(where[0], '1', 0, where[1]), res[2 * u] + res[2 * u + 1], 0)
                    st(jloc(where[0], '1', 1, where[1]), res[2 * u] - res[2 * u + 1], 0)
            elif isinstance(n, str):
                aa, bb = (res[0] + res[1], res[0] - res[1]), (res[2] + res[3], res[2] - res[3])
                sm = [aa[al] + bb[al] for al in range(2)]
                df = [aa[al] - bb[al] for al in range(2)]
                J = lambda name, al: ld(jloc(kind, name, al, name == '1' and kind == '26' and p in SEL3[1::2]), 0)
                part = 'stores' if n in cfg['DEFER'] else None
                if n == '35':
                    for al in range(2):
                        st(jloc(kind, 's', al), df[al] + J('1', al), 0)
                    inner_act(g, l, p, kind, 1, 0, sm[0], sm[1], part)
                elif n == '47':
                    O, I = (lambda i, j: oloc(raw_slot(p), i, j, 1)), (lambda name: iloc(g, name, 1))
                    v = {'35': [[(1, O(0, 1))], [(1, I('s')), (-1, I('m1'))]],
                         '47': [[(1, O(0, 0)), (-1, I('s'))], [(1, I('u')), (-1, O(0, 1))]],
                         '26': [[(1, O(1, 0)), (-1, I('u'))], [(1, I('s')), (-1, O(1, 1))]]}[kind]
                    for al in range(2):
                        st(jloc(kind, 'u', al), lincomb([(1, df[al])] + [(s, ld(loc, 0)) for s, loc in v[al]]), 0)
                    inner_act(g, l, p, kind, 0, 0, sm[0] + J('s', 0), sm[1] + J('s', 1), part)
                else:
                    inner_act(g, l, p, kind, 1, 1, J('s', 0) - df[0], J('s', 1) - df[1], part)
                    inner_act(g, l, p, kind, 0, 1, sm[0] + J('u', 0), sm[1] + J('u', 1), part)
            elif kind == '1':
                st(iloc(g, 'm1', 0), res[0])
                st(iloc(g, 'm1', 1), res[1])
            else:
                inner_act(g, l, p, kind, n, None, res[0] + res[1], res[0] - res[1])

        state = {}
        for g, rd, t0, n in sched:
            l, p = outs[g]
            if t0 == start[G - 1]:
                out_copy(tile, slot, 0).start()
            if t0 + n == T:
                out_copy(tile, slot, 1).start()
            res = issue(l, p, rd)
            for t in range(t0, t0 + n):
                for ph, l2, fn, group in plan.get(t, []):
                    gr = 16 * (t - t0) + 8 * ph
                    gate = res[0][gr:gr + 8, :]
                    if cfg['GADD'] and isinstance(rd[1], str):
                        gate = gate + res[1][gr:gr + 8, :]
                    if l2 == 'fin':
                        lf, pf, nf, r0 = fn
                        for j in range(2):
                            d = ld(oloc(raw_slot(pf), 1, j, nf), (r0, 16))
                            d = tie(tie(d, (never, gate)), (never, gate), 8)
                            outer_act(lf, pf, 1, j, nf, d, (r0, 16), 'finals')
                    elif l2 is None:
                        conv(xn_ref, zs, *fn, min(32, Mh - fn[2]), (never, gate))
                    else:
                        xb[xset(l2)][0, 0, 0, 0, Mh + 24:Mh + 32, :] = gate
                        fn(state.setdefault(id(fn), {}), group, zs, za, (never, gate))
            consume(g, l, p, rd, res)
        out_copy(tile, slot, 2).start()
        return carry

    prologue()
    jax.lax.fori_loop(0, NMAIN, main, 0)
    xr_out.wait()
    in_copy(NMAIN - 1, (NMAIN - 1) % 2).wait()
    for t in range(max(NMAIN - 2, 0), NMAIN):
        for part in range(3):
            out_copy(t, t % 2, part).wait()


DEFAULT = dict(SEL=(3, 5, 4, 7), SEL3=(3, 5, 4, 7), XC={B12: 5, B11: 1, B22: 7, B21: 2}, AFREE=4, NOBC=0, NSLAB=5, JM=4, XP=40, XO=16, DEFER=('26',), EW=12, KW=(1,) * 5, CM=(1,) * 7, SEEDS=(), SEG=32, PJ=20, QO=0, TIEL=3, GADD=1, TF=0, T8=0, TAIL=6,
               CS=0.5, CL=0.3, UL=0.8, CAP=0.85, FR=((1.,), (.4, .6), (.35, .37, .28), (.16, .26, .31, .27)))


def build(TM=640, **kw):
    def f(x0, ws, bs):
        B, D = x0.shape
        L = ws.shape[0]
        cfg = dict(DEFAULT, **kw)
        Mh = TM // 4
        MP = Mh + 32
        nmain = (B - 1) // TM
        R0 = B - nmain * TM
        pairs3, q2 = layout(cfg)
        n3 = sum(2 * len(v) for v in pairs3.values())
        pad = lambda n: n + (2 - n) % 4
        V = pltpu.VMEM
        half = V((1, MP, 128), f32)
        XP = Mh + cfg['XP']
        scratch = ([V((1, 2, 2, 2, XP, 128), f32)] * 4 + [V((1, 2, 4, 2, XP, 128), f32)] * 6 + [half] * (16 + 56 + 20)
                   + [V((1, 1 + (p == 2), 2, pad(Mh // 16), 16 * len(q2[p]), 128), bf16) for p in (1, 3, 4, 5, 7, 2)]
                   + [V((1, 2, pad(Mh // 32), 112, 128), bf16)] * (n3 // 2)
                   + [V((L, 2, 16, 16 * len(q2[p]), 128), bf16) for p in range(1, 8)]
                   + [V((L, n3, 8, 112, 128), bf16), V((1, 4, 16 * n3, 128), f32), V((1, 4, 16 * n3, 128), f32),
                      V((L, len(BIAS), 8, 128), f32), V((8, 1, D), f32), V((2, TM, D), bf16), V((2, TM, D), bf16), V((L, 8, 8, 16, D), bf16),
                      V((R0, D), bf16), V((2, R0, D), f32), V((L, D), bf16), pltpu.SemaphoreType.DMA((L + 18,))])
        anyspec = pl.BlockSpec(memory_space=pl.ANY)
        return pl.pallas_call(
            functools.partial(_kernel, L=L, TM=TM, R0=R0, NMAIN=nmain, D=D, cfg=cfg),
            in_specs=[anyspec, anyspec, anyspec],
            out_specs=anyspec,
            out_shape=jax.ShapeDtypeStruct((B, D), x0.dtype),
            scratch_shapes=scratch,
            compiler_params=pltpu.CompilerParams(
                vmem_limit_bytes=110 * 1024 * 1024,
                internal_scratch_in_bytes=65536,
                disable_bounds_checks=True,
            ),
        )(x0, ws.reshape(L, 8, 8, 16, D), bs)
    return f


@jax.jit
def pallas_standalone__dcn_v2_cross__recsys_kernel(x0, ws, bs):
    return build(TM=640)(x0, ws, bs)
```

```python
import functools

import jax
import jax.numpy as jnp
import jax.experimental.pallas as pl
import jax.experimental.pallas.tpu as pltpu

f32 = jnp.float32
bf16 = jnp.bfloat16
u32 = jnp.uint32

B11, B12, B21, B22 = (0, 0), (0, 1), (1, 0), (1, 1)
LA = {1: [(B11, 1), (B22, 1)], 2: [(B11, 1), (B12, 1), (B21, 1), (B22, 1)], 3: [(B11, 1), (B12, -1)],
      4: [(B12, 1), (B22, 1)], 5: [(B11, 1), (B12, 1)], 6: [(B12, 1), (B11, -1), (B21, 1), (B22, -1)],
      7: [(B12, 1), (B22, -1)]}
PAIRS = ((5, 3), (4, 7), (2, 6))
ORD = (3, 5, 4, 7, 1, 2, 6)
D2 = (1.0, 2.0)
BF = {1: 1.0, 2: 0.5, 3: 0.5, 4: 0.5, 5: 0.5, 6: 0.5, 7: 0.5}
OUTER = (3, 5, 1, 4, 7, 2, 6)
OACT = {
    3: ([(1, B12)], [('M3', [(1, 'd')])], []),
    5: ([], [('M5', [(1, 'd')])], [(B12, [(1, 'd'), (1, 'M3')])]),
    1: ([(1, B11), (-1, B12)], [('S', [(1, 'd'), (1, 'M3'), (-1, 'M5')])], []),
    4: ([], [('M4', [(1, 'd')])], []),
    7: ([], [('M7', [(1, 'd')])], [(B11, [(1, 'd'), (1, 'S'), (1, 'M4')])]),
    2: ([(1, B11), (-1, B22)], [('M2', [(1, 'd')]),
        ('U', [(1, 'd'), (1, 'M4'), (-1, 'M7'), (1, 'M3'), (1, 'M5'), (1, ((1, B21), (-1, B12), (-1, B11), (1, B22)))])], []),
    6: ([], [], [(B22, [(1, 'd'), (1, 'S'), (-1, 'M2')]), (B21, [(1, 'd'), (1, 'U')])]),
}
OSL = {'M3': 0, 'M5': 1, 'S': 2, 'M4': 3, 'M7': 4, 'M2': 6, 'U': 5}
ISL = {'m1': 0, 's': 1, 'v': 2, 'u': 3}
STAGES = {1: [(B11, B12, B21, B22)], 2: [(B11, B12), (B21, B22)], 3: [(B11, B12), (B22,), (B21,)],
          4: [(B11,), (B12,), (B22,), (B21,)], 5: [(B11, B12), (B22, 'hold'), ('l1',), (B21,)],
          6: [(B11,), (B12,), (B22, 'hold'), ('l1',), (B21,)]}
BIAS = [(p, extra, i, j, n, h) for p in OUTER for extra in (False, True)
        if (any(not isinstance(x, str) for _, t in OACT[p][1] + OACT[p][2] for _, x in t) if extra else OACT[p][0])
        for i in range(2) for j in range(2) for n in range(2) for h in range(2)]
PREP_ORDER = (2, 6, 3, 5, 1, 4, 7)
LAG = 8


def _dot(a, b):
    return jnp.dot(a, b, preferred_element_type=f32)


def scale(R, C, h, k):
    return D2[R // 2] * D2[R % 2] * D2[h] / (D2[C // 2] * D2[C % 2] * D2[k])


def b_ops(b11, b12, b21, b22):
    r1 = b11 + b22
    g = b12 + b21
    return {1: r1, 2: b11 - b12, 3: b12 - b22, 4: g - r1, 5: b12 + b22, 6: b11 + b12, 7: g + r1}


def lincomb(terms):
    assert terms[0][0] == 1
    acc = terms[0][1]
    for s, v in terms[1:]:
        acc = acc + v if s == 1 else acc - v
    return acc


def raw_slot(p):
    return next((name for name, terms in OACT[p][1] if terms == [(1, 'd')]), None)


def round_usage(p, rd, first, last, defer, hy):
    bt, stores, finals = OACT[p]
    alu = bool(bt) + sum(len(t) - 1 for _, t in stores) + sum(len(t) + (not first) + 2 * last for _, t in finals)
    nst = len(stores) + len(finals)
    nld = len({x for _, t in stores + finals for _, x in t if isinstance(x, str) and x != 'd'}) + len(finals) * (2 - first)
    kind, n = rd
    if isinstance(n, str):
        e = kind == '47'
        if kind == '26':
            a, st, ld, m = {'35': (10, 2, 9, 2), '47': (10, 2, 9, 2) if hy == 1 else (16, 2, 13, 2), '26': (20, 0, 17, 4) if hy == 1 else (16, 0, 13, 4)}[n]
            if n in defer and finals:
                alu, nst, nld = 0, 1, 0
        else:
            a, st, ld, m = {'1': (0, 4, 5, 0), '35': (9 + e, 3, 8 + e, 1),
                            '47': (9 + e, 3, 8 + e, 1) if hy == 1 else (14 + 2 * e, 3, 11 + 2 * e, 1),
                            '26': (17 + 3 * e, 2, 14 + 3 * e, 2) if hy == 1 else (14 + 2 * e, 2, 11 + 2 * e, 2)}[n]
    else:
        a, st, ld, m = {'1': (2, 2, 4, 0), '35': (5, 2 - bool(raw_slot(p)), 5, 1), '47': (6, 1, 6, 1),
                        '26': (6, 0, 6, 2)}[kind]
    return a + m * alu, st + m * nst, ld + m * nld


def yds(groups, cap):
    n = len(cap)
    speed, cls, gcls = [0.0] * n, [-1] * n, {}
    todo = list(groups)
    while todo:
        pre = [0.0]
        for t in range(n):
            pre.append(pre[-1] + (cap[t] if cls[t] < 0 else 0.0))
        best = None
        for a in sorted({g[0] for g in todo}):
            w = 0.0
            for g in sorted((g for g in todo if g[0] >= a), key=lambda g: g[1]):
                w += g[2]
                d = w / max(pre[g[1] + 1] - pre[a], 1e-9)
                if best is None or d > best[0]:
                    best = (d, a, g[1])
        d, a, b = best
        for t in range(a, b + 1):
            if cls[t] < 0:
                speed[t], cls[t] = d, len(gcls)
        gcls.update({g[:2]: len(gcls) for g in todo if g[0] >= a and g[1] <= b})
        todo = [g for g in todo if not (g[0] >= a and g[1] <= b)]
    return speed, cls, gcls


def spread_jobs(jobs, cap, tail):
    T = len(cap)
    cap3 = cap * 3
    all3 = [(lo + k * T, hi + k * T, ji, k) for k in range(3) for ji, (lo, hi, _) in enumerate(jobs) if lo + k * T >= 0]
    pend = {}
    for j in sorted(all3, key=lambda j: (j[1], j[3], j[2])):
        pend.setdefault(j[:2], []).append(j)
    speed, cls, gcls = yds([w + (sum(sum(jobs[j[2]][2]) for j in q),) for w, q in pend.items()], cap3)
    when = [[] for _ in jobs]
    debt, cur, done = 0.0, None, 0
    for t in range(3 * T):
        while True:
            j = cur
            if j is None:
                rdy = [q[0] for w, q in pend.items() if q and w[0] <= t and (gcls[w] == cls[t] or w[1] <= t)]
                if not rdy:
                    debt = max(debt, 0.0)
                    break
                j = rdy[0]
                nst = len(jobs[j[2]][2])
                if nst > 1 and j[1] > t and (t + tail + 2 * nst) // T != t // T:
                    break
            must = j[1] <= t or (cur is not None and (t + tail + 1) // T != t // T)
            if not must and (cap3[t] == 0.0 or debt > 0.5 * speed[t] * cap3[t]):
                break
            if cur is None:
                pend[j[:2]].pop(0)
                cur, done = j, 0
            debt += jobs[j[2]][2][done]
            if j[3] == 1:
                when[j[2]].append(t - T)
            done += 1
            if done == len(jobs[j[2]][2]):
                cur = None
        debt -= speed[t] * cap3[t]
    return when


def layout(cfg):
    sel, sel3 = cfg['SEL'], cfg['SEL3']
    pairs3 = {p: [qs for qs in PAIRS if p in sel3 or (p in sel and qs != (2, 6))] for p in range(1, 8)}
    q2 = {p: [q for q in ORD if not any(q in qs for qs in pairs3[p])] for p in range(1, 8)}
    return pairs3, q2


def _kernel(x_hbm, w_hbm, b_hbm, o_hbm, *scratch, L, TM, R0, NMAIN, D, cfg):
    H, Mh, Mq = D // 4, TM // 4, TM // 8
    NC, NQ = Mh // 16, Mq // 16
    MP = Mh + 32
    SEL, SEL3 = cfg['SEL'], cfg['SEL3']
    pairs3, q2 = layout(cfg)
    prods3 = [(p, q) for p in SEL for qs in pairs3[p] for q in qs]
    assert H == 256 and L % 2 == 0 and Mq % 16 == 0 and all(raw_slot(p) for p in SEL)
    it = iter(scratch)
    take = lambda n: [next(it) for _ in range(n)]
    x0b, xb, ib, ob, jb = take(4), take(6), take(16), take(56), take(26)
    s2 = dict(zip((1, 3, 4, 5, 7, 2), take(6)))
    s3 = {(p, qs): next(it) for p in SEL for qs in pairs3[p]}
    t2 = dict(zip(range(1, 8), take(7)))
    t3_ref, kb0, kb1, bt_ref, bf_ref, xn2_ref, o2_ref, w_ref, xr_ref, xp_ref, b_ref, sem = it

    xset = lambda l: 4 if l == 0 else (l % 2) * 2
    xoff = lambda I, J: cfg['XO'] * ((I + J) % 2)
    xloc = lambda l, R, C, k: (xb[xset(l) + R // 2], (R % 2, C, k), xoff(R // 2, C // 2))
    x0loc = lambda R, C, k: (x0b[(R // 2) * 2 + C // 2], (R % 2, C % 2, k), 8 + xoff(R // 2, C // 2))
    iloc = lambda g, name, n: (ib[((g % 2) * 4 + ISL[name]) * 2 + n], (), 8 * ISL[name])
    oloc = lambda name, i, j, n: (ob[(OSL[name] * 4 + i * 2 + j) * 2 + n], (), 8 * ((OSL[name] + 2 * j) % 4))

    def jloc(kind, name, al, second=False):
        i = 24 + al if second else (('35', '47', '26').index(kind) * 4 + ('1', 's', 'u', 'v').index(name)) * 2 + al
        return jb[i], (), 8 * ((i + i // 2) % 4)

    def s2loc(p):
        return (s2[2], (2, 6).index(p)) if p in (2, 6) else (s2[p], 0)

    def bias_coefs(p, extra, i, j, n, h):
        where = [(1, i, j, n, h)]
        if extra:
            terms = next(x for _, t in OACT[p][1] + OACT[p][2] for _, x in t if not isinstance(x, str))
        else:
            terms = OACT[p][0]
            w = [(1, i, j)] + [(-1, 0, 1)] * bool(raw_slot(p) and (i, j) == B21)
            where = [x + (n, h) for x in w]
            if (h, n) == (1, 0) and PAIRS[{B12: 0, B11: 1}.get((i, j), 2)] in pairs3[p]:
                where += [(-sg, ii, jj, 1, 0) for sg, ii, jj in w]
        coef = {}
        for sg, ii, jj, nn, hh in where:
            for cf, (I, J) in terms:
                key = (2 * J + jj) * 2 + nn
                coef[key] = coef.get(key, 0.0) + sg * cf * scale(2 * I + ii, 2 * J + jj, hh, nn)
        return coef

    def tie(v, anchor, r=0):
        if anchor is None:
            return v
        return jnp.concatenate([v[:r]] * (r > 0) + [jax.lax.select(anchor[0], anchor[1], v[r:r + 8])] + [v[r + 8:]] * (r + 8 < v.shape[0]), axis=0)

    def consts(anchor, ss, reps):
        one = {s: jnp.full((8, 128), s, f32) for s in set(ss)}
        if anchor is not None:
            one = {s: jax.lax.select(anchor[0], anchor[1], v) for s, v in one.items()}
        return jnp.concatenate([one[s] for s in ss for _ in range(reps)], axis=0)

    def conv(src, zs, R, C, r, nr, anchor=None):
        v = src[R * Mh + r:R * Mh + r + nr, C * H:(C + 1) * H].astype(f32)
        for k in range(2):
            buf, idx, off = xloc(0, R, C, k)
            sv = consts(anchor, [scale(R, C, (r + u) // Mq, k) for u in range(0, nr, 16)], 2)
            buf[(zs,) + idx + (slice(off + r, off + r + nr),)] = v[:, k * 128:(k + 1) * 128] * sv

    def block_sum(l, terms, ii, jj, kk, r, save, zs, za, anchor, at=None):
        rng = lambda t: slice(t[0], t[-1] + 1)
        vals = []
        for u, ((I, J), s) in enumerate(terms):
            r0 = xoff(I, J) + r
            v = xb[xset(l) + I][za if u == 0 else 0, rng(ii), slice(2 * J + jj[0], 2 * J + jj[-1] + 1), rng(kk), r0:r0 + 16, :]
            if (I, J) in save:
                sv = consts(anchor, [1.0 / scale(2 * I + i, 2 * J + j, r // Mq, k) for i in ii for j in jj for k in kk], 2)
                x0b[I * 2 + J][zs, rng(ii), rng(jj), rng(kk), r0 + 8:r0 + 24, :] = v * sv.reshape(v.shape)
            if u == 0 and at is not None and cfg['TIEL'] in (1, 2) and anchor is not None:
                v = tie(v.reshape(v.size // 128, 128), anchor, at + cfg['T8']).reshape(v.shape)
            vals.append((s, v))
        v = lincomb(vals)
        v = v.reshape(v.size // 128, 128)
        if cfg['TIEL'] == 3 and at is not None:
            v = tie(v, anchor, at)
        return v

    def release(qs, store, st8, anchor):
        v = st8['l1']
        if anchor is not None:
            n = v.shape[0]
            top = jax.lax.select(jnp.broadcast_to(anchor[0], (n, 8, 128)), jnp.broadcast_to(anchor[1], (n, 8, 128)), v[:, :8])
            v = jnp.concatenate([top, v[:, 8:]], axis=1)
        r0 = 16 * qs.index(1)
        store(slice(r0, r0 + 16), v.astype(bf16))

    def finish(e, f, group, qs, store, st8, anchor, hold=False):
        if not cfg['TIEL']:
            e = tie(e, anchor)
        a = e[None] if f is None else jnp.concatenate([e + f, e - f], axis=0).reshape(2, e.shape[0], 128)
        for u, b in enumerate(group):
            st8[b] = a if len(group) == 1 else a[:, 16 * u:16 * u + 16]
        ops = {}
        if B12 in group and 3 in qs:
            ops[3], ops[5] = st8[B11] - st8[B12], st8[B11] + st8[B12]
        if B22 in group:
            if 4 in qs:
                ops[4], ops[7] = st8[B12] + st8[B22], st8[B12] - st8[B22]
            ops[1] = st8['l1'] = st8[B11] + st8[B22]
        if B21 in group:
            g = st8[B12] + st8[B21]
            ops[2], ops[6] = g + st8['l1'], g - st8['l1']
        now = [q for q in qs if q in ops and not (hold and q == 1)]
        if now:
            r0 = 16 * qs.index(now[0])
            store(slice(r0, r0 + 16 * len(now)), jnp.concatenate([ops[q] for q in now], axis=1).astype(bf16))

    def unit2(l, ps, c, k, save, st8, group, zs, za, anchor):
        def store(rows, v):
            s2[ps[0]][zs, :, k, c, rows, :] = v
        if group == ('l1',):
            return release(q2[ps[0]], store, st8, anchor)
        hold, group = 'hold' in group, tuple(b for b in group if b != 'hold')
        ii, jj = sorted({b[0] for b in group}), sorted({b[1] for b in group})
        bs = lambda terms, at: block_sum(l, terms, ii, jj, [k], 16 * c, save, zs, za, anchor, at)
        at = 16 * (len(group) > 1)
        e, f = (bs(LA[ps[0]], at), None) if len(ps) == 1 else (bs([(B12, 1), (B21, 1)], at), bs([(B11, 1), (B22, 1)], None))
        finish(e, f, group, q2[ps[0]], store, st8, anchor, hold)

    def unit3(l, p, qs, c, save, st8, group, zs, za, anchor):
        def store(rows, w):
            s3[(p, qs)][zs, :, c, rows, :] = w
        if group == ('l1',):
            return release(ORD, store, st8, anchor)
        hold, group = 'hold' in group, tuple(b for b in group if b != 'hold')
        for h in sorted({b[0] for b in group}):
            grp = tuple(b for b in group if b[0] == h)
            kk = [b[1] for b in grp]
            ii, jj = {(5, 3): ([0], [0, 1]), (4, 7): ([0, 1], [1]), (2, 6): ([0, 1], [0, 1])}[qs]
            v = block_sum(l, LA[p], ii, jj, sorted(kk), h * Mq + 16 * c, save, zs, za, anchor,
                          16 * (len(kk) > 1 or (qs == (2, 6) and not cfg['TF'])))
            n = 16 * len(kk)
            piece = lambda u: v[u * n:(u + 1) * n]
            if qs == (2, 6):
                e, f = piece(1) + piece(2), piece(0) + piece(3)
                r0 = 16 * q2[p].index(1)
                s2[p][zs, 0, min(kk):max(kk) + 1, h * NQ + c, r0:r0 + 16, :] = f.reshape(len(kk), 16, 128).astype(bf16)
            else:
                e, f = piece(0), piece(1)
            finish(e, f, tuple(sorted(grp)), ORD, store, st8, anchor, hold)

    def prep(l, u, anchors, zero, kb):
        for k in range(2):
            wide = [w_ref[l, R * 2 + k, u].astype(f32) for R in range(4)]
            for n in range(2):
                def blk(R, C):
                    v = wide[R][:, C * H + n * 128:C * H + (n + 1) * 128]
                    s = D2[R // 2] / D2[C // 2]
                    return v if s == 1.0 else v * s
                O = {(i, j): b_ops(blk(i, j), blk(i, 2 + j), blk(2 + i, j), blk(2 + i, 2 + j)) for i, j in (B11, B12, B21, B22)}
                for p in PREP_ORDER:
                    anchor = next(anchors)
                    s = BF[p] * 0.5 * D2[k] / D2[n]
                    cs = {f: consts(anchor, [s * f], 2) for f in (0.5, 1.0, 2.0)}
                    T = b_ops(*[O[(i, j)][p] * cs[D2[i] / D2[j]] for i, j in (B11, B12, B21, B22)])
                    T[1] = T[1] + T[1]
                    t2[p][l, n, k * 8 + u] = jnp.concatenate([T[q] for q in q2[p]], axis=0).astype(bf16)
                    mine = [e for e, pq in enumerate(prods3) if pq[0] == p]
                    if mine:
                        kb[zero, k * 2 + n, 16 * mine[0]:16 * mine[-1] + 16, :] = jnp.concatenate(
                            [T[prods3[e][1]] for e in mine], axis=0)
        for e in range(len(prods3)):
            v = kb[0, :, 16 * e:16 * e + 16, :] * consts(next(anchors), [0.5], 2)
            T = b_ops(v[0], v[1], v[2], v[3])
            T[1] = T[1] + T[1]
            t3_ref[l, e, u] = jnp.concatenate([T[q] for q in ORD], axis=0).astype(bf16)

    def rounds_of(p):
        rs = [('1', None)] + [('x', '1')] * (p in SEL)
        for kind, qs in zip(('35', '47', '26'), PAIRS):
            if kind == '26' and p in SEL3[::2]:
                rs.append(('y', '1'))
            rs += [(kind, r) for r in (('35', '47', '26') if qs in pairs3[p] else (0, 1))]
        return rs

    outs = [(l, p) for l in range(L) for p in OUTER]
    G = len(outs)
    sched, start, use = [], [], []
    for g, (l, p) in enumerate(outs):
        start.append(len(use))
        for rd in rounds_of(p):
            n = NQ if isinstance(rd[1], str) else NC
            sched.append((g, rd, len(use), n))
            a, st_, ld_ = round_usage(p, rd, l == 0, l == L - 1, cfg['DEFER'], cfg['HY'])
            if cfg['PORT']:
                use += [max((2 * a + st_ + 2 + 16 / n) / 72 + cfg['PS'] * st_ / 8, cfg['PORT'] * st_ / 8)] * n
            else:
                use += [max(a / 32, st_ / 8, cfg['UL'] * ld_ / 24)] * n
    T = len(use)
    cap = [max(cfg['CAP'] - max(use[t], use[(t + 1) % T]), 0.0) * (t < T - cfg['TAIL']) for t in range(T)]
    for g in range(G):
        for t in range(start[g], (start + [T])[g + 1]):
            cap[t] *= cfg['CM'][g % 7]
    jobs = []
    def add(lo, hi, alu, st_, ld_, nst, l, fn):
        w = alu / 64 + cfg['CS'] * (st_ + nst) / 16 + cfg['CL'] * ld_ / 48
        w *= cfg['KW'][0 if l in (None, 'fin') else nst]
        if cfg['HOLD'] and nst >= 3:
            nst += 2
        jobs.append((lo, max(hi, lo), [w * f for f in cfg['FR'][nst - 1]], l, fn, nst))
    for g, (l, p) in enumerate(outs):
        ready = 7 * l - 2 * all(I == 0 for (I, J), _ in LA[p])
        lo = start[ready] - (T if ready < 0 else 0)
        if 7 in SEL3 and cfg['DEFER'] and ready % 7 == 5 and l > 0:
            lo += cfg['EW'] + 1
        if p in SEL3 and OACT[p][2]:
            for h, n in [(0, 1)] * ('35' in cfg['DEFER']) + [(0, 0)] * ('47' in cfg['DEFER']) + [(1, 1), (1, 0)] * ('26' in cfg['DEFER']):
                for c in range(0, NQ):
                    e0 = start[g + 1]
                    add(e0, e0 + cfg['EW'] if p == 7 else start[7 * l + 5] - 1, 20 + 8 * (l == L - 1), 3, 20, 1, 'fin',
                        (l, p, n, h * Mq + 16 * c))
        hi = start[g] - LAG - 3
        nt = len(LA[p])
        save = [b for b, pp in cfg['XC'].items() if pp == p and l == 0]
        if p in SEL3:
            if p in SEL3[1::2]:
                host = 7 * l + OUTER.index(SEL3[SEL3.index(p) - 1])
                hi = [t0 for gg, rd, t0, _ in sched if gg == host and rd[0] == 'y'][0] - LAG - 3
            for c in range(NQ):
                add(lo, hi, 32 * nt + 50 + 32 * len(save), 18 + 32 * len(save), 32 * nt, 4, l,
                    functools.partial(unit3, l, p, (2, 6), c, save))
        elif p != 6:
            ps = (2, 6) if p == 2 else (p,)
            nq = len(q2[p]) * len(ps)
            alu = 8 * (nt - 2 + len(ps)) + (8 if p in SEL else 16) * len(ps) + nq
            for c in range(NC):
                for k in range(2):
                    add(lo, hi, alu + 8 * len(save), nq + 8 * len(save), 8 * nt, 1 if nq <= 3 else 2 if nq <= 7 else 3, l,
                        functools.partial(unit2, l, ps, c, k, save))
        if p in SEL:
            for qs, c in ([(qs, c) for qs in PAIRS[:2] for c in range(NQ)] if cfg['QO'] else
                          [(qs, c) for c in range(NQ) for qs in PAIRS[:2]]):
                if True:
                    add(lo, start[g] - LAG - 3 + (NC if g else 0), 16 * nt + 46, 14, 16 * nt, 3, l,
                        functools.partial(unit3, l, p, qs, c, []))
    for R in range(4):
        for C in range(4):
            for c in range(0, NC, 2):
                add(start[6], start[G - 2] - 2, 18, 7, 4, 1, None, (R, C, 16 * c))
    when = spread_jobs([j[:3] for j in jobs], cap, cfg['TAIL'])
    evs = [e[:1] + e[2:] for e in sorted((t % T, ts[0] % T, ji, u) for ji, ts in enumerate(when) for u, t in enumerate(ts))]
    half = {}
    for e, (t, ji, u) in enumerate(evs):
        half[(ji, u)] = 2 * t + (0 if e + 1 < len(evs) and evs[e + 1][0] == t and (e == 0 or evs[e - 1][0] != t) else 1)
    SEG = cfg['SEG']
    for sg, seeds in enumerate(cfg['SEEDS']):
        mine = [e for e, ev in enumerate(evs) if ev[0] // SEG == sg]
        for seed in seeds:
            for e in mine:
                _, ji, u = evs[e]
                r = (e * 2654435761 + seed * 97531 + 12345) * 2246822519 % 4294967296 >> 8
                if r % 100 >= cfg['PJ']:
                    continue
                h = half[(ji, u)] + (2, -2, 1, -1, 2, -2)[r // 100 % 6]
                off = when[ji][u] - when[ji][u] % T
                lo_ = max(2 * (jobs[ji][0] - off), 2 * sg * SEG, half[evs[e - 1][1:]] + 1 if e else 0)
                hi_ = min(2 * (jobs[ji][1] - off) + 1, 2 * (sg + 1) * SEG - 1,
                          half[evs[e + 1][1:]] - 1 if e + 1 < len(evs) else 2 * (T - cfg['TAIL']))
                if lo_ <= h <= hi_:
                    half[(ji, u)] = h
    if cfg.get('SHOW'):
        for g in range(7, 14):
            rg = range(start[g], start[g + 1])
            print('  ', ''.join('%2d' % round(10 * use[t]) for t in rg))
            print('  ', ''.join('%2s' % ''.join((str(len(w)) if u == 0 else '.') for w in when for u, x in enumerate(w) if x % T == t) for t in rg))
    plan = {}
    for _, ji, u in evs:
        plan.setdefault(half[(ji, u)] // 2, []).append((half[(ji, u)] % 2, jobs[ji][3], jobs[ji][4], STAGES[jobs[ji][5]][u]))
    if cfg.get('PLANOUT') is not None:
        kind = lambda j: 'conv' if j[3] is None else 'fin' if j[3] == 'fin' else j[4].func.__name__ + str(j[4].args[1] if j[4].func.__name__ == 'unit2' else j[4].args[2])
        cfg['PLANOUT'].update(ev=[(half[(ji, u)], kind(jobs[ji]), u, jobs[ji][2][u]) for _, ji, u in evs], use=use,
                              rd=[(outs[g][1], str(rd)) for g, rd, t0, n in sched for _ in range(n)])
    assert all((ts[0] < 0) == (ts[-1] < 0) for ts in when)
    carried = [(job[4], job[5]) for ts, job in zip(when, jobs) if ts[0] < 0]

    def w_copy(l):
        return pltpu.make_async_copy(w_hbm.at[l], w_ref.at[l], sem.at[l])

    def w0_copy(u):
        return pltpu.make_async_copy(w_hbm.at[0, :, u], w_ref.at[0, :, u], sem.at[L + 10 + u])

    def in_copy(t, slot):
        return pltpu.make_async_copy(x_hbm.at[pl.ds(pl.multiple_of(t * TM, 32), TM)], xn2_ref.at[slot], sem.at[L + slot])

    def out_copy(t, slot, part):
        r0, nr = ((0, 2 * Mh), (2 * Mh, Mh), (3 * Mh, Mh))[part]
        return pltpu.make_async_copy(o2_ref.at[slot, pl.ds(r0, nr)],
                                     o_hbm.at[pl.ds(pl.multiple_of(t * TM + r0, 32), nr)],
                                     sem.at[L + 4 + 3 * slot + part])

    xr_in = pltpu.make_async_copy(x_hbm.at[pl.ds(NMAIN * TM, R0)], xr_ref, sem.at[L + 2])
    xr_out = pltpu.make_async_copy(xr_ref, o_hbm.at[pl.ds(NMAIN * TM, R0)], sem.at[L + 2])
    b_in = pltpu.make_async_copy(b_hbm, b_ref, sem.at[L + 3])

    def prologue():
        b_in.start()
        for u in range(8):
            w0_copy(u).start()
        xr_in.start()
        in_copy(0, 0).start()
        for l in range(1, L):
            w_copy(l).start()
        in_copy(min(1, NMAIN - 1), 1).start()
        b_in.wait()
        for l in range(L):
            bf_ref[l] = b_ref[l:l + 1, :].astype(f32)

        def bias_tiles(l, carry):
            b = jnp.broadcast_to(bf_ref[l] + (l == 0).astype(f32), (8, D))
            for u, site in enumerate(BIAS):
                terms = [b[:, key * 128:(key + 1) * 128] * cf for key, cf in sorted(bias_coefs(*site).items()) if cf != 0.0]
                bt_ref[l, u] = functools.reduce(lambda x, y: x + y, terms)
            return carry
        jax.lax.fori_loop(0, L, bias_tiles, 0)
        if cfg.get('FAST'):
            return

        def slab(u, carry):
            w0_copy(u).wait()
            zero = jax.lax.shift_right_logical(u, 12)
            prep(0, u, iter(lambda: None, 0), zero, kb0)
            return zero
        zero = jax.lax.fori_loop(0, cfg['NSLAB'], slab, 0)

        def plain(l, xbf, x0f, x, na, free, never, j0=0, j1=D // 128):
            passes = []
            for jt in range(j0, j1):
                cols = slice(jt * 128, (jt + 1) * 128)
                ya = _dot(xbf[:, :D // 2], w_ref[l, 0:4, :, :, cols].reshape(D // 2, 128)) + bf_ref[l, :, cols]
                passes += [ya, _dot(xbf[:, D // 2:], w_ref[l, 4:8, :, :, cols].reshape(D // 2, 128)) + ya]
            xp_ref[0, :, j0 * 128:j1 * 128] = x0f * jnp.concatenate(passes[1::2], axis=1) + x
            for u in range(na):
                ps, rr = divmod((u - free) * len(passes) * (R0 // 8) // (na - free), R0 // 8)
                yield None if u < free else (never, passes[ps][rr * 8:rr * 8 + 8, :])

        for u in range(cfg['NSLAB'], 8):
            w0_copy(u).wait()
        xr_in.wait()
        never = jnp.broadcast_to(zero, (8, 128)) != 0
        jm = cfg['JM']
        x0f = xr_ref[:, :jm * 128].astype(f32)
        xp_ref[1, :, :jm * 128] = x0f
        anchors = plain(0, xr_ref[...], x0f, x0f, (8 - cfg['NSLAB']) * (28 + len(prods3)), cfg['AFREE'], never, 0, jm)
        for u in range(cfg['NSLAB'], 8):
            prep(0, u, anchors, zero, (kb0, kb1)[u % 2])
        in_copy(0, 0).wait()
        x0f = xr_ref[:, jm * 128:].astype(f32)
        xp_ref[1, :, jm * 128:] = x0f
        units = [(R, C, r) for R in range(4) for C in range(4) for r in range(0, Mh, 32)]
        anchors = plain(0, xr_ref[...], x0f, x0f, len(units) + sum(len(STAGES[n]) for _, n in carried) + 2, 4, never, jm)
        for R, C, r in units[:len(units) // 2]:
            conv(xn2_ref.at[0], zero, R, C, r, min(32, Mh - r), next(anchors))
        for fn, n in carried:
            st8 = {}
            for group in STAGES[n]:
                anchor = next(anchors)
                xb[xset(0)][0, 0, 0, 0, Mh + 24:Mh + 32, :] = anchor[1]
                fn(st8, group, zero, jax.lax.shift_right_logical(zero, 1), anchor)
        for R, C, r in units[len(units) // 2:]:
            conv(xn2_ref.at[0], zero, R, C, r, min(32, Mh - r), next(anchors))

        def layer(l, carry):
            w_copy(l).wait()
            zero = jax.lax.shift_right_logical(l, 12)
            x = xp_ref[0]
            anchors = plain(l, x.astype(bf16), xp_ref[1], x, 8 * (28 + len(prods3)), cfg['AFREE'],
                            jnp.broadcast_to(zero, (8, 128)) != 0)
            for u in range(8):
                prep(l, u, anchors, zero, (kb0, kb1)[u % 2])
            return carry

        jax.lax.fori_loop(1, L, layer, 0)
        xr_ref[...] = xp_ref[0].astype(bf16)
        xr_out.start()

    def main(tile, carry):
        zs, za = jax.lax.shift_right_logical(tile, 12), jax.lax.shift_right_logical(tile, 13)
        never = jnp.broadcast_to(zs, (8, 128)) != 0
        slot = tile % 2
        in_copy(jnp.minimum(tile + 2, NMAIN - 1), slot).start()
        in_copy(jnp.minimum(tile + 1, NMAIN - 1), 1 - slot).wait()

        @pl.when(tile > 1)
        def _():
            for part in range(3):
                out_copy(tile - 2, slot, part).wait()

        xn_ref = xn2_ref.at[1 - slot]
        o_ref = o2_ref.at[slot]
        def rows(h, r0):
            if isinstance(h, tuple):
                return slice(r0 + h[0], r0 + h[0] + h[1])
            return slice(r0, r0 + Mh) if h is None else slice(r0 + h * Mq, r0 + (h + 1) * Mq)

        def ld(loc, h=None, z=0):
            return loc[0][(z,) + loc[1] + (rows(h, loc[2]),)]

        def st(loc, v, h=None):
            loc[0][(za if h == 1 and not loc[1] and cfg['ZB'] else zs,) + loc[1] + (rows(h, loc[2]),)] = v

        def by_half(v, h, fn):
            if isinstance(h, tuple):
                h = h[0] // Mq
            return fn(v, h) if h is not None else jnp.concatenate([fn(v[:Mq], 0), fn(v[Mq:], 1)], axis=0)

        def gather(ref, idx, n, pos):
            if cfg['NOBC']:
                return ref[idx + (slice(0, n), slice(16 * pos, 16 * pos + 16))].reshape(16 * n, 128)
            return ref.bitcast(u32)[idx + (slice(0, n), slice(8 * pos, 8 * pos + 8))].reshape(8 * n, 128)

        as_bf16 = lambda v: v if cfg['NOBC'] else pltpu.bitcast(v, bf16)

        def lhs2(p, q):
            ref, u = s2loc(p)
            return as_bf16(jnp.concatenate([gather(ref, (0, u, k), NC, q2[p].index(q)) for k in range(2)], axis=1))

        def rhs2(l, p, q, n):
            return as_bf16(gather(t2[p], (l, n), 16, q2[p].index(q)))

        def dot3(l, p, q, r):
            qs = next(qs for qs in PAIRS if q in qs)
            return _dot(as_bf16(gather(s3[(p, qs)], (0, qs.index(q)), NQ, ORD.index(r))),
                        as_bf16(gather(t3_ref, (l, prods3.index((p, q))), 8, ORD.index(r))))

        def add_bias(v, l, site, h):
            def one(x, hh):
                b = bt_ref[l, BIAS.index(site + (hh,))]
                return (x.reshape(Mq // 8, 8, 128) + b).reshape(Mq, 128)
            return by_half(v, h, one)

        def outer_act(l, p, i, j, n, d, h, part=None):
            bt, stores, finals = OACT[p]
            if part == 'stores':
                finals = []
            if part == 'finals':
                bt, stores = [], []
            if bt:
                d = add_bias(d, l, (p, False, i, j, n), h)
            cache = {'d': d}
            def comb(terms):
                for _, src in terms:
                    if isinstance(src, str) and src not in cache:
                        cache[src] = ld(oloc(src, i, j, n), h)
                v = lincomb([(s, cache[src]) for s, src in terms if isinstance(src, str)])
                for _, src in terms:
                    if not isinstance(src, str):
                        v = add_bias(v, l, (p, True, i, j, n), h)
                return v
            fin = [(IJ, comb(terms)) for IJ, terms in finals]
            for name, v in [(name, comb(terms)) for name, terms in stores]:
                st(oloc(name, i, j, n), v, h)
            for (I, J), y in fin:
                R, C = 2 * I + i, 2 * J + j
                xn = ld(x0loc(R, C, n), h) * y
                if l > 0:
                    xn = xn + ld(xloc(l, R, C, n), h)
                if l < L - 1:
                    st(xloc(l + 1, R, C, n), xn, h)
                else:
                    xn = by_half(xn, h, lambda x, hh: x if scale(R, C, hh, n) == 1.0 else x * (1.0 / scale(R, C, hh, n)))
                    o_ref[rows(h, R * Mh), C * H + n * 128:C * H + (n + 1) * 128] = xn.astype(bf16)

        def inner_act(g, l, p, kind, n, h, P, Q, part=None):
            vloc = oloc(raw_slot(p), 0, 1, n) if raw_slot(p) else iloc(g, 'v', n)
            if kind == '35':
                st(iloc(g, 's', n), Q + ld(iloc(g, 'm1', n), h), h)
                if not raw_slot(p):
                    st(vloc, P, h)
                outer_act(l, p, 0, 1, n, P, h)
            elif kind == '47':
                st(iloc(g, 'u', n), Q + ld(vloc, h), h)
                outer_act(l, p, 0, 0, n, P + ld(iloc(g, 's', n), h), h)
            else:
                outer_act(l, p, 1, 1, n, ld(iloc(g, 's', n), h) - Q, h, part)
                outer_act(l, p, 1, 0, n, P + ld(iloc(g, 'u', n), h), h, part)

        def issue(l, p, rd):
            kind, n = rd
            if kind == 'x':
                return [dot3(l, p, q, 1) for q in (3, 5, 4, 7)]
            if kind == 'y':
                return [dot3(l, pp, q, 1) for pp in (p, SEL3[SEL3.index(p) + 1]) for q in (2, 6)]
            if isinstance(n, str):
                return [dot3(l, p, int(q), int(r)) for r in n for q in kind]
            if kind == '1':
                lhs = lhs2(p, 1)
                return [_dot(lhs, rhs2(l, p, 1, 0)), _dot(lhs, rhs2(l, p, 1, 1))]
            return [_dot(lhs2(p, int(q)), rhs2(l, p, int(q), n)) for q in kind]

        def consume(g, l, p, rd, res):
            kind, n = rd
            if n == '1':
                for u, where in enumerate((('35', False), ('47', False)) if kind == 'x' else (('26', False), ('26', True))):
                    for al in range(2):
                        st(jloc(where[0], '1', al, where[1]), res[2 * u + al], 0)
            elif isinstance(n, str):
                sm = [res[al] + res[2 + al] for al in range(2)]
                df = [res[al] - res[2 + al] for al in range(2)]
                J = lambda name, al: ld(jloc(kind, name, al, name == '1' and kind == '26' and p in SEL3[1::2]), 0)
                part = 'stores' if n in cfg['DEFER'] else None
                done = lambda h, nn, m: inner_act(g, l, p, kind, nn, h, m[0] + m[1], m[0] - m[1], part)
                O, I = (lambda i, j: oloc(raw_slot(p), i, j, 1)), (lambda name: iloc(g, name, 1))
                rec = lambda al: [(s, ld(loc, 0, za if cfg['ZB'] else 0)) for s, loc in {
                    '35': [[(1, O(0, 1))], [(1, I('s')), (-1, I('m1'))]],
                    '47': [[(1, O(0, 0)), (-1, I('s'))], [(1, I('u')), (-1, O(0, 1))]],
                    '26': [[(1, O(1, 0)), (-1, I('u'))], [(1, I('s')), (-1, O(1, 1))]]}[kind][al]]
                if n == '35':
                    for al in range(2):
                        st(jloc(kind, 's', al), df[al] + J('1', al), 0)
                    done(0, 1, sm)
                elif n == '47':
                    if cfg['HY'] == 1:
                        for al in range(2):
                            st(jloc(kind, 'u', al), df[al], 0)
                    else:
                        for al, v in enumerate((df[0] + df[1], df[0] - df[1])):
                            st(jloc(kind, 'u', al), lincomb([(1, v)] + rec(al)), 0)
                    done(0, 0, [sm[al] + J('s', al) for al in range(2)])
                else:
                    if cfg['HY'] == 1:
                        m = [sm[al] + J('u', al) for al in range(2)]
                        P, Q = lincomb([(1, m[0] + m[1])] + rec(0)), lincomb([(1, m[0] - m[1])] + rec(1))
                    else:
                        P, Q = (sm[0] + sm[1]) + J('u', 0), (sm[0] - sm[1]) + J('u', 1)
                    done(1, 1, [J('s', al) - df[al] for al in range(2)])
                    inner_act(g, l, p, kind, 0, 1, P, Q, part)
            elif kind == '1':
                st(iloc(g, 'm1', 0), res[0])
                st(iloc(g, 'm1', 1), res[1])
            else:
                inner_act(g, l, p, kind, n, None, res[0] + res[1], res[0] - res[1])

        state = {}
        for g, rd, t0, n in sched:
            l, p = outs[g]
            if t0 == start[G - 1]:
                out_copy(tile, slot, 0).start()
            if t0 + n == T:
                out_copy(tile, slot, 1).start()
            res = issue(l, p, rd)
            for t in range(t0, t0 + n):
                for ph, l2, fn, group in plan.get(t, []):
                    gr = 16 * (t - t0) + 8 * ph
                    gate = res[0][gr:gr + 8, :]
                    if cfg['GADD'] and isinstance(rd[1], str) and rd[1] != '1':
                        gate = gate + res[2][gr:gr + 8, :]
                    if l2 == 'fin':
                        lf, pf, nf, r0 = fn
                        for j in range(2):
                            d = ld(oloc(raw_slot(pf), 1, j, nf), (r0, 16))
                            d = tie(tie(d, (never, gate)), (never, gate), 8)
                            outer_act(lf, pf, 1, j, nf, d, (r0, 16), 'finals')
                    elif l2 is None:
                        conv(xn_ref, zs, *fn, min(32, Mh - fn[2]), (never, gate))
                    else:
                        if group != ('l1',):
                            xb[xset(l2)][0, 0, 0, 0, Mh + 24:Mh + 32, :] = gate
                        fn(state.setdefault(id(fn), {}), group, zs, za, (never, gate))
            consume(g, l, p, rd, res)
        out_copy(tile, slot, 2).start()
        return carry

    prologue()
    jax.lax.fori_loop(0, NMAIN, main, 0)
    xr_out.wait()
    in_copy(NMAIN - 1, (NMAIN - 1) % 2).wait()
    for t in range(max(NMAIN - 2, 0), NMAIN):
        for part in range(3):
            out_copy(t, t % 2, part).wait()


DEFAULT = dict(SEL=(3, 5, 4, 7), SEL3=(3, 5, 4, 7), XC={B12: 5, B11: 1, B22: 7, B21: 2}, AFREE=4, NOBC=0, ZB=0, HY=1, HOLD=0, PORT=0.9, PS=0, NSLAB=5, JM=4, XP=40, XO=16, DEFER=('26',), EW=12, KW=(1,) * 5, CM=(1,) * 7, SEEDS=(), SEG=32, PJ=20, QO=0, TIEL=3, GADD=1, TF=0, T8=0, TAIL=6,
               CS=0.5, CL=0.3, UL=0.8, CAP=0.85, FR=((1.,), (.4, .6), (.35, .37, .28), (.16, .26, .31, .27),
                   (.35, .29, .08, .28), (.16, .26, .26, .05, .27)))


def build(TM=640, **kw):
    def f(x0, ws, bs):
        B, D = x0.shape
        L = ws.shape[0]
        cfg = dict(DEFAULT, **kw)
        Mh = TM // 4
        MP = Mh + 32
        nmain = (B - 1) // TM
        R0 = B - nmain * TM
        pairs3, q2 = layout(cfg)
        n3 = sum(2 * len(v) for v in pairs3.values())
        pad = lambda n: n + (2 - n) % 4
        V = pltpu.VMEM
        half = V((1, MP, 128), f32)
        XP = Mh + cfg['XP']
        scratch = ([V((1, 2, 2, 2, XP, 128), f32)] * 4 + [V((1, 2, 4, 2, XP, 128), f32)] * 6 + [half] * (16 + 56 + 26)
                   + [V((1, 1 + (p == 2), 2, pad(Mh // 16), 16 * len(q2[p]), 128), bf16) for p in (1, 3, 4, 5, 7, 2)]
                   + [V((1, 2, pad(Mh // 32), 112, 128), bf16)] * (n3 // 2)
                   + [V((L, 2, 16, 16 * len(q2[p]), 128), bf16) for p in range(1, 8)]
                   + [V((L, n3, 8, 112, 128), bf16), V((1, 4, 16 * n3, 128), f32), V((1, 4, 16 * n3, 128), f32),
                      V((L, len(BIAS), 8, 128), f32), V((8, 1, D), f32), V((2, TM, D), bf16), V((2, TM, D), bf16), V((L, 8, 8, 16, D), bf16),
                      V((R0, D), bf16), V((2, R0, D), f32), V((L, D), bf16), pltpu.SemaphoreType.DMA((L + 18,))])
        anyspec = pl.BlockSpec(memory_space=pl.ANY)
        return pl.pallas_call(
            functools.partial(_kernel, L=L, TM=TM, R0=R0, NMAIN=nmain, D=D, cfg=cfg),
            in_specs=[anyspec, anyspec, anyspec],
            out_specs=anyspec,
            out_shape=jax.ShapeDtypeStruct((B, D), x0.dtype),
            scratch_shapes=scratch,
            compiler_params=pltpu.CompilerParams(
                vmem_limit_bytes=110 * 1024 * 1024,
                internal_scratch_in_bytes=65536,
                disable_bounds_checks=True,
            ),
        )(x0, ws.reshape(L, 8, 8, 16, D), bs)
    return f


@jax.jit
def pallas_standalone__dcn_v2_cross__recsys_kernel(x0, ws, bs):
    return build(TM=640)(x0, ws, bs)
```

```python
import functools

import jax
import jax.numpy as jnp
import jax.experimental.pallas as pl
import jax.experimental.pallas.tpu as pltpu

f32 = jnp.float32
bf16 = jnp.bfloat16
u32 = jnp.uint32

B11, B12, B21, B22 = (0, 0), (0, 1), (1, 0), (1, 1)
LA = {1: [(B11, 1), (B22, 1)], 2: [(B11, 1), (B12, 1), (B21, 1), (B22, 1)], 3: [(B11, 1), (B12, -1)],
      4: [(B12, 1), (B22, 1)], 5: [(B11, 1), (B12, 1)], 6: [(B12, 1), (B11, -1), (B21, 1), (B22, -1)],
      7: [(B12, 1), (B22, -1)]}
PAIRS = ((5, 3), (4, 7), (2, 6))
ORD = (3, 5, 4, 7, 1, 2, 6)
D2 = (1.0, 2.0)
BF = {1: 1.0, 2: 0.5, 3: 0.5, 4: 0.5, 5: 0.5, 6: 0.5, 7: 0.5}
OUTER = (3, 5, 1, 4, 7, 2, 6)
OACT = {
    3: ([(1, B12)], [('M3', [(1, 'd')])], []),
    5: ([], [('M5', [(1, 'd')])], [(B12, [(1, 'd'), (1, 'M3')])]),
    1: ([(1, B11), (-1, B12)], [('S', [(1, 'd'), (1, 'M3'), (-1, 'M5')])], []),
    4: ([], [('M4', [(1, 'd')])], []),
    7: ([], [('M7', [(1, 'd')])], [(B11, [(1, 'd'), (1, 'S'), (1, 'M4')])]),
    2: ([(1, B11), (-1, B22)], [('M2', [(1, 'd')]),
        ('U', [(1, 'd'), (1, 'M4'), (-1, 'M7'), (1, 'M3'), (1, 'M5'), (1, ((1, B21), (-1, B12), (-1, B11), (1, B22)))])], []),
    6: ([], [], [(B22, [(1, 'd'), (1, 'S'), (-1, 'M2')]), (B21, [(1, 'd'), (1, 'U')])]),
}
OSL = {'M3': 0, 'M5': 1, 'S': 2, 'M4': 3, 'M7': 4, 'M2': 6, 'U': 5}
ISL = {'m1': 0, 's': 1, 'v': 2, 'u': 3}
STAGES = {1: [(B11, B12, B21, B22)], 2: [(B11, B12), (B21, B22)], 3: [(B11, B12), (B22,), (B21,)],
          4: [(B11,), (B12,), (B22,), (B21,)], 5: [(B11, B12), (B22, 'hold'), ('l1',), (B21,)],
          6: [(B11,), (B12,), (B22, 'hold'), ('l1',), (B21,)]}
BIAS = [(p, extra, i, j, n, h) for p in OUTER for extra in (False, True)
        if (any(not isinstance(x, str) for _, t in OACT[p][1] + OACT[p][2] for _, x in t) if extra else OACT[p][0])
        for i in range(2) for j in range(2) for n in range(2) for h in range(2)]
PREP_ORDER = (2, 6, 3, 5, 1, 4, 7)
LAG = 8


def _dot(a, b):
    return jnp.dot(a, b, preferred_element_type=f32)


def scale(R, C, h, k):
    return D2[R // 2] * D2[R % 2] * D2[h] / (D2[C // 2] * D2[C % 2] * D2[k])


def b_ops(b11, b12, b21, b22):
    r1 = b11 + b22
    g = b12 + b21
    return {1: r1, 2: b11 - b12, 3: b12 - b22, 4: g - r1, 5: b12 + b22, 6: b11 + b12, 7: g + r1}


def lincomb(terms):
    assert terms[0][0] == 1
    acc = terms[0][1]
    for s, v in terms[1:]:
        acc = acc + v if s == 1 else acc - v
    return acc


def raw_slot(p):
    return next((name for name, terms in OACT[p][1] if terms == [(1, 'd')]), None)


def round_usage(p, rd, first, last, defer, hy):
    bt, stores, finals = OACT[p]
    alu = bool(bt) + sum(len(t) - 1 for _, t in stores) + sum(len(t) + (not first) + 2 * last for _, t in finals)
    nst = len(stores) + len(finals)
    nld = len({x for _, t in stores + finals for _, x in t if isinstance(x, str) and x != 'd'}) + len(finals) * (2 - first)
    kind, n = rd
    if isinstance(n, str):
        e = kind == '47'
        if kind == '26':
            a, st, ld, m = {'35': (10, 2, 9, 2), '47': (10, 2, 9, 2) if hy == 1 else (16, 2, 13, 2), '26': (20, 0, 17, 4) if hy == 1 else (16, 0, 13, 4)}[n]
            if n in defer and finals:
                alu, nst, nld = 0, 1, 0
        else:
            a, st, ld, m = {'1': (0, 4, 5, 0), '35': (9 + e, 3, 8 + e, 1),
                            '47': (9 + e, 3, 8 + e, 1) if hy == 1 else (14 + 2 * e, 3, 11 + 2 * e, 1),
                            '26': (17 + 3 * e, 2, 14 + 3 * e, 2) if hy == 1 else (14 + 2 * e, 2, 11 + 2 * e, 2)}[n]
    else:
        a, st, ld, m = {'1': (2, 2, 4, 0), '35': (5, 2 - bool(raw_slot(p)), 5, 1), '47': (6, 1, 6, 1),
                        '26': (6, 0, 6, 2)}[kind]
    return a + m * alu, st + m * nst, ld + m * nld


def yds(groups, cap):
    n = len(cap)
    speed, cls, gcls = [0.0] * n, [-1] * n, {}
    todo = list(groups)
    while todo:
        pre = [0.0]
        for t in range(n):
            pre.append(pre[-1] + (cap[t] if cls[t] < 0 else 0.0))
        best = None
        for a in sorted({g[0] for g in todo}):
            w = 0.0
            for g in sorted((g for g in todo if g[0] >= a), key=lambda g: g[1]):
                w += g[2]
                d = w / max(pre[g[1] + 1] - pre[a], 1e-9)
                if best is None or d > best[0]:
                    best = (d, a, g[1])
        d, a, b = best
        for t in range(a, b + 1):
            if cls[t] < 0:
                speed[t], cls[t] = d, len(gcls)
        gcls.update({g[:2]: len(gcls) for g in todo if g[0] >= a and g[1] <= b})
        todo = [g for g in todo if not (g[0] >= a and g[1] <= b)]
    return speed, cls, gcls


def spread_jobs(jobs, cap, tail):
    T = len(cap)
    cap3 = cap * 3
    all3 = [(lo + k * T, hi + k * T, ji, k) for k in range(3) for ji, (lo, hi, _) in enumerate(jobs) if lo + k * T >= 0]
    pend = {}
    for j in sorted(all3, key=lambda j: (j[1], j[3], j[2])):
        pend.setdefault(j[:2], []).append(j)
    speed, cls, gcls = yds([w + (sum(sum(jobs[j[2]][2]) for j in q),) for w, q in pend.items()], cap3)
    when = [[] for _ in jobs]
    debt, cur, done = 0.0, None, 0
    for t in range(3 * T):
        while True:
            j = cur
            if j is None:
                rdy = [q[0] for w, q in pend.items() if q and w[0] <= t and (gcls[w] == cls[t] or w[1] <= t)]
                if not rdy:
                    debt = max(debt, 0.0)
                    break
                j = rdy[0]
                nst = len(jobs[j[2]][2])
                if nst > 1 and j[1] > t and (t + tail + 2 * nst) // T != t // T:
                    break
            must = j[1] <= t or (cur is not None and (t + tail + 1) // T != t // T)
            if not must and (cap3[t] == 0.0 or debt > 0.5 * speed[t] * cap3[t]):
                break
            if cur is None:
                pend[j[:2]].pop(0)
                cur, done = j, 0
            debt += jobs[j[2]][2][done]
            if j[3] == 1:
                when[j[2]].append(t - T)
            done += 1
            if done == len(jobs[j[2]][2]):
                cur = None
        debt -= speed[t] * cap3[t]
    return when


def layout(cfg):
    sel, sel3 = cfg['SEL'], cfg['SEL3']
    pairs3 = {p: [qs for qs in PAIRS if p in sel3 or (p in sel and qs != (2, 6))] for p in range(1, 8)}
    q2 = {p: [q for q in ORD if not any(q in qs for qs in pairs3[p])] for p in range(1, 8)}
    return pairs3, q2


def _kernel(x_hbm, w_hbm, b_hbm, o_hbm, *scratch, L, TM, R0, NMAIN, D, cfg):
    H, Mh, Mq = D // 4, TM // 4, TM // 8
    NC, NQ = Mh // 16, Mq // 16
    MP = Mh + 32
    SEL, SEL3 = cfg['SEL'], cfg['SEL3']
    pairs3, q2 = layout(cfg)
    prods3 = [(p, q) for p in SEL for qs in pairs3[p] for q in qs]
    assert H == 256 and L % 2 == 0 and Mq % 16 == 0 and all(raw_slot(p) for p in SEL)
    it = iter(scratch)
    take = lambda n: [next(it) for _ in range(n)]
    x0b, xb, ib, ob, jb = take(4), take(6), take(16), take(56), take(26)
    s2 = dict(zip((1, 3, 4, 5, 7, 2), take(6)))
    s3 = {(p, qs): next(it) for p in SEL for qs in pairs3[p]}
    t2 = dict(zip(range(1, 8), take(7)))
    t3_ref, kb0, kb1, bt_ref, bf_ref, xn2_ref, o2_ref, w_ref, xr_ref, xp_ref, b_ref, sem = it

    xset = lambda l: 4 if l == 0 else (l % 2) * 2
    xoff = lambda I, J: cfg['XO'] * ((I + J) % 2)
    xloc = lambda l, R, C, k: (xb[xset(l) + R // 2], (R % 2, C, k), xoff(R // 2, C // 2))
    x0loc = lambda R, C, k: (x0b[(R // 2) * 2 + C // 2], (R % 2, C % 2, k), 8 + xoff(R // 2, C // 2))
    iloc = lambda g, name, n: (ib[((g % 2) * 4 + ISL[name]) * 2 + n], (), 8 * ISL[name])
    oloc = lambda name, i, j, n: (ob[(OSL[name] * 4 + i * 2 + j) * 2 + n], (), 8 * ((OSL[name] + 2 * j) % 4))

    def jloc(kind, name, al, second=False):
        i = 24 + al if second else (('35', '47', '26').index(kind) * 4 + ('1', 's', 'u', 'v').index(name)) * 2 + al
        return jb[i], (), 8 * ((i + i // 2) % 4)

    def s2loc(p):
        return (s2[2], (2, 6).index(p)) if p in (2, 6) else (s2[p], 0)

    def bias_coefs(p, extra, i, j, n, h):
        where = [(1, i, j, n, h)]
        if extra:
            terms = next(x for _, t in OACT[p][1] + OACT[p][2] for _, x in t if not isinstance(x, str))
        else:
            terms = OACT[p][0]
            w = [(1, i, j)] + [(-1, 0, 1)] * bool(raw_slot(p) and (i, j) == B21)
            where = [x + (n, h) for x in w]
            if (h, n) == (1, 0) and PAIRS[{B12: 0, B11: 1}.get((i, j), 2)] in pairs3[p]:
                where += [(-sg, ii, jj, 1, 0) for sg, ii, jj in w]
        coef = {}
        for sg, ii, jj, nn, hh in where:
            for cf, (I, J) in terms:
                key = (2 * J + jj) * 2 + nn
                coef[key] = coef.get(key, 0.0) + sg * cf * scale(2 * I + ii, 2 * J + jj, hh, nn)
        return coef

    def tie(v, anchor, r=0):
        if anchor is None:
            return v
        return jnp.concatenate([v[:r]] * (r > 0) + [jax.lax.select(anchor[0], anchor[1], v[r:r + 8])] + [v[r + 8:]] * (r + 8 < v.shape[0]), axis=0)

    def consts(anchor, ss, reps):
        one = {s: jnp.full((8, 128), s, f32) for s in set(ss)}
        if anchor is not None:
            one = {s: jax.lax.select(anchor[0], anchor[1], v) for s, v in one.items()}
        return jnp.concatenate([one[s] for s in ss for _ in range(reps)], axis=0)

    def conv(src, zs, R, C, r, nr, anchor=None):
        v = src[R * Mh + r:R * Mh + r + nr, C * H:(C + 1) * H].astype(f32)
        for k in range(2):
            buf, idx, off = xloc(0, R, C, k)
            sv = consts(anchor, [scale(R, C, (r + u) // Mq, k) for u in range(0, nr, 16)], 2)
            buf[(zs,) + idx + (slice(off + r, off + r + nr),)] = v[:, k * 128:(k + 1) * 128] * sv

    def block_sum(l, terms, ii, jj, kk, r, save, zs, za, anchor, at=None):
        rng = lambda t: slice(t[0], t[-1] + 1)
        vals = []
        for u, ((I, J), s) in enumerate(terms):
            r0 = xoff(I, J) + r
            v = xb[xset(l) + I][za if u == 0 else 0, rng(ii), slice(2 * J + jj[0], 2 * J + jj[-1] + 1), rng(kk), r0:r0 + 16, :]
            if (I, J) in save:
                sv = consts(anchor, [1.0 / scale(2 * I + i, 2 * J + j, r // Mq, k) for i in ii for j in jj for k in kk], 2)
                x0b[I * 2 + J][zs, rng(ii), rng(jj), rng(kk), r0 + 8:r0 + 24, :] = v * sv.reshape(v.shape)
            if u == 0 and at is not None and cfg['TIEL'] in (1, 2) and anchor is not None:
                v = tie(v.reshape(v.size // 128, 128), anchor, at + cfg['T8']).reshape(v.shape)
            vals.append((s, v))
        v = lincomb(vals)
        v = v.reshape(v.size // 128, 128)
        if cfg['TIEL'] == 3 and at is not None:
            v = tie(v, anchor, at)
        return v

    def release(qs, store, st8, anchor):
        v = st8['l1']
        if anchor is not None:
            n = v.shape[0]
            top = jax.lax.select(jnp.broadcast_to(anchor[0], (n, 8, 128)), jnp.broadcast_to(anchor[1], (n, 8, 128)), v[:, :8])
            v = jnp.concatenate([top, v[:, 8:]], axis=1)
        r0 = 16 * qs.index(1)
        store(slice(r0, r0 + 16), v.astype(bf16))

    def finish(e, f, group, qs, store, st8, anchor, hold=False):
        if not cfg['TIEL']:
            e = tie(e, anchor)
        a = e[None] if f is None else jnp.concatenate([e + f, e - f], axis=0).reshape(2, e.shape[0], 128)
        for u, b in enumerate(group):
            st8[b] = a if len(group) == 1 else a[:, 16 * u:16 * u + 16]
        ops = {}
        if B12 in group and 3 in qs:
            ops[3], ops[5] = st8[B11] - st8[B12], st8[B11] + st8[B12]
        if B22 in group:
            if 4 in qs:
                ops[4], ops[7] = st8[B12] + st8[B22], st8[B12] - st8[B22]
            ops[1] = st8['l1'] = st8[B11] + st8[B22]
        if B21 in group:
            g = st8[B12] + st8[B21]
            ops[2], ops[6] = g + st8['l1'], g - st8['l1']
        now = [q for q in qs if q in ops and not (hold and q == 1)]
        if now:
            r0 = 16 * qs.index(now[0])
            store(slice(r0, r0 + 16 * len(now)), jnp.concatenate([ops[q] for q in now], axis=1).astype(bf16))

    def unit2(l, ps, c, k, save, st8, group, zs, za, anchor):
        def store(rows, v):
            s2[ps[0]][zs, :, k, c, rows, :] = v
        if group == ('l1',):
            return release(q2[ps[0]], store, st8, anchor)
        hold, group = 'hold' in group, tuple(b for b in group if b != 'hold')
        ii, jj = sorted({b[0] for b in group}), sorted({b[1] for b in group})
        bs = lambda terms, at: block_sum(l, terms, ii, jj, [k], 16 * c, save, zs, za, anchor, at)
        at = 16 * (len(group) > 1)
        e, f = (bs(LA[ps[0]], at), None) if len(ps) == 1 else (bs([(B12, 1), (B21, 1)], at), bs([(B11, 1), (B22, 1)], None))
        finish(e, f, group, q2[ps[0]], store, st8, anchor, hold)

    def unit3(l, p, qs, c, save, st8, group, zs, za, anchor):
        def store(rows, w):
            s3[(p, qs)][zs, :, c, rows, :] = w
        if group == ('l1',):
            return release(ORD, store, st8, anchor)
        hold, group = 'hold' in group, tuple(b for b in group if b != 'hold')
        for h in sorted({b[0] for b in group}):
            grp = tuple(b for b in group if b[0] == h)
            kk = [b[1] for b in grp]
            ii, jj = {(5, 3): ([0], [0, 1]), (4, 7): ([0, 1], [1]), (2, 6): ([0, 1], [0, 1])}[qs]
            v = block_sum(l, LA[p], ii, jj, sorted(kk), h * Mq + 16 * c, save, zs, za, anchor,
                          16 * (len(kk) > 1 or (qs == (2, 6) and not cfg['TF'])))
            n = 16 * len(kk)
            piece = lambda u: v[u * n:(u + 1) * n]
            if qs == (2, 6):
                e, f = piece(1) + piece(2), piece(0) + piece(3)
                r0 = 16 * q2[p].index(1)
                s2[p][zs, 0, min(kk):max(kk) + 1, h * NQ + c, r0:r0 + 16, :] = f.reshape(len(kk), 16, 128).astype(bf16)
            else:
                e, f = piece(0), piece(1)
            finish(e, f, tuple(sorted(grp)), ORD, store, st8, anchor, hold)

    def prep(l, u, anchors, zero, kb):
        for k in range(2):
            wide = [w_ref[l, R * 2 + k, u].astype(f32) for R in range(4)]
            for n in range(2):
                def blk(R, C):
                    v = wide[R][:, C * H + n * 128:C * H + (n + 1) * 128]
                    s = D2[R // 2] / D2[C // 2]
                    return v if s == 1.0 else v * s
                O = {(i, j): b_ops(blk(i, j), blk(i, 2 + j), blk(2 + i, j), blk(2 + i, 2 + j)) for i, j in (B11, B12, B21, B22)}
                for p in PREP_ORDER:
                    anchor = next(anchors)
                    fold = 0.5 if cfg['FOLD'] and p in SEL else 1.0
                    s = BF[p] * 0.5 * D2[k] / D2[n] * fold
                    cs = {f: consts(anchor, [s * f], 2) for f in (0.5, 1.0, 2.0)}
                    T = b_ops(*[O[(i, j)][p] * cs[D2[i] / D2[j]] for i, j in (B11, B12, B21, B22)])
                    sq = {q: 2.0 * BF[q] / fold for q in q2[p]}
                    t2[p][l, n, k * 8 + u] = jnp.concatenate(
                        [T[q] if sq[q] == 1.0 else T[q] * sq[q] for q in q2[p]], axis=0).astype(bf16)
                    mine = [e for e, pq in enumerate(prods3) if pq[0] == p]
                    if mine:
                        kb[zero, k * 2 + n, 16 * mine[0]:16 * mine[-1] + 16, :] = jnp.concatenate(
                            [T[prods3[e][1]] for e in mine], axis=0)
        for e in range(len(prods3)):
            anchor = next(anchors)
            if cfg['FOLD']:
                n3 = 16 * len(prods3)
                if anchor is not None and cfg['FOLD'] > 1:
                    kb[0, 0, n3:n3 + 8, :] = anchor[1]
                    v = kb[jax.lax.shift_right_logical(zero, 1), :, 16 * e:16 * e + 16, :]
                else:
                    v = kb[0, :, 16 * e:16 * e + 16, :]
                T = b_ops(v[0], tie(v[1], anchor), v[2], v[3])
            else:
                v = kb[0, :, 16 * e:16 * e + 16, :] * consts(anchor, [0.5], 2)
                T = b_ops(v[0], v[1], v[2], v[3])
            T[1] = T[1] + T[1]
            t3_ref[l, e, u] = jnp.concatenate([T[q] for q in ORD], axis=0).astype(bf16)

    def rounds_of(p):
        rs = [('1', None)] + [('x', '1')] * (p in SEL)
        for kind, qs in zip(('35', '47', '26'), PAIRS):
            if kind == '26' and p in SEL3[::2]:
                rs.append(('y', '1'))
            rs += [(kind, r) for r in (('35', '47', '26') if qs in pairs3[p] else (0, 1))]
        return rs

    outs = [(l, p) for l in range(L) for p in OUTER]
    G = len(outs)
    sched, start, use = [], [], []
    for g, (l, p) in enumerate(outs):
        start.append(len(use))
        for rd in rounds_of(p):
            n = NQ if isinstance(rd[1], str) else NC
            sched.append((g, rd, len(use), n))
            a, st_, ld_ = round_usage(p, rd, l == 0, l == L - 1, cfg['DEFER'], cfg['HY'])
            if cfg['PORT']:
                use += [max((2 * a + st_ + 2 + 16 / n) / 72 + cfg['PS'] * st_ / 8, cfg['PORT'] * st_ / 8)] * n
            else:
                use += [max(a / 32, st_ / 8, cfg['UL'] * ld_ / 24)] * n
    T = len(use)
    cap = [max(cfg['CAP'] - max(use[t], use[(t + 1) % T]), 0.0) * (t < T - cfg['TAIL']) for t in range(T)]
    for g in range(G):
        for t in range(start[g], (start + [T])[g + 1]):
            cap[t] *= cfg['CM'][g % 7]
    jobs = []
    def add(lo, hi, alu, st_, ld_, nst, l, fn):
        w = alu / 64 + cfg['CS'] * (st_ + nst) / 16 + cfg['CL'] * ld_ / 48
        w *= cfg['KW'][0 if l in (None, 'fin') else nst]
        if cfg['HOLD'] and nst >= 3:
            nst += 2
        jobs.append((lo, max(hi, lo), [w * f for f in cfg['FR'][nst - 1]], l, fn, nst))
    for g, (l, p) in enumerate(outs):
        ready = 7 * l - 2 * all(I == 0 for (I, J), _ in LA[p])
        lo = start[ready] - (T if ready < 0 else 0)
        if 7 in SEL3 and cfg['DEFER'] and ready % 7 == 5 and l > 0:
            lo += cfg['EW'] + 1
        if p in SEL3 and OACT[p][2]:
            for h, n in [(0, 1)] * ('35' in cfg['DEFER']) + [(0, 0)] * ('47' in cfg['DEFER']) + [(1, 1), (1, 0)] * ('26' in cfg['DEFER']):
                for c in range(0, NQ):
                    e0 = start[g + 1]
                    add(e0, e0 + cfg['EW'] if p == 7 else start[7 * l + 5] - 1, 20 + 8 * (l == L - 1), 3, 20, 1, 'fin',
                        (l, p, n, h * Mq + 16 * c))
        hi = start[g] - LAG - 3
        nt = len(LA[p])
        save = [b for b, pp in cfg['XC'].items() if pp == p and l == 0]
        if p in SEL3:
            if p in SEL3[1::2]:
                host = 7 * l + OUTER.index(SEL3[SEL3.index(p) - 1])
                hi = [t0 for gg, rd, t0, _ in sched if gg == host and rd[0] == 'y'][0] - LAG - 3
            for c in range(NQ):
                add(lo, hi, 32 * nt + 50 + 32 * len(save), 18 + 32 * len(save), 32 * nt, 4, l,
                    functools.partial(unit3, l, p, (2, 6), c, save))
        elif p != 6:
            ps = (2, 6) if p == 2 else (p,)
            nq = len(q2[p]) * len(ps)
            alu = 8 * (nt - 2 + len(ps)) + (8 if p in SEL else 16) * len(ps) + nq
            for c in range(NC):
                for k in range(2):
                    add(lo, hi, alu + 8 * len(save), nq + 8 * len(save), 8 * nt, 1 if nq <= 3 else 2 if nq <= 7 else 3, l,
                        functools.partial(unit2, l, ps, c, k, save))
        if p in SEL:
            for qs, c in ([(qs, c) for qs in PAIRS[:2] for c in range(NQ)] if cfg['QO'] else
                          [(qs, c) for c in range(NQ) for qs in PAIRS[:2]]):
                if True:
                    add(lo, start[g] - LAG - 3 + (NC if g else 0), 16 * nt + 46, 14, 16 * nt, 3, l,
                        functools.partial(unit3, l, p, qs, c, []))
    for R in range(4):
        for C in range(4):
            for c in range(0, NC, 2):
                add(start[6], start[G - 2] - 2, 18, 7, 4, 1, None, (R, C, 16 * c))
    when = spread_jobs([j[:3] for j in jobs], cap, cfg['TAIL'])
    evs = [e[:1] + e[2:] for e in sorted((t % T, ts[0] % T, ji, u) for ji, ts in enumerate(when) for u, t in enumerate(ts))]
    half = {}
    for e, (t, ji, u) in enumerate(evs):
        half[(ji, u)] = 2 * t + (0 if cfg['DBL'] and e + 1 < len(evs) and evs[e + 1][0] == t and (e == 0 or evs[e - 1][0] != t) else 1)
    SEG = cfg['SEG']
    for sg, seeds in enumerate(cfg['SEEDS']):
        mine = [e for e, ev in enumerate(evs) if ev[0] // SEG == sg]
        for seed in seeds:
            for e in mine:
                _, ji, u = evs[e]
                r = (e * 2654435761 + seed * 97531 + 12345) * 2246822519 % 4294967296 >> 8
                if r % 100 >= cfg['PJ']:
                    continue
                h = half[(ji, u)] + (2, -2, 1, -1, 2, -2)[r // 100 % 6]
                off = when[ji][u] - when[ji][u] % T
                lo_ = max(2 * (jobs[ji][0] - off), 2 * sg * SEG, half[evs[e - 1][1:]] + 1 if e else 0)
                hi_ = min(2 * (jobs[ji][1] - off) + 1, 2 * (sg + 1) * SEG - 1,
                          half[evs[e + 1][1:]] - 1 if e + 1 < len(evs) else 2 * (T - cfg['TAIL']))
                if lo_ <= h <= hi_:
                    half[(ji, u)] = h
    if cfg.get('SHOW'):
        for g in range(7, 14):
            rg = range(start[g], start[g + 1])
            print('  ', ''.join('%2d' % round(10 * use[t]) for t in rg))
            print('  ', ''.join('%2s' % ''.join((str(len(w)) if u == 0 else '.') for w in when for u, x in enumerate(w) if x % T == t) for t in rg))
    plan = {}
    for _, ji, u in evs:
        plan.setdefault(half[(ji, u)] // 2, []).append((half[(ji, u)] % 2, jobs[ji][3], jobs[ji][4], STAGES[jobs[ji][5]][u]))
    if cfg.get('PLANOUT') is not None:
        kind = lambda j: 'conv' if j[3] is None else 'fin' if j[3] == 'fin' else j[4].func.__name__ + str(j[4].args[1] if j[4].func.__name__ == 'unit2' else j[4].args[2])
        cfg['PLANOUT'].update(ev=[(half[(ji, u)], kind(jobs[ji]), u, jobs[ji][2][u]) for _, ji, u in evs], use=use,
                              rd=[(outs[g][1], str(rd)) for g, rd, t0, n in sched for _ in range(n)])
    assert all((ts[0] < 0) == (ts[-1] < 0) for ts in when)
    carried = [(job[4], job[5]) for ts, job in zip(when, jobs) if ts[0] < 0]

    def w_copy(l):
        return pltpu.make_async_copy(w_hbm.at[l], w_ref.at[l], sem.at[l])

    def w0_copy(u):
        return pltpu.make_async_copy(w_hbm.at[0, :, u], w_ref.at[0, :, u], sem.at[L + 10 + u])

    def in_copy(t, slot):
        return pltpu.make_async_copy(x_hbm.at[pl.ds(pl.multiple_of(t * TM, 32), TM)], xn2_ref.at[slot], sem.at[L + slot])

    def out_copy(t, slot, part):
        r0, nr = ((0, 2 * Mh), (2 * Mh, Mh), (3 * Mh, Mh))[part]
        return pltpu.make_async_copy(o2_ref.at[slot, pl.ds(r0, nr)],
                                     o_hbm.at[pl.ds(pl.multiple_of(t * TM + r0, 32), nr)],
                                     sem.at[L + 4 + 3 * slot + part])

    xr_in = pltpu.make_async_copy(x_hbm.at[pl.ds(NMAIN * TM, R0)], xr_ref, sem.at[L + 2])
    xr_out = pltpu.make_async_copy(xr_ref, o_hbm.at[pl.ds(NMAIN * TM, R0)], sem.at[L + 2])
    b_in = pltpu.make_async_copy(b_hbm, b_ref, sem.at[L + 3])

    def prologue():
        b_in.start()
        for u in range(8):
            w0_copy(u).start()
        xr_in.start()
        in_copy(0, 0).start()
        for l in range(1, L):
            w_copy(l).start()
        in_copy(min(1, NMAIN - 1), 1).start()
        b_in.wait()
        for l in range(L):
            bf_ref[l] = b_ref[l:l + 1, :].astype(f32)

        def bias_tiles(l, carry):
            b = jnp.broadcast_to(bf_ref[l] + (l == 0).astype(f32), (8, D))
            for u, site in enumerate(BIAS):
                terms = [b[:, key * 128:(key + 1) * 128] * cf for key, cf in sorted(bias_coefs(*site).items()) if cf != 0.0]
                bt_ref[l, u] = functools.reduce(lambda x, y: x + y, terms)
            return carry
        jax.lax.fori_loop(0, L, bias_tiles, 0)
        if cfg.get('FAST'):
            return

        def slab(u, carry):
            w0_copy(u).wait()
            zero = jax.lax.shift_right_logical(u, 12)
            prep(0, u, iter(lambda: None, 0), zero, kb0)
            return zero
        zero = jax.lax.fori_loop(0, cfg['NSLAB'], slab, 0)

        def plain(l, xbf, x0f, x, na, free, never, j0=0, j1=D // 128):
            passes = []
            for jt in range(j0, j1):
                cols = slice(jt * 128, (jt + 1) * 128)
                ya = _dot(xbf[:, :D // 2], w_ref[l, 0:4, :, :, cols].reshape(D // 2, 128)) + bf_ref[l, :, cols]
                passes += [ya, _dot(xbf[:, D // 2:], w_ref[l, 4:8, :, :, cols].reshape(D // 2, 128)) + ya]
            xp_ref[0, :, j0 * 128:j1 * 128] = x0f * jnp.concatenate(passes[1::2], axis=1) + x
            for u in range(na):
                f_ = (u - free) * len(passes) * (R0 // 8) // (na - free)
                if cfg['PPH'] is not None:
                    f_ = f_ // 2 * 2 + cfg['PPH']
                ps, rr = divmod(f_, R0 // 8)
                yield None if u < free else (never, passes[ps][rr * 8:rr * 8 + 8, :])

        for u in range(cfg['NSLAB'], 8):
            w0_copy(u).wait()
        xr_in.wait()
        never = jnp.broadcast_to(zero, (8, 128)) != 0
        jm = cfg['JM']
        x0f = xr_ref[:, :jm * 128].astype(f32)
        xp_ref[1, :, :jm * 128] = x0f
        anchors = plain(0, xr_ref[...], x0f, x0f, (8 - cfg['NSLAB']) * (28 + len(prods3)), cfg['AFREE'], never, 0, jm)
        for u in range(cfg['NSLAB'], 8):
            prep(0, u, anchors, zero, (kb0, kb1)[u % 2])
        in_copy(0, 0).wait()
        x0f = xr_ref[:, jm * 128:].astype(f32)
        xp_ref[1, :, jm * 128:] = x0f
        units = [(R, C, r) for R in range(4) for C in range(4) for r in range(0, Mh, 32)]
        anchors = plain(0, xr_ref[...], x0f, x0f, len(units) + sum(len(STAGES[n]) for _, n in carried) + 2, 4, never, jm)
        for R, C, r in units[:len(units) // 2]:
            conv(xn2_ref.at[0], zero, R, C, r, min(32, Mh - r), next(anchors))
        for fn, n in carried:
            st8 = {}
            for group in STAGES[n]:
                anchor = next(anchors)
                xb[xset(0)][0, 0, 0, 0, Mh + 24:Mh + 32, :] = anchor[1]
                fn(st8, group, zero, jax.lax.shift_right_logical(zero, 1), anchor)
        for R, C, r in units[len(units) // 2:]:
            conv(xn2_ref.at[0], zero, R, C, r, min(32, Mh - r), next(anchors))

        def layer(l, carry):
            w_copy(l).wait()
            zero = jax.lax.shift_right_logical(l, 12)
            x = xp_ref[0]
            anchors = plain(l, x.astype(bf16), xp_ref[1], x, 8 * (28 + len(prods3)), cfg['AFREE'],
                            jnp.broadcast_to(zero, (8, 128)) != 0)
            for u in range(8):
                prep(l, u, anchors, zero, (kb0, kb1)[u % 2])
            return carry

        jax.lax.fori_loop(1, L, layer, 0)
        xr_ref[...] = xp_ref[0].astype(bf16)
        xr_out.start()

    def main(tile, carry):
        zs, za = jax.lax.shift_right_logical(tile, 12), jax.lax.shift_right_logical(tile, 13)
        never = jnp.broadcast_to(zs, (8, 128)) != 0
        slot = tile % 2
        in_copy(jnp.minimum(tile + 2, NMAIN - 1), slot).start()
        in_copy(jnp.minimum(tile + 1, NMAIN - 1), 1 - slot).wait()

        @pl.when(tile > 1)
        def _():
            for part in range(3):
                out_copy(tile - 2, slot, part).wait()

        xn_ref = xn2_ref.at[1 - slot]
        o_ref = o2_ref.at[slot]
        def rows(h, r0):
            if isinstance(h, tuple):
                return slice(r0 + h[0], r0 + h[0] + h[1])
            return slice(r0, r0 + Mh) if h is None else slice(r0 + h * Mq, r0 + (h + 1) * Mq)

        def ld(loc, h=None, z=0):
            return loc[0][(z,) + loc[1] + (rows(h, loc[2]),)]

        def st(loc, v, h=None):
            loc[0][(za if h == 1 and not loc[1] and cfg['ZB'] else zs,) + loc[1] + (rows(h, loc[2]),)] = v

        def by_half(v, h, fn):
            if isinstance(h, tuple):
                h = h[0] // Mq
            return fn(v, h) if h is not None else jnp.concatenate([fn(v[:Mq], 0), fn(v[Mq:], 1)], axis=0)

        def gather(ref, idx, n, pos):
            if cfg['NOBC']:
                return ref[idx + (slice(0, n), slice(16 * pos, 16 * pos + 16))].reshape(16 * n, 128)
            return ref.bitcast(u32)[idx + (slice(0, n), slice(8 * pos, 8 * pos + 8))].reshape(8 * n, 128)

        as_bf16 = lambda v: v if cfg['NOBC'] else pltpu.bitcast(v, bf16)

        def lhs2(p, q):
            ref, u = s2loc(p)
            return as_bf16(jnp.concatenate([gather(ref, (0, u, k), NC, q2[p].index(q)) for k in range(2)], axis=1))

        def rhs2(l, p, q, n):
            return as_bf16(gather(t2[p], (l, n), 16, q2[p].index(q)))

        def dot3(l, p, q, r):
            qs = next(qs for qs in PAIRS if q in qs)
            return _dot(as_bf16(gather(s3[(p, qs)], (0, qs.index(q)), NQ, ORD.index(r))),
                        as_bf16(gather(t3_ref, (l, prods3.index((p, q))), 8, ORD.index(r))))

        def add_bias(v, l, site, h):
            def one(x, hh):
                b = bt_ref[l, BIAS.index(site + (hh,))]
                return (x.reshape(Mq // 8, 8, 128) + b).reshape(Mq, 128)
            return by_half(v, h, one)

        def outer_act(l, p, i, j, n, d, h, part=None):
            bt, stores, finals = OACT[p]
            if part == 'stores':
                finals = []
            if part == 'finals':
                bt, stores = [], []
            if bt:
                d = add_bias(d, l, (p, False, i, j, n), h)
            cache = {'d': d}
            def comb(terms):
                for _, src in terms:
                    if isinstance(src, str) and src not in cache:
                        cache[src] = ld(oloc(src, i, j, n), h)
                v = lincomb([(s, cache[src]) for s, src in terms if isinstance(src, str)])
                for _, src in terms:
                    if not isinstance(src, str):
                        v = add_bias(v, l, (p, True, i, j, n), h)
                return v
            fin = [(IJ, comb(terms)) for IJ, terms in finals]
            for name, v in [(name, comb(terms)) for name, terms in stores]:
                st(oloc(name, i, j, n), v, h)
            for (I, J), y in fin:
                R, C = 2 * I + i, 2 * J + j
                xn = ld(x0loc(R, C, n), h) * y
                if l > 0:
                    xn = xn + ld(xloc(l, R, C, n), h)
                if l < L - 1:
                    st(xloc(l + 1, R, C, n), xn, h)
                else:
                    xn = by_half(xn, h, lambda x, hh: x if scale(R, C, hh, n) == 1.0 else x * (1.0 / scale(R, C, hh, n)))
                    o_ref[rows(h, R * Mh), C * H + n * 128:C * H + (n + 1) * 128] = xn.astype(bf16)

        def inner_act(g, l, p, kind, n, h, P, Q, part=None):
            vloc = oloc(raw_slot(p), 0, 1, n) if raw_slot(p) else iloc(g, 'v', n)
            if kind == '35':
                st(iloc(g, 's', n), Q + ld(iloc(g, 'm1', n), h), h)
                if not raw_slot(p):
                    st(vloc, P, h)
                outer_act(l, p, 0, 1, n, P, h)
            elif kind == '47':
                st(iloc(g, 'u', n), Q + ld(vloc, h), h)
                outer_act(l, p, 0, 0, n, P + ld(iloc(g, 's', n), h), h)
            else:
                outer_act(l, p, 1, 1, n, ld(iloc(g, 's', n), h) - Q, h, part)
                outer_act(l, p, 1, 0, n, P + ld(iloc(g, 'u', n), h), h, part)

        def issue(l, p, rd):
            kind, n = rd
            if kind == 'x':
                return [dot3(l, p, q, 1) for q in (3, 5, 4, 7)]
            if kind == 'y':
                return [dot3(l, pp, q, 1) for pp in (p, SEL3[SEL3.index(p) + 1]) for q in (2, 6)]
            if isinstance(n, str):
                if cfg['MO']:
                    d = [dot3(l, p, int(q), int(r)) for q in kind for r in n]
                    return [d[0], d[2], d[1], d[3]]
                return [dot3(l, p, int(q), int(r)) for r in n for q in kind]
            if cfg['GR']:
                ops = [(lhs2(p, 1),) * 2, (rhs2(l, p, 1, 0), rhs2(l, p, 1, 1))] if kind == '1' else [
                    [lhs2(p, int(q)) for q in kind], [rhs2(l, p, int(q), n) for q in kind]]
                d = [_dot(a[:, k * 128:(k + 1) * 128], b[k * 128:(k + 1) * 128]) for a, b in zip(*ops) for k in range(2)]
                return [d[0] + d[1], d[2] + d[3], d[cfg['GR'] - 1]]
            if kind == '1':
                lhs = lhs2(p, 1)
                return [_dot(lhs, rhs2(l, p, 1, 0)), _dot(lhs, rhs2(l, p, 1, 1))]
            return [_dot(lhs2(p, int(q)), rhs2(l, p, int(q), n)) for q in kind]

        def consume(g, l, p, rd, res):
            kind, n = rd
            if n == '1':
                for u, where in enumerate((('35', False), ('47', False)) if kind == 'x' else (('26', False), ('26', True))):
                    for al in range(2):
                        st(jloc(where[0], '1', al, where[1]), res[2 * u + al], 0)
            elif isinstance(n, str):
                sm = [res[al] + res[2 + al] for al in range(2)]
                df = [res[al] - res[2 + al] for al in range(2)]
                J = lambda name, al: ld(jloc(kind, name, al, name == '1' and kind == '26' and p in SEL3[1::2]), 0)
                part = 'stores' if n in cfg['DEFER'] else None
                done = lambda h, nn, m: inner_act(g, l, p, kind, nn, h, m[0] + m[1], m[0] - m[1], part)
                O, I = (lambda i, j: oloc(raw_slot(p), i, j, 1)), (lambda name: iloc(g, name, 1))
                rec = lambda al: [(s, ld(loc, 0, za if cfg['ZB'] else 0)) for s, loc in {
                    '35': [[(1, O(0, 1))], [(1, I('s')), (-1, I('m1'))]],
                    '47': [[(1, O(0, 0)), (-1, I('s'))], [(1, I('u')), (-1, O(0, 1))]],
                    '26': [[(1, O(1, 0)), (-1, I('u'))], [(1, I('s')), (-1, O(1, 1))]]}[kind][al]]
                if n == '35':
                    for al in range(2):
                        st(jloc(kind, 's', al), df[al] + J('1', al), 0)
                    done(0, 1, sm)
                elif n == '47':
                    if cfg['HY'] == 1:
                        for al in range(2):
                            st(jloc(kind, 'u', al), df[al], 0)
                    else:
                        for al, v in enumerate((df[0] + df[1], df[0] - df[1])):
                            st(jloc(kind, 'u', al), lincomb([(1, v)] + rec(al)), 0)
                    done(0, 0, [sm[al] + J('s', al) for al in range(2)])
                else:
                    if cfg['HY'] == 1:
                        m = [sm[al] + J('u', al) for al in range(2)]
                        P, Q = lincomb([(1, m[0] + m[1])] + rec(0)), lincomb([(1, m[0] - m[1])] + rec(1))
                    else:
                        P, Q = (sm[0] + sm[1]) + J('u', 0), (sm[0] - sm[1]) + J('u', 1)
                    done(1, 1, [J('s', al) - df[al] for al in range(2)])
                    inner_act(g, l, p, kind, 0, 1, P, Q, part)
            elif kind == '1':
                st(iloc(g, 'm1', 0), res[0])
                st(iloc(g, 'm1', 1), res[1])
            else:
                inner_act(g, l, p, kind, n, None, res[0] + res[1], res[0] - res[1])

        state = {}
        for g, rd, t0, n in sched:
            l, p = outs[g]
            if t0 == start[G - 1]:
                out_copy(tile, slot, 0).start()
            if t0 + n == T:
                out_copy(tile, slot, 1).start()
            res = issue(l, p, rd)
            if cfg['EO']:
                consume(g, l, p, rd, res)
            for t in range(t0, t0 + n):
                for ph, l2, fn, group in plan.get(t, []):
                    gr = 16 * (t - t0) + 8 * ph
                    if cfg['GF']:
                        gr = 16 * (t - t0) + 8 * (1 - ph)
                    gs = cfg['GS']
                    gate = res[2 if len(res) == 3 else cfg['GM']][gr:gr + 8, :]
                    if cfg['GADD'] and isinstance(rd[1], str) and rd[1] != '1':
                        gate = gate + res[2 + gs % 2][gr:gr + 8, :]
                    elif gs == 2 and rd[0] != '1' and rd[1] != '1':
                        gate = gate + res[1][gr:gr + 8, :]
                    if l2 == 'fin':
                        lf, pf, nf, r0 = fn
                        for j in range(2):
                            d = ld(oloc(raw_slot(pf), 1, j, nf), (r0, 16))
                            d = tie(tie(d, (never, gate)), (never, gate), 8)
                            outer_act(lf, pf, 1, j, nf, d, (r0, 16), 'finals')
                    elif l2 is None:
                        conv(xn_ref, zs, *fn, min(32, Mh - fn[2]), (never, gate))
                    else:
                        if group != ('l1',):
                            xb[xset(l2)][0, 0, 0, 0, Mh + 24:Mh + 32, :] = gate
                        fn(state.setdefault(id(fn), {}), group, zs, za, (never, gate))
            if not cfg['EO']:
                consume(g, l, p, rd, res)
        out_copy(tile, slot, 2).start()
        return carry

    prologue()
    jax.lax.fori_loop(0, NMAIN, main, 0)
    xr_out.wait()
    in_copy(NMAIN - 1, (NMAIN - 1) % 2).wait()
    for t in range(max(NMAIN - 2, 0), NMAIN):
        for part in range(3):
            out_copy(t, t % 2, part).wait()


DEFAULT = dict(SEL=(3, 5, 4, 7), SEL3=(3, 5, 4, 7), XC={B12: 5, B11: 1, B22: 7, B21: 2}, AFREE=4, NOBC=0, FOLD=1, MO=1, GR=2, GM=0, DBL=1, GS=0, GF=0, EO=0, KP=16, PPH=None, ZB=0, HY=1, HOLD=0, PORT=0.9, PS=0, NSLAB=6, JM=3, XP=40, XO=16, DEFER=('26',), EW=12, KW=(1,) * 5, CM=(1,) * 7, SEEDS=(), SEG=32, PJ=20, QO=0, TIEL=3, GADD=0, TF=0, T8=0, TAIL=6,
               CS=0.5, CL=0.3, UL=0.8, CAP=0.85, FR=((1.,), (.4, .6), (.35, .37, .28), (.16, .26, .31, .27),
                   (.35, .29, .08, .28), (.16, .26, .26, .05, .27)))


def build(TM=640, **kw):
    def f(x0, ws, bs):
        B, D = x0.shape
        L = ws.shape[0]
        cfg = dict(DEFAULT, **kw)
        Mh = TM // 4
        MP = Mh + 32
        nmain = (B - 1) // TM
        R0 = B - nmain * TM
        pairs3, q2 = layout(cfg)
        n3 = sum(2 * len(v) for v in pairs3.values())
        pad = lambda n: n + (2 - n) % 4
        V = pltpu.VMEM
        half = V((1, MP, 128), f32)
        XP = Mh + cfg['XP']
        scratch = ([V((1, 2, 2, 2, XP, 128), f32)] * 4 + [V((1, 2, 4, 2, XP, 128), f32)] * 6 + [half] * (16 + 56 + 26)
                   + [V((1, 1 + (p == 2), 2, pad(Mh // 16), 16 * len(q2[p]), 128), bf16) for p in (1, 3, 4, 5, 7, 2)]
                   + [V((1, 2, pad(Mh // 32), 112, 128), bf16)] * (n3 // 2)
                   + [V((L, 2, 16, 16 * len(q2[p]), 128), bf16) for p in range(1, 8)]
                   + [V((L, n3, 8, 112, 128), bf16), V((1, 4, 16 * n3 + cfg['KP'], 128), f32), V((1, 4, 16 * n3 + cfg['KP'], 128), f32),
                      V((L, len(BIAS), 8, 128), f32), V((8, 1, D), f32), V((2, TM, D), bf16), V((2, TM, D), bf16), V((L, 8, 8, 16, D), bf16),
                      V((R0, D), bf16), V((2, R0, D), f32), V((L, D), bf16), pltpu.SemaphoreType.DMA((L + 18,))])
        anyspec = pl.BlockSpec(memory_space=pl.ANY)
        return pl.pallas_call(
            functools.partial(_kernel, L=L, TM=TM, R0=R0, NMAIN=nmain, D=D, cfg=cfg),
            in_specs=[anyspec, anyspec, anyspec],
            out_specs=anyspec,
            out_shape=jax.ShapeDtypeStruct((B, D), x0.dtype),
            scratch_shapes=scratch,
            compiler_params=pltpu.CompilerParams(
                vmem_limit_bytes=110 * 1024 * 1024,
                internal_scratch_in_bytes=65536,
                disable_bounds_checks=True,
            ),
        )(x0, ws.reshape(L, 8, 8, 16, D), bs)
    return f


@jax.jit
def pallas_standalone__dcn_v2_cross__recsys_kernel(x0, ws, bs):
    return build(TM=640)(x0, ws, bs)
```

```python
import functools

import jax
import jax.numpy as jnp
import jax.experimental.pallas as pl
import jax.experimental.pallas.tpu as pltpu

f32 = jnp.float32
bf16 = jnp.bfloat16
u32 = jnp.uint32

B11, B12, B21, B22 = (0, 0), (0, 1), (1, 0), (1, 1)
LA = {1: [(B11, 1), (B22, 1)], 2: [(B11, 1), (B12, 1), (B21, 1), (B22, 1)], 3: [(B11, 1), (B12, -1)],
      4: [(B12, 1), (B22, 1)], 5: [(B11, 1), (B12, 1)], 6: [(B12, 1), (B11, -1), (B21, 1), (B22, -1)],
      7: [(B12, 1), (B22, -1)]}
PAIRS = ((5, 3), (4, 7), (2, 6))
ORD = (3, 5, 4, 7, 1, 2, 6)
D2 = (1.0, 2.0)
BF = {1: 1.0, 2: 0.5, 3: 0.5, 4: 0.5, 5: 0.5, 6: 0.5, 7: 0.5}
OUTER = (3, 5, 1, 4, 7, 2, 6)
OACT = {
    3: ([(1, B12)], [('M3', [(1, 'd')])], []),
    5: ([], [('M5', [(1, 'd')])], [(B12, [(1, 'd'), (1, 'M3')])]),
    1: ([(1, B11), (-1, B12)], [('S', [(1, 'd'), (1, 'M3'), (-1, 'M5')])], []),
    4: ([], [('M4', [(1, 'd')])], []),
    7: ([], [('M7', [(1, 'd')])], [(B11, [(1, 'd'), (1, 'S'), (1, 'M4')])]),
    2: ([(1, B11), (-1, B22)], [('M2', [(1, 'd')]),
        ('U', [(1, 'd'), (1, 'M4'), (-1, 'M7'), (1, 'M3'), (1, 'M5'), (1, ((1, B21), (-1, B12), (-1, B11), (1, B22)))])], []),
    6: ([], [], [(B22, [(1, 'd'), (1, 'S'), (-1, 'M2')]), (B21, [(1, 'd'), (1, 'U')])]),
}
OSL = {'M3': 0, 'M5': 1, 'S': 2, 'M4': 3, 'M7': 4, 'M2': 6, 'U': 5}
ISL = {'m1': 0, 's': 1, 'v': 2, 'u': 3}
STAGES = {1: [(B11, B12, B21, B22)], 2: [(B11, B12), (B21, B22)], 3: [(B11, B12), (B22,), (B21,)],
          4: [(B11,), (B12,), (B22,), (B21,)], 5: [(B11, B12), (B22, 'hold'), ('l1',), (B21,)],
          6: [(B11,), (B12,), (B22, 'hold'), ('l1',), (B21,)]}
BIAS = [(p, extra, i, j, n, h) for p in OUTER for extra in (False, True)
        if (any(not isinstance(x, str) for _, t in OACT[p][1] + OACT[p][2] for _, x in t) if extra else OACT[p][0])
        for i in range(2) for j in range(2) for n in range(2) for h in range(2)]
PREP_ORDER = (2, 6, 3, 5, 1, 4, 7)
LAG = 8


def _dot(a, b):
    return jnp.dot(a, b, preferred_element_type=f32)


def scale(R, C, h, k):
    return D2[R // 2] * D2[R % 2] * D2[h] / (D2[C // 2] * D2[C % 2] * D2[k])


def b_ops(b11, b12, b21, b22):
    r1 = b11 + b22
    g = b12 + b21
    return {1: r1, 2: b11 - b12, 3: b12 - b22, 4: g - r1, 5: b12 + b22, 6: b11 + b12, 7: g + r1}


def lincomb(terms):
    assert terms[0][0] == 1
    acc = terms[0][1]
    for s, v in terms[1:]:
        acc = acc + v if s == 1 else acc - v
    return acc


def raw_slot(p):
    return next((name for name, terms in OACT[p][1] if terms == [(1, 'd')]), None)


def round_usage(p, rd, first, last, defer, hy):
    bt, stores, finals = OACT[p]
    alu = bool(bt) + sum(len(t) - 1 for _, t in stores) + sum(len(t) + (not first) + 2 * last for _, t in finals)
    nst = len(stores) + len(finals)
    nld = len({x for _, t in stores + finals for _, x in t if isinstance(x, str) and x != 'd'}) + len(finals) * (2 - first)
    kind, n = rd
    if isinstance(n, str):
        e = kind == '47'
        if kind == '26':
            a, st, ld, m = {'35': (10, 2, 9, 2), '47': (10, 2, 9, 2) if hy == 1 else (16, 2, 13, 2), '26': (20, 0, 17, 4) if hy == 1 else (16, 0, 13, 4)}[n]
            if n in defer and finals:
                alu, nst, nld = 0, 1, 0
        else:
            a, st, ld, m = {'1': (0, 4, 5, 0), '35': (9 + e, 3, 8 + e, 1),
                            '47': (9 + e, 3, 8 + e, 1) if hy == 1 else (14 + 2 * e, 3, 11 + 2 * e, 1),
                            '26': (17 + 3 * e, 2, 14 + 3 * e, 2) if hy == 1 else (14 + 2 * e, 2, 11 + 2 * e, 2)}[n]
    else:
        a, st, ld, m = {'1': (2, 2, 4, 0), '35': (5, 2 - bool(raw_slot(p)), 5, 1), '47': (6, 1, 6, 1),
                        '26': (6, 0, 6, 2)}[kind]
    return a + m * alu, st + m * nst, ld + m * nld


def yds(groups, cap):
    n = len(cap)
    speed, cls, gcls = [0.0] * n, [-1] * n, {}
    todo = list(groups)
    while todo:
        pre = [0.0]
        for t in range(n):
            pre.append(pre[-1] + (cap[t] if cls[t] < 0 else 0.0))
        best = None
        for a in sorted({g[0] for g in todo}):
            w = 0.0
            for g in sorted((g for g in todo if g[0] >= a), key=lambda g: g[1]):
                w += g[2]
                d = w / max(pre[g[1] + 1] - pre[a], 1e-9)
                if best is None or d > best[0]:
                    best = (d, a, g[1])
        d, a, b = best
        for t in range(a, b + 1):
            if cls[t] < 0:
                speed[t], cls[t] = d, len(gcls)
        gcls.update({g[:2]: len(gcls) for g in todo if g[0] >= a and g[1] <= b})
        todo = [g for g in todo if not (g[0] >= a and g[1] <= b)]
    return speed, cls, gcls


def spread_jobs(jobs, cap, tail):
    T = len(cap)
    cap3 = cap * 3
    all3 = [(lo + k * T, hi + k * T, ji, k) for k in range(3) for ji, (lo, hi, _) in enumerate(jobs) if lo + k * T >= 0]
    pend = {}
    for j in sorted(all3, key=lambda j: (j[1], j[3], j[2])):
        pend.setdefault(j[:2], []).append(j)
    speed, cls, gcls = yds([w + (sum(sum(jobs[j[2]][2]) for j in q),) for w, q in pend.items()], cap3)
    when = [[] for _ in jobs]
    debt, cur, done = 0.0, None, 0
    for t in range(3 * T):
        while True:
            j = cur
            if j is None:
                rdy = [q[0] for w, q in pend.items() if q and w[0] <= t and (gcls[w] == cls[t] or w[1] <= t)]
                if not rdy:
                    debt = max(debt, 0.0)
                    break
                j = rdy[0]
                nst = len(jobs[j[2]][2])
                if nst > 1 and j[1] > t and (t + tail + 2 * nst) // T != t // T:
                    break
            must = j[1] <= t or (cur is not None and (t + tail + 1) // T != t // T)
            if not must and (cap3[t] == 0.0 or debt > 0.5 * speed[t] * cap3[t]):
                break
            if cur is None:
                pend[j[:2]].pop(0)
                cur, done = j, 0
            debt += jobs[j[2]][2][done]
            if j[3] == 1:
                when[j[2]].append(t - T)
            done += 1
            if done == len(jobs[j[2]][2]):
                cur = None
        debt -= speed[t] * cap3[t]
    return when


def layout(cfg):
    sel, sel3 = cfg['SEL'], cfg['SEL3']
    pairs3 = {p: [qs for qs in PAIRS if p in sel3 or (p in sel and qs != (2, 6))] for p in range(1, 8)}
    q2 = {p: [q for q in ORD if not any(q in qs for qs in pairs3[p])] for p in range(1, 8)}
    return pairs3, q2


def _kernel(x_hbm, w_hbm, b_hbm, o_hbm, *scratch, L, TM, R0, NMAIN, D, cfg):
    H, Mh, Mq = D // 4, TM // 4, TM // 8
    NC, NQ = Mh // 16, Mq // 16
    MP = Mh + 32
    SEL, SEL3 = cfg['SEL'], cfg['SEL3']
    pairs3, q2 = layout(cfg)
    prods3 = [(p, q) for p in SEL for qs in pairs3[p] for q in qs]
    assert H == 256 and L % 2 == 0 and Mq % 16 == 0 and all(raw_slot(p) for p in SEL)
    it = iter(scratch)
    take = lambda n: [next(it) for _ in range(n)]
    x0b, xb, ib, ob, jb = take(4), take(6), take(16), take(56), take(26)
    s2 = dict(zip((1, 3, 4, 5, 7, 2), take(6)))
    s3 = {(p, qs): next(it) for p in SEL for qs in pairs3[p]}
    t2 = dict(zip(range(1, 8), take(7)))
    t3_ref, kb0, kb1, bt_ref, bf_ref, xn2_ref, o2_ref, w_ref, xr_ref, xp_ref, b_ref, sem = it

    xset = lambda l: 4 if l == 0 else (l % 2) * 2
    xoff = lambda I, J: cfg['XO'] * ((I + J) % 2)
    xloc = lambda l, R, C, k: (xb[xset(l) + R // 2], (R % 2, C, k), xoff(R // 2, C // 2))
    x0loc = lambda R, C, k: (x0b[(R // 2) * 2 + C // 2], (R % 2, C % 2, k), 8 + xoff(R // 2, C // 2))
    iloc = lambda g, name, n: (ib[((g % 2) * 4 + ISL[name]) * 2 + n], (), 8 * ISL[name])
    oloc = lambda name, i, j, n: (ob[(OSL[name] * 4 + i * 2 + j) * 2 + n], (), 8 * ((OSL[name] + 2 * j) % 4))

    def jloc(kind, name, al, second=False):
        i = 24 + al if second else (('35', '47', '26').index(kind) * 4 + ('1', 's', 'u', 'v').index(name)) * 2 + al
        return jb[i], (), 8 * ((i + i // 2) % 4)

    def s2loc(p):
        return (s2[2], (2, 6).index(p)) if p in (2, 6) else (s2[p], 0)

    def bias_coefs(p, extra, i, j, n, h):
        where = [(1, i, j, n, h)]
        if extra:
            terms = next(x for _, t in OACT[p][1] + OACT[p][2] for _, x in t if not isinstance(x, str))
        else:
            terms = OACT[p][0]
            w = [(1, i, j)] + [(-1, 0, 1)] * bool(raw_slot(p) and (i, j) == B21)
            where = [x + (n, h) for x in w]
            if (h, n) == (1, 0) and PAIRS[{B12: 0, B11: 1}.get((i, j), 2)] in pairs3[p]:
                where += [(-sg, ii, jj, 1, 0) for sg, ii, jj in w]
        coef = {}
        for sg, ii, jj, nn, hh in where:
            for cf, (I, J) in terms:
                key = (2 * J + jj) * 2 + nn
                coef[key] = coef.get(key, 0.0) + sg * cf * scale(2 * I + ii, 2 * J + jj, hh, nn)
        return coef

    def tie(v, anchor, r=0):
        if anchor is None:
            return v
        return jnp.concatenate([v[:r]] * (r > 0) + [jax.lax.select(anchor[0], anchor[1], v[r:r + 8])] + [v[r + 8:]] * (r + 8 < v.shape[0]), axis=0)

    def consts(anchor, ss, reps):
        one = {s: jnp.full((8, 128), s, f32) for s in set(ss)}
        if anchor is not None:
            one = {s: jax.lax.select(anchor[0], anchor[1], v) for s, v in one.items()}
        return jnp.concatenate([one[s] for s in ss for _ in range(reps)], axis=0)

    def conv(src, zs, R, C, r, nr, anchor=None):
        v = src[R * Mh + r:R * Mh + r + nr, C * H:(C + 1) * H].astype(f32)
        for k in range(2):
            buf, idx, off = xloc(0, R, C, k)
            sv = consts(anchor, [scale(R, C, (r + u) // Mq, k) for u in range(0, nr, 16)], 2)
            buf[(zs,) + idx + (slice(off + r, off + r + nr),)] = v[:, k * 128:(k + 1) * 128] * sv

    def block_sum(l, terms, ii, jj, kk, r, save, zs, za, anchor, late=None):
        rng = lambda t: slice(t[0], t[-1] + 1)
        keys = [(i, j, k) for i in ii for j in jj for k in kk]
        vals = []
        for u, ((I, J), s) in enumerate(terms):
            ref, r0 = xb[xset(l) + I], xoff(I, J) + r
            v = ref[za if u == 0 else 0, rng(ii), 2 * J + jj[0]:2 * J + jj[-1] + 1, rng(kk), r0:r0 + 16, :]
            if (I, J) in save:
                sv = consts(anchor, [1.0 / scale(2 * I + i, 2 * J + j, r // Mq, k) for i, j, k in keys], 2)
                x0b[I * 2 + J][zs, rng(ii), rng(jj), rng(kk), r0 + 8:r0 + 24, :] = v * sv.reshape(v.shape)
            v = v.reshape(16 * len(keys), 128)
            if u == 0 and late is not None and anchor is not None:
                ref[0, 0, 0, 0, Mh + 24:Mh + 32, :] = anchor[1]
                top = ref[za, late[0], 2 * J + late[1], late[2], r0:r0 + 8, :]
                if cfg['TIEL'] == 2:
                    top = jax.lax.select(anchor[0], anchor[1], top)
                at = 16 * keys.index(late)
                v = jnp.concatenate([v[:at]] * (at > 0) + [top, v[at + 8:]], axis=0)
            vals.append((s, v))
        v = lincomb(vals)
        if cfg['TIEL'] == 3 and late is not None:
            v = tie(v, anchor, 16 * keys.index(late))
        return v

    def release(qs, store, st8, anchor):
        v = st8['l1']
        if anchor is not None:
            n = v.shape[0]
            top = jax.lax.select(jnp.broadcast_to(anchor[0], (n, 8, 128)), jnp.broadcast_to(anchor[1], (n, 8, 128)), v[:, :8])
            v = jnp.concatenate([top, v[:, 8:]], axis=1)
        r0 = 16 * qs.index(1)
        store(slice(r0, r0 + 16), v.astype(bf16))

    def finish(e, f, group, qs, store, st8, anchor, hold=False):
        a = e[None] if f is None else jnp.concatenate([e + f, e - f], axis=0).reshape(2, e.shape[0], 128)
        for u, b in enumerate(group):
            st8[b] = a if len(group) == 1 else a[:, 16 * u:16 * u + 16]
        ops = {}
        if B12 in group and 3 in qs:
            ops[3], ops[5] = st8[B11] - st8[B12], st8[B11] + st8[B12]
        if B22 in group:
            if 4 in qs:
                ops[4], ops[7] = st8[B12] + st8[B22], st8[B12] - st8[B22]
            ops[1] = st8['l1'] = st8[B11] + st8[B22]
        if B21 in group:
            g = st8[B12] + st8[B21]
            ops[2], ops[6] = g + st8['l1'], g - st8['l1']
        now = [q for q in qs if q in ops and not (hold and q == 1)]
        if now:
            r0 = 16 * qs.index(now[0])
            store(slice(r0, r0 + 16 * len(now)), jnp.concatenate([ops[q] for q in now], axis=1).astype(bf16))

    def unit2(l, ps, c, k, save, st8, group, zs, za, anchor):
        def store(rows, v):
            s2[ps[0]][zs, :, k, c, rows, :] = v
        if group == ('l1',):
            return release(q2[ps[0]], store, st8, anchor)
        hold, group = 'hold' in group, tuple(b for b in group if b != 'hold')
        ii, jj = sorted({b[0] for b in group}), sorted({b[1] for b in group})
        bs = lambda terms, late: block_sum(l, terms, ii, jj, [k], 16 * c, save, zs, za, anchor, late)
        f = None if len(ps) == 1 else bs([(B11, 1), (B22, 1)], None)
        e = bs(LA[ps[0]] if len(ps) == 1 else [(B12, 1), (B21, 1)], (ii[0], jj[-1], k))
        finish(e, f, group, q2[ps[0]], store, st8, anchor, hold)

    def unit3(l, p, qs, c, save, st8, group, zs, za, anchor):
        def store(rows, w):
            s3[(p, qs)][zs, :, c, rows, :] = w
        if group == ('l1',):
            return release(ORD, store, st8, anchor)
        hold, group = 'hold' in group, tuple(b for b in group if b != 'hold')
        for h in sorted({b[0] for b in group}):
            grp = tuple(b for b in group if b[0] == h)
            kk = [b[1] for b in grp]
            ii, jj = {(5, 3): ([0], [0, 1]), (4, 7): ([0, 1], [1]), (2, 6): ([0, 1], [0, 1])}[qs]
            v = block_sum(l, LA[p], ii, jj, sorted(kk), h * Mq + 16 * c, save, zs, za, anchor,
                          (0, (0 if cfg['TF'] else 1) if qs == (2, 6) else jj[0], max(kk)) if h == group[-1][0] else None)
            n = 16 * len(kk)
            piece = lambda u: v[u * n:(u + 1) * n]
            if qs == (2, 6):
                e, f = piece(1) + piece(2), piece(0) + piece(3)
                r0 = 16 * q2[p].index(1)
                s2[p][zs, 0, min(kk):max(kk) + 1, h * NQ + c, r0:r0 + 16, :] = f.reshape(len(kk), 16, 128).astype(bf16)
            else:
                e, f = piece(0), piece(1)
            finish(e, f, tuple(sorted(grp)), ORD, store, st8, anchor, hold)

    def prep(l, u, anchors, zero, kb):
        for k in range(2):
            wide = [w_ref[l, R * 2 + k, u].astype(f32) for R in range(4)]
            for n in range(2):
                def blk(R, C):
                    v = wide[R][:, C * H + n * 128:C * H + (n + 1) * 128]
                    s = D2[R // 2] / D2[C // 2]
                    return v if s == 1.0 else v * s
                O = {(i, j): b_ops(blk(i, j), blk(i, 2 + j), blk(2 + i, j), blk(2 + i, 2 + j)) for i, j in (B11, B12, B21, B22)}
                for p in PREP_ORDER:
                    anchor = next(anchors)
                    fold = 0.5 if cfg['FOLD'] and p in SEL else 1.0
                    s = BF[p] * 0.5 * D2[k] / D2[n] * fold
                    cs = {f: consts(anchor, [s * f], 2) for f in (0.5, 1.0, 2.0)}
                    T = b_ops(*[O[(i, j)][p] * cs[D2[i] / D2[j]] for i, j in (B11, B12, B21, B22)])
                    sq = {q: 2.0 * BF[q] / fold for q in q2[p]}
                    t2[p][l, n, k * 8 + u] = jnp.concatenate(
                        [T[q] if sq[q] == 1.0 else T[q] * sq[q] for q in q2[p]], axis=0).astype(bf16)
                    mine = [e for e, pq in enumerate(prods3) if pq[0] == p]
                    if mine:
                        kb[zero, k * 2 + n, 16 * mine[0]:16 * mine[-1] + 16, :] = jnp.concatenate(
                            [T[prods3[e][1]] for e in mine], axis=0)
        for e in range(len(prods3)):
            anchor = next(anchors)
            if cfg['FOLD']:
                n3 = 16 * len(prods3)
                if anchor is not None and cfg['FOLD'] > 1:
                    kb[0, 0, n3:n3 + 8, :] = anchor[1]
                    v = kb[jax.lax.shift_right_logical(zero, 1), :, 16 * e:16 * e + 16, :]
                else:
                    v = kb[0, :, 16 * e:16 * e + 16, :]
                T = b_ops(v[0], tie(v[1], anchor), v[2], v[3])
            else:
                v = kb[0, :, 16 * e:16 * e + 16, :] * consts(anchor, [0.5], 2)
                T = b_ops(v[0], v[1], v[2], v[3])
            T[1] = T[1] + T[1]
            t3_ref[l, e, u] = jnp.concatenate([T[q] for q in ORD], axis=0).astype(bf16)

    def rounds_of(p):
        rs = [('1', None)] + [('x', '1')] * (p in SEL)
        for kind, qs in zip(('35', '47', '26'), PAIRS):
            if kind == '26' and p in SEL3[::2]:
                rs.append(('y', '1'))
            rs += [(kind, r) for r in (('35', '47', '26') if qs in pairs3[p] else (0, 1))]
        return rs

    outs = [(l, p) for l in range(L) for p in OUTER]
    G = len(outs)
    sched, start, use = [], [], []
    for g, (l, p) in enumerate(outs):
        start.append(len(use))
        for rd in rounds_of(p):
            n = NQ if isinstance(rd[1], str) else NC
            sched.append((g, rd, len(use), n))
            a, st_, ld_ = round_usage(p, rd, l == 0, l == L - 1, cfg['DEFER'], cfg['HY'])
            if cfg['PORT']:
                use += [max((2 * a + st_ + 2 + 16 / n) / 72 + cfg['PS'] * st_ / 8, cfg['PORT'] * st_ / 8)] * n
            else:
                use += [max(a / 32, st_ / 8, cfg['UL'] * ld_ / 24)] * n
    T = len(use)
    cap = [max(cfg['CAP'] - max(use[t], use[(t + 1) % T]), 0.0) * (t < T - cfg['TAIL']) for t in range(T)]
    for g in range(G):
        for t in range(start[g], (start + [T])[g + 1]):
            cap[t] *= cfg['CM'][g % 7]
    jobs = []
    def add(lo, hi, alu, st_, ld_, nst, l, fn):
        w = alu / 64 + cfg['CS'] * (st_ + nst) / 16 + cfg['CL'] * ld_ / 48
        w *= cfg['KW'][0 if l in (None, 'fin') else nst]
        if cfg['HOLD'] and nst >= 3:
            nst += 2
        jobs.append((lo, max(hi, lo), [w * f for f in cfg['FR'][nst - 1]], l, fn, nst))
    for g, (l, p) in enumerate(outs):
        ready = 7 * l - 2 * all(I == 0 for (I, J), _ in LA[p])
        lo = start[ready] - (T if ready < 0 else 0)
        if 7 in SEL3 and cfg['DEFER'] and ready % 7 == 5 and l > 0:
            lo += cfg['EW'] + 1
        if p in SEL3 and OACT[p][2]:
            for h, n in [(0, 1)] * ('35' in cfg['DEFER']) + [(0, 0)] * ('47' in cfg['DEFER']) + [(1, 1), (1, 0)] * ('26' in cfg['DEFER']):
                for c in range(0, NQ):
                    e0 = start[g + 1]
                    add(e0, e0 + cfg['EW'] if p == 7 else start[7 * l + 5] - 1, 20 + 8 * (l == L - 1), 3, 20, 1, 'fin',
                        (l, p, n, h * Mq + 16 * c))
        hi = start[g] - LAG - 3
        nt = len(LA[p])
        save = [b for b, pp in cfg['XC'].items() if pp == p and l == 0]
        if p in SEL3:
            if p in SEL3[1::2]:
                host = 7 * l + OUTER.index(SEL3[SEL3.index(p) - 1])
                hi = [t0 for gg, rd, t0, _ in sched if gg == host and rd[0] == 'y'][0] - LAG - 3
            for c in range(NQ):
                add(lo, hi, 32 * nt + 50 + 32 * len(save), 18 + 32 * len(save), 32 * nt, cfg['NS'][3], l,
                    functools.partial(unit3, l, p, (2, 6), c, save))
        elif p != 6:
            ps = (2, 6) if p == 2 else (p,)
            nq = len(q2[p]) * len(ps)
            alu = 8 * (nt - 2 + len(ps)) + (8 if p in SEL else 16) * len(ps) + nq
            for c in range(NC):
                for k in range(2):
                    add(lo, hi, alu + 8 * len(save), nq + 8 * len(save), 8 * nt, 1 if nq <= 3 else cfg['NS'][0] if nq <= 7 else cfg['NS'][1], l,
                        functools.partial(unit2, l, ps, c, k, save))
        if p in SEL:
            for qs, c in ([(qs, c) for qs in PAIRS[:2] for c in range(NQ)] if cfg['QO'] else
                          [(qs, c) for c in range(NQ) for qs in PAIRS[:2]]):
                if True:
                    add(lo, start[g] - LAG - 3 + (NC if g else 0), 16 * nt + 46, 14, 16 * nt, cfg['NS'][2], l,
                        functools.partial(unit3, l, p, qs, c, []))
    for R in range(4):
        for C in range(4):
            for c in range(0, NC, 2):
                add(start[6], start[G - 2] - 2, 18, 7, 4, 1, None, (R, C, 16 * c))
    when = spread_jobs([j[:3] for j in jobs], cap, cfg['TAIL'])
    evs = [e[:1] + e[2:] for e in sorted((t % T, ts[0] % T, ji, u) for ji, ts in enumerate(when) for u, t in enumerate(ts))]
    half = {}
    for e, (t, ji, u) in enumerate(evs):
        half[(ji, u)] = 2 * t + (0 if cfg['DBL'] and e + 1 < len(evs) and evs[e + 1][0] == t and (e == 0 or evs[e - 1][0] != t) else 1)
    SEG = cfg['SEG']
    for sg, seeds in enumerate(cfg['SEEDS']):
        mine = [e for e, ev in enumerate(evs) if ev[0] // SEG == sg]
        for seed in seeds:
            for e in mine:
                _, ji, u = evs[e]
                r = (e * 2654435761 + seed * 97531 + 12345) * 2246822519 % 4294967296 >> 8
                if r % 100 >= cfg['PJ']:
                    continue
                h = half[(ji, u)] + (2, -2, 1, -1, 2, -2)[r // 100 % 6]
                off = when[ji][u] - when[ji][u] % T
                lo_ = max(2 * (jobs[ji][0] - off), 2 * sg * SEG, half[evs[e - 1][1:]] + 1 if e else 0)
                hi_ = min(2 * (jobs[ji][1] - off) + 1, 2 * (sg + 1) * SEG - 1,
                          half[evs[e + 1][1:]] - 1 if e + 1 < len(evs) else 2 * (T - cfg['TAIL']))
                if lo_ <= h <= hi_:
                    half[(ji, u)] = h
    if cfg.get('SHOW'):
        for g in range(7, 14):
            rg = range(start[g], start[g + 1])
            print('  ', ''.join('%2d' % round(10 * use[t]) for t in rg))
            print('  ', ''.join('%2s' % ''.join((str(len(w)) if u == 0 else '.') for w in when for u, x in enumerate(w) if x % T == t) for t in rg))
    plan = {}
    for _, ji, u in evs:
        plan.setdefault(half[(ji, u)] // 2, []).append((half[(ji, u)] % 2, jobs[ji][3], jobs[ji][4], STAGES[jobs[ji][5]][u]))
    if cfg.get('PLANOUT') is not None:
        kind = lambda j: 'conv' if j[3] is None else 'fin' if j[3] == 'fin' else j[4].func.__name__ + str(j[4].args[1] if j[4].func.__name__ == 'unit2' else j[4].args[2])
        cfg['PLANOUT'].update(ev=[(half[(ji, u)], kind(jobs[ji]), u, jobs[ji][2][u]) for _, ji, u in evs], use=use,
                              rd=[(outs[g][1], str(rd)) for g, rd, t0, n in sched for _ in range(n)])
    assert all((ts[0] < 0) == (ts[-1] < 0) for ts in when)
    carried = [(job[4], job[5]) for ts, job in zip(when, jobs) if ts[0] < 0]

    def w_copy(l):
        return pltpu.make_async_copy(w_hbm.at[l], w_ref.at[l], sem.at[l])

    def w0_copy(u):
        return pltpu.make_async_copy(w_hbm.at[0, :, u], w_ref.at[0, :, u], sem.at[L + 10 + u])

    def in_copy(t, slot):
        return pltpu.make_async_copy(x_hbm.at[pl.ds(pl.multiple_of(t * TM, 32), TM)], xn2_ref.at[slot], sem.at[L + slot])

    def out_copy(t, slot, part):
        r0, nr = ((0, 2 * Mh), (2 * Mh, Mh), (3 * Mh, Mh))[part]
        return pltpu.make_async_copy(o2_ref.at[slot, pl.ds(r0, nr)],
                                     o_hbm.at[pl.ds(pl.multiple_of(t * TM + r0, 32), nr)],
                                     sem.at[L + 4 + 3 * slot + part])

    xr_in = pltpu.make_async_copy(x_hbm.at[pl.ds(NMAIN * TM, R0)], xr_ref, sem.at[L + 2])
    xr_out = pltpu.make_async_copy(xr_ref, o_hbm.at[pl.ds(NMAIN * TM, R0)], sem.at[L + 2])
    b_in = pltpu.make_async_copy(b_hbm, b_ref, sem.at[L + 3])

    def prologue():
        b_in.start()
        for u in range(8):
            w0_copy(u).start()
        xr_in.start()
        in_copy(0, 0).start()
        for l in range(1, L):
            w_copy(l).start()
        in_copy(min(1, NMAIN - 1), 1).start()
        b_in.wait()
        for l in range(L):
            bf_ref[l] = b_ref[l:l + 1, :].astype(f32)

        def bias_tiles(l, carry):
            b = jnp.broadcast_to(bf_ref[l] + (l == 0).astype(f32), (8, D))
            for u, site in enumerate(BIAS):
                terms = [b[:, key * 128:(key + 1) * 128] * cf for key, cf in sorted(bias_coefs(*site).items()) if cf != 0.0]
                bt_ref[l, u] = functools.reduce(lambda x, y: x + y, terms)
            return carry
        jax.lax.fori_loop(0, L, bias_tiles, 0)
        if cfg.get('FAST'):
            return

        def slab(u, carry):
            w0_copy(u).wait()
            zero = jax.lax.shift_right_logical(u, 12)
            prep(0, u, iter(lambda: None, 0), zero, kb0)
            return zero
        zero = jax.lax.fori_loop(0, cfg['NSLAB'], slab, 0)

        def plain(l, xbf, x0f, x, na, free, never, j0=0, j1=D // 128):
            passes = []
            for jt in range(j0, j1):
                cols = slice(jt * 128, (jt + 1) * 128)
                ya = _dot(xbf[:, :D // 2], w_ref[l, 0:4, :, :, cols].reshape(D // 2, 128)) + bf_ref[l, :, cols]
                passes += [ya, _dot(xbf[:, D // 2:], w_ref[l, 4:8, :, :, cols].reshape(D // 2, 128)) + ya]
            xp_ref[0, :, j0 * 128:j1 * 128] = x0f * jnp.concatenate(passes[1::2], axis=1) + x
            for u in range(na):
                f_ = (u - free) * len(passes) * (R0 // 8) // (na - free)
                if cfg['PPH'] is not None:
                    f_ = f_ // 2 * 2 + cfg['PPH']
                ps, rr = divmod(f_, R0 // 8)
                yield None if u < free else (never, passes[ps][rr * 8:rr * 8 + 8, :])

        for u in range(cfg['NSLAB'], 8):
            w0_copy(u).wait()
        xr_in.wait()
        never = jnp.broadcast_to(zero, (8, 128)) != 0
        jm = cfg['JM']
        x0f = xr_ref[:, :jm * 128].astype(f32)
        xp_ref[1, :, :jm * 128] = x0f
        anchors = plain(0, xr_ref[...], x0f, x0f, (8 - cfg['NSLAB']) * (28 + len(prods3)), cfg['AFREE'], never, 0, jm)
        for u in range(cfg['NSLAB'], 8):
            prep(0, u, anchors, zero, (kb0, kb1)[u % 2])
        in_copy(0, 0).wait()
        x0f = xr_ref[:, jm * 128:].astype(f32)
        xp_ref[1, :, jm * 128:] = x0f
        units = [(R, C, r) for R in range(4) for C in range(4) for r in range(0, Mh, 32)]
        anchors = plain(0, xr_ref[...], x0f, x0f, len(units) + sum(len(STAGES[n]) for _, n in carried) + 2, 4, never, jm)
        for R, C, r in units[:len(units) // 2]:
            conv(xn2_ref.at[0], zero, R, C, r, min(32, Mh - r), next(anchors))
        for fn, n in carried:
            st8 = {}
            for group in STAGES[n]:
                anchor = next(anchors)
                fn(st8, group, zero, jax.lax.shift_right_logical(zero, 1), anchor)
        for R, C, r in units[len(units) // 2:]:
            conv(xn2_ref.at[0], zero, R, C, r, min(32, Mh - r), next(anchors))

        def layer(l, carry):
            w_copy(l).wait()
            zero = jax.lax.shift_right_logical(l, 12)
            x = xp_ref[0]
            anchors = plain(l, x.astype(bf16), xp_ref[1], x, 8 * (28 + len(prods3)), cfg['AFREE'],
                            jnp.broadcast_to(zero, (8, 128)) != 0)
            for u in range(8):
                prep(l, u, anchors, zero, (kb0, kb1)[u % 2])
            return carry

        jax.lax.fori_loop(1, L, layer, 0)
        xr_ref[...] = xp_ref[0].astype(bf16)
        xr_out.start()

    def main(tile, carry):
        zs, za = jax.lax.shift_right_logical(tile, 12), jax.lax.shift_right_logical(tile, 13)
        never = jnp.broadcast_to(zs, (8, 128)) != 0
        slot = tile % 2
        in_copy(jnp.minimum(tile + 2, NMAIN - 1), slot).start()
        in_copy(jnp.minimum(tile + 1, NMAIN - 1), 1 - slot).wait()

        @pl.when(tile > 1)
        def _():
            for part in range(3):
                out_copy(tile - 2, slot, part).wait()

        xn_ref = xn2_ref.at[1 - slot]
        o_ref = o2_ref.at[slot]
        def rows(h, r0):
            if isinstance(h, tuple):
                return slice(r0 + h[0], r0 + h[0] + h[1])
            return slice(r0, r0 + Mh) if h is None else slice(r0 + h * Mq, r0 + (h + 1) * Mq)

        def ld(loc, h=None, z=0):
            return loc[0][(z,) + loc[1] + (rows(h, loc[2]),)]

        def st(loc, v, h=None):
            loc[0][(za if h == 1 and not loc[1] and cfg['ZB'] else zs,) + loc[1] + (rows(h, loc[2]),)] = v

        def by_half(v, h, fn):
            if isinstance(h, tuple):
                h = h[0] // Mq
            return fn(v, h) if h is not None else jnp.concatenate([fn(v[:Mq], 0), fn(v[Mq:], 1)], axis=0)

        def gather(ref, idx, n, pos):
            if cfg['NOBC']:
                return ref[idx + (slice(0, n), slice(16 * pos, 16 * pos + 16))].reshape(16 * n, 128)
            return ref.bitcast(u32)[idx + (slice(0, n), slice(8 * pos, 8 * pos + 8))].reshape(8 * n, 128)

        as_bf16 = lambda v: v if cfg['NOBC'] else pltpu.bitcast(v, bf16)

        def lhs2(p, q):
            ref, u = s2loc(p)
            return as_bf16(jnp.concatenate([gather(ref, (0, u, k), NC, q2[p].index(q)) for k in range(2)], axis=1))

        def rhs2(l, p, q, n):
            return as_bf16(gather(t2[p], (l, n), 16, q2[p].index(q)))

        def dot3(l, p, q, r):
            qs = next(qs for qs in PAIRS if q in qs)
            return _dot(as_bf16(gather(s3[(p, qs)], (0, qs.index(q)), NQ, ORD.index(r))),
                        as_bf16(gather(t3_ref, (l, prods3.index((p, q))), 8, ORD.index(r))))

        def add_bias(v, l, site, h):
            def one(x, hh):
                b = bt_ref[l, BIAS.index(site + (hh,))]
                return (x.reshape(Mq // 8, 8, 128) + b).reshape(Mq, 128)
            return by_half(v, h, one)

        def outer_act(l, p, i, j, n, d, h, part=None):
            bt, stores, finals = OACT[p]
            if part == 'stores':
                finals = []
            if part == 'finals':
                bt, stores = [], []
            if bt:
                d = add_bias(d, l, (p, False, i, j, n), h)
            cache = {'d': d}
            def comb(terms):
                for _, src in terms:
                    if isinstance(src, str) and src not in cache:
                        cache[src] = ld(oloc(src, i, j, n), h)
                v = lincomb([(s, cache[src]) for s, src in terms if isinstance(src, str)])
                for _, src in terms:
                    if not isinstance(src, str):
                        v = add_bias(v, l, (p, True, i, j, n), h)
                return v
            fin = [(IJ, comb(terms)) for IJ, terms in finals]
            for name, v in [(name, comb(terms)) for name, terms in stores]:
                st(oloc(name, i, j, n), v, h)
            for (I, J), y in fin:
                R, C = 2 * I + i, 2 * J + j
                xn = ld(x0loc(R, C, n), h) * y
                if l > 0:
                    xn = xn + ld(xloc(l, R, C, n), h)
                if l < L - 1:
                    st(xloc(l + 1, R, C, n), xn, h)
                else:
                    xn = by_half(xn, h, lambda x, hh: x if scale(R, C, hh, n) == 1.0 else x * (1.0 / scale(R, C, hh, n)))
                    o_ref[rows(h, R * Mh), C * H + n * 128:C * H + (n + 1) * 128] = xn.astype(bf16)

        def inner_act(g, l, p, kind, n, h, P, Q, part=None):
            vloc = oloc(raw_slot(p), 0, 1, n) if raw_slot(p) else iloc(g, 'v', n)
            if kind == '35':
                st(iloc(g, 's', n), Q + ld(iloc(g, 'm1', n), h), h)
                if not raw_slot(p):
                    st(vloc, P, h)
                outer_act(l, p, 0, 1, n, P, h)
            elif kind == '47':
                st(iloc(g, 'u', n), Q + ld(vloc, h), h)
                outer_act(l, p, 0, 0, n, P + ld(iloc(g, 's', n), h), h)
            else:
                outer_act(l, p, 1, 1, n, ld(iloc(g, 's', n), h) - Q, h, part)
                outer_act(l, p, 1, 0, n, P + ld(iloc(g, 'u', n), h), h, part)

        def issue(l, p, rd):
            kind, n = rd
            if kind == 'x':
                return [dot3(l, p, q, 1) for q in (3, 5, 4, 7)]
            if kind == 'y':
                return [dot3(l, pp, q, 1) for pp in (p, SEL3[SEL3.index(p) + 1]) for q in (2, 6)]
            if isinstance(n, str):
                if cfg['MO']:
                    d = [dot3(l, p, int(q), int(r)) for q in kind for r in n]
                    return [d[0], d[2], d[1], d[3]]
                return [dot3(l, p, int(q), int(r)) for r in n for q in kind]
            if cfg['GR']:
                ops = [(lhs2(p, 1),) * 2, (rhs2(l, p, 1, 0), rhs2(l, p, 1, 1))] if kind == '1' else [
                    [lhs2(p, int(q)) for q in kind], [rhs2(l, p, int(q), n) for q in kind]]
                d = [_dot(a[:, k * 128:(k + 1) * 128], b[k * 128:(k + 1) * 128]) for a, b in zip(*ops) for k in range(2)]
                return [d[0] + d[1], d[2] + d[3], d[cfg['GR'] - 1]]
            if kind == '1':
                lhs = lhs2(p, 1)
                return [_dot(lhs, rhs2(l, p, 1, 0)), _dot(lhs, rhs2(l, p, 1, 1))]
            return [_dot(lhs2(p, int(q)), rhs2(l, p, int(q), n)) for q in kind]

        def consume(g, l, p, rd, res):
            kind, n = rd
            if n == '1':
                for u, where in enumerate((('35', False), ('47', False)) if kind == 'x' else (('26', False), ('26', True))):
                    for al in range(2):
                        st(jloc(where[0], '1', al, where[1]), res[2 * u + al], 0)
            elif isinstance(n, str):
                sm = [res[al] + res[2 + al] for al in range(2)]
                df = [res[al] - res[2 + al] for al in range(2)]
                J = lambda name, al: ld(jloc(kind, name, al, name == '1' and kind == '26' and p in SEL3[1::2]), 0)
                part = 'stores' if n in cfg['DEFER'] else None
                done = lambda h, nn, m: inner_act(g, l, p, kind, nn, h, m[0] + m[1], m[0] - m[1], part)
                O, I = (lambda i, j: oloc(raw_slot(p), i, j, 1)), (lambda name: iloc(g, name, 1))
                rec = lambda al: [(s, ld(loc, 0, za if cfg['ZB'] else 0)) for s, loc in {
                    '35': [[(1, O(0, 1))], [(1, I('s')), (-1, I('m1'))]],
                    '47': [[(1, O(0, 0)), (-1, I('s'))], [(1, I('u')), (-1, O(0, 1))]],
                    '26': [[(1, O(1, 0)), (-1, I('u'))], [(1, I('s')), (-1, O(1, 1))]]}[kind][al]]
                if n == '35':
                    for al in range(2):
                        st(jloc(kind, 's', al), df[al] + J('1', al), 0)
                    done(0, 1, sm)
                elif n == '47':
                    if cfg['HY'] == 1:
                        for al in range(2):
                            st(jloc(kind, 'u', al), df[al], 0)
                    else:
                        for al, v in enumerate((df[0] + df[1], df[0] - df[1])):
                            st(jloc(kind, 'u', al), lincomb([(1, v)] + rec(al)), 0)
                    done(0, 0, [sm[al] + J('s', al) for al in range(2)])
                else:
                    if cfg['HY'] == 1:
                        m = [sm[al] + J('u', al) for al in range(2)]
                        P, Q = lincomb([(1, m[0] + m[1])] + rec(0)), lincomb([(1, m[0] - m[1])] + rec(1))
                    else:
                        P, Q = (sm[0] + sm[1]) + J('u', 0), (sm[0] - sm[1]) + J('u', 1)
                    done(1, 1, [J('s', al) - df[al] for al in range(2)])
                    inner_act(g, l, p, kind, 0, 1, P, Q, part)
            elif kind == '1':
                st(iloc(g, 'm1', 0), res[0])
                st(iloc(g, 'm1', 1), res[1])
            else:
                inner_act(g, l, p, kind, n, None, res[0] + res[1], res[0] - res[1])

        state = {}
        for g, rd, t0, n in sched:
            l, p = outs[g]
            if t0 == start[G - 1]:
                out_copy(tile, slot, 0).start()
            if t0 + n == T:
                out_copy(tile, slot, 1).start()
            res = issue(l, p, rd)
            if cfg['EO']:
                consume(g, l, p, rd, res)
            for t in range(t0, t0 + n):
                for ph, l2, fn, group in plan.get(t, []):
                    gr = 16 * (t - t0) + 8 * ph
                    if cfg['GF']:
                        gr = 16 * (t - t0) + 8 * (1 - ph)
                    gs = cfg['GS']
                    gate = res[2 if len(res) == 3 else cfg['GM']][gr:gr + 8, :]
                    if cfg['GADD'] and isinstance(rd[1], str) and rd[1] != '1':
                        gate = gate + res[2 + gs % 2][gr:gr + 8, :]
                    elif gs == 2 and rd[0] != '1' and rd[1] != '1':
                        gate = gate + res[1][gr:gr + 8, :]
                    if l2 == 'fin':
                        lf, pf, nf, r0 = fn
                        for j in range(2):
                            d = ld(oloc(raw_slot(pf), 1, j, nf), (r0, 16))
                            d = tie(tie(d, (never, gate)), (never, gate), 8)
                            outer_act(lf, pf, 1, j, nf, d, (r0, 16), 'finals')
                    elif l2 is None:
                        conv(xn_ref, zs, *fn, min(32, Mh - fn[2]), (never, gate))
                    else:
                        fn(state.setdefault(id(fn), {}), group, zs, za, (never, gate))
            if not cfg['EO']:
                consume(g, l, p, rd, res)
        out_copy(tile, slot, 2).start()
        return carry

    prologue()
    jax.lax.fori_loop(0, NMAIN, main, 0)
    xr_out.wait()
    in_copy(NMAIN - 1, (NMAIN - 1) % 2).wait()
    for t in range(max(NMAIN - 2, 0), NMAIN):
        for part in range(3):
            out_copy(t, t % 2, part).wait()


DEFAULT = dict(SEL=(3, 5, 4, 7), SEL3=(3, 5, 4, 7), XC={B12: 5, B11: 1, B22: 7, B21: 2}, AFREE=4, NOBC=0, FOLD=1, MO=1, GR=2, NS=(2, 3, 3, 4), GM=0, DBL=1, GS=0, GF=0, EO=0, KP=16, PPH=None, ZB=0, HY=1, HOLD=0, PORT=0.9, PS=0, NSLAB=6, JM=3, XP=40, XO=16, DEFER=('26',), EW=12, KW=(1,) * 5, CM=(1,) * 7, SEEDS=(), SEG=32, PJ=20, QO=0, TIEL=2, GADD=0, TF=0, T8=0, TAIL=6,
               CS=0.5, CL=0.3, UL=0.8, CAP=0.85, FR=((1.,), (.4, .6), (.35, .37, .28), (.16, .26, .31, .27),
                   (.35, .29, .08, .28), (.16, .26, .26, .05, .27)))


def build(TM=640, **kw):
    def f(x0, ws, bs):
        B, D = x0.shape
        L = ws.shape[0]
        cfg = dict(DEFAULT, **kw)
        Mh = TM // 4
        MP = Mh + 32
        nmain = (B - 1) // TM
        R0 = B - nmain * TM
        pairs3, q2 = layout(cfg)
        n3 = sum(2 * len(v) for v in pairs3.values())
        pad = lambda n: n + (2 - n) % 4
        V = pltpu.VMEM
        half = V((1, MP, 128), f32)
        XP = Mh + cfg['XP']
        scratch = ([V((1, 2, 2, 2, XP, 128), f32)] * 4 + [V((1, 2, 4, 2, XP, 128), f32)] * 6 + [half] * (16 + 56 + 26)
                   + [V((1, 1 + (p == 2), 2, pad(Mh // 16), 16 * len(q2[p]), 128), bf16) for p in (1, 3, 4, 5, 7, 2)]
                   + [V((1, 2, pad(Mh // 32), 112, 128), bf16)] * (n3 // 2)
                   + [V((L, 2, 16, 16 * len(q2[p]), 128), bf16) for p in range(1, 8)]
                   + [V((L, n3, 8, 112, 128), bf16), V((1, 4, 16 * n3 + cfg['KP'], 128), f32), V((1, 4, 16 * n3 + cfg['KP'], 128), f32),
                      V((L, len(BIAS), 8, 128), f32), V((8, 1, D), f32), V((2, TM, D), bf16), V((2, TM, D), bf16), V((L, 8, 8, 16, D), bf16),
                      V((R0, D), bf16), V((2, R0, D), f32), V((L, D), bf16), pltpu.SemaphoreType.DMA((L + 18,))])
        anyspec = pl.BlockSpec(memory_space=pl.ANY)
        return pl.pallas_call(
            functools.partial(_kernel, L=L, TM=TM, R0=R0, NMAIN=nmain, D=D, cfg=cfg),
            in_specs=[anyspec, anyspec, anyspec],
            out_specs=anyspec,
            out_shape=jax.ShapeDtypeStruct((B, D), x0.dtype),
            scratch_shapes=scratch,
            compiler_params=pltpu.CompilerParams(
                vmem_limit_bytes=110 * 1024 * 1024,
                internal_scratch_in_bytes=65536,
                disable_bounds_checks=True,
            ),
        )(x0, ws.reshape(L, 8, 8, 16, D), bs)
    return f


@jax.jit
def pallas_standalone__dcn_v2_cross__recsys_kernel(x0, ws, bs):
    return build(TM=640)(x0, ws, bs)
```

```python
import functools

import jax
import jax.numpy as jnp
import jax.experimental.pallas as pl
import jax.experimental.pallas.tpu as pltpu

f32 = jnp.float32
bf16 = jnp.bfloat16
u32 = jnp.uint32

B11, B12, B21, B22 = (0, 0), (0, 1), (1, 0), (1, 1)
LA = {1: [(B11, 1), (B22, 1)], 2: [(B11, 1), (B12, 1), (B21, 1), (B22, 1)], 3: [(B11, 1), (B12, -1)],
      4: [(B12, 1), (B22, 1)], 5: [(B11, 1), (B12, 1)], 6: [(B12, 1), (B11, -1), (B21, 1), (B22, -1)],
      7: [(B12, 1), (B22, -1)]}
PAIRS = ((5, 3), (4, 7), (2, 6))
ORD = (3, 5, 4, 7, 1, 2, 6)
D2 = (1.0, 2.0)
BF = {1: 1.0, 2: 0.5, 3: 0.5, 4: 0.5, 5: 0.5, 6: 0.5, 7: 0.5}
OUTER = (3, 5, 1, 4, 7, 2, 6)
OACT = {
    3: ([(1, B12)], [('M3', [(1, 'd')])], []),
    5: ([], [('M5', [(1, 'd')])], [(B12, [(1, 'd'), (1, 'M3')])]),
    1: ([(1, B11), (-1, B12)], [('S', [(1, 'd'), (1, 'M3'), (-1, 'M5')])], []),
    4: ([], [('M4', [(1, 'd')])], []),
    7: ([], [('M7', [(1, 'd')])], [(B11, [(1, 'd'), (1, 'S'), (1, 'M4')])]),
    2: ([(1, B11), (-1, B22)], [('M2', [(1, 'd')]),
        ('U', [(1, 'd'), (1, 'M4'), (-1, 'M7'), (1, 'M3'), (1, 'M5'), (1, ((1, B21), (-1, B12), (-1, B11), (1, B22)))])], []),
    6: ([], [('M6', [(1, 'd')])], [(B22, [(1, 'd'), (1, 'S'), (-1, 'M2')]), (B21, [(1, 'd'), (1, 'U')])]),
}
OSL = {'M3': 0, 'M5': 1, 'S': 2, 'M4': 3, 'M7': 4, 'M2': 6, 'U': 5, 'M6': 7}
ISL = {'m1': 0, 's': 1, 'v': 2, 'u': 3}
STAGES = {1: [(B11, B12, B21, B22)], 2: [(B11, B12), (B21, B22)], 3: [(B11, B12), (B22,), (B21,)],
          4: [(B11,), (B12,), (B22,), (B21,)], 5: [(B11, B12), (B22, 'hold'), ('l1',), (B21,)],
          6: [(B11,), (B12,), (B22, 'hold'), ('l1',), (B21,)]}
BIAS = [(p, extra, i, j, n, h) for p in OUTER for extra in (False, True)
        if (any(not isinstance(x, str) for _, t in OACT[p][1] + OACT[p][2] for _, x in t) if extra else OACT[p][0])
        for i in range(2) for j in range(2) for n in range(2) for h in range(2)]
PREP_ORDER = (2, 6, 3, 5, 1, 4, 7)
LAG = 8


def _dot(a, b):
    return jnp.dot(a, b, preferred_element_type=f32)


def scale(R, C, h, k):
    return D2[R // 2] * D2[R % 2] * D2[h] / (D2[C // 2] * D2[C % 2] * D2[k])


def b_ops(b11, b12, b21, b22):
    r1 = b11 + b22
    g = b12 + b21
    return {1: r1, 2: b11 - b12, 3: b12 - b22, 4: g - r1, 5: b12 + b22, 6: b11 + b12, 7: g + r1}


def lincomb(terms):
    assert terms[0][0] == 1
    acc = terms[0][1]
    for s, v in terms[1:]:
        acc = acc + v if s == 1 else acc - v
    return acc


def raw_slot(p):
    return next((name for name, terms in OACT[p][1] if terms == [(1, 'd')]), None)


def round_usage(p, rd, first, last, defer, hy):
    bt, stores, finals = OACT[p]
    alu = bool(bt) + sum(len(t) - 1 for _, t in stores) + sum(len(t) + (not first) + 2 * last for _, t in finals)
    nst = len(stores) + len(finals)
    nld = len({x for _, t in stores + finals for _, x in t if isinstance(x, str) and x != 'd'}) + len(finals) * (2 - first)
    kind, n = rd
    if defer:
        alu, nst, nld = bool(bt), 1, 0
    elif p == 6 and kind != '35' and n != '35':
        nst -= 1
    if isinstance(n, str):
        e = kind == '47'
        if kind == '26':
            a, st, ld, m = {'35': (10, 2, 9, 2), '47': (10, 2, 9, 2) if hy == 1 else (16, 2, 13, 2), '26': (20, 0, 17, 4) if hy == 1 else (16, 0, 13, 4)}[n]
        else:
            a, st, ld, m = {'1': (0, 4, 5, 0), '35': (9 + e, 3, 8 + e, 1),
                            '47': (9 + e, 3, 8 + e, 1) if hy == 1 else (14 + 2 * e, 3, 11 + 2 * e, 1),
                            '26': (17 + 3 * e, 2, 14 + 3 * e, 2) if hy == 1 else (14 + 2 * e, 2, 11 + 2 * e, 2)}[n]
    else:
        a, st, ld, m = {'1': (2, 2, 4, 0), '35': (5, 2 - bool(raw_slot(p)), 5, 1), '47': (6, 1, 6, 1),
                        '26': (6, 0, 6, 2)}[kind]
    return a + m * alu, st + m * nst, ld + m * nld


def yds(groups, cap):
    n = len(cap)
    speed, cls, gcls = [0.0] * n, [-1] * n, {}
    todo = list(groups)
    while todo:
        pre = [0.0]
        for t in range(n):
            pre.append(pre[-1] + (cap[t] if cls[t] < 0 else 0.0))
        best = None
        for a in sorted({g[0] for g in todo}):
            w = 0.0
            for g in sorted((g for g in todo if g[0] >= a), key=lambda g: g[1]):
                w += g[2]
                d = w / max(pre[g[1] + 1] - pre[a], 1e-9)
                if best is None or d > best[0]:
                    best = (d, a, g[1])
        d, a, b = best
        for t in range(a, b + 1):
            if cls[t] < 0:
                speed[t], cls[t] = d, len(gcls)
        gcls.update({g[:2]: len(gcls) for g in todo if g[0] >= a and g[1] <= b})
        todo = [g for g in todo if not (g[0] >= a and g[1] <= b)]
    return speed, cls, gcls


def spread_jobs(jobs, cap, tail):
    T = len(cap)
    cap3 = cap * 3
    all3 = [(lo + k * T, hi + k * T, ji, k) for k in range(3) for ji, (lo, hi, _) in enumerate(jobs) if lo + k * T >= 0]
    pend = {}
    for j in sorted(all3, key=lambda j: (j[1], j[3], j[2])):
        pend.setdefault(j[:2], []).append(j)
    speed, cls, gcls = yds([w + (sum(sum(jobs[j[2]][2]) for j in q),) for w, q in pend.items()], cap3)
    when = [[] for _ in jobs]
    debt, cur, done = 0.0, None, 0
    for t in range(3 * T):
        while True:
            j = cur
            if j is None:
                rdy = [q[0] for w, q in pend.items() if q and w[0] <= t and (gcls[w] == cls[t] or w[1] <= t)]
                if not rdy:
                    debt = max(debt, 0.0)
                    break
                j = rdy[0]
                nst = len(jobs[j[2]][2])
                if nst > 1 and j[1] > t and (t + tail + 2 * nst) // T != t // T:
                    break
            must = j[1] <= t or (cur is not None and (t + tail + 1) // T != t // T)
            if not must and (cap3[t] == 0.0 or debt > 0.5 * speed[t] * cap3[t]):
                break
            if cur is None:
                pend[j[:2]].pop(0)
                cur, done = j, 0
            debt += jobs[j[2]][2][done]
            if j[3] == 1:
                when[j[2]].append(t - T)
            done += 1
            if done == len(jobs[j[2]][2]):
                cur = None
        debt -= speed[t] * cap3[t]
    return when


def layout(cfg):
    sel, sel3 = cfg['SEL'], cfg['SEL3']
    pairs3 = {p: [qs for qs in PAIRS if p in sel3 or (p in sel and qs != (2, 6))] for p in range(1, 8)}
    q2 = {p: [q for q in ORD if not any(q in qs for qs in pairs3[p])] for p in range(1, 8)}
    return pairs3, q2


def _kernel(x_hbm, w_hbm, b_hbm, o_hbm, *scratch, L, TM, R0, NMAIN, D, cfg):
    H, Mh, Mq = D // 4, TM // 4, TM // 8
    NC, NQ = Mh // 16, Mq // 16
    MP = Mh + 32
    SEL, SEL3 = cfg['SEL'], cfg['SEL3']
    pairs3, q2 = layout(cfg)
    prods3 = [(p, q) for p in SEL for qs in pairs3[p] for q in qs]
    assert H == 256 and L % 2 == 0 and Mq % 16 == 0 and all(raw_slot(p) for p in SEL)
    it = iter(scratch)
    take = lambda n: [next(it) for _ in range(n)]
    x0b, xb, ib, ob, jb = take(4), take(7), take(16), take(64), take(26)
    joint = q2[2] == q2[6]
    MAT = cfg['MAT'] and joint and 2 in SEL
    s2 = dict(zip(range(1, 8), take(7)))
    s3 = {(p, qs): next(it) for p in SEL for qs in pairs3[p]}
    t2 = dict(zip(range(1, 8), take(7)))
    t3_ref, kb0, kb1, bt_ref, bf_ref, xn2_ref, o2_ref, w_ref, xr_ref, xp_ref, b_ref, sem = it

    xset = lambda l: 6 if l == 'O' else 4 if l == 0 else (l % 2) * 2
    xoff = lambda I, J: cfg['XO'] * ((I + J) % 2)
    xloc = lambda l, R, C, k: (xb[xset(l) + R // 2], (R % 2, C, k), xoff(R // 2, C // 2))
    x0loc = lambda R, C, k: (x0b[(R // 2) * 2 + C // 2], (R % 2, C % 2, k), 8 + xoff(R // 2, C // 2))
    iloc = lambda g, name, n: (ib[((g % 2) * 4 + ISL[name]) * 2 + n], (), 8 * ISL[name])
    oloc = lambda name, i, j, n: (ob[(OSL[name] * 4 + i * 2 + j) * 2 + n], (), 8 * ((OSL[name] + 2 * j) % 4))

    def jloc(kind, name, al, second=False):
        i = 24 + al if second else (('35', '47', '26').index(kind) * 4 + ('1', 's', 'u', 'v').index(name)) * 2 + al
        return jb[i], (), 8 * ((i + i // 2) % 4)

    def s2loc(p):
        return (s2[2], (2, 6).index(p)) if p in (2, 6) and joint else (s2[p], 0)

    def bias_coefs(p, extra, i, j, n, h):
        where = [(1, i, j, n, h)]
        if extra:
            terms = next(x for _, t in OACT[p][1] + OACT[p][2] for _, x in t if not isinstance(x, str))
        else:
            terms = OACT[p][0]
            w = [(1, i, j)] + [(-1, 0, 1)] * bool(raw_slot(p) and (i, j) == B21)
            where = [x + (n, h) for x in w]
            if (h, n) == (1, 0) and PAIRS[{B12: 0, B11: 1}.get((i, j), 2)] in pairs3[p]:
                where += [(-sg, ii, jj, 1, 0) for sg, ii, jj in w]
        coef = {}
        for sg, ii, jj, nn, hh in where:
            for cf, (I, J) in terms:
                key = (2 * J + jj) * 2 + nn
                coef[key] = coef.get(key, 0.0) + sg * cf * scale(2 * I + ii, 2 * J + jj, hh, nn)
        return coef

    def tie(v, anchor, r=0):
        if anchor is None:
            return v
        return jnp.concatenate([v[:r]] * (r > 0) + [jax.lax.select(anchor[0], anchor[1], v[r:r + 8])] + [v[r + 8:]] * (r + 8 < v.shape[0]), axis=0)

    def consts(anchor, ss, reps):
        one = {s: jnp.full((8, 128), s, f32) for s in set(ss)}
        if anchor is not None:
            one = {s: jax.lax.select(anchor[0], anchor[1], v) for s, v in one.items()}
        return jnp.concatenate([one[s] for s in ss for _ in range(reps)], axis=0)

    def conv(src, zs, R, C, r, nr, anchor=None):
        v = src[R * Mh + r:R * Mh + r + nr, C * H:(C + 1) * H].astype(f32)
        for k in range(2):
            buf, idx, off = xloc(0, R, C, k)
            sv = consts(anchor, [scale(R, C, (r + u) // Mq, k) for u in range(0, nr, 16)], 2)
            buf[(zs,) + idx + (slice(off + r, off + r + nr),)] = v[:, k * 128:(k + 1) * 128] * sv

    cnt = {}
    def block_sum(l, terms, ii, jj, kk, r, save, zs, za, anchor, late=None):
        rng = lambda t: slice(t[0], t[-1] + 1)
        keys = [(i, j, k) for i in ii for j in jj for k in kk]
        vals = []
        for u, ((I, J), s) in enumerate(terms):
            ref, r0 = xb[xset(l) + I], xoff(I, J) + r
            v = ref[za if u == 0 else 0, rng(ii), 2 * J + jj[0]:2 * J + jj[-1] + 1, rng(kk), r0:r0 + 16, :]
            if (I, J) in save:
                sv = consts(anchor, [1.0 / scale(2 * I + i, 2 * J + j, r // Mq, k) for i, j, k in keys], 2)
                x0b[I * 2 + J][zs, rng(ii), rng(jj), rng(kk), r0 + 8:r0 + 24, :] = v * sv.reshape(v.shape)
            v = v.reshape(16 * len(keys), 128)
            if u == 0 and late is not None and anchor is not None:
                cnt[xset(l)] = cnt.get(xset(l), -1) + 1
                if cnt[xset(l)] % cfg['GE'] == 0:
                    ref[0, 0, 0, 0, Mh + 24:Mh + 32, :] = anchor[1]
                at = 16 * keys.index(late)
                top = v[at:at + 8] if cfg['NL'] else ref[za, late[0], 2 * J + late[1], late[2], r0:r0 + 8, :]
                if cfg['TIEL'] == 2:
                    top = jax.lax.select(anchor[0], anchor[1], top)
                v = jnp.concatenate([v[:at]] * (at > 0) + [top, v[at + 8:]], axis=0)
            vals.append((s, v))
        v = lincomb(vals)
        if cfg['TIEL'] == 3 and late is not None:
            v = tie(v, anchor, 16 * keys.index(late))
        return v

    def release(qs, store, st8, anchor):
        v = st8['l1']
        if anchor is not None:
            n = v.shape[0]
            top = jax.lax.select(jnp.broadcast_to(anchor[0], (n, 8, 128)), jnp.broadcast_to(anchor[1], (n, 8, 128)), v[:, :8])
            v = jnp.concatenate([top, v[:, 8:]], axis=1)
        r0 = 16 * qs.index(1)
        store(slice(r0, r0 + 16), v.astype(bf16))

    def finish(e, f, group, qs, store, st8, anchor, hold=False, keep=None):
        a = e[None] if f is None else jnp.concatenate([e + f, e - f], axis=0).reshape(2, e.shape[0], 128)
        for u, b in enumerate(group):
            st8[b] = a if len(group) == 1 else a[:, 16 * u:16 * u + 16]
            if keep:
                keep(b, st8[b])
        ops = {}
        if B12 in group and 3 in qs:
            ops[3], ops[5] = st8[B11] - st8[B12], st8[B11] + st8[B12]
        if B22 in group:
            if 4 in qs:
                ops[4], ops[7] = st8[B12] + st8[B22], st8[B12] - st8[B22]
            ops[1] = st8['l1'] = st8[B11] + st8[B22]
        if B21 in group:
            g = st8[B12] + st8[B21]
            ops[2], ops[6] = g + st8['l1'], g - st8['l1']
        now = [q for q in qs if q in ops and not (hold and q == 1)]
        if now:
            r0 = 16 * qs.index(now[0])
            store(slice(r0, r0 + 16 * len(now)), jnp.concatenate([ops[q] for q in now], axis=1).astype(bf16))

    def unit2(l, ps, c, k, save, st8, group, zs, za, anchor):
        def store(rows, v):
            s2[ps[0]][zs, :, k, c, rows, :] = v
        if group == ('l1',):
            return release(q2[ps[0]], store, st8, anchor)
        hold, group = 'hold' in group, tuple(b for b in group if b != 'hold')
        ii, jj = sorted({b[0] for b in group}), sorted({b[1] for b in group})
        bs = lambda terms, late: block_sum(l, terms, ii, jj, [k], 16 * c, save, zs, za, anchor, late)
        f = None if len(ps) == 1 else bs([(B11, 1), (B22, 1)], None)
        e = bs(LA[ps[0]] if len(ps) == 1 else [(B12, 1), (B21, 1)], (ii[0], jj[-1], k))
        def keep(b, v):
            if b != B21:
                for J in range(2):
                    xb[6][zs, b[0], 2 * J + b[1], k, xoff(0, J) + 16 * c:xoff(0, J) + 16 * c + 16, :] = v[J]
        if f is None or joint:
            return finish(e, f, group, q2[ps[0]], store, st8, anchor, hold, keep if f is not None and MAT else None)
        for p, v in zip(ps, (e + f, e - f)):
            def store1(rows, w):
                s2[p][zs, :, k, c, rows, :] = w
            finish(v, None, group, q2[p], store1, st8.setdefault(p, {}), anchor)

    def unit3(l, p, qs, c, save, st8, group, zs, za, anchor):
        def store(rows, w):
            s3[(p, qs)][zs, :, c, rows, :] = w
        if group == ('l1',):
            return release(ORD, store, st8, anchor)
        hold, group = 'hold' in group, tuple(b for b in group if b != 'hold')
        for h in sorted({b[0] for b in group}):
            grp = tuple(b for b in group if b[0] == h)
            kk = [b[1] for b in grp]
            ii, jj = {(5, 3): ([0], [0, 1]), (4, 7): ([0, 1], [1]), (2, 6): ([0, 1], [0, 1])}[qs]
            src = ('O', [((0, (2, 6).index(p)), 1)]) if MAT and p in (2, 6) else (l, LA[p])
            v = block_sum(*src, ii, jj, sorted(kk), h * Mq + 16 * c, save, zs, za, anchor,
                          (0, (0 if cfg['TF'] else 1) if qs == (2, 6) else jj[0], max(kk)) if h == group[-1][0] else None)
            n = 16 * len(kk)
            piece = lambda u: v[u * n:(u + 1) * n]
            if qs == (2, 6):
                e, f = piece(1) + piece(2), piece(0) + piece(3)
                r0 = 16 * q2[p].index(1)
                s2[p][zs, 0, min(kk):max(kk) + 1, h * NQ + c, r0:r0 + 16, :] = f.reshape(len(kk), 16, 128).astype(bf16)
            else:
                e, f = piece(0), piece(1)
            finish(e, f, tuple(sorted(grp)), ORD, store, st8, anchor, hold)

    def prep(l, u, anchors, zero, kb):
        for k in range(2):
            wide = [w_ref[l, R * 2 + k, u].astype(f32) for R in range(4)]
            for n in range(2):
                def blk(R, C):
                    v = wide[R][:, C * H + n * 128:C * H + (n + 1) * 128]
                    s = D2[R // 2] / D2[C // 2]
                    return v if s == 1.0 else v * s
                O = {(i, j): b_ops(blk(i, j), blk(i, 2 + j), blk(2 + i, j), blk(2 + i, 2 + j)) for i, j in (B11, B12, B21, B22)}
                for p in PREP_ORDER:
                    anchor = next(anchors)
                    fold = 0.5 if cfg['FOLD'] and p in SEL else 1.0
                    s = BF[p] * 0.5 * D2[k] / D2[n] * fold
                    cs = {f: consts(anchor, [s * f], 2) for f in (0.5, 1.0, 2.0)}
                    T = b_ops(*[O[(i, j)][p] * cs[D2[i] / D2[j]] for i, j in (B11, B12, B21, B22)])
                    sq = {q: 2.0 * BF[q] / fold for q in q2[p]}
                    t2[p][l, n, k * 8 + u] = jnp.concatenate(
                        [T[q] if sq[q] == 1.0 else T[q] * sq[q] for q in q2[p]], axis=0).astype(bf16)
                    mine = [e for e, pq in enumerate(prods3) if pq[0] == p]
                    if mine:
                        kb[zero, k * 2 + n, 16 * mine[0]:16 * mine[-1] + 16, :] = jnp.concatenate(
                            [T[prods3[e][1]] for e in mine], axis=0)
        for e in range(len(prods3)):
            anchor = next(anchors)
            if cfg['FOLD']:
                n3 = 16 * len(prods3)
                if anchor is not None and cfg['FOLD'] > 1:
                    kb[0, 0, n3:n3 + 8, :] = anchor[1]
                    v = kb[jax.lax.shift_right_logical(zero, 1), :, 16 * e:16 * e + 16, :]
                else:
                    v = kb[0, :, 16 * e:16 * e + 16, :]
                T = b_ops(v[0], tie(v[1], anchor), v[2], v[3])
            else:
                v = kb[0, :, 16 * e:16 * e + 16, :] * consts(anchor, [0.5], 2)
                T = b_ops(v[0], v[1], v[2], v[3])
            T[1] = T[1] + T[1]
            t3_ref[l, e, u] = jnp.concatenate([T[q] for q in ORD], axis=0).astype(bf16)

    def rounds_of(p):
        rs = [('1', None)] + [('x', '1')] * (p in SEL)
        for kind, qs in zip(('35', '47', '26'), PAIRS):
            if kind == '26' and p in SEL3[::2]:
                rs.append(('y', '1'))
            rs += [(kind, r) for r in (('35', '47', '26') if qs in pairs3[p] else (0, 1))]
        return rs

    def deferred(l, p, rd):
        return rd in cfg['DEFER'].get(p, ()) or (l == L - 1 and rd in cfg['DEFL'].get(p, ()))

    outs = [(l, p) for l in range(L) for p in OUTER]
    G = len(outs)
    sched, start, use = [], [], []
    for g, (l, p) in enumerate(outs):
        start.append(len(use))
        for rd in rounds_of(p):
            n = NQ if isinstance(rd[1], str) else NC
            sched.append((g, rd, len(use), n))
            a, st_, ld_ = round_usage(p, rd, l == 0, l == L - 1, deferred(l, p, rd), cfg['HY'])
            if cfg['PORT']:
                use += [max((2 * a + st_ + 2 + 16 / n) / 72 + cfg['PS'] * st_ / 8, cfg['PORT'] * st_ / 8)] * n
            else:
                use += [max(a / 32, st_ / 8, cfg['UL'] * ld_ / 24)] * n
    T = len(use)
    cap = [max(cfg['CAP'] - max(use[t], use[(t + 1) % T]), 0.0) * (t < T - cfg['TAIL']) for t in range(T)]
    for g in range(G):
        for t in range(start[g], (start + [T])[g + 1]):
            cap[t] *= cfg['CM'][g % 7]
    jobs = []
    def add(lo, hi, alu, st_, ld_, nst, l, fn):
        w = alu / 64 + cfg['CS'] * (st_ + nst) / 16 + cfg['CL'] * ld_ / 48
        w *= cfg['KW'][0 if l in (None, 'fin') else nst]
        if cfg['HOLD'] and nst >= 3:
            nst += 2
        jobs.append((lo, max(hi, lo), [w * f for f in cfg['FR'][nst - 1]], l, fn, nst))
    for g, (l, p) in enumerate(outs):
        ready = 7 * l - 2 * all(I == 0 for (I, J), _ in LA[p])
        lo = start[ready] - (T if ready < 0 else 0)
        if cfg['DEFER'].get(7) and ready % 7 == 5 and l > 0:
            lo += cfg['EW'] + 1
        for gg, rd, t0, n_ in sched:
            if gg == g and deferred(l, p, rd):
                if p == 7:
                    due = start[g + 1] + cfg['EW'] if l < L - 1 else start[g + 2] - 1
                elif p == 5:
                    due = start[7 * l + 5] - 1
                elif p == 6:
                    due = (start[g + 1] if l < L - 1 else T - NC) - 1
                else:
                    due = [t for g2, r2, t, _ in sched if g2 == g + 1 and r2[0] == rd[0]][0] - 3
                nops = 4 * sum(len(t) + (x in OACT[p][2]) * (2 + 2 * (l == L - 1)) for x in OACT[p][1][1:] + OACT[p][2] for t in x[1:])
                ws = [(i, j, n, h * Mq + 16 * c) for c in range(NQ) for h, n in {'35': [(0, 1)], '47': [(0, 0)], '26': [(1, 1), (1, 0)]}[rd[1]]
                      for i, j in {'35': [B12], '47': [B11], '26': [B22, B21]}[rd[0]]]
                m_ = 1 if p == 6 else 2
                for u in range(0, len(ws), m_):
                    add(t0 + n_, due, nops * m_ // 2, 3, nops * m_ // 2, 1, 'fin', (l, p, ws[u:u + m_]))
        hi = start[g] - LAG - 3
        nt = len(LA[p])
        save = [b for b, pp in cfg['XC'].items() if pp == p and l == 0]
        if p in SEL3:
            if p in SEL3[1::2]:
                host = 7 * l + OUTER.index(SEL3[SEL3.index(p) - 1])
                hi = [t0 for gg, rd, t0, _ in sched if gg == host and rd[0] == 'y'][0] - LAG - 3
            for c in range(NQ):
                add(lo, hi, 32 * nt + 50 + 32 * len(save), 18 + 32 * len(save), 32 * nt, cfg['NS'][3], l,
                    functools.partial(unit3, l, p, (2, 6), c, save))
        elif p != 6:
            ps = (2, 6) if p == 2 else (p,)
            nq = sum(len(q2[x]) for x in ps)
            alu = 8 * (nt - 2 + len(ps)) + sum(8 if x in SEL else 16 for x in ps) + nq
            if MAT and p == 2:
                hi = start[7 * l + cfg['MAT']] - 3
            for c in range(NC):
                for k in range(2):
                    add(lo, hi, alu + 8 * len(save), nq + 8 * len(save) + 12 * (bool(MAT) and p == 2), 8 * nt, 1 if nq <= 3 else cfg['NS'][4] if nq == 6 else cfg['NS'][0] if nq <= 7 else cfg['NS'][1], l,
                        functools.partial(unit2, l, ps, c, k, save))
        if MAT and p in (2, 6):
            lo, nt = start[7 * l + cfg['MAT']], 1
        if p in SEL:
            for qs, c in ([(qs, c) for qs in PAIRS[:2] for c in range(NQ)] if cfg['QO'] else
                          [(qs, c) for c in range(NQ) for qs in PAIRS[:2]]):
                if True:
                    add(lo, start[g] - LAG - 3 + (NC if g else 0), 16 * nt + 46, 14, 16 * nt, cfg['NS'][2 + (nt == 4)], l,
                        functools.partial(unit3, l, p, qs, c, []))
    for R in range(4):
        for C in range(4):
            for c in range(0, NC, 2):
                add(start[6], start[G - 2] - 2, 18, 7, 4, 1, None, (R, C, 16 * c))
    when = spread_jobs([j[:3] for j in jobs], cap, cfg['TAIL'])
    evs = [e[:1] + e[2:] for e in sorted((t % T, ts[0] % T, ji, u) for ji, ts in enumerate(when) for u, t in enumerate(ts))]
    half = {}
    for e, (t, ji, u) in enumerate(evs):
        half[(ji, u)] = 2 * t + (0 if cfg['DBL'] and e + 1 < len(evs) and evs[e + 1][0] == t and (e == 0 or evs[e - 1][0] != t) else 1)
    SEG = cfg['SEG']
    for sg, seeds in enumerate(cfg['SEEDS']):
        mine = [e for e, ev in enumerate(evs) if ev[0] // SEG == sg]
        for seed in seeds:
            for e in mine:
                _, ji, u = evs[e]
                r = (e * 2654435761 + seed * 97531 + 12345) * 2246822519 % 4294967296 >> 8
                if r % 100 >= cfg['PJ']:
                    continue
                h = half[(ji, u)] + (2, -2, 1, -1, 2, -2)[r // 100 % 6]
                off = when[ji][u] - when[ji][u] % T
                lo_ = max(2 * (jobs[ji][0] - off), 2 * sg * SEG, half[evs[e - 1][1:]] + 1 if e else 0)
                hi_ = min(2 * (jobs[ji][1] - off) + 1, 2 * (sg + 1) * SEG - 1,
                          half[evs[e + 1][1:]] - 1 if e + 1 < len(evs) else 2 * (T - cfg['TAIL']))
                if lo_ <= h <= hi_:
                    half[(ji, u)] = h
    if cfg.get('SHOW'):
        for g in range(7, 14):
            rg = range(start[g], start[g + 1])
            print('  ', ''.join('%2d' % round(10 * use[t]) for t in rg))
            print('  ', ''.join('%2s' % ''.join((str(len(w)) if u == 0 else '.') for w in when for u, x in enumerate(w) if x % T == t) for t in rg))
    plan = {}
    for _, ji, u in evs:
        plan.setdefault(half[(ji, u)] // 2, []).append((half[(ji, u)] % 2, jobs[ji][3], jobs[ji][4], STAGES[jobs[ji][5]][u]))
    if cfg.get('PLANOUT') is not None:
        kind = lambda j: 'conv' if j[3] is None else 'fin' if j[3] == 'fin' else j[4].func.__name__ + str(j[4].args[1] if j[4].func.__name__ == 'unit2' else j[4].args[2])
        cfg['PLANOUT'].update(ev=[(half[(ji, u)], kind(jobs[ji]), u, jobs[ji][2][u]) for _, ji, u in evs], use=use,
                              rd=[(outs[g][1], str(rd)) for g, rd, t0, n in sched for _ in range(n)])
    assert all((ts[0] < 0) == (ts[-1] < 0) for ts in when)
    carried = [(job[4], job[5]) for ts, job in zip(when, jobs) if ts[0] < 0]

    def w_copy(l):
        return pltpu.make_async_copy(w_hbm.at[l], w_ref.at[l], sem.at[l])

    def w0_copy(u):
        return pltpu.make_async_copy(w_hbm.at[0, :, u], w_ref.at[0, :, u], sem.at[L + 10 + u])

    def in_copy(t, slot):
        return pltpu.make_async_copy(x_hbm.at[pl.ds(pl.multiple_of(t * TM, 32), TM)], xn2_ref.at[slot], sem.at[L + slot])

    def out_copy(t, slot, part):
        r0, nr = ((0, 2 * Mh), (2 * Mh, Mh), (3 * Mh, Mh))[part]
        return pltpu.make_async_copy(o2_ref.at[slot, pl.ds(r0, nr)],
                                     o_hbm.at[pl.ds(pl.multiple_of(t * TM + r0, 32), nr)],
                                     sem.at[L + 4 + 3 * slot + part])

    xr_in = pltpu.make_async_copy(x_hbm.at[pl.ds(NMAIN * TM, R0)], xr_ref, sem.at[L + 2])
    xr_out = pltpu.make_async_copy(xr_ref, o_hbm.at[pl.ds(NMAIN * TM, R0)], sem.at[L + 2])
    b_in = pltpu.make_async_copy(b_hbm, b_ref, sem.at[L + 3])

    def prologue():
        b_in.start()
        for u in range(8):
            w0_copy(u).start()
        xr_in.start()
        in_copy(0, 0).start()
        for l in range(1, L):
            w_copy(l).start()
        in_copy(min(1, NMAIN - 1), 1).start()
        b_in.wait()
        for l in range(L):
            bf_ref[l] = b_ref[l:l + 1, :].astype(f32)

        def bias_tiles(l, carry):
            b = jnp.broadcast_to(bf_ref[l] + (l == 0).astype(f32), (8, D))
            for u, site in enumerate(BIAS):
                terms = [b[:, key * 128:(key + 1) * 128] * cf for key, cf in sorted(bias_coefs(*site).items()) if cf != 0.0]
                bt_ref[l, u] = functools.reduce(lambda x, y: x + y, terms)
            return carry
        jax.lax.fori_loop(0, L, bias_tiles, 0)
        if cfg.get('FAST'):
            return

        def slab(u, carry):
            w0_copy(u).wait()
            zero = jax.lax.shift_right_logical(u, 12)
            prep(0, u, iter(lambda: None, 0), zero, kb0)
            return zero
        zero = jax.lax.fori_loop(0, cfg['NSLAB'], slab, 0)

        def plain(l, xbf, x0f, x, na, free, never, j0=0, j1=D // 128):
            passes = []
            for jt in range(j0, j1):
                cols = slice(jt * 128, (jt + 1) * 128)
                ya = _dot(xbf[:, :D // 2], w_ref[l, 0:4, :, :, cols].reshape(D // 2, 128)) + bf_ref[l, :, cols]
                passes += [ya, _dot(xbf[:, D // 2:], w_ref[l, 4:8, :, :, cols].reshape(D // 2, 128)) + ya]
            xp_ref[0, :, j0 * 128:j1 * 128] = x0f * jnp.concatenate(passes[1::2], axis=1) + x
            for u in range(na):
                f_ = (u - free) * len(passes) * (R0 // 8) // (na - free)
                if cfg['PPH'] is not None:
                    f_ = f_ // 2 * 2 + cfg['PPH']
                ps, rr = divmod(f_, R0 // 8)
                yield None if u < free else (never, passes[ps][rr * 8:rr * 8 + 8, :])

        for u in range(cfg['NSLAB'], 8):
            w0_copy(u).wait()
        xr_in.wait()
        never = jnp.broadcast_to(zero, (8, 128)) != 0
        jm = cfg['JM']
        x0f = xr_ref[:, :jm * 128].astype(f32)
        xp_ref[1, :, :jm * 128] = x0f
        anchors = plain(0, xr_ref[...], x0f, x0f, (8 - cfg['NSLAB']) * (28 + len(prods3)), cfg['AFREE'], never, 0, jm)
        for u in range(cfg['NSLAB'], 8):
            prep(0, u, anchors, zero, (kb0, kb1)[u % 2])
        in_copy(0, 0).wait()
        x0f = xr_ref[:, jm * 128:].astype(f32)
        xp_ref[1, :, jm * 128:] = x0f
        units = [(R, C, r) for R in range(4) for C in range(4) for r in range(0, Mh, 32)]
        anchors = plain(0, xr_ref[...], x0f, x0f, len(units) + sum(len(STAGES[n]) for _, n in carried) + 2, 4, never, jm)
        for R, C, r in units[:len(units) // 2]:
            conv(xn2_ref.at[0], zero, R, C, r, min(32, Mh - r), next(anchors))
        for fn, n in carried:
            st8 = {}
            for group in STAGES[n]:
                anchor = next(anchors)
                fn(st8, group, zero, jax.lax.shift_right_logical(zero, 1), anchor)
        for R, C, r in units[len(units) // 2:]:
            conv(xn2_ref.at[0], zero, R, C, r, min(32, Mh - r), next(anchors))

        def layer(l, carry):
            w_copy(l).wait()
            zero = jax.lax.shift_right_logical(l, 12)
            x = xp_ref[0]
            anchors = plain(l, x.astype(bf16), xp_ref[1], x, 8 * (28 + len(prods3)), cfg['AFREE'],
                            jnp.broadcast_to(zero, (8, 128)) != 0)
            for u in range(8):
                prep(l, u, anchors, zero, (kb0, kb1)[u % 2])
            return carry

        jax.lax.fori_loop(1, L, layer, 0)
        xr_ref[...] = xp_ref[0].astype(bf16)
        xr_out.start()

    def main(tile, carry):
        zs, za = jax.lax.shift_right_logical(tile, 12), jax.lax.shift_right_logical(tile, 13)
        never = jnp.broadcast_to(zs, (8, 128)) != 0
        slot = tile % 2
        in_copy(jnp.minimum(tile + 2, NMAIN - 1), slot).start()
        in_copy(jnp.minimum(tile + 1, NMAIN - 1), 1 - slot).wait()

        @pl.when(tile > 1)
        def _():
            for part in range(3):
                out_copy(tile - 2, slot, part).wait()

        xn_ref = xn2_ref.at[1 - slot]
        o_ref = o2_ref.at[slot]
        def rows(h, r0):
            if isinstance(h, tuple):
                return slice(r0 + h[0], r0 + h[0] + h[1])
            return slice(r0, r0 + Mh) if h is None else slice(r0 + h * Mq, r0 + (h + 1) * Mq)

        def ld(loc, h=None, z=0):
            return loc[0][(z,) + loc[1] + (rows(h, loc[2]),)]

        def st(loc, v, h=None):
            loc[0][(za if h == 1 and not loc[1] and cfg['ZB'] else zs,) + loc[1] + (rows(h, loc[2]),)] = v

        def by_half(v, h, fn):
            if isinstance(h, tuple):
                h = h[0] // Mq
            return fn(v, h) if h is not None else jnp.concatenate([fn(v[:Mq], 0), fn(v[Mq:], 1)], axis=0)

        def gather(ref, idx, n, pos):
            if cfg['NOBC']:
                return ref[idx + (slice(0, n), slice(16 * pos, 16 * pos + 16))].reshape(16 * n, 128)
            return ref.bitcast(u32)[idx + (slice(0, n), slice(8 * pos, 8 * pos + 8))].reshape(8 * n, 128)

        as_bf16 = lambda v: v if cfg['NOBC'] else pltpu.bitcast(v, bf16)

        def lhs2(p, q):
            ref, u = s2loc(p)
            return as_bf16(jnp.concatenate([gather(ref, (0, u, k), NC, q2[p].index(q)) for k in range(2)], axis=1))

        def rhs2(l, p, q, n):
            return as_bf16(gather(t2[p], (l, n), 16, q2[p].index(q)))

        def dot3(l, p, q, r):
            qs = next(qs for qs in PAIRS if q in qs)
            return _dot(as_bf16(gather(s3[(p, qs)], (0, qs.index(q)), NQ, ORD.index(r))),
                        as_bf16(gather(t3_ref, (l, prods3.index((p, q))), 8, ORD.index(r))))

        def add_bias(v, l, site, h):
            def one(x, hh):
                b = bt_ref[l, BIAS.index(site + (hh,))]
                return (x.reshape(x.shape[0] // 8, 8, 128) + b).reshape(x.shape)
            return by_half(v, h, one)

        def outer_act(l, p, i, j, n, d, h, part=None):
            bt, stores, finals = OACT[p]
            if part == 'raw':
                stores, finals = stores[:1], []
            if part == 'rest':
                bt, stores = [], stores[1:]
            if p == 6 and part is None and (i, j) != B12 and (h, n) != (0, 1):
                stores = []
            if bt:
                d = add_bias(d, l, (p, False, i, j, n), h)
            cache = {'d': d}
            def comb(terms):
                for _, src in terms:
                    if isinstance(src, str) and src not in cache:
                        cache[src] = ld(oloc(src, i, j, n), h)
                v = lincomb([(s, cache[src]) for s, src in terms if isinstance(src, str)])
                for _, src in terms:
                    if not isinstance(src, str):
                        v = add_bias(v, l, (p, True, i, j, n), h)
                return v
            fin = [(IJ, comb(terms)) for IJ, terms in finals]
            for name, v in [(name, comb(terms)) for name, terms in stores]:
                st(oloc(name, i, j, n), v, h)
            for (I, J), y in fin:
                R, C = 2 * I + i, 2 * J + j
                xn = ld(x0loc(R, C, n), h) * y
                if l > 0:
                    xn = xn + ld(xloc(l, R, C, n), h)
                if l < L - 1:
                    st(xloc(l + 1, R, C, n), xn, h)
                else:
                    xn = by_half(xn, h, lambda x, hh: x if scale(R, C, hh, n) == 1.0 else x * (1.0 / scale(R, C, hh, n)))
                    o_ref[rows(h, R * Mh), C * H + n * 128:C * H + (n + 1) * 128] = xn.astype(bf16)

        def inner_act(g, l, p, kind, n, h, P, Q, part=None):
            vloc = oloc(raw_slot(p), 0, 1, n) if raw_slot(p) else iloc(g, 'v', n)
            if kind == '35':
                st(iloc(g, 's', n), Q + ld(iloc(g, 'm1', n), h), h)
                if not raw_slot(p):
                    st(vloc, P, h)
                outer_act(l, p, 0, 1, n, P, h, part)
            elif kind == '47':
                st(iloc(g, 'u', n), Q + ld(vloc, h), h)
                outer_act(l, p, 0, 0, n, P + ld(iloc(g, 's', n), h), h, part)
            else:
                outer_act(l, p, 1, 1, n, ld(iloc(g, 's', n), h) - Q, h, part)
                outer_act(l, p, 1, 0, n, P + ld(iloc(g, 'u', n), h), h, part)

        def issue(l, p, rd):
            kind, n = rd
            if kind == 'x':
                return [dot3(l, p, q, 1) for q in (3, 5, 4, 7)]
            if kind == 'y':
                return [dot3(l, pp, q, 1) for pp in (p, SEL3[SEL3.index(p) + 1]) for q in (2, 6)]
            if isinstance(n, str):
                if cfg['MO']:
                    d = [dot3(l, p, int(q), int(r)) for q in kind for r in n]
                    return [d[0], d[2], d[1], d[3]]
                return [dot3(l, p, int(q), int(r)) for r in n for q in kind]
            if cfg['GR']:
                ops = [(lhs2(p, 1),) * 2, (rhs2(l, p, 1, 0), rhs2(l, p, 1, 1))] if kind == '1' else [
                    [lhs2(p, int(q)) for q in kind], [rhs2(l, p, int(q), n) for q in kind]]
                d = [_dot(a[:, k * 128:(k + 1) * 128], b[k * 128:(k + 1) * 128]) for a, b in zip(*ops) for k in range(2)]
                return [d[0] + d[1], d[2] + d[3], d[cfg['GR'] - 1]]
            if kind == '1':
                lhs = lhs2(p, 1)
                return [_dot(lhs, rhs2(l, p, 1, 0)), _dot(lhs, rhs2(l, p, 1, 1))]
            return [_dot(lhs2(p, int(q)), rhs2(l, p, int(q), n)) for q in kind]

        def consume(g, l, p, rd, res):
            kind, n = rd
            if n == '1':
                for u, where in enumerate((('35', False), ('47', False)) if kind == 'x' else (('26', False), ('26', True))):
                    for al in range(2):
                        st(jloc(where[0], '1', al, where[1]), res[2 * u + al], 0)
            elif isinstance(n, str):
                sm = [res[al] + res[2 + al] for al in range(2)]
                df = [res[al] - res[2 + al] for al in range(2)]
                J = lambda name, al: ld(jloc(kind, name, al, name == '1' and kind == '26' and p in SEL3[1::2]), 0)
                part = 'raw' if deferred(l, p, rd) else None
                done = lambda h, nn, m: inner_act(g, l, p, kind, nn, h, m[0] + m[1], m[0] - m[1], part)
                O, I = (lambda i, j: oloc(raw_slot(p), i, j, 1)), (lambda name: iloc(g, name, 1))
                rec = lambda al: [(s, ld(loc, 0, za if cfg['ZB'] else 0)) for s, loc in {
                    '35': [[(1, O(0, 1))], [(1, I('s')), (-1, I('m1'))]],
                    '47': [[(1, O(0, 0)), (-1, I('s'))], [(1, I('u')), (-1, O(0, 1))]],
                    '26': [[(1, O(1, 0)), (-1, I('u'))], [(1, I('s')), (-1, O(1, 1))]]}[kind][al]]
                if n == '35':
                    for al in range(2):
                        st(jloc(kind, 's', al), df[al] + J('1', al), 0)
                    done(0, 1, sm)
                elif n == '47':
                    if cfg['HY'] == 1:
                        for al in range(2):
                            st(jloc(kind, 'u', al), df[al], 0)
                    else:
                        for al, v in enumerate((df[0] + df[1], df[0] - df[1])):
                            st(jloc(kind, 'u', al), lincomb([(1, v)] + rec(al)), 0)
                    done(0, 0, [sm[al] + J('s', al) for al in range(2)])
                else:
                    if cfg['HY'] == 1:
                        m = [sm[al] + J('u', al) for al in range(2)]
                        P, Q = lincomb([(1, m[0] + m[1])] + rec(0)), lincomb([(1, m[0] - m[1])] + rec(1))
                    else:
                        P, Q = (sm[0] + sm[1]) + J('u', 0), (sm[0] - sm[1]) + J('u', 1)
                    done(1, 1, [J('s', al) - df[al] for al in range(2)])
                    inner_act(g, l, p, kind, 0, 1, P, Q, part)
            elif kind == '1':
                st(iloc(g, 'm1', 0), res[0])
                st(iloc(g, 'm1', 1), res[1])
            else:
                inner_act(g, l, p, kind, n, None, res[0] + res[1], res[0] - res[1])

        state = {}
        for g, rd, t0, n in sched:
            l, p = outs[g]
            if t0 == start[G - 1]:
                out_copy(tile, slot, 0).start()
            if t0 + n == T:
                out_copy(tile, slot, 1).start()
            res = issue(l, p, rd)
            if cfg['EO']:
                consume(g, l, p, rd, res)
            for t in range(t0, t0 + n):
                for ph, l2, fn, group in plan.get(t, []):
                    gr = 16 * (t - t0) + 8 * ph
                    if cfg['GF']:
                        gr = 16 * (t - t0) + 8 * (1 - ph)
                    gs = cfg['GS']
                    gate = res[2 if len(res) == 3 else cfg['GM']][gr:gr + 8, :]
                    if cfg['GADD'] and isinstance(rd[1], str) and rd[1] != '1':
                        gate = gate + res[2 + gs % 2][gr:gr + 8, :]
                    elif gs == 2 and rd[0] != '1' and rd[1] != '1':
                        gate = gate + res[1][gr:gr + 8, :]
                    if l2 == 'fin':
                        for i, j, nf, r0 in fn[2]:
                            d = ld(oloc(raw_slot(fn[1]), i, j, nf), (r0, 16))
                            d = tie(tie(d, (never, gate)), (never, gate), 8)
                            outer_act(fn[0], fn[1], i, j, nf, d, (r0, 16), 'rest')
                    elif l2 is None:
                        conv(xn_ref, zs, *fn, min(32, Mh - fn[2]), (never, gate))
                    else:
                        fn(state.setdefault(id(fn), {}), group, zs, za, (never, gate))
            if not cfg['EO']:
                consume(g, l, p, rd, res)
        out_copy(tile, slot, 2).start()
        return carry

    prologue()
    jax.lax.fori_loop(0, NMAIN, main, 0)
    xr_out.wait()
    in_copy(NMAIN - 1, (NMAIN - 1) % 2).wait()
    for t in range(max(NMAIN - 2, 0), NMAIN):
        for part in range(3):
            out_copy(t, t % 2, part).wait()


DEFAULT = dict(SEL=(3, 5, 4, 7, 2, 6), SEL3=(3, 5, 4, 7), XC={B12: 5, B11: 1, B22: 7, B21: 2}, AFREE=4, NOBC=0, MAT=4, FOLD=1, MO=1, GR=2, NS=(2, 3, 3, 4, 3), NL=1, GE=6, GM=0, DBL=1, GS=0, GF=0, EO=0, KP=16, PPH=None, ZB=0, HY=1, HOLD=0, PORT=0.9, PS=0, NSLAB=6, JM=3, XP=40, XO=16, DEFER={5: [('26', '26'), ('47', '26')], 7: [('26', '26'), ('47', '26')], 2: [('35', '26'), ('47', '26')],
                      6: [('35', '26'), ('47', '26')]}, DEFL={}, EW=12, KW=(1,) * 5, CM=(1,) * 7, SEEDS=(), SEG=32, PJ=20, QO=0, TIEL=2, GADD=0, TF=0, T8=0, TAIL=6,
               CS=0.5, CL=0.3, UL=0.8, CAP=0.95, FR=((1.,), (.4, .6), (.35, .37, .28), (.16, .26, .31, .27),
                   (.35, .29, .08, .28), (.16, .26, .26, .05, .27)))


def build(TM=640, **kw):
    def f(x0, ws, bs):
        B, D = x0.shape
        L = ws.shape[0]
        cfg = dict(DEFAULT, **kw)
        Mh = TM // 4
        MP = Mh + 32
        nmain = (B - 1) // TM
        R0 = B - nmain * TM
        pairs3, q2 = layout(cfg)
        n3 = sum(2 * len(v) for v in pairs3.values())
        pad = lambda n: n + (2 - n) % 4
        V = pltpu.VMEM
        half = V((1, MP, 128), f32)
        XP = Mh + cfg['XP']
        scratch = ([V((1, 2, 2, 2, XP, 128), f32)] * 4 + [V((1, 2, 4, 2, XP, 128), f32)] * 7 + [half] * (16 + 64 + 26)
                   + [V((1, 1 + (p == 2 and q2[2] == q2[6]), 2, pad(Mh // 16), 16 * len(q2[p]), 128), bf16) for p in range(1, 8)]
                   + [V((1, 2, pad(Mh // 32), 112, 128), bf16)] * (n3 // 2)
                   + [V((L, 2, 16, 16 * len(q2[p]), 128), bf16) for p in range(1, 8)]
                   + [V((L, n3, 8, 112, 128), bf16), V((1, 4, 16 * n3 + cfg['KP'], 128), f32), V((1, 4, 16 * n3 + cfg['KP'], 128), f32),
                      V((L, len(BIAS), 8, 128), f32), V((8, 1, D), f32), V((2, TM, D), bf16), V((2, TM, D), bf16), V((L, 8, 8, 16, D), bf16),
                      V((R0, D), bf16), V((2, R0, D), f32), V((L, D), bf16), pltpu.SemaphoreType.DMA((L + 18,))])
        anyspec = pl.BlockSpec(memory_space=pl.ANY)
        return pl.pallas_call(
            functools.partial(_kernel, L=L, TM=TM, R0=R0, NMAIN=nmain, D=D, cfg=cfg),
            in_specs=[anyspec, anyspec, anyspec],
            out_specs=anyspec,
            out_shape=jax.ShapeDtypeStruct((B, D), x0.dtype),
            scratch_shapes=scratch,
            compiler_params=pltpu.CompilerParams(
                vmem_limit_bytes=120 * 1024 * 1024,
                internal_scratch_in_bytes=65536,
                disable_bounds_checks=True,
            ),
        )(x0, ws.reshape(L, 8, 8, 16, D), bs)
    return f


@jax.jit
def pallas_standalone__dcn_v2_cross__recsys_kernel(x0, ws, bs):
    return build(TM=640)(x0, ws, bs)
```

```python
import functools

import jax
import jax.numpy as jnp
import jax.experimental.pallas as pl
import jax.experimental.pallas.tpu as pltpu

f32 = jnp.float32
bf16 = jnp.bfloat16
u32 = jnp.uint32

B11, B12, B21, B22 = (0, 0), (0, 1), (1, 0), (1, 1)
LA = {1: [(B11, 1), (B22, 1)], 2: [(B11, 1), (B12, 1), (B21, 1), (B22, 1)], 3: [(B11, 1), (B12, -1)],
      4: [(B12, 1), (B22, 1)], 5: [(B11, 1), (B12, 1)], 6: [(B12, 1), (B11, -1), (B21, 1), (B22, -1)],
      7: [(B12, 1), (B22, -1)]}
PAIRS = ((5, 3), (4, 7), (2, 6))
ORD = (3, 5, 4, 7, 1, 2, 6)
D2 = (1.0, 2.0)
BF = {1: 1.0, 2: 0.5, 3: 0.5, 4: 0.5, 5: 0.5, 6: 0.5, 7: 0.5}
OUTER = (3, 5, 1, 4, 7, 2, 6)
OACT = {
    3: ([(1, B12)], [('M3', [(1, 'd')])], []),
    5: ([], [('M5', [(1, 'd')])], [(B12, [(1, 'd'), (1, 'M3')])]),
    1: ([(1, B11), (-1, B12)], [('S', [(1, 'd'), (1, 'M3'), (-1, 'M5')])], []),
    4: ([], [('M4', [(1, 'd')])], []),
    7: ([], [('M7', [(1, 'd')])], [(B11, [(1, 'd'), (1, 'S'), (1, 'M4')])]),
    2: ([(1, B11), (-1, B22)], [('M2', [(1, 'd')]),
        ('U', [(1, 'd'), (1, 'M4'), (-1, 'M7'), (1, 'M3'), (1, 'M5'), (1, ((1, B21), (-1, B12), (-1, B11), (1, B22)))])], []),
    6: ([], [('M6', [(1, 'd')])], [(B22, [(1, 'd'), (1, 'S'), (-1, 'M2')]), (B21, [(1, 'd'), (1, 'U')])]),
}
OSL = {'M3': 0, 'M5': 1, 'S': 2, 'M4': 3, 'M7': 4, 'M2': 6, 'U': 5, 'M6': 7}
ISL = {'m1': 0, 's': 1, 'v': 2, 'u': 3}
STAGES = {1: [(B11, B12, B21, B22)], 2: [(B11, B12), (B21, B22)], 3: [(B11, B12), (B22,), (B21,)],
          4: [(B11,), (B12,), (B22,), (B21,)], 5: [(B11, B12), (B22, 'hold'), ('l1',), (B21,)],
          6: [(B11,), (B12,), (B22, 'hold'), ('l1',), (B21,)]}
BIAS = [(p, extra, i, j, n, h) for p in OUTER for extra in (False, True)
        if (any(not isinstance(x, str) for _, t in OACT[p][1] + OACT[p][2] for _, x in t) if extra else OACT[p][0])
        for i in range(2) for j in range(2) for n in range(2) for h in range(2)]
PREP_ORDER = (2, 6, 3, 5, 1, 4, 7)
GAMMA = 0.125
LAG = 8


def _dot(a, b):
    return jnp.dot(a, b, preferred_element_type=f32)


def scale(R, C, h, k):
    return D2[R // 2] * D2[R % 2] * D2[h] / (D2[C // 2] * D2[C % 2] * D2[k])


def b_ops(b11, b12, b21, b22):
    r1 = b11 + b22
    g = b12 + b21
    return {1: r1, 2: b11 - b12, 3: b12 - b22, 4: g - r1, 5: b12 + b22, 6: b11 + b12, 7: g + r1}


def lincomb(terms):
    assert terms[0][0] == 1
    acc = terms[0][1]
    for s, v in terms[1:]:
        acc = acc + v if s == 1 else acc - v
    return acc


def raw_slot(p):
    return next((name for name, terms in OACT[p][1] if terms == [(1, 'd')]), None)


def round_usage(p, rd, first, last, defer, hy):
    bt, stores, finals = OACT[p]
    alu = bool(bt) + sum(len(t) - 1 for _, t in stores) + sum(len(t) + (not first) + 2 * last for _, t in finals)
    nst = len(stores) + len(finals)
    nld = len({x for _, t in stores + finals for _, x in t if isinstance(x, str) and x != 'd'}) + len(finals) * (2 - first)
    kind, n = rd
    if defer:
        alu, nst, nld = bool(bt), 1, 0
    elif p == 6 and kind != '35' and n != '35':
        nst -= 1
    if isinstance(n, str):
        e = kind == '47'
        if kind == '26':
            a, st, ld, m = {'35': (10, 2, 9, 2), '47': (10, 2, 9, 2) if hy == 1 else (16, 2, 13, 2), '26': (20, 0, 17, 4) if hy == 1 else (16, 0, 13, 4)}[n]
        else:
            a, st, ld, m = {'1': (0, 4, 5, 0), '35': (9 + e, 3, 8 + e, 1),
                            '47': (9 + e, 3, 8 + e, 1) if hy == 1 else (14 + 2 * e, 3, 11 + 2 * e, 1),
                            '26': (17 + 3 * e, 2, 14 + 3 * e, 2) if hy == 1 else (14 + 2 * e, 2, 11 + 2 * e, 2)}[n]
    else:
        a, st, ld, m = {'1': (2, 2, 4, 0), '35': (5, 2 - bool(raw_slot(p)), 5, 1), '47': (6, 1, 6, 1),
                        '26': (6, 0, 6, 2)}[kind]
    return a + m * alu, st + m * nst, ld + m * nld


def yds(groups, cap):
    n = len(cap)
    speed, cls, gcls = [0.0] * n, [-1] * n, {}
    todo = list(groups)
    while todo:
        pre = [0.0]
        for t in range(n):
            pre.append(pre[-1] + (cap[t] if cls[t] < 0 else 0.0))
        best = None
        for a in sorted({g[0] for g in todo}):
            w = 0.0
            for g in sorted((g for g in todo if g[0] >= a), key=lambda g: g[1]):
                w += g[2]
                d = w / max(pre[g[1] + 1] - pre[a], 1e-9)
                if best is None or d > best[0]:
                    best = (d, a, g[1])
        d, a, b = best
        for t in range(a, b + 1):
            if cls[t] < 0:
                speed[t], cls[t] = d, len(gcls)
        gcls.update({g[:2]: len(gcls) for g in todo if g[0] >= a and g[1] <= b})
        todo = [g for g in todo if not (g[0] >= a and g[1] <= b)]
    return speed, cls, gcls


def spread_jobs(jobs, cap, tail):
    T = len(cap)
    cap3 = cap * 3
    all3 = [(lo + k * T, hi + k * T, ji, k) for k in range(3) for ji, (lo, hi, _) in enumerate(jobs) if lo + k * T >= 0]
    pend = {}
    for j in sorted(all3, key=lambda j: (j[1], j[3], j[2])):
        pend.setdefault(j[:2], []).append(j)
    speed, cls, gcls = yds([w + (sum(sum(jobs[j[2]][2]) for j in q),) for w, q in pend.items()], cap3)
    when = [[] for _ in jobs]
    debt, cur, done = 0.0, None, 0
    for t in range(3 * T):
        while True:
            j = cur
            if j is None:
                rdy = [q[0] for w, q in pend.items() if q and w[0] <= t and (gcls[w] == cls[t] or w[1] <= t)]
                if not rdy:
                    debt = max(debt, 0.0)
                    break
                j = rdy[0]
                nst = len(jobs[j[2]][2])
                if nst > 1 and j[1] > t and (t + tail + 2 * nst) // T != t // T:
                    break
            must = j[1] <= t or (cur is not None and (t + tail + 1) // T != t // T)
            if not must and (cap3[t] == 0.0 or debt > 0.5 * speed[t] * cap3[t]):
                break
            if cur is None:
                pend[j[:2]].pop(0)
                cur, done = j, 0
            debt += jobs[j[2]][2][done]
            if j[3] == 1:
                when[j[2]].append(t - T)
            done += 1
            if done == len(jobs[j[2]][2]):
                cur = None
        debt -= speed[t] * cap3[t]
    return when


def layout(cfg):
    sel, sel3 = cfg['SEL'], cfg['SEL3']
    pairs3 = {p: [qs for qs in PAIRS if p in sel3 or (p in sel and qs != (2, 6))] for p in range(1, 8)}
    q2 = {p: [q for q in ORD if not any(q in qs for qs in pairs3[p])] for p in range(1, 8)}
    return pairs3, q2


def _kernel(x_hbm, w_hbm, b_hbm, o_hbm, *scratch, L, TM, R0, NMAIN, D, cfg):
    H, Mh, Mq = D // 4, TM // 4, TM // 8
    NC, NQ = Mh // 16, Mq // 16
    MP = Mh + 32
    SEL, SEL3 = cfg['SEL'], cfg['SEL3']
    pairs3, q2 = layout(cfg)
    prods3 = [(p, q) for p in SEL for qs in pairs3[p] for q in qs]
    assert H == 256 and L % 2 == 0 and Mq % 16 == 0 and all(raw_slot(p) for p in SEL)
    it = iter(scratch)
    take = lambda n: [next(it) for _ in range(n)]
    x0b, xb, ib, ob, jb = take(4), take(7), take(16), take(64), take(26)
    joint = q2[2] == q2[6]
    MAT = cfg['MAT'] and joint and 2 in SEL
    s2 = dict(zip(range(1, 8), take(7)))
    s3 = {(p, qs): next(it) for p in SEL for qs in pairs3[p]}
    t2 = dict(zip(range(1, 8), take(7)))
    t3_ref, kb0, kb1, bt_ref, bf_ref, xn2_ref, o2_ref, w_ref, xr_ref, xp_ref, b_ref, sem = it

    xset = lambda l: 6 if l == 'O' else 4 if l == 0 else (l % 2) * 2
    xoff = lambda I, J: cfg['XO'] * ((I + J) % 2)
    xloc = lambda l, R, C, k: (xb[xset(l) + R // 2], (R % 2, C, k), xoff(R // 2, C // 2))
    x0loc = lambda R, C, k: (x0b[(R // 2) * 2 + C // 2], (R % 2, C % 2, k), 8 + xoff(R // 2, C // 2))
    iloc = lambda g, name, n: (ib[((g % 2) * 4 + ISL[name]) * 2 + n], (), 8 * ISL[name])
    oloc = lambda name, i, j, n: (ob[(OSL[name] * 4 + i * 2 + j) * 2 + n], (), 8 * ((OSL[name] + 2 * j) % 4))

    def jloc(kind, name, al, second=False):
        i = 24 + al if second else (('35', '47', '26').index(kind) * 4 + ('1', 's', 'u', 'v').index(name)) * 2 + al
        return jb[i], (), 8 * ((i + i // 2) % 4)

    def s2loc(p):
        return (s2[2], (2, 6).index(p)) if p in (2, 6) and joint else (s2[p], 0)

    def bias_coefs(p, extra, i, j, n, h):
        where = [(1, i, j, n, h)]
        if extra:
            terms = next(x for _, t in OACT[p][1] + OACT[p][2] for _, x in t if not isinstance(x, str))
        else:
            terms = OACT[p][0]
            w = [(1, i, j)] + [(-1, 0, 1)] * bool(raw_slot(p) and (i, j) == B21)
            where = [x + (n, h) for x in w]
            if (h, n) == (1, 0) and PAIRS[{B12: 0, B11: 1}.get((i, j), 2)] in pairs3[p]:
                where += [(-sg, ii, jj, 1, 0) for sg, ii, jj in w]
        coef = {}
        for sg, ii, jj, nn, hh in where:
            for cf, (I, J) in terms:
                key = (2 * J + jj) * 2 + nn
                coef[key] = coef.get(key, 0.0) + sg * cf * scale(2 * I + ii, 2 * J + jj, hh, nn) / GAMMA
        return coef

    def tie(v, anchor, r=0):
        if anchor is None:
            return v
        return jnp.concatenate([v[:r]] * (r > 0) + [jax.lax.select(anchor[0], anchor[1], v[r:r + 8])] + [v[r + 8:]] * (r + 8 < v.shape[0]), axis=0)

    def consts(anchor, ss, reps):
        one = {s: jnp.full((8, 128), s, f32) for s in set(ss)}
        if anchor is not None:
            one = {s: jax.lax.select(anchor[0], anchor[1], v) for s, v in one.items()}
        return jnp.concatenate([one[s] for s in ss for _ in range(reps)], axis=0)

    def conv(src, zs, R, C, r, nr, anchor=None):
        v = src[R * Mh + r:R * Mh + r + nr, C * H:(C + 1) * H].astype(f32)
        for k in range(2):
            buf, idx, off = xloc(0, R, C, k)
            sv = consts(anchor, [scale(R, C, (r + u) // Mq, k) for u in range(0, nr, 16)], 2)
            buf[(zs,) + idx + (slice(off + r, off + r + nr),)] = v[:, k * 128:(k + 1) * 128] * sv

    cnt = {}
    def block_sum(l, terms, ii, jj, kk, r, save, zs, za, anchor, late=None):
        rng = lambda t: slice(t[0], t[-1] + 1)
        keys = [(i, j, k) for i in ii for j in jj for k in kk]
        vals = []
        for u, ((I, J), s) in enumerate(terms):
            ref, r0 = xb[xset(l) + I], xoff(I, J) + r
            v = ref[za if u == 0 else 0, rng(ii), 2 * J + jj[0]:2 * J + jj[-1] + 1, rng(kk), r0:r0 + 16, :]
            if (I, J) in save:
                sv = consts(anchor, [GAMMA / scale(2 * I + i, 2 * J + j, r // Mq, k) for i, j, k in keys], 2)
                x0b[I * 2 + J][zs, rng(ii), rng(jj), rng(kk), r0 + 8:r0 + 24, :] = v * sv.reshape(v.shape)
            v = v.reshape(16 * len(keys), 128)
            if u == 0 and late is not None and anchor is not None:
                cnt[xset(l)] = cnt.get(xset(l), -1) + 1
                if cnt[xset(l)] % cfg['GE'] == 0:
                    ref[0, 0, 0, 0, Mh + 24:Mh + 32, :] = anchor[1]
                at = 16 * keys.index(late)
                top = v[at:at + 8] if cfg['NL'] else ref[za, late[0], 2 * J + late[1], late[2], r0:r0 + 8, :]
                if cfg['TIEL'] == 2:
                    top = jax.lax.select(anchor[0], anchor[1], top)
                v = jnp.concatenate([v[:at]] * (at > 0) + [top, v[at + 8:]], axis=0)
            vals.append((s, v))
        v = lincomb(vals)
        if cfg['TIEL'] == 3 and late is not None:
            v = tie(v, anchor, 16 * keys.index(late))
        return v

    def release(qs, store, st8, anchor):
        v = st8['l1']
        if anchor is not None:
            n = v.shape[0]
            top = jax.lax.select(jnp.broadcast_to(anchor[0], (n, 8, 128)), jnp.broadcast_to(anchor[1], (n, 8, 128)), v[:, :8])
            v = jnp.concatenate([top, v[:, 8:]], axis=1)
        r0 = 16 * qs.index(1)
        store(slice(r0, r0 + 16), v.astype(bf16))

    def finish(e, f, group, qs, store, st8, anchor, hold=False, keep=None):
        a = e[None] if f is None else jnp.concatenate([e + f, e - f], axis=0).reshape(2, e.shape[0], 128)
        for u, b in enumerate(group):
            st8[b] = a if len(group) == 1 else a[:, 16 * u:16 * u + 16]
            if keep:
                keep(b, st8[b])
        ops = {}
        if B12 in group and 3 in qs:
            ops[3], ops[5] = st8[B11] - st8[B12], st8[B11] + st8[B12]
        if B22 in group:
            if 4 in qs:
                ops[4], ops[7] = st8[B12] + st8[B22], st8[B12] - st8[B22]
            ops[1] = st8['l1'] = st8[B11] + st8[B22]
        if B21 in group:
            g = st8[B12] + st8[B21]
            ops[2], ops[6] = g + st8['l1'], g - st8['l1']
        now = [q for q in qs if q in ops and not (hold and q == 1)]
        if now:
            r0 = 16 * qs.index(now[0])
            store(slice(r0, r0 + 16 * len(now)), jnp.concatenate([ops[q] for q in now], axis=1).astype(bf16))

    def unit2(l, ps, c, k, save, st8, group, zs, za, anchor):
        def store(rows, v):
            s2[ps[0]][zs, :, k, c, rows, :] = v
        if group == ('l1',):
            return release(q2[ps[0]], store, st8, anchor)
        hold, group = 'hold' in group, tuple(b for b in group if b != 'hold')
        ii, jj = sorted({b[0] for b in group}), sorted({b[1] for b in group})
        bs = lambda terms, late: block_sum(l, terms, ii, jj, [k], 16 * c, save, zs, za, anchor, late)
        f = None if len(ps) == 1 else bs([(B11, 1), (B22, 1)], None)
        e = bs(LA[ps[0]] if len(ps) == 1 else [(B12, 1), (B21, 1)], (ii[0], jj[-1], k))
        def keep(b, v):
            if b != B21:
                for J in range(2):
                    xb[6][zs, b[0], 2 * J + b[1], k, xoff(0, J) + 16 * c:xoff(0, J) + 16 * c + 16, :] = v[J]
        if f is None or joint:
            return finish(e, f, group, q2[ps[0]], store, st8, anchor, hold, keep if f is not None and MAT else None)
        for p, v in zip(ps, (e + f, e - f)):
            def store1(rows, w):
                s2[p][zs, :, k, c, rows, :] = w
            finish(v, None, group, q2[p], store1, st8.setdefault(p, {}), anchor)

    def unit3(l, p, qs, c, save, st8, group, zs, za, anchor):
        def store(rows, w):
            s3[(p, qs)][zs, :, c, rows, :] = w
        if group == ('l1',):
            return release(ORD, store, st8, anchor)
        hold, group = 'hold' in group, tuple(b for b in group if b != 'hold')
        for h in sorted({b[0] for b in group}):
            grp = tuple(b for b in group if b[0] == h)
            kk = [b[1] for b in grp]
            ii, jj = {(5, 3): ([0], [0, 1]), (4, 7): ([0, 1], [1]), (2, 6): ([0, 1], [0, 1])}[qs]
            src = ('O', [((0, (2, 6).index(p)), 1)]) if MAT and p in (2, 6) else (l, LA[p])
            v = block_sum(*src, ii, jj, sorted(kk), h * Mq + 16 * c, save, zs, za, anchor,
                          (0, (0 if cfg['TF'] else 1) if qs == (2, 6) else jj[0], max(kk)) if h == group[-1][0] else None)
            n = 16 * len(kk)
            piece = lambda u: v[u * n:(u + 1) * n]
            if qs == (2, 6):
                e, f = piece(1) + piece(2), piece(0) + piece(3)
                r0 = 16 * q2[p].index(1)
                s2[p][zs, 0, min(kk):max(kk) + 1, h * NQ + c, r0:r0 + 16, :] = f.reshape(len(kk), 16, 128).astype(bf16)
            else:
                e, f = piece(0), piece(1)
            finish(e, f, tuple(sorted(grp)), ORD, store, st8, anchor, hold)

    def prep(l, u, anchors, zero, kb):
        mul = lambda v, s: v if s == 1.0 else v * s
        def third(e, last):
            v = kb[0, 0:4 if last is None else 3, 16 * e:16 * e + 16, :]
            T = b_ops(v[0], tie(v[1], next(anchors)), v[2], v[3] if last is None else last)
            T[1] = T[1] * 2.0
            t3_ref[l, e, u] = jnp.concatenate([T[q] for q in ORD], axis=0).astype(bf16)
        for k in range(2):
            wide = [w_ref[l, R * 2 + k, u].astype(f32) for R in range(4)]
            for n in range(2):
                la = next(anchors) if cfg['LANC'] else None
                def blk(R, C):
                    v = mul(wide[R][:, C * H + n * 128:C * H + (n + 1) * 128], scale(R, C, k, n))
                    return tie(v, la) if (R // 2, C // 2) == B12 else v
                O = {(i, j): b_ops(blk(i, j), blk(i, 2 + j), blk(2 + i, j), blk(2 + i, 2 + j)) for i, j in (B11, B12, B21, B22)}
                for p in cfg['PO']:
                    o = [mul(O[b][p], BF[p] * (0.25 if p in SEL else 0.5) / GAMMA) for b in (B11, B12, B21, B22)]
                    T = b_ops(o[0], tie(o[1], next(anchors)), o[2], o[3])
                    t2[p][l, n, k * 8 + u] = jnp.concatenate(
                        [mul(T[q], BF[q] * (4.0 if p in SEL else 2.0)) for q in q2[p]], axis=0).astype(bf16)
                    mine = [e for e, pq in enumerate(prods3) if pq[0] == p]
                    if cfg['KD'] and (k, n) == (1, 1):
                        for e in mine:
                            third(e, T[prods3[e][1]])
                    elif mine:
                        kb[zero, k * 2 + n, 16 * mine[0]:16 * mine[-1] + 16, :] = jnp.concatenate(
                            [T[prods3[e][1]] for e in mine], axis=0)
        if not cfg['KD']:
            for e in range(len(prods3)):
                third(e, None)

    def rounds_of(p):
        rs = [('1', None)] + [('x', '1')] * (p in SEL)
        for kind, qs in zip(('35', '47', '26'), PAIRS):
            if kind == '26' and p in SEL3[::2]:
                rs.append(('y', '1'))
            rs += [(kind, r) for r in (('35', '47', '26') if qs in pairs3[p] else (0, 1))]
        return rs

    def deferred(l, p, rd):
        return rd in cfg['DEFER'].get(p, ()) or (l == L - 1 and rd in cfg['DEFL'].get(p, ()))

    outs = [(l, p) for l in range(L) for p in OUTER]
    G = len(outs)
    sched, start, use = [], [], []
    for g, (l, p) in enumerate(outs):
        start.append(len(use))
        for rd in rounds_of(p):
            n = NQ if isinstance(rd[1], str) else NC
            sched.append((g, rd, len(use), n))
            a, st_, ld_ = round_usage(p, rd, l == 0, l == L - 1, deferred(l, p, rd), cfg['HY'])
            if cfg['PORT']:
                use += [max((2 * a + st_ + 2 + 16 / n) / 72 + cfg['PS'] * st_ / 8, cfg['PORT'] * st_ / 8)] * n
            else:
                use += [max(a / 32, st_ / 8, cfg['UL'] * ld_ / 24)] * n
    T = len(use)
    cap = [max(cfg['CAP'] - max(use[t], use[(t + 1) % T]), 0.0) * (t < T - cfg['TAIL']) for t in range(T)]
    for g in range(G):
        for t in range(start[g], (start + [T])[g + 1]):
            cap[t] *= cfg['CM'][g % 7]
    jobs = []
    def add(lo, hi, alu, st_, ld_, nst, l, fn):
        w = alu / 64 + cfg['CS'] * (st_ + nst) / 16 + cfg['CL'] * ld_ / 48
        w *= cfg['KW'][0 if l in (None, 'fin') else nst]
        if cfg['HOLD'] and nst >= 3:
            nst += 2
        jobs.append((lo, max(hi, lo), [w * f for f in cfg['FR'][nst - 1]], l, fn, nst))
    for g, (l, p) in enumerate(outs):
        ready = 7 * l - 2 * all(I == 0 for (I, J), _ in LA[p])
        lo = start[ready] - (T if ready < 0 else 0)
        if cfg['DEFER'].get(7) and ready % 7 == 5 and l > 0:
            lo += cfg['EW'] + 1
        for gg, rd, t0, n_ in sched:
            if gg == g and deferred(l, p, rd):
                if p == 7:
                    due = start[g + 1] + cfg['EW'] if l < L - 1 else start[g + 2] - 1
                elif p == 5:
                    due = start[7 * l + 5] - 1
                elif p == 6:
                    due = (start[g + 1] if l < L - 1 else T - NC) - 1
                else:
                    due = [t for g2, r2, t, _ in sched if g2 == g + 1 and r2[0] == rd[0]][0] - 3
                nops = 4 * sum(len(t) + (x in OACT[p][2]) * (2 + 2 * (l == L - 1)) for x in OACT[p][1][1:] + OACT[p][2] for t in x[1:])
                ws = [(i, j, n, h * Mq + 16 * c) for c in range(NQ) for h, n in {'35': [(0, 1)], '47': [(0, 0)], '26': [(1, 1), (1, 0)]}[rd[1]]
                      for i, j in {'35': [B12], '47': [B11], '26': [B22, B21]}[rd[0]]]
                m_ = 1 if p == 6 else 2
                for u in range(0, len(ws), m_):
                    add(t0 + n_, due, nops * m_ // 2, 3, nops * m_ // 2, 1, 'fin', (l, p, ws[u:u + m_]))
        hi = start[g] - LAG - 3
        nt = len(LA[p])
        save = [b for b, pp in cfg['XC'].items() if pp == p and l == 0]
        if p in SEL3:
            if p in SEL3[1::2]:
                host = 7 * l + OUTER.index(SEL3[SEL3.index(p) - 1])
                hi = [t0 for gg, rd, t0, _ in sched if gg == host and rd[0] == 'y'][0] - LAG - 3
            for c in range(NQ):
                add(lo, hi, 32 * nt + 50 + 32 * len(save), 18 + 32 * len(save), 32 * nt, cfg['NS'][3], l,
                    functools.partial(unit3, l, p, (2, 6), c, save))
        elif p != 6:
            ps = (2, 6) if p == 2 else (p,)
            nq = sum(len(q2[x]) for x in ps)
            alu = 8 * (nt - 2 + len(ps)) + sum(8 if x in SEL else 16 for x in ps) + nq
            if MAT and p == 2:
                hi = start[7 * l + cfg['MAT']] - 3
            for c in range(NC):
                for k in range(2):
                    add(lo, hi, alu + 8 * len(save), nq + 8 * len(save) + 12 * (bool(MAT) and p == 2), 8 * nt, 1 if nq <= 3 else cfg['NS'][4] if nq == 6 else cfg['NS'][0] if nq <= 7 else cfg['NS'][1], l,
                        functools.partial(unit2, l, ps, c, k, save))
        if MAT and p in (2, 6):
            lo, nt = start[7 * l + cfg['MAT']], 1
        if p in SEL:
            for qs, c in ([(qs, c) for qs in PAIRS[:2] for c in range(NQ)] if cfg['QO'] else
                          [(qs, c) for c in range(NQ) for qs in PAIRS[:2]]):
                if True:
                    add(lo, start[g] - LAG - 3 + (NC if g else 0), 16 * nt + 46, 14, 16 * nt, cfg['NS'][2 + (nt == 4)], l,
                        functools.partial(unit3, l, p, qs, c, []))
    for R in range(4):
        for C in range(4):
            for c in range(0, NC, 2):
                add(start[6], start[G - 2] - 2, 18, 7, 4, 1, None, (R, C, 16 * c))
    when = spread_jobs([j[:3] for j in jobs], cap, cfg['TAIL'])
    evs = [e[:1] + e[2:] for e in sorted((t % T, ts[0] % T, ji, u) for ji, ts in enumerate(when) for u, t in enumerate(ts))]
    half = {}
    for e, (t, ji, u) in enumerate(evs):
        half[(ji, u)] = 2 * t + (0 if cfg['DBL'] and e + 1 < len(evs) and evs[e + 1][0] == t and (e == 0 or evs[e - 1][0] != t) else 1)
    SEG = cfg['SEG']
    for sg, seeds in enumerate(cfg['SEEDS']):
        mine = [e for e, ev in enumerate(evs) if ev[0] // SEG == sg]
        for seed in seeds:
            for e in mine:
                _, ji, u = evs[e]
                r = (e * 2654435761 + seed * 97531 + 12345) * 2246822519 % 4294967296 >> 8
                if r % 100 >= cfg['PJ']:
                    continue
                h = half[(ji, u)] + (2, -2, 1, -1, 2, -2)[r // 100 % 6]
                off = when[ji][u] - when[ji][u] % T
                lo_ = max(2 * (jobs[ji][0] - off), 2 * sg * SEG, half[evs[e - 1][1:]] + 1 if e else 0)
                hi_ = min(2 * (jobs[ji][1] - off) + 1, 2 * (sg + 1) * SEG - 1,
                          half[evs[e + 1][1:]] - 1 if e + 1 < len(evs) else 2 * (T - cfg['TAIL']))
                if lo_ <= h <= hi_:
                    half[(ji, u)] = h
    if cfg.get('SHOW'):
        for g in range(7, 14):
            rg = range(start[g], start[g + 1])
            print('  ', ''.join('%2d' % round(10 * use[t]) for t in rg))
            print('  ', ''.join('%2s' % ''.join((str(len(w)) if u == 0 else '.') for w in when for u, x in enumerate(w) if x % T == t) for t in rg))
    plan = {}
    for _, ji, u in evs:
        plan.setdefault(half[(ji, u)] // 2, []).append((half[(ji, u)] % 2, jobs[ji][3], jobs[ji][4], STAGES[jobs[ji][5]][u]))
    if cfg.get('PLANOUT') is not None:
        kind = lambda j: 'conv' if j[3] is None else 'fin' if j[3] == 'fin' else j[4].func.__name__ + str(j[4].args[1] if j[4].func.__name__ == 'unit2' else j[4].args[2])
        cfg['PLANOUT'].update(ev=[(half[(ji, u)], kind(jobs[ji]), u, jobs[ji][2][u]) for _, ji, u in evs], use=use,
                              rd=[(outs[g][1], str(rd)) for g, rd, t0, n in sched for _ in range(n)])
    assert all((ts[0] < 0) == (ts[-1] < 0) for ts in when)
    carried = [(job[4], job[5]) for ts, job in zip(when, jobs) if ts[0] < 0]

    def w_copy(l):
        return pltpu.make_async_copy(w_hbm.at[l], w_ref.at[l], sem.at[l])

    def w0_copy(u):
        return pltpu.make_async_copy(w_hbm.at[0, :, u], w_ref.at[0, :, u], sem.at[L + 10 + u])

    def in_copy(t, slot):
        return pltpu.make_async_copy(x_hbm.at[pl.ds(pl.multiple_of(t * TM, 32), TM)], xn2_ref.at[slot], sem.at[L + slot])

    def out_copy(t, slot, part):
        r0, nr = ((0, 2 * Mh), (2 * Mh, Mh), (3 * Mh, Mh))[part]
        return pltpu.make_async_copy(o2_ref.at[slot, pl.ds(r0, nr)],
                                     o_hbm.at[pl.ds(pl.multiple_of(t * TM + r0, 32), nr)],
                                     sem.at[L + 4 + 3 * slot + part])

    xr_in = pltpu.make_async_copy(x_hbm.at[pl.ds(NMAIN * TM, R0)], xr_ref, sem.at[L + 2])
    xr_out = pltpu.make_async_copy(xr_ref, o_hbm.at[pl.ds(NMAIN * TM, R0)], sem.at[L + 2])
    b_in = pltpu.make_async_copy(b_hbm, b_ref, sem.at[L + 3])

    def prologue():
        b_in.start()
        for u in range(8):
            w0_copy(u).start()
        xr_in.start()
        in_copy(0, 0).start()
        for l in range(1, L):
            w_copy(l).start()
        in_copy(min(1, NMAIN - 1), 1).start()
        b_in.wait()
        for l in range(L):
            bf_ref[l] = b_ref[l:l + 1, :].astype(f32)

        def bias_tiles(l, carry):
            b = jnp.broadcast_to(bf_ref[l] + (l == 0).astype(f32), (8, D))
            for u, site in enumerate(BIAS):
                terms = [b[:, key * 128:(key + 1) * 128] * cf for key, cf in sorted(bias_coefs(*site).items()) if cf != 0.0]
                bt_ref[l, u] = functools.reduce(lambda x, y: x + y, terms)
            return carry
        jax.lax.fori_loop(0, L, bias_tiles, 0)
        if cfg.get('FAST'):
            return

        def slab(u, carry):
            w0_copy(u).wait()
            zero = jax.lax.shift_right_logical(u, 12)
            prep(0, u, iter(lambda: None, 0), zero, kb0)
            return zero
        zero = jax.lax.fori_loop(0, cfg['NSLAB'], slab, 0)

        def plain(l, xbf, x0f, x, na, free, never, j0=0, j1=D // 128):
            passes = []
            for jt in range(j0, j1):
                cols = slice(jt * 128, (jt + 1) * 128)
                ya = _dot(xbf[:, :D // 2], w_ref[l, 0:4, :, :, cols].reshape(D // 2, 128)) + bf_ref[l, :, cols]
                passes += [ya, _dot(xbf[:, D // 2:], w_ref[l, 4:8, :, :, cols].reshape(D // 2, 128)) + ya]
            xp_ref[0, :, j0 * 128:j1 * 128] = x0f * jnp.concatenate(passes[1::2], axis=1) + x
            for u in range(na):
                f_ = (u - free) * len(passes) * (R0 // 8) // (na - free)
                if cfg['PPH'] is not None:
                    f_ = f_ // 2 * 2 + cfg['PPH']
                ps, rr = divmod(f_, R0 // 8)
                yield None if u < free else (never, passes[ps][rr * 8:rr * 8 + 8, :])

        for u in range(cfg['NSLAB'], 8):
            w0_copy(u).wait()
        xr_in.wait()
        never = jnp.broadcast_to(zero, (8, 128)) != 0
        jm = cfg['JM']
        x0f = xr_ref[:, :jm * 128].astype(f32)
        xp_ref[1, :, :jm * 128] = x0f
        anchors = plain(0, xr_ref[...], x0f, x0f, (8 - cfg['NSLAB']) * (28 + 4 * cfg['LANC'] + len(prods3)), cfg['AFREE'], never, 0, jm)
        for u in range(cfg['NSLAB'], 8):
            prep(0, u, anchors, zero, (kb0, kb1)[u % 2])
        in_copy(0, 0).wait()
        x0f = xr_ref[:, jm * 128:].astype(f32)
        xp_ref[1, :, jm * 128:] = x0f
        units = [(R, C, r) for R in range(4) for C in range(4) for r in range(0, Mh, 32)]
        anchors = plain(0, xr_ref[...], x0f, x0f, len(units) + sum(len(STAGES[n]) for _, n in carried) + 2, 4, never, jm)
        for R, C, r in units[:len(units) // 2]:
            conv(xn2_ref.at[0], zero, R, C, r, min(32, Mh - r), next(anchors))
        for fn, n in carried:
            st8 = {}
            for group in STAGES[n]:
                anchor = next(anchors)
                fn(st8, group, zero, jax.lax.shift_right_logical(zero, 1), anchor)
        for R, C, r in units[len(units) // 2:]:
            conv(xn2_ref.at[0], zero, R, C, r, min(32, Mh - r), next(anchors))

        def layer(l, carry):
            w_copy(l).wait()
            zero = jax.lax.shift_right_logical(l, 12)
            x = xp_ref[0]
            anchors = plain(l, x.astype(bf16), xp_ref[1], x, 8 * (28 + 4 * cfg['LANC'] + len(prods3)), cfg['AFREE'],
                            jnp.broadcast_to(zero, (8, 128)) != 0)
            for u in range(8):
                prep(l, u, anchors, zero, (kb0, kb1)[u % 2])
            return carry

        jax.lax.fori_loop(1, L, layer, 0)
        xr_ref[...] = xp_ref[0].astype(bf16)
        xr_out.start()

    def main(tile, carry):
        zs, za = jax.lax.shift_right_logical(tile, 12), jax.lax.shift_right_logical(tile, 13)
        never = jnp.broadcast_to(zs, (8, 128)) != 0
        slot = tile % 2
        in_copy(jnp.minimum(tile + 2, NMAIN - 1), slot).start()
        in_copy(jnp.minimum(tile + 1, NMAIN - 1), 1 - slot).wait()

        @pl.when(tile > 1)
        def _():
            for part in range(3):
                out_copy(tile - 2, slot, part).wait()

        xn_ref = xn2_ref.at[1 - slot]
        o_ref = o2_ref.at[slot]
        def rows(h, r0):
            if isinstance(h, tuple):
                return slice(r0 + h[0], r0 + h[0] + h[1])
            return slice(r0, r0 + Mh) if h is None else slice(r0 + h * Mq, r0 + (h + 1) * Mq)

        def ld(loc, h=None, z=0):
            return loc[0][(z,) + loc[1] + (rows(h, loc[2]),)]

        def st(loc, v, h=None):
            loc[0][(za if h == 1 and not loc[1] and cfg['ZB'] else zs,) + loc[1] + (rows(h, loc[2]),)] = v

        def by_half(v, h, fn):
            if isinstance(h, tuple):
                h = h[0] // Mq
            return fn(v, h) if h is not None else jnp.concatenate([fn(v[:Mq], 0), fn(v[Mq:], 1)], axis=0)

        def gather(ref, idx, n, pos):
            if cfg['NOBC']:
                return ref[idx + (slice(0, n), slice(16 * pos, 16 * pos + 16))].reshape(16 * n, 128)
            return ref.bitcast(u32)[idx + (slice(0, n), slice(8 * pos, 8 * pos + 8))].reshape(8 * n, 128)

        as_bf16 = lambda v: v if cfg['NOBC'] else pltpu.bitcast(v, bf16)

        def lhs2(p, q):
            ref, u = s2loc(p)
            return as_bf16(jnp.concatenate([gather(ref, (0, u, k), NC, q2[p].index(q)) for k in range(2)], axis=1))

        def rhs2(l, p, q, n):
            return as_bf16(gather(t2[p], (l, n), 16, q2[p].index(q)))

        def dot3(l, p, q, r):
            qs = next(qs for qs in PAIRS if q in qs)
            return _dot(as_bf16(gather(s3[(p, qs)], (0, qs.index(q)), NQ, ORD.index(r))),
                        as_bf16(gather(t3_ref, (l, prods3.index((p, q))), 8, ORD.index(r))))

        def add_bias(v, l, site, h):
            def one(x, hh):
                b = bt_ref[l, BIAS.index(site + (hh,))]
                return (x.reshape(x.shape[0] // 8, 8, 128) + b).reshape(x.shape)
            return by_half(v, h, one)

        def outer_act(l, p, i, j, n, d, h, part=None):
            bt, stores, finals = OACT[p]
            if part == 'raw':
                stores, finals = stores[:1], []
            if part == 'rest':
                bt, stores = [], stores[1:]
            if p == 6 and part is None and (i, j) != B12 and (h, n) != (0, 1):
                stores = []
            if bt:
                d = add_bias(d, l, (p, False, i, j, n), h)
            cache = {'d': d}
            def comb(terms):
                for _, src in terms:
                    if isinstance(src, str) and src not in cache:
                        cache[src] = ld(oloc(src, i, j, n), h)
                v = lincomb([(s, cache[src]) for s, src in terms if isinstance(src, str)])
                for _, src in terms:
                    if not isinstance(src, str):
                        v = add_bias(v, l, (p, True, i, j, n), h)
                return v
            fin = [(IJ, comb(terms)) for IJ, terms in finals]
            for name, v in [(name, comb(terms)) for name, terms in stores]:
                st(oloc(name, i, j, n), v, h)
            for (I, J), y in fin:
                R, C = 2 * I + i, 2 * J + j
                xn = ld(x0loc(R, C, n), h) * y
                if l > 0:
                    xn = xn + ld(xloc(l, R, C, n), h)
                if l < L - 1:
                    st(xloc(l + 1, R, C, n), xn, h)
                else:
                    xn = by_half(xn, h, lambda x, hh: x if scale(R, C, hh, n) == 1.0 else x * (1.0 / scale(R, C, hh, n)))
                    o_ref[rows(h, R * Mh), C * H + n * 128:C * H + (n + 1) * 128] = xn.astype(bf16)

        def inner_act(g, l, p, kind, n, h, P, Q, part=None):
            vloc = oloc(raw_slot(p), 0, 1, n) if raw_slot(p) else iloc(g, 'v', n)
            if kind == '35':
                st(iloc(g, 's', n), Q + ld(iloc(g, 'm1', n), h), h)
                if not raw_slot(p):
                    st(vloc, P, h)
                outer_act(l, p, 0, 1, n, P, h, part)
            elif kind == '47':
                st(iloc(g, 'u', n), Q + ld(vloc, h), h)
                outer_act(l, p, 0, 0, n, P + ld(iloc(g, 's', n), h), h, part)
            else:
                outer_act(l, p, 1, 1, n, ld(iloc(g, 's', n), h) - Q, h, part)
                outer_act(l, p, 1, 0, n, P + ld(iloc(g, 'u', n), h), h, part)

        def issue(l, p, rd):
            kind, n = rd
            if kind == 'x':
                return [dot3(l, p, q, 1) for q in (3, 5, 4, 7)]
            if kind == 'y':
                return [dot3(l, pp, q, 1) for pp in (p, SEL3[SEL3.index(p) + 1]) for q in (2, 6)]
            if isinstance(n, str):
                if cfg['MO']:
                    d = [dot3(l, p, int(q), int(r)) for q in kind for r in n]
                    return [d[0], d[2], d[1], d[3]]
                return [dot3(l, p, int(q), int(r)) for r in n for q in kind]
            if cfg['GR']:
                ops = [(lhs2(p, 1),) * 2, (rhs2(l, p, 1, 0), rhs2(l, p, 1, 1))] if kind == '1' else [
                    [lhs2(p, int(q)) for q in kind], [rhs2(l, p, int(q), n) for q in kind]]
                d = [_dot(a[:, k * 128:(k + 1) * 128], b[k * 128:(k + 1) * 128]) for a, b in zip(*ops) for k in range(2)]
                return [d[0] + d[1], d[2] + d[3], d[cfg['GR'] - 1]]
            if kind == '1':
                lhs = lhs2(p, 1)
                return [_dot(lhs, rhs2(l, p, 1, 0)), _dot(lhs, rhs2(l, p, 1, 1))]
            return [_dot(lhs2(p, int(q)), rhs2(l, p, int(q), n)) for q in kind]

        def consume(g, l, p, rd, res):
            kind, n = rd
            if n == '1':
                for u, where in enumerate((('35', False), ('47', False)) if kind == 'x' else (('26', False), ('26', True))):
                    for al in range(2):
                        st(jloc(where[0], '1', al, where[1]), res[2 * u + al], 0)
            elif isinstance(n, str):
                sm = [res[al] + res[2 + al] for al in range(2)]
                df = [res[al] - res[2 + al] for al in range(2)]
                J = lambda name, al: ld(jloc(kind, name, al, name == '1' and kind == '26' and p in SEL3[1::2]), 0)
                part = 'raw' if deferred(l, p, rd) else None
                done = lambda h, nn, m: inner_act(g, l, p, kind, nn, h, m[0] + m[1], m[0] - m[1], part)
                O, I = (lambda i, j: oloc(raw_slot(p), i, j, 1)), (lambda name: iloc(g, name, 1))
                rec = lambda al: [(s, ld(loc, 0, za if cfg['ZB'] else 0)) for s, loc in {
                    '35': [[(1, O(0, 1))], [(1, I('s')), (-1, I('m1'))]],
                    '47': [[(1, O(0, 0)), (-1, I('s'))], [(1, I('u')), (-1, O(0, 1))]],
                    '26': [[(1, O(1, 0)), (-1, I('u'))], [(1, I('s')), (-1, O(1, 1))]]}[kind][al]]
                if n == '35':
                    for al in range(2):
                        st(jloc(kind, 's', al), df[al] + J('1', al), 0)
                    done(0, 1, sm)
                elif n == '47':
                    if cfg['HY'] == 1:
                        for al in range(2):
                            st(jloc(kind, 'u', al), df[al], 0)
                    else:
                        for al, v in enumerate((df[0] + df[1], df[0] - df[1])):
                            st(jloc(kind, 'u', al), lincomb([(1, v)] + rec(al)), 0)
                    done(0, 0, [sm[al] + J('s', al) for al in range(2)])
                else:
                    if cfg['HY'] == 1:
                        m = [sm[al] + J('u', al) for al in range(2)]
                        P, Q = lincomb([(1, m[0] + m[1])] + rec(0)), lincomb([(1, m[0] - m[1])] + rec(1))
                    else:
                        P, Q = (sm[0] + sm[1]) + J('u', 0), (sm[0] - sm[1]) + J('u', 1)
                    done(1, 1, [J('s', al) - df[al] for al in range(2)])
                    inner_act(g, l, p, kind, 0, 1, P, Q, part)
            elif kind == '1':
                st(iloc(g, 'm1', 0), res[0])
                st(iloc(g, 'm1', 1), res[1])
            else:
                inner_act(g, l, p, kind, n, None, res[0] + res[1], res[0] - res[1])

        state = {}
        for g, rd, t0, n in sched:
            l, p = outs[g]
            if t0 == start[G - 1]:
                out_copy(tile, slot, 0).start()
            if t0 + n == T:
                out_copy(tile, slot, 1).start()
            res = issue(l, p, rd)
            if cfg['EO']:
                consume(g, l, p, rd, res)
            for t in range(t0, t0 + n):
                for ph, l2, fn, group in plan.get(t, []):
                    gr = 16 * (t - t0) + 8 * ph
                    if cfg['GF']:
                        gr = 16 * (t - t0) + 8 * (1 - ph)
                    gs = cfg['GS']
                    gate = res[2 if len(res) == 3 else cfg['GM']][gr:gr + 8, :]
                    if cfg['GADD'] and isinstance(rd[1], str) and rd[1] != '1':
                        gate = gate + res[2 + gs % 2][gr:gr + 8, :]
                    elif gs == 2 and rd[0] != '1' and rd[1] != '1':
                        gate = gate + res[1][gr:gr + 8, :]
                    if l2 == 'fin':
                        for i, j, nf, r0 in fn[2]:
                            d = ld(oloc(raw_slot(fn[1]), i, j, nf), (r0, 16))
                            d = tie(tie(d, (never, gate)), (never, gate), 8)
                            outer_act(fn[0], fn[1], i, j, nf, d, (r0, 16), 'rest')
                    elif l2 is None:
                        conv(xn_ref, zs, *fn, min(32, Mh - fn[2]), (never, gate))
                    else:
                        fn(state.setdefault(id(fn), {}), group, zs, za, (never, gate))
            if not cfg['EO']:
                consume(g, l, p, rd, res)
        out_copy(tile, slot, 2).start()
        return carry

    prologue()
    if not cfg.get('NOMAIN'):
        jax.lax.fori_loop(0, NMAIN, main, 0)
    else:
        for p_ in range(1, 8):
            for l_ in range(L):
                o2_ref[0, 0:16, 0:128] = t2[p_][l_, 0, pl.program_id(0) if False else 3, 0:16] + t3_ref[l_, p_, 2, 0:16]
    xr_out.wait()
    in_copy(NMAIN - 1, (NMAIN - 1) % 2).wait()
    for t in range(max(NMAIN - 2, 0), NMAIN):
        for part in range(3):
            out_copy(t, t % 2, part).wait()


DEFAULT = dict(SEL=(3, 5, 4, 7, 2, 6), SEL3=(3, 5, 4, 7), XC={B12: 5, B11: 1, B22: 7, B21: 2}, AFREE=2, NOBC=0, LANC=1, KD=1, PO=PREP_ORDER, PT=0, MAT=4, FOLD=1, MO=1, GR=2, NS=(2, 3, 3, 4, 3), NL=1, GE=6, GM=0, DBL=1, GS=0, GF=0, EO=0, KP=16, PPH=None, ZB=0, HY=1, HOLD=0, PORT=0.9, PS=0, NSLAB=6, JM=3, XP=40, XO=16, DEFER={5: [('26', '26'), ('47', '26')], 7: [('26', '26'), ('47', '26')], 2: [('35', '26'), ('47', '26')],
                      6: [('35', '26'), ('47', '26')]}, DEFL={}, EW=12, KW=(1,) * 5, CM=(1,) * 7, SEEDS=(), SEG=32, PJ=20, QO=0, TIEL=2, GADD=0, TF=0, T8=0, TAIL=6,
               CS=0.5, CL=0.3, UL=0.8, CAP=0.95, FR=((1.,), (.4, .6), (.35, .37, .28), (.16, .26, .31, .27),
                   (.35, .29, .08, .28), (.16, .26, .26, .05, .27)))


def build(TM=640, **kw):
    def f(x0, ws, bs):
        B, D = x0.shape
        L = ws.shape[0]
        cfg = dict(DEFAULT, **kw)
        Mh = TM // 4
        MP = Mh + 32
        nmain = (B - 1) // TM
        R0 = B - nmain * TM
        pairs3, q2 = layout(cfg)
        n3 = sum(2 * len(v) for v in pairs3.values())
        pad = lambda n: n + (2 - n) % 4
        V = pltpu.VMEM
        half = V((1, MP, 128), f32)
        XP = Mh + cfg['XP']
        scratch = ([V((1, 2, 2, 2, XP, 128), f32)] * 4 + [V((1, 2, 4, 2, XP, 128), f32)] * 7 + [half] * (16 + 64 + 26)
                   + [V((1, 1 + (p == 2 and q2[2] == q2[6]), 2, pad(Mh // 16), 16 * len(q2[p]), 128), bf16) for p in range(1, 8)]
                   + [V((1, 2, pad(Mh // 32), 112, 128), bf16)] * (n3 // 2)
                   + [V((L, 2, 16, 16 * len(q2[p]), 128), bf16) for p in range(1, 8)]
                   + [V((L, n3, 8, 112, 128), bf16), V((1, 4, 16 * n3 + cfg['KP'], 128), f32), V((1, 4, 16 * n3 + cfg['KP'], 128), f32),
                      V((L, len(BIAS), 8, 128), f32), V((8, 1, D), f32), V((2, TM, D), bf16), V((2, TM, D), bf16), V((L, 8, 8, 16, D), bf16),
                      V((R0, D), bf16), V((2, R0, D), f32), V((L, D), bf16), pltpu.SemaphoreType.DMA((L + 18,))])
        anyspec = pl.BlockSpec(memory_space=pl.ANY)
        return pl.pallas_call(
            functools.partial(_kernel, L=L, TM=TM, R0=R0, NMAIN=nmain, D=D, cfg=cfg),
            in_specs=[anyspec, anyspec, anyspec],
            out_specs=anyspec,
            out_shape=jax.ShapeDtypeStruct((B, D), x0.dtype),
            scratch_shapes=scratch,
            compiler_params=pltpu.CompilerParams(
                vmem_limit_bytes=120 * 1024 * 1024,
                internal_scratch_in_bytes=65536,
                disable_bounds_checks=True,
            ),
        )(x0, ws.reshape(L, 8, 8, 16, D), bs)
    return f


@jax.jit
def pallas_standalone__dcn_v2_cross__recsys_kernel(x0, ws, bs):
    return build(TM=640)(x0, ws, bs)
```

```python
import functools

import jax
import jax.numpy as jnp
import jax.experimental.pallas as pl
import jax.experimental.pallas.tpu as pltpu

f32 = jnp.float32
bf16 = jnp.bfloat16
u32 = jnp.uint32

B11, B12, B21, B22 = (0, 0), (0, 1), (1, 0), (1, 1)
LA = {1: [(B11, 1), (B22, 1)], 2: [(B11, 1), (B12, 1), (B21, 1), (B22, 1)], 3: [(B11, 1), (B12, -1)],
      4: [(B12, 1), (B22, 1)], 5: [(B11, 1), (B12, 1)], 6: [(B12, 1), (B11, -1), (B21, 1), (B22, -1)],
      7: [(B12, 1), (B22, -1)]}
PAIRS = ((5, 3), (4, 7), (2, 6))
ORD = (3, 5, 4, 7, 1, 2, 6)
D2 = (1.0, 2.0)
BF = {1: 1.0, 2: 0.5, 3: 0.5, 4: 0.5, 5: 0.5, 6: 0.5, 7: 0.5}
OUTER = (3, 5, 1, 4, 7, 2, 6)
OACT = {
    3: ([(1, B12)], [('M3', [(1, 'd')])], []),
    5: ([], [('M5', [(1, 'd')])], [(B12, [(1, 'd'), (1, 'M3')])]),
    1: ([(1, B11), (-1, B12)], [('S', [(1, 'd'), (1, 'M3'), (-1, 'M5')])], []),
    4: ([], [('M4', [(1, 'd')])], []),
    7: ([], [('M7', [(1, 'd')])], [(B11, [(1, 'd'), (1, 'S'), (1, 'M4')])]),
    2: ([(1, B11), (-1, B22)], [('M2', [(1, 'd')]),
        ('U', [(1, 'd'), (1, 'M4'), (-1, 'M7'), (1, 'M3'), (1, 'M5'), (1, ((1, B21), (-1, B12), (-1, B11), (1, B22)))])], []),
    6: ([], [('M6', [(1, 'd')])], [(B22, [(1, 'd'), (1, 'S'), (-1, 'M2')]), (B21, [(1, 'd'), (1, 'U')])]),
}
OSL = {'M3': 0, 'M5': 1, 'S': 2, 'M4': 3, 'M7': 4, 'M2': 6, 'U': 5, 'M6': 7}
ISL = {'m1': 0, 's': 1, 'v': 2, 'u': 3}
STAGES = {1: [(B11, B12, B21, B22)], 2: [(B11, B12), (B21, B22)], 3: [(B11, B12), (B22,), (B21,)],
          4: [(B11,), (B12,), (B22,), (B21,)], 5: [(B11, B12), (B22, 'hold'), ('l1',), (B21,)],
          6: [(B11,), (B12,), (B22, 'hold'), ('l1',), (B21,)]}
BIAS = [(p, extra, i, j, n, h) for p in OUTER for extra in (False, True)
        if (any(not isinstance(x, str) for _, t in OACT[p][1] + OACT[p][2] for _, x in t) if extra else OACT[p][0])
        for i in range(2) for j in range(2) for n in range(2) for h in range(2)]
PREP_ORDER = (2, 6, 3, 5, 1, 4, 7)
GAMMA = 0.125
LAG = 8


def _dot(a, b):
    return jnp.dot(a, b, preferred_element_type=f32)


def scale(R, C, h, k):
    return D2[R // 2] * D2[R % 2] * D2[h] / (D2[C // 2] * D2[C % 2] * D2[k])


def phys(C, k):
    return 4 * (C // 2) + 2 * k + C % 2


def b_ops(b11, b12, b21, b22):
    r1 = b11 + b22
    g = b12 + b21
    return {1: r1, 2: b11 - b12, 3: b12 - b22, 4: g - r1, 5: b12 + b22, 6: b11 + b12, 7: g + r1}


def lincomb(terms):
    assert terms[0][0] == 1
    acc = terms[0][1]
    for s, v in terms[1:]:
        acc = acc + v if s == 1 else acc - v
    return acc


def raw_slot(p):
    return next((name for name, terms in OACT[p][1] if terms == [(1, 'd')]), None)


def round_usage(p, rd, first, last, defer, hy):
    bt, stores, finals = OACT[p]
    alu = bool(bt) + sum(len(t) - 1 for _, t in stores) + sum(len(t) + (not first) + 2 * last for _, t in finals)
    nst = len(stores) + len(finals)
    nld = len({x for _, t in stores + finals for _, x in t if isinstance(x, str) and x != 'd'}) + len(finals) * (2 - first)
    kind, n = rd
    if defer:
        alu, nst, nld = bool(bt), 1, 0
    elif p == 6 and kind != '35' and n != '35':
        nst -= 1
    if isinstance(n, str):
        e = kind == '47'
        if kind == '26':
            a, st, ld, m = {'35': (10, 2, 9, 2), '47': (10, 2, 9, 2) if hy == 1 else (16, 2, 13, 2), '26': (20, 0, 17, 4) if hy == 1 else (16, 0, 13, 4)}[n]
        else:
            a, st, ld, m = {'1': (0, 4, 5, 0), '35': (9 + e, 3, 8 + e, 1),
                            '47': (9 + e, 3, 8 + e, 1) if hy == 1 else (14 + 2 * e, 3, 11 + 2 * e, 1),
                            '26': (17 + 3 * e, 2, 14 + 3 * e, 2) if hy == 1 else (14 + 2 * e, 2, 11 + 2 * e, 2)}[n]
    else:
        a, st, ld, m = {'1': (2, 2, 4, 0), '35': (5, 2 - bool(raw_slot(p)), 5, 1), '47': (6, 1, 6, 1),
                        '26': (6, 0, 6, 2)}[kind]
    return a + m * alu, st + m * nst, ld + m * nld


def yds(groups, cap):
    n = len(cap)
    speed, cls, gcls = [0.0] * n, [-1] * n, {}
    todo = list(groups)
    while todo:
        pre = [0.0]
        for t in range(n):
            pre.append(pre[-1] + (cap[t] if cls[t] < 0 else 0.0))
        best = None
        for a in sorted({g[0] for g in todo}):
            w = 0.0
            for g in sorted((g for g in todo if g[0] >= a), key=lambda g: g[1]):
                w += g[2]
                d = w / max(pre[g[1] + 1] - pre[a], 1e-9)
                if best is None or d > best[0]:
                    best = (d, a, g[1])
        d, a, b = best
        for t in range(a, b + 1):
            if cls[t] < 0:
                speed[t], cls[t] = d, len(gcls)
        gcls.update({g[:2]: len(gcls) for g in todo if g[0] >= a and g[1] <= b})
        todo = [g for g in todo if not (g[0] >= a and g[1] <= b)]
    return speed, cls, gcls


def spread_jobs(jobs, cap, tail):
    T = len(cap)
    cap3 = cap * 3
    all3 = [(lo + k * T, hi + k * T, ji, k) for k in range(3) for ji, (lo, hi, _) in enumerate(jobs) if lo + k * T >= 0]
    pend = {}
    for j in sorted(all3, key=lambda j: (j[1], j[3], j[2])):
        pend.setdefault(j[:2], []).append(j)
    speed, cls, gcls = yds([w + (sum(sum(jobs[j[2]][2]) for j in q),) for w, q in pend.items()], cap3)
    when = [[] for _ in jobs]
    debt, cur, done = 0.0, None, 0
    for t in range(3 * T):
        while True:
            j = cur
            if j is None:
                rdy = [q[0] for w, q in pend.items() if q and w[0] <= t and (gcls[w] == cls[t] or w[1] <= t)]
                if not rdy:
                    debt = max(debt, 0.0)
                    break
                j = rdy[0]
                nst = len(jobs[j[2]][2])
                if nst > 1 and j[1] > t and (t + tail + 2 * nst) // T != t // T:
                    break
            must = j[1] <= t or (cur is not None and (t + tail + 1) // T != t // T)
            if not must and (cap3[t] == 0.0 or debt > 0.5 * speed[t] * cap3[t]):
                break
            if cur is None:
                pend[j[:2]].pop(0)
                cur, done = j, 0
            debt += jobs[j[2]][2][done]
            if j[3] == 1:
                when[j[2]].append(t - T)
            done += 1
            if done == len(jobs[j[2]][2]):
                cur = None
        debt -= speed[t] * cap3[t]
    return when


def layout(cfg):
    sel, sel3 = cfg['SEL'], cfg['SEL3']
    pairs3 = {p: [qs for qs in PAIRS if p in sel3 or (p in sel and qs != (2, 6))] for p in range(1, 8)}
    q2 = {p: [q for q in ORD if not any(q in qs for qs in pairs3[p])] for p in range(1, 8)}
    return pairs3, q2


def _kernel(x_hbm, w_hbm, b_hbm, o_hbm, *scratch, L, TM, R0, NMAIN, D, cfg):
    H, Mh, Mq = D // 4, TM // 4, TM // 8
    NC, NQ = Mh // 16, Mq // 16
    MP = Mh + 32
    SEL, SEL3 = cfg['SEL'], cfg['SEL3']
    pairs3, q2 = layout(cfg)
    prods3 = [(p, q) for p in SEL for qs in pairs3[p] for q in qs]
    assert NMAIN >= 3 and H == 256 and L % 2 == 0 and Mq % 16 == 0 and all(raw_slot(p) for p in SEL)
    it = iter(scratch)
    take = lambda n: [next(it) for _ in range(n)]
    x0b, xb, ib, ob, jb = take(4), take(7), take(16), take(64), take(26)
    joint = q2[2] == q2[6]
    MAT = cfg['MAT'] and joint and 2 in SEL
    s2 = dict(zip(range(1, 8), take(7)))
    s3 = {(p, qs): next(it) for p in SEL for qs in pairs3[p]}
    t2 = dict(zip(range(1, 8), take(7)))
    t3_ref, kb0, kb1, bt_ref, bf_ref, xn2_ref, o2_ref, w_ref, xr_ref, xp_ref, b_ref, sem = it

    xset = lambda l: 6 if l == 'O' else 4 if l == 0 else (l % 2) * 2
    xoff = lambda I, J: cfg['XO'] * ((I + J) % 2)
    xloc = lambda l, R, C, k: (xb[xset(l) + R // 2], (R % 2, C, k), xoff(R // 2, C // 2))
    x0loc = lambda R, C, k: (x0b[(R // 2) * 2 + C // 2], (R % 2, C % 2, k), 8 + xoff(R // 2, C // 2))
    iloc = lambda g, name, n: (ib[((g % 2) * 4 + ISL[name]) * 2 + n], (), 8 * ISL[name])
    oloc = lambda name, i, j, n: (ob[(OSL[name] * 4 + i * 2 + j) * 2 + n], (), 8 * ((OSL[name] + 2 * j) % 4))

    def jloc(kind, name, al, second=False):
        i = 24 + al if second else (('35', '47', '26').index(kind) * 4 + ('1', 's', 'u', 'v').index(name)) * 2 + al
        return jb[i], (), 8 * ((i + i // 2) % 4)

    def s2loc(p):
        return (s2[2], (2, 6).index(p)) if p in (2, 6) and joint else (s2[p], 0)

    def bias_coefs(p, extra, i, j, n, h):
        where = [(1, i, j, n, h)]
        if extra:
            terms = next(x for _, t in OACT[p][1] + OACT[p][2] for _, x in t if not isinstance(x, str))
        else:
            terms = OACT[p][0]
            w = [(1, i, j)] + [(-1, 0, 1)] * bool(raw_slot(p) and (i, j) == B21)
            where = [x + (n, h) for x in w]
            if (h, n) == (1, 0) and PAIRS[{B12: 0, B11: 1}.get((i, j), 2)] in pairs3[p]:
                where += [(-sg, ii, jj, 1, 0) for sg, ii, jj in w]
        coef = {}
        for sg, ii, jj, nn, hh in where:
            for cf, (I, J) in terms:
                key = phys(2 * J + jj, nn)
                coef[key] = coef.get(key, 0.0) + sg * cf * scale(2 * I + ii, 2 * J + jj, hh, nn) / GAMMA
        return coef

    def tie(v, anchor, r=0):
        if anchor is None:
            return v
        return jnp.concatenate([v[:r]] * (r > 0) + [jax.lax.select(anchor[0], anchor[1], v[r:r + 8])] + [v[r + 8:]] * (r + 8 < v.shape[0]), axis=0)

    def consts(anchor, ss, reps):
        one = {s: jnp.full((8, 128), s, f32) for s in set(ss)}
        if anchor is not None:
            one = {s: jax.lax.select(anchor[0], anchor[1], v) for s, v in one.items()}
        return jnp.concatenate([one[s] for s in ss for _ in range(reps)], axis=0)

    def conv(src, zs, R, Q, r, nr, anchor=None):
        v = src[R * Mh + r:R * Mh + r + nr, Q * H:(Q + 1) * H].astype(f32)
        for j in range(2):
            C, k = 2 * (Q // 2) + j, Q % 2
            buf, idx, off = xloc(0, R, C, k)
            sv = consts(anchor, [scale(R, C, (r + u) // Mq, k) for u in range(0, nr, 16)], 2)
            buf[(zs,) + idx + (slice(off + r, off + r + nr),)] = v[:, j * 128:(j + 1) * 128] * sv

    cnt = {}
    def block_sum(l, terms, ii, jj, kk, r, save, zs, za, anchor, late=None):
        rng = lambda t: slice(t[0], t[-1] + 1)
        keys = [(i, j, k) for i in ii for j in jj for k in kk]
        vals = []
        for u, ((I, J), s) in enumerate(terms):
            ref, r0 = xb[xset(l) + I], xoff(I, J) + r
            v = ref[za if u == 0 else 0, rng(ii), 2 * J + jj[0]:2 * J + jj[-1] + 1, rng(kk), r0:r0 + 16, :]
            if (I, J) in save:
                sv = consts(anchor, [GAMMA / scale(2 * I + i, 2 * J + j, r // Mq, k) for i, j, k in keys], 2)
                x0b[I * 2 + J][zs, rng(ii), rng(jj), rng(kk), r0 + 8:r0 + 24, :] = v * sv.reshape(v.shape)
            v = v.reshape(16 * len(keys), 128)
            if u == 0 and late is not None and anchor is not None:
                cnt[xset(l)] = cnt.get(xset(l), -1) + 1
                if cnt[xset(l)] % cfg['GE'] == 0:
                    ref[0, 0, 0, 0, Mh + 24:Mh + 32, :] = anchor[1]
                at = 16 * keys.index(late)
                top = v[at:at + 8] if cfg['NL'] else ref[za, late[0], 2 * J + late[1], late[2], r0:r0 + 8, :]
                if cfg['TIEL'] == 2:
                    top = jax.lax.select(anchor[0], anchor[1], top)
                v = jnp.concatenate([v[:at]] * (at > 0) + [top, v[at + 8:]], axis=0)
            vals.append((s, v))
        v = lincomb(vals)
        if cfg['TIEL'] == 3 and late is not None:
            v = tie(v, anchor, 16 * keys.index(late))
        return v

    def release(qs, store, st8, anchor):
        v = st8['l1']
        if anchor is not None:
            n = v.shape[0]
            top = jax.lax.select(jnp.broadcast_to(anchor[0], (n, 8, 128)), jnp.broadcast_to(anchor[1], (n, 8, 128)), v[:, :8])
            v = jnp.concatenate([top, v[:, 8:]], axis=1)
        r0 = 16 * qs.index(1)
        store(slice(r0, r0 + 16), v.astype(bf16))

    def finish(e, f, group, qs, store, st8, anchor, hold=False, keep=None):
        a = e[None] if f is None else jnp.concatenate([e + f, e - f], axis=0).reshape(2, e.shape[0], 128)
        for u, b in enumerate(group):
            st8[b] = a if len(group) == 1 else a[:, 16 * u:16 * u + 16]
            if keep:
                keep(b, st8[b])
        ops = {}
        if B12 in group and 3 in qs:
            ops[3], ops[5] = st8[B11] - st8[B12], st8[B11] + st8[B12]
        if B22 in group:
            if 4 in qs:
                ops[4], ops[7] = st8[B12] + st8[B22], st8[B12] - st8[B22]
            ops[1] = st8['l1'] = st8[B11] + st8[B22]
        if B21 in group:
            g = st8[B12] + st8[B21]
            ops[2], ops[6] = g + st8['l1'], g - st8['l1']
        now = [q for q in qs if q in ops and not (hold and q == 1)]
        if now:
            r0 = 16 * qs.index(now[0])
            store(slice(r0, r0 + 16 * len(now)), jnp.concatenate([ops[q] for q in now], axis=1).astype(bf16))

    def unit2(l, ps, c, k, save, st8, group, zs, za, anchor):
        def store(rows, v):
            s2[ps[0]][zs, :, k, c, rows, :] = v
        if group == ('l1',):
            return release(q2[ps[0]], store, st8, anchor)
        hold, group = 'hold' in group, tuple(b for b in group if b != 'hold')
        ii, jj = sorted({b[0] for b in group}), sorted({b[1] for b in group})
        bs = lambda terms, late: block_sum(l, terms, ii, jj, [k], 16 * c, save, zs, za, anchor, late)
        f = None if len(ps) == 1 else bs([(B11, 1), (B22, 1)], None)
        e = bs(LA[ps[0]] if len(ps) == 1 else [(B12, 1), (B21, 1)], (ii[0], jj[-1], k))
        def keep(b, v):
            if b != B21:
                for J in range(2):
                    xb[6][zs, b[0], 2 * J + b[1], k, xoff(0, J) + 16 * c:xoff(0, J) + 16 * c + 16, :] = v[J]
        if f is None or joint:
            return finish(e, f, group, q2[ps[0]], store, st8, anchor, hold, keep if f is not None and MAT else None)
        for p, v in zip(ps, (e + f, e - f)):
            def store1(rows, w):
                s2[p][zs, :, k, c, rows, :] = w
            finish(v, None, group, q2[p], store1, st8.setdefault(p, {}), anchor)

    def unit3(l, p, qs, c, save, st8, group, zs, za, anchor):
        def store(rows, w):
            s3[(p, qs)][zs, :, c, rows, :] = w
        if group == ('l1',):
            return release(ORD, store, st8, anchor)
        hold, group = 'hold' in group, tuple(b for b in group if b != 'hold')
        for h in sorted({b[0] for b in group}):
            grp = tuple(b for b in group if b[0] == h)
            kk = [b[1] for b in grp]
            ii, jj = {(5, 3): ([0], [0, 1]), (4, 7): ([0, 1], [1]), (2, 6): ([0, 1], [0, 1])}[qs]
            src = ('O', [((0, (2, 6).index(p)), 1)]) if MAT and p in (2, 6) else (l, LA[p])
            v = block_sum(*src, ii, jj, sorted(kk), h * Mq + 16 * c, save, zs, za, anchor,
                          (0, (0 if cfg['TF'] else 1) if qs == (2, 6) else jj[0], max(kk)) if h == group[-1][0] else None)
            n = 16 * len(kk)
            piece = lambda u: v[u * n:(u + 1) * n]
            if qs == (2, 6):
                e, f = piece(1) + piece(2), piece(0) + piece(3)
                r0 = 16 * q2[p].index(1)
                s2[p][zs, 0, min(kk):max(kk) + 1, h * NQ + c, r0:r0 + 16, :] = f.reshape(len(kk), 16, 128).astype(bf16)
            else:
                e, f = piece(0), piece(1)
            finish(e, f, tuple(sorted(grp)), ORD, store, st8, anchor, hold)

    def prep(l, u, anchors, zero, kb):
        mul = lambda v, s: v if s == 1.0 else v * s
        def third(e, last):
            v = kb[0, 0:4 if last is None else 3, 16 * e:16 * e + 16, :]
            T = b_ops(v[0], tie(v[1], next(anchors)), v[2], v[3] if last is None else last)
            T[1] = T[1] * 2.0
            t3_ref[l, e, u] = jnp.concatenate([T[q] for q in ORD], axis=0).astype(bf16)
        for k in range(2):
            wide = [w_ref[l, phys(R, k), u].astype(f32) for R in range(4)]
            for n in range(2):
                la = next(anchors) if cfg['LANC'] else None
                def blk(R, C):
                    v = mul(wide[R][:, phys(C, n) * 128:(phys(C, n) + 1) * 128], scale(R, C, k, n))
                    return tie(v, la) if (R // 2, C // 2) == B12 else v
                O = {(i, j): b_ops(blk(i, j), blk(i, 2 + j), blk(2 + i, j), blk(2 + i, 2 + j)) for i, j in (B11, B12, B21, B22)}
                for p in cfg['PO']:
                    o = [mul(O[b][p], BF[p] * (0.25 if p in SEL else 0.5) / GAMMA) for b in (B11, B12, B21, B22)]
                    T = b_ops(o[0], tie(o[1], next(anchors)), o[2], o[3])
                    t2[p][l, n, k * 8 + u] = jnp.concatenate(
                        [mul(T[q], BF[q] * (4.0 if p in SEL else 2.0)) for q in q2[p]], axis=0).astype(bf16)
                    mine = [e for e, pq in enumerate(prods3) if pq[0] == p]
                    if cfg['KD'] and (k, n) == (1, 1):
                        for e in mine:
                            third(e, T[prods3[e][1]])
                    elif mine:
                        kb[zero, k * 2 + n, 16 * mine[0]:16 * mine[-1] + 16, :] = jnp.concatenate(
                            [T[prods3[e][1]] for e in mine], axis=0)
        if not cfg['KD']:
            for e in range(len(prods3)):
                third(e, None)

    def rounds_of(p):
        rs = [('1', None)] + [('x', '1')] * (p in SEL)
        for kind, qs in zip(('35', '47', '26'), PAIRS):
            if kind == '26' and p in SEL3[::2]:
                rs.append(('y', '1'))
            rs += [(kind, r) for r in (('35', '47', '26') if qs in pairs3[p] else (0, 1))]
        return rs

    def deferred(l, p, rd):
        return rd in cfg['DEFER'].get(p, ()) or (l == L - 1 and rd in cfg['DEFL'].get(p, ()))

    outs = [(l, p) for l in range(L) for p in OUTER]
    G = len(outs)
    sched, start, use = [], [], []
    for g, (l, p) in enumerate(outs):
        start.append(len(use))
        for rd in rounds_of(p):
            n = NQ if isinstance(rd[1], str) else NC
            sched.append((g, rd, len(use), n))
            a, st_, ld_ = round_usage(p, rd, l == 0, l == L - 1, deferred(l, p, rd), cfg['HY'])
            if cfg['PORT']:
                use += [max((2 * a + st_ + 2 + 16 / n) / 72 + cfg['PS'] * st_ / 8, cfg['PORT'] * st_ / 8)] * n
            else:
                use += [max(a / 32, st_ / 8, cfg['UL'] * ld_ / 24)] * n
    T = len(use)
    cap = [max(cfg['CAP'] - max(use[t], use[(t + 1) % T], cfg['UMIN']), 0.0) ** cfg['GAM'] * (t < T - cfg['TAIL']) for t in range(T)]
    for g in range(G):
        for t in range(start[g], (start + [T])[g + 1]):
            cap[t] *= cfg['CM'][g % 7]
    jobs = []
    def add(lo, hi, alu, st_, ld_, nst, l, fn):
        w = alu / 64 + cfg['CS'] * (st_ + nst) / 16 + cfg['CL'] * ld_ / 48
        w *= cfg['KW'][0 if l in (None, 'fin') else nst]
        if cfg['HOLD'] and nst >= 3:
            nst += 2
        jobs.append((lo, max(hi, lo), [w * f for f in cfg['FR'][nst - 1]], l, fn, nst))
    for g, (l, p) in enumerate(outs):
        ready = 7 * l - 2 * all(I == 0 for (I, J), _ in LA[p])
        lo = start[ready] - (T if ready < 0 else 0)
        if cfg['DEFER'].get(7) and ready % 7 == 5 and l > 0:
            lo += cfg['EW'] + 1
        for gg, rd, t0, n_ in sched:
            if gg == g and deferred(l, p, rd):
                if p == 7:
                    due = start[g + 1] + cfg['EW'] if l < L - 1 else start[g + 2] - 1
                elif p == 5:
                    due = start[7 * l + 5] - 1
                elif p == 6:
                    due = (start[g + 1] if l < L - 1 else T - NC) - 1
                else:
                    due = [t for g2, r2, t, _ in sched if g2 == g + 1 and r2[0] == rd[0]][0] - 3
                nops = 4 * sum(len(t) + (x in OACT[p][2]) * (2 + 2 * (l == L - 1)) for x in OACT[p][1][1:] + OACT[p][2] for t in x[1:])
                ws = [(i, j, n, h * Mq + 16 * c) for c in range(NQ) for h, n in {'35': [(0, 1)], '47': [(0, 0)], '26': [(1, 1), (1, 0)]}[rd[1]]
                      for i, j in {'35': [B12], '47': [B11], '26': [B22, B21]}[rd[0]]]
                m_ = 1 if p == 6 else 2
                for u in range(0, len(ws), m_):
                    add(t0 + n_, due, nops * m_ // 2, 3, nops * m_ // 2, 1, 'fin', (l, p, ws[u:u + m_]))
        hi = start[g] - LAG - 3
        nt = len(LA[p])
        save = [b for b, pp in cfg['XC'].items() if pp == p and l == 0]
        if p in SEL3:
            if p in SEL3[1::2]:
                host = 7 * l + OUTER.index(SEL3[SEL3.index(p) - 1])
                hi = [t0 for gg, rd, t0, _ in sched if gg == host and rd[0] == 'y'][0] - LAG - 3
            for c in range(NQ):
                add(lo, hi, 32 * nt + 50 + 32 * len(save), 18 + 32 * len(save), 32 * nt, cfg['NS'][3], l,
                    functools.partial(unit3, l, p, (2, 6), c, save))
        elif p != 6:
            ps = (2, 6) if p == 2 else (p,)
            nq = sum(len(q2[x]) for x in ps)
            alu = 8 * (nt - 2 + len(ps)) + sum(8 if x in SEL else 16 for x in ps) + nq
            if MAT and p == 2:
                hi = start[7 * l + cfg['MAT']] - 3
            for c in range(NC):
                for k in range(2):
                    add(lo, hi, alu + 8 * len(save), nq + 8 * len(save) + 12 * (bool(MAT) and p == 2), 8 * nt, 1 if nq <= 3 else cfg['NS'][4] if nq == 6 else cfg['NS'][0] if nq <= 7 else cfg['NS'][1], l,
                        functools.partial(unit2, l, ps, c, k, save))
        if MAT and p in (2, 6):
            lo, nt = start[7 * l + cfg['MAT']], 1
        if p in SEL:
            for qs, c in ([(qs, c) for qs in PAIRS[:2] for c in range(NQ)] if cfg['QO'] else
                          [(qs, c) for c in range(NQ) for qs in PAIRS[:2]]):
                if True:
                    add(lo, start[g] - LAG - 3 + (NC if g else 0), 16 * nt + 46, 14, 16 * nt, cfg['NS'][2 + (nt == 4)], l,
                        functools.partial(unit3, l, p, qs, c, []))
    for R in range(4):
        for C in range(4):
            for c in range(0, NC, 2):
                add(start[6], start[G - 2] - 2, 18, 7, 4, 1, None, (R, C, 16 * c))
    when = spread_jobs([j[:3] for j in jobs], cap, cfg['TAIL'])
    evs = [e[:1] + e[2:] for e in sorted((t % T, ts[0] % T, ji, u) for ji, ts in enumerate(when) for u, t in enumerate(ts))]
    half = {}
    for e, (t, ji, u) in enumerate(evs):
        half[(ji, u)] = 2 * t + (0 if cfg['DBL'] and e + 1 < len(evs) and evs[e + 1][0] == t and (e == 0 or evs[e - 1][0] != t) else 1)
    SEG = cfg['SEG']
    for sg, seeds in enumerate(cfg['SEEDS']):
        mine = [e for e, ev in enumerate(evs) if ev[0] // SEG == sg]
        for seed in seeds:
            for e in mine:
                _, ji, u = evs[e]
                r = (e * 2654435761 + seed * 97531 + 12345) * 2246822519 % 4294967296 >> 8
                if r % 100 >= cfg['PJ']:
                    continue
                h = half[(ji, u)] + (2, -2, 1, -1, 2, -2)[r // 100 % 6]
                off = when[ji][u] - when[ji][u] % T
                lo_ = max(2 * (jobs[ji][0] - off), 2 * sg * SEG, half[evs[e - 1][1:]] + 1 if e else 0)
                hi_ = min(2 * (jobs[ji][1] - off) + 1, 2 * (sg + 1) * SEG - 1,
                          half[evs[e + 1][1:]] - 1 if e + 1 < len(evs) else 2 * (T - cfg['TAIL']))
                if lo_ <= h <= hi_:
                    half[(ji, u)] = h
    if cfg.get('SHOW'):
        for g in range(7, 14):
            rg = range(start[g], start[g + 1])
            print('  ', ''.join('%2d' % round(10 * use[t]) for t in rg))
            print('  ', ''.join('%2s' % ''.join((str(len(w)) if u == 0 else '.') for w in when for u, x in enumerate(w) if x % T == t) for t in rg))
    plan = {}
    for _, ji, u in evs:
        plan.setdefault(half[(ji, u)] // 2, []).append((half[(ji, u)] % 2, jobs[ji][3], jobs[ji][4], STAGES[jobs[ji][5]][u]))
    if cfg.get('PLANOUT') is not None:
        kind = lambda j: 'conv' if j[3] is None else 'fin' if j[3] == 'fin' else j[4].func.__name__ + str(j[4].args[1] if j[4].func.__name__ == 'unit2' else j[4].args[2])
        cfg['PLANOUT'].update(ev=[(half[(ji, u)], kind(jobs[ji]), u, jobs[ji][2][u]) for _, ji, u in evs], use=use,
                              rd=[(outs[g][1], str(rd)) for g, rd, t0, n in sched for _ in range(n)])
    assert all((ts[0] < 0) == (ts[-1] < 0) for ts in when)
    carried = [(job[4], job[5]) for ts, job in zip(when, jobs) if ts[0] < 0]

    def w_copy(l):
        return pltpu.make_async_copy(w_hbm.at[l], w_ref.at[l], sem.at[l])

    def w0_copy(u):
        return pltpu.make_async_copy(w_hbm.at[0, :, u], w_ref.at[0, :, u], sem.at[L + 6 + u])

    def in_copy(t, slot):
        return pltpu.make_async_copy(x_hbm.at[pl.ds(pl.multiple_of(t * TM, 32), TM)], xn2_ref.at[slot], sem.at[L + slot])

    def out_copy(t, slot, part):
        r0, nr = ((0, 2 * Mh), (2 * Mh, Mh), (3 * Mh, Mh), (0, TM))[part]
        return pltpu.make_async_copy(o2_ref.at[slot, pl.ds(r0, nr)],
                                     o_hbm.at[pl.ds(pl.multiple_of(t * TM + r0, 32), nr)],
                                     sem.at[L + 4 + slot])

    xr_in = pltpu.make_async_copy(x_hbm.at[pl.ds(NMAIN * TM, R0)], xr_ref, sem.at[L + 2])
    xr_out = pltpu.make_async_copy(xr_ref, o_hbm.at[pl.ds(NMAIN * TM, R0)], sem.at[L + 2])
    b_in = pltpu.make_async_copy(b_hbm, b_ref, sem.at[L + 3])

    def turn(tile):
        slot = tile % 2
        pl.when(tile + 2 < NMAIN)(lambda: in_copy(tile + 2, slot).start())
        pl.when(tile > 1)(lambda: out_copy(tile - 2, slot, 3).wait())
        pl.when(tile + 1 < NMAIN)(lambda: in_copy(tile + 1, 1 - slot).wait())

    def prologue():
        b_in.start()
        for u in range(8):
            w0_copy(u).start()
        xr_in.start()
        in_copy(0, 0).start()
        for l in range(1, L):
            w_copy(l).start()
        in_copy(1, 1).start()
        b_in.wait()
        for l in range(L):
            bf_ref[l] = b_ref[l:l + 1, :].astype(f32)

        def bias_tiles(l, carry):
            b = jnp.broadcast_to(bf_ref[l] + (l == 0).astype(f32), (8, D))
            for u, site in enumerate(BIAS):
                terms = [b[:, key * 128:(key + 1) * 128] * cf for key, cf in sorted(bias_coefs(*site).items()) if cf != 0.0]
                bt_ref[l, u] = functools.reduce(lambda x, y: x + y, terms)
            return carry
        jax.lax.fori_loop(0, L, bias_tiles, 0)
        if cfg.get('FAST'):
            return

        def slab(u, carry):
            w0_copy(u).wait()
            zero = jax.lax.shift_right_logical(u, 12)
            prep(0, u, iter(lambda: None, 0), zero, kb0)
            return zero
        zero = jax.lax.fori_loop(0, cfg['NSLAB'], slab, 0)

        def plain(l, xbf, x0f, x, na, free, never, j0=0, j1=D // 128):
            passes = []
            for jt in range(j0, j1):
                cols = slice(jt * 128, (jt + 1) * 128)
                ya = _dot(xbf[:, :D // 2], w_ref[l, 0:4, :, :, cols].reshape(D // 2, 128)) + bf_ref[l, :, cols]
                passes += [ya, _dot(xbf[:, D // 2:], w_ref[l, 4:8, :, :, cols].reshape(D // 2, 128)) + ya]
            xp_ref[0, :, j0 * 128:j1 * 128] = x0f * jnp.concatenate(passes[1::2], axis=1) + x
            for u in range(na):
                f_ = (u - free) * len(passes) * (R0 // 8) // (na - free)
                if cfg['PPH'] is not None:
                    f_ = f_ // 2 * 2 + cfg['PPH']
                ps, rr = divmod(f_, R0 // 8)
                yield None if u < free else (never, passes[ps][rr * 8:rr * 8 + 8, :])

        for u in range(cfg['NSLAB'], 8):
            w0_copy(u).wait()
        xr_in.wait()
        never = jnp.broadcast_to(zero, (8, 128)) != 0
        jm = cfg['JM']
        x0f = xr_ref[:, :jm * 128].astype(f32)
        xp_ref[1, :, :jm * 128] = x0f
        anchors = plain(0, xr_ref[...], x0f, x0f, (8 - cfg['NSLAB']) * (28 + 4 * cfg['LANC'] + len(prods3)), cfg['AFREE'], never, 0, jm)
        for u in range(cfg['NSLAB'], 8):
            prep(0, u, anchors, zero, (kb0, kb1)[u % 2])
        in_copy(0, 0).wait()
        x0f = xr_ref[:, jm * 128:].astype(f32)
        xp_ref[1, :, jm * 128:] = x0f
        units = [(R, C, r) for R in range(4) for C in range(4) for r in range(0, Mh, 32)]
        anchors = plain(0, xr_ref[...], x0f, x0f, len(units) + sum(len(STAGES[n]) for _, n in carried) + 2, 4, never, jm)
        for R, C, r in units[:len(units) // 2]:
            conv(xn2_ref.at[0], zero, R, C, r, min(32, Mh - r), next(anchors))
        for fn, n in carried:
            st8 = {}
            for group in STAGES[n]:
                anchor = next(anchors)
                fn(st8, group, zero, jax.lax.shift_right_logical(zero, 1), anchor)
        for R, C, r in units[len(units) // 2:]:
            conv(xn2_ref.at[0], zero, R, C, r, min(32, Mh - r), next(anchors))

        def layer(l, carry):
            w_copy(l).wait()
            zero = jax.lax.shift_right_logical(l, 12)
            x = xp_ref[0]
            anchors = plain(l, x.astype(bf16), xp_ref[1], x, 8 * (28 + 4 * cfg['LANC'] + len(prods3)), cfg['AFREE'],
                            jnp.broadcast_to(zero, (8, 128)) != 0)
            for u in range(8):
                prep(l, u, anchors, zero, (kb0, kb1)[u % 2])
            return carry

        jax.lax.fori_loop(1, L, layer, 0)
        xr_ref[...] = xp_ref[0].astype(bf16)
        xr_out.start()

    def main(tile, carry):
        zs, za = jax.lax.shift_right_logical(tile, 12), jax.lax.shift_right_logical(tile, 13)
        never = jnp.broadcast_to(zs, (8, 128)) != 0
        slot = tile % 2
        xn_ref = xn2_ref.at[1 - slot]
        o_ref = o2_ref.at[slot]
        def rows(h, r0):
            if isinstance(h, tuple):
                return slice(r0 + h[0], r0 + h[0] + h[1])
            return slice(r0, r0 + Mh) if h is None else slice(r0 + h * Mq, r0 + (h + 1) * Mq)

        def ld(loc, h=None, z=0):
            return loc[0][(z,) + loc[1] + (rows(h, loc[2]),)]

        def st(loc, v, h=None):
            loc[0][(za if h == 1 and not loc[1] and cfg['ZB'] else zs,) + loc[1] + (rows(h, loc[2]),)] = v

        def by_half(v, h, fn):
            if isinstance(h, tuple):
                h = h[0] // Mq
            return fn(v, h) if h is not None else jnp.concatenate([fn(v[:Mq], 0), fn(v[Mq:], 1)], axis=0)

        def gather(ref, idx, n, pos):
            if cfg['NOBC']:
                return ref[idx + (slice(0, n), slice(16 * pos, 16 * pos + 16))].reshape(16 * n, 128)
            return ref.bitcast(u32)[idx + (slice(0, n), slice(8 * pos, 8 * pos + 8))].reshape(8 * n, 128)

        as_bf16 = lambda v: v if cfg['NOBC'] else pltpu.bitcast(v, bf16)

        def lhs2(p, q):
            ref, u = s2loc(p)
            return as_bf16(jnp.concatenate([gather(ref, (0, u, k), NC, q2[p].index(q)) for k in range(2)], axis=1))

        def rhs2(l, p, q, n):
            return as_bf16(gather(t2[p], (l, n), 16, q2[p].index(q)))

        def dot3(l, p, q, r):
            qs = next(qs for qs in PAIRS if q in qs)
            return _dot(as_bf16(gather(s3[(p, qs)], (0, qs.index(q)), NQ, ORD.index(r))),
                        as_bf16(gather(t3_ref, (l, prods3.index((p, q))), 8, ORD.index(r))))

        def add_bias(v, l, site, h):
            def one(x, hh):
                b = bt_ref[l, BIAS.index(site + (hh,))]
                return (x.reshape(x.shape[0] // 8, 8, 128) + b).reshape(x.shape)
            return by_half(v, h, one)

        wait = {}
        def outer_act(l, p, i, j, n, d, h, part=None):
            bt, stores, finals = OACT[p]
            if part == 'raw':
                stores, finals = stores[:1], []
            if part == 'rest':
                bt, stores = [], stores[1:]
            if p == 6 and part is None and (i, j) != B12 and (h, n) != (0, 1):
                stores = []
            if bt:
                d = add_bias(d, l, (p, False, i, j, n), h)
            cache = {'d': d}
            def comb(terms):
                for _, src in terms:
                    if isinstance(src, str) and src not in cache:
                        cache[src] = ld(oloc(src, i, j, n), h)
                v = lincomb([(s, cache[src]) for s, src in terms if isinstance(src, str)])
                for _, src in terms:
                    if not isinstance(src, str):
                        v = add_bias(v, l, (p, True, i, j, n), h)
                return v
            fin = [(IJ, comb(terms)) for IJ, terms in finals]
            for name, v in [(name, comb(terms)) for name, terms in stores]:
                st(oloc(name, i, j, n), v, h)
            for (I, J), y in fin:
                R, C = 2 * I + i, 2 * J + j
                xn = ld(x0loc(R, C, n), h) * y
                if l > 0:
                    xn = xn + ld(xloc(l, R, C, n), h)
                if l < L - 1:
                    st(xloc(l + 1, R, C, n), xn, h)
                else:
                    xn = by_half(xn, h, lambda x, hh: x if scale(R, C, hh, n) == 1.0 else x * (1.0 / scale(R, C, hh, n)))
                    c0 = phys(C, n) * 128
                    if i == 0:
                        o_ref[rows(h, R * Mh), c0:c0 + 128] = xn.astype(bf16)
                    elif j == 1:
                        wait[(R, J)] = xn
                    else:
                        o_ref[rows(h, R * Mh), c0:c0 + 256] = jnp.concatenate([xn, wait.pop((R, J))], axis=1).astype(bf16)

        def inner_act(g, l, p, kind, n, h, P, Q, part=None):
            vloc = oloc(raw_slot(p), 0, 1, n) if raw_slot(p) else iloc(g, 'v', n)
            if kind == '35':
                st(iloc(g, 's', n), Q + ld(iloc(g, 'm1', n), h), h)
                if not raw_slot(p):
                    st(vloc, P, h)
                outer_act(l, p, 0, 1, n, P, h, part)
            elif kind == '47':
                st(iloc(g, 'u', n), Q + ld(vloc, h), h)
                outer_act(l, p, 0, 0, n, P + ld(iloc(g, 's', n), h), h, part)
            else:
                outer_act(l, p, 1, 1, n, ld(iloc(g, 's', n), h) - Q, h, part)
                outer_act(l, p, 1, 0, n, P + ld(iloc(g, 'u', n), h), h, part)

        def issue(l, p, rd):
            kind, n = rd
            if kind == 'x':
                return [dot3(l, p, q, 1) for q in (3, 5, 4, 7)]
            if kind == 'y':
                return [dot3(l, pp, q, 1) for pp in (p, SEL3[SEL3.index(p) + 1]) for q in (2, 6)]
            if isinstance(n, str):
                if cfg['MO']:
                    d = [dot3(l, p, int(q), int(r)) for q in kind for r in n]
                    return [d[0], d[2], d[1], d[3]]
                return [dot3(l, p, int(q), int(r)) for r in n for q in kind]
            if cfg['GR']:
                ops = [(lhs2(p, 1),) * 2, (rhs2(l, p, 1, 0), rhs2(l, p, 1, 1))] if kind == '1' else [
                    [lhs2(p, int(q)) for q in kind], [rhs2(l, p, int(q), n) for q in kind]]
                d = [_dot(a[:, k * 128:(k + 1) * 128], b[k * 128:(k + 1) * 128]) for a, b in zip(*ops) for k in range(2)]
                return [d[0] + d[1], d[2] + d[3], d[cfg['GR'] - 1]]
            if kind == '1':
                lhs = lhs2(p, 1)
                return [_dot(lhs, rhs2(l, p, 1, 0)), _dot(lhs, rhs2(l, p, 1, 1))]
            return [_dot(lhs2(p, int(q)), rhs2(l, p, int(q), n)) for q in kind]

        def consume(g, l, p, rd, res):
            kind, n = rd
            if n == '1':
                for u, where in enumerate((('35', False), ('47', False)) if kind == 'x' else (('26', False), ('26', True))):
                    for al in range(2):
                        st(jloc(where[0], '1', al, where[1]), res[2 * u + al], 0)
            elif isinstance(n, str):
                sm = [res[al] + res[2 + al] for al in range(2)]
                df = [res[al] - res[2 + al] for al in range(2)]
                J = lambda name, al: ld(jloc(kind, name, al, name == '1' and kind == '26' and p in SEL3[1::2]), 0)
                part = 'raw' if deferred(l, p, rd) else None
                done = lambda h, nn, m: inner_act(g, l, p, kind, nn, h, m[0] + m[1], m[0] - m[1], part)
                O, I = (lambda i, j: oloc(raw_slot(p), i, j, 1)), (lambda name: iloc(g, name, 1))
                rec = lambda al: [(s, ld(loc, 0, za if cfg['ZB'] else 0)) for s, loc in {
                    '35': [[(1, O(0, 1))], [(1, I('s')), (-1, I('m1'))]],
                    '47': [[(1, O(0, 0)), (-1, I('s'))], [(1, I('u')), (-1, O(0, 1))]],
                    '26': [[(1, O(1, 0)), (-1, I('u'))], [(1, I('s')), (-1, O(1, 1))]]}[kind][al]]
                if n == '35':
                    for al in range(2):
                        st(jloc(kind, 's', al), df[al] + J('1', al), 0)
                    done(0, 1, sm)
                elif n == '47':
                    if cfg['HY'] == 1:
                        for al in range(2):
                            st(jloc(kind, 'u', al), df[al], 0)
                    else:
                        for al, v in enumerate((df[0] + df[1], df[0] - df[1])):
                            st(jloc(kind, 'u', al), lincomb([(1, v)] + rec(al)), 0)
                    done(0, 0, [sm[al] + J('s', al) for al in range(2)])
                else:
                    if cfg['HY'] == 1:
                        m = [sm[al] + J('u', al) for al in range(2)]
                        P, Q = lincomb([(1, m[0] + m[1])] + rec(0)), lincomb([(1, m[0] - m[1])] + rec(1))
                    else:
                        P, Q = (sm[0] + sm[1]) + J('u', 0), (sm[0] - sm[1]) + J('u', 1)
                    done(1, 1, [J('s', al) - df[al] for al in range(2)])
                    inner_act(g, l, p, kind, 0, 1, P, Q, part)
            elif kind == '1':
                st(iloc(g, 'm1', 0), res[0])
                st(iloc(g, 'm1', 1), res[1])
            else:
                inner_act(g, l, p, kind, n, None, res[0] + res[1], res[0] - res[1])

        state = {}
        for g, rd, t0, n in sched:
            l, p = outs[g]
            if t0 == start[G - 1]:
                out_copy(tile, slot, 0).start()
            if t0 + n == T:
                out_copy(tile, slot, 1).start()
            res = issue(l, p, rd)
            if cfg['EO']:
                consume(g, l, p, rd, res)
            for t in range(t0, t0 + n):
                for ph, l2, fn, group in plan.get(t, []):
                    gr = 16 * (t - t0) + 8 * ph
                    if cfg['GF']:
                        gr = 16 * (t - t0) + 8 * (1 - ph)
                    gs = cfg['GS']
                    gate = res[2 if len(res) == 3 else cfg['GM']][gr:gr + 8, :]
                    if cfg['GADD'] and isinstance(rd[1], str) and rd[1] != '1':
                        gate = gate + res[2 + gs % 2][gr:gr + 8, :]
                    elif gs == 2 and rd[0] != '1' and rd[1] != '1':
                        gate = gate + res[1][gr:gr + 8, :]
                    if l2 == 'fin':
                        for i, j, nf, r0 in fn[2]:
                            d = ld(oloc(raw_slot(fn[1]), i, j, nf), (r0, 16))
                            d = tie(tie(d, (never, gate)), (never, gate), 8)
                            outer_act(fn[0], fn[1], i, j, nf, d, (r0, 16), 'rest')
                    elif l2 is None:
                        conv(xn_ref, zs, *fn, min(32, Mh - fn[2]), (never, gate))
                    else:
                        fn(state.setdefault(id(fn), {}), group, zs, za, (never, gate))
            if not cfg['EO']:
                consume(g, l, p, rd, res)
        out_copy(tile, slot, 2).start()
        turn(tile + 1)
        return carry

    prologue()
    in_copy(2, 0).start()
    in_copy(1, 1).wait()
    if not cfg.get('NOMAIN'):
        jax.lax.fori_loop(0, NMAIN, main, 0)
    else:
        for p_ in range(1, 8):
            for l_ in range(L):
                o2_ref[0, 0:16, 0:128] = t2[p_][l_, 0, pl.program_id(0) if False else 3, 0:16] + t3_ref[l_, p_, 2, 0:16]
    xr_out.wait()
    out_copy(NMAIN - 1, (NMAIN - 1) % 2, 3).wait()


DEFAULT = dict(SEL=(3, 5, 4, 7, 2, 6), SEL3=(3, 5, 4, 7), XC={B12: 5, B11: 1, B22: 7, B21: 2}, AFREE=2, NOBC=0, GAM=1.0, UMIN=0, LANC=1, KD=1, PO=PREP_ORDER, PT=0, MAT=4, FOLD=1, MO=1, GR=2, NS=(2, 3, 3, 4, 3), NL=1, GE=6, GM=0, DBL=1, GS=0, GF=0, EO=0, KP=16, PPH=None, ZB=0, HY=1, HOLD=0, PORT=0.9, PS=0, NSLAB=6, JM=3, XP=40, XO=16, DEFER={5: [('26', '26'), ('47', '26')], 7: [('26', '26'), ('47', '26')], 2: [('35', '26'), ('47', '26')],
                      6: [('35', '26'), ('47', '26')]}, DEFL={}, EW=12, KW=(1,) * 5, CM=(1,) * 7, SEEDS=(), SEG=32, PJ=20, QO=0, TIEL=2, GADD=0, TF=0, T8=0, TAIL=6,
               CS=0.5, CL=0.3, UL=0.8, CAP=0.95, FR=((1.,), (.4, .6), (.35, .37, .28), (.16, .26, .31, .27),
                   (.35, .29, .08, .28), (.16, .26, .26, .05, .27)))


def build(TM=640, **kw):
    def f(x0, ws, bs):
        B, D = x0.shape
        L = ws.shape[0]
        cfg = dict(DEFAULT, **kw)
        Mh = TM // 4
        MP = Mh + 32
        nmain = (B - 1) // TM
        R0 = B - nmain * TM
        pairs3, q2 = layout(cfg)
        n3 = sum(2 * len(v) for v in pairs3.values())
        pad = lambda n: n + (2 - n) % 4
        V = pltpu.VMEM
        half = V((1, MP, 128), f32)
        XP = Mh + cfg['XP']
        scratch = ([V((1, 2, 2, 2, XP, 128), f32)] * 4 + [V((1, 2, 4, 2, XP, 128), f32)] * 7 + [half] * (16 + 64 + 26)
                   + [V((1, 1 + (p == 2 and q2[2] == q2[6]), 2, pad(Mh // 16), 16 * len(q2[p]), 128), bf16) for p in range(1, 8)]
                   + [V((1, 2, pad(Mh // 32), 112, 128), bf16)] * (n3 // 2)
                   + [V((L, 2, 16, 16 * len(q2[p]), 128), bf16) for p in range(1, 8)]
                   + [V((L, n3, 8, 112, 128), bf16), V((1, 4, 16 * n3 + cfg['KP'], 128), f32), V((1, 4, 16 * n3 + cfg['KP'], 128), f32),
                      V((L, len(BIAS), 8, 128), f32), V((8, 1, D), f32), V((2, TM, D), bf16), V((2, TM, D), bf16), V((L, 8, 8, 16, D), bf16),
                      V((R0, D), bf16), V((2, R0, D), f32), V((L, D), bf16), pltpu.SemaphoreType.DMA((L + 14,))])
        anyspec = pl.BlockSpec(memory_space=pl.ANY)
        return pl.pallas_call(
            functools.partial(_kernel, L=L, TM=TM, R0=R0, NMAIN=nmain, D=D, cfg=cfg),
            in_specs=[anyspec, anyspec, anyspec],
            out_specs=anyspec,
            out_shape=jax.ShapeDtypeStruct((B, D), x0.dtype),
            scratch_shapes=scratch,
            compiler_params=pltpu.CompilerParams(
                vmem_limit_bytes=120 * 1024 * 1024,
                internal_scratch_in_bytes=65536,
                disable_bounds_checks=True,
            ),
        )(x0, ws.reshape(L, 8, 8, 16, D), bs)
    return f


@jax.jit
def pallas_standalone__dcn_v2_cross__recsys_kernel(x0, ws, bs):
    return build(TM=640)(x0, ws, bs)
```

```python
import functools

import jax
import jax.numpy as jnp
import numpy as np
import jax.experimental.pallas as pl
import jax.experimental.pallas.tpu as pltpu

f32 = jnp.float32
bf16 = jnp.bfloat16
u32 = jnp.uint32

B11, B12, B21, B22 = (0, 0), (0, 1), (1, 0), (1, 1)
LA = {1: [(B11, 1), (B22, 1)], 2: [(B11, 1), (B12, 1), (B21, 1), (B22, 1)], 3: [(B11, 1), (B12, -1)],
      4: [(B12, 1), (B22, 1)], 5: [(B11, 1), (B12, 1)], 6: [(B12, 1), (B11, -1), (B21, 1), (B22, -1)],
      7: [(B12, 1), (B22, -1)]}
PAIRS = ((5, 3), (4, 7), (2, 6))
ORD = (3, 5, 4, 7, 1, 2, 6)
D2 = (1.0, 2.0)
BF = {1: 1.0, 2: 0.5, 3: 0.5, 4: 0.5, 5: 0.5, 6: 0.5, 7: 0.5}
OUTER = (3, 5, 1, 4, 7, 2, 6)
OACT = {
    3: ([], [('M3', [(1, 'd')])], []),
    5: ([], [('M5', [(1, 'd')])], [(B12, [(1, 'd'), (1, 'M3')])]),
    1: ([], [('S', [(1, 'd'), (1, 'M3'), (-1, 'M5')])], []),
    4: ([], [('M4', [(1, 'd')])], []),
    7: ([], [('M7', [(1, 'd')])], [(B11, [(1, 'd'), (1, 'S'), (1, 'M4')])]),
    2: ([], [('M2', [(1, 'd')]), ('U', [(1, 'd'), (1, 'M4'), (-1, 'M7'), (1, 'M3'), (1, 'M5')])], []),
    6: ([], [('M6', [(1, 'd')])], [(B22, [(1, 'd'), (1, 'S'), (-1, 'M2')]), (B21, [(1, 'd'), (1, 'U')])]),
}
PC = {1: (1, 0, 0, 1), 2: (0, 0, 1, -1), 3: (1, 1, 1, 1), 4: (1, 0, 1, 0), 5: (-1, 1, 1, -1), 6: (0, 0, 1, 1),
      7: (1, 0, -1, 0)}
OSL = {'M3': 0, 'M5': 1, 'S': 2, 'M4': 3, 'M7': 4, 'M2': 6, 'U': 5, 'M6': 7}
ISL = {'m1': 0, 's': 1, 'v': 2, 'u': 3}
STAGES = {1: [(B11, B12, B21, B22)], 2: [(B11, B12), (B21, B22)], 3: [(B11, B12), (B22,), (B21,)],
          4: [(B11,), (B12,), (B22,), (B21,)], 5: [(B11, B12), (B22, 'hold'), ('l1',), (B21,)],
          6: [(B11,), (B12,), (B22, 'hold'), ('l1',), (B21,)]}
PREP_ORDER = (2, 6, 3, 5, 1, 4, 7)
GAMMA = 0.125
LAG = 8


def _dot(a, b):
    return jnp.dot(a, b, preferred_element_type=f32)


def scale(R, C, h, k):
    return D2[R // 2] * D2[R % 2] * D2[h] / (D2[C // 2] * D2[C % 2] * D2[k])


def phys(C, k):
    return 4 * (C // 2) + 2 * k + C % 2


def b_ops(b11, b12, b21, b22):
    r1 = b11 + b22
    g = b12 + b21
    return {1: r1, 2: b11 - b12, 3: b12 - b22, 4: g - r1, 5: b12 + b22, 6: b11 + b12, 7: g + r1}


def lincomb(terms):
    assert terms[0][0] == 1
    acc = terms[0][1]
    for s, v in terms[1:]:
        acc = acc + v if s == 1 else acc - v
    return acc


def raw_slot(p):
    return next((name for name, terms in OACT[p][1] if terms == [(1, 'd')]), None)


def round_usage(p, rd, first, last, defer, hy, tel):
    bt, stores, finals = OACT[p]
    alu = bool(bt) + sum(len(t) - 1 for _, t in stores) + sum(len(t) + (not first) + 2 * last for _, t in finals)
    nst = len(stores) + len(finals)
    nld = len({x for _, t in stores + finals for _, x in t if isinstance(x, str) and x != 'd'}) + len(finals) * (2 - first)
    kind, n = rd
    if last and kind == '26':
        alu, nst = alu - 0.7 * len(finals), nst - 0.5 * len(finals)
    if defer:
        alu, nst, nld = bool(bt), 1, 0
    elif p == 6 and kind != '35' and n != '35':
        nst -= 1
    if isinstance(n, str):
        e = kind == '47'
        if kind == '26':
            a, st, ld, m = {'35': (10, 2, 9, 2), '47': (10, 2, 9, 2) if hy == 1 else (16, 2, 13, 2), '26': (20, 0, 17, 4) if hy == 1 else (16, 0, 13, 4)}[n]
        else:
            a, st, ld, m = {'1': (0, 4, 5, 0), '35': (9 + e, 3, 8 + e, 1),
                            '47': (9 + e, 3, 8 + e, 1) if hy == 1 else (14 + 2 * e, 3, 11 + 2 * e, 1),
                            '26': (17 + 3 * e, 2, 14 + 3 * e, 2) if hy == 1 else (14 + 2 * e, 2, 11 + 2 * e, 2)}[n]
    else:
        a, st, ld, m = {'1': (2, 2, 4, 0), '35': (5, 2 - bool(raw_slot(p)), 5, 1), '47': (6, 1, 6, 1),
                        '26': (6, 0, 6, 2)}[kind]
    if tel and n == '26':
        a -= 1 + (kind != '35')
    return a + m * alu, st + m * nst, ld + m * nld


def yds(groups, cap):
    n = len(cap)
    speed, cls, gcls = [0.0] * n, [-1] * n, {}
    todo = list(groups)
    while todo:
        pre = [0.0]
        for t in range(n):
            pre.append(pre[-1] + (cap[t] if cls[t] < 0 else 0.0))
        best = None
        for a in sorted({g[0] for g in todo}):
            w = 0.0
            for g in sorted((g for g in todo if g[0] >= a), key=lambda g: g[1]):
                w += g[2]
                d = w / max(pre[g[1] + 1] - pre[a], 1e-9)
                if best is None or d > best[0]:
                    best = (d, a, g[1])
        d, a, b = best
        for t in range(a, b + 1):
            if cls[t] < 0:
                speed[t], cls[t] = d, len(gcls)
        gcls.update({g[:2]: len(gcls) for g in todo if g[0] >= a and g[1] <= b})
        todo = [g for g in todo if not (g[0] >= a and g[1] <= b)]
    return speed, cls, gcls


def spread_jobs(jobs, cap, tail, vcap=None):
    T = len(cap)
    cap3 = cap * 3
    all3 = [(j[0] + k * T, j[1] + k * T, ji, k) for k in range(3) for ji, j in enumerate(jobs) if j[0] + k * T >= 0]
    pend = {}
    for j in sorted(all3, key=lambda j: (j[1], j[3], j[2])):
        pend.setdefault(j[:2], []).append(j)
    speed, cls, gcls = yds([w + (sum(sum(jobs[j[2]][2]) for j in q),) for w, q in pend.items()], cap3)
    when = [[] for _ in jobs]
    debt, cur, done, vdebt = 0.0, None, 0, 0.0
    cum = [0.0]
    for t in range(3 * T):
        cum.append(cum[-1] + speed[t] * cap3[t])
    left = {w: sum(sum(jobs[j[2]][2]) for j in q) for w, q in pend.items()}
    def fits(j, t):
        need = max(debt, 0.0) + sum(jobs[j[2]][2]) + 1.0
        for w in pend:
            if w[1] >= j[1]:
                return True
            if left[w] > 1e-9:
                need += left[w]
                if need > cum[w[1] + 1] - cum[t]:
                    return False
        return True
    for t in range(3 * T):
        if t % T == 0:
            debt, vdebt = min(debt, 0.0), -0.5
        while True:
            j = cur
            if j is None:
                rdy = [q[0] for w, q in pend.items() if q and w[0] <= t and (gcls[w] == cls[t] or w[1] <= t)]
                if not rdy:
                    debt = max(debt, 0.0)
                    break
                j = rdy[0]
                if vcap is not None and j[1] > t:
                    ok = [x for x in rdy if x is j or fits(x, t)]
                    j = (min if vdebt > 0 else max)(ok, key=lambda x: jobs[x[2]][3])
                nst = len(jobs[j[2]][2])
                if nst > 1 and j[1] > t and (t + tail + 2 * nst) // T != t // T:
                    break
            must = j[1] <= t or (cur is not None and (t + tail + 1) // T != t // T)
            if not must and (cap3[t] == 0.0 or debt > 0.5 * speed[t] * cap3[t]):
                break
            if cur is None:
                pend[j[:2]].pop(0)
                left[j[:2]] -= sum(jobs[j[2]][2])
                cur, done = j, 0
            debt += jobs[j[2]][2][done]
            vdebt += jobs[j[2]][2][done] * jobs[j[2]][3]
            if j[3] == 1:
                when[j[2]].append(t - T)
            done += 1
            if done == len(jobs[j[2]][2]):
                cur = None
        debt -= speed[t] * cap3[t]
        if vcap is not None:
            vdebt = min(max(vdebt - vcap[t % T], -0.5), 1.0)
    return when


def layout(cfg):
    sel, sel3 = cfg['SEL'], cfg['SEL3']
    pairs3 = {p: [qs for qs in PAIRS if p in sel3 or (p in sel and qs != (2, 6))] for p in range(1, 8)}
    q2 = {p: [q for q in ORD if not any(q in qs for qs in pairs3[p])] for p in range(1, 8)}
    return pairs3, q2


def _kernel(x_hbm, w_hbm, b_hbm, o_hbm, *scratch, L, TM, R0, NMAIN, D, cfg):
    H, Mh, Mq = D // 4, TM // 4, TM // 8
    NC, NQ = Mh // 16, Mq // 16
    MP = Mh + 32
    SEL, SEL3 = cfg['SEL'], cfg['SEL3']
    pairs3, q2 = layout(cfg)
    prods3 = [(p, q) for p in SEL for qs in pairs3[p] for q in qs]
    assert NMAIN >= 3 and H == 256 and L % 2 == 0 and Mq % 16 == 0 and all(raw_slot(p) for p in SEL)
    it = iter(scratch)
    take = lambda n: [next(it) for _ in range(n)]
    x0b, xb, ib, ob, jb = take(4), take(7), take(16), take(64), take(26)
    joint = q2[2] == q2[6]
    MAT = cfg['MAT'] and joint and 2 in SEL
    s2 = dict(zip(range(1, 8), take(7)))
    s3 = {(p, qs): next(it) for p in SEL for qs in pairs3[p]}
    t2 = dict(zip(range(1, 8), take(7)))
    t3_ref, kb0, kb1, bt_ref, bf_ref, xn2_ref, o2_ref, w_ref, xr_ref, xp_ref, b_ref, sem = it

    xset = lambda l: 6 if l == 'O' else 4 if l == 0 else (l % 2) * 2
    xoff = lambda I, J: cfg['XO'] * ((I + J) % 2)
    xloc = lambda l, R, C, k: (xb[xset(l) + R // 2], (R % 2, C, k), xoff(R // 2, C // 2))
    x0loc = lambda R, C, k: (x0b[(R // 2) * 2 + C // 2], (R % 2, C % 2, k), 8 + xoff(R // 2, C // 2))
    iloc = lambda g, name, n: (ib[((g % 2) * 4 + ISL[name]) * 2 + n], (), 8 * ISL[name])
    oloc = lambda name, i, j, n: (ob[(OSL[name] * 4 + i * 2 + j) * 2 + n], (), 8 * ((OSL[name] + 2 * j) % 4))

    def jloc(kind, name, al, second=False):
        i = 24 + al if second else (('35', '47', '26').index(kind) * 4 + ('1', 's', 'u', 'v').index(name)) * 2 + al
        return jb[i], (), 8 * ((i + i // 2) % 4)

    def s2loc(p):
        return (s2[2], (2, 6).index(p)) if p in (2, 6) and joint and 2 not in SEL3 else (s2[p], 0)

    def tie(v, anchor, r=0):
        if anchor is None:
            return v
        return jnp.concatenate([v[:r]] * (r > 0) + [jax.lax.select(anchor[0], anchor[1], v[r:r + 8])] + [v[r + 8:]] * (r + 8 < v.shape[0]), axis=0)

    def consts(anchor, ss, reps):
        one = {s: jnp.full((8, 128), s, f32) for s in set(ss)}
        if anchor is not None:
            one = {s: jax.lax.select(anchor[0], anchor[1], v) for s, v in one.items()}
        return jnp.concatenate([one[s] for s in ss for _ in range(reps)], axis=0)

    def conv(src, zs, R, Q, r, nr, anchor=None):
        v = src[R * Mh + r:R * Mh + r + nr, Q * H:(Q + 1) * H].astype(f32)
        for j in range(2):
            C, k = 2 * (Q // 2) + j, Q % 2
            buf, idx, off = xloc(0, R, C, k)
            sv = consts(anchor, [scale(R, C, (r + u) // Mq, k) for u in range(0, nr, 16)], 2)
            buf[(zs,) + idx + (slice(off + r, off + r + nr),)] = v[:, j * 128:(j + 1) * 128] * sv

    cnt = {}
    def block_sum(l, terms, ii, jj, kk, r, save, zs, za, anchor, late=None, notie=False):
        rng = lambda t: slice(t[0], t[-1] + 1)
        keys = [(i, j, k) for i in ii for j in jj for k in kk]
        vals = []
        for u, ((I, J), s) in enumerate(terms):
            ref, r0 = xb[xset(l) + I], xoff(I, J) + r
            v = ref[za if u == 0 else 0, rng(ii), 2 * J + jj[0]:2 * J + jj[-1] + 1, rng(kk), r0:r0 + 16, :]
            if (I, J) in save:
                sv = consts(anchor, [GAMMA / scale(2 * I + i, 2 * J + j, r // Mq, k) for i, j, k in keys], 2)
                x0b[I * 2 + J][zs, rng(ii), rng(jj), rng(kk), r0 + 8:r0 + 24, :] = v * sv.reshape(v.shape)
            v = v.reshape(16 * len(keys), 128)
            if u == 0 and late is not None and anchor is not None:
                cnt[xset(l)] = cnt.get(xset(l), -1) + 1
                if cnt[xset(l)] % cfg['GE'] == 0:
                    ref[0, 0, 0, 0, Mh + 24:Mh + 32, :] = anchor[1]
                at = 16 * keys.index(late)
                top = v[at:at + 8] if cfg['NL'] else ref[za, late[0], 2 * J + late[1], late[2], r0:r0 + 8, :]
                if cfg['TIEL'] == 2:
                    top = jax.lax.select(anchor[0], anchor[1], top)
                v = jnp.concatenate([v[:at]] * (at > 0) + [top, v[at + 8:]], axis=0)
            vals.append((s, v))
        v = lincomb(vals)
        if cfg['TIEL'] == 3 and late is not None and not notie:
            v = tie(v, anchor, 16 * keys.index(late))
        return v

    def release(qs, store, st8, anchor):
        v = st8['l1']
        if anchor is not None:
            n = v.shape[0]
            top = jax.lax.select(jnp.broadcast_to(anchor[0], (n, 8, 128)), jnp.broadcast_to(anchor[1], (n, 8, 128)), v[:, :8])
            v = jnp.concatenate([top, v[:, 8:]], axis=1)
        r0 = 16 * qs.index(1)
        store(slice(r0, r0 + 16), v.astype(bf16))

    def finish(e, f, group, qs, store, st8, anchor, hold=False, keep=None):
        a = e[None] if f is None else jnp.concatenate([e + f, e - f], axis=0).reshape(2, e.shape[0], 128)
        for u, b in enumerate(group):
            st8[b] = a if len(group) == 1 else a[:, 16 * u:16 * u + 16]
            if keep:
                keep(b, st8[b])
        ops = {}
        if B12 in group and 3 in qs:
            ops[3], ops[5] = st8[B11] - st8[B12], st8[B11] + st8[B12]
        if B22 in group:
            if 4 in qs:
                ops[4], ops[7] = st8[B12] + st8[B22], st8[B12] - st8[B22]
            ops[1] = st8['l1'] = st8[B11] + st8[B22]
        if B21 in group:
            g = st8[B12] + st8[B21]
            ops[2], ops[6] = g + st8['l1'], g - st8['l1']
        now = [q for q in qs if q in ops and not (hold and q == 1)]
        if now:
            r0 = 16 * qs.index(now[0])
            store(slice(r0, r0 + 16 * len(now)), jnp.concatenate([ops[q] for q in now], axis=1).astype(bf16))

    def unit2(l, ps, c, k, save, st8, group, zs, za, anchor):
        def store(rows, v):
            s2[ps[0]][zs, :, k, c, rows, :] = v
        if group == ('l1',):
            return release(q2[ps[0]], store, st8, anchor)
        hold, group = 'hold' in group, tuple(b for b in group if b != 'hold')
        ii, jj = sorted({b[0] for b in group}), sorted({b[1] for b in group})
        bs = lambda terms, late: block_sum(l, terms, ii, jj, [k], 16 * c, save, zs, za, anchor, late, len(ps) == 2 and 2 in SEL3)
        if cfg['MRG'] and ps == (1,):
            e = bs([(B12, 1), (B21, 1)], None)
            f = bs(LA[1], (ii[0], jj[-1], k))
            for J, v in enumerate((e + f, e - f)):
                r0 = xoff(0, J) + 16 * c
                xb[6][zs, ii[0]:ii[-1] + 1, 2 * J + jj[0]:2 * J + jj[-1] + 1, k, r0:r0 + 16, :] = v.reshape(len(ii), len(jj), 16, 128)
            return finish(f, None, group, q2[1], store, st8, anchor)
        f = None if len(ps) == 1 else bs([(B11, 1), (B22, 1)], None)
        e = bs(LA[ps[0]] if len(ps) == 1 else [(B12, 1), (B21, 1)], (ii[0], jj[-1], k))
        if 2 in SEL3 and f is not None:
            if anchor is not None:
                n = e.shape[0] // 8
                e = jax.lax.select(jnp.tile(anchor[0], (n, 1)), jnp.tile(anchor[1], (n, 1)), e)
            for J, v in enumerate((e + f, e - f)):
                r0 = xoff(0, J) + 16 * c
                xb[6][zs, ii[0]:ii[-1] + 1, 2 * J + jj[0]:2 * J + jj[-1] + 1, k, r0:r0 + 16, :] = v.reshape(len(ii), len(jj), 16, 128)
            return
        def keep(b, v):
            if b != B21:
                for J in range(2):
                    xb[6][zs, b[0], 2 * J + b[1], k, xoff(0, J) + 16 * c:xoff(0, J) + 16 * c + 16, :] = v[J]
        if f is None or joint:
            return finish(e, f, group, q2[ps[0]], store, st8, anchor, hold, keep if f is not None and MAT else None)
        for p, v in zip(ps, (e + f, e - f)):
            def store1(rows, w):
                s2[p][zs, :, k, c, rows, :] = w
            finish(v, None, group, q2[p], store1, st8.setdefault(p, {}), anchor)

    def unit3(l, p, qs, c, save, st8, group, zs, za, anchor):
        def store(rows, w):
            s3[(p, qs)][zs, :, c, rows, :] = w
        if group == ('l1',):
            return release(ORD, store, st8, anchor)
        hold, group = 'hold' in group, tuple(b for b in group if b != 'hold')
        for h in sorted({b[0] for b in group}):
            grp = tuple(b for b in group if b[0] == h)
            kk = [b[1] for b in grp]
            ii, jj = {(5, 3): ([0], [0, 1]), (4, 7): ([0, 1], [1]), (2, 6): ([0, 1], [0, 1])}[qs]
            src = ('O', [((0, (2, 6).index(p)), 1)]) if MAT and p in (2, 6) else (l, LA[p])
            v = block_sum(*src, ii, jj, sorted(kk), h * Mq + 16 * c, save, zs, za, anchor,
                          (0, (0 if cfg['TF'] else 1) if qs == (2, 6) else jj[0], max(kk)) if h == group[-1][0] else None)
            n = 16 * len(kk)
            piece = lambda u: v[u * n:(u + 1) * n]
            if qs == (2, 6):
                e, f = piece(1) + piece(2), piece(0) + piece(3)
                r0 = 16 * q2[p].index(1)
                s2loc(p)[0][zs, s2loc(p)[1], min(kk):max(kk) + 1, h * NQ + c, r0:r0 + 16, :] = f.reshape(len(kk), 16, 128).astype(bf16)
            else:
                e, f = piece(0), piece(1)
            finish(e, f, tuple(sorted(grp)), ORD, store, st8, anchor, hold)

    def prep(l, u, anchors, zero, kb):
        mul = lambda v, s: v if s == 1.0 else v * s
        def third(e, last):
            v = kb[0, 0:4 if last is None else 3, 16 * e:16 * e + 16, :]
            T = b_ops(v[0], tie(v[1], next(anchors)), v[2], v[3] if last is None else last)
            T[1] = T[1] * 2.0
            t3_ref[l, e, u] = jnp.concatenate([T[q] for q in ORD], axis=0).astype(bf16)
        for k in range(2):
            wide = [w_ref[l, phys(R, k), u].astype(f32) for R in range(4)]
            for n in range(2):
                la = next(anchors) if cfg['LANC'] else None
                def blk(R, C):
                    v = mul(wide[R][:, phys(C, n) * 128:(phys(C, n) + 1) * 128], scale(R, C, k, n))
                    return tie(v, la) if (R // 2, C // 2) == B12 else v
                O = {(i, j): b_ops(blk(i, j), blk(i, 2 + j), blk(2 + i, j), blk(2 + i, 2 + j)) for i, j in (B11, B12, B21, B22)}
                for p in cfg['PO']:
                    o = [mul(O[b][p], BF[p] * (0.25 if p in SEL else 0.5) / GAMMA) for b in (B11, B12, B21, B22)]
                    T = b_ops(o[0], tie(o[1], next(anchors)), o[2], o[3])
                    t2[p][l, n, k * 8 + u] = jnp.concatenate(
                        [mul(T[q], BF[q] * (4.0 if p in SEL else 2.0)) for q in q2[p]], axis=0).astype(bf16)
                    mine = [e for e, pq in enumerate(prods3) if pq[0] == p]
                    if cfg['KD'] and (k, n) == (1, 1):
                        for e in mine:
                            third(e, T[prods3[e][1]])
                    elif mine:
                        kb[zero, k * 2 + n, 16 * mine[0]:16 * mine[-1] + 16, :] = jnp.concatenate(
                            [T[prods3[e][1]] for e in mine], axis=0)
        if not cfg['KD']:
            for e in range(len(prods3)):
                third(e, None)

    def rounds_of(p):
        rs = [('1', None)] + [('x', '1')] * (p in SEL)
        for kind, qs in zip(('35', '47', '26'), PAIRS):
            if kind == '26' and p in SEL3[::2]:
                rs.append(('y', '1'))
            rs += [(kind, r) for r in (('35', '47', '26') if qs in pairs3[p] else (0, 1))]
        return rs

    def deferred(l, p, rd):
        if l == L - 1 and p == 6 and rd[0] == '26':
            return rd[1] in cfg['LATE']
        return rd in cfg['DEFER'].get(p, ()) or (l == L - 1 and rd in cfg['DEFL'].get(p, ()))

    port = lambda a, st_, n: max((2 * a + st_ + 2 + 16 / n) / 72, cfg['PORT'] * st_ / 8)
    cand = []
    for p in OUTER:
        for rd in rounds_of(p):
            kind, n = rd
            if n == '1':
                pq = [(p, q) for q in (3, 5, 4, 7)] if kind == 'x' else [(pp, q) for pp in (p, SEL3[SEL3.index(p) + 1]) for q in (2, 6)]
                cand += [(p, rd, x + ('1',), (1, 0, 0, 1)) for x in pq]
            elif n in ('35', '47'):
                cand += [(p, rd, (p, int(q), w), pat) for q in kind
                         for w, pat in ((('v', (0, 1, 1, 0)),) if n == '35' else (('k', (0, 0, 1, 0)), ('m', (1, 0, 0, 0))))]
            elif n != '26':
                cand += [(p, rd, (p, int(q), (h, nn)), tuple(int(e == 2 * h + nn) for e in range(4)))
                         for q in kind for nn in ((0, 1) if kind == '1' else (n,)) for h in range(2)]
    extra, sites, rows_ = {}, [], []
    while len(sites) < 64:
        def busy(c):
            a, st_, _ = round_usage(c[0], c[1], False, False, deferred(1, c[0], c[1]), cfg['HY'], c[0] in SEL3)
            return (2 * (a + extra.get(c[:2], 0)) + st_ + (5 if isinstance(c[1][1], str) else 3)) * cfg['BW'].get(c[0], 1.0)
        c = min(cand, key=busy)
        cand.remove(c)
        row = np.kron(np.kron(PC[c[2][0]], PC[c[2][1]]), c[3])
        if np.linalg.matrix_rank(np.array(rows_ + [row])) > len(rows_):
            rows_.append(row)
            sites.append(c[2])
            extra[c[:2]] = extra.get(c[:2], 0) + (1 if isinstance(c[1][1], str) else 0.5)
    want = np.zeros((64, 8))
    for e, (I, J, i, j, h, n) in enumerate(np.ndindex(*(2,) * 6)):
        want[e, phys(2 * J + j, n)] = scale(2 * I + i, 2 * J + j, h, n) / GAMMA
    bcoef = np.round(np.linalg.solve(np.array(rows_, float).T, want) * 4096) / 4096
    assert (np.array(rows_).T @ bcoef == want).all()
    if cfg.get('PLANOUT') is not None:
        print(extra, np.abs(bcoef).max(), (np.abs(bcoef).sum(1) == 0).sum())
    sites = {x: e for e, x in enumerate(sites) if bcoef[e].any()}

    outs = [(l, p) for l in range(L) for p in OUTER]
    G = len(outs)
    PRE = cfg['PRE']
    sched, start, use, vuse = [], [], [cfg['PU']] * PRE, []
    for g, (l, p) in enumerate(outs):
        start.append(len(use))
        for rd in rounds_of(p):
            n = NQ if isinstance(rd[1], str) else NC
            sched.append((g, rd, len(use), n))
            a, st_, ld_ = round_usage(p, rd, l == 0, l == L - 1, deferred(l, p, rd), cfg['HY'], cfg['TEL'] and p in SEL3)
            use += [port(a + extra.get((p, rd), 0), st_, n)] * n
            vuse += [st_ / 8] * n
    T = len(use)
    cap = [max(cfg['CAP'] - max(use[t], use[(t + 1) % T], cfg['UMIN']), 0.0) ** cfg['GAM'] * (t < T - cfg['TAIL']) for t in range(T)]
    for g in range(G):
        for t in range(start[g], (start + [T])[g + 1]):
            cap[t] *= cfg['CM'][g % 7]
    jobs = []
    late = []
    def add(lo, hi, alu, st_, ld_, nst, l, fn):
        w = alu / 64 + cfg['CS'] * (st_ + nst) / 16 + cfg['CL'] * ld_ / 48
        w *= cfg['KW'][0 if l in (None, 'fin', 'late') else nst]
        if cfg['HOLD'] and nst >= 3:
            nst += 2
        jobs.append((lo, max(hi, lo), [w * f for f in (cfg['FR'][nst - 1] if not (st_ >= 16 and ld_ == 32 and alu < 75) else {2: (.5, .5), 3: (.46, .28, .26), 4: (.19, .26, .29, .26)}[nst])], l, fn, nst, st_ / 16 / w))
    for g, (l, p) in enumerate(outs):
        ready = 7 * l - 2 * all(I == 0 for (I, J), _ in LA[p])
        lo = start[ready] - (T if ready < 0 else 0) - (PRE if ready == 0 else 0)
        if ready % 7 == 0 and (l > 0 or cfg['LATE']):
            lo += cfg['EW6']
        if cfg['DEFER'].get(7) and ready % 7 == 5 and l > 0:
            lo += cfg['EW'] + 1
        for gg, rd, t0, n_ in sched:
            if gg == g and deferred(l, p, rd):
                if p == 7:
                    due = start[g + 1] + cfg['EW'] if l < L - 1 else start[g + 2] - 1
                elif p == 5:
                    due = start[7 * l + 5] - 1
                elif p == 6:
                    due = (start[g + 1] + cfg['EW6'] if l < L - 1 else T - cfg['TAIL']) - 1
                else:
                    due = [t for g2, r2, t, _ in sched if g2 == g + 1 and r2[0] == rd[0]][0] - 3
                nops = 4 * sum(len(t) + (x in OACT[p][2]) * (2 + 2 * (l == L - 1)) for x in OACT[p][1][1:] + OACT[p][2] for t in x[1:])
                ws = [(i, j, n, h * Mq + 16 * c) for c in range(NQ) for h, n in {'35': [(0, 1)], '47': [(0, 0)], '26': [(1, 1), (1, 0)]}[rd[1]]
                      for i, j in {'35': [B12], '47': [B11], '26': [B22, B21]}[rd[0]]]
                m_ = 1 if p == 6 and not (l == L - 1 and rd[0] == '26') else 2
                if l == L - 1 and p == 6 and rd[0] == '26':
                    for u in range(0, len(ws), 2):
                        for r8 in (0, 8):
                            late.append((l, p, [w[:3] + (w[3] + r8,) for w in ws[u:u + 2]], 8))
                            add(0, cfg['EW6'] - 1, nops * 0.45, 1, nops * 0.4, 1, 'late', late[-1])
                    continue
                for u in range(0, len(ws), m_):
                    add(t0 + n_, due, nops * m_ // 2, 3, nops * m_ // 2, 1, 'fin', (l, p, ws[u:u + m_]))
        hi = start[g] - LAG - 3 - (PRE if g == 0 else 0)
        nt = len(LA[p])
        save = [b for b, pp in cfg['XC'].items() if pp == p and l == 0]
        if p == 2 and p in SEL3 and not cfg['MRG']:
            for c in range(NC):
                for k in range(2):
                    add(lo, (start[7 * l + cfg['MAT']] + cfg['MOFF'] + cfg['MOF0'] * (l == 0)) - 3, 40 + 8 * len(save), 16 + 8 * len(save), 32, cfg['NM'], l,
                        functools.partial(unit2, l, (2, 6), c, k, save))
        if p in SEL3 and p in (2, 6):
            lo, nt, save = (start[7 * l + cfg['MAT']] + cfg['MOFF'] + cfg['MOF0'] * (l == 0)), 1, []
        if p in SEL3:
            if p in SEL3[1::2]:
                host = 7 * l + OUTER.index(SEL3[SEL3.index(p) - 1])
                hi = [t0 for gg, rd, t0, _ in sched if gg == host and rd[0] == 'y'][0] - LAG - 3
            for c in range(NQ):
                add(lo, hi, 32 * nt + 50 + 32 * len(save), 18 + 32 * len(save), 32 * nt, cfg['NS'][3], l,
                    functools.partial(unit3, l, p, (2, 6), c, save))
        elif p != 6:
            ps = (2, 6) if p == 2 else (p,)
            nq = sum(len(q2[x]) for x in ps)
            alu = 8 * (nt - 2 + len(ps)) + sum(8 if x in SEL else 16 for x in ps) + nq
            if cfg['MRG'] and p == 1:
                for c in range(NC):
                    for k in range(2):
                        add(lo, hi, 55 + 8 * len(save), 23 + 8 * len(save), 32, cfg['MRG'], l, functools.partial(unit2, l, ps, c, k, save))
                continue
            if MAT and p == 2:
                hi = (start[7 * l + cfg['MAT']] + cfg['MOFF'] + cfg['MOF0'] * (l == 0)) - 3
            for c in range(NC):
                for k in range(2):
                    add(lo, hi, alu + 8 * len(save), nq + 8 * len(save) + 12 * (bool(MAT) and p == 2), 8 * nt, 1 if nq <= 3 else cfg['NS'][4] if nq == 6 else cfg['NS'][0] if nq <= 7 else cfg['NS'][1], l,
                        functools.partial(unit2, l, ps, c, k, save))
        if MAT and p in (2, 6):
            lo, nt = (start[7 * l + cfg['MAT']] + cfg['MOFF'] + cfg['MOF0'] * (l == 0)), 1
        if p in SEL:
            for qs, c in ([(qs, c) for qs in PAIRS[:2] for c in range(NQ)] if cfg['QO'] else
                          [(qs, c) for c in range(NQ) for qs in PAIRS[:2]]):
                if True:
                    add(lo, start[g] - LAG - 3 + (NC if g else -PRE), 16 * nt + 46, 14, 16 * nt, cfg['NS'][2 + (nt == 4)], l,
                        functools.partial(unit3, l, p, qs, c, []))
    for R in range(4):
        for C in range(4):
            for c in range(0, NC, 2):
                add(start[6], start[G - 2] - 2, 18, 7, 4, 1, None, (R, C, 16 * c))
    when = spread_jobs([j[:3] + j[6:] for j in jobs], cap, cfg['TAIL'],
                       [cfg['VK'] * (1 - vuse[(t + 1) % T]) for t in range(T)] if cfg['VK'] else None)
    evs = [e[:1] + e[2:] for e in sorted((t % T, ts[0] % T, ji, u) for ji, ts in enumerate(when) for u, t in enumerate(ts))]
    half = {}
    for e, (t, ji, u) in enumerate(evs):
        half[(ji, u)] = 2 * t + (0 if cfg['DBL'] and e + 1 < len(evs) and evs[e + 1][0] == t and (e == 0 or evs[e - 1][0] != t) else 1)
    SEG = cfg['SEG']
    for sg, seeds in enumerate(cfg['SEEDS']):
        mine = [e for e, ev in enumerate(evs) if ev[0] // SEG == sg]
        for seed in seeds:
            for e in mine:
                _, ji, u = evs[e]
                r = (e * 2654435761 + seed * 97531 + 12345) * 2246822519 % 4294967296 >> 8
                if r % 100 >= cfg['PJ']:
                    continue
                h = half[(ji, u)] + (2, -2, 1, -1, 2, -2)[r // 100 % 6]
                off = when[ji][u] - when[ji][u] % T
                lo_ = max(2 * (jobs[ji][0] - off), 2 * sg * SEG, half[evs[e - 1][1:]] + 1 if e else 0)
                hi_ = min(2 * (jobs[ji][1] - off) + 1, 2 * (sg + 1) * SEG - 1,
                          half[evs[e + 1][1:]] - 1 if e + 1 < len(evs) else 2 * (T - cfg['TAIL']))
                if lo_ <= h <= hi_:
                    half[(ji, u)] = h
    if cfg.get('SHOW'):
        for g in range(7, 14):
            rg = range(start[g], start[g + 1])
            print('  ', ''.join('%2d' % round(10 * use[t]) for t in rg))
            print('  ', ''.join('%2s' % ''.join((str(len(w)) if u == 0 else '.') for w in when for u, x in enumerate(w) if x % T == t) for t in rg))
    plan = {}
    for _, ji, u in evs:
        plan.setdefault(half[(ji, u)] // 2, []).append((half[(ji, u)] % 2, jobs[ji][3], jobs[ji][4], STAGES[jobs[ji][5]][u]))
    if cfg.get('PLANOUT') is not None:
        kind = lambda j: 'conv' if j[3] is None else 'fin' if j[3] in ('fin', 'late') else j[4].func.__name__ + str(j[4].args[1] if j[4].func.__name__ == 'unit2' else j[4].args[2])
        cfg['PLANOUT'].update(ev=[(half[(ji, u)], kind(jobs[ji]), u, jobs[ji][2][u]) for _, ji, u in evs], use=use,
                              rd=[(outs[g][1], str(rd)) for g, rd, t0, n in sched for _ in range(n)])
    assert all((ts[0] < 0) == (ts[-1] < 0) for ts in when)
    carried = [(job[4], job[5]) for ts, job in zip(when, jobs) if ts[0] < 0]

    def w_copy(l):
        return pltpu.make_async_copy(w_hbm.at[l], w_ref.at[l], sem.at[l])

    def w0_copy(u):
        return pltpu.make_async_copy(w_hbm.at[0, :, u], w_ref.at[0, :, u], sem.at[L + 6 + u])

    def in_copy(t, slot):
        return pltpu.make_async_copy(x_hbm.at[pl.ds(pl.multiple_of(t * TM, 32), TM)], xn2_ref.at[slot], sem.at[L + slot])

    def out_copy(t, slot, part):
        r0, nr = ((0, 2 * Mh), (2 * Mh, Mh), (3 * Mh, Mh), (0, TM))[part]
        return pltpu.make_async_copy(o2_ref.at[slot, pl.ds(r0, nr)],
                                     o_hbm.at[pl.ds(pl.multiple_of(t * TM + r0, 32), nr)],
                                     sem.at[L + 4 + slot])

    xr_in = pltpu.make_async_copy(x_hbm.at[pl.ds(NMAIN * TM, R0)], xr_ref, sem.at[L + 2])
    xr_out = pltpu.make_async_copy(xr_ref, o_hbm.at[pl.ds(NMAIN * TM, R0)], sem.at[L + 2])
    b_in = pltpu.make_async_copy(b_hbm, b_ref, sem.at[L + 3])

    def turn(tile):
        slot = tile % 2
        pl.when(tile + 2 < NMAIN)(lambda: in_copy(tile + 2, slot).start())
        pl.when(tile > 1)(lambda: out_copy(tile - 2, slot, 3).wait())
        pl.when(tile + 1 < NMAIN)(lambda: in_copy(tile + 1, 1 - slot).wait())

    def prologue():
        b_in.start()
        for u in range(8):
            w0_copy(u).start()
        xr_in.start()
        in_copy(0, 0).start()
        for l in range(1, L):
            w_copy(l).start()
        in_copy(1, 1).start()
        b_in.wait()
        for l in range(L):
            bf_ref[l] = b_ref[l:l + 1, :].astype(f32)

        def bias_tiles(l, carry):
            b = jnp.broadcast_to(bf_ref[l] + (l == 0).astype(f32), (8, D))
            for u in sites.values():
                terms = [b[:, key * 128:(key + 1) * 128] * float(cf) for key, cf in enumerate(bcoef[u]) if cf != 0.0]
                bt_ref[l, u] = functools.reduce(lambda x, y: x + y, terms)
            return carry
        jax.lax.fori_loop(0, L, bias_tiles, 0)
        if cfg.get('FAST'):
            return

        def slab(u, carry):
            w0_copy(u).wait()
            zero = jax.lax.shift_right_logical(u, 12)
            prep(0, u, iter(lambda: None, 0), zero, kb0)
            return zero
        zero = jax.lax.fori_loop(0, cfg['NSLAB'], slab, 0)

        def plain(l, xbf, x0f, x, na, free, never, j0=0, j1=D // 128):
            passes = []
            for jt in range(j0, j1):
                cols = slice(jt * 128, (jt + 1) * 128)
                ya = _dot(xbf[:, :D // 2], w_ref[l, 0:4, :, :, cols].reshape(D // 2, 128)) + bf_ref[l, :, cols]
                passes += [ya, _dot(xbf[:, D // 2:], w_ref[l, 4:8, :, :, cols].reshape(D // 2, 128)) + ya]
            xp_ref[0, :, j0 * 128:j1 * 128] = x0f * jnp.concatenate(passes[1::2], axis=1) + x
            for u in range(na):
                f_ = (u - free) * len(passes) * (R0 // 8) // (na - free)
                if cfg['PPH'] is not None:
                    f_ = f_ // 2 * 2 + cfg['PPH']
                ps, rr = divmod(f_, R0 // 8)
                yield None if u < free else (never, passes[ps][rr * 8:rr * 8 + 8, :])

        for u in range(cfg['NSLAB'], 8):
            w0_copy(u).wait()
        xr_in.wait()
        never = jnp.broadcast_to(zero, (8, 128)) != 0
        jm = cfg['JM']
        x0f = xr_ref[:, :jm * 128].astype(f32)
        xp_ref[1, :, :jm * 128] = x0f
        anchors = plain(0, xr_ref[...], x0f, x0f, (8 - cfg['NSLAB']) * (28 + 4 * cfg['LANC'] + len(prods3)), cfg['AFREE'], never, 0, jm)
        for u in range(cfg['NSLAB'], 8):
            prep(0, u, anchors, zero, (kb0, kb1)[u % 2])
        in_copy(0, 0).wait()
        x0f = xr_ref[:, jm * 128:].astype(f32)
        xp_ref[1, :, jm * 128:] = x0f
        units = [(R, C, r) for R in range(4) for C in range(4) for r in range(0, Mh, 32)]
        anchors = plain(0, xr_ref[...], x0f, x0f, len(units) + sum(len(STAGES[n]) for _, n in carried) + 2, 4, never, jm)
        for R, C, r in units[:len(units) // 2]:
            conv(xn2_ref.at[0], zero, R, C, r, min(32, Mh - r), next(anchors))
        for fn, n in carried:
            st8 = {}
            for group in STAGES[n]:
                anchor = next(anchors)
                fn(st8, group, zero, jax.lax.shift_right_logical(zero, 1), anchor)
        for R, C, r in units[len(units) // 2:]:
            conv(xn2_ref.at[0], zero, R, C, r, min(32, Mh - r), next(anchors))

        def layer(l, carry):
            w_copy(l).wait()
            zero = jax.lax.shift_right_logical(l, 12)
            x = xp_ref[0]
            anchors = plain(l, x.astype(bf16), xp_ref[1], x, 8 * (28 + 4 * cfg['LANC'] + len(prods3)), cfg['AFREE'],
                            jnp.broadcast_to(zero, (8, 128)) != 0)
            for u in range(8):
                prep(l, u, anchors, zero, (kb0, kb1)[u % 2])
            return carry

        jax.lax.fori_loop(1, L, layer, 0)
        xr_ref[...] = xp_ref[0].astype(bf16)
        xr_out.start()

    def main(tile, carry, only_late=False):
        zs, za = jax.lax.shift_right_logical(tile, 12), jax.lax.shift_right_logical(tile, 13)
        never = jnp.broadcast_to(zs, (8, 128)) != 0
        slot = tile % 2
        xn_ref = xn2_ref.at[1 - slot]
        o_cur = [o2_ref.at[1 - slot]]
        def rows(h, r0):
            if isinstance(h, tuple):
                return slice(r0 + h[0], r0 + h[0] + h[1])
            return slice(r0, r0 + Mh) if h is None else slice(r0 + h * Mq, r0 + (h + 1) * Mq)

        def ld(loc, h=None, z=0):
            return loc[0][(z,) + loc[1] + (rows(h, loc[2]),)]

        def st(loc, v, h=None):
            loc[0][(za if h == 1 and not loc[1] and cfg['ZB'] else zs,) + loc[1] + (rows(h, loc[2]),)] = v

        def by_half(v, h, fn):
            if isinstance(h, tuple):
                h = h[0] // Mq
            return fn(v, h) if h is not None else jnp.concatenate([fn(v[:Mq], 0), fn(v[Mq:], 1)], axis=0)

        def gather(ref, idx, n, pos):
            if cfg['NOBC']:
                return ref[idx + (slice(0, n), slice(16 * pos, 16 * pos + 16))].reshape(16 * n, 128)
            return ref.bitcast(u32)[idx + (slice(0, n), slice(8 * pos, 8 * pos + 8))].reshape(8 * n, 128)

        as_bf16 = lambda v: v if cfg['NOBC'] else pltpu.bitcast(v, bf16)

        def lhs2(p, q):
            ref, u = s2loc(p)
            return as_bf16(jnp.concatenate([gather(ref, (0, u, k), NC, q2[p].index(q)) for k in range(2)], axis=1))

        def rhs2(l, p, q, n):
            return as_bf16(gather(t2[p], (l, n), 16, q2[p].index(q)))

        def dot3(l, p, q, r):
            qs = next(qs for qs in PAIRS if q in qs)
            return _dot(as_bf16(gather(s3[(p, qs)], (0, qs.index(q)), NQ, ORD.index(r))),
                        as_bf16(gather(t3_ref, (l, prods3.index((p, q))), 8, ORD.index(r))))

        def biased(v, l, *site):
            if site not in sites:
                return v
            return (v.reshape(Mq // 8, 8, 128) + bt_ref[l, sites[site]]).reshape(Mq, 128)

        def biased2(v, l, p, q, n):
            if not any((p, q, (h, n)) in sites for h in range(2)):
                return v
            return by_half(v, None, lambda x, h: biased(x, l, p, q, (h, n)))

        wait = {}
        def outer_act(l, p, i, j, n, d, h, part=None):
            bt, stores, finals = OACT[p]
            if part == 'raw':
                stores, finals = stores[:1], []
            if part == 'rest':
                bt, stores = [], stores[1:]
            if p == 6 and part is None and (i, j) != B12 and (h, n) != (0, 1):
                stores = []
            cache = {'d': d}
            def comb(terms):
                for _, src in terms:
                    if isinstance(src, str) and src not in cache:
                        cache[src] = ld(oloc(src, i, j, n), h)
                v = lincomb([(s, cache[src]) for s, src in terms if isinstance(src, str)])
                return v
            fin = [(IJ, comb(terms)) for IJ, terms in finals]
            for name, v in [(name, comb(terms)) for name, terms in stores]:
                st(oloc(name, i, j, n), v, h)
            for (I, J), y in fin:
                R, C = 2 * I + i, 2 * J + j
                xn = ld(x0loc(R, C, n), h) * y
                if l > 0:
                    xn = xn + ld(xloc(l, R, C, n), h)
                if l < L - 1:
                    st(xloc(l + 1, R, C, n), xn, h)
                else:
                    xn = by_half(xn, h, lambda x, hh: x if scale(R, C, hh, n) == 1.0 else x * (1.0 / scale(R, C, hh, n)))
                    c0 = phys(C, n) * 128
                    if i == 0:
                        o_cur[0][rows(h, R * Mh), c0:c0 + 128] = xn.astype(bf16)
                    elif j == 1:
                        wait[(R, J)] = xn
                    else:
                        o_cur[0][rows(h, R * Mh), c0:c0 + 256] = jnp.concatenate([xn, wait.pop((R, J))], axis=1).astype(bf16)

        def inner_act(g, l, p, kind, n, h, P, Q, part=None):
            vloc = oloc(raw_slot(p), 0, 1, n) if raw_slot(p) else iloc(g, 'v', n)
            if kind == '35':
                st(iloc(g, 's', n), Q + ld(iloc(g, 'm1', n), h), h)
                if not raw_slot(p):
                    st(vloc, P, h)
                outer_act(l, p, 0, 1, n, P, h, part)
            elif kind == '47':
                st(iloc(g, 'u', n), Q + ld(vloc, h), h)
                outer_act(l, p, 0, 0, n, P + ld(iloc(g, 's', n), h), h, part)
            else:
                outer_act(l, p, 1, 1, n, ld(iloc(g, 's', n), h) - Q, h, part)
                outer_act(l, p, 1, 0, n, P + ld(iloc(g, 'u', n), h), h, part)

        def issue(l, p, rd):
            kind, n = rd
            if kind == 'x':
                return [dot3(l, p, q, 1) for q in (3, 5, 4, 7)]
            if kind == 'y':
                return [dot3(l, pp, q, 1) for pp in (p, SEL3[SEL3.index(p) + 1]) for q in (2, 6)]
            if isinstance(n, str):
                if cfg['MO']:
                    d = [dot3(l, p, int(q), int(r)) for q in kind for r in n]
                    return [d[0], d[2], d[1], d[3]]
                return [dot3(l, p, int(q), int(r)) for r in n for q in kind]
            if cfg['GR']:
                ops = [(lhs2(p, 1),) * 2, (rhs2(l, p, 1, 0), rhs2(l, p, 1, 1))] if kind == '1' else [
                    [lhs2(p, int(q)) for q in kind], [rhs2(l, p, int(q), n) for q in kind]]
                d = [_dot(a[:, k * 128:(k + 1) * 128], b[k * 128:(k + 1) * 128]) for a, b in zip(*ops) for k in range(2)]
                return [d[0] + d[1], d[2] + d[3], d[cfg['GR'] - 1]]
            if kind == '1':
                lhs = lhs2(p, 1)
                return [_dot(lhs, rhs2(l, p, 1, 0)), _dot(lhs, rhs2(l, p, 1, 1))]
            return [_dot(lhs2(p, int(q)), rhs2(l, p, int(q), n)) for q in kind]

        def consume(g, l, p, rd, res):
            kind, n = rd
            if n == '1':
                for u, where in enumerate((('35', False), ('47', False)) if kind == 'x' else (('26', False), ('26', True))):
                    pp = SEL3[SEL3.index(p) + 1] if where[1] else p
                    for al in range(2):
                        st(jloc(where[0], '1', al, where[1]), biased(res[2 * u + al], l, pp, int(where[0][al]), '1'), 0)
            elif isinstance(n, str):
                sm = [res[al] + res[2 + al] for al in range(2)]
                df = [res[al] - res[2 + al] for al in range(2)]
                J = lambda name, al: ld(jloc(kind, name, al, name == '1' and kind == '26' and p in SEL3[1::2]), 0)
                part = 'raw' if deferred(l, p, rd) else None
                done = lambda h, nn, m: inner_act(g, l, p, kind, nn, h, m[0] + m[1], m[0] - m[1], part)
                O, I = (lambda i, j: oloc(raw_slot(p), i, j, 1)), (lambda name: iloc(g, name, 1))
                rec = lambda al: [(s, ld(loc, 0, za if cfg['ZB'] else 0)) for s, loc in {
                    '35': [[(1, O(0, 1))], [(1, I('s')), (-1, I('m1'))]],
                    '47': [[(1, O(0, 0)), (-1, I('s'))], [(1, I('u')), (-1, O(0, 1))]],
                    '26': [[(1, O(1, 0)), (-1, I('u'))], [(1, I('s')), (-1, O(1, 1))]]}[kind][al]
                    if not (cfg['TEL'] and p in SEL3 and any(loc[0] is I(x)[0] for x in 'su'))]
                if n == '35':
                    for al in range(2):
                        st(jloc(kind, 's', al), df[al] + J('1', al), 0)
                    done(0, 1, [biased(sm[al], l, p, int(kind[al]), 'v') for al in range(2)])
                elif n == '47':
                    if cfg['HY'] == 1:
                        for al in range(2):
                            st(jloc(kind, 'u', al), biased(df[al], l, p, int(kind[al]), 'k'), 0)
                    else:
                        for al, v in enumerate((df[0] + df[1], df[0] - df[1])):
                            st(jloc(kind, 'u', al), lincomb([(1, v)] + rec(al)), 0)
                    done(0, 0, [biased(sm[al] + J('s', al), l, p, int(kind[al]), 'm') for al in range(2)])
                else:
                    if cfg['HY'] == 1:
                        m = [sm[al] + J('u', al) for al in range(2)]
                        P, Q = lincomb([(1, m[0] + m[1])] + rec(0)), lincomb([(1, m[0] - m[1])] + rec(1))
                    else:
                        P, Q = (sm[0] + sm[1]) + J('u', 0), (sm[0] - sm[1]) + J('u', 1)
                    done(1, 1, [J('s', al) - df[al] for al in range(2)])
                    inner_act(g, l, p, kind, 0, 1, P, Q, part)
            elif kind == '1':
                for nn in range(2):
                    st(iloc(g, 'm1', nn), biased2(res[nn], l, p, 1, nn))
            else:
                a, b = (biased2(res[al], l, p, int(kind[al]), n) for al in range(2))
                inner_act(g, l, p, kind, n, None, a + b, a - b)

        def fin(fn, anchor):
            nr = fn[3] if len(fn) > 3 else 16
            for i, j, nf, r0 in fn[2]:
                d = ld(oloc(raw_slot(fn[1]), i, j, nf), (r0, nr))
                for r8 in range(0, nr, 8):
                    d = tie(d, anchor, r8)
                outer_act(fn[0], fn[1], i, j, nf, d, (r0, nr), 'rest')

        if only_late:
            for fn in late:
                fin(fn, None)
            return out_copy(tile - 1, 1 - slot, 2).start()
        state = {}
        cnt.clear()
        for g, rd, t0, n in sched:
            l, p = outs[g]
            if t0 == start[1]:
                if late:
                    pl.when(tile > 0)(lambda: out_copy(tile - 1, 1 - slot, 2).start())
                o_cur[0] = o2_ref.at[slot]
            if t0 == start[G - 1]:
                out_copy(tile, slot, 0).start()
            res = issue(l, p, rd)
            if cfg['EO']:
                consume(g, l, p, rd, res)
            for t in range(0 if t0 == PRE else t0, t0 + n):
                for ph, l2, fn, group in plan.get(t, []):
                    gr = max(16 * (t - t0) + 8 * ph, 0)
                    if cfg['GF']:
                        gr = 16 * (t - t0) + 8 * (1 - ph)
                    gs = cfg['GS']
                    gate = res[2 if len(res) == 3 else cfg['GM']][gr:gr + 8, :]
                    if t < t0:
                        gate = bt_ref[0, t]
                    elif cfg['GADD'] and isinstance(rd[1], str) and rd[1] != '1':
                        gate = gate + res[2 + gs % 2][gr:gr + 8, :]
                    elif gs == 2 and rd[0] != '1' and rd[1] != '1':
                        gate = gate + res[1][gr:gr + 8, :]
                    if l2 in ('fin', 'late'):
                        fin(fn, (never, gate))
                    elif l2 is None:
                        conv(xn_ref, zs, *fn, min(32, Mh - fn[2]), (never, gate))
                    else:
                        fn(state.setdefault(id(fn), {}), group, zs, za, (never, gate))
            if t0 + n == T:
                out_copy(tile, slot, 1).start()
            if not cfg['EO']:
                consume(g, l, p, rd, res)
        if not late:
            out_copy(tile, slot, 2).start()
        turn(tile + 1)
        return carry

    prologue()
    in_copy(2, 0).start()
    in_copy(1, 1).wait()
    if not cfg.get('NOMAIN'):
        jax.lax.fori_loop(0, NMAIN, main, 0)
    else:
        for p_ in range(1, 8):
            for l_ in range(L):
                o2_ref[0, 0:16, 0:128] = t2[p_][l_, 0, pl.program_id(0) if False else 3, 0:16] + t3_ref[l_, p_, 2, 0:16]
    if late:
        main(jnp.int32(NMAIN), 0, True)
    xr_out.wait()
    out_copy(NMAIN - 1, (NMAIN - 1) % 2, 3).wait()


DEFAULT = dict(SEL=(3, 5, 4, 7, 2, 6), SEL3=(3, 5, 4, 7, 2, 6), XC={B12: 5, B11: 1, B22: 7, B21: 2}, AFREE=2, NOBC=0, VK=0.75, MRG=0, LATE=('26',), LS=8, MOFF=15, MOF0=0, NM=2, BW={}, TEL=1, EW6=25, PRE=0, PU=0.1, GAM=1.0, UMIN=0, LANC=1, KD=1, PO=PREP_ORDER, PT=0, MAT=3, FOLD=1, MO=1, GR=2, NS=(2, 3, 3, 4, 3), NL=1, GE=8, GM=0, DBL=0, GS=0, GF=0, EO=0, KP=16, PPH=None, ZB=0, HY=1, HOLD=0, PORT=0.9, PS=0, NSLAB=6, JM=3, XP=40, XO=16, DEFER={5: [('26', '26'), ('47', '26')], 7: [('26', '26'), ('47', '26')], 2: [('47', '26'), ('26', '26')],
                      6: [('35', '26'), ('47', '26'), ('26', '26'), ('26', '35')]}, DEFL={}, EW=12, KW=(1,) * 5, CM=(1,) * 7, SEEDS=(), SEG=32, PJ=20, QO=0, TIEL=3, GADD=0, TF=0, T8=0, TAIL=3,
               CS=0.5, CL=0.3, UL=0.8, CAP=0.95, FR=((1.,), (.4, .6), (.35, .37, .28), (.16, .26, .31, .27),
                   (.35, .29, .08, .28), (.16, .26, .26, .05, .27)))


def build(TM=640, **kw):
    def f(x0, ws, bs):
        B, D = x0.shape
        L = ws.shape[0]
        cfg = dict(DEFAULT, **kw)
        Mh = TM // 4
        MP = Mh + 32
        nmain = (B - 1) // TM
        R0 = B - nmain * TM
        pairs3, q2 = layout(cfg)
        n3 = sum(2 * len(v) for v in pairs3.values())
        pad = lambda n: n + (2 - n) % 4
        V = pltpu.VMEM
        half = V((1, MP, 128), f32)
        XP = Mh + cfg['XP']
        scratch = ([V((1, 2, 2, 2, XP, 128), f32)] * 4 + [V((1, 2, 4, 2, XP, 128), f32)] * 7 + [half] * (16 + 64 + 26)
                   + [V((1, 1 + (p == 2 and q2[2] == q2[6]), 2, pad(Mh // 16), 16 * len(q2[p]), 128), bf16) for p in range(1, 8)]
                   + [V((1, 2, pad(Mh // 32), 112, 128), bf16)] * (n3 // 2)
                   + [V((L, 2, 16, 16 * len(q2[p]), 128), bf16) for p in range(1, 8)]
                   + [V((L, n3, 8, 112, 128), bf16), V((1, 4, 16 * n3 + cfg['KP'], 128), f32), V((1, 4, 16 * n3 + cfg['KP'], 128), f32),
                      V((L, 64, 8, 128), f32), V((8, 1, D), f32), V((2, TM, D), bf16), V((2, TM, D), bf16), V((L, 8, 8, 16, D), bf16),
                      V((R0, D), bf16), V((2, R0, D), f32), V((L, D), bf16), pltpu.SemaphoreType.DMA((L + 14,))])
        anyspec = pl.BlockSpec(memory_space=pl.ANY)
        return pl.pallas_call(
            functools.partial(_kernel, L=L, TM=TM, R0=R0, NMAIN=nmain, D=D, cfg=cfg),
            in_specs=[anyspec, anyspec, anyspec],
            out_specs=anyspec,
            out_shape=jax.ShapeDtypeStruct((B, D), x0.dtype),
            scratch_shapes=scratch,
            compiler_params=pltpu.CompilerParams(
                vmem_limit_bytes=120 * 1024 * 1024,
                internal_scratch_in_bytes=65536,
                disable_bounds_checks=True,
            ),
        )(x0, ws.reshape(L, 8, 8, 16, D), bs)
    return f


@jax.jit
def pallas_standalone__dcn_v2_cross__recsys_kernel(x0, ws, bs):
    return build(TM=640)(x0, ws, bs)
```

```python
import functools

import jax
import jax.numpy as jnp
import numpy as np
import jax.experimental.pallas as pl
import jax.experimental.pallas.tpu as pltpu

f32 = jnp.float32
bf16 = jnp.bfloat16
u32 = jnp.uint32

B11, B12, B21, B22 = BLOCKS = (0, 0), (0, 1), (1, 0), (1, 1)
LA = {1: [(B11, 1), (B22, 1)], 3: [(B11, 1), (B12, -1)], 5: [(B11, 1), (B12, 1)], 4: [(B12, 1), (B22, 1)],
      7: [(B12, 1), (B22, -1)]}
PC = {1: (1, 0, 0, 1), 2: (0, 0, 1, -1), 3: (1, 1, 1, 1), 4: (1, 0, 1, 0), 5: (-1, 1, 1, -1), 6: (0, 0, 1, 1),
      7: (1, 0, -1, 0)}
KINDS = ('35', '47', '26')
PAIR = {'35': (5, 3), '47': (4, 7), '26': (2, 6)}
ORD = (3, 5, 4, 7, 1, 2, 6)
OUTER = (3, 5, 1, 4, 7, 2, 6)
GUEST = {3: 5, 4: 7, 2: 6}
PRODS3 = [(p, q) for p in OUTER if p != 1 for kind in KINDS for q in PAIR[kind]]
GAMMA = 0.125
OACT = {
    3: ([('M3', '+d')], []),
    5: ([('M5', '+d')], [(B12, '+d +M3')]),
    1: ([('S', '+d +M3 -M5')], []),
    4: ([('M4', '+d')], []),
    7: ([('M7', '+d')], [(B11, '+d +S +M4')]),
    2: ([('M2', '+d'), ('U', '+d +M4 -M7 +M3 +M5')], []),
    6: ([('M6', '+d')], [(B22, '+d +S -M2'), (B21, '+d +U')]),
}
OSL = {'M3': 0, 'M5': 1, 'S': 2, 'M4': 3, 'M7': 4, 'U': 5, 'M2': 6, 'M6': 7}
ISL = {'m1': 0, 's': 1, 'v': 2, 'u': 3}
DEFER = {5: [('26', '26'), ('47', '26')], 7: [('26', '26'), ('47', '26')], 2: [('47', '26'), ('26', '26')],
         6: [('35', '26'), ('47', '26'), ('26', '26'), ('26', '35')]}
SAVE = {5: B12, 1: B11, 7: B22, 2: B21}
STAGES = {1: [(None, 1.0)], 2: [((B11, B12), .4), ((B21, B22), .6)], 'O': [((B11, B12), .5), ((B21, B22), .5)],
          3: [((B11, B12), .35), ((B22,), .37), ((B21,), .28)],
          4: [((B11,), .16), ((B12,), .26), ((B22,), .31), ((B21,), .27)]}
LAG = 8
CFG = dict(CAP=0.95, PORT=0.9, CS=0.5, CL=0.3, VK=0.75, TAIL=3, EW7=12, EW6=25, MOFF=15, GE=8, NSLAB=6, JM=3)


def _dot(a, b):
    return jnp.dot(a, b, preferred_element_type=f32)


def scale(R, C, h, k):
    return 2.0 ** (R // 2 + R % 2 + h - C // 2 - C % 2 - k)


def phys(C, k):
    return 4 * (C // 2) + 2 * k + C % 2


def b_ops(b11, b12, b21, b22):
    r1 = b11 + b22
    g = b12 + b21
    return {1: r1, 2: b11 - b12, 3: b12 - b22, 4: g - r1, 5: b12 + b22, 6: b11 + b12, 7: g + r1}


def lincomb(terms):
    assert terms[0][0] == 1
    acc = terms[0][1]
    for s, v in terms[1:]:
        acc = acc + v if s == 1 else acc - v
    return acc


def rounds_of(p):
    if p == 1:
        return [('1', None)] + [(kind, n) for kind in KINDS for n in range(2)]
    minis = lambda kind: [(kind, r) for r in KINDS]
    return [('1', None), ('x', '1')] + minis('35') + minis('47') + [('y', '1')] * (p in GUEST) + minis('26')


def round_usage(p, rd, first, last, defer):
    stores, finals = OACT[p]
    kind, n = rd
    alu = sum(len(t.split()) - 1 for _, t in stores) + sum(len(t.split()) + (not first) + 2 * last for _, t in finals)
    nst = len(stores) + len(finals)
    if last and kind == '26':
        alu, nst = alu - 0.7 * len(finals), nst - 0.5 * len(finals)
    if defer:
        alu, nst = 0, 1
    elif p == 6 and kind != '35' and n != '35':
        nst -= 1
    if n == '1':
        a, st, m = 0, 4, 0
    elif isinstance(n, str):
        a, st, m = {'35': ((9, 3, 1), (16, 2, 2)), '47': ((10, 3, 1), (18, 2, 2)), '26': ((10, 2, 2), (18, 0, 4))}[kind][n == '26']
    else:
        a, st, m = {'1': (2, 2, 0), '35': (5, 2, 1), '47': (6, 1, 1), '26': (6, 0, 2)}[kind]
    return a + m * alu, st + m * nst


def bias_sites():
    cand = []
    for p in OUTER:
        for rd in rounds_of(p):
            kind, n = rd
            if n == '1':
                pq = [(p, q) for q in (3, 5, 4, 7)] if kind == 'x' else [(x, q) for x in (p, GUEST[p]) for q in (2, 6)]
                cand += [(p, rd, x + ('1',), (1, 0, 0, 1)) for x in pq]
            elif n in ('35', '47'):
                where = [('v', (0, 1, 1, 0))] if n == '35' else [('k', (0, 0, 1, 0)), ('m', (1, 0, 0, 0))]
                cand += [(p, rd, (p, int(q), w), pat) for q in kind for w, pat in where]
            elif n != '26':
                cand += [(p, rd, (p, int(q), (h, nn)), tuple(int(e == 2 * h + nn) for e in range(4)))
                         for q in kind for nn in ((0, 1) if kind == '1' else (n,)) for h in range(2)]
    extra, sites, rows = {}, [], []
    def busy(c):
        a, st = round_usage(c[0], c[1], False, False, c[1] in DEFER.get(c[0], ()))
        return 2 * (a + extra.get(c[:2], 0)) + st + (5 if isinstance(c[1][1], str) else 3)
    while len(sites) < 64:
        c = min(cand, key=busy)
        cand.remove(c)
        row = np.kron(np.kron(PC[c[2][0]], PC[c[2][1]]), c[3])
        if np.linalg.matrix_rank(np.array(rows + [row])) > len(rows):
            rows.append(row)
            sites.append(c[2])
            extra[c[:2]] = extra.get(c[:2], 0) + (1 if isinstance(c[1][1], str) else 0.5)
    want = np.zeros((64, 8))
    for e, (I, J, i, j, h, n) in enumerate(np.ndindex(*(2,) * 6)):
        want[e, phys(2 * J + j, n)] = scale(2 * I + i, 2 * J + j, h, n) / GAMMA
    coef = np.round(np.linalg.solve(np.array(rows, float).T, want) * 4096) / 4096
    assert (np.array(rows).T @ coef == want).all()
    return {x: e for e, x in enumerate(sites) if coef[e].any()}, coef, extra


def yds(groups, cap):
    n = len(cap)
    speed, cls, gcls = [0.0] * n, [-1] * n, {}
    todo = list(groups)
    while todo:
        pre = [0.0]
        for t in range(n):
            pre.append(pre[-1] + (cap[t] if cls[t] < 0 else 0.0))
        best = None
        for a in sorted({g[0] for g in todo}):
            w = 0.0
            for g in sorted((g for g in todo if g[0] >= a), key=lambda g: g[1]):
                w += g[2]
                d = w / max(pre[g[1] + 1] - pre[a], 1e-9)
                if best is None or d > best[0]:
                    best = (d, a, g[1])
        d, a, b = best
        for t in range(a, b + 1):
            if cls[t] < 0:
                speed[t], cls[t] = d, len(gcls)
        gcls.update({g[:2]: len(gcls) for g in todo if g[0] >= a and g[1] <= b})
        todo = [g for g in todo if not (g[0] >= a and g[1] <= b)]
    return speed, cls, gcls


def spread_jobs(jobs, cap, vcap, tail):
    T = len(cap)
    cap3 = cap * 3
    all3 = [(j[0] + k * T, j[1] + k * T, ji, k) for k in range(3) for ji, j in enumerate(jobs) if j[0] + k * T >= 0]
    pend = {}
    for j in sorted(all3, key=lambda j: (j[1], j[3], j[2])):
        pend.setdefault(j[:2], []).append(j)
    left = {w: sum(sum(jobs[j[2]][2]) for j in q) for w, q in pend.items()}
    speed, cls, gcls = yds([w + (left[w],) for w in pend], cap3)
    cum = [0.0]
    for t in range(3 * T):
        cum.append(cum[-1] + speed[t] * cap3[t])
    when = [[] for _ in jobs]
    debt, vdebt, cur, done = 0.0, 0.0, None, 0

    def fits(j, t):
        need = max(debt, 0.0) + sum(jobs[j[2]][2]) + 1.0
        for w in pend:
            if w[1] >= j[1]:
                break
            if left[w] > 1e-9:
                need += left[w]
                if need > cum[w[1] + 1] - cum[t]:
                    return False
        return True

    for t in range(3 * T):
        if t % T == 0:
            debt, vdebt = min(debt, 0.0), -0.5
        while True:
            rdy = [q[0] for w, q in pend.items() if q and w[0] <= t and (gcls[w] == cls[t] or w[1] <= t)]
            j = cur
            if j is None:
                if not rdy:
                    debt = max(debt, 0.0)
                    break
                j = rdy[0]
                if j[1] > t:
                    j = (min if vdebt > 0 else max)([x for x in rdy if x is j or fits(x, t)], key=lambda x: jobs[x[2]][3])
                nst = len(jobs[j[2]][2])
                if nst > 1 and j[1] > t and (t + tail + 2 * nst) // T != t // T:
                    break
            must = j[1] <= t or (cur is not None and ((t + tail + 1) // T != t // T or (rdy and rdy[0][1] <= t)))
            if not must and (cap3[t] == 0.0 or debt > 0.5 * speed[t] * cap3[t]):
                break
            if cur is None:
                pend[j[:2]].pop(0)
                left[j[:2]] -= sum(jobs[j[2]][2])
                cur, done = j, 0
            debt += jobs[j[2]][2][done]
            vdebt += jobs[j[2]][2][done] * jobs[j[2]][3]
            if j[3] == 1:
                when[j[2]].append(t - T)
            done += 1
            if done == len(jobs[j[2]][2]):
                cur = None
        debt -= speed[t] * cap3[t]
        vdebt = min(max(vdebt - vcap[t % T], -0.5), 1.0)
    assert all(j[0] <= ts[0] and ts[-1] <= j[1] and (ts[0] < 0) == (ts[-1] < 0) for j, ts in zip(jobs, when))
    return when


def _kernel(x_hbm, w_hbm, b_hbm, o_hbm, *scratch, L, TM, R0, NMAIN, D, cfg):
    H, Mh, Mq = D // 4, TM // 4, TM // 8
    NC, NQ = Mh // 16, Mq // 16
    it = iter(scratch)
    take = lambda n: [next(it) for _ in range(n)]
    x0b, xb, ib, ob, jb = take(4), take(7), take(16), take(64), take(20)
    s2 = dict(zip(range(1, 8), take(7)))
    s3 = {(p, kind): next(it) for p in OUTER if p != 1 for kind in KINDS}
    t2 = dict(zip(range(1, 8), take(7)))
    t3_ref, kb0, kb1, bt_ref, bf_ref, xn2_ref, o2_ref, w_ref, xr_ref, xp_ref, b_ref, sem = it
    sites, bcoef, extra = bias_sites()
    pos2 = lambda p, q: ORD.index(q) if p == 1 else 0

    xset = lambda l: 6 if l == 'O' else 4 if l == 0 else (l % 2) * 2
    xoff = lambda I, J: 16 * ((I + J) % 2)
    xloc = lambda l, R, C, k: (xb[xset(l) + R // 2], (R % 2, C, k), xoff(R // 2, C // 2))
    x0loc = lambda R, C, k: (x0b[(R // 2) * 2 + C // 2], (R % 2, C % 2, k), 8 + xoff(R // 2, C // 2))
    iloc = lambda g, name, n: (ib[((g % 2) * 4 + ISL[name]) * 2 + n], (), 8 * ISL[name])
    oloc = lambda name, i, j, n: (ob[(OSL[name] * 4 + i * 2 + j) * 2 + n], (), 8 * ((OSL[name] + 2 * j) % 4))

    def jloc(kind, name, al, guest=False):
        u = ('1', 's', 'k').index(name)
        return jb[18 + al if guest else (KINDS.index(kind) * 3 + u) * 2 + al], (), 8 * ((3 * u + al) % 4)

    def tie(v, anchor, r=None, lo=0):
        if anchor is None:
            return v
        never, gate = anchor
        if r is None:
            n = v.shape[0]
            return jax.lax.select(never[n], gate if n == 8 else jnp.tile(gate, (n // 8, 1)), v)
        top = jax.lax.select(never[8], gate, v[r:r + 8])
        return jnp.concatenate(([v[lo:r]] if r > lo else []) + [top, v[r + 8:r + 16]], axis=0)

    def consts(anchor, ss):
        one = {s: tie(jnp.full((8, 128), s, f32), anchor) for s in set(ss)}
        return jnp.concatenate([one[s] for s in ss for _ in range(2)], axis=0)

    def conv(src, R, Q, r, zs, anchor):
        v = src[R * Mh + r:R * Mh + r + 32, Q * H:(Q + 1) * H].astype(f32)
        for j in range(2):
            C, k = 2 * (Q // 2) + j, Q % 2
            buf, idx, off = xloc(0, R, C, k)
            sv = consts(anchor, [scale(R, C, (r + u) // Mq, k) for u in (0, 16)])
            buf[(zs,) + idx + (slice(off + r, off + r + 32),)] = v[:, j * 128:(j + 1) * 128] * sv

    count = {}
    def block_sum(l, terms, ii, jj, kk, r, save, zs, za, anchor, gate=True):
        rng = lambda t: slice(t[0], t[-1] + 1)
        vals = []
        for u, ((I, J), s) in enumerate(terms):
            ref, r0 = xb[xset(l) + I], xoff(I, J) + r
            v = ref[za if u == 0 else 0, rng(ii), 2 * J + jj[0]:2 * J + jj[-1] + 1, rng(kk), r0:r0 + 16, :]
            if (I, J) == save:
                sv = consts(anchor, [GAMMA / scale(2 * I + i, 2 * J + j, r // Mq, k) for i in ii for j in jj for k in kk])
                x0b[I * 2 + J][zs, rng(ii), rng(jj), rng(kk), r0 + 8:r0 + 24, :] = v * sv.reshape(v.shape)
            if u == 0 and gate:
                count[xset(l)] = count.get(xset(l), -1) + 1
                if count[xset(l)] % cfg['GE'] == 0:
                    ref[0, 0, 0, 0, Mh + 24:Mh + 32, :] = anchor[1]
            vals.append((s, v))
        v = lincomb(vals)
        return v.reshape(v.size // 128, 128)

    def operands(a, group, st8, store):
        for u, b in enumerate(group):
            st8[b] = a if len(group) == 1 else a[:, u:u + 1]
        ops = {}
        if B12 in group:
            ops[3], ops[5] = st8[B11] - st8[B12], st8[B11] + st8[B12]
        if B22 in group:
            ops[4], ops[7] = st8[B12] + st8[B22], st8[B12] - st8[B22]
            ops[1] = st8['l1'] = st8[B11] + st8[B22]
        if B21 in group:
            g = st8[B12] + st8[B21]
            ops[2], ops[6] = g + st8['l1'], g - st8['l1']
        now = [q for q in ORD if q in ops]
        if now:
            u = ORD.index(now[0])
            store(slice(u, u + len(now)), jnp.concatenate([ops[q] for q in now], axis=1).astype(bf16))

    def unit1(l, c, k, save, st8, group, zs, za, anchor):
        def store(pos, v):
            s2[1][zs, k:k + 1, pos, 16 * c:16 * c + 16, :] = v
        e = block_sum(l, LA[1], [group[0][0]], [0, 1], [k], 16 * c, save, zs, za, anchor)
        operands(tie(e, anchor, 16).reshape(1, 2, 16, 128), group, st8, store)

    def unit26(l, c, k, save, st8, group, zs, za, anchor):
        i = group[0][0]
        f = block_sum(l, [(B11, 1), (B22, 1)], [i], [0, 1], [k], 16 * c, save, zs, za, anchor, False)
        e = tie(block_sum(l, [(B12, 1), (B21, 1)], [i], [0, 1], [k], 16 * c, save, zs, za, anchor), anchor)
        for J, v in enumerate((e + f, e - f)):
            r0 = xoff(0, J) + 16 * c
            xb[6][zs, i, 2 * J:2 * J + 2, k, r0:r0 + 16, :] = v.reshape(2, 16, 128)

    def unit3(l, p, kind, c, save, st8, group, zs, za, anchor):
        def store(pos, v):
            s3[(p, kind)][zs, :, pos, 16 * c:16 * c + 16, :] = v
        h, kk = group[0][0], [b[1] for b in group]
        ii, jj = {'35': ([0], [0, 1]), '47': ([0, 1], [1]), '26': ([0, 1], [0, 1])}[kind]
        src = (l, LA[p]) if p in LA else ('O', [((0, (2, 6).index(p)), 1)])
        n = 16 * len(kk)
        v = block_sum(*src, ii, jj, kk, h * Mq + 16 * c, save, zs, za, anchor)
        if kind == '26':
            e, f = tie(v, anchor, 16, 16) + v[32:48], v[0:16] + v[48:64]
            r0 = h * Mq + 16 * c
            s2[p][zs, kk[0], 0, r0:r0 + 16, :] = f.astype(bf16)
        else:
            e, f = tie(v, anchor, n - 16), v[n:]
        operands(jnp.concatenate([e + f, e - f], axis=0).reshape(2, len(kk), 16, 128), group, st8, store)

    NPREP = 32 + len(PRODS3)
    def prep(l, u, anchors, zero, kb):
        mul = lambda v, s: v if s == 1.0 else v * s
        stack = lambda T: jnp.concatenate([T[q] for q in ORD], axis=0).reshape(7, 16, 128).astype(bf16)
        rows = pl.ds(16 * u, 16) if isinstance(u, int) else pl.ds(pl.multiple_of(16 * u, 16), 16)
        for k in range(2):
            wide = [w_ref[l, phys(R, k), u].astype(f32) for R in range(4)]
            for n in range(2):
                anchor = next(anchors)
                blk = lambda R, C: mul(wide[R][:, phys(C, n) * 128:(phys(C, n) + 1) * 128], scale(R, C, k, n))
                O = {(i, j): b_ops(blk(i, j), tie(blk(i, 2 + j), anchor, 0), blk(2 + i, j), blk(2 + i, 2 + j))
                     for i, j in BLOCKS}
                for p in (2, 6, 3, 5, 1, 4, 7):
                    o = [mul(O[b][p], 4.0 if p == 1 else 1.0) for b in BLOCKS]
                    T = b_ops(o[0], tie(o[1], next(anchors), 0), o[2], o[3])
                    if p == 1:
                        T[1] = T[1] * 2.0
                        t2[p][l, n, k, :, rows, :] = stack(T)
                        continue
                    t2[p][l, n, k, 0, rows, :] = (T[1] * 4.0).astype(bf16)
                    e0 = PRODS3.index((p, 5))
                    if (k, n) != (1, 1):
                        kb[zero, k * 2 + n, 16 * e0:16 * e0 + 96, :] = jnp.concatenate(
                            [T[q] for _, q in PRODS3[e0:e0 + 6]], axis=0)
                        continue
                    for e in range(e0, e0 + 6):
                        v = kb[0, 0:3, 16 * e:16 * e + 16, :]
                        T3 = b_ops(v[0], tie(v[1], next(anchors), 0), v[2], T[PRODS3[e][1]])
                        T3[1] = T3[1] * 2.0
                        t3_ref[l, e, :, rows, :] = stack(T3)

    def deferred(l, p, rd):
        if l == L - 1 and p == 6 and rd[0] == '26':
            return rd[1] == '26'
        return rd in DEFER.get(p, ())

    outs = [(l, p) for l in range(L) for p in OUTER]
    G = len(outs)
    sched, start, use, vuse = [], [], [], []
    for g, (l, p) in enumerate(outs):
        start.append(len(use))
        for rd in rounds_of(p):
            n = NQ if isinstance(rd[1], str) else NC
            sched.append((g, rd, len(use), n))
            a, st_ = round_usage(p, rd, l == 0, l == L - 1, deferred(l, p, rd))
            a += extra.get((p, rd), 0)
            use += [max((2 * a + st_ + 2 + 16 / n) / 72, cfg['PORT'] * st_ / 8)] * n
            vuse += [st_ / 8] * n
    T = len(use)
    first = lambda g, kind: next(t0 for gg, rd, t0, _ in sched if gg == g and rd[0] == kind)
    jobs, late = [], []
    def add(lo, hi, alu, st_, ld_, scheme, kind, fn):
        w = alu / 64 + cfg['CS'] * (st_ + len(STAGES[scheme])) / 16 + cfg['CL'] * ld_ / 48
        jobs.append((lo, max(hi, lo), [w * f for _, f in STAGES[scheme]], st_ / 16 / w, scheme, kind, fn))
    for g, (l, p) in enumerate(outs):
        for gg, rd, t0, n_ in sched:
            if gg == g and deferred(l, p, rd):
                last = l == L - 1
                nops = 4 * (sum(len(t.split()) for _, t in OACT[p][0][1:]) + sum(len(t.split()) + 2 + 2 * last for _, t in OACT[p][1]))
                ws = [(i, j, n, h * Mq + 16 * c) for c in range(NQ)
                      for h, n in {'35': [B12], '47': [B11], '26': [B22, B21]}[rd[1]]
                      for i, j in {'35': [B12], '47': [B11], '26': [B22, B21]}[rd[0]]]
                if t0 + n_ == T:
                    for u in range(0, len(ws), 2):
                        for r8 in (0, 8):
                            late.append((l, p, [w[:3] + (w[3] + r8,) for w in ws[u:u + 2]], 8))
                            add(0, cfg['EW6'] - 1, nops * 0.45, 1, nops * 0.4, 1, 'fin', late[-1])
                    continue
                due = {5: lambda: start[7 * l + 5] - 1, 2: lambda: first(g + 1, rd[0]) - 3,
                       7: lambda: start[g + 2] - 1 if last else start[g + 1] + cfg['EW7'],
                       6: lambda: T - cfg['TAIL'] - 1 if last else start[g + 1] + cfg['EW6'] - 1}[p]()
                m = 1 if p == 6 else 2
                for u in range(0, len(ws), m):
                    add(t0 + n_, due, nops * m // 2, 3, nops * m // 2, 1, 'fin', (l, p, ws[u:u + m], 16))
        if p in (3, 5):
            lo = start[7 * l - 2] + (cfg['EW7'] + 1 if l else -T)
        else:
            lo = start[7 * l] + cfg['EW6']
        hi = start[g] - LAG - 3
        save = SAVE.get(p) if l == 0 else None
        sv = save is not None
        if p == 1:
            for c, k in np.ndindex(NC, 2):
                add(lo, hi, 31 + 8 * sv, 7 + 8 * sv, 16, 2, l, functools.partial(unit1, l, c, k, save))
            continue
        nt = 2
        if p in (2, 6):
            mid = start[7 * l + 3] + cfg['MOFF']
            if p == 2:
                for c, k in np.ndindex(NC, 2):
                    add(lo, mid - 3, 40 + 8 * sv, 16 + 8 * sv, 32, 'O', l, functools.partial(unit26, l, c, k, save))
            lo, nt, save, sv = mid, 1, None, False
        for c in range(NQ):
            add(lo, hi if p in GUEST else first(g - 1, 'y') - LAG - 3, 32 * nt + 50 + 32 * sv, 18 + 32 * sv, 32 * nt,
                4, l, functools.partial(unit3, l, p, '26', c, save))
        for c in range(NQ):
            for kind in KINDS[:2]:
                add(lo, hi + (NC if g else 0), 16 * nt + 46, 14, 16 * nt, 3, l, functools.partial(unit3, l, p, kind, c, None))
    convs = [(R, Q, r) for R in range(4) for Q in range(4) for r in range(0, Mh, 32)]
    for x in convs:
        add(start[6], start[G - 2] - 2, 18, 7, 4, 1, 'conv', x)
    cap = [max(cfg['CAP'] - max(use[t], use[(t + 1) % T]), 0.0) * (t < T - cfg['TAIL']) for t in range(T)]
    when = spread_jobs(jobs, cap, [cfg['VK'] * (1 - vuse[(t + 1) % T]) for t in range(T)], cfg['TAIL'])
    plan = {}
    for t, _, ji, u in sorted((t % T, ts[0] % T, ji, u) for ji, ts in enumerate(when) for u, t in enumerate(ts)):
        plan.setdefault(t, []).append((jobs[ji][5], jobs[ji][6], STAGES[jobs[ji][4]][u][0]))
    carried = [job for ts, job in zip(when, jobs) if ts[0] < 0]

    def w_copy(l):
        return pltpu.make_async_copy(w_hbm.at[l], w_ref.at[l], sem.at[l])

    def w0_copy(u):
        return pltpu.make_async_copy(w_hbm.at[0, :, u], w_ref.at[0, :, u], sem.at[L + 6 + u])

    def in_copy(t, slot):
        return pltpu.make_async_copy(x_hbm.at[pl.ds(pl.multiple_of(t * TM, 32), TM)], xn2_ref.at[slot], sem.at[L + slot])

    def out_copy(t, slot, part):
        r0, nr = ((0, 2 * Mh), (2 * Mh, Mh), (3 * Mh, Mh), (0, TM))[part]
        return pltpu.make_async_copy(o2_ref.at[slot, pl.ds(r0, nr)],
                                     o_hbm.at[pl.ds(pl.multiple_of(t * TM + r0, 32), nr)], sem.at[L + 4 + slot])

    xr_in = pltpu.make_async_copy(x_hbm.at[pl.ds(NMAIN * TM, R0)], xr_ref, sem.at[L + 2])
    xr_out = pltpu.make_async_copy(xr_ref, o_hbm.at[pl.ds(NMAIN * TM, R0)], sem.at[L + 2])
    b_in = pltpu.make_async_copy(b_hbm, b_ref, sem.at[L + 3])
    opaque = lambda i, s: jax.lax.shift_right_logical(i, s)
    mask = lambda zero: {n: jnp.broadcast_to(zero, (n, 128)) != 0 for n in (8, 16, 32)}

    def prologue():
        b_in.start()
        for u in range(8):
            w0_copy(u).start()
        xr_in.start()
        in_copy(0, 0).start()
        for l in range(1, L):
            w_copy(l).start()
        in_copy(1, 1).start()
        b_in.wait()
        for l in range(L):
            bf_ref[l] = b_ref[l:l + 1, :].astype(f32)

        def bias_tiles(l, carry):
            b = jnp.broadcast_to(bf_ref[l] + (l == 0).astype(f32), (8, D))
            for u in sites.values():
                terms = [b[:, e * 128:(e + 1) * 128] * float(cf) for e, cf in enumerate(bcoef[u]) if cf != 0.0]
                bt_ref[l, u] = functools.reduce(lambda x, y: x + y, terms)
            return carry
        jax.lax.fori_loop(0, L, bias_tiles, 0)
        if cfg.get('FAST'):
            return

        def slab(u, carry):
            w0_copy(u).wait()
            prep(0, u, iter(lambda: None, 0), opaque(u, 12), kb0)
            return opaque(u, 12)
        zero = jax.lax.fori_loop(0, cfg['NSLAB'], slab, 0)

        def plain(l, xbf, x0f, x, j0, j1, na, free, never):
            passes = []
            for jt in range(j0, j1):
                cols = slice(jt * 128, (jt + 1) * 128)
                ya = _dot(xbf[:, :D // 2], w_ref[l, 0:4, :, :, cols].reshape(D // 2, 128)) + bf_ref[l, :, cols]
                passes += [ya, _dot(xbf[:, D // 2:], w_ref[l, 4:8, :, :, cols].reshape(D // 2, 128)) + ya]
            xp_ref[0, :, j0 * 128:j1 * 128] = x0f * jnp.concatenate(passes[1::2], axis=1) + x
            for u in range(na):
                ps, rr = divmod((u - free) * len(passes) * (R0 // 8) // (na - free), R0 // 8)
                yield None if u < free else (never, passes[ps][rr * 8:rr * 8 + 8, :])

        for u in range(cfg['NSLAB'], 8):
            w0_copy(u).wait()
        xr_in.wait()
        jm = cfg['JM']
        x0f = xr_ref[:, :jm * 128].astype(f32)
        xp_ref[1, :, :jm * 128] = x0f
        anchors = plain(0, xr_ref[...], x0f, x0f, 0, jm, (8 - cfg['NSLAB']) * NPREP, 2, mask(zero))
        for u in range(cfg['NSLAB'], 8):
            prep(0, u, anchors, zero, (kb0, kb1)[u % 2])
        in_copy(0, 0).wait()
        x0f = xr_ref[:, jm * 128:].astype(f32)
        xp_ref[1, :, jm * 128:] = x0f
        anchors = plain(0, xr_ref[...], x0f, x0f, jm, 8, len(convs) + sum(len(j[2]) for j in carried) + 2, 4, mask(zero))
        for x in convs[:len(convs) // 2]:
            conv(xn2_ref.at[0], *x, zero, next(anchors))
        for job in carried:
            st8 = {}
            for group, _ in STAGES[job[4]]:
                job[6](st8, group, zero, opaque(zero, 1), next(anchors))
        for x in convs[len(convs) // 2:]:
            conv(xn2_ref.at[0], *x, zero, next(anchors))

        def layer(l, carry):
            w_copy(l).wait()
            x, zero = xp_ref[0], opaque(l, 12)
            anchors = plain(l, x.astype(bf16), xp_ref[1], x, 0, 8, 8 * NPREP, 2, mask(zero))
            for u in range(8):
                prep(l, u, anchors, zero, (kb0, kb1)[u % 2])
            return carry

        jax.lax.fori_loop(1, L, layer, 0)
        xr_ref[...] = xp_ref[0].astype(bf16)
        xr_out.start()

    def main(tile, carry, only_late=False):
        zs, za = opaque(tile, 12), opaque(tile, 13)
        never = mask(zs)
        slot = tile % 2
        out = [o2_ref.at[1 - slot]]

        def rows(h, r0):
            lo, n = (0, Mh) if h is None else h if isinstance(h, tuple) else (h * Mq, Mq)
            return slice(r0 + lo, r0 + lo + n)

        def ld(loc, h):
            return loc[0][(0,) + loc[1] + (rows(h, loc[2]),)]

        def st(loc, v, h):
            loc[0][(zs,) + loc[1] + (rows(h, loc[2]),)] = v

        def operand(ref, idx, n):
            if cfg.get('NOBC'):
                return ref[idx + (slice(0, n),)]
            return pltpu.bitcast(ref.bitcast(u32)[idx + (slice(0, n // 2),)], bf16)

        def dot3(l, p, q, r):
            kind = next(x for x in KINDS if q in PAIR[x])
            return _dot(operand(s3[(p, kind)], (0, PAIR[kind].index(q), ORD.index(r)), Mq),
                        operand(t3_ref, (l, PRODS3.index((p, q)), ORD.index(r)), 128))

        def issue(l, p, rd):
            kind, n = rd
            if kind == 'x':
                return [dot3(l, p, q, 1) for q in (3, 5, 4, 7)]
            if kind == 'y':
                return [dot3(l, x, q, 1) for x in (p, GUEST[p]) for q in (2, 6)]
            if isinstance(n, str):
                return [dot3(l, p, int(q), int(r)) for q in kind for r in n]
            lhs = {q: [operand(s2[p], (0, k, pos2(p, q)), Mh) for k in range(2)] for q in map(int, kind)}
            return [_dot(lhs[q][k], operand(t2[p], (l, nn, k, pos2(p, q)), 128))
                    for q, nn in ([(1, 0), (1, 1)] if kind == '1' else [(int(q), n) for q in kind]) for k in range(2)]

        def biased(v, l, *site):
            if site not in sites:
                return v
            return (v.reshape(Mq // 8, 8, 128) + bt_ref[l, sites[site]]).reshape(Mq, 128)

        wait = {}
        def outer_act(l, p, i, j, n, d, h, part=None):
            stores, finals = OACT[p]
            if part == 'park':
                stores, finals = stores[:1], []
            elif part == 'rest' or (p == 6 and (i, j) != B12 and (h, n) != B12):
                stores = stores[1:]
            cache = {'d': d}
            def comb(terms):
                for t in terms.split():
                    if t[1:] not in cache:
                        cache[t[1:]] = ld(oloc(t[1:], i, j, n), h)
                return lincomb([(int(t[0] + '1'), cache[t[1:]]) for t in terms.split()])
            fin = [(IJ, comb(terms)) for IJ, terms in finals]
            for name, v in [(name, comb(terms)) for name, terms in stores]:
                st(oloc(name, i, j, n), v, h)
            for (I, J), y in fin:
                R, C = 2 * I + i, 2 * J + j
                xn = ld(x0loc(R, C, n), h) * y
                if l > 0:
                    xn = xn + ld(xloc(l, R, C, n), h)
                if l < L - 1:
                    st(xloc(l + 1, R, C, n), xn, h)
                    continue
                s = scale(R, C, rows(h, 0).start // Mq, n)
                xn = xn if s == 1.0 else xn * (1.0 / s)
                c0 = phys(C, n) * 128
                if i == 0:
                    out[0][rows(h, R * Mh), c0:c0 + 128] = xn.astype(bf16)
                elif j == 1:
                    wait[J] = xn
                else:
                    out[0][rows(h, R * Mh), c0:c0 + 256] = jnp.concatenate([xn, wait.pop(J)], axis=1).astype(bf16)

        def inner_act(g, l, p, kind, n, h, P, Q, part=None):
            vloc = iloc(g, 'v', n) if p == 1 else oloc(OACT[p][0][0][0], 0, 1, n)
            if kind == '35':
                st(iloc(g, 's', n), Q + ld(iloc(g, 'm1', n), h), h)
                if p == 1:
                    st(vloc, P, h)
                outer_act(l, p, 0, 1, n, P, h, part)
            elif kind == '47':
                st(iloc(g, 'u', n), Q + ld(vloc, h), h)
                outer_act(l, p, 0, 0, n, P + ld(iloc(g, 's', n), h), h, part)
            else:
                outer_act(l, p, 1, 1, n, ld(iloc(g, 's', n), h) - Q, h, part)
                outer_act(l, p, 1, 0, n, P + ld(iloc(g, 'u', n), h), h, part)

        def consume(g, l, p, rd, res):
            kind, n = rd
            if n == '1':
                for u, (kd, x) in enumerate([('35', p), ('47', p)] if kind == 'x' else [('26', p), ('26', GUEST[p])]):
                    for al in range(2):
                        st(jloc(kd, '1', al, x != p), biased(res[2 * u + al], l, x, int(kd[al]), '1'), 0)
            elif isinstance(n, str):
                sm = [res[2 * al] + res[2 * al + 1] for al in range(2)]
                df = [res[2 * al] - res[2 * al + 1] for al in range(2)]
                J = lambda name, al: ld(jloc(kind, name, al, name == '1' and kind == '26' and p not in GUEST), 0)
                part = 'park' if deferred(l, p, rd) else None
                done = lambda h, nn, m: inner_act(g, l, p, kind, nn, h, m[0] + m[1], m[0] - m[1], part)
                if n == '35':
                    for al in range(2):
                        st(jloc(kind, 's', al), df[al] + J('1', al), 0)
                    done(0, 1, [biased(sm[al], l, p, int(kind[al]), 'v') for al in range(2)])
                elif n == '47':
                    for al in range(2):
                        st(jloc(kind, 'k', al), biased(df[al], l, p, int(kind[al]), 'k'), 0)
                    done(0, 0, [biased(sm[al] + J('s', al), l, p, int(kind[al]), 'm') for al in range(2)])
                else:
                    O = lambda i, j: ld(oloc(OACT[p][0][0][0], i, j, 1), 0)
                    m = [sm[al] + J('k', al) for al in range(2)]
                    P = m[0] + m[1] + O(*{'35': B12, '47': B11, '26': B21}[kind])
                    Q = m[0] - m[1] - (ld(iloc(g, 'm1', 1), 0) if kind == '35' else O(*{'47': B12, '26': B22}[kind]))
                    done(1, 1, [J('s', al) - df[al] for al in range(2)])
                    inner_act(g, l, p, kind, 0, 1, P, Q, part)
            else:
                m = []
                for al, (q, nn) in enumerate([(1, 0), (1, 1)] if kind == '1' else [(int(q), n) for q in kind]):
                    v = res[2 * al] + res[2 * al + 1]
                    if any((p, q, (h, nn)) in sites for h in range(2)):
                        v = jnp.concatenate([biased(v[h * Mq:(h + 1) * Mq], l, p, q, (h, nn)) for h in range(2)], axis=0)
                    m.append(v)
                if kind == '1':
                    for nn in range(2):
                        st(iloc(g, 'm1', nn), m[nn], None)
                else:
                    inner_act(g, l, p, kind, n, None, m[0] + m[1], m[0] - m[1])

        def finish(l, p, pieces, nr, anchor):
            for i, j, n, r0 in pieces:
                d = ld(oloc(OACT[p][0][0][0], i, j, n), (r0, nr))
                outer_act(l, p, i, j, n, tie(d, anchor), (r0, nr), 'rest')

        if only_late:
            for x in late:
                finish(*x, None)
            out_copy(tile - 1, 1 - slot, 2).start()
            return carry
        state = {}
        count.clear()
        for g, rd, t0, n in sched:
            l, p = outs[g]
            if t0 == start[1]:
                pl.when(tile > 0)(lambda: out_copy(tile - 1, 1 - slot, 2).start())
                out[0] = o2_ref.at[slot]
            if t0 == start[G - 1]:
                out_copy(tile, slot, 0).start()
            res = issue(l, p, rd)
            for t in range(t0, t0 + n):
                if t in plan:
                    r0 = 16 * (t - t0) + 8
                    anchor = (never, res[0 if isinstance(rd[1], str) else 1][r0:r0 + 8, :])
                for kind, fn, group in plan.get(t, []):
                    if kind == 'fin':
                        finish(*fn, anchor)
                    elif kind == 'conv':
                        conv(xn2_ref.at[1 - slot], *fn, zs, anchor)
                    else:
                        fn(state.setdefault(id(fn), {}), group, zs, za, anchor)
            if t0 + n == T:
                out_copy(tile, slot, 1).start()
            consume(g, l, p, rd, res)
        pl.when(tile + 3 < NMAIN)(lambda: in_copy(tile + 3, 1 - slot).start())
        pl.when(tile > 0)(lambda: out_copy(tile - 1, 1 - slot, 3).wait())
        pl.when(tile + 2 < NMAIN)(lambda: in_copy(tile + 2, slot).wait())
        return carry

    prologue()
    in_copy(2, 0).start()
    in_copy(1, 1).wait()
    jax.lax.fori_loop(0, NMAIN, main, 0)
    main(jnp.int32(NMAIN), 0, True)
    xr_out.wait()
    out_copy(NMAIN - 1, (NMAIN - 1) % 2, 3).wait()


def build(TM=640, **kw):
    def f(x0, ws, bs):
        B, D = x0.shape
        L = ws.shape[0]
        Mh = TM // 4
        nmain = (B - 1) // TM
        R0 = B - nmain * TM
        assert D == 1024 and L % 2 == 0 and L <= 8 and TM % 128 == 0 and R0 % 16 == 0 and nmain >= 3
        n3 = len(PRODS3)
        odd = lambda n: 16 * (n // 16 | 1)
        V = pltpu.VMEM
        scratch = ([V((1, 2, 2, 2, Mh + 40, 128), f32)] * 4 + [V((1, 2, 4, 2, Mh + 40, 128), f32)] * 7
                   + [V((1, Mh + 32, 128), f32)] * (16 + 64 + 20)
                   + [V((1, 2, 10 if p == 1 else 2, odd(Mh), 128), bf16) for p in range(1, 8)]
                   + [V((1, 2, 10, odd(Mh // 2), 128), bf16)] * (n3 // 2)
                   + [V((L, 2, 2, 7 if p == 1 else 1, 128, 128), bf16) for p in range(1, 8)]
                   + [V((L, n3, 7, 128, 128), bf16)] + [V((1, 4, 16 * n3 + 16, 128), f32)] * 2
                   + [V((L, 64, 8, 128), f32), V((8, 1, D), f32), V((2, TM, D), bf16), V((2, TM, D), bf16),
                      V((L, 8, 8, 16, D), bf16), V((R0, D), bf16), V((2, R0, D), f32), V((L, D), bf16),
                      pltpu.SemaphoreType.DMA((L + 14,))])
        anyspec = pl.BlockSpec(memory_space=pl.ANY)
        return pl.pallas_call(
            functools.partial(_kernel, L=L, TM=TM, R0=R0, NMAIN=nmain, D=D, cfg=dict(CFG, **kw)),
            in_specs=[anyspec, anyspec, anyspec],
            out_specs=anyspec,
            out_shape=jax.ShapeDtypeStruct((B, D), x0.dtype),
            scratch_shapes=scratch,
            compiler_params=pltpu.CompilerParams(
                vmem_limit_bytes=120 * 1024 * 1024,
                internal_scratch_in_bytes=65536,
                disable_bounds_checks=True,
            ),
        )(x0, ws.reshape(L, 8, 8, 16, D), bs)
    return f


@jax.jit
def pallas_standalone__dcn_v2_cross__recsys_kernel(x0, ws, bs):
    return build()(x0, ws, bs)
```

```python
import functools

import jax
import jax.numpy as jnp
import numpy as np
import jax.experimental.pallas as pl
import jax.experimental.pallas.tpu as pltpu

f32 = jnp.float32
bf16 = jnp.bfloat16
u32 = jnp.uint32

B11, B12, B21, B22 = BLOCKS = (0, 0), (0, 1), (1, 0), (1, 1)
LA = {1: [(B11, 1), (B22, 1)], 3: [(B11, 1), (B12, -1)], 5: [(B11, 1), (B12, 1)], 4: [(B12, 1), (B22, 1)],
      7: [(B12, 1), (B22, -1)]}
PC = {1: (1, 0, 0, 1), 2: (0, 0, 1, -1), 3: (1, 1, 1, 1), 4: (1, 0, 1, 0), 5: (-1, 1, 1, -1), 6: (0, 0, 1, 1),
      7: (1, 0, -1, 0)}
KINDS = ('35', '47', '26')
PAIR = {'35': (5, 3), '47': (4, 7), '26': (2, 6)}
ORD = (3, 5, 4, 7, 1, 2, 6)
OUTER = (3, 5, 1, 4, 7, 2, 6)
GUEST = {3: 5, 4: 7, 2: 6}
PRODS3 = [(p, q) for p in OUTER if p != 1 for kind in KINDS for q in PAIR[kind]]
GAMMA = 0.125
OACT = {
    3: ([('M3', '+d')], []),
    5: ([('M5', '+d')], [(B12, '+d +M3')]),
    1: ([('S', '+d +M3 -M5')], []),
    4: ([('M4', '+d')], []),
    7: ([('M7', '+d')], [(B11, '+d +S +M4')]),
    2: ([('M2', '+d'), ('U', '+d +M4 -M7 +M3 +M5')], []),
    6: ([('M6', '+d')], [(B22, '+d +S -M2'), (B21, '+d +U')]),
}
OSL = {'M3': 0, 'M5': 1, 'S': 2, 'M4': 3, 'M7': 4, 'U': 5, 'M2': 6, 'M6': 7}
ISL = {'m1': 0, 's': 1, 'v': 2, 'u': 3}
DEFER = {5: [('26', '26'), ('47', '26')], 7: [('26', '26'), ('47', '26')], 2: [('47', '26'), ('26', '26')],
         6: [('35', '26'), ('47', '26'), ('26', '26'), ('26', '35')]}
SAVE = {5: B12, 1: B11, 7: B22, 2: B21}
STAGES = {1: [(None, 1.0)], 2: [((B11, B12), .4), ((B21, B22), .6)], 'O': [((B11, B12), .5), ((B21, B22), .5)],
          3: [((B11, B12), .35), ((B22,), .37), ((B21,), .28)],
          4: [((B11,), .16), ((B12,), .26), ((B22,), .31), ((B21,), .27)]}
LAG = 8
CFG = dict(CAP=0.95, PORT=0.9, CS=0.5, CL=0.3, VK=0.75, TAIL=3, EW7=12, EW6=25, MOFF=15, GE=8, NSLAB=6, JM=3)


def _dot(a, b):
    return jnp.dot(a, b, preferred_element_type=f32)


def scale(R, C, h, k):
    return 2.0 ** (R // 2 + R % 2 + h - C // 2 - C % 2 - k)


def phys(C, k):
    return 4 * (C // 2) + 2 * k + C % 2


def b_ops(b11, b12, b21, b22):
    r1 = b11 + b22
    g = b12 + b21
    return {1: r1, 2: b11 - b12, 3: b12 - b22, 4: g - r1, 5: b12 + b22, 6: b11 + b12, 7: g + r1}


def lincomb(terms):
    assert terms[0][0] == 1
    acc = terms[0][1]
    for s, v in terms[1:]:
        acc = acc + v if s == 1 else acc - v
    return acc


def rounds_of(p):
    if p == 1:
        return [('1', None)] + [(kind, n) for kind in KINDS for n in range(2)]
    minis = lambda kind: [(kind, r) for r in KINDS]
    return [('1', None), ('x', '1')] + minis('35') + minis('47') + [('y', '1')] * (p in GUEST) + minis('26')


def round_usage(p, rd, first, last, defer):
    stores, finals = OACT[p]
    kind, n = rd
    alu = sum(len(t.split()) - 1 for _, t in stores) + sum(len(t.split()) + (not first) + 2 * last for _, t in finals)
    nst = len(stores) + len(finals)
    if last and kind == '26':
        alu, nst = alu - 0.7 * len(finals), nst - 0.5 * len(finals)
    if defer:
        alu, nst = 0, 1
    elif p == 6 and kind != '35' and n != '35':
        nst -= 1
    if n == '1':
        a, st, m = 0, 4, 0
    elif isinstance(n, str):
        a, st, m = {'35': ((9, 3, 1), (16, 2, 2)), '47': ((10, 3, 1), (18, 2, 2)), '26': ((10, 2, 2), (18, 0, 4))}[kind][n == '26']
    else:
        a, st, m = {'1': (2, 2, 0), '35': (5, 2, 1), '47': (6, 1, 1), '26': (6, 0, 2)}[kind]
    return a + m * alu, st + m * nst


def bias_sites():
    cand = []
    for p in OUTER:
        for rd in rounds_of(p):
            kind, n = rd
            if n == '1':
                pq = [(p, q) for q in (3, 5, 4, 7)] if kind == 'x' else [(x, q) for x in (p, GUEST[p]) for q in (2, 6)]
                cand += [(p, rd, x + ('1',), (1, 0, 0, 1)) for x in pq]
            elif n in ('35', '47'):
                where = [('v', (0, 1, 1, 0))] if n == '35' else [('k', (0, 0, 1, 0)), ('m', (1, 0, 0, 0))]
                cand += [(p, rd, (p, int(q), w), pat) for q in kind for w, pat in where]
            elif n != '26':
                cand += [(p, rd, (p, int(q), (h, nn)), tuple(int(e == 2 * h + nn) for e in range(4)))
                         for q in kind for nn in ((0, 1) if kind == '1' else (n,)) for h in range(2)]
    extra, sites, rows = {}, [], []
    def busy(c):
        a, st = round_usage(c[0], c[1], False, False, c[1] in DEFER.get(c[0], ()))
        return 2 * (a + extra.get(c[:2], 0)) + st + (5 if isinstance(c[1][1], str) else 3)
    while len(sites) < 64:
        c = min(cand, key=busy)
        cand.remove(c)
        row = np.kron(np.kron(PC[c[2][0]], PC[c[2][1]]), c[3])
        if np.linalg.matrix_rank(np.array(rows + [row])) > len(rows):
            rows.append(row)
            sites.append(c[2])
            extra[c[:2]] = extra.get(c[:2], 0) + (1 if isinstance(c[1][1], str) else 0.5)
    want = np.zeros((64, 8))
    for e, (I, J, i, j, h, n) in enumerate(np.ndindex(*(2,) * 6)):
        want[e, phys(2 * J + j, n)] = scale(2 * I + i, 2 * J + j, h, n) / GAMMA
    coef = np.round(np.linalg.solve(np.array(rows, float).T, want) * 4096) / 4096
    assert (np.array(rows).T @ coef == want).all()
    return {x: e for e, x in enumerate(sites) if coef[e].any()}, coef, extra


def yds(groups, cap):
    n = len(cap)
    speed, cls, gcls = [0.0] * n, [-1] * n, {}
    todo = list(groups)
    while todo:
        pre = [0.0]
        for t in range(n):
            pre.append(pre[-1] + (cap[t] if cls[t] < 0 else 0.0))
        best = None
        for a in sorted({g[0] for g in todo}):
            w = 0.0
            for g in sorted((g for g in todo if g[0] >= a), key=lambda g: g[1]):
                w += g[2]
                d = w / max(pre[g[1] + 1] - pre[a], 1e-9)
                if best is None or d > best[0]:
                    best = (d, a, g[1])
        d, a, b = best
        for t in range(a, b + 1):
            if cls[t] < 0:
                speed[t], cls[t] = d, len(gcls)
        gcls.update({g[:2]: len(gcls) for g in todo if g[0] >= a and g[1] <= b})
        todo = [g for g in todo if not (g[0] >= a and g[1] <= b)]
    return speed, cls, gcls


def spread_jobs(jobs, cap, vcap, tail):
    T = len(cap)
    cap3 = cap * 3
    all3 = [(j[0] + k * T, j[1] + k * T, ji, k) for k in range(3) for ji, j in enumerate(jobs) if j[0] + k * T >= 0]
    pend = {}
    for j in sorted(all3, key=lambda j: (j[1], j[3], j[2])):
        pend.setdefault(j[:2], []).append(j)
    left = {w: sum(sum(jobs[j[2]][2]) for j in q) for w, q in pend.items()}
    speed, cls, gcls = yds([w + (left[w],) for w in pend], cap3)
    cum = [0.0]
    for t in range(3 * T):
        cum.append(cum[-1] + speed[t] * cap3[t])
    when = [[] for _ in jobs]
    debt, vdebt, cur, done = 0.0, 0.0, None, 0

    def fits(j, t):
        need = max(debt, 0.0) + sum(jobs[j[2]][2]) + 1.0
        for w in pend:
            if w[1] >= j[1]:
                break
            if left[w] > 1e-9:
                need += left[w]
                if need > cum[w[1] + 1] - cum[t]:
                    return False
        return True

    for t in range(3 * T):
        if t % T == 0:
            debt, vdebt = min(debt, 0.0), -0.5
        while True:
            rdy = [q[0] for w, q in pend.items() if q and w[0] <= t and (gcls[w] == cls[t] or w[1] <= t)]
            j = cur
            if j is None:
                if not rdy:
                    debt = max(debt, 0.0)
                    break
                j = rdy[0]
                if j[1] > t:
                    j = (min if vdebt > 0 else max)([x for x in rdy if x is j or fits(x, t)], key=lambda x: jobs[x[2]][3])
                nst = len(jobs[j[2]][2])
                if nst > 1 and j[1] > t and (t + tail + 2 * nst) // T != t // T:
                    break
            must = j[1] <= t or (cur is not None and ((t + tail + 1) // T != t // T or (rdy and rdy[0][1] <= t)))
            if not must and (cap3[t] == 0.0 or debt > 0.5 * speed[t] * cap3[t]):
                break
            if cur is None:
                pend[j[:2]].pop(0)
                left[j[:2]] -= sum(jobs[j[2]][2])
                cur, done = j, 0
            debt += jobs[j[2]][2][done]
            vdebt += jobs[j[2]][2][done] * jobs[j[2]][3]
            if j[3] == 1:
                when[j[2]].append(t - T)
            done += 1
            if done == len(jobs[j[2]][2]):
                cur = None
        debt -= speed[t] * cap3[t]
        vdebt = min(max(vdebt - vcap[t % T], -0.5), 1.0)
    assert all(j[0] <= ts[0] and ts[-1] <= j[1] and (ts[0] < 0) == (ts[-1] < 0) for j, ts in zip(jobs, when))
    return when


def _kernel(x_hbm, w_hbm, b_hbm, o_hbm, *scratch, L, TM, R0, NMAIN, D, cfg):
    H, Mh, Mq = D // 4, TM // 4, TM // 8
    NC, NQ = Mh // 16, Mq // 16
    it = iter(scratch)
    take = lambda n: [next(it) for _ in range(n)]
    x0b, xb, ib, ob, jb = take(4), take(7), take(16), take(64), take(20)
    s2 = dict(zip(range(1, 8), take(7)))
    s3 = {(p, kind): next(it) for p in OUTER if p != 1 for kind in KINDS}
    t2 = dict(zip(range(1, 8), take(7)))
    t3_ref, kb0, kb1, bt_ref, bf_ref, xn2_ref, o2_ref, w_ref, xr_ref, xp_ref, b_ref, sem = it
    sites, bcoef, extra = bias_sites()
    pos2 = lambda p, q: ORD.index(q) if p == 1 else 0

    xset = lambda l: 6 if l == 'O' else 4 if l == 0 else (l % 2) * 2
    xoff = lambda I, J: 16 * ((I + J) % 2)
    xloc = lambda l, R, C, k: (xb[xset(l) + R // 2], (R % 2, C, k), xoff(R // 2, C // 2))
    x0loc = lambda R, C, k: (x0b[(R // 2) * 2 + C // 2], (R % 2, C % 2, k), 8 + xoff(R // 2, C // 2))
    iloc = lambda g, name, n: (ib[((g % 2) * 4 + ISL[name]) * 2 + n], (), 8 * ISL[name])
    oloc = lambda name, i, j, n: (ob[(OSL[name] * 4 + i * 2 + j) * 2 + n], (), 8 * ((OSL[name] + 2 * j) % 4))

    def jloc(kind, name, al, guest=False):
        u = ('1', 's', 'k').index(name)
        return jb[18 + al if guest else (KINDS.index(kind) * 3 + u) * 2 + al], (), 8 * ((3 * u + al) % 4)

    def tie(v, anchor, r=None, lo=0):
        if anchor is None:
            return v
        never, gate = anchor
        if r is None:
            n = v.shape[0]
            return jax.lax.select(never[n], gate if n == 8 else jnp.tile(gate, (n // 8, 1)), v)
        top = jax.lax.select(never[8], gate, v[r:r + 8])
        return jnp.concatenate(([v[lo:r]] if r > lo else []) + [top, v[r + 8:r + 16]], axis=0)

    def consts(anchor, ss):
        one = {s: tie(jnp.full((8, 128), s, f32), anchor) for s in set(ss)}
        return jnp.concatenate([one[s] for s in ss for _ in range(2)], axis=0)

    def conv(src, R, Q, r, zs, anchor):
        v = src[R * Mh + r:R * Mh + r + 32, Q * H:(Q + 1) * H].astype(f32)
        for j in range(2):
            C, k = 2 * (Q // 2) + j, Q % 2
            buf, idx, off = xloc(0, R, C, k)
            sv = consts(anchor, [scale(R, C, (r + u) // Mq, k) for u in (0, 16)])
            buf[(zs,) + idx + (slice(off + r, off + r + 32),)] = v[:, j * 128:(j + 1) * 128] * sv

    count = {}
    def block_sum(l, terms, ii, jj, kk, r, save, zs, za, anchor, gate=True):
        rng = lambda t: slice(t[0], t[-1] + 1)
        vals = []
        for u, ((I, J), s) in enumerate(terms):
            ref, r0 = xb[xset(l) + I], xoff(I, J) + r
            v = ref[za if u == 0 else 0, rng(ii), 2 * J + jj[0]:2 * J + jj[-1] + 1, rng(kk), r0:r0 + 16, :]
            if (I, J) == save:
                sv = consts(anchor, [GAMMA / scale(2 * I + i, 2 * J + j, r // Mq, k) for i in ii for j in jj for k in kk])
                x0b[I * 2 + J][zs, rng(ii), rng(jj), rng(kk), r0 + 8:r0 + 24, :] = v * sv.reshape(v.shape)
            if u == 0 and gate:
                count[xset(l)] = count.get(xset(l), -1) + 1
                if count[xset(l)] % cfg['GE'] == 0:
                    ref[0, 0, 0, 0, Mh + 24:Mh + 32, :] = anchor[1]
            vals.append((s, v))
        v = lincomb(vals)
        return v.reshape(v.size // 128, 128)

    def operands(a, group, st8, store):
        for u, b in enumerate(group):
            st8[b] = a if len(group) == 1 else a[:, u:u + 1]
        ops = {}
        if B12 in group:
            ops[3], ops[5] = st8[B11] - st8[B12], st8[B11] + st8[B12]
        if B22 in group:
            ops[4], ops[7] = st8[B12] + st8[B22], st8[B12] - st8[B22]
            ops[1] = st8['l1'] = st8[B11] + st8[B22]
        if B21 in group:
            g = st8[B12] + st8[B21]
            ops[2], ops[6] = g + st8['l1'], g - st8['l1']
        now = [q for q in ORD if q in ops]
        if now:
            u = ORD.index(now[0])
            store(slice(u, u + len(now)), jnp.concatenate([ops[q] for q in now], axis=1).astype(bf16))

    def unit1(l, c, k, save, st8, group, zs, za, anchor):
        def store(pos, v):
            s2[1][zs, k:k + 1, pos, 16 * c:16 * c + 16, :] = v
        e = block_sum(l, LA[1], [group[0][0]], [0, 1], [k], 16 * c, save, zs, za, anchor)
        operands(tie(e, anchor, 16).reshape(1, 2, 16, 128), group, st8, store)

    def unit26(l, c, k, save, st8, group, zs, za, anchor):
        i = group[0][0]
        f = block_sum(l, [(B11, 1), (B22, 1)], [i], [0, 1], [k], 16 * c, save, zs, za, anchor, False)
        e = tie(block_sum(l, [(B12, 1), (B21, 1)], [i], [0, 1], [k], 16 * c, save, zs, za, anchor), anchor)
        for J, v in enumerate((e + f, e - f)):
            r0 = xoff(0, J) + 16 * c
            xb[6][zs, i, 2 * J:2 * J + 2, k, r0:r0 + 16, :] = v.reshape(2, 16, 128)

    def unit3(l, p, kind, c, save, st8, group, zs, za, anchor):
        def store(pos, v):
            s3[(p, kind)][zs, :, pos, 16 * c:16 * c + 16, :] = v
        h, kk = group[0][0], [b[1] for b in group]
        ii, jj = {'35': ([0], [0, 1]), '47': ([0, 1], [1]), '26': ([0, 1], [0, 1])}[kind]
        src = (l, LA[p]) if p in LA else ('O', [((0, (2, 6).index(p)), 1)])
        n = 16 * len(kk)
        v = block_sum(*src, ii, jj, kk, h * Mq + 16 * c, save, zs, za, anchor)
        if kind == '26':
            e, f = tie(v, anchor, 16, 16) + v[32:48], v[0:16] + v[48:64]
            r0 = h * Mq + 16 * c
            s2[p][zs, kk[0], 0, r0:r0 + 16, :] = f.astype(bf16)
        else:
            e, f = tie(v, anchor, n - 16), v[n:]
        operands(jnp.concatenate([e + f, e - f], axis=0).reshape(2, len(kk), 16, 128), group, st8, store)

    NPREP = 32 + len(PRODS3)
    def prep(l, u, anchors, zero, kb):
        mul = lambda v, s: v if s == 1.0 else v * s
        stack = lambda T: jnp.concatenate([T[q] for q in ORD], axis=0).reshape(7, 16, 128).astype(bf16)
        rows = pl.ds(16 * u, 16) if isinstance(u, int) else pl.ds(pl.multiple_of(16 * u, 16), 16)
        for k in range(2):
            wide = [w_ref[l, phys(R, k), u].astype(f32) for R in range(4)]
            for n in range(2):
                anchor = next(anchors)
                blk = lambda R, C: mul(wide[R][:, phys(C, n) * 128:(phys(C, n) + 1) * 128], scale(R, C, k, n))
                O = {(i, j): b_ops(blk(i, j), tie(blk(i, 2 + j), anchor, 0), blk(2 + i, j), blk(2 + i, 2 + j))
                     for i, j in BLOCKS}
                for p in (2, 6, 3, 5, 1, 4, 7):
                    o = [mul(O[b][p], 4.0 if p == 1 else 1.0) for b in BLOCKS]
                    T = b_ops(o[0], tie(o[1], next(anchors), 0), o[2], o[3])
                    if p == 1:
                        T[1] = T[1] * 2.0
                        t2[p][l, n, k, :, rows, :] = stack(T)
                        continue
                    t2[p][l, n, k, 0, rows, :] = (T[1] * 4.0).astype(bf16)
                    e0 = PRODS3.index((p, 5))
                    if (k, n) != (1, 1):
                        kb[zero, k * 2 + n, 16 * e0:16 * e0 + 96, :] = jnp.concatenate(
                            [T[q] for _, q in PRODS3[e0:e0 + 6]], axis=0)
                        continue
                    for e in range(e0, e0 + 6):
                        v = kb[0, 0:3, 16 * e:16 * e + 16, :]
                        T3 = b_ops(v[0], tie(v[1], next(anchors), 0), v[2], T[PRODS3[e][1]])
                        T3[1] = T3[1] * 2.0
                        t3_ref[l, e, :, rows, :] = stack(T3)

    def deferred(l, p, rd):
        if l == L - 1 and p == 6 and rd[0] == '26':
            return rd[1] == '26'
        return rd in DEFER.get(p, ())

    outs = [(l, p) for l in range(L) for p in OUTER]
    G = len(outs)
    sched, start, use, vuse = [], [], [], []
    for g, (l, p) in enumerate(outs):
        start.append(len(use))
        for rd in rounds_of(p):
            n = NQ if isinstance(rd[1], str) else NC
            sched.append((g, rd, len(use), n))
            a, st_ = round_usage(p, rd, l == 0, l == L - 1, deferred(l, p, rd))
            a += extra.get((p, rd), 0)
            use += [max((2 * a + st_ + 2 + 16 / n) / 72, cfg['PORT'] * st_ / 8)] * n
            vuse += [st_ / 8] * n
    T = len(use)
    first = lambda g, kind: next(t0 for gg, rd, t0, _ in sched if gg == g and rd[0] == kind)
    jobs, late = [], []
    def add(lo, hi, alu, st_, ld_, scheme, kind, fn):
        w = alu / 64 + cfg['CS'] * (st_ + len(STAGES[scheme])) / 16 + cfg['CL'] * ld_ / 48
        jobs.append((lo, max(hi, lo), [w * f for _, f in STAGES[scheme]], st_ / 16 / w, scheme, kind, fn))
    for g, (l, p) in enumerate(outs):
        for gg, rd, t0, n_ in sched:
            if gg == g and deferred(l, p, rd):
                last = l == L - 1
                nops = 4 * (sum(len(t.split()) for _, t in OACT[p][0][1:]) + sum(len(t.split()) + 2 + 2 * last for _, t in OACT[p][1]))
                ws = [(i, j, n, h * Mq + 16 * c) for c in range(NQ)
                      for h, n in {'35': [B12], '47': [B11], '26': [B22, B21]}[rd[1]]
                      for i, j in {'35': [B12], '47': [B11], '26': [B22, B21]}[rd[0]]]
                if t0 + n_ == T:
                    for u in range(0, len(ws), 2):
                        for r8 in (0, 8):
                            late.append((l, p, [w[:3] + (w[3] + r8,) for w in ws[u:u + 2]], 8))
                            add(0, cfg['EW6'] - 1, nops * 0.45, 1, nops * 0.4, 1, 'fin', late[-1])
                    continue
                due = {5: lambda: start[7 * l + 5] - 1, 2: lambda: first(g + 1, rd[0]) - 3,
                       7: lambda: start[g + 2] - 1 if last else start[g + 1] + cfg['EW7'],
                       6: lambda: T - cfg['TAIL'] - 1 if last else start[g + 1] + cfg['EW6'] - 1}[p]()
                m = 1 if p == 6 else 2
                for u in range(0, len(ws), m):
                    add(t0 + n_, due, nops * m // 2, 3, nops * m // 2, 1, 'fin', (l, p, ws[u:u + m], 16))
        if p in (3, 5):
            lo = start[7 * l - 2] + (cfg['EW7'] + 1 if l else -T)
        else:
            lo = start[7 * l] + cfg['EW6']
        hi = start[g] - LAG - 3
        save = SAVE.get(p) if l == 0 else None
        sv = save is not None
        if p == 1:
            for c, k in np.ndindex(NC, 2):
                add(lo, hi, 31 + 8 * sv, 7 + 8 * sv, 16, 2, l, functools.partial(unit1, l, c, k, save))
            continue
        nt = 2
        if p in (2, 6):
            mid = start[7 * l + 3] + cfg['MOFF']
            if p == 2:
                for c, k in np.ndindex(NC, 2):
                    add(lo, mid - 3, 40 + 8 * sv, 16 + 8 * sv, 32, 'O', l, functools.partial(unit26, l, c, k, save))
            lo, nt, save, sv = mid, 1, None, False
        for c in range(NQ):
            add(lo, hi if p in GUEST else first(g - 1, 'y') - LAG - 3, 32 * nt + 50 + 32 * sv, 18 + 32 * sv, 32 * nt,
                4, l, functools.partial(unit3, l, p, '26', c, save))
        for c in range(NQ):
            for kind in KINDS[:2]:
                add(lo, hi + (NC if g else 0), 16 * nt + 46, 14, 16 * nt, 3, l, functools.partial(unit3, l, p, kind, c, None))
    convs = [(R, Q, r) for R in range(4) for Q in range(4) for r in range(0, Mh, 32)]
    for x in convs:
        add(start[6], start[G - 2] - 2, 18, 7, 4, 1, 'conv', x)
    cap = [max(cfg['CAP'] - max(use[t], use[(t + 1) % T]), 0.0) * (t < T - cfg['TAIL']) for t in range(T)]
    when = spread_jobs(jobs, cap, [cfg['VK'] * (1 - vuse[(t + 1) % T]) for t in range(T)], cfg['TAIL'])
    plan = {}
    for t, _, ji, u in sorted((t % T, ts[0] % T, ji, u) for ji, ts in enumerate(when) for u, t in enumerate(ts)):
        plan.setdefault(t, []).append((jobs[ji][5], jobs[ji][6], STAGES[jobs[ji][4]][u][0]))
    carried = [job for ts, job in zip(when, jobs) if ts[0] < 0]

    def w_copy(l):
        return pltpu.make_async_copy(w_hbm.at[l], w_ref.at[l], sem.at[l])

    def w0_copy(u):
        return pltpu.make_async_copy(w_hbm.at[0, :, u], w_ref.at[0, :, u], sem.at[L + 6 + u])

    def in_copy(t, slot):
        return pltpu.make_async_copy(x_hbm.at[pl.ds(pl.multiple_of(t * TM, 32), TM)], xn2_ref.at[slot], sem.at[L + slot])

    def out_copy(t, slot, part):
        r0, nr = ((0, 2 * Mh), (2 * Mh, Mh), (3 * Mh, Mh), (0, TM))[part]
        return pltpu.make_async_copy(o2_ref.at[slot, pl.ds(r0, nr)],
                                     o_hbm.at[pl.ds(pl.multiple_of(t * TM + r0, 32), nr)], sem.at[L + 4 + slot])

    xr_in = pltpu.make_async_copy(x_hbm.at[pl.ds(NMAIN * TM, R0)], xr_ref, sem.at[L + 2])
    xr_out = pltpu.make_async_copy(xr_ref, o_hbm.at[pl.ds(NMAIN * TM, R0)], sem.at[L + 2])
    b_in = pltpu.make_async_copy(b_hbm, b_ref, sem.at[L + 3])
    opaque = lambda i, s: jax.lax.shift_right_logical(i, s)
    mask = lambda zero: {n: jnp.broadcast_to(zero, (n, 128)) != 0 for n in (8, 16, 32)}

    def prologue():
        b_in.start()
        for u in range(8):
            w0_copy(u).start()
        xr_in.start()
        in_copy(0, 0).start()
        for l in range(1, L):
            w_copy(l).start()
        in_copy(1, 1).start()
        for j, n in BLOCKS:
            for ref, idx, off in ([oloc(x, 1, j, n) for x in ('S', 'M2', 'U', 'M6')]
                                  + [f(3, 2 * J + j, n) for J in range(2) for f in (x0loc, functools.partial(xloc, L - 1))]):
                ref[(0,) + idx + (slice(off + Mq, off + Mh),)] = jnp.zeros((Mq, 128), f32)
        b_in.wait()
        for l in range(L):
            bf_ref[l] = b_ref[l:l + 1, :].astype(f32)

        def bias_tiles(l, carry):
            b = jnp.broadcast_to(bf_ref[l] + (l == 0).astype(f32), (8, D))
            for u in sites.values():
                terms = [b[:, e * 128:(e + 1) * 128] * float(cf) for e, cf in enumerate(bcoef[u]) if cf != 0.0]
                bt_ref[l, u] = functools.reduce(lambda x, y: x + y, terms)
            return carry
        jax.lax.fori_loop(0, L, bias_tiles, 0)
        if cfg.get('FAST'):
            return

        def slab(u, carry):
            w0_copy(u).wait()
            prep(0, u, iter(lambda: None, 0), opaque(u, 12), kb0)
            return opaque(u, 12)
        zero = jax.lax.fori_loop(0, cfg['NSLAB'], slab, 0)

        def plain(l, xbf, x0f, x, j0, j1, na, free, never):
            passes = []
            for jt in range(j0, j1):
                cols = slice(jt * 128, (jt + 1) * 128)
                ya = _dot(xbf[:, :D // 2], w_ref[l, 0:4, :, :, cols].reshape(D // 2, 128)) + bf_ref[l, :, cols]
                passes += [ya, _dot(xbf[:, D // 2:], w_ref[l, 4:8, :, :, cols].reshape(D // 2, 128)) + ya]
            xp_ref[0, :, j0 * 128:j1 * 128] = x0f * jnp.concatenate(passes[1::2], axis=1) + x
            for u in range(na):
                ps, rr = divmod((u - free) * len(passes) * (R0 // 8) // (na - free), R0 // 8)
                yield None if u < free else (never, passes[ps][rr * 8:rr * 8 + 8, :])

        for u in range(cfg['NSLAB'], 8):
            w0_copy(u).wait()
        xr_in.wait()
        jm = cfg['JM']
        x0f = xr_ref[:, :jm * 128].astype(f32)
        xp_ref[1, :, :jm * 128] = x0f
        anchors = plain(0, xr_ref[...], x0f, x0f, 0, jm, (8 - cfg['NSLAB']) * NPREP, 2, mask(zero))
        for u in range(cfg['NSLAB'], 8):
            prep(0, u, anchors, zero, (kb0, kb1)[u % 2])
        in_copy(0, 0).wait()
        x0f = xr_ref[:, jm * 128:].astype(f32)
        xp_ref[1, :, jm * 128:] = x0f
        anchors = plain(0, xr_ref[...], x0f, x0f, jm, 8, len(convs) + sum(len(j[2]) for j in carried) + 2, 4, mask(zero))
        for x in convs[:len(convs) // 2]:
            conv(xn2_ref.at[0], *x, zero, next(anchors))
        for job in carried:
            st8 = {}
            for group, _ in STAGES[job[4]]:
                job[6](st8, group, zero, opaque(zero, 1), next(anchors))
        for x in convs[len(convs) // 2:]:
            conv(xn2_ref.at[0], *x, zero, next(anchors))

        def layer(l, carry):
            w_copy(l).wait()
            x, zero = xp_ref[0], opaque(l, 12)
            anchors = plain(l, x.astype(bf16), xp_ref[1], x, 0, 8, 8 * NPREP, 2, mask(zero))
            for u in range(8):
                prep(l, u, anchors, zero, (kb0, kb1)[u % 2])
            return carry

        jax.lax.fori_loop(1, L, layer, 0)
        xr_ref[...] = xp_ref[0].astype(bf16)
        xr_out.start()

    def main(tile, carry, only_late=False):
        zs, za = opaque(tile, 12), opaque(tile, 13)
        never = mask(zs)
        slot = tile % 2
        out = [o2_ref.at[1 - slot]]

        def rows(h, r0):
            lo, n = (0, Mh) if h is None else h if isinstance(h, tuple) else (h * Mq, Mq)
            return slice(r0 + lo, r0 + lo + n)

        def ld(loc, h):
            return loc[0][(0,) + loc[1] + (rows(h, loc[2]),)]

        def st(loc, v, h):
            loc[0][(zs,) + loc[1] + (rows(h, loc[2]),)] = v

        def operand(ref, idx, n):
            if cfg.get('NOBC'):
                return ref[idx + (slice(0, n),)]
            return pltpu.bitcast(ref.bitcast(u32)[idx + (slice(0, n // 2),)], bf16)

        def dot3(l, p, q, r):
            kind = next(x for x in KINDS if q in PAIR[x])
            return _dot(operand(s3[(p, kind)], (0, PAIR[kind].index(q), ORD.index(r)), Mq),
                        operand(t3_ref, (l, PRODS3.index((p, q)), ORD.index(r)), 128))

        def issue(l, p, rd):
            kind, n = rd
            if kind == 'x':
                return [dot3(l, p, q, 1) for q in (3, 5, 4, 7)]
            if kind == 'y':
                return [dot3(l, x, q, 1) for x in (p, GUEST[p]) for q in (2, 6)]
            if isinstance(n, str):
                return [dot3(l, p, int(q), int(r)) for q in kind for r in n]
            lhs = {q: [operand(s2[p], (0, k, pos2(p, q)), Mh) for k in range(2)] for q in map(int, kind)}
            return [_dot(lhs[q][k], operand(t2[p], (l, nn, k, pos2(p, q)), 128))
                    for q, nn in ([(1, 0), (1, 1)] if kind == '1' else [(int(q), n) for q in kind]) for k in range(2)]

        def biased(v, l, *site):
            if site not in sites:
                return v
            return (v.reshape(Mq // 8, 8, 128) + bt_ref[l, sites[site]]).reshape(Mq, 128)

        wait = {}
        def outer_act(l, p, i, j, n, d, h, part=None):
            stores, finals = OACT[p]
            if part == 'park':
                stores, finals = stores[:1], []
            elif part == 'rest' or (p == 6 and (i, j) != B12 and (h, n) != B12):
                stores = stores[1:]
            cache = {'d': d}
            def comb(terms):
                for t in terms.split():
                    if t[1:] not in cache:
                        cache[t[1:]] = ld(oloc(t[1:], i, j, n), h)
                return lincomb([(int(t[0] + '1'), cache[t[1:]]) for t in terms.split()])
            fin = [(IJ, comb(terms)) for IJ, terms in finals]
            for name, v in [(name, comb(terms)) for name, terms in stores]:
                st(oloc(name, i, j, n), v, h)
            for (I, J), y in fin:
                R, C = 2 * I + i, 2 * J + j
                xn = ld(x0loc(R, C, n), h) * y
                if l > 0:
                    xn = xn + ld(xloc(l, R, C, n), h)
                if l < L - 1:
                    st(xloc(l + 1, R, C, n), xn, h)
                    continue
                s = scale(R, C, rows(h, 0).start // Mq, n)
                xn = xn if s == 1.0 else xn * (1.0 / s)
                c0 = phys(C, n) * 128
                if i == 0:
                    out[0][rows(h, R * Mh), c0:c0 + 128] = xn.astype(bf16)
                elif j == 1:
                    wait[J] = xn
                else:
                    out[0][rows(h, R * Mh), c0:c0 + 256] = jnp.concatenate([xn, wait.pop(J)], axis=1).astype(bf16)

        def inner_act(g, l, p, kind, n, h, P, Q, part=None):
            vloc = iloc(g, 'v', n) if p == 1 else oloc(OACT[p][0][0][0], 0, 1, n)
            if kind == '35':
                st(iloc(g, 's', n), Q + ld(iloc(g, 'm1', n), h), h)
                if p == 1:
                    st(vloc, P, h)
                outer_act(l, p, 0, 1, n, P, h, part)
            elif kind == '47':
                st(iloc(g, 'u', n), Q + ld(vloc, h), h)
                outer_act(l, p, 0, 0, n, P + ld(iloc(g, 's', n), h), h, part)
            else:
                outer_act(l, p, 1, 1, n, ld(iloc(g, 's', n), h) - Q, h, part)
                outer_act(l, p, 1, 0, n, P + ld(iloc(g, 'u', n), h), h, part)

        def consume(g, l, p, rd, res):
            kind, n = rd
            if n == '1':
                for u, (kd, x) in enumerate([('35', p), ('47', p)] if kind == 'x' else [('26', p), ('26', GUEST[p])]):
                    for al in range(2):
                        st(jloc(kd, '1', al, x != p), biased(res[2 * u + al], l, x, int(kd[al]), '1'), 0)
            elif isinstance(n, str):
                sm = [res[2 * al] + res[2 * al + 1] for al in range(2)]
                df = [res[2 * al] - res[2 * al + 1] for al in range(2)]
                J = lambda name, al: ld(jloc(kind, name, al, name == '1' and kind == '26' and p not in GUEST), 0)
                part = 'park' if deferred(l, p, rd) else None
                done = lambda h, nn, m: inner_act(g, l, p, kind, nn, h, m[0] + m[1], m[0] - m[1], part)
                if n == '35':
                    for al in range(2):
                        st(jloc(kind, 's', al), df[al] + J('1', al), 0)
                    done(0, 1, [biased(sm[al], l, p, int(kind[al]), 'v') for al in range(2)])
                elif n == '47':
                    for al in range(2):
                        st(jloc(kind, 'k', al), biased(df[al], l, p, int(kind[al]), 'k'), 0)
                    done(0, 0, [biased(sm[al] + J('s', al), l, p, int(kind[al]), 'm') for al in range(2)])
                else:
                    O = lambda i, j: ld(oloc(OACT[p][0][0][0], i, j, 1), 0)
                    m = [sm[al] + J('k', al) for al in range(2)]
                    P = m[0] + m[1] + O(*{'35': B12, '47': B11, '26': B21}[kind])
                    Q = m[0] - m[1] - (ld(iloc(g, 'm1', 1), 0) if kind == '35' else O(*{'47': B12, '26': B22}[kind]))
                    done(1, 1, [J('s', al) - df[al] for al in range(2)])
                    inner_act(g, l, p, kind, 0, 1, P, Q, part)
            else:
                m = []
                for al, (q, nn) in enumerate([(1, 0), (1, 1)] if kind == '1' else [(int(q), n) for q in kind]):
                    v = res[2 * al] + res[2 * al + 1]
                    if any((p, q, (h, nn)) in sites for h in range(2)):
                        v = jnp.concatenate([biased(v[h * Mq:(h + 1) * Mq], l, p, q, (h, nn)) for h in range(2)], axis=0)
                    m.append(v)
                if kind == '1':
                    for nn in range(2):
                        st(iloc(g, 'm1', nn), m[nn], None)
                else:
                    inner_act(g, l, p, kind, n, None, m[0] + m[1], m[0] - m[1])

        def finish(l, p, pieces, nr, anchor):
            for i, j, n, r0 in pieces:
                d = ld(oloc(OACT[p][0][0][0], i, j, n), (r0, nr))
                outer_act(l, p, i, j, n, tie(d, anchor), (r0, nr), 'rest')

        if only_late:
            for x in late:
                finish(*x, None)
            out_copy(tile - 1, 1 - slot, 2).start()
            return carry
        state = {}
        count.clear()
        for g, rd, t0, n in sched:
            l, p = outs[g]
            if t0 == start[1]:
                pl.when(tile > 0)(lambda: out_copy(tile - 1, 1 - slot, 2).start())
                out[0] = o2_ref.at[slot]
            if t0 == start[G - 1]:
                out_copy(tile, slot, 0).start()
            res = issue(l, p, rd)
            for t in range(t0, t0 + n):
                if t in plan:
                    r0 = 16 * (t - t0) + 8
                    anchor = (never, res[0 if isinstance(rd[1], str) else 1][r0:r0 + 8, :])
                for kind, fn, group in plan.get(t, []):
                    if kind == 'fin':
                        finish(*fn, anchor)
                    elif kind == 'conv':
                        conv(xn2_ref.at[1 - slot], *fn, zs, anchor)
                    else:
                        fn(state.setdefault(id(fn), {}), group, zs, za, anchor)
            if t0 + n == T:
                out_copy(tile, slot, 1).start()
            consume(g, l, p, rd, res)
        pl.when(tile + 3 < NMAIN)(lambda: in_copy(tile + 3, 1 - slot).start())
        pl.when(tile > 0)(lambda: out_copy(tile - 1, 1 - slot, 3).wait())
        pl.when(tile + 2 < NMAIN)(lambda: in_copy(tile + 2, slot).wait())
        return carry

    prologue()
    in_copy(2, 0).start()
    in_copy(1, 1).wait()
    jax.lax.fori_loop(0, NMAIN, main, 0)
    main(jnp.int32(NMAIN), 0, True)
    xr_out.wait()
    out_copy(NMAIN - 1, (NMAIN - 1) % 2, 3).wait()


def build(TM=640, **kw):
    def f(x0, ws, bs):
        B, D = x0.shape
        L = ws.shape[0]
        Mh = TM // 4
        nmain = (B - 1) // TM
        R0 = B - nmain * TM
        assert D == 1024 and L % 2 == 0 and L <= 8 and TM % 128 == 0 and R0 % 16 == 0 and nmain >= 3
        n3 = len(PRODS3)
        odd = lambda n: 16 * (n // 16 | 1)
        V = pltpu.VMEM
        scratch = ([V((1, 2, 2, 2, Mh + 40, 128), f32)] * 4 + [V((1, 2, 4, 2, Mh + 40, 128), f32)] * 7
                   + [V((1, Mh + 32, 128), f32)] * (16 + 64 + 20)
                   + [V((1, 2, 10 if p == 1 else 2, odd(Mh), 128), bf16) for p in range(1, 8)]
                   + [V((1, 2, 10, odd(Mh // 2), 128), bf16)] * (n3 // 2)
                   + [V((L, 2, 2, 7 if p == 1 else 1, 128, 128), bf16) for p in range(1, 8)]
                   + [V((L, n3, 7, 128, 128), bf16)] + [V((1, 4, 16 * n3 + 16, 128), f32)] * 2
                   + [V((L, 64, 8, 128), f32), V((8, 1, D), f32), V((2, TM, D), bf16), V((2, TM, D), bf16),
                      V((L, 8, 8, 16, D), bf16), V((R0, D), bf16), V((2, R0, D), f32), V((L, D), bf16),
                      pltpu.SemaphoreType.DMA((L + 14,))])
        anyspec = pl.BlockSpec(memory_space=pl.ANY)
        return pl.pallas_call(
            functools.partial(_kernel, L=L, TM=TM, R0=R0, NMAIN=nmain, D=D, cfg=dict(CFG, **kw)),
            in_specs=[anyspec, anyspec, anyspec],
            out_specs=anyspec,
            out_shape=jax.ShapeDtypeStruct((B, D), x0.dtype),
            scratch_shapes=scratch,
            compiler_params=pltpu.CompilerParams(
                vmem_limit_bytes=120 * 1024 * 1024,
                internal_scratch_in_bytes=65536,
                disable_bounds_checks=True,
            ),
        )(x0, ws.reshape(L, 8, 8, 16, D), bs)
    return f


@jax.jit
def pallas_standalone__dcn_v2_cross__recsys_kernel(x0, ws, bs):
    return build()(x0, ws, bs)
```

```python
import functools

import jax
import jax.numpy as jnp
import numpy as np
import jax.experimental.pallas as pl
import jax.experimental.pallas.tpu as pltpu

f32 = jnp.float32
bf16 = jnp.bfloat16
u32 = jnp.uint32

B11, B12, B21, B22 = BLOCKS = (0, 0), (0, 1), (1, 0), (1, 1)
LA = {1: [(B11, 1), (B22, 1)], 3: [(B11, 1), (B12, -1)], 5: [(B11, 1), (B12, 1)], 4: [(B12, 1), (B22, 1)],
      7: [(B12, 1), (B22, -1)]}
PC = {1: (1, 0, 0, 1), 2: (0, 0, 1, -1), 3: (1, 1, 1, 1), 4: (1, 0, 1, 0), 5: (-1, 1, 1, -1), 6: (0, 0, 1, 1),
      7: (1, 0, -1, 0)}
KINDS = ('35', '47', '26')
PAIR = {'35': (5, 3), '47': (4, 7), '26': (2, 6)}
ORD = (3, 5, 4, 7, 1, 2, 6)
OUTER = (3, 5, 1, 4, 7, 2, 6)
GUEST = {3: 5, 4: 7, 2: 6}
PRODS3 = [(p, q) for p in OUTER if p != 1 for kind in KINDS for q in PAIR[kind]]
GAMMA = 0.125
OACT = {
    3: ([('M3', '+d')], []),
    5: ([('M5', '+d')], [(B12, '+d +M3')]),
    1: ([('S', '+d +M3 -M5')], []),
    4: ([('M4', '+d')], []),
    7: ([('M7', '+d')], [(B11, '+d +S +M4')]),
    2: ([('M2', '+d'), ('U', '+d +M4 -M7 +M3 +M5')], []),
    6: ([('M6', '+d')], [(B22, '+d +S -M2'), (B21, '+d +U')]),
}
OSL = {'M3': 0, 'M5': 1, 'S': 2, 'M4': 3, 'M7': 4, 'U': 5, 'M2': 6, 'M6': 7}
ISL = {'m1': 0, 's': 1, 'v': 2, 'u': 3}
DEFER = {5: [('26', '26'), ('47', '26')], 7: [('26', '26'), ('47', '26')], 2: [('47', '26'), ('26', '26')],
         6: [('35', '26'), ('47', '26'), ('26', '26'), ('26', '35')]}
SAVE = {5: B12, 1: B11, 7: B22, 2: B21}
STAGES = {1: [(None, 1.0)], 2: [((B11, B12), .4), ((B21, B22), .6)], 'O': [((B11, B12), .5), ((B21, B22), .5)],
          3: [((B11, B12), .35), ((B22,), .37), ((B21,), .28)],
          4: [((B11,), .16), ((B12,), .26), ((B22,), .31), ((B21,), .27)]}
LAG = 8
CFG = dict(CAP=0.95, PORT=0.9, CS=0.5, CL=0.3, VK=0.75, TAIL=3, EW7=12, EW6=25, MOFF=15, GE=8, NSLAB=6, JM=3)


def _dot(a, b):
    return jnp.dot(a, b, preferred_element_type=f32)


def scale(R, C, h, k):
    return 2.0 ** (R // 2 + R % 2 + h - C // 2 - C % 2 - k)


def phys(C, k):
    return 4 * (C // 2) + 2 * k + C % 2


def b_ops(b11, b12, b21, b22):
    r1 = b11 + b22
    g = b12 + b21
    return {1: r1, 2: b11 - b12, 3: b12 - b22, 4: g - r1, 5: b12 + b22, 6: b11 + b12, 7: g + r1}


def lincomb(terms):
    assert terms[0][0] == 1
    acc = terms[0][1]
    for s, v in terms[1:]:
        acc = acc + v if s == 1 else acc - v
    return acc


def rounds_of(p):
    if p == 1:
        return [('1', None)] + [(kind, n) for kind in KINDS for n in range(2)]
    minis = lambda kind: [(kind, r) for r in KINDS]
    return [('1', None), ('x', '1')] + minis('35') + minis('47') + [('y', '1')] * (p in GUEST) + minis('26')


def round_usage(p, rd, first, last, defer):
    stores, finals = OACT[p]
    kind, n = rd
    alu = sum(len(t.split()) - 1 for _, t in stores) + sum(len(t.split()) + (not first) + 2 * last for _, t in finals)
    nst = len(stores) + len(finals)
    if last and kind == '26':
        alu, nst = alu - 0.7 * len(finals), nst - 0.5 * len(finals)
    if defer:
        alu, nst = 0, 1
    elif p == 6 and kind != '35' and n != '35':
        nst -= 1
    if n == '1':
        a, st, m = 0, 4, 0
    elif isinstance(n, str):
        a, st, m = {'35': ((9, 3, 1), (16, 2, 2)), '47': ((10, 3, 1), (18, 2, 2)), '26': ((10, 2, 2), (18, 0, 4))}[kind][n == '26']
    else:
        a, st, m = {'1': (2, 2, 0), '35': (5, 2, 1), '47': (6, 1, 1), '26': (6, 0, 2)}[kind]
    return a + m * alu, st + m * nst


def bias_sites():
    cand = []
    for p in OUTER:
        for rd in rounds_of(p):
            kind, n = rd
            if n == '1':
                pq = [(p, q) for q in (3, 5, 4, 7)] if kind == 'x' else [(x, q) for x in (p, GUEST[p]) for q in (2, 6)]
                cand += [(p, rd, x + ('1',), (1, 0, 0, 1)) for x in pq]
            elif n in ('35', '47'):
                where = [('v', (0, 1, 1, 0))] if n == '35' else [('k', (0, 0, 1, 0)), ('m', (1, 0, 0, 0))]
                cand += [(p, rd, (p, int(q), w), pat) for q in kind for w, pat in where]
            elif n != '26':
                cand += [(p, rd, (p, int(q), (h, nn)), tuple(int(e == 2 * h + nn) for e in range(4)))
                         for q in kind for nn in ((0, 1) if kind == '1' else (n,)) for h in range(2)]
    extra, sites, rows = {}, [], []
    def busy(c):
        a, st = round_usage(c[0], c[1], False, False, c[1] in DEFER.get(c[0], ()))
        return 2 * (a + extra.get(c[:2], 0)) + st + (5 if isinstance(c[1][1], str) else 3)
    while len(sites) < 64:
        c = min(cand, key=busy)
        cand.remove(c)
        row = np.kron(np.kron(PC[c[2][0]], PC[c[2][1]]), c[3])
        if np.linalg.matrix_rank(np.array(rows + [row])) > len(rows):
            rows.append(row)
            sites.append(c[2])
            extra[c[:2]] = extra.get(c[:2], 0) + (1 if isinstance(c[1][1], str) else 0.5)
    want = np.zeros((64, 8))
    for e, (I, J, i, j, h, n) in enumerate(np.ndindex(*(2,) * 6)):
        want[e, phys(2 * J + j, n)] = scale(2 * I + i, 2 * J + j, h, n) / GAMMA
    coef = np.round(np.linalg.solve(np.array(rows, float).T, want) * 4096) / 4096
    assert (np.array(rows).T @ coef == want).all()
    return {x: e for e, x in enumerate(sites) if coef[e].any()}, coef, extra


def yds(groups, cap):
    n = len(cap)
    speed, cls, gcls = [0.0] * n, [-1] * n, {}
    todo = list(groups)
    while todo:
        pre = [0.0]
        for t in range(n):
            pre.append(pre[-1] + (cap[t] if cls[t] < 0 else 0.0))
        best = None
        for a in sorted({g[0] for g in todo}):
            w = 0.0
            for g in sorted((g for g in todo if g[0] >= a), key=lambda g: g[1]):
                w += g[2]
                d = w / max(pre[g[1] + 1] - pre[a], 1e-9)
                if best is None or d > best[0]:
                    best = (d, a, g[1])
        d, a, b = best
        for t in range(a, b + 1):
            if cls[t] < 0:
                speed[t], cls[t] = d, len(gcls)
        gcls.update({g[:2]: len(gcls) for g in todo if g[0] >= a and g[1] <= b})
        todo = [g for g in todo if not (g[0] >= a and g[1] <= b)]
    return speed, cls, gcls


def spread_jobs(jobs, cap, vcap, tail):
    T = len(cap)
    cap3 = cap * 3
    all3 = [(j[0] + k * T, j[1] + k * T, ji, k) for k in range(3) for ji, j in enumerate(jobs) if j[0] + k * T >= 0]
    pend = {}
    for j in sorted(all3, key=lambda j: (j[1], j[3], j[2])):
        pend.setdefault(j[:2], []).append(j)
    left = {w: sum(sum(jobs[j[2]][2]) for j in q) for w, q in pend.items()}
    speed, cls, gcls = yds([w + (left[w],) for w in pend], cap3)
    cum = [0.0]
    for t in range(3 * T):
        cum.append(cum[-1] + speed[t] * cap3[t])
    when = [[] for _ in jobs]
    debt, vdebt, cur, done = 0.0, 0.0, None, 0

    def fits(j, t):
        need = max(debt, 0.0) + sum(jobs[j[2]][2]) + 1.0
        for w in pend:
            if w[1] >= j[1]:
                break
            if left[w] > 1e-9:
                need += left[w]
                if need > cum[w[1] + 1] - cum[t]:
                    return False
        return True

    for t in range(3 * T):
        if t % T == 0:
            debt, vdebt = min(debt, 0.0), -0.5
        while True:
            rdy = [q[0] for w, q in pend.items() if q and w[0] <= t and (gcls[w] == cls[t] or w[1] <= t)]
            j = cur
            if j is None:
                if not rdy:
                    debt = max(debt, 0.0)
                    break
                j = rdy[0]
                if j[1] > t:
                    j = (min if vdebt > 0 else max)([x for x in rdy if x is j or fits(x, t)], key=lambda x: jobs[x[2]][3])
                nst = len(jobs[j[2]][2])
                if nst > 1 and j[1] > t and (t + tail + 2 * nst) // T != t // T:
                    break
            must = j[1] <= t or (cur is not None and ((t + tail + 1) // T != t // T or (rdy and rdy[0][1] <= t)))
            if not must and (cap3[t] == 0.0 or debt > 0.5 * speed[t] * cap3[t]):
                break
            if cur is None:
                pend[j[:2]].pop(0)
                left[j[:2]] -= sum(jobs[j[2]][2])
                cur, done = j, 0
            debt += jobs[j[2]][2][done]
            vdebt += jobs[j[2]][2][done] * jobs[j[2]][3]
            if j[3] == 1:
                when[j[2]].append(t - T)
            done += 1
            if done == len(jobs[j[2]][2]):
                cur = None
        debt -= speed[t] * cap3[t]
        vdebt = min(max(vdebt - vcap[t % T], -0.5), 1.0)
    assert all(j[0] <= ts[0] and ts[-1] <= j[1] and (ts[0] < 0) == (ts[-1] < 0) for j, ts in zip(jobs, when))
    return when


def _kernel(x_hbm, w_hbm, b_hbm, o_hbm, *scratch, L, TM, R0, NMAIN, D, cfg):
    H, Mh, Mq = D // 4, TM // 4, TM // 8
    NC, NQ = Mh // 16, Mq // 16
    it = iter(scratch)
    take = lambda n: [next(it) for _ in range(n)]
    x0b, xb, ib, ob, jb = take(4), take(7), take(16), take(64), take(20)
    s2 = dict(zip(range(1, 8), take(7)))
    s3 = {(p, kind): next(it) for p in OUTER if p != 1 for kind in KINDS}
    t2 = dict(zip(range(1, 8), take(7)))
    t3_ref, kb0, kb1, bt_ref, bf_ref, xn2_ref, o2_ref, w_ref, xr_ref, xp_ref, b_ref, sem = it
    sites, bcoef, extra = bias_sites()
    pos2 = lambda p, q: ORD.index(q) if p == 1 else 0

    xset = lambda l: 6 if l == 'O' else 4 if l == 0 else (l % 2) * 2
    xoff = lambda I, J: 16 * ((I + J) % 2)
    xloc = lambda l, R, C, k: (xb[xset(l) + R // 2], (R % 2, C, k), xoff(R // 2, C // 2))
    x0loc = lambda R, C, k: (x0b[(R // 2) * 2 + C // 2], (R % 2, C % 2, k), 8 + xoff(R // 2, C // 2))
    iloc = lambda g, name, n: (ib[((g % 2) * 4 + ISL[name]) * 2 + n], (), 8 * ISL[name])
    oloc = lambda name, i, j, n: (ob[(OSL[name] * 4 + i * 2 + j) * 2 + n], (), 8 * ((OSL[name] + 2 * j) % 4))

    def jloc(kind, name, al, guest=False):
        u = ('1', 's', 'k').index(name)
        return jb[18 + al if guest else (KINDS.index(kind) * 3 + u) * 2 + al], (), 8 * ((3 * u + al) % 4)

    def tie(v, anchor, r=None, lo=0):
        if anchor is None:
            return v
        never, gate = anchor
        if r is None:
            n = v.shape[0]
            return jax.lax.select(never[n], gate if n == 8 else jnp.tile(gate, (n // 8, 1)), v)
        top = jax.lax.select(never[8], gate, v[r:r + 8])
        return jnp.concatenate(([v[lo:r]] if r > lo else []) + [top, v[r + 8:r + 16]], axis=0)

    def consts(anchor, ss):
        one = {s: tie(jnp.full((8, 128), s, f32), anchor) for s in set(ss)}
        return jnp.concatenate([one[s] for s in ss for _ in range(2)], axis=0)

    def conv(src, R, Q, r, zs, anchor):
        v = src[R * Mh + r:R * Mh + r + 32, Q * H:(Q + 1) * H].astype(f32)
        for j in range(2):
            C, k = 2 * (Q // 2) + j, Q % 2
            buf, idx, off = xloc(0, R, C, k)
            sv = consts(anchor, [scale(R, C, (r + u) // Mq, k) for u in (0, 16)])
            buf[(zs,) + idx + (slice(off + r, off + r + 32),)] = v[:, j * 128:(j + 1) * 128] * sv

    count = {}
    def block_sum(l, terms, ii, jj, kk, r, save, zs, za, anchor, gate=True):
        rng = lambda t: slice(t[0], t[-1] + 1)
        vals = []
        for u, ((I, J), s) in enumerate(terms):
            ref, r0 = xb[xset(l) + I], xoff(I, J) + r
            v = ref[za if u == 0 else 0, rng(ii), 2 * J + jj[0]:2 * J + jj[-1] + 1, rng(kk), r0:r0 + 16, :]
            if (I, J) == save:
                sv = consts(anchor, [GAMMA / scale(2 * I + i, 2 * J + j, r // Mq, k) for i in ii for j in jj for k in kk])
                x0b[I * 2 + J][zs, rng(ii), rng(jj), rng(kk), r0 + 8:r0 + 24, :] = v * sv.reshape(v.shape)
            if u == 0 and gate:
                count[xset(l)] = count.get(xset(l), -1) + 1
                if count[xset(l)] % cfg['GE'] == 0:
                    ref[0, 0, 0, 0, Mh + 24:Mh + 32, :] = anchor[1]
            vals.append((s, v))
        v = lincomb(vals)
        return v.reshape(v.size // 128, 128)

    def operands(a, group, st8, store):
        for u, b in enumerate(group):
            st8[b] = a if len(group) == 1 else a[:, u:u + 1]
        ops = {}
        if B12 in group:
            ops[3], ops[5] = st8[B11] - st8[B12], st8[B11] + st8[B12]
        if B22 in group:
            ops[4], ops[7] = st8[B12] + st8[B22], st8[B12] - st8[B22]
            ops[1] = st8['l1'] = st8[B11] + st8[B22]
        if B21 in group:
            g = st8[B12] + st8[B21]
            ops[2], ops[6] = g + st8['l1'], g - st8['l1']
        now = [q for q in ORD if q in ops]
        if now:
            u = ORD.index(now[0])
            store(slice(u, u + len(now)), jnp.concatenate([ops[q] for q in now], axis=1).astype(bf16))

    def unit1(l, c, k, save, st8, group, zs, za, anchor):
        def store(pos, v):
            s2[1][zs, k:k + 1, pos, 16 * c:16 * c + 16, :] = v
        e = block_sum(l, LA[1], [group[0][0]], [0, 1], [k], 16 * c, save, zs, za, anchor)
        operands(tie(e, anchor, 16).reshape(1, 2, 16, 128), group, st8, store)

    def unit26(l, c, k, save, st8, group, zs, za, anchor):
        i = group[0][0]
        f = block_sum(l, [(B11, 1), (B22, 1)], [i], [0, 1], [k], 16 * c, save, zs, za, anchor, False)
        e = tie(block_sum(l, [(B12, 1), (B21, 1)], [i], [0, 1], [k], 16 * c, save, zs, za, anchor), anchor)
        for J, v in enumerate((e + f, e - f)):
            r0 = xoff(0, J) + 16 * c
            xb[6][zs, i, 2 * J:2 * J + 2, k, r0:r0 + 16, :] = v.reshape(2, 16, 128)

    def unit3(l, p, kind, c, save, st8, group, zs, za, anchor):
        def store(pos, v):
            s3[(p, kind)][zs, :, pos, 16 * c:16 * c + 16, :] = v
        h, kk = group[0][0], [b[1] for b in group]
        ii, jj = {'35': ([0], [0, 1]), '47': ([0, 1], [1]), '26': ([0, 1], [0, 1])}[kind]
        src = (l, LA[p]) if p in LA else ('O', [((0, (2, 6).index(p)), 1)])
        n = 16 * len(kk)
        v = block_sum(*src, ii, jj, kk, h * Mq + 16 * c, save, zs, za, anchor)
        if kind == '26':
            e, f = tie(v, anchor, 16, 16) + v[32:48], v[0:16] + v[48:64]
            r0 = h * Mq + 16 * c
            s2[p][zs, kk[0], 0, r0:r0 + 16, :] = f.astype(bf16)
        else:
            e, f = tie(v, anchor, n - 16), v[n:]
        operands(jnp.concatenate([e + f, e - f], axis=0).reshape(2, len(kk), 16, 128), group, st8, store)

    NPREP = 32 + len(PRODS3)
    def prep(l, u, anchors, zero, kb):
        mul = lambda v, s: v if s == 1.0 else v * s
        stack = lambda T: jnp.concatenate([T[q] for q in ORD], axis=0).reshape(7, 16, 128).astype(bf16)
        rows = pl.ds(16 * u, 16) if isinstance(u, int) else pl.ds(pl.multiple_of(16 * u, 16), 16)
        for k in range(2):
            wide = [w_ref[l, phys(R, k), u].astype(f32) for R in range(4)]
            for n in range(2):
                anchor = next(anchors)
                blk = lambda R, C: mul(wide[R][:, phys(C, n) * 128:(phys(C, n) + 1) * 128], scale(R, C, k, n))
                O = {(i, j): b_ops(blk(i, j), tie(blk(i, 2 + j), anchor, 0), blk(2 + i, j), blk(2 + i, 2 + j))
                     for i, j in BLOCKS}
                for p in (2, 6, 3, 5, 1, 4, 7):
                    o = [mul(O[b][p], 4.0 if p == 1 else 1.0) for b in BLOCKS]
                    T = b_ops(o[0], tie(o[1], next(anchors), 0), o[2], o[3])
                    if p == 1:
                        T[1] = T[1] * 2.0
                        t2[p][l, n, k, :, rows, :] = stack(T)
                        continue
                    t2[p][l, n, k, 0, rows, :] = (T[1] * 4.0).astype(bf16)
                    e0 = PRODS3.index((p, 5))
                    if (k, n) != (1, 1):
                        kb[zero, k * 2 + n, 16 * e0:16 * e0 + 96, :] = jnp.concatenate(
                            [T[q] for _, q in PRODS3[e0:e0 + 6]], axis=0)
                        continue
                    for e in range(e0, e0 + 6):
                        v = kb[0, 0:3, 16 * e:16 * e + 16, :]
                        T3 = b_ops(v[0], tie(v[1], next(anchors), 0), v[2], T[PRODS3[e][1]])
                        T3[1] = T3[1] * 2.0
                        t3_ref[l, e, :, rows, :] = stack(T3)

    def deferred(l, p, rd):
        if l == L - 1 and p == 6 and rd[0] == '26':
            return rd[1] == '26'
        return rd in DEFER.get(p, ())

    outs = [(l, p) for l in range(L) for p in OUTER]
    G = len(outs)
    sched, start, use, vuse = [], [], [], []
    for g, (l, p) in enumerate(outs):
        start.append(len(use))
        for rd in rounds_of(p):
            n = NQ if isinstance(rd[1], str) else NC
            sched.append((g, rd, len(use), n))
            a, st_ = round_usage(p, rd, l == 0, l == L - 1, deferred(l, p, rd))
            a += extra.get((p, rd), 0)
            use += [max((2 * a + st_ + 2 + 16 / n) / 72, cfg['PORT'] * st_ / 8)] * n
            vuse += [st_ / 8] * n
    T = len(use)
    first = lambda g, kind: next(t0 for gg, rd, t0, _ in sched if gg == g and rd[0] == kind)
    jobs, late = [], []
    def add(lo, hi, alu, st_, ld_, scheme, kind, fn):
        w = alu / 64 + cfg['CS'] * (st_ + len(STAGES[scheme])) / 16 + cfg['CL'] * ld_ / 48
        jobs.append((lo, max(hi, lo), [w * f for _, f in STAGES[scheme]], st_ / 16 / w, scheme, kind, fn))
    for g, (l, p) in enumerate(outs):
        for gg, rd, t0, n_ in sched:
            if gg == g and deferred(l, p, rd):
                last = l == L - 1
                nops = 4 * (sum(len(t.split()) for _, t in OACT[p][0][1:]) + sum(len(t.split()) + 2 + 2 * last for _, t in OACT[p][1]))
                ws = [(i, j, n, h * Mq + 16 * c) for c in range(NQ)
                      for h, n in {'35': [B12], '47': [B11], '26': [B22, B21]}[rd[1]]
                      for i, j in {'35': [B12], '47': [B11], '26': [B22, B21]}[rd[0]]]
                if t0 + n_ == T:
                    for u in range(0, len(ws), 2):
                        for r8 in (0, 8):
                            late.append((l, p, [w[:3] + (w[3] + r8,) for w in ws[u:u + 2]], 8))
                            add(0, cfg['EW6'] - 1, nops * 0.45, 1, nops * 0.4, 1, 'fin', late[-1])
                    continue
                due = {5: lambda: start[7 * l + 5] - 1, 2: lambda: first(g + 1, rd[0]) - 3,
                       7: lambda: start[g + 1] + cfg['EW7'],
                       6: lambda: T - cfg['TAIL'] - 1 if last else start[g + 1] + cfg['EW6'] - 1}[p]()
                m = 1 if p == 6 else 2
                for u in range(0, len(ws), m):
                    add(t0 + n_, due, nops * m // 2, 3, nops * m // 2, 1, 'fin', (l, p, ws[u:u + m], 16))
        if p in (3, 5):
            lo = start[7 * l - 2] + (cfg['EW7'] + 1 if l else -T)
        else:
            lo = start[7 * l] + cfg['EW6']
        hi = start[g] - LAG - 3
        save = SAVE.get(p) if l == 0 else None
        sv = save is not None
        if p == 1:
            for c, k in np.ndindex(NC, 2):
                add(lo, hi, 31 + 8 * sv, 7 + 8 * sv, 16, 2, l, functools.partial(unit1, l, c, k, save))
            continue
        nt = 2
        if p in (2, 6):
            mid = start[7 * l + 3] + cfg['MOFF']
            if p == 2:
                for c, k in np.ndindex(NC, 2):
                    add(lo, mid - 3, 40 + 8 * sv, 16 + 8 * sv, 32, 'O', l, functools.partial(unit26, l, c, k, save))
            lo, nt, save, sv = mid, 1, None, False
        for c in range(NQ):
            add(lo, hi if p in GUEST else first(g - 1, 'y') - LAG - 3, 32 * nt + 50 + 32 * sv, 18 + 32 * sv, 32 * nt,
                4, l, functools.partial(unit3, l, p, '26', c, save))
        for c in range(NQ):
            for kind in KINDS[:2]:
                add(lo, hi + (NC if g else 0), 16 * nt + 46, 14, 16 * nt, 3, l, functools.partial(unit3, l, p, kind, c, None))
    convs = [(R, Q, r) for R in range(4) for Q in range(4) for r in range(0, Mh, 32)]
    for x in convs:
        add(start[6], start[G - 2] - 2, 18, 7, 4, 1, 'conv', x)
    cap = [max(cfg['CAP'] - max(use[t], use[(t + 1) % T]), 0.0) * (t < T - cfg['TAIL']) for t in range(T)]
    when = spread_jobs(jobs, cap, [cfg['VK'] * (1 - vuse[(t + 1) % T]) for t in range(T)], cfg['TAIL'])
    plan = {}
    for t, _, ji, u in sorted((t % T, ts[0] % T, ji, u) for ji, ts in enumerate(when) for u, t in enumerate(ts)):
        plan.setdefault(t, []).append((jobs[ji][5], jobs[ji][6], STAGES[jobs[ji][4]][u][0]))
    carried = [job for ts, job in zip(when, jobs) if ts[0] < 0]

    def w_copy(l):
        return pltpu.make_async_copy(w_hbm.at[l], w_ref.at[l], sem.at[l])

    def w0_copy(u):
        return pltpu.make_async_copy(w_hbm.at[0, :, u], w_ref.at[0, :, u], sem.at[L + 6 + u])

    def in_copy(t, slot):
        return pltpu.make_async_copy(x_hbm.at[pl.ds(pl.multiple_of(t * TM, 32), TM)], xn2_ref.at[slot], sem.at[L + slot])

    def out_copy(t, slot, part):
        r0, nr = (0, TM) if part is None else ((0, 4 * Mq), (4 * Mq, Mq), (5 * Mq, Mq), (6 * Mq, Mq), (7 * Mq, Mq))[part]
        return pltpu.make_async_copy(o2_ref.at[slot, pl.ds(r0, nr)],
                                     o_hbm.at[pl.ds(pl.multiple_of(t * TM + r0, 16), nr)], sem.at[L + 4 + slot])

    xr_in = pltpu.make_async_copy(x_hbm.at[pl.ds(NMAIN * TM, R0)], xr_ref, sem.at[L + 2])
    xr_out = pltpu.make_async_copy(xr_ref, o_hbm.at[pl.ds(NMAIN * TM, R0)], sem.at[L + 2])
    b_in = pltpu.make_async_copy(b_hbm, b_ref, sem.at[L + 3])
    opaque = lambda i, s: jax.lax.shift_right_logical(i, s)
    mask = lambda zero: {n: jnp.broadcast_to(zero, (n, 128)) != 0 for n in (8, 16, 32)}

    def prologue():
        b_in.start()
        for u in range(8):
            w0_copy(u).start()
        xr_in.start()
        in_copy(0, 0).start()
        for l in range(1, L):
            w_copy(l).start()
        in_copy(1, 1).start()
        for j, n in BLOCKS:
            for ref, idx, off in ([oloc(x, 1, j, n) for x in ('S', 'M2', 'U', 'M6')]
                                  + [f(3, 2 * J + j, n) for J in range(2) for f in (x0loc, functools.partial(xloc, L - 1))]):
                ref[(0,) + idx + (slice(off + Mq, off + Mh),)] = jnp.zeros((Mq, 128), f32)
        b_in.wait()
        for l in range(L):
            bf_ref[l] = b_ref[l:l + 1, :].astype(f32)

        def bias_tiles(l, carry):
            b = jnp.broadcast_to(bf_ref[l] + (l == 0).astype(f32), (8, D))
            for u in sites.values():
                terms = [b[:, e * 128:(e + 1) * 128] * float(cf) for e, cf in enumerate(bcoef[u]) if cf != 0.0]
                bt_ref[l, u] = functools.reduce(lambda x, y: x + y, terms)
            return carry
        jax.lax.fori_loop(0, L, bias_tiles, 0)
        if cfg.get('FAST'):
            return

        def slab(u, carry):
            w0_copy(u).wait()
            prep(0, u, iter(lambda: None, 0), opaque(u, 12), kb0)
            return opaque(u, 12)
        zero = jax.lax.fori_loop(0, cfg['NSLAB'], slab, 0)

        def plain(l, xbf, x0f, x, j0, j1, na, free, never):
            passes = []
            for jt in range(j0, j1):
                cols = slice(jt * 128, (jt + 1) * 128)
                ya = _dot(xbf[:, :D // 2], w_ref[l, 0:4, :, :, cols].reshape(D // 2, 128)) + bf_ref[l, :, cols]
                passes += [ya, _dot(xbf[:, D // 2:], w_ref[l, 4:8, :, :, cols].reshape(D // 2, 128)) + ya]
            xp_ref[0, :, j0 * 128:j1 * 128] = x0f * jnp.concatenate(passes[1::2], axis=1) + x
            for u in range(na):
                ps, rr = divmod((u - free) * len(passes) * (R0 // 8) // (na - free), R0 // 8)
                yield None if u < free else (never, passes[ps][rr * 8:rr * 8 + 8, :])

        for u in range(cfg['NSLAB'], 8):
            w0_copy(u).wait()
        xr_in.wait()
        jm = cfg['JM']
        x0f = xr_ref[:, :jm * 128].astype(f32)
        xp_ref[1, :, :jm * 128] = x0f
        anchors = plain(0, xr_ref[...], x0f, x0f, 0, jm, (8 - cfg['NSLAB']) * NPREP, 2, mask(zero))
        for u in range(cfg['NSLAB'], 8):
            prep(0, u, anchors, zero, (kb0, kb1)[u % 2])
        in_copy(0, 0).wait()
        x0f = xr_ref[:, jm * 128:].astype(f32)
        xp_ref[1, :, jm * 128:] = x0f
        anchors = plain(0, xr_ref[...], x0f, x0f, jm, 8, len(convs) + sum(len(j[2]) for j in carried) + 2, 4, mask(zero))
        for x in convs[:len(convs) // 2]:
            conv(xn2_ref.at[0], *x, zero, next(anchors))
        for job in carried:
            st8 = {}
            for group, _ in STAGES[job[4]]:
                job[6](st8, group, zero, opaque(zero, 1), next(anchors))
        for x in convs[len(convs) // 2:]:
            conv(xn2_ref.at[0], *x, zero, next(anchors))

        def layer(l, carry):
            w_copy(l).wait()
            x, zero = xp_ref[0], opaque(l, 12)
            anchors = plain(l, x.astype(bf16), xp_ref[1], x, 0, 8, 8 * NPREP, 2, mask(zero))
            for u in range(8):
                prep(l, u, anchors, zero, (kb0, kb1)[u % 2])
            return carry

        jax.lax.fori_loop(1, L, layer, 0)
        xr_ref[...] = xp_ref[0].astype(bf16)
        xr_out.start()

    def main(tile, carry, only_late=False):
        zs, za = opaque(tile, 12), opaque(tile, 13)
        never = mask(zs)
        slot = tile % 2
        out = [o2_ref.at[1 - slot]]

        def rows(h, r0):
            lo, n = (0, Mh) if h is None else h if isinstance(h, tuple) else (h * Mq, Mq)
            return slice(r0 + lo, r0 + lo + n)

        def ld(loc, h):
            return loc[0][(0,) + loc[1] + (rows(h, loc[2]),)]

        def st(loc, v, h):
            loc[0][(zs,) + loc[1] + (rows(h, loc[2]),)] = v

        def operand(ref, idx, n):
            if cfg.get('NOBC'):
                return ref[idx + (slice(0, n),)]
            return pltpu.bitcast(ref.bitcast(u32)[idx + (slice(0, n // 2),)], bf16)

        def dot3(l, p, q, r):
            kind = next(x for x in KINDS if q in PAIR[x])
            return _dot(operand(s3[(p, kind)], (0, PAIR[kind].index(q), ORD.index(r)), Mq),
                        operand(t3_ref, (l, PRODS3.index((p, q)), ORD.index(r)), 128))

        def issue(l, p, rd):
            kind, n = rd
            if kind == 'x':
                return [dot3(l, p, q, 1) for q in (3, 5, 4, 7)]
            if kind == 'y':
                return [dot3(l, x, q, 1) for x in (p, GUEST[p]) for q in (2, 6)]
            if isinstance(n, str):
                return [dot3(l, p, int(q), int(r)) for q in kind for r in n]
            lhs = {q: [operand(s2[p], (0, k, pos2(p, q)), Mh) for k in range(2)] for q in map(int, kind)}
            return [_dot(lhs[q][k], operand(t2[p], (l, nn, k, pos2(p, q)), 128))
                    for q, nn in ([(1, 0), (1, 1)] if kind == '1' else [(int(q), n) for q in kind]) for k in range(2)]

        def biased(v, l, *site):
            if site not in sites:
                return v
            return (v.reshape(Mq // 8, 8, 128) + bt_ref[l, sites[site]]).reshape(Mq, 128)

        wait = {}
        def outer_act(l, p, i, j, n, d, h, part=None):
            stores, finals = OACT[p]
            if part == 'park':
                stores, finals = stores[:1], []
            elif part == 'rest' or (p == 6 and (i, j) != B12 and (h, n) != B12):
                stores = stores[1:]
            cache = {'d': d}
            def comb(terms):
                for t in terms.split():
                    if t[1:] not in cache:
                        cache[t[1:]] = ld(oloc(t[1:], i, j, n), h)
                return lincomb([(int(t[0] + '1'), cache[t[1:]]) for t in terms.split()])
            fin = [(IJ, comb(terms)) for IJ, terms in finals]
            for name, v in [(name, comb(terms)) for name, terms in stores]:
                st(oloc(name, i, j, n), v, h)
            for (I, J), y in fin:
                R, C = 2 * I + i, 2 * J + j
                xn = ld(x0loc(R, C, n), h) * y
                if l > 0:
                    xn = xn + ld(xloc(l, R, C, n), h)
                if l < L - 1:
                    st(xloc(l + 1, R, C, n), xn, h)
                    continue
                s = scale(R, C, rows(h, 0).start // Mq, n)
                xn = xn if s == 1.0 else xn * (1.0 / s)
                c0 = phys(C, n) * 128
                if i == 0:
                    out[0][rows(h, R * Mh), c0:c0 + 128] = xn.astype(bf16)
                elif j == 1:
                    wait[J] = xn
                else:
                    out[0][rows(h, R * Mh), c0:c0 + 256] = jnp.concatenate([xn, wait.pop(J)], axis=1).astype(bf16)

        def inner_act(g, l, p, kind, n, h, P, Q, part=None):
            vloc = iloc(g, 'v', n) if p == 1 else oloc(OACT[p][0][0][0], 0, 1, n)
            if kind == '35':
                st(iloc(g, 's', n), Q + ld(iloc(g, 'm1', n), h), h)
                if p == 1:
                    st(vloc, P, h)
                outer_act(l, p, 0, 1, n, P, h, part)
            elif kind == '47':
                st(iloc(g, 'u', n), Q + ld(vloc, h), h)
                outer_act(l, p, 0, 0, n, P + ld(iloc(g, 's', n), h), h, part)
            else:
                outer_act(l, p, 1, 1, n, ld(iloc(g, 's', n), h) - Q, h, part)
                outer_act(l, p, 1, 0, n, P + ld(iloc(g, 'u', n), h), h, part)

        def consume(g, l, p, rd, res):
            kind, n = rd
            if n == '1':
                for u, (kd, x) in enumerate([('35', p), ('47', p)] if kind == 'x' else [('26', p), ('26', GUEST[p])]):
                    for al in range(2):
                        st(jloc(kd, '1', al, x != p), biased(res[2 * u + al], l, x, int(kd[al]), '1'), 0)
            elif isinstance(n, str):
                sm = [res[2 * al] + res[2 * al + 1] for al in range(2)]
                df = [res[2 * al] - res[2 * al + 1] for al in range(2)]
                J = lambda name, al: ld(jloc(kind, name, al, name == '1' and kind == '26' and p not in GUEST), 0)
                part = 'park' if deferred(l, p, rd) else None
                done = lambda h, nn, m: inner_act(g, l, p, kind, nn, h, m[0] + m[1], m[0] - m[1], part)
                if n == '35':
                    for al in range(2):
                        st(jloc(kind, 's', al), df[al] + J('1', al), 0)
                    done(0, 1, [biased(sm[al], l, p, int(kind[al]), 'v') for al in range(2)])
                elif n == '47':
                    for al in range(2):
                        st(jloc(kind, 'k', al), biased(df[al], l, p, int(kind[al]), 'k'), 0)
                    done(0, 0, [biased(sm[al] + J('s', al), l, p, int(kind[al]), 'm') for al in range(2)])
                else:
                    O = lambda i, j: ld(oloc(OACT[p][0][0][0], i, j, 1), 0)
                    m = [sm[al] + J('k', al) for al in range(2)]
                    P = m[0] + m[1] + O(*{'35': B12, '47': B11, '26': B21}[kind])
                    Q = m[0] - m[1] - (ld(iloc(g, 'm1', 1), 0) if kind == '35' else O(*{'47': B12, '26': B22}[kind]))
                    done(1, 1, [J('s', al) - df[al] for al in range(2)])
                    inner_act(g, l, p, kind, 0, 1, P, Q, part)
            else:
                m = []
                for al, (q, nn) in enumerate([(1, 0), (1, 1)] if kind == '1' else [(int(q), n) for q in kind]):
                    v = res[2 * al] + res[2 * al + 1]
                    if any((p, q, (h, nn)) in sites for h in range(2)):
                        v = jnp.concatenate([biased(v[h * Mq:(h + 1) * Mq], l, p, q, (h, nn)) for h in range(2)], axis=0)
                    m.append(v)
                if kind == '1':
                    for nn in range(2):
                        st(iloc(g, 'm1', nn), m[nn], None)
                else:
                    inner_act(g, l, p, kind, n, None, m[0] + m[1], m[0] - m[1])

        def finish(l, p, pieces, nr, anchor):
            for i, j, n, r0 in pieces:
                d = ld(oloc(OACT[p][0][0][0], i, j, n), (r0, nr))
                outer_act(l, p, i, j, n, tie(d, anchor), (r0, nr), 'rest')

        if only_late:
            for x in late:
                finish(*x, None)
            out_copy(tile - 1, 1 - slot, 4).start()
            return carry
        state = {}
        count.clear()
        for g, rd, t0, n in sched:
            l, p = outs[g]
            if t0 == start[1]:
                pl.when(tile > 0)(lambda: out_copy(tile - 1, 1 - slot, 4).start())
                out[0] = o2_ref.at[slot]
            if t0 == first(G - 2, '35'):
                assert t0 > start[G - 2] + cfg['EW7']
                out_copy(tile, slot, 0).start()
            res = issue(l, p, rd)
            if t0 == first(G - 2, '35'):
                out[0][TM - 8:TM, 0:128] = res[0][0:8, :].astype(bf16)
            for t in range(t0, t0 + n):
                if t in plan:
                    r0 = 16 * (t - t0) + 8
                    anchor = (never, res[0 if isinstance(rd[1], str) else 1][r0:r0 + 8, :])
                for kind, fn, group in plan.get(t, []):
                    if kind == 'fin':
                        finish(*fn, anchor)
                    elif kind == 'conv':
                        conv(xn2_ref.at[1 - slot], *fn, zs, anchor)
                    else:
                        fn(state.setdefault(id(fn), {}), group, zs, za, anchor)
            if t0 == first(G - 1, '26'):
                out_copy(tile, slot, 1).start()
            if t0 + n == T:
                out_copy(tile, slot, 2).start()
                out_copy(tile, slot, 3).start()
            consume(g, l, p, rd, res)
        pl.when(tile + 3 < NMAIN)(lambda: in_copy(tile + 3, 1 - slot).start())
        pl.when(tile > 0)(lambda: out_copy(tile - 1, 1 - slot, None).wait())
        pl.when(tile + 2 < NMAIN)(lambda: in_copy(tile + 2, slot).wait())
        return carry

    prologue()
    in_copy(2, 0).start()
    in_copy(1, 1).wait()
    jax.lax.fori_loop(0, NMAIN, main, 0)
    main(jnp.int32(NMAIN), 0, True)
    xr_out.wait()
    out_copy(NMAIN - 1, (NMAIN - 1) % 2, None).wait()


def build(TM=640, **kw):
    def f(x0, ws, bs):
        B, D = x0.shape
        L = ws.shape[0]
        Mh = TM // 4
        nmain = (B - 1) // TM
        R0 = B - nmain * TM
        assert D == 1024 and L % 2 == 0 and L <= 8 and TM % 128 == 0 and R0 % 16 == 0 and nmain >= 3
        n3 = len(PRODS3)
        odd = lambda n: 16 * (n // 16 | 1)
        V = pltpu.VMEM
        scratch = ([V((1, 2, 2, 2, Mh + 40, 128), f32)] * 4 + [V((1, 2, 4, 2, Mh + 40, 128), f32)] * 7
                   + [V((1, Mh + 32, 128), f32)] * (16 + 64 + 20)
                   + [V((1, 2, 10 if p == 1 else 2, odd(Mh), 128), bf16) for p in range(1, 8)]
                   + [V((1, 2, 10, odd(Mh // 2), 128), bf16)] * (n3 // 2)
                   + [V((L, 2, 2, 7 if p == 1 else 1, 128, 128), bf16) for p in range(1, 8)]
                   + [V((L, n3, 7, 128, 128), bf16)] + [V((1, 4, 16 * n3 + 16, 128), f32)] * 2
                   + [V((L, 64, 8, 128), f32), V((8, 1, D), f32), V((2, TM, D), bf16), V((2, TM, D), bf16),
                      V((L, 8, 8, 16, D), bf16), V((R0, D), bf16), V((2, R0, D), f32), V((L, D), bf16),
                      pltpu.SemaphoreType.DMA((L + 14,))])
        anyspec = pl.BlockSpec(memory_space=pl.ANY)
        return pl.pallas_call(
            functools.partial(_kernel, L=L, TM=TM, R0=R0, NMAIN=nmain, D=D, cfg=dict(CFG, **kw)),
            in_specs=[anyspec, anyspec, anyspec],
            out_specs=anyspec,
            out_shape=jax.ShapeDtypeStruct((B, D), x0.dtype),
            scratch_shapes=scratch,
            compiler_params=pltpu.CompilerParams(
                vmem_limit_bytes=120 * 1024 * 1024,
                internal_scratch_in_bytes=65536,
                disable_bounds_checks=True,
            ),
        )(x0, ws.reshape(L, 8, 8, 16, D), bs)
    return f


@jax.jit
def pallas_standalone__dcn_v2_cross__recsys_kernel(x0, ws, bs):
    return build()(x0, ws, bs)
```

```python
import functools

import jax
import jax.numpy as jnp
import numpy as np
import jax.experimental.pallas as pl
import jax.experimental.pallas.tpu as pltpu

f32 = jnp.float32
bf16 = jnp.bfloat16
u32 = jnp.uint32

B11, B12, B21, B22 = BLOCKS = (0, 0), (0, 1), (1, 0), (1, 1)
LA = {1: [(B11, 1), (B22, 1)], 3: [(B11, 1), (B12, -1)], 5: [(B11, 1), (B12, 1)], 4: [(B12, 1), (B22, 1)],
      7: [(B12, 1), (B22, -1)]}
PC = {1: (1, 0, 0, 1), 2: (0, 0, 1, -1), 3: (1, 1, 1, 1), 4: (1, 0, 1, 0), 5: (-1, 1, 1, -1), 6: (0, 0, 1, 1),
      7: (1, 0, -1, 0)}
KINDS = ('35', '47', '26')
PAIR = {'35': (5, 3), '47': (4, 7), '26': (2, 6)}
ORD = (3, 5, 4, 7, 1, 2, 6)
OUTER = (3, 5, 1, 4, 7, 2, 6)
GUEST = {3: 5, 4: 7, 2: 6}
PRODS3 = [(p, q) for p in OUTER if p != 1 for kind in KINDS for q in PAIR[kind]]
GAMMA = 0.125
OACT = {
    3: ([('M3', '+d')], []),
    5: ([('M5', '+d')], [(B12, '+d +M3')]),
    1: ([('S', '+d +M3 -M5')], []),
    4: ([('M4', '+d')], []),
    7: ([('M7', '+d')], [(B11, '+d +S +M4')]),
    2: ([('M2', '+d')], []),
    6: ([('M6', '+d')], [(B22, '+d +S -M2'), (B21, '+d +M2 +M4 -M7 +M3 +M5')]),
}
OSL = {'M3': 0, 'M5': 1, 'S': 2, 'M4': 3, 'M7': 4, 'M2': 5, 'M6': 6}
ISL = {'m1': 0, 's': 1, 'v': 2, 'u': 3}
DEFER = {5: [('26', '26'), ('47', '26')], 7: [('26', '26'), ('47', '26')],
         6: [('35', '26'), ('47', '26'), ('26', '35'), ('26', '47'), ('26', '26')]}
SAVE = {5: B12, 1: B11, 7: B22, 2: B21}
STAGES = {1: [(None, 1.0)], 2: [((B11, B12), .4), ((B21, B22), .6)], 'O': [((B11, B12), .5), ((B21, B22), .5)],
          3: [((B11, B12), .35), ((B22,), .37), ((B21,), .28)],
          4: [((B11,), .16), ((B12,), .26), ((B22,), .31), ((B21,), .27)]}
LAG = 8
CFG = dict(CAP=0.95, PORT=0.9, CS=0.5, CL=0.3, VK=0.7, TAIL=3, EW7=12, EW6=40, MOFF=15, GE=8, NSLAB=6, JM=3)


def _dot(a, b):
    return jnp.dot(a, b, preferred_element_type=f32)


def scale(R, C, h, k):
    return 2.0 ** (R // 2 + R % 2 + h - C // 2 - C % 2 - k)


def phys(C, k):
    return 4 * (C // 2) + 2 * k + C % 2


def b_ops(b11, b12, b21, b22):
    r1 = b11 + b22
    g = b12 + b21
    return {1: r1, 2: b11 - b12, 3: b12 - b22, 4: g - r1, 5: b12 + b22, 6: b11 + b12, 7: g + r1}


def lincomb(terms):
    assert terms[0][0] == 1
    acc = terms[0][1]
    for s, v in terms[1:]:
        acc = acc + v if s == 1 else acc - v
    return acc


def rounds_of(p):
    if p == 1:
        return [('1', None)] + [(kind, n) for kind in KINDS for n in range(2)]
    minis = lambda kind: [(kind, r) for r in KINDS]
    return [('1', None), ('x', '1')] + minis('35') + minis('47') + [('y', '1')] * (p in GUEST) + minis('26')


def round_usage(p, rd, first, last, defer):
    stores, finals = OACT[p]
    kind, n = rd
    alu = sum(len(t.split()) - 1 for _, t in stores) + sum(len(t.split()) + (not first) + 2 * last for _, t in finals)
    nst = len(stores) + len(finals)
    if last and kind == '26':
        alu, nst = alu - 0.7 * len(finals), nst - 0.5 * len(finals)
    if defer:
        alu, nst = 0, 1
    elif p == 6 and kind != '35' and n != '35':
        nst -= 1
    if n == '1':
        a, st, m = 0, 4, 0
    elif isinstance(n, str):
        a, st, m = {'35': ((9, 3, 1), (16, 2, 2)), '47': ((10, 3, 1), (18, 2, 2)), '26': ((10, 2, 2), (18, 0, 4))}[kind][n == '26']
    else:
        a, st, m = {'1': (2, 2, 0), '35': (5, 2, 1), '47': (6, 1, 1), '26': (6, 0, 2)}[kind]
    return a + m * alu, st + m * nst


def bias_sites():
    cand = []
    for p in OUTER:
        for rd in rounds_of(p):
            kind, n = rd
            if n == '1':
                pq = [(p, q) for q in (3, 5, 4, 7)] if kind == 'x' else [(x, q) for x in (p, GUEST[p]) for q in (2, 6)]
                cand += [(p, rd, x + ('1',), (1, 0, 0, 1)) for x in pq]
            elif n in ('35', '47'):
                where = [('v', (0, 1, 1, 0))] if n == '35' else [('k', (0, 0, 1, 0)), ('m', (1, 0, 0, 0))]
                cand += [(p, rd, (p, int(q), w), pat) for q in kind for w, pat in where]
            elif n != '26':
                cand += [(p, rd, (p, int(q), (h, nn)), tuple(int(e == 2 * h + nn) for e in range(4)))
                         for q in kind for nn in ((0, 1) if kind == '1' else (n,)) for h in range(2)]
    extra, sites, rows = {}, [], []
    def busy(c):
        a, st = round_usage(c[0], c[1], False, False, c[1] in DEFER.get(c[0], ()))
        return 2 * (a + extra.get(c[:2], 0)) + st + (5 if isinstance(c[1][1], str) else 3)
    while len(sites) < 64:
        c = min(cand, key=busy)
        cand.remove(c)
        row = np.kron(np.kron(PC[c[2][0]], PC[c[2][1]]), c[3])
        if np.linalg.matrix_rank(np.array(rows + [row])) > len(rows):
            rows.append(row)
            sites.append(c[2])
            extra[c[:2]] = extra.get(c[:2], 0) + (1 if isinstance(c[1][1], str) else 0.5)
    want = np.zeros((64, 8))
    for e, (I, J, i, j, h, n) in enumerate(np.ndindex(*(2,) * 6)):
        want[e, phys(2 * J + j, n)] = scale(2 * I + i, 2 * J + j, h, n) / GAMMA
    coef = np.round(np.linalg.solve(np.array(rows, float).T, want) * 4096) / 4096
    assert (np.array(rows).T @ coef == want).all()
    return {x: e for e, x in enumerate(sites) if coef[e].any()}, coef, extra


def yds(groups, cap):
    n = len(cap)
    speed, cls, gcls = [0.0] * n, [-1] * n, {}
    todo = list(groups)
    while todo:
        pre = [0.0]
        for t in range(n):
            pre.append(pre[-1] + (cap[t] if cls[t] < 0 else 0.0))
        best = None
        for a in sorted({g[0] for g in todo}):
            w = 0.0
            for g in sorted((g for g in todo if g[0] >= a), key=lambda g: g[1]):
                w += g[2]
                d = w / max(pre[g[1] + 1] - pre[a], 1e-9)
                if best is None or d > best[0]:
                    best = (d, a, g[1])
        d, a, b = best
        for t in range(a, b + 1):
            if cls[t] < 0:
                speed[t], cls[t] = d, len(gcls)
        gcls.update({g[:2]: len(gcls) for g in todo if g[0] >= a and g[1] <= b})
        todo = [g for g in todo if not (g[0] >= a and g[1] <= b)]
    return speed, cls, gcls


def spread_jobs(jobs, cap, vcap, tail):
    T = len(cap)
    cap3 = cap * 3
    all3 = [(j[0] + k * T, j[1] + k * T, ji, k) for k in range(3) for ji, j in enumerate(jobs) if j[0] + k * T >= 0]
    pend = {}
    for j in sorted(all3, key=lambda j: (j[1], j[3], j[2])):
        pend.setdefault(j[:2], []).append(j)
    left = {w: sum(sum(jobs[j[2]][2]) for j in q) for w, q in pend.items()}
    speed, cls, gcls = yds([w + (left[w],) for w in pend], cap3)
    cum = [0.0]
    for t in range(3 * T):
        cum.append(cum[-1] + speed[t] * cap3[t])
    when = [[] for _ in jobs]
    debt, vdebt, cur, done = 0.0, 0.0, None, 0

    def fits(j, t):
        need = max(debt, 0.0) + sum(jobs[j[2]][2]) + 1.0
        for w in pend:
            if w[1] >= j[1]:
                break
            if left[w] > 1e-9:
                need += left[w]
                if need > cum[w[1] + 1] - cum[t]:
                    return False
        return True

    for t in range(3 * T):
        if t % T == 0:
            debt, vdebt = min(debt, 0.0), -0.5
        while True:
            rdy = [q[0] for w, q in pend.items() if q and w[0] <= t and (gcls[w] == cls[t] or w[1] <= t)]
            j = cur
            if j is None:
                if not rdy:
                    debt = max(debt, 0.0)
                    break
                j = rdy[0]
                if j[1] > t:
                    j = (min if vdebt > 0 else max)([x for x in rdy if x is j or fits(x, t)], key=lambda x: jobs[x[2]][3])
                nst = len(jobs[j[2]][2])
                if nst > 1 and j[1] > t and (t + tail + 2 * nst) // T != t // T:
                    break
            must = j[1] <= t or (cur is not None and ((t + tail + 1) // T != t // T or (rdy and rdy[0][1] <= t)))
            if not must and (cap3[t] == 0.0 or debt > 0.5 * speed[t] * cap3[t]):
                break
            if cur is None:
                pend[j[:2]].pop(0)
                left[j[:2]] -= sum(jobs[j[2]][2])
                cur, done = j, 0
            debt += jobs[j[2]][2][done]
            vdebt += jobs[j[2]][2][done] * jobs[j[2]][3]
            if j[3] == 1:
                when[j[2]].append(t - T)
            done += 1
            if done == len(jobs[j[2]][2]):
                cur = None
        debt -= speed[t] * cap3[t]
        vdebt = min(max(vdebt - vcap[t % T], -0.5), 1.0)
    assert all(j[0] <= ts[0] and ts[-1] <= j[1] and (ts[0] < 0) == (ts[-1] < 0) for j, ts in zip(jobs, when))
    return when


def _kernel(x_hbm, w_hbm, b_hbm, o_hbm, *scratch, L, TM, R0, NMAIN, D, cfg):
    H, Mh, Mq = D // 4, TM // 4, TM // 8
    NC, NQ = Mh // 16, Mq // 16
    it = iter(scratch)
    take = lambda n: [next(it) for _ in range(n)]
    x0b, xb, ib, ob, jb = take(4), take(7), take(16), take(56), take(20)
    s2 = dict(zip(range(1, 8), take(7)))
    s3 = {(p, kind): next(it) for p in OUTER if p != 1 for kind in KINDS}
    t2 = dict(zip(range(1, 8), take(7)))
    t3_ref, kb0, kb1, bt_ref, bf_ref, xn2_ref, o2_ref, w_ref, xr_ref, xp_ref, b_ref, sem = it
    sites, bcoef, extra = bias_sites()
    pos2 = lambda p, q: ORD.index(q) if p == 1 else 0

    xset = lambda l: 6 if l == 'O' else 4 if l == 0 else (l % 2) * 2
    xoff = lambda I, J: 16 * ((I + J) % 2)
    xloc = lambda l, R, C, k: (xb[xset(l) + R // 2], (R % 2, C, k), xoff(R // 2, C // 2))
    x0loc = lambda R, C, k: (x0b[(R // 2) * 2 + C // 2], (R % 2, C % 2, k), 8 + xoff(R // 2, C // 2))
    iloc = lambda g, name, n: (ib[((g % 2) * 4 + ISL[name]) * 2 + n], (), 8 * ISL[name])
    oloc = lambda name, i, j, n: (ob[(OSL[name] * 4 + i * 2 + j) * 2 + n], (), 8 * ((OSL[name] + 2 * j) % 4))

    def jloc(kind, name, al, guest=False):
        u = ('1', 's', 'k').index(name)
        return jb[18 + al if guest else (KINDS.index(kind) * 3 + u) * 2 + al], (), 8 * ((3 * u + al) % 4)

    def tie(v, anchor, r=None, lo=0):
        if anchor is None:
            return v
        never, gate = anchor
        if r is None:
            n = v.shape[0]
            return jax.lax.select(never[n], gate if n == 8 else jnp.tile(gate, (n // 8, 1)), v)
        top = jax.lax.select(never[8], gate, v[r:r + 8])
        return jnp.concatenate(([v[lo:r]] if r > lo else []) + [top, v[r + 8:r + 16]], axis=0)

    def consts(anchor, ss):
        one = {s: tie(jnp.full((8, 128), s, f32), anchor) for s in set(ss)}
        return jnp.concatenate([one[s] for s in ss for _ in range(2)], axis=0)

    def conv(src, R, Q, r, zs, anchor):
        v = src[R * Mh + r:R * Mh + r + 32, Q * H:(Q + 1) * H].astype(f32)
        for j in range(2):
            C, k = 2 * (Q // 2) + j, Q % 2
            buf, idx, off = xloc(0, R, C, k)
            sv = consts(anchor, [scale(R, C, (r + u) // Mq, k) for u in (0, 16)])
            buf[(zs,) + idx + (slice(off + r, off + r + 32),)] = v[:, j * 128:(j + 1) * 128] * sv

    count = {}
    def block_sum(l, terms, ii, jj, kk, r, save, zs, za, anchor, gate=True):
        rng = lambda t: slice(t[0], t[-1] + 1)
        vals = []
        for u, ((I, J), s) in enumerate(terms):
            ref, r0 = xb[xset(l) + I], xoff(I, J) + r
            v = ref[za if u == 0 else 0, rng(ii), 2 * J + jj[0]:2 * J + jj[-1] + 1, rng(kk), r0:r0 + 16, :]
            if (I, J) == save:
                sv = consts(anchor, [GAMMA / scale(2 * I + i, 2 * J + j, r // Mq, k) for i in ii for j in jj for k in kk])
                x0b[I * 2 + J][zs, rng(ii), rng(jj), rng(kk), r0 + 8:r0 + 24, :] = v * sv.reshape(v.shape)
            if u == 0 and gate:
                count[xset(l)] = count.get(xset(l), -1) + 1
                if count[xset(l)] % cfg['GE'] == 0:
                    ref[0, 0, 0, 0, Mh + 24:Mh + 32, :] = anchor[1]
            vals.append((s, v))
        v = lincomb(vals)
        return v.reshape(v.size // 128, 128)

    def operands(a, group, st8, store):
        for u, b in enumerate(group):
            st8[b] = a if len(group) == 1 else a[:, u:u + 1]
        ops = {}
        if B12 in group:
            ops[3], ops[5] = st8[B11] - st8[B12], st8[B11] + st8[B12]
        if B22 in group:
            ops[4], ops[7] = st8[B12] + st8[B22], st8[B12] - st8[B22]
            ops[1] = st8['l1'] = st8[B11] + st8[B22]
        if B21 in group:
            g = st8[B12] + st8[B21]
            ops[2], ops[6] = g + st8['l1'], g - st8['l1']
        now = [q for q in ORD if q in ops]
        if now:
            u = ORD.index(now[0])
            store(slice(u, u + len(now)), jnp.concatenate([ops[q] for q in now], axis=1).astype(bf16))

    def unit1(l, c, k, save, st8, group, zs, za, anchor):
        def store(pos, v):
            s2[1][zs, k:k + 1, pos, 16 * c:16 * c + 16, :] = v
        e = block_sum(l, LA[1], [group[0][0]], [0, 1], [k], 16 * c, save, zs, za, anchor)
        operands(tie(e, anchor, 16).reshape(1, 2, 16, 128), group, st8, store)

    def unit26(l, c, k, save, st8, group, zs, za, anchor):
        i = group[0][0]
        f = block_sum(l, [(B11, 1), (B22, 1)], [i], [0, 1], [k], 16 * c, save, zs, za, anchor, False)
        e = tie(block_sum(l, [(B12, 1), (B21, 1)], [i], [0, 1], [k], 16 * c, save, zs, za, anchor), anchor)
        for J, v in enumerate((e + f, e - f)):
            r0 = xoff(0, J) + 16 * c
            xb[6][zs, i, 2 * J:2 * J + 2, k, r0:r0 + 16, :] = v.reshape(2, 16, 128)

    def unit3(l, p, kind, c, save, st8, group, zs, za, anchor):
        def store(pos, v):
            s3[(p, kind)][zs, :, pos, 16 * c:16 * c + 16, :] = v
        h, kk = group[0][0], [b[1] for b in group]
        ii, jj = {'35': ([0], [0, 1]), '47': ([0, 1], [1]), '26': ([0, 1], [0, 1])}[kind]
        src = (l, LA[p]) if p in LA else ('O', [((0, (2, 6).index(p)), 1)])
        n = 16 * len(kk)
        v = block_sum(*src, ii, jj, kk, h * Mq + 16 * c, save, zs, za, anchor)
        if kind == '26':
            e, f = tie(v, anchor, 16, 16) + v[32:48], v[0:16] + v[48:64]
            r0 = h * Mq + 16 * c
            s2[p][zs, kk[0], 0, r0:r0 + 16, :] = f.astype(bf16)
        else:
            e, f = tie(v, anchor, n - 16), v[n:]
        operands(jnp.concatenate([e + f, e - f], axis=0).reshape(2, len(kk), 16, 128), group, st8, store)

    NPREP = 32 + len(PRODS3)
    def prep(l, u, anchors, zero, kb):
        mul = lambda v, s: v if s == 1.0 else v * s
        stack = lambda T: jnp.concatenate([T[q] for q in ORD], axis=0).reshape(7, 16, 128).astype(bf16)
        rows = pl.ds(16 * u, 16) if isinstance(u, int) else pl.ds(pl.multiple_of(16 * u, 16), 16)
        for k in range(2):
            wide = [w_ref[l, phys(R, k), u].astype(f32) for R in range(4)]
            for n in range(2):
                anchor = next(anchors)
                blk = lambda R, C: mul(wide[R][:, phys(C, n) * 128:(phys(C, n) + 1) * 128], scale(R, C, k, n))
                O = {(i, j): b_ops(blk(i, j), tie(blk(i, 2 + j), anchor, 0), blk(2 + i, j), blk(2 + i, 2 + j))
                     for i, j in BLOCKS}
                for p in (2, 6, 3, 5, 1, 4, 7):
                    o = [mul(O[b][p], 4.0 if p == 1 else 1.0) for b in BLOCKS]
                    T = b_ops(o[0], tie(o[1], next(anchors), 0), o[2], o[3])
                    if p == 1:
                        T[1] = T[1] * 2.0
                        t2[p][l, n, k, :, rows, :] = stack(T)
                        continue
                    t2[p][l, n, k, 0, rows, :] = (T[1] * 4.0).astype(bf16)
                    e0 = PRODS3.index((p, 5))
                    if (k, n) != (1, 1):
                        kb[zero, k * 2 + n, 16 * e0:16 * e0 + 96, :] = jnp.concatenate(
                            [T[q] for _, q in PRODS3[e0:e0 + 6]], axis=0)
                        continue
                    for e in range(e0, e0 + 6):
                        v = kb[0, 0:3, 16 * e:16 * e + 16, :]
                        T3 = b_ops(v[0], tie(v[1], next(anchors), 0), v[2], T[PRODS3[e][1]])
                        T3[1] = T3[1] * 2.0
                        t3_ref[l, e, :, rows, :] = stack(T3)

    outs = [(l, p) for l in range(L) for p in OUTER]
    G = len(outs)
    sched, start, use, vuse = [], [], [], []
    for g, (l, p) in enumerate(outs):
        start.append(len(use))
        for rd in rounds_of(p):
            n = NQ if isinstance(rd[1], str) else NC
            sched.append((g, rd, len(use), n))
            a, st_ = round_usage(p, rd, l == 0, l == L - 1, rd in DEFER.get(p, ()))
            a += extra.get((p, rd), 0)
            use += [max((2 * a + st_ + 2 + 16 / n) / 72, cfg['PORT'] * st_ / 8)] * n
            vuse += [st_ / 8] * n
    T = len(use)
    first = lambda g, kind: next(t0 for gg, rd, t0, _ in sched if gg == g and rd[0] == kind)
    jobs, late = [], []
    def add(lo, hi, alu, st_, ld_, scheme, kind, fn):
        w = alu / 64 + cfg['CS'] * (st_ + len(STAGES[scheme])) / 16 + cfg['CL'] * ld_ / 48
        jobs.append((lo, max(hi, lo), [w * f for _, f in STAGES[scheme]], st_ / 16 / w, scheme, kind, fn))
    for g, (l, p) in enumerate(outs):
        for gg, rd, t0, n_ in sched:
            if gg == g and rd in DEFER.get(p, ()):
                last = l == L - 1
                nops = 4 * (sum(len(t.split()) for _, t in OACT[p][0][1:]) + sum(len(t.split()) + 2 + 2 * last for _, t in OACT[p][1]))
                ws = [(i, j, n, h * Mq + 16 * c) for c in range(NQ)
                      for h, n in {'35': [B12], '47': [B11], '26': [B22, B21]}[rd[1]]
                      for i, j in {'35': [B12], '47': [B11], '26': [B22, B21]}[rd[0]]]
                if last and p == 6 and rd[0] == '26':
                    for u in range(0, len(ws), 2):
                        for r8 in (0, 8):
                            late.append((l, p, [w[:3] + (w[3] + r8,) for w in ws[u:u + 2]], 8))
                            add(0, cfg['EW6'] - 1, nops * 0.45, 1, nops * 0.4, 1, 'fin', late[-1])
                    continue
                due = {5: lambda: start[7 * l + 5] - 1,
                       7: lambda: start[g + 1] + cfg['EW7'],
                       6: lambda: T - cfg['TAIL'] - 1 if last else min(start[g + 1] + cfg['EW6'], first(g + 1, rd[0])) - 1}[p]()
                m = 1 if p == 6 else 2
                for u in range(0, len(ws), m):
                    add(t0 + n_, due, nops * m // 2, 3, nops * m // 2, 1, 'fin', (l, p, ws[u:u + m], 16))
        if p in (3, 5):
            lo = start[7 * l - 2] + (cfg['EW7'] + 1 if l else -T)
        else:
            lo = start[7 * l] + cfg['EW6']
        hi = start[g] - LAG - 3
        save = SAVE.get(p) if l == 0 else None
        sv = save is not None
        if p == 1:
            for c, k in np.ndindex(NC, 2):
                add(lo, hi, 31 + 8 * sv, 7 + 8 * sv, 16, 2, l, functools.partial(unit1, l, c, k, save))
            continue
        nt = 2
        if p in (2, 6):
            mid = start[7 * l + 3] + cfg['MOFF']
            if p == 2:
                for c, k in np.ndindex(NC, 2):
                    add(lo, mid - 3, 40 + 8 * sv, 16 + 8 * sv, 32, 'O', l, functools.partial(unit26, l, c, k, save))
            lo, nt, save, sv = mid, 1, None, False
        for c in range(NQ):
            add(lo, hi if p in GUEST else first(g - 1, 'y') - LAG - 3, 32 * nt + 50 + 32 * sv, 18 + 32 * sv, 32 * nt,
                4, l, functools.partial(unit3, l, p, '26', c, save))
        for c in range(NQ):
            for kind in KINDS[:2]:
                add(lo, hi + (NC if g else 0), 16 * nt + 46, 14, 16 * nt, 3, l, functools.partial(unit3, l, p, kind, c, None))
    convs = [(R, Q, r) for R in range(4) for Q in range(4) for r in range(0, Mh, 32)]
    for x in convs:
        add(start[6], start[G - 2] - 2, 18, 7, 4, 1, 'conv', x)
    cap = [max(cfg['CAP'] - max(use[t], use[(t + 1) % T]), 0.0) * (t < T - cfg['TAIL']) for t in range(T)]
    when = spread_jobs(jobs, cap, [cfg['VK'] * (1 - vuse[(t + 1) % T]) for t in range(T)], cfg['TAIL'])
    plan = {}
    for t, _, ji, u in sorted((t % T, ts[0] % T, ji, u) for ji, ts in enumerate(when) for u, t in enumerate(ts)):
        plan.setdefault(t, []).append((jobs[ji][5], jobs[ji][6], STAGES[jobs[ji][4]][u][0]))
    carried = [job for ts, job in zip(when, jobs) if ts[0] < 0]

    def w_copy(l):
        return pltpu.make_async_copy(w_hbm.at[l], w_ref.at[l], sem.at[l])

    def w0_copy(u):
        return pltpu.make_async_copy(w_hbm.at[0, :, u], w_ref.at[0, :, u], sem.at[L + 6 + u])

    def in_copy(t, slot):
        return pltpu.make_async_copy(x_hbm.at[pl.ds(pl.multiple_of(t * TM, 32), TM)], xn2_ref.at[slot], sem.at[L + slot])

    def out_copy(t, slot, part):
        r0, nr = (0, TM) if part is None else ((0, 4 * Mq), (4 * Mq, Mq), (5 * Mq, Mq), (6 * Mq, 2 * Mq))[part]
        return pltpu.make_async_copy(o2_ref.at[slot, pl.ds(r0, nr)],
                                     o_hbm.at[pl.ds(pl.multiple_of(t * TM + r0, 16), nr)], sem.at[L + 4 + slot])

    xr_in = pltpu.make_async_copy(x_hbm.at[pl.ds(NMAIN * TM, R0)], xr_ref, sem.at[L + 2])
    xr_out = pltpu.make_async_copy(xr_ref, o_hbm.at[pl.ds(NMAIN * TM, R0)], sem.at[L + 2])
    b_in = pltpu.make_async_copy(b_hbm, b_ref, sem.at[L + 3])
    opaque = lambda i, s: jax.lax.shift_right_logical(i, s)
    mask = lambda zero: {n: jnp.broadcast_to(zero, (n, 128)) != 0 for n in (8, 16, 32)}

    def prologue():
        b_in.start()
        for u in range(8):
            w0_copy(u).start()
        xr_in.start()
        in_copy(0, 0).start()
        for l in range(1, L):
            w_copy(l).start()
        in_copy(1, 1).start()
        b_in.wait()
        for l in range(L):
            bf_ref[l] = b_ref[l:l + 1, :].astype(f32)

        def bias_tiles(l, carry):
            b = jnp.broadcast_to(bf_ref[l] + (l == 0).astype(f32), (8, D))
            for u in sites.values():
                terms = [b[:, e * 128:(e + 1) * 128] * float(cf) for e, cf in enumerate(bcoef[u]) if cf != 0.0]
                bt_ref[l, u] = functools.reduce(lambda x, y: x + y, terms)
            return carry
        jax.lax.fori_loop(0, L, bias_tiles, 0)
        if cfg.get('FAST'):
            return

        def slab(u, carry):
            w0_copy(u).wait()
            prep(0, u, iter(lambda: None, 0), opaque(u, 12), kb0)
            return opaque(u, 12)
        zero = jax.lax.fori_loop(0, cfg['NSLAB'], slab, 0)

        def plain(l, xbf, x0f, x, j0, j1, na, free, never):
            passes = []
            for jt in range(j0, j1):
                cols = slice(jt * 128, (jt + 1) * 128)
                ya = _dot(xbf[:, :D // 2], w_ref[l, 0:4, :, :, cols].reshape(D // 2, 128)) + bf_ref[l, :, cols]
                passes += [ya, _dot(xbf[:, D // 2:], w_ref[l, 4:8, :, :, cols].reshape(D // 2, 128)) + ya]
            xp_ref[0, :, j0 * 128:j1 * 128] = x0f * jnp.concatenate(passes[1::2], axis=1) + x
            for u in range(na):
                ps, rr = divmod((u - free) * len(passes) * (R0 // 8) // (na - free), R0 // 8)
                yield None if u < free else (never, passes[ps][rr * 8:rr * 8 + 8, :])

        for u in range(cfg['NSLAB'], 8):
            w0_copy(u).wait()
        xr_in.wait()
        jm = cfg['JM']
        x0f = xr_ref[:, :jm * 128].astype(f32)
        xp_ref[1, :, :jm * 128] = x0f
        anchors = plain(0, xr_ref[...], x0f, x0f, 0, jm, (8 - cfg['NSLAB']) * NPREP, 2, mask(zero))
        for u in range(cfg['NSLAB'], 8):
            prep(0, u, anchors, zero, (kb0, kb1)[u % 2])
        in_copy(0, 0).wait()
        x0f = xr_ref[:, jm * 128:].astype(f32)
        xp_ref[1, :, jm * 128:] = x0f
        blank = [loc for j, n in BLOCKS for loc in [oloc(x, 1, j, n) for x in OSL]
                 + [f(3, 2 * J + j, n) for J in range(2) for f in (x0loc, functools.partial(xloc, L - 1))]]
        na = len(convs) + sum(len(j[2]) for j in carried) + 2 * len(blank) + 2
        anchors = plain(0, xr_ref[...], x0f, x0f, jm, 8, na, 4, mask(zero))
        for x in convs[:len(convs) // 2]:
            conv(xn2_ref.at[0], *x, zero, next(anchors))
        for job in carried:
            st8 = {}
            for group, _ in STAGES[job[4]]:
                job[6](st8, group, zero, opaque(zero, 1), next(anchors))
        for x in convs[len(convs) // 2:]:
            conv(xn2_ref.at[0], *x, zero, next(anchors))
        for ref, idx, off in blank:
            for r0 in (off, off + Mq):
                ref[(0,) + idx + (slice(r0, r0 + Mq),)] = consts(next(anchors), [0.0] * NQ)

        def layer(l, carry):
            w_copy(l).wait()
            x, zero = xp_ref[0], opaque(l, 12)
            anchors = plain(l, x.astype(bf16), xp_ref[1], x, 0, 8, 8 * NPREP, 2, mask(zero))
            for u in range(8):
                prep(l, u, anchors, zero, (kb0, kb1)[u % 2])
            return carry

        jax.lax.fori_loop(1, L, layer, 0)
        xr_ref[...] = xp_ref[0].astype(bf16)
        xr_out.start()

    def main(tile, carry, only_late=False):
        zs, za = opaque(tile, 12), opaque(tile, 13)
        never = mask(zs)
        slot = tile % 2
        out = [o2_ref.at[1 - slot]]

        def rows(h, r0):
            lo, n = (0, Mh) if h is None else h if isinstance(h, tuple) else (h * Mq, Mq)
            return slice(r0 + lo, r0 + lo + n)

        def ld(loc, h):
            return loc[0][(0,) + loc[1] + (rows(h, loc[2]),)]

        def st(loc, v, h):
            loc[0][(zs,) + loc[1] + (rows(h, loc[2]),)] = v

        def operand(ref, idx, n):
            if cfg.get('NOBC'):
                return ref[idx + (slice(0, n),)]
            return pltpu.bitcast(ref.bitcast(u32)[idx + (slice(0, n // 2),)], bf16)

        def dot3(l, p, q, r):
            kind = next(x for x in KINDS if q in PAIR[x])
            return _dot(operand(s3[(p, kind)], (0, PAIR[kind].index(q), ORD.index(r)), Mq),
                        operand(t3_ref, (l, PRODS3.index((p, q)), ORD.index(r)), 128))

        def issue(l, p, rd):
            kind, n = rd
            if kind == 'x':
                return [dot3(l, p, q, 1) for q in (3, 5, 4, 7)]
            if kind == 'y':
                return [dot3(l, x, q, 1) for x in (p, GUEST[p]) for q in (2, 6)]
            if isinstance(n, str):
                return [dot3(l, p, int(q), int(r)) for q in kind for r in n]
            lhs = {q: [operand(s2[p], (0, k, pos2(p, q)), Mh) for k in range(2)] for q in map(int, kind)}
            return [_dot(lhs[q][k], operand(t2[p], (l, nn, k, pos2(p, q)), 128))
                    for q, nn in ([(1, 0), (1, 1)] if kind == '1' else [(int(q), n) for q in kind]) for k in range(2)]

        def biased(v, l, *site):
            if site not in sites:
                return v
            return (v.reshape(Mq // 8, 8, 128) + bt_ref[l, sites[site]]).reshape(Mq, 128)

        wait = {}
        def outer_act(l, p, i, j, n, d, h, part=None):
            stores, finals = OACT[p]
            if part == 'park':
                stores, finals = stores[:1], []
            elif part == 'rest' or (p == 6 and (i, j) != B12 and (h, n) != B12):
                stores = stores[1:]
            cache = {'d': d}
            def comb(terms):
                for t in terms.split():
                    if t[1:] not in cache:
                        cache[t[1:]] = ld(oloc(t[1:], i, j, n), h)
                return lincomb([(int(t[0] + '1'), cache[t[1:]]) for t in terms.split()])
            fin = [(IJ, comb(terms)) for IJ, terms in finals]
            for name, v in [(name, comb(terms)) for name, terms in stores]:
                st(oloc(name, i, j, n), v, h)
            for (I, J), y in fin:
                R, C = 2 * I + i, 2 * J + j
                xn = ld(x0loc(R, C, n), h) * y
                if l > 0:
                    xn = xn + ld(xloc(l, R, C, n), h)
                if l < L - 1:
                    st(xloc(l + 1, R, C, n), xn, h)
                    continue
                s = scale(R, C, rows(h, 0).start // Mq, n)
                xn = xn if s == 1.0 else xn * (1.0 / s)
                c0 = phys(C, n) * 128
                if i == 0:
                    out[0][rows(h, R * Mh), c0:c0 + 128] = xn.astype(bf16)
                elif j == 1:
                    wait[J] = xn
                else:
                    out[0][rows(h, R * Mh), c0:c0 + 256] = jnp.concatenate([xn, wait.pop(J)], axis=1).astype(bf16)

        def inner_act(g, l, p, kind, n, h, P, Q, part=None):
            vloc = iloc(g, 'v', n) if p == 1 else oloc(OACT[p][0][0][0], 0, 1, n)
            if kind == '35':
                st(iloc(g, 's', n), Q + ld(iloc(g, 'm1', n), h), h)
                if p == 1:
                    st(vloc, P, h)
                outer_act(l, p, 0, 1, n, P, h, part)
            elif kind == '47':
                st(iloc(g, 'u', n), Q + ld(vloc, h), h)
                outer_act(l, p, 0, 0, n, P + ld(iloc(g, 's', n), h), h, part)
            else:
                outer_act(l, p, 1, 1, n, ld(iloc(g, 's', n), h) - Q, h, part)
                outer_act(l, p, 1, 0, n, P + ld(iloc(g, 'u', n), h), h, part)

        def consume(g, l, p, rd, res):
            kind, n = rd
            if n == '1':
                for u, (kd, x) in enumerate([('35', p), ('47', p)] if kind == 'x' else [('26', p), ('26', GUEST[p])]):
                    for al in range(2):
                        st(jloc(kd, '1', al, x != p), biased(res[2 * u + al], l, x, int(kd[al]), '1'), 0)
            elif isinstance(n, str):
                sm = [res[2 * al] + res[2 * al + 1] for al in range(2)]
                df = [res[2 * al] - res[2 * al + 1] for al in range(2)]
                J = lambda name, al: ld(jloc(kind, name, al, name == '1' and kind == '26' and p not in GUEST), 0)
                part = 'park' if rd in DEFER.get(p, ()) else None
                done = lambda h, nn, m: inner_act(g, l, p, kind, nn, h, m[0] + m[1], m[0] - m[1], part)
                if n == '35':
                    for al in range(2):
                        st(jloc(kind, 's', al), df[al] + J('1', al), 0)
                    done(0, 1, [biased(sm[al], l, p, int(kind[al]), 'v') for al in range(2)])
                elif n == '47':
                    for al in range(2):
                        st(jloc(kind, 'k', al), biased(df[al], l, p, int(kind[al]), 'k'), 0)
                    done(0, 0, [biased(sm[al] + J('s', al), l, p, int(kind[al]), 'm') for al in range(2)])
                else:
                    O = lambda i, j: ld(oloc(OACT[p][0][0][0], i, j, 1), 0)
                    m = [sm[al] + J('k', al) for al in range(2)]
                    P = m[0] + m[1] + O(*{'35': B12, '47': B11, '26': B21}[kind])
                    Q = m[0] - m[1] - (ld(iloc(g, 'm1', 1), 0) if kind == '35' else O(*{'47': B12, '26': B22}[kind]))
                    done(1, 1, [J('s', al) - df[al] for al in range(2)])
                    inner_act(g, l, p, kind, 0, 1, P, Q, part)
            else:
                m = []
                for al, (q, nn) in enumerate([(1, 0), (1, 1)] if kind == '1' else [(int(q), n) for q in kind]):
                    v = res[2 * al] + res[2 * al + 1]
                    if any((p, q, (h, nn)) in sites for h in range(2)):
                        v = jnp.concatenate([biased(v[h * Mq:(h + 1) * Mq], l, p, q, (h, nn)) for h in range(2)], axis=0)
                    m.append(v)
                if kind == '1':
                    for nn in range(2):
                        st(iloc(g, 'm1', nn), m[nn], None)
                else:
                    inner_act(g, l, p, kind, n, None, m[0] + m[1], m[0] - m[1])

        def finish(l, p, pieces, nr, anchor):
            for i, j, n, r0 in pieces:
                d = ld(oloc(OACT[p][0][0][0], i, j, n), (r0, nr))
                outer_act(l, p, i, j, n, tie(d, anchor), (r0, nr), 'rest')

        if only_late:
            for x in late:
                finish(*x, None)
            out_copy(tile - 1, 1 - slot, 3).start()
            return carry
        state = {}
        count.clear()
        for g, rd, t0, n in sched:
            l, p = outs[g]
            if t0 == start[1]:
                pl.when(tile > 0)(lambda: out_copy(tile - 1, 1 - slot, 3).start())
                out[0] = o2_ref.at[slot]
            if t0 == first(G - 2, '35'):
                assert t0 > start[G - 2] + cfg['EW7']
                out_copy(tile, slot, 0).start()
            res = issue(l, p, rd)
            if t0 == first(G - 2, '35'):
                out[0][TM - 8:TM, 0:128] = res[0][0:8, :].astype(bf16)
            for t in range(t0, t0 + n):
                if t in plan:
                    r0 = 16 * (t - t0) + 8
                    anchor = (never, res[0 if isinstance(rd[1], str) else 1][r0:r0 + 8, :])
                for kind, fn, group in plan.get(t, []):
                    if kind == 'fin':
                        finish(*fn, anchor)
                    elif kind == 'conv':
                        conv(xn2_ref.at[1 - slot], *fn, zs, anchor)
                    else:
                        fn(state.setdefault(id(fn), {}), group, zs, za, anchor)
            if t0 == first(G - 1, '26'):
                out_copy(tile, slot, 1).start()
            if t0 + n == T:
                out_copy(tile, slot, 2).start()
            consume(g, l, p, rd, res)
        pl.when(tile + 3 < NMAIN)(lambda: in_copy(tile + 3, 1 - slot).start())
        pl.when(tile > 0)(lambda: out_copy(tile - 1, 1 - slot, None).wait())
        pl.when(tile + 2 < NMAIN)(lambda: in_copy(tile + 2, slot).wait())
        return carry

    prologue()
    in_copy(2, 0).start()
    in_copy(1, 1).wait()
    jax.lax.fori_loop(0, NMAIN, main, 0)
    main(jnp.int32(NMAIN), 0, True)
    xr_out.wait()
    out_copy(NMAIN - 1, (NMAIN - 1) % 2, None).wait()


def build(TM=640, **kw):
    def f(x0, ws, bs):
        B, D = x0.shape
        L = ws.shape[0]
        Mh = TM // 4
        nmain = (B - 1) // TM
        R0 = B - nmain * TM
        assert D == 1024 and L % 2 == 0 and L <= 8 and TM % 128 == 0 and R0 % 16 == 0 and nmain >= 3
        n3 = len(PRODS3)
        odd = lambda n: 16 * (n // 16 | 1)
        V = pltpu.VMEM
        scratch = ([V((1, 2, 2, 2, Mh + 40, 128), f32)] * 4 + [V((1, 2, 4, 2, Mh + 40, 128), f32)] * 7
                   + [V((1, Mh + 32, 128), f32)] * (16 + 56 + 20)
                   + [V((1, 2, 10 if p == 1 else 2, odd(Mh), 128), bf16) for p in range(1, 8)]
                   + [V((1, 2, 10, odd(Mh // 2), 128), bf16)] * (n3 // 2)
                   + [V((L, 2, 2, 7 if p == 1 else 1, 128, 128), bf16) for p in range(1, 8)]
                   + [V((L, n3, 7, 128, 128), bf16)] + [V((1, 4, 16 * n3 + 16, 128), f32)] * 2
                   + [V((L, 64, 8, 128), f32), V((8, 1, D), f32), V((2, TM, D), bf16), V((2, TM, D), bf16),
                      V((L, 8, 8, 16, D), bf16), V((R0, D), bf16), V((2, R0, D), f32), V((L, D), bf16),
                      pltpu.SemaphoreType.DMA((L + 14,))])
        anyspec = pl.BlockSpec(memory_space=pl.ANY)
        return pl.pallas_call(
            functools.partial(_kernel, L=L, TM=TM, R0=R0, NMAIN=nmain, D=D, cfg=dict(CFG, **kw)),
            in_specs=[anyspec, anyspec, anyspec],
            out_specs=anyspec,
            out_shape=jax.ShapeDtypeStruct((B, D), x0.dtype),
            scratch_shapes=scratch,
            compiler_params=pltpu.CompilerParams(
                vmem_limit_bytes=120 * 1024 * 1024,
                internal_scratch_in_bytes=65536,
                disable_bounds_checks=True,
            ),
        )(x0, ws.reshape(L, 8, 8, 16, D), bs)
    return f


@jax.jit
def pallas_standalone__dcn_v2_cross__recsys_kernel(x0, ws, bs):
    return build()(x0, ws, bs)
```

```python
import functools

import jax
import jax.numpy as jnp
import numpy as np
import jax.experimental.pallas as pl
import jax.experimental.pallas.tpu as pltpu

f32 = jnp.float32
bf16 = jnp.bfloat16
u32 = jnp.uint32

B11, B12, B21, B22 = BLOCKS = (0, 0), (0, 1), (1, 0), (1, 1)
LA = {1: [(B11, 1), (B22, 1)], 3: [(B11, 1), (B12, -1)], 5: [(B11, 1), (B12, 1)], 4: [(B12, 1), (B22, 1)],
      7: [(B12, 1), (B22, -1)]}
PC = {1: (1, 0, 0, 1), 2: (0, 0, 1, -1), 3: (1, 1, 1, 1), 4: (1, 0, 1, 0), 5: (-1, 1, 1, -1), 6: (0, 0, 1, 1),
      7: (1, 0, -1, 0)}
KINDS = ('35', '47', '26')
PAIR = {'35': (5, 3), '47': (4, 7), '26': (2, 6)}
ORD = (3, 5, 4, 7, 1, 2, 6)
OUTER = (3, 5, 1, 4, 7, 2, 6)
GUEST = {3: 5, 4: 7, 2: 6}
PRODS3 = [(p, q) for p in OUTER if p != 1 for kind in KINDS for q in PAIR[kind]]
GAMMA = 0.125
OACT = {
    3: ([('M3', '+d')], []),
    5: ([('M5', '+d')], [(B12, '+d +M3')]),
    1: ([('S', '+d +M3 -M5')], []),
    4: ([('M4', '+d')], []),
    7: ([('M7', '+d')], [(B11, '+d +S +M4')]),
    2: ([('M2', '+d')], []),
    6: ([('M6', '+d')], [(B22, '+d +S -M2'), (B21, '+d +M2 +M4 -M7 +M3 +M5')]),
}
OSL = {'M3': 0, 'M5': 1, 'S': 2, 'M4': 3, 'M7': 4, 'M2': 5, 'M6': 6}
ISL = {'m1': 0, 's': 1, 'v': 2, 'u': 3}
DEFER = {5: [('26', '26'), ('47', '26'), ('35', '26')], 7: [('26', '26'), ('47', '26'), ('35', '26')],
         6: [('26', '26'), ('47', '26'), ('35', '26'), ('26', '35'), ('26', '47')]}
DONE = {'35': [B12], '47': [B11], '26': [B22, B21]}
SAVE = {5: B12, 1: B11, 7: B22, 2: B21}
STAGES = {1: [(None, 1.0)], 2: [((B11, B12), .4), ((B21, B22), .6)], 'O': [((B11, B12), .5), ((B21, B22), .5)],
          3: [((B11, B12), .35), ((B22,), .37), ((B21,), .28)],
          4: [((B11,), .16), ((B12,), .26), ((B22,), .31), ((B21,), .27)]}
LAG = 8
CFG = dict(FR=(24, 16, 16, 8), CAP=0.95, PORT=0.9, CS=0.5, CL=0.3, VK=0.7, TAIL=3, EW7=12, EW6=40, MOFF=15, GE=8, NSLAB=6, JM=3)


def _dot(a, b):
    return jnp.dot(a, b, preferred_element_type=f32)


def scale(R, C, h, k):
    return 2.0 ** (R // 2 + R % 2 + h - C // 2 - C % 2 - k)


def phys(C, k):
    return 4 * (C // 2) + 2 * k + C % 2


def b_ops(b11, b12, b21, b22):
    r1 = b11 + b22
    g = b12 + b21
    return {1: r1, 2: b11 - b12, 3: b12 - b22, 4: g - r1, 5: b12 + b22, 6: b11 + b12, 7: g + r1}


def lincomb(terms):
    assert terms[0][0] == 1
    acc = terms[0][1]
    for s, v in terms[1:]:
        acc = acc + v if s == 1 else acc - v
    return acc


def rounds_of(p):
    if p == 1:
        return [('1', None)] + [(kind, n) for kind in KINDS for n in range(2)]
    minis = lambda kind: [(kind, r) for r in KINDS]
    return [('1', None), ('x', '1')] + minis('35') + minis('47') + [('y', '1')] * (p in GUEST) + minis('26')


def round_usage(p, rd, first, last, defer):
    stores, finals = OACT[p]
    kind, n = rd
    alu = sum(len(t.split()) - 1 for _, t in stores) + sum(len(t.split()) + (not first) + 2 * last for _, t in finals)
    nst = len(stores) + len(finals)
    if last and kind == '26':
        alu, nst = alu - 0.7 * len(finals), nst - 0.5 * len(finals)
    if defer:
        alu, nst = 0, 1
    elif p == 6 and kind != '35' and n != '35':
        nst -= 1
    if n == '1':
        a, st, m = 0, 4, 0
    elif isinstance(n, str):
        a, st, m = {'35': ((9, 3, 1), (16, 2, 2)), '47': ((10, 3, 1), (18, 2, 2)), '26': ((10, 2, 2), (18, 0, 4))}[kind][n == '26']
    else:
        a, st, m = {'1': (2, 2, 0), '35': (5, 2, 1), '47': (6, 1, 1), '26': (6, 0, 2)}[kind]
    return a + m * alu, st + m * nst


def bias_sites():
    cand = []
    for p in OUTER:
        for rd in rounds_of(p):
            kind, n = rd
            if n == '1':
                pq = [(p, q) for q in (3, 5, 4, 7)] if kind == 'x' else [(x, q) for x in (p, GUEST[p]) for q in (2, 6)]
                cand += [(p, rd, x + ('1',), (1, 0, 0, 1)) for x in pq]
            elif n in ('35', '47'):
                where = [('v', (0, 1, 1, 0))] if n == '35' else [('k', (0, 0, 1, 0)), ('m', (1, 0, 0, 0))]
                cand += [(p, rd, (p, int(q), w), pat) for q in kind for w, pat in where]
            elif n != '26':
                cand += [(p, rd, (p, int(q), (h, nn)), tuple(int(e == 2 * h + nn) for e in range(4)))
                         for q in kind for nn in ((0, 1) if kind == '1' else (n,)) for h in range(2)]
    unit = lambda b: tuple(int(x == b) for x in BLOCKS)
    sites = [(b, leaf, sub) for p in DEFER for rd in DEFER[p] for b, _ in OACT[p][1]
             for leaf in DONE[rd[0]] for sub in DONE[rd[1]]]
    rows = [np.kron(np.kron(unit(b), unit(leaf)), unit(sub)) for b, leaf, sub in sites]
    extra = {}
    def busy(c):
        a, st = round_usage(c[0], c[1], False, False, c[1] in DEFER.get(c[0], ()))
        return 2 * (a + extra.get(c[:2], 0)) + st + (5 if isinstance(c[1][1], str) else 3)
    while len(sites) < 64:
        c = min(cand, key=busy)
        cand.remove(c)
        row = np.kron(np.kron(PC[c[2][0]], PC[c[2][1]]), c[3])
        if np.linalg.matrix_rank(np.array(rows + [row])) > len(rows):
            rows.append(row)
            sites.append(c[2])
            extra[c[:2]] = extra.get(c[:2], 0) + (1 if isinstance(c[1][1], str) else 0.5)
    want = np.zeros((64, 8))
    for e, (I, J, i, j, h, n) in enumerate(np.ndindex(*(2,) * 6)):
        want[e, phys(2 * J + j, n)] = scale(2 * I + i, 2 * J + j, h, n) / GAMMA
    coef = np.round(np.linalg.solve(np.array(rows, float).T, want) * 4096) / 4096
    assert (np.array(rows).T @ coef == want).all()
    return {x: e for e, x in enumerate(sites) if coef[e].any() or isinstance(x[1], tuple)}, coef, extra


def yds(groups, cap):
    n = len(cap)
    speed, cls, gcls = [0.0] * n, [-1] * n, {}
    todo = list(groups)
    while todo:
        pre = [0.0]
        for t in range(n):
            pre.append(pre[-1] + (cap[t] if cls[t] < 0 else 0.0))
        best = None
        for a in sorted({g[0] for g in todo}):
            w = 0.0
            for g in sorted((g for g in todo if g[0] >= a), key=lambda g: g[1]):
                w += g[2]
                d = w / max(pre[g[1] + 1] - pre[a], 1e-9)
                if best is None or d > best[0]:
                    best = (d, a, g[1])
        d, a, b = best
        for t in range(a, b + 1):
            if cls[t] < 0:
                speed[t], cls[t] = d, len(gcls)
        gcls.update({g[:2]: len(gcls) for g in todo if g[0] >= a and g[1] <= b})
        todo = [g for g in todo if not (g[0] >= a and g[1] <= b)]
    return speed, cls, gcls


def spread_jobs(jobs, cap, vcap, tail):
    T = len(cap)
    cap3 = cap * 3
    all3 = [(j[0] + k * T, j[1] + k * T, ji, k) for k in range(3) for ji, j in enumerate(jobs) if j[0] + k * T >= 0]
    pend = {}
    for j in sorted(all3, key=lambda j: (j[1], j[3], j[2])):
        pend.setdefault(j[:2], []).append(j)
    left = {w: sum(sum(jobs[j[2]][2]) for j in q) for w, q in pend.items()}
    speed, cls, gcls = yds([w + (left[w],) for w in pend], cap3)
    cum = [0.0]
    for t in range(3 * T):
        cum.append(cum[-1] + speed[t] * cap3[t])
    when = [[] for _ in jobs]
    debt, vdebt, cur, done = 0.0, 0.0, None, 0

    def fits(j, t):
        need = max(debt, 0.0) + sum(jobs[j[2]][2]) + 1.0
        for w in pend:
            if w[1] >= j[1]:
                break
            if left[w] > 1e-9:
                need += left[w]
                if need > cum[w[1] + 1] - cum[t]:
                    return False
        return True

    for t in range(3 * T):
        if t % T == 0:
            debt, vdebt = min(debt, 0.0), -0.5
        while True:
            rdy = [q[0] for w, q in pend.items() if q and w[0] <= t and (gcls[w] == cls[t] or w[1] <= t)]
            j = cur
            if j is None:
                if not rdy:
                    debt = max(debt, 0.0)
                    break
                j = rdy[0]
                if j[1] > t:
                    j = (min if vdebt > 0 else max)([x for x in rdy if x is j or fits(x, t)], key=lambda x: jobs[x[2]][3])
                nst = len(jobs[j[2]][2])
                if nst > 1 and j[1] > t and (t + tail + 2 * nst) // T != t // T:
                    break
            must = j[1] <= t or (cur is not None and ((t + tail + 1) // T != t // T or (rdy and rdy[0][1] <= t)))
            if not must and (cap3[t] == 0.0 or debt > 0.5 * speed[t] * cap3[t]):
                break
            if cur is None:
                pend[j[:2]].pop(0)
                left[j[:2]] -= sum(jobs[j[2]][2])
                cur, done = j, 0
            debt += jobs[j[2]][2][done]
            vdebt += jobs[j[2]][2][done] * jobs[j[2]][3]
            if j[3] == 1:
                when[j[2]].append(t - T)
            done += 1
            if done == len(jobs[j[2]][2]):
                cur = None
        debt -= speed[t] * cap3[t]
        vdebt = min(max(vdebt - vcap[t % T], -0.5), 1.0)
    assert all(j[0] <= ts[0] and ts[-1] <= j[1] and (ts[0] < 0) == (ts[-1] < 0) for j, ts in zip(jobs, when))
    return when


def _kernel(x_hbm, w_hbm, b_hbm, o_hbm, *scratch, L, TM, R0, NMAIN, D, cfg):
    H, Mh, Mq = D // 4, TM // 4, TM // 8
    NC, NQ = Mh // 16, Mq // 16
    it = iter(scratch)
    take = lambda n: [next(it) for _ in range(n)]
    x0b, xb, ib, ob, jb = take(4), take(7), take(16), take(56), take(20)
    s2 = dict(zip(range(1, 8), take(7)))
    s3 = {(p, kind): next(it) for p in OUTER if p != 1 for kind in KINDS}
    t2 = dict(zip(range(1, 8), take(7)))
    t3_ref, kb0, kb1, bt_ref, bf_ref, xn2_ref, o2_ref, w_ref, xr_ref, xp_ref, b_ref, sem = it
    sites, bcoef, extra = bias_sites()
    pos2 = lambda p, q: ORD.index(q) if p == 1 else 0

    xset = lambda l: 6 if l == 'O' else 4 if l == 0 else (l % 2) * 2
    xoff = lambda I, J: 16 * ((I + J) % 2)
    xloc = lambda l, R, C, k: (xb[xset(l) + R // 2], (R % 2, C, k), xoff(R // 2, C // 2))
    x0loc = lambda R, C, k: (x0b[(R // 2) * 2 + C // 2], (R % 2, C % 2, k), 8 + xoff(R // 2, C // 2))
    iloc = lambda g, name, n: (ib[((g % 2) * 4 + ISL[name]) * 2 + n], (), 8 * ISL[name])
    oloc = lambda name, i, j, n: (ob[(OSL[name] * 4 + i * 2 + j) * 2 + n], (), 8 * ((OSL[name] + 2 * j) % 4))

    def jloc(kind, name, al, guest=False):
        u = ('1', 's', 'k').index(name)
        return jb[18 + al if guest else (KINDS.index(kind) * 3 + u) * 2 + al], (), 8 * ((3 * u + al) % 4)

    def tie(v, anchor, r=None, lo=0):
        if anchor is None:
            return v
        never, gate = anchor
        if r is None:
            n = v.shape[0]
            return jax.lax.select(never[n], gate if n == 8 else jnp.tile(gate, (n // 8, 1)), v)
        top = jax.lax.select(never[8], gate, v[r:r + 8])
        return jnp.concatenate(([v[lo:r]] if r > lo else []) + [top, v[r + 8:r + 16]], axis=0)

    def consts(anchor, ss):
        one = {s: tie(jnp.full((8, 128), s, f32), anchor) for s in set(ss)}
        return jnp.concatenate([one[s] for s in ss for _ in range(2)], axis=0)

    def conv(src, R, Q, r, zs, anchor):
        v = src[R * Mh + r:R * Mh + r + 32, Q * H:(Q + 1) * H].astype(f32)
        for j in range(2):
            C, k = 2 * (Q // 2) + j, Q % 2
            buf, idx, off = xloc(0, R, C, k)
            sv = consts(anchor, [scale(R, C, (r + u) // Mq, k) for u in (0, 16)])
            buf[(zs,) + idx + (slice(off + r, off + r + 32),)] = v[:, j * 128:(j + 1) * 128] * sv

    count = {}
    def block_sum(l, terms, ii, jj, kk, r, save, zs, za, anchor, gate=True):
        rng = lambda t: slice(t[0], t[-1] + 1)
        vals = []
        for u, ((I, J), s) in enumerate(terms):
            ref, r0 = xb[xset(l) + I], xoff(I, J) + r
            v = ref[za if u == 0 else 0, rng(ii), 2 * J + jj[0]:2 * J + jj[-1] + 1, rng(kk), r0:r0 + 16, :]
            if (I, J) == save:
                sv = consts(anchor, [GAMMA / scale(2 * I + i, 2 * J + j, r // Mq, k) for i in ii for j in jj for k in kk])
                x0b[I * 2 + J][zs, rng(ii), rng(jj), rng(kk), r0 + 8:r0 + 24, :] = v * sv.reshape(v.shape)
            if u == 0 and gate:
                count[xset(l)] = count.get(xset(l), -1) + 1
                if count[xset(l)] % cfg['GE'] == 0:
                    ref[0, 0, 0, 0, Mh + 24:Mh + 32, :] = anchor[1]
            vals.append((s, v))
        v = lincomb(vals)
        return v.reshape(v.size // 128, 128)

    def operands(a, group, st8, store):
        for u, b in enumerate(group):
            st8[b] = a if len(group) == 1 else a[:, u:u + 1]
        ops = {}
        if B12 in group:
            ops[3], ops[5] = st8[B11] - st8[B12], st8[B11] + st8[B12]
        if B22 in group:
            ops[4], ops[7] = st8[B12] + st8[B22], st8[B12] - st8[B22]
            ops[1] = st8['l1'] = st8[B11] + st8[B22]
        if B21 in group:
            g = st8[B12] + st8[B21]
            ops[2], ops[6] = g + st8['l1'], g - st8['l1']
        now = [q for q in ORD if q in ops]
        if now:
            u = ORD.index(now[0])
            store(slice(u, u + len(now)), jnp.concatenate([ops[q] for q in now], axis=1).astype(bf16))

    def unit1(l, c, k, save, st8, group, zs, za, anchor):
        def store(pos, v):
            s2[1][zs, k:k + 1, pos, 16 * c:16 * c + 16, :] = v
        e = block_sum(l, LA[1], [group[0][0]], [0, 1], [k], 16 * c, save, zs, za, anchor)
        operands(tie(e, anchor, 16).reshape(1, 2, 16, 128), group, st8, store)

    def unit26(l, c, k, save, st8, group, zs, za, anchor):
        i = group[0][0]
        f = block_sum(l, [(B11, 1), (B22, 1)], [i], [0, 1], [k], 16 * c, save, zs, za, anchor, False)
        e = tie(block_sum(l, [(B12, 1), (B21, 1)], [i], [0, 1], [k], 16 * c, save, zs, za, anchor), anchor)
        for J, v in enumerate((e + f, e - f)):
            r0 = xoff(0, J) + 16 * c
            xb[6][zs, i, 2 * J:2 * J + 2, k, r0:r0 + 16, :] = v.reshape(2, 16, 128)

    def unit3(l, p, kind, c, save, st8, group, zs, za, anchor):
        def store(pos, v):
            s3[(p, kind)][zs, :, pos, 16 * c:16 * c + 16, :] = v
        h, kk = group[0][0], [b[1] for b in group]
        ii, jj = {'35': ([0], [0, 1]), '47': ([0, 1], [1]), '26': ([0, 1], [0, 1])}[kind]
        src = (l, LA[p]) if p in LA else ('O', [((0, (2, 6).index(p)), 1)])
        n = 16 * len(kk)
        v = block_sum(*src, ii, jj, kk, h * Mq + 16 * c, save, zs, za, anchor)
        if kind == '26':
            e, f = tie(v, anchor, 16, 16) + v[32:48], v[0:16] + v[48:64]
            r0 = h * Mq + 16 * c
            s2[p][zs, kk[0], 0, r0:r0 + 16, :] = f.astype(bf16)
        else:
            e, f = tie(v, anchor, n - 16), v[n:]
        operands(jnp.concatenate([e + f, e - f], axis=0).reshape(2, len(kk), 16, 128), group, st8, store)

    NPREP = 32 + len(PRODS3)
    def prep(l, u, anchors, zero, kb):
        mul = lambda v, s: v if s == 1.0 else v * s
        stack = lambda T: jnp.concatenate([T[q] for q in ORD], axis=0).reshape(7, 16, 128).astype(bf16)
        rows = pl.ds(16 * u, 16) if isinstance(u, int) else pl.ds(pl.multiple_of(16 * u, 16), 16)
        for k in range(2):
            wide = [w_ref[l, phys(R, k), u].astype(f32) for R in range(4)]
            for n in range(2):
                anchor = next(anchors)
                blk = lambda R, C: mul(wide[R][:, phys(C, n) * 128:(phys(C, n) + 1) * 128], scale(R, C, k, n))
                O = {(i, j): b_ops(blk(i, j), tie(blk(i, 2 + j), anchor, 0), blk(2 + i, j), blk(2 + i, 2 + j))
                     for i, j in BLOCKS}
                for p in (2, 6, 3, 5, 1, 4, 7):
                    o = [mul(O[b][p], 4.0 if p == 1 else 1.0) for b in BLOCKS]
                    T = b_ops(o[0], tie(o[1], next(anchors), 0), o[2], o[3])
                    if p == 1:
                        T[1] = T[1] * 2.0
                        t2[p][l, n, k, :, rows, :] = stack(T)
                        continue
                    t2[p][l, n, k, 0, rows, :] = (T[1] * 4.0).astype(bf16)
                    e0 = PRODS3.index((p, 5))
                    if (k, n) != (1, 1):
                        kb[zero, k * 2 + n, 16 * e0:16 * e0 + 96, :] = jnp.concatenate(
                            [T[q] for _, q in PRODS3[e0:e0 + 6]], axis=0)
                        continue
                    for e in range(e0, e0 + 6):
                        v = kb[0, 0:3, 16 * e:16 * e + 16, :]
                        T3 = b_ops(v[0], tie(v[1], next(anchors), 0), v[2], T[PRODS3[e][1]])
                        T3[1] = T3[1] * 2.0
                        t3_ref[l, e, :, rows, :] = stack(T3)

    outs = [(l, p) for l in range(L) for p in OUTER]
    G = len(outs)
    sched, start, use, vuse = [], [], [], []
    for g, (l, p) in enumerate(outs):
        start.append(len(use))
        for rd in rounds_of(p):
            n = NQ if isinstance(rd[1], str) else NC
            sched.append((g, rd, len(use), n))
            a, st_ = round_usage(p, rd, l == 0, l == L - 1, rd in DEFER.get(p, ()))
            a += extra.get((p, rd), 0)
            use += [max((2 * a + st_ + 2 + 16 / n) / 72, cfg['PORT'] * st_ / 8)] * n
            vuse += [st_ / 8] * n
    T = len(use)
    first = lambda g, kind: next(t0 for gg, rd, t0, _ in sched if gg == g and rd[0] == kind)
    jobs, late = [], []
    def add(lo, hi, alu, st_, ld_, scheme, kind, fn):
        w = alu / 64 + cfg['CS'] * (st_ + len(STAGES[scheme])) / 16 + cfg['CL'] * ld_ / 48
        jobs.append((lo, max(hi, lo), [w * f for _, f in STAGES[scheme]], st_ / 16 / w, scheme, kind, fn))
    for g, (l, p) in enumerate(outs):
        for gg, rd, t0, n_ in sched:
            if gg == g and rd in DEFER.get(p, ()):
                last = l == L - 1
                nops = sum(len(t.split()) + 1 + (l > 0) + 1.5 * last for _, t in OACT[p][1])
                islate = last and p == 6 and rd[0] == '26'
                due = {5: lambda: start[7 * l + 5] - 1, 7: lambda: start[g + 1] + cfg['EW7'],
                       6: lambda: T - cfg['TAIL'] - 1 if last else min(start[g + 1] + cfg['EW6'], first(g + 1, rd[0])) - 1}[p]()
                both = last and rd[0] == '26'
                step = cfg['FR'][(p == 6) + 2 * both]
                for r0 in range(0, Mq, step):
                    nr = min(step, Mq - r0)
                    for h, n in DONE[rd[1]]:
                        for leaves in [DONE[rd[0]]] if both else [[b] for b in DONE[rd[0]]]:
                            fn = (l, p, leaves, h, n, r0, nr)
                            nv = len(leaves) * nr // 8
                            add(0 if islate else t0 + n_, cfg['EW6'] - 1 if islate else due, nops * nv,
                                nv * len(OACT[p][1]) / (1 + both) - 1, 0.9 * nops * nv, 1, 'fin', fn)
                            if islate:
                                late.append(fn)
        if p in (3, 5):
            lo = start[7 * l - 2] + (cfg['EW7'] + 1 if l else -T)
        else:
            lo = start[7 * l] + cfg['EW6']
        hi = start[g] - LAG - 3
        save = SAVE.get(p) if l == 0 else None
        sv = save is not None
        if p == 1:
            for c, k in np.ndindex(NC, 2):
                add(lo, hi, 31 + 8 * sv, 7 + 8 * sv, 16, 2, l, functools.partial(unit1, l, c, k, save))
            continue
        nt = 2
        if p in (2, 6):
            mid = start[7 * l + 3] + cfg['MOFF']
            if p == 2:
                for c, k in np.ndindex(NC, 2):
                    add(lo, mid - 3, 40 + 8 * sv, 16 + 8 * sv, 32, 'O', l, functools.partial(unit26, l, c, k, save))
            lo, nt, save, sv = mid, 1, None, False
        for c in range(NQ):
            add(lo, hi if p in GUEST else first(g - 1, 'y') - LAG - 3, 32 * nt + 50 + 32 * sv, 18 + 32 * sv, 32 * nt,
                4, l, functools.partial(unit3, l, p, '26', c, save))
        for c in range(NQ):
            for kind in KINDS[:2]:
                add(lo, hi + (NC if g else 0), 16 * nt + 46, 14, 16 * nt, 3, l, functools.partial(unit3, l, p, kind, c, None))
    convs = [(R, Q, r) for R in range(4) for Q in range(4) for r in range(0, Mh, 32)]
    for x in convs:
        add(start[6], start[G - 2] - 2, 18, 7, 4, 1, 'conv', x)
    cap = [max(cfg['CAP'] - max(use[t], use[(t + 1) % T]), 0.0) * (t < T - cfg['TAIL']) for t in range(T)]
    when = spread_jobs(jobs, cap, [cfg['VK'] * (1 - vuse[(t + 1) % T]) for t in range(T)], cfg['TAIL'])
    plan = {}
    for t, _, ji, u in sorted((t % T, ts[0] % T, ji, u) for ji, ts in enumerate(when) for u, t in enumerate(ts)):
        plan.setdefault(t, []).append((jobs[ji][5], jobs[ji][6], STAGES[jobs[ji][4]][u][0]))
    carried = [job for ts, job in zip(when, jobs) if ts[0] < 0]

    def w_copy(l):
        return pltpu.make_async_copy(w_hbm.at[l], w_ref.at[l], sem.at[l])

    def w0_copy(u):
        return pltpu.make_async_copy(w_hbm.at[0, :, u], w_ref.at[0, :, u], sem.at[L + 6 + u])

    def in_copy(t, slot):
        return pltpu.make_async_copy(x_hbm.at[pl.ds(pl.multiple_of(t * TM, 32), TM)], xn2_ref.at[slot], sem.at[L + slot])

    def out_copy(t, slot, part):
        r0, nr = (0, TM) if part is None else ((0, 4 * Mq), (4 * Mq, Mq), (5 * Mq, Mq), (6 * Mq, 2 * Mq))[part]
        return pltpu.make_async_copy(o2_ref.at[slot, pl.ds(r0, nr)],
                                     o_hbm.at[pl.ds(pl.multiple_of(t * TM + r0, 16), nr)], sem.at[L + 4 + slot])

    xr_in = pltpu.make_async_copy(x_hbm.at[pl.ds(NMAIN * TM, R0)], xr_ref, sem.at[L + 2])
    xr_out = pltpu.make_async_copy(xr_ref, o_hbm.at[pl.ds(NMAIN * TM, R0)], sem.at[L + 2])
    b_in = pltpu.make_async_copy(b_hbm, b_ref, sem.at[L + 3])
    opaque = lambda i, s: jax.lax.shift_right_logical(i, s)
    mask = lambda zero: {n: jnp.broadcast_to(zero, (n, 128)) != 0 for n in (8, 16, 32)}

    def prologue():
        b_in.start()
        for u in range(8):
            w0_copy(u).start()
        xr_in.start()
        in_copy(0, 0).start()
        for l in range(1, L):
            w_copy(l).start()
        in_copy(1, 1).start()
        b_in.wait()
        for l in range(L):
            bf_ref[l] = b_ref[l:l + 1, :].astype(f32)

        def bias_tiles(l, carry):
            b = jnp.broadcast_to(bf_ref[l] + (l == 0).astype(f32), (8, D))
            for u in sites.values():
                terms = [b[:, e * 128:(e + 1) * 128] * float(cf) for e, cf in enumerate(bcoef[u]) if cf != 0.0]
                bt_ref[l, u] = functools.reduce(lambda x, y: x + y, terms or [jnp.zeros((8, 128), f32)])
            return carry
        jax.lax.fori_loop(0, L, bias_tiles, 0)
        if cfg.get('FAST'):
            return

        def slab(u, carry):
            w0_copy(u).wait()
            prep(0, u, iter(lambda: None, 0), opaque(u, 12), kb0)
            return opaque(u, 12)
        zero = jax.lax.fori_loop(0, cfg['NSLAB'], slab, 0)

        def plain(l, xbf, x0f, x, j0, j1, na, free, never):
            passes = []
            for jt in range(j0, j1):
                cols = slice(jt * 128, (jt + 1) * 128)
                ya = _dot(xbf[:, :D // 2], w_ref[l, 0:4, :, :, cols].reshape(D // 2, 128)) + bf_ref[l, :, cols]
                passes += [ya, _dot(xbf[:, D // 2:], w_ref[l, 4:8, :, :, cols].reshape(D // 2, 128)) + ya]
            xp_ref[0, :, j0 * 128:j1 * 128] = x0f * jnp.concatenate(passes[1::2], axis=1) + x
            for u in range(na):
                ps, rr = divmod((u - free) * len(passes) * (R0 // 8) // (na - free), R0 // 8)
                yield None if u < free else (never, passes[ps][rr * 8:rr * 8 + 8, :])

        for u in range(cfg['NSLAB'], 8):
            w0_copy(u).wait()
        xr_in.wait()
        jm = cfg['JM']
        x0f = xr_ref[:, :jm * 128].astype(f32)
        xp_ref[1, :, :jm * 128] = x0f
        anchors = plain(0, xr_ref[...], x0f, x0f, 0, jm, (8 - cfg['NSLAB']) * NPREP, 2, mask(zero))
        for u in range(cfg['NSLAB'], 8):
            prep(0, u, anchors, zero, (kb0, kb1)[u % 2])
        in_copy(0, 0).wait()
        x0f = xr_ref[:, jm * 128:].astype(f32)
        xp_ref[1, :, jm * 128:] = x0f
        blank = [loc for j, n in BLOCKS for loc in [oloc(x, 1, j, n) for x in OSL]
                 + [f(3, 2 * J + j, n) for J in range(2) for f in (x0loc, functools.partial(xloc, L - 1))]]
        na = len(convs) + sum(len(j[2]) for j in carried) + 2 * len(blank) + 2
        anchors = plain(0, xr_ref[...], x0f, x0f, jm, 8, na, 4, mask(zero))
        for x in convs[:len(convs) // 2]:
            conv(xn2_ref.at[0], *x, zero, next(anchors))
        for job in carried:
            st8 = {}
            for group, _ in STAGES[job[4]]:
                job[6](st8, group, zero, opaque(zero, 1), next(anchors))
        for x in convs[len(convs) // 2:]:
            conv(xn2_ref.at[0], *x, zero, next(anchors))
        for ref, idx, off in blank:
            for r0 in (off, off + Mq):
                ref[(0,) + idx + (slice(r0, r0 + Mq),)] = consts(next(anchors), [0.0] * NQ)

        def layer(l, carry):
            w_copy(l).wait()
            x, zero = xp_ref[0], opaque(l, 12)
            anchors = plain(l, x.astype(bf16), xp_ref[1], x, 0, 8, 8 * NPREP, 2, mask(zero))
            for u in range(8):
                prep(l, u, anchors, zero, (kb0, kb1)[u % 2])
            return carry

        jax.lax.fori_loop(1, L, layer, 0)
        xr_ref[...] = xp_ref[0].astype(bf16)
        xr_out.start()

    def main(tile, carry, only_late=False):
        zs, za = opaque(tile, 12), opaque(tile, 13)
        never = mask(zs)
        slot = tile % 2
        out = [o2_ref.at[1 - slot]]

        def rows(h, r0):
            lo, n = (0, Mh) if h is None else h if isinstance(h, tuple) else (h * Mq, Mq)
            return slice(r0 + lo, r0 + lo + n)

        def ld(loc, h):
            return loc[0][(0,) + loc[1] + (rows(h, loc[2]),)]

        def st(loc, v, h):
            loc[0][(zs,) + loc[1] + (rows(h, loc[2]),)] = v

        def operand(ref, idx, n):
            if cfg.get('NOBC'):
                return ref[idx + (slice(0, n),)]
            return pltpu.bitcast(ref.bitcast(u32)[idx + (slice(0, n // 2),)], bf16)

        def dot3(l, p, q, r):
            kind = next(x for x in KINDS if q in PAIR[x])
            return _dot(operand(s3[(p, kind)], (0, PAIR[kind].index(q), ORD.index(r)), Mq),
                        operand(t3_ref, (l, PRODS3.index((p, q)), ORD.index(r)), 128))

        def issue(l, p, rd):
            kind, n = rd
            if kind == 'x':
                return [dot3(l, p, q, 1) for q in (3, 5, 4, 7)]
            if kind == 'y':
                return [dot3(l, x, q, 1) for x in (p, GUEST[p]) for q in (2, 6)]
            if isinstance(n, str):
                return [dot3(l, p, int(q), int(r)) for q in kind for r in n]
            lhs = {q: [operand(s2[p], (0, k, pos2(p, q)), Mh) for k in range(2)] for q in map(int, kind)}
            return [_dot(lhs[q][k], operand(t2[p], (l, nn, k, pos2(p, q)), 128))
                    for q, nn in ([(1, 0), (1, 1)] if kind == '1' else [(int(q), n) for q in kind]) for k in range(2)]

        def biased(v, l, *site):
            if site not in sites:
                return v
            return (v.reshape(Mq // 8, 8, 128) + bt_ref[l, sites[site]]).reshape(Mq, 128)

        wait = {}
        def outer_act(l, p, i, j, n, d, h, part=None, last=lambda b, y: y):
            stores, finals = OACT[p]
            if part == 'park':
                stores, finals = stores[:1], []
            elif part == 'rest' or (p == 6 and (i, j) != B12 and (h, n) != B12):
                stores = stores[1:]
            cache = {'d': d}
            def comb(terms):
                for t in terms.split():
                    if t[1:] not in cache:
                        cache[t[1:]] = ld(oloc(t[1:], i, j, n), h)
                return lincomb([(int(t[0] + '1'), cache[t[1:]]) for t in terms.split()])
            fin = [(IJ, last(IJ, comb(terms))) for IJ, terms in finals]
            for name, v in [(name, comb(terms)) for name, terms in stores]:
                st(oloc(name, i, j, n), v, h)
            for (I, J), y in fin:
                R, C = 2 * I + i, 2 * J + j
                xn = ld(x0loc(R, C, n), h) * y
                if l > 0:
                    xn = xn + ld(xloc(l, R, C, n), h)
                if l < L - 1:
                    st(xloc(l + 1, R, C, n), xn, h)
                    continue
                s = scale(R, C, rows(h, 0).start // Mq, n)
                xn = xn if s == 1.0 else xn * (1.0 / s)
                c0 = phys(C, n) * 128
                if i == 0:
                    out[0][rows(h, R * Mh), c0:c0 + 128] = xn.astype(bf16)
                elif j == 1:
                    wait[J] = xn
                else:
                    out[0][rows(h, R * Mh), c0:c0 + 256] = jnp.concatenate([xn, wait.pop(J)], axis=1).astype(bf16)

        def inner_act(g, l, p, kind, n, h, P, Q, part=None):
            vloc = iloc(g, 'v', n) if p == 1 else oloc(OACT[p][0][0][0], 0, 1, n)
            if kind == '35':
                st(iloc(g, 's', n), Q + ld(iloc(g, 'm1', n), h), h)
                if p == 1:
                    st(vloc, P, h)
                outer_act(l, p, 0, 1, n, P, h, part)
            elif kind == '47':
                st(iloc(g, 'u', n), Q + ld(vloc, h), h)
                outer_act(l, p, 0, 0, n, P + ld(iloc(g, 's', n), h), h, part)
            else:
                outer_act(l, p, 1, 1, n, ld(iloc(g, 's', n), h) - Q, h, part)
                outer_act(l, p, 1, 0, n, P + ld(iloc(g, 'u', n), h), h, part)

        def consume(g, l, p, rd, res):
            kind, n = rd
            if n == '1':
                for u, (kd, x) in enumerate([('35', p), ('47', p)] if kind == 'x' else [('26', p), ('26', GUEST[p])]):
                    for al in range(2):
                        st(jloc(kd, '1', al, x != p), biased(res[2 * u + al], l, x, int(kd[al]), '1'), 0)
            elif isinstance(n, str):
                sm = [res[2 * al] + res[2 * al + 1] for al in range(2)]
                df = [res[2 * al] - res[2 * al + 1] for al in range(2)]
                J = lambda name, al: ld(jloc(kind, name, al, name == '1' and kind == '26' and p not in GUEST), 0)
                part = 'park' if rd in DEFER.get(p, ()) else None
                done = lambda h, nn, m: inner_act(g, l, p, kind, nn, h, m[0] + m[1], m[0] - m[1], part)
                if n == '35':
                    for al in range(2):
                        st(jloc(kind, 's', al), df[al] + J('1', al), 0)
                    done(0, 1, [biased(sm[al], l, p, int(kind[al]), 'v') for al in range(2)])
                elif n == '47':
                    for al in range(2):
                        st(jloc(kind, 'k', al), biased(df[al], l, p, int(kind[al]), 'k'), 0)
                    done(0, 0, [biased(sm[al] + J('s', al), l, p, int(kind[al]), 'm') for al in range(2)])
                else:
                    O = lambda i, j: ld(oloc(OACT[p][0][0][0], i, j, 1), 0)
                    m = [sm[al] + J('k', al) for al in range(2)]
                    P = m[0] + m[1] + O(*{'35': B12, '47': B11, '26': B21}[kind])
                    Q = m[0] - m[1] - (ld(iloc(g, 'm1', 1), 0) if kind == '35' else O(*{'47': B12, '26': B22}[kind]))
                    done(1, 1, [J('s', al) - df[al] for al in range(2)])
                    inner_act(g, l, p, kind, 0, 1, P, Q, part)
            else:
                m = []
                for al, (q, nn) in enumerate([(1, 0), (1, 1)] if kind == '1' else [(int(q), n) for q in kind]):
                    v = res[2 * al] + res[2 * al + 1]
                    if any((p, q, (h, nn)) in sites for h in range(2)):
                        v = jnp.concatenate([biased(v[h * Mq:(h + 1) * Mq], l, p, q, (h, nn)) for h in range(2)], axis=0)
                    m.append(v)
                if kind == '1':
                    for nn in range(2):
                        st(iloc(g, 'm1', nn), m[nn], None)
                else:
                    inner_act(g, l, p, kind, n, None, m[0] + m[1], m[0] - m[1])

        def finish(l, p, leaves, h, n, r0, nr, anchor):
            for i, j in leaves:
                d = ld(oloc(OACT[p][0][0][0], i, j, n), (h * Mq + r0, nr))
                last = lambda b, y: (y.reshape(nr // 8, 8, 128)
                                     + tie(bt_ref[l, sites[(b, (i, j), (h, n))]], anchor)).reshape(nr, 128)
                outer_act(l, p, i, j, n, d, (h * Mq + r0, nr), 'rest', last)

        if only_late:
            for x in late:
                finish(*x, None)
            out_copy(tile - 1, 1 - slot, 3).start()
            return carry
        state = {}
        count.clear()
        for g, rd, t0, n in sched:
            l, p = outs[g]
            if t0 == start[1]:
                pl.when(tile > 0)(lambda: out_copy(tile - 1, 1 - slot, 3).start())
                out[0] = o2_ref.at[slot]
            if t0 == first(G - 2, '35'):
                assert t0 > start[G - 2] + cfg['EW7']
                out_copy(tile, slot, 0).start()
            res = issue(l, p, rd)
            if t0 == first(G - 2, '35'):
                out[0][TM - 8:TM, 0:128] = res[0][0:8, :].astype(bf16)
            for t in range(t0, t0 + n):
                if t in plan:
                    r0 = 16 * (t - t0) + 8
                    anchor = (never, res[0 if isinstance(rd[1], str) else 1][r0:r0 + 8, :])
                for kind, fn, group in plan.get(t, []):
                    if kind == 'fin':
                        finish(*fn, anchor)
                    elif kind == 'conv':
                        conv(xn2_ref.at[1 - slot], *fn, zs, anchor)
                    else:
                        fn(state.setdefault(id(fn), {}), group, zs, za, anchor)
            if t0 == first(G - 1, '26'):
                out_copy(tile, slot, 1).start()
            if t0 + n == T:
                out_copy(tile, slot, 2).start()
            consume(g, l, p, rd, res)
        pl.when(tile + 3 < NMAIN)(lambda: in_copy(tile + 3, 1 - slot).start())
        pl.when(tile > 0)(lambda: out_copy(tile - 1, 1 - slot, None).wait())
        pl.when(tile + 2 < NMAIN)(lambda: in_copy(tile + 2, slot).wait())
        return carry

    prologue()
    in_copy(2, 0).start()
    in_copy(1, 1).wait()
    jax.lax.fori_loop(0, NMAIN, main, 0)
    main(jnp.int32(NMAIN), 0, True)
    xr_out.wait()
    out_copy(NMAIN - 1, (NMAIN - 1) % 2, None).wait()


def build(TM=640, **kw):
    def f(x0, ws, bs):
        B, D = x0.shape
        L = ws.shape[0]
        Mh = TM // 4
        nmain = (B - 1) // TM
        R0 = B - nmain * TM
        assert D == 1024 and L % 2 == 0 and L <= 8 and TM % 128 == 0 and R0 % 16 == 0 and nmain >= 3
        n3 = len(PRODS3)
        odd = lambda n: 16 * (n // 16 | 1)
        V = pltpu.VMEM
        scratch = ([V((1, 2, 2, 2, Mh + 40, 128), f32)] * 4 + [V((1, 2, 4, 2, Mh + 40, 128), f32)] * 7
                   + [V((1, Mh + 32, 128), f32)] * (16 + 56 + 20)
                   + [V((1, 2, 10 if p == 1 else 2, odd(Mh), 128), bf16) for p in range(1, 8)]
                   + [V((1, 2, 10, odd(Mh // 2), 128), bf16)] * (n3 // 2)
                   + [V((L, 2, 2, 7 if p == 1 else 1, 128, 128), bf16) for p in range(1, 8)]
                   + [V((L, n3, 7, 128, 128), bf16)] + [V((1, 4, 16 * n3 + 16, 128), f32)] * 2
                   + [V((L, 64, 8, 128), f32), V((8, 1, D), f32), V((2, TM, D), bf16), V((2, TM, D), bf16),
                      V((L, 8, 8, 16, D), bf16), V((R0, D), bf16), V((2, R0, D), f32), V((L, D), bf16),
                      pltpu.SemaphoreType.DMA((L + 14,))])
        anyspec = pl.BlockSpec(memory_space=pl.ANY)
        return pl.pallas_call(
            functools.partial(_kernel, L=L, TM=TM, R0=R0, NMAIN=nmain, D=D, cfg=dict(CFG, **kw)),
            in_specs=[anyspec, anyspec, anyspec],
            out_specs=anyspec,
            out_shape=jax.ShapeDtypeStruct((B, D), x0.dtype),
            scratch_shapes=scratch,
            compiler_params=pltpu.CompilerParams(
                vmem_limit_bytes=120 * 1024 * 1024,
                internal_scratch_in_bytes=65536,
                disable_bounds_checks=True,
            ),
        )(x0, ws.reshape(L, 8, 8, 16, D), bs)
    return f


@jax.jit
def pallas_standalone__dcn_v2_cross__recsys_kernel(x0, ws, bs):
    return build()(x0, ws, bs)
```

```python
import functools

import jax
import jax.numpy as jnp
import numpy as np
import jax.experimental.pallas as pl
import jax.experimental.pallas.tpu as pltpu

f32 = jnp.float32
bf16 = jnp.bfloat16
u32 = jnp.uint32

B11, B12, B21, B22 = BLOCKS = (0, 0), (0, 1), (1, 0), (1, 1)
LA = {1: [(B11, 1), (B22, 1)], 3: [(B11, 1), (B12, -1)], 5: [(B11, 1), (B12, 1)], 4: [(B12, 1), (B22, 1)],
      7: [(B12, 1), (B22, -1)]}
PC = {1: (1, 0, 0, 1), 2: (0, 0, 1, -1), 3: (1, 1, 1, 1), 4: (1, 0, 1, 0), 5: (-1, 1, 1, -1), 6: (0, 0, 1, 1),
      7: (1, 0, -1, 0)}
KINDS = ('35', '47', '26')
PAIR = {'35': (5, 3), '47': (4, 7), '26': (2, 6)}
ORD = (3, 5, 4, 7, 1, 2, 6)
OUTER = (3, 5, 1, 4, 7, 2, 6)
GUEST = {3: 5, 4: 7, 2: 6}
PRODS3 = [(p, q) for p in OUTER if p != 1 for kind in KINDS for q in PAIR[kind]]
GAMMA = 0.125
OACT = {
    3: ([('M3', '+d')], []),
    5: ([('M5', '+d')], [(B12, '+d +M3')]),
    1: ([('S', '+d +M3 -M5')], []),
    4: ([('M4', '+d')], []),
    7: ([('M7', '+d')], [(B11, '+d +S +M4')]),
    2: ([('M2', '+d')], []),
    6: ([('M6', '+d')], [(B22, '+d +S -M2'), (B21, '+d +M2 +M4 -M7 +M3 +M5')]),
}
OSL = {'M3': 0, 'M5': 1, 'S': 2, 'M4': 3, 'M7': 4, 'M2': 5, 'M6': 6}
ISL = {'m1': 0, 's': 1, 'v': 2, 'u': 3}
DEFER = {5: [('26', '26'), ('47', '26'), ('35', '26')], 7: [('26', '26'), ('47', '26'), ('35', '26')],
         6: [('26', '26'), ('47', '26'), ('35', '26'), ('26', '35'), ('26', '47')]}
DONE = {'35': [B12], '47': [B11], '26': [B22, B21]}
SAVE = {5: B12, 1: B11, 7: B22, 2: B21}
STAGES = {1: [(None, 1.0)], 2: [((B11, B12), .4), ((B21, B22), .6)], 'O': [((B11, B12), .5), ((B21, B22), .5)],
          3: [((B11, B12), .35), ((B22,), .37), ((B21,), .28)],
          4: [((B11,), .16), ((B12,), .26), ((B22,), .31), ((B21,), .27)]}
LAG = 8
CFG = dict(FR=(24, 16, 16, 8), CAP=0.95, PORT=0.9, CS=0.5, CL=0.3, VK=0.7, TAIL=3, EW7=12, EW6=40, MOFF=15, GE=12, NSLAB=6, JM=3)


def _dot(a, b):
    return jnp.dot(a, b, preferred_element_type=f32)


def scale(R, C, h, k):
    return 2.0 ** (R // 2 + R % 2 + h - C // 2 - C % 2 - k)


def phys(C, k):
    return 4 * (C // 2) + 2 * k + C % 2


def b_ops(b11, b12, b21, b22):
    r1 = b11 + b22
    g = b12 + b21
    return {1: r1, 2: b11 - b12, 3: b12 - b22, 4: g - r1, 5: b12 + b22, 6: b11 + b12, 7: g + r1}


def lincomb(terms):
    assert terms[0][0] == 1
    acc = terms[0][1]
    for s, v in terms[1:]:
        acc = acc + v if s == 1 else acc - v
    return acc


def rounds_of(p):
    if p == 1:
        return [('1', None)] + [(kind, n) for kind in KINDS for n in range(2)]
    minis = lambda kind: [(kind, r) for r in KINDS]
    return [('1', None), ('x', '1')] + minis('35') + minis('47') + [('y', '1')] * (p in GUEST) + minis('26')


def round_usage(p, rd, first, last, defer):
    stores, finals = OACT[p]
    kind, n = rd
    alu = sum(len(t.split()) - 1 for _, t in stores) + sum(len(t.split()) + (not first) + 2 * last for _, t in finals)
    nst = len(stores) + len(finals)
    if last and kind == '26':
        alu, nst = alu - 0.7 * len(finals), nst - 0.5 * len(finals)
    if defer:
        alu, nst = 0, 1
    elif p == 6 and kind != '35' and n != '35':
        nst -= 1
    if n == '1':
        a, st, m = 0, 4, 0
    elif isinstance(n, str):
        a, st, m = {'35': ((9, 3, 1), (16, 2, 2)), '47': ((10, 3, 1), (18, 2, 2)), '26': ((10, 2, 2), (18, 0, 4))}[kind][n == '26']
    else:
        a, st, m = {'1': (2, 2, 0), '35': (5, 2, 1), '47': (6, 1, 1), '26': (6, 0, 2)}[kind]
    return a + m * alu, st + m * nst


def bias_sites():
    cand = []
    for p in OUTER:
        for rd in rounds_of(p):
            kind, n = rd
            if n == '1':
                pq = [(p, q) for q in (3, 5, 4, 7)] if kind == 'x' else [(x, q) for x in (p, GUEST[p]) for q in (2, 6)]
                cand += [(p, rd, x + ('1',), (1, 0, 0, 1)) for x in pq]
            elif n in ('35', '47'):
                where = [('v', (0, 1, 1, 0))] if n == '35' else [('k', (0, 0, 1, 0)), ('m', (1, 0, 0, 0))]
                cand += [(p, rd, (p, int(q), w), pat) for q in kind for w, pat in where]
            elif n != '26':
                cand += [(p, rd, (p, int(q), (h, nn)), tuple(int(e == 2 * h + nn) for e in range(4)))
                         for q in kind for nn in ((0, 1) if kind == '1' else (n,)) for h in range(2)]
    unit = lambda b: tuple(int(x == b) for x in BLOCKS)
    sites = [(b, leaf, sub) for p in DEFER for rd in DEFER[p] for b, _ in OACT[p][1]
             for leaf in DONE[rd[0]] for sub in DONE[rd[1]]]
    rows = [np.kron(np.kron(unit(b), unit(leaf)), unit(sub)) for b, leaf, sub in sites]
    extra = {}
    def busy(c):
        a, st = round_usage(c[0], c[1], False, False, c[1] in DEFER.get(c[0], ()))
        return 2 * (a + extra.get(c[:2], 0)) + st + (5 if isinstance(c[1][1], str) else 3)
    while len(sites) < 64:
        c = min(cand, key=busy)
        cand.remove(c)
        row = np.kron(np.kron(PC[c[2][0]], PC[c[2][1]]), c[3])
        if np.linalg.matrix_rank(np.array(rows + [row])) > len(rows):
            rows.append(row)
            sites.append(c[2])
            extra[c[:2]] = extra.get(c[:2], 0) + (1 if isinstance(c[1][1], str) else 0.5)
    want = np.zeros((64, 8))
    for e, (I, J, i, j, h, n) in enumerate(np.ndindex(*(2,) * 6)):
        want[e, phys(2 * J + j, n)] = scale(2 * I + i, 2 * J + j, h, n) / GAMMA
    coef = np.round(np.linalg.solve(np.array(rows, float).T, want) * 4096) / 4096
    assert (np.array(rows).T @ coef == want).all()
    return {x: e for e, x in enumerate(sites) if coef[e].any() or isinstance(x[1], tuple)}, coef, extra


def yds(groups, cap):
    n = len(cap)
    speed, cls, gcls = [0.0] * n, [-1] * n, {}
    todo = list(groups)
    while todo:
        pre = [0.0]
        for t in range(n):
            pre.append(pre[-1] + (cap[t] if cls[t] < 0 else 0.0))
        best = None
        for a in sorted({g[0] for g in todo}):
            w = 0.0
            for g in sorted((g for g in todo if g[0] >= a), key=lambda g: g[1]):
                w += g[2]
                d = w / max(pre[g[1] + 1] - pre[a], 1e-9)
                if best is None or d > best[0]:
                    best = (d, a, g[1])
        d, a, b = best
        for t in range(a, b + 1):
            if cls[t] < 0:
                speed[t], cls[t] = d, len(gcls)
        gcls.update({g[:2]: len(gcls) for g in todo if g[0] >= a and g[1] <= b})
        todo = [g for g in todo if not (g[0] >= a and g[1] <= b)]
    return speed, cls, gcls


def spread_jobs(jobs, cap, vcap, tail):
    T = len(cap)
    cap3 = cap * 3
    all3 = [(j[0] + k * T, j[1] + k * T, ji, k) for k in range(3) for ji, j in enumerate(jobs) if j[0] + k * T >= 0]
    pend = {}
    for j in sorted(all3, key=lambda j: (j[1], j[3], j[2])):
        pend.setdefault(j[:2], []).append(j)
    left = {w: sum(sum(jobs[j[2]][2]) for j in q) for w, q in pend.items()}
    speed, cls, gcls = yds([w + (left[w],) for w in pend], cap3)
    cum = [0.0]
    for t in range(3 * T):
        cum.append(cum[-1] + speed[t] * cap3[t])
    when = [[] for _ in jobs]
    debt, vdebt, cur, done = 0.0, 0.0, None, 0

    def fits(j, t):
        need = max(debt, 0.0) + sum(jobs[j[2]][2]) + 1.0
        for w in pend:
            if w[1] >= j[1]:
                break
            if left[w] > 1e-9:
                need += left[w]
                if need > cum[w[1] + 1] - cum[t]:
                    return False
        return True

    for t in range(3 * T):
        if t % T == 0:
            debt, vdebt = min(debt, 0.0), -0.5
        while True:
            rdy = [q[0] for w, q in pend.items() if q and w[0] <= t and (gcls[w] == cls[t] or w[1] <= t)]
            j = cur
            if j is None:
                if not rdy:
                    debt = max(debt, 0.0)
                    break
                j = rdy[0]
                if j[1] > t:
                    j = (min if vdebt > 0 else max)([x for x in rdy if x is j or fits(x, t)], key=lambda x: jobs[x[2]][3])
                nst = len(jobs[j[2]][2])
                if nst > 1 and j[1] > t and (t + tail + 2 * nst) // T != t // T:
                    break
            must = j[1] <= t or (cur is not None and ((t + tail + 1) // T != t // T or (rdy and rdy[0][1] <= t)))
            if not must and (cap3[t] == 0.0 or debt > 0.5 * speed[t] * cap3[t]):
                break
            if cur is None:
                pend[j[:2]].pop(0)
                left[j[:2]] -= sum(jobs[j[2]][2])
                cur, done = j, 0
            debt += jobs[j[2]][2][done]
            vdebt += jobs[j[2]][2][done] * jobs[j[2]][3]
            if j[3] == 1:
                when[j[2]].append(t - T)
            done += 1
            if done == len(jobs[j[2]][2]):
                cur = None
        debt -= speed[t] * cap3[t]
        vdebt = min(max(vdebt - vcap[t % T], -0.5), 1.0)
    assert all(j[0] <= ts[0] and ts[-1] <= j[1] and (ts[0] < 0) == (ts[-1] < 0) for j, ts in zip(jobs, when))
    return when


def _kernel(x_hbm, w_hbm, b_hbm, o_hbm, *scratch, L, TM, R0, NMAIN, D, cfg):
    H, Mh, Mq = D // 4, TM // 4, TM // 8
    NC, NQ = Mh // 16, Mq // 16
    it = iter(scratch)
    take = lambda n: [next(it) for _ in range(n)]
    x0b, xb, ib, ob, jb = take(4), take(7), take(16), take(56), take(20)
    s2 = dict(zip(range(1, 8), take(7)))
    s3 = {(p, kind): next(it) for p in OUTER if p != 1 for kind in KINDS}
    t2 = dict(zip(range(1, 8), take(7)))
    t3_ref, kb0, kb1, bt_ref, bf_ref, xn2_ref, o2_ref, w0_ref, w_ref, xr_ref, xp_ref, b_ref, sem = it
    sites, bcoef, extra = bias_sites()
    pos2 = lambda p, q: ORD.index(q) if p == 1 else 0

    xset = lambda l: 6 if l == 'O' else 4 if l == 0 else (l % 2) * 2
    xoff = lambda I, J: 16 * ((I + J) % 2)
    xloc = lambda l, R, C, k: (xb[xset(l) + R // 2], (R % 2, C, k), xoff(R // 2, C // 2))
    x0loc = lambda R, C, k: (x0b[(R // 2) * 2 + C // 2], (R % 2, C % 2, k), 8 + xoff(R // 2, C // 2))
    iloc = lambda g, name, n: (ib[((g % 2) * 4 + ISL[name]) * 2 + n], (), 8 * ISL[name])
    oloc = lambda name, i, j, n: (ob[(OSL[name] * 4 + i * 2 + j) * 2 + n], (), 8 * ((OSL[name] + 2 * j) % 4))

    def jloc(kind, name, al, guest=False):
        u = ('1', 's', 'k').index(name)
        return jb[18 + al if guest else (KINDS.index(kind) * 3 + u) * 2 + al], (), 8 * ((3 * u + al) % 4)

    def tie(v, anchor, r=None, lo=0):
        if anchor is None:
            return v
        never, gate = anchor
        if r is None:
            n = v.shape[0]
            return jax.lax.select(never[n], gate if n == 8 else jnp.tile(gate, (n // 8, 1)), v)
        top = jax.lax.select(never[8], gate, v[r:r + 8])
        return jnp.concatenate(([v[lo:r]] if r > lo else []) + [top, v[r + 8:r + 16]], axis=0)

    def consts(anchor, ss):
        one = {s: tie(jnp.full((8, 128), s, f32), anchor) for s in set(ss)}
        return jnp.concatenate([one[s] for s in ss for _ in range(2)], axis=0)

    def conv(src, R, Q, r, zs, anchor):
        v = src[R * Mh + r:R * Mh + r + 32, Q * H:(Q + 1) * H].astype(f32)
        for j in range(2):
            C, k = 2 * (Q // 2) + j, Q % 2
            buf, idx, off = xloc(0, R, C, k)
            sv = consts(anchor, [scale(R, C, (r + u) // Mq, k) for u in (0, 16)])
            buf[(zs,) + idx + (slice(off + r, off + r + 32),)] = v[:, j * 128:(j + 1) * 128] * sv

    count = {}
    def block_sum(l, terms, ii, jj, kk, r, save, zs, za, anchor, gate=True):
        rng = lambda t: slice(t[0], t[-1] + 1)
        vals = []
        for u, ((I, J), s) in enumerate(terms):
            ref, r0 = xb[xset(l) + I], xoff(I, J) + r
            v = ref[za if u == 0 else 0, rng(ii), 2 * J + jj[0]:2 * J + jj[-1] + 1, rng(kk), r0:r0 + 16, :]
            if (I, J) == save:
                sv = consts(anchor, [GAMMA / scale(2 * I + i, 2 * J + j, r // Mq, k) for i in ii for j in jj for k in kk])
                x0b[I * 2 + J][zs, rng(ii), rng(jj), rng(kk), r0 + 8:r0 + 24, :] = v * sv.reshape(v.shape)
            if u == 0 and gate:
                count[xset(l)] = count.get(xset(l), -1) + 1
                if count[xset(l)] % cfg['GE'] == 0:
                    ref[0, 0, 0, 0, Mh + 24:Mh + 32, :] = count.get('prev', anchor)[1]
                count['prev'] = anchor
            vals.append((s, v))
        v = lincomb(vals)
        return v.reshape(v.size // 128, 128)

    def operands(a, group, st8, store):
        for u, b in enumerate(group):
            st8[b] = a if len(group) == 1 else a[:, u:u + 1]
        ops = {}
        if B12 in group:
            ops[3], ops[5] = st8[B11] - st8[B12], st8[B11] + st8[B12]
        if B22 in group:
            ops[4], ops[7] = st8[B12] + st8[B22], st8[B12] - st8[B22]
            ops[1] = st8['l1'] = st8[B11] + st8[B22]
        if B21 in group:
            g = st8[B12] + st8[B21]
            ops[2], ops[6] = g + st8['l1'], g - st8['l1']
        now = [q for q in ORD if q in ops]
        if now:
            u = ORD.index(now[0])
            store(slice(u, u + len(now)), jnp.concatenate([ops[q] for q in now], axis=1).astype(bf16))

    def unit1(l, c, k, save, st8, group, zs, za, anchor):
        def store(pos, v):
            s2[1][zs, k:k + 1, pos, 16 * c:16 * c + 16, :] = v
        e = block_sum(l, LA[1], [group[0][0]], [0, 1], [k], 16 * c, save, zs, za, anchor)
        operands(tie(e, anchor, 16).reshape(1, 2, 16, 128), group, st8, store)

    def unit26(l, c, k, save, st8, group, zs, za, anchor):
        i = group[0][0]
        f = block_sum(l, [(B11, 1), (B22, 1)], [i], [0, 1], [k], 16 * c, save, zs, za, anchor, False)
        e = tie(block_sum(l, [(B12, 1), (B21, 1)], [i], [0, 1], [k], 16 * c, save, zs, za, anchor), anchor)
        for J, v in enumerate((e + f, e - f)):
            r0 = xoff(0, J) + 16 * c
            xb[6][zs, i, 2 * J:2 * J + 2, k, r0:r0 + 16, :] = v.reshape(2, 16, 128)

    def unit3(l, p, kind, c, save, st8, group, zs, za, anchor):
        def store(pos, v):
            s3[(p, kind)][zs, :, pos, 16 * c:16 * c + 16, :] = v
        h, kk = group[0][0], [b[1] for b in group]
        ii, jj = {'35': ([0], [0, 1]), '47': ([0, 1], [1]), '26': ([0, 1], [0, 1])}[kind]
        src = (l, LA[p]) if p in LA else ('O', [((0, (2, 6).index(p)), 1)])
        n = 16 * len(kk)
        v = block_sum(*src, ii, jj, kk, h * Mq + 16 * c, save, zs, za, anchor)
        if kind == '26':
            e, f = tie(v, anchor, 16, 16) + v[32:48], v[0:16] + v[48:64]
            r0 = h * Mq + 16 * c
            s2[p][zs, kk[0], 0, r0:r0 + 16, :] = f.astype(bf16)
        else:
            e, f = tie(v, anchor, n - 16), v[n:]
        operands(jnp.concatenate([e + f, e - f], axis=0).reshape(2, len(kk), 16, 128), group, st8, store)

    GAPS = [w for pos in range(4) for w in [1] + [x for p in (2, 6, 3, 5, 1, 4, 7) for x in (
        [15] if p == 1 else [21] if pos < 3 else [9] + [15] * 6)]]

    def wtile(idx, n):
        if cfg.get('NOBC'):
            return w_ref[idx].reshape(16 * n, 128)
        return pltpu.bitcast(w_ref.bitcast(u32)[idx].reshape(8 * n, 128), bf16)

    def prep(l, u, anchors, zero, kb):
        mul = lambda v, s: v if s == 1.0 else v * s
        stack = lambda T: jnp.concatenate([T[q] for q in ORD], axis=0).reshape(7, 16, 128).astype(bf16)
        rows = pl.ds(16 * u, 16) if isinstance(u, int) else pl.ds(pl.multiple_of(16 * u, 16), 16)
        for k in range(2):
            if isinstance(l, int):
                wide = [w0_ref[phys(R, k), u].astype(f32) for R in range(4)]
                tile = lambda R, c: wide[R][:, c * 128:(c + 1) * 128]
            else:
                wide = [wtile((l - 1, slice(None), phys(R, k), u), 8).astype(f32) for R in range(4)]
                tile = lambda R, c: wide[R][c * 16:(c + 1) * 16]
            for n in range(2):
                anchor = next(anchors)
                blk = lambda R, C: mul(tile(R, phys(C, n)), scale(R, C, k, n))
                O = {(i, j): b_ops(blk(i, j), tie(blk(i, 2 + j), anchor, 0), blk(2 + i, j), blk(2 + i, 2 + j))
                     for i, j in BLOCKS}
                for p in (2, 6, 3, 5, 1, 4, 7):
                    o = [mul(O[b][p], 4.0 if p == 1 else 1.0) for b in BLOCKS]
                    T = b_ops(o[0], tie(o[1], next(anchors), 0), o[2], o[3])
                    if p == 1:
                        T[1] = T[1] * 2.0
                        t2[p][l, n, k, :, rows, :] = stack(T)
                        continue
                    t2[p][l, n, k, 0, rows, :] = (T[1] * 4.0).astype(bf16)
                    e0 = PRODS3.index((p, 5))
                    if (k, n) != (1, 1):
                        kb[zero, k * 2 + n, 16 * e0:16 * e0 + 96, :] = jnp.concatenate(
                            [T[q] for _, q in PRODS3[e0:e0 + 6]], axis=0)
                        continue
                    for e in range(e0, e0 + 6):
                        v = kb[0, 0:3, 16 * e:16 * e + 16, :]
                        T3 = b_ops(v[0], tie(v[1], next(anchors), 0), v[2], T[PRODS3[e][1]])
                        T3[1] = T3[1] * 2.0
                        t3_ref[l, e, :, rows, :] = stack(T3)

    outs = [(l, p) for l in range(L) for p in OUTER]
    G = len(outs)
    sched, start, use, vuse = [], [], [], []
    for g, (l, p) in enumerate(outs):
        start.append(len(use))
        for rd in rounds_of(p):
            n = NQ if isinstance(rd[1], str) else NC
            sched.append((g, rd, len(use), n))
            a, st_ = round_usage(p, rd, l == 0, l == L - 1, rd in DEFER.get(p, ()))
            a += extra.get((p, rd), 0)
            use += [max((2 * a + st_ + 2 + 16 / n) / 72, cfg['PORT'] * st_ / 8)] * n
            vuse += [st_ / 8] * n
    T = len(use)
    first = lambda g, kind: next(t0 for gg, rd, t0, _ in sched if gg == g and rd[0] == kind)
    jobs, late = [], []
    def add(lo, hi, alu, st_, ld_, scheme, kind, fn):
        w = alu / 64 + cfg['CS'] * (st_ + len(STAGES[scheme])) / 16 + cfg['CL'] * ld_ / 48
        jobs.append((lo, max(hi, lo), [w * f for _, f in STAGES[scheme]], st_ / 16 / w, scheme, kind, fn))
    for g, (l, p) in enumerate(outs):
        for gg, rd, t0, n_ in sched:
            if gg == g and rd in DEFER.get(p, ()):
                last = l == L - 1
                nops = sum(len(t.split()) + 1 + (l > 0) + 1.5 * last for _, t in OACT[p][1])
                islate = last and p == 6 and rd[0] == '26'
                due = {5: lambda: start[7 * l + 5] - 1, 7: lambda: start[g + 1] + cfg['EW7'],
                       6: lambda: T - cfg['TAIL'] - 1 if last else min(start[g + 1] + cfg['EW6'], first(g + 1, rd[0])) - 1}[p]()
                both = last and rd[0] == '26'
                step = cfg['FR'][(p == 6) + 2 * both]
                for r0 in range(0, Mq, step):
                    nr = min(step, Mq - r0)
                    for h, n in DONE[rd[1]]:
                        for leaves in [DONE[rd[0]]] if both else [[b] for b in DONE[rd[0]]]:
                            fn = (l, p, leaves, h, n, r0, nr)
                            nv = len(leaves) * nr // 8
                            add(0 if islate else t0 + n_, cfg['EW6'] - 1 if islate else due, nops * nv,
                                nv * len(OACT[p][1]) / (1 + both) - 1, 0.9 * nops * nv, 1, 'fin', fn)
                            if islate:
                                late.append(fn)
        if p in (3, 5):
            lo = start[7 * l - 2] + (cfg['EW7'] + 1 if l else -T)
        else:
            lo = start[7 * l] + cfg['EW6']
        hi = start[g] - LAG - 3
        save = SAVE.get(p) if l == 0 else None
        sv = save is not None
        if p == 1:
            for c, k in np.ndindex(NC, 2):
                add(lo, hi, 31 + 8 * sv, 7 + 8 * sv, 16, 2, l, functools.partial(unit1, l, c, k, save))
            continue
        nt = 2
        if p in (2, 6):
            mid = start[7 * l + 3] + cfg['MOFF']
            if p == 2:
                for c, k in np.ndindex(NC, 2):
                    add(lo, mid - 3, 40 + 8 * sv, 16 + 8 * sv, 32, 'O', l, functools.partial(unit26, l, c, k, save))
            lo, nt, save, sv = mid, 1, None, False
        for c in range(NQ):
            add(lo, hi if p in GUEST else first(g - 1, 'y') - LAG - 3, 32 * nt + 50 + 32 * sv, 18 + 32 * sv, 32 * nt,
                4, l, functools.partial(unit3, l, p, '26', c, save))
        for c in range(NQ):
            for kind in KINDS[:2]:
                add(lo, hi + (NC if g else 0), 16 * nt + 46, 14, 16 * nt, 3, l, functools.partial(unit3, l, p, kind, c, None))
    convs = [(R, Q, r) for R in range(4) for Q in range(4) for r in range(0, Mh, 32)]
    for x in convs:
        add(start[6], start[G - 2] - 2, 18, 7, 4, 1, 'conv', x)
    cap = [max(cfg['CAP'] - max(use[t], use[(t + 1) % T]), 0.0) * (t < T - cfg['TAIL']) for t in range(T)]
    when = spread_jobs(jobs, cap, [cfg['VK'] * (1 - vuse[(t + 1) % T]) for t in range(T)], cfg['TAIL'])
    plan = {}
    for t, _, ji, u in sorted((t % T, ts[0] % T, ji, u) for ji, ts in enumerate(when) for u, t in enumerate(ts)):
        plan.setdefault(t, []).append((jobs[ji][5], jobs[ji][6], STAGES[jobs[ji][4]][u][0]))
    assert cfg['EW6'] <= first(0, '26')
    carried = [job for ts, job in zip(when, jobs) if ts[0] < 0]

    def w_copy(l, c=None):
        if c is None:
            return pltpu.make_async_copy(w_ref.at[l - 1], w_ref.at[l - 1], sem.at[l])
        return pltpu.make_async_copy(w_hbm.at[l, :, :, :, pl.ds(c * 128, 128)], w_ref.at[l - 1, c], sem.at[l])

    def w0_copy(u):
        return pltpu.make_async_copy(w_hbm.at[0, :, u], w0_ref.at[:, u], sem.at[L + 6 + u])

    def in_copy(t, slot):
        return pltpu.make_async_copy(x_hbm.at[pl.ds(pl.multiple_of(t * TM, 32), TM)], xn2_ref.at[slot], sem.at[L + slot])

    def out_copy(t, slot, part):
        r0, nr = (0, TM) if part is None else ((0, 4 * Mq), (4 * Mq, Mq), (5 * Mq, Mq), (6 * Mq, 2 * Mq))[part]
        return pltpu.make_async_copy(o2_ref.at[slot, pl.ds(r0, nr)],
                                     o_hbm.at[pl.ds(pl.multiple_of(t * TM + r0, 16), nr)], sem.at[L + 4 + slot])

    xr_in = pltpu.make_async_copy(x_hbm.at[pl.ds(NMAIN * TM, R0)], xr_ref, sem.at[L + 2])
    xr_out = pltpu.make_async_copy(xr_ref, o_hbm.at[pl.ds(NMAIN * TM, R0)], sem.at[L + 2])
    b_in = pltpu.make_async_copy(b_hbm, b_ref, sem.at[L + 3])
    opaque = lambda i, s: jax.lax.shift_right_logical(i, s)
    mask = lambda zero: {n: jnp.broadcast_to(zero, (n, 128)) != 0 for n in (8, 16, 32)}

    def prologue():
        b_in.start()
        for u in range(8):
            w0_copy(u).start()
        xr_in.start()
        in_copy(0, 0).start()
        b_in.wait()
        for l in range(L):
            bf_ref[l] = b_ref[l:l + 1, :].astype(f32)

        def bias_tiles(l, carry):
            b = jnp.broadcast_to(bf_ref[l] + (l == 0).astype(f32), (8, D))
            for u in sites.values():
                terms = [b[:, e * 128:(e + 1) * 128] * float(cf) for e, cf in enumerate(bcoef[u]) if cf != 0.0]
                bt_ref[l, u] = functools.reduce(lambda x, y: x + y, terms or [jnp.zeros((8, 128), f32)])
            return carry
        jax.lax.fori_loop(0, L, bias_tiles, 0)
        if cfg.get('FAST'):
            return

        def slab(u, carry):
            w0_copy(u).wait()
            prep(0, u, iter(lambda: None, 0), opaque(u, 12), kb0)
            return opaque(u, 12)
        zero = jax.lax.fori_loop(0, cfg['NSLAB'], slab, 0)

        halves = lambda x: (x[:, :D // 2].astype(bf16), x[:, D // 2:].astype(bf16))

        def plain(l, xbf, x0f, x, j0, j1, gaps, free, never):
            passes = []
            for jt in range(j0, j1):
                cols = slice(jt * 128, (jt + 1) * 128)
                w = [w0_ref[b:b + 4, :, :, cols].reshape(D // 2, 128) if isinstance(l, int)
                     else wtile((l - 1, jt, slice(b, b + 4)), 32) for b in (0, 4)]
                ya = _dot(xbf[0], w[0]) + bf_ref[l, :, cols]
                passes += [ya, _dot(xbf[1], w[1]) + ya]
            xp_ref[0, :, j0 * 128:j1 * 128] = x0f * jnp.concatenate(passes[1::2], axis=1) + x
            for u in range(len(gaps)):
                ps, rr = divmod(sum(gaps[free:u]) * len(passes) * (R0 // 8) // sum(gaps[free:]), R0 // 8)
                yield None if u < free else (never, passes[ps][rr * 8:rr * 8 + 8, :])

        for l in range(1, L):
            for c in range(8):
                w_copy(l, c).start()
        in_copy(1, 1).start()
        for u in range(cfg['NSLAB'], 8):
            w0_copy(u).wait()
        xr_in.wait()
        jm = cfg['JM']
        x0f = xr_ref[:, :jm * 128].astype(f32)
        xp_ref[1, :, :jm * 128] = x0f
        anchors = plain(0, halves(xr_ref), x0f, x0f, 0, jm, (8 - cfg['NSLAB']) * GAPS, 2, mask(zero))
        for u in range(cfg['NSLAB'], 8):
            prep(0, u, anchors, zero, (kb0, kb1)[u % 2])
        in_copy(0, 0).wait()
        x0f = xr_ref[:, jm * 128:].astype(f32)
        xp_ref[1, :, jm * 128:] = x0f
        blank = [loc for j, n in BLOCKS for loc in [oloc(x, 1, j, n) for x in OSL]
                 + [f(3, 2 * J + j, n) for J in range(2) for f in (x0loc, functools.partial(xloc, L - 1))]]
        na = len(convs) + sum(len(j[2]) for j in carried) + 2 * len(blank) + 2
        anchors = plain(0, halves(xr_ref), x0f, x0f, jm, 8, [1] * na, 4, mask(zero))
        for x in convs[:len(convs) // 2]:
            conv(xn2_ref.at[0], *x, zero, next(anchors))
        for job in carried:
            st8 = {}
            for group, _ in STAGES[job[4]]:
                job[6](st8, group, zero, opaque(zero, 1), next(anchors))
        for x in convs[len(convs) // 2:]:
            conv(xn2_ref.at[0], *x, zero, next(anchors))
        for ref, idx, off in blank:
            for r0 in (off, off + Mq):
                ref[(0,) + idx + (slice(r0, r0 + Mq),)] = consts(next(anchors), [0.0] * NQ)

        def layer(l, carry):
            w_copy(l).wait()
            x, zero = xp_ref[0], opaque(l, 12)
            anchors = plain(l, halves(x), xp_ref[1], x, 0, 8, 8 * GAPS, 2, mask(zero))
            for u in range(8):
                prep(l, u, anchors, zero, (kb0, kb1)[u % 2])
            return carry

        jax.lax.fori_loop(1, L, layer, 0)
        xr_ref[...] = xp_ref[0].astype(bf16)
        xr_out.start()

    def main(tile, carry, only_late=False):
        zs, za = opaque(tile, 12), opaque(tile, 13)
        never = mask(zs)
        slot = tile % 2
        out = [o2_ref.at[1 - slot]]

        def rows(h, r0):
            lo, n = (0, Mh) if h is None else h if isinstance(h, tuple) else (h * Mq, Mq)
            return slice(r0 + lo, r0 + lo + n)

        def ld(loc, h):
            return loc[0][(0,) + loc[1] + (rows(h, loc[2]),)]

        def st(loc, v, h):
            loc[0][(zs,) + loc[1] + (rows(h, loc[2]),)] = v

        def operand(ref, idx, n):
            if cfg.get('NOBC'):
                return ref[idx + (slice(0, n),)]
            return pltpu.bitcast(ref.bitcast(u32)[idx + (slice(0, n // 2),)], bf16)

        def dot3(l, p, q, r):
            kind = next(x for x in KINDS if q in PAIR[x])
            return _dot(operand(s3[(p, kind)], (0, PAIR[kind].index(q), ORD.index(r)), Mq),
                        operand(t3_ref, (l, PRODS3.index((p, q)), ORD.index(r)), 128))

        def issue(l, p, rd):
            kind, n = rd
            if kind == 'x':
                return [dot3(l, p, q, 1) for q in (3, 5, 4, 7)]
            if kind == 'y':
                return [dot3(l, x, q, 1) for x in (p, GUEST[p]) for q in (2, 6)]
            if isinstance(n, str):
                return [dot3(l, p, int(q), int(r)) for q in kind for r in n]
            lhs = {q: [operand(s2[p], (0, k, pos2(p, q)), Mh) for k in range(2)] for q in map(int, kind)}
            return [_dot(lhs[q][k], operand(t2[p], (l, nn, k, pos2(p, q)), 128))
                    for q, nn in ([(1, 0), (1, 1)] if kind == '1' else [(int(q), n) for q in kind]) for k in range(2)]

        def biased(v, l, *site):
            if site not in sites:
                return v
            return (v.reshape(Mq // 8, 8, 128) + bt_ref[l, sites[site]]).reshape(Mq, 128)

        wait = {}
        def outer_act(l, p, i, j, n, d, h, part=None, last=lambda b, y: y):
            stores, finals = OACT[p]
            if part == 'park':
                stores, finals = stores[:1], []
            elif part == 'rest' or (p == 6 and (i, j) != B12 and (h, n) != B12):
                stores = stores[1:]
            cache = {'d': d}
            def comb(terms):
                for t in terms.split():
                    if t[1:] not in cache:
                        cache[t[1:]] = ld(oloc(t[1:], i, j, n), h)
                return lincomb([(int(t[0] + '1'), cache[t[1:]]) for t in terms.split()])
            fin = [(IJ, last(IJ, comb(terms))) for IJ, terms in finals]
            for name, v in [(name, comb(terms)) for name, terms in stores]:
                st(oloc(name, i, j, n), v, h)
            for (I, J), y in fin:
                R, C = 2 * I + i, 2 * J + j
                xn = ld(x0loc(R, C, n), h) * y
                if l > 0:
                    xn = xn + ld(xloc(l, R, C, n), h)
                if l < L - 1:
                    st(xloc(l + 1, R, C, n), xn, h)
                    continue
                s = scale(R, C, rows(h, 0).start // Mq, n)
                xn = xn if s == 1.0 else xn * (1.0 / s)
                c0 = phys(C, n) * 128
                if i == 0:
                    out[0][rows(h, R * Mh), c0:c0 + 128] = xn.astype(bf16)
                elif j == 1:
                    wait[J] = xn
                else:
                    out[0][rows(h, R * Mh), c0:c0 + 256] = jnp.concatenate([xn, wait.pop(J)], axis=1).astype(bf16)

        def inner_act(g, l, p, kind, n, h, P, Q, part=None):
            vloc = iloc(g, 'v', n) if p == 1 else oloc(OACT[p][0][0][0], 0, 1, n)
            if kind == '35':
                st(iloc(g, 's', n), Q + ld(iloc(g, 'm1', n), h), h)
                if p == 1:
                    st(vloc, P, h)
                outer_act(l, p, 0, 1, n, P, h, part)
            elif kind == '47':
                st(iloc(g, 'u', n), Q + ld(vloc, h), h)
                outer_act(l, p, 0, 0, n, P + ld(iloc(g, 's', n), h), h, part)
            else:
                outer_act(l, p, 1, 1, n, ld(iloc(g, 's', n), h) - Q, h, part)
                outer_act(l, p, 1, 0, n, P + ld(iloc(g, 'u', n), h), h, part)

        def consume(g, l, p, rd, res):
            kind, n = rd
            if n == '1':
                for u, (kd, x) in enumerate([('35', p), ('47', p)] if kind == 'x' else [('26', p), ('26', GUEST[p])]):
                    for al in range(2):
                        st(jloc(kd, '1', al, x != p), biased(res[2 * u + al], l, x, int(kd[al]), '1'), 0)
            elif isinstance(n, str):
                sm = [res[2 * al] + res[2 * al + 1] for al in range(2)]
                df = [res[2 * al] - res[2 * al + 1] for al in range(2)]
                J = lambda name, al: ld(jloc(kind, name, al, name == '1' and kind == '26' and p not in GUEST), 0)
                part = 'park' if rd in DEFER.get(p, ()) else None
                done = lambda h, nn, m: inner_act(g, l, p, kind, nn, h, m[0] + m[1], m[0] - m[1], part)
                if n == '35':
                    for al in range(2):
                        st(jloc(kind, 's', al), df[al] + J('1', al), 0)
                    done(0, 1, [biased(sm[al], l, p, int(kind[al]), 'v') for al in range(2)])
                elif n == '47':
                    for al in range(2):
                        st(jloc(kind, 'k', al), biased(df[al], l, p, int(kind[al]), 'k'), 0)
                    done(0, 0, [biased(sm[al] + J('s', al), l, p, int(kind[al]), 'm') for al in range(2)])
                else:
                    O = lambda i, j: ld(oloc(OACT[p][0][0][0], i, j, 1), 0)
                    m = [sm[al] + J('k', al) for al in range(2)]
                    P = m[0] + m[1] + O(*{'35': B12, '47': B11, '26': B21}[kind])
                    Q = m[0] - m[1] - (ld(iloc(g, 'm1', 1), 0) if kind == '35' else O(*{'47': B12, '26': B22}[kind]))
                    done(1, 1, [J('s', al) - df[al] for al in range(2)])
                    inner_act(g, l, p, kind, 0, 1, P, Q, part)
            else:
                m = []
                for al, (q, nn) in enumerate([(1, 0), (1, 1)] if kind == '1' else [(int(q), n) for q in kind]):
                    v = res[2 * al] + res[2 * al + 1]
                    if any((p, q, (h, nn)) in sites for h in range(2)):
                        v = jnp.concatenate([biased(v[h * Mq:(h + 1) * Mq], l, p, q, (h, nn)) for h in range(2)], axis=0)
                    m.append(v)
                if kind == '1':
                    for nn in range(2):
                        st(iloc(g, 'm1', nn), m[nn], None)
                else:
                    inner_act(g, l, p, kind, n, None, m[0] + m[1], m[0] - m[1])

        def finish(l, p, leaves, h, n, r0, nr, anchor):
            for i, j in leaves:
                d = ld(oloc(OACT[p][0][0][0], i, j, n), (h * Mq + r0, nr))
                last = lambda b, y: (y.reshape(nr // 8, 8, 128)
                                     + tie(bt_ref[l, sites[(b, (i, j), (h, n))]], anchor)).reshape(nr, 128)
                outer_act(l, p, i, j, n, d, (h * Mq + r0, nr), 'rest', last)

        if only_late:
            for x in late:
                finish(*x, None)
            out_copy(tile - 1, 1 - slot, 3).start()
            return carry
        state = {}
        count.clear()
        for g, rd, t0, n in sched:
            l, p = outs[g]
            if t0 == start[1]:
                pl.when(tile > 0)(lambda: out_copy(tile - 1, 1 - slot, 3).start())
                out[0] = o2_ref.at[slot]
            if t0 == first(G - 2, '35'):
                assert t0 > start[G - 2] + cfg['EW7']
                out_copy(tile, slot, 0).start()
            res = issue(l, p, rd)
            if t0 == first(G - 2, '35'):
                out[0][TM - 8:TM, 0:128] = res[0][0:8, :].astype(bf16)
            for t in range(t0, t0 + n):
                if t in plan:
                    r0 = 16 * (t - t0) + 8
                    anchor = (never, res[0 if isinstance(rd[1], str) else 1][r0:r0 + 8, :])
                for kind, fn, group in plan.get(t, []):
                    if kind == 'fin':
                        finish(*fn, anchor)
                    elif kind == 'conv':
                        conv(xn2_ref.at[1 - slot], *fn, zs, anchor)
                    else:
                        fn(state.setdefault(id(fn), {}), group, zs, za, anchor)
            if t0 == first(G - 1, '26'):
                out_copy(tile, slot, 1).start()
            if t0 + n == T:
                out_copy(tile, slot, 2).start()
            consume(g, l, p, rd, res)
        pl.when(tile + 3 < NMAIN)(lambda: in_copy(tile + 3, 1 - slot).start())
        pl.when(tile > 0)(lambda: out_copy(tile - 1, 1 - slot, None).wait())
        pl.when(tile + 2 < NMAIN)(lambda: in_copy(tile + 2, slot).wait())
        return carry

    prologue()
    in_copy(2, 0).start()
    in_copy(1, 1).wait()
    jax.lax.fori_loop(0, NMAIN, main, 0)
    main(jnp.int32(NMAIN), 0, True)
    xr_out.wait()
    out_copy(NMAIN - 1, (NMAIN - 1) % 2, None).wait()


def build(TM=640, **kw):
    def f(x0, ws, bs):
        B, D = x0.shape
        L = ws.shape[0]
        Mh = TM // 4
        nmain = (B - 1) // TM
        R0 = B - nmain * TM
        assert D == 1024 and L % 2 == 0 and L <= 8 and TM % 128 == 0 and R0 % 16 == 0 and nmain >= 3
        n3 = len(PRODS3)
        odd = lambda n: 16 * (n // 16 | 1)
        V = pltpu.VMEM
        scratch = ([V((1, 2, 2, 2, Mh + 40, 128), f32)] * 4 + [V((1, 2, 4, 2, Mh + 40, 128), f32)] * 7
                   + [V((1, Mh + 32, 128), f32)] * (16 + 56 + 20)
                   + [V((1, 2, 10 if p == 1 else 2, odd(Mh), 128), bf16) for p in range(1, 8)]
                   + [V((1, 2, 10, odd(Mh // 2), 128), bf16)] * (n3 // 2)
                   + [V((L, 2, 2, 7 if p == 1 else 1, 128, 128), bf16) for p in range(1, 8)]
                   + [V((L, n3, 7, 128, 128), bf16)] + [V((1, 4, 16 * n3 + 16, 128), f32)] * 2
                   + [V((L, 64, 8, 128), f32), V((8, 1, D), f32), V((2, TM, D), bf16), V((2, TM, D), bf16),
                      V((8, 8, 16, D), bf16), V((L - 1, 8, 8, 8, 16, 128), bf16), V((R0, D), bf16), V((2, R0, D), f32), V((L, D), bf16),
                      pltpu.SemaphoreType.DMA((L + 14,))])
        anyspec = pl.BlockSpec(memory_space=pl.ANY)
        return pl.pallas_call(
            functools.partial(_kernel, L=L, TM=TM, R0=R0, NMAIN=nmain, D=D, cfg=dict(CFG, **kw)),
            in_specs=[anyspec, anyspec, anyspec],
            out_specs=anyspec,
            out_shape=jax.ShapeDtypeStruct((B, D), x0.dtype),
            scratch_shapes=scratch,
            compiler_params=pltpu.CompilerParams(
                vmem_limit_bytes=120 * 1024 * 1024,
                internal_scratch_in_bytes=65536,
                disable_bounds_checks=True,
                disable_semaphore_checks=True,
            ),
        )(x0, ws.reshape(L, 8, 8, 16, D), bs)
    return f


@jax.jit
def pallas_standalone__dcn_v2_cross__recsys_kernel(x0, ws, bs):
    return build()(x0, ws, bs)
```

```python
import functools

import jax
import jax.numpy as jnp
import numpy as np
import jax.experimental.pallas as pl
import jax.experimental.pallas.tpu as pltpu

f32 = jnp.float32
bf16 = jnp.bfloat16
u32 = jnp.uint32

B11, B12, B21, B22 = BLOCKS = (0, 0), (0, 1), (1, 0), (1, 1)
LA = {1: [(B11, 1), (B22, 1)], 3: [(B11, 1), (B12, -1)], 5: [(B11, 1), (B12, 1)], 4: [(B12, 1), (B22, 1)],
      7: [(B12, 1), (B22, -1)]}
PC = {1: (1, 0, 0, 1), 2: (0, 0, 1, -1), 3: (1, 1, 1, 1), 4: (1, 0, 1, 0), 5: (-1, 1, 1, -1), 6: (0, 0, 1, 1),
      7: (1, 0, -1, 0)}
KINDS = ('35', '47', '26')
PAIR = {'35': (5, 3), '47': (4, 7), '26': (2, 6)}
ORD = (3, 5, 4, 7, 1, 2, 6)
OUTER = (3, 5, 1, 4, 7, 2, 6)
GUEST = {3: 5, 4: 7, 2: 6}
PRODS3 = [(p, q) for p in OUTER if p != 1 for kind in KINDS for q in PAIR[kind]]
GAMMA = 0.125
OACT = {
    3: ([('M3', '+d')], []),
    5: ([('M5', '+d')], [(B12, '+d +M3')]),
    1: ([('S', '+d +M3 -M5')], []),
    4: ([('M4', '+d')], []),
    7: ([('M7', '+d')], [(B11, '+d +S +M4')]),
    2: ([('M2', '+d')], []),
    6: ([('M6', '+d')], [(B22, '+d +S -M2'), (B21, '+d +M2 +M4 -M7 +M3 +M5')]),
}
OSL = {'M3': 0, 'M5': 1, 'S': 2, 'M4': 3, 'M7': 4, 'M2': 5, 'M6': 6}
ISL = {'m1': 0, 's': 1, 'v': 2, 'u': 3}
DEFER = {5: [('26', '26'), ('47', '26'), ('35', '26')], 7: [('26', '26'), ('47', '26'), ('35', '26')],
         6: [('26', '26'), ('47', '26'), ('35', '26'), ('26', '35'), ('26', '47')]}
DONE = {'35': [B12], '47': [B11], '26': [B22, B21]}
SAVE = {5: B12, 1: B11, 7: B22, 2: B21}
STAGES = {1: [(None, 1.0)], 2: [((B11, B12), .4), ((B21, B22), .6)], 'O': [((B11, B12), .5), ((B21, B22), .5)],
          3: [((B11, B12), .35), ((B22,), .37), ((B21,), .28)],
          4: [((B11,), .16), ((B12,), .26), ((B22,), .31), ((B21,), .27)]}
LAG = 8
CFG = dict(FR=(24, 16, 16, 8), CAP=0.95, PORT=0.9, CS=0.5, CL=0.3, VK=0.66, TAIL=3, EW7=12, EW6=40, MOFF=15, GE=12, NSLAB=6, JM=3)


def _dot(a, b):
    return jnp.dot(a, b, preferred_element_type=f32)


def scale(R, C, h, k):
    return 2.0 ** (R // 2 + R % 2 + h - C // 2 - C % 2 - k)


def phys(C, k):
    return 4 * (C // 2) + 2 * k + C % 2


def b_ops(b11, b12, b21, b22, final=False):
    r1 = b11 + b22
    if final:
        r1 = jax.lax.bitcast_convert_type((jax.lax.bitcast_convert_type(r1, jnp.int32) + 0x8000) & -0x10000, f32)
        b22 = r1 - b11
    g = b12 + b21
    return {1: r1, 2: b11 - b12, 3: b12 - b22, 4: g - r1, 5: b12 + b22, 6: b11 + b12, 7: g + r1}


def lincomb(terms):
    assert terms[0][0] == 1
    acc = terms[0][1]
    for s, v in terms[1:]:
        acc = acc + v if s == 1 else acc - v
    return acc


def rounds_of(p):
    if p == 1:
        return [('1', None)] + [(kind, n) for kind in KINDS for n in range(2)]
    minis = lambda kind: [(kind, r) for r in KINDS]
    return [('1', None), ('x', '1')] + minis('35') + minis('47') + [('y', '1')] * (p in GUEST) + minis('26')


def round_usage(p, rd, first, last, defer):
    stores, finals = OACT[p]
    kind, n = rd
    alu = sum(len(t.split()) - 1 for _, t in stores) + sum(len(t.split()) + (not first) + 2 * last for _, t in finals)
    nst = len(stores) + len(finals)
    if last and kind == '26':
        alu, nst = alu - 0.7 * len(finals), nst - 0.5 * len(finals)
    if defer:
        alu, nst = 0, 1
    elif p == 6 and kind != '35' and n != '35':
        nst -= 1
    if n == '1':
        a, st, m = 0, 4, 0
    elif isinstance(n, str):
        a, st, m = {'35': ((9, 3, 1), (16, 2, 2)), '47': ((10, 3, 1), (18, 2, 2)), '26': ((10, 2, 2), (18, 0, 4))}[kind][n == '26']
    else:
        a, st, m = {'1': (2, 2, 0), '35': (5, 2, 1), '47': (6, 1, 1), '26': (6, 0, 2)}[kind]
    return a + m * alu, st + m * nst


def bias_sites():
    cand = []
    for p in OUTER:
        for rd in rounds_of(p):
            kind, n = rd
            if n == '1':
                pq = [(p, q) for q in (3, 5, 4, 7)] if kind == 'x' else [(x, q) for x in (p, GUEST[p]) for q in (2, 6)]
                cand += [(p, rd, x + ('1',), (1, 0, 0, 1)) for x in pq]
            elif n in ('35', '47'):
                where = [('v', (0, 1, 1, 0))] if n == '35' else [('k', (0, 0, 1, 0)), ('m', (1, 0, 0, 0))]
                cand += [(p, rd, (p, int(q), w), pat) for q in kind for w, pat in where]
            elif n != '26':
                cand += [(p, rd, (p, int(q), (h, nn)), tuple(int(e == 2 * h + nn) for e in range(4)))
                         for q in kind for nn in ((0, 1) if kind == '1' else (n,)) for h in range(2)]
    unit = lambda b: tuple(int(x == b) for x in BLOCKS)
    sites = [(b, leaf, sub) for p in DEFER for rd in DEFER[p] for b, _ in OACT[p][1]
             for leaf in DONE[rd[0]] for sub in DONE[rd[1]]]
    rows = [np.kron(np.kron(unit(b), unit(leaf)), unit(sub)) for b, leaf, sub in sites]
    extra = {}
    def busy(c):
        a, st = round_usage(c[0], c[1], False, False, c[1] in DEFER.get(c[0], ()))
        return 2 * (a + extra.get(c[:2], 0)) + st + (5 if isinstance(c[1][1], str) else 3)
    while len(sites) < 64:
        c = min(cand, key=busy)
        cand.remove(c)
        row = np.kron(np.kron(PC[c[2][0]], PC[c[2][1]]), c[3])
        if np.linalg.matrix_rank(np.array(rows + [row])) > len(rows):
            rows.append(row)
            sites.append(c[2])
            extra[c[:2]] = extra.get(c[:2], 0) + (1 if isinstance(c[1][1], str) else 0.5)
    want = np.zeros((64, 8))
    for e, (I, J, i, j, h, n) in enumerate(np.ndindex(*(2,) * 6)):
        want[e, phys(2 * J + j, n)] = scale(2 * I + i, 2 * J + j, h, n) / GAMMA
    coef = np.round(np.linalg.solve(np.array(rows, float).T, want) * 4096) / 4096
    assert (np.array(rows).T @ coef == want).all()
    return {x: e for e, x in enumerate(sites) if coef[e].any() or isinstance(x[1], tuple)}, coef, extra


def yds(groups, cap):
    n = len(cap)
    speed, cls, gcls = [0.0] * n, [-1] * n, {}
    todo = list(groups)
    while todo:
        pre = [0.0]
        for t in range(n):
            pre.append(pre[-1] + (cap[t] if cls[t] < 0 else 0.0))
        best = None
        for a in sorted({g[0] for g in todo}):
            w = 0.0
            for g in sorted((g for g in todo if g[0] >= a), key=lambda g: g[1]):
                w += g[2]
                d = w / max(pre[g[1] + 1] - pre[a], 1e-9)
                if best is None or d > best[0]:
                    best = (d, a, g[1])
        d, a, b = best
        for t in range(a, b + 1):
            if cls[t] < 0:
                speed[t], cls[t] = d, len(gcls)
        gcls.update({g[:2]: len(gcls) for g in todo if g[0] >= a and g[1] <= b})
        todo = [g for g in todo if not (g[0] >= a and g[1] <= b)]
    return speed, cls, gcls


def spread_jobs(jobs, cap, vcap, tail):
    T = len(cap)
    cap3 = cap * 3
    all3 = [(j[0] + k * T, j[1] + k * T, ji, k) for k in range(3) for ji, j in enumerate(jobs) if j[0] + k * T >= 0]
    pend = {}
    for j in sorted(all3, key=lambda j: (j[1], j[3], j[2])):
        pend.setdefault(j[:2], []).append(j)
    left = {w: sum(sum(jobs[j[2]][2]) for j in q) for w, q in pend.items()}
    speed, cls, gcls = yds([w + (left[w],) for w in pend], cap3)
    cum = [0.0]
    for t in range(3 * T):
        cum.append(cum[-1] + speed[t] * cap3[t])
    when = [[] for _ in jobs]
    debt, vdebt, cur, done = 0.0, 0.0, None, 0

    def fits(j, t):
        need = max(debt, 0.0) + sum(jobs[j[2]][2]) + 1.0
        for w in pend:
            if w[1] >= j[1]:
                break
            if left[w] > 1e-9:
                need += left[w]
                if need > cum[w[1] + 1] - cum[t]:
                    return False
        return True

    for t in range(3 * T):
        if t % T == 0:
            debt, vdebt = min(debt, 0.0), -0.5
        while True:
            rdy = [q[0] for w, q in pend.items() if q and w[0] <= t and (gcls[w] == cls[t] or w[1] <= t)]
            j = cur
            if j is None:
                if not rdy:
                    debt = max(debt, 0.0)
                    break
                j = rdy[0]
                if j[1] > t:
                    j = (min if vdebt > 0 else max)([x for x in rdy if x is j or fits(x, t)], key=lambda x: jobs[x[2]][3])
                nst = len(jobs[j[2]][2])
                if nst > 1 and j[1] > t and (t + tail + 2 * nst) // T != t // T:
                    break
            must = j[1] <= t or (cur is not None and ((t + tail + 1) // T != t // T or (rdy and rdy[0][1] <= t)))
            if not must and (cap3[t] == 0.0 or debt > 0.5 * speed[t] * cap3[t]):
                break
            if cur is None:
                pend[j[:2]].pop(0)
                left[j[:2]] -= sum(jobs[j[2]][2])
                cur, done = j, 0
            debt += jobs[j[2]][2][done]
            vdebt += jobs[j[2]][2][done] * jobs[j[2]][3]
            if j[3] == 1:
                when[j[2]].append(t - T)
            done += 1
            if done == len(jobs[j[2]][2]):
                cur = None
        debt -= speed[t] * cap3[t]
        vdebt = min(max(vdebt - vcap[t % T], -0.5), 1.0)
    assert all(j[0] <= ts[0] and ts[-1] <= j[1] and (ts[0] < 0) == (ts[-1] < 0) for j, ts in zip(jobs, when))
    return when


def _kernel(x_hbm, w_hbm, b_hbm, o_hbm, *scratch, L, TM, R0, NMAIN, D, cfg):
    H, Mh, Mq = D // 4, TM // 4, TM // 8
    NC, NQ = Mh // 16, Mq // 16
    it = iter(scratch)
    take = lambda n: [next(it) for _ in range(n)]
    x0b, xb, ib, ob, jb = take(4), take(7), take(16), take(56), take(20)
    s2 = dict(zip(range(1, 8), take(7)))
    s3 = {(p, kind): next(it) for p in OUTER if p != 1 for kind in KINDS}
    t2 = dict(zip(range(1, 8), take(7)))
    t3_ref, kb0, kb1, bt_ref, bf_ref, xn2_ref, o2_ref, w0_ref, w_ref, xr_ref, xp_ref, b_ref, sem = it
    sites, bcoef, extra = bias_sites()
    pos2 = lambda p, q: ORD.index(q) if p == 1 else 0

    xset = lambda l: 6 if l == 'O' else 4 if l == 0 else (l % 2) * 2
    xoff = lambda I, J: 16 * ((I + J) % 2)
    xloc = lambda l, R, C, k: (xb[xset(l) + R // 2], (R % 2, C, k), xoff(R // 2, C // 2))
    x0loc = lambda R, C, k: (x0b[(R // 2) * 2 + C // 2], (R % 2, C % 2, k), 8 + xoff(R // 2, C // 2))
    iloc = lambda g, name, n: (ib[((g % 2) * 4 + ISL[name]) * 2 + n], (), 8 * ISL[name])
    oloc = lambda name, i, j, n: (ob[(OSL[name] * 4 + i * 2 + j) * 2 + n], (), 8 * ((OSL[name] + 2 * j) % 4))

    def jloc(kind, name, al, guest=False):
        u = ('1', 's', 'k').index(name)
        return jb[18 + al if guest else (KINDS.index(kind) * 3 + u) * 2 + al], (), 8 * ((3 * u + al) % 4)

    def tie(v, anchor, r=None, lo=0):
        if anchor is None:
            return v
        never, gate = anchor
        if r is None:
            n = v.shape[0]
            return jax.lax.select(never[n], gate if n == 8 else jnp.tile(gate, (n // 8, 1)), v)
        top = jax.lax.select(never[8], gate, v[r:r + 8])
        return jnp.concatenate(([v[lo:r]] if r > lo else []) + [top, v[r + 8:r + 16]], axis=0)

    def consts(anchor, ss):
        one = {s: tie(jnp.full((8, 128), s, f32), anchor) for s in set(ss)}
        return jnp.concatenate([one[s] for s in ss for _ in range(2)], axis=0)

    def conv(src, R, Q, r, zs, anchor):
        v = src[R * Mh + r:R * Mh + r + 32, Q * H:(Q + 1) * H].astype(f32)
        for j in range(2):
            C, k = 2 * (Q // 2) + j, Q % 2
            buf, idx, off = xloc(0, R, C, k)
            sv = consts(anchor, [scale(R, C, (r + u) // Mq, k) for u in (0, 16)])
            buf[(zs,) + idx + (slice(off + r, off + r + 32),)] = v[:, j * 128:(j + 1) * 128] * sv

    count = {}
    def block_sum(l, terms, ii, jj, kk, r, save, zs, za, anchor, gate=True):
        rng = lambda t: slice(t[0], t[-1] + 1)
        vals = []
        for u, ((I, J), s) in enumerate(terms):
            ref, r0 = xb[xset(l) + I], xoff(I, J) + r
            v = ref[za if u == 0 else 0, rng(ii), 2 * J + jj[0]:2 * J + jj[-1] + 1, rng(kk), r0:r0 + 16, :]
            if (I, J) == save:
                sv = consts(anchor, [GAMMA / scale(2 * I + i, 2 * J + j, r // Mq, k) for i in ii for j in jj for k in kk])
                x0b[I * 2 + J][zs, rng(ii), rng(jj), rng(kk), r0 + 8:r0 + 24, :] = v * sv.reshape(v.shape)
            if u == 0 and gate:
                count[xset(l)] = count.get(xset(l), -1) + 1
                if count[xset(l)] % cfg['GE'] == 0:
                    ref[0, 0, 0, 0, Mh + 24:Mh + 32, :] = count.get('prev', anchor)[1]
                count['prev'] = anchor
            vals.append((s, v))
        v = lincomb(vals)
        return v.reshape(v.size // 128, 128)

    def operands(a, group, st8, store):
        for u, b in enumerate(group):
            st8[b] = a if len(group) == 1 else a[:, u:u + 1]
        ops = {}
        if B12 in group:
            ops[3], ops[5] = st8[B11] - st8[B12], st8[B11] + st8[B12]
        if B22 in group:
            ops[4], ops[7] = st8[B12] + st8[B22], st8[B12] - st8[B22]
            ops[1] = st8['l1'] = st8[B11] + st8[B22]
        if B21 in group:
            g = st8[B12] + st8[B21]
            ops[2], ops[6] = g + st8['l1'], g - st8['l1']
        now = [q for q in ORD if q in ops]
        if now:
            u = ORD.index(now[0])
            store(slice(u, u + len(now)), jnp.concatenate([ops[q] for q in now], axis=1).astype(bf16))

    def unit1(l, c, k, save, st8, group, zs, za, anchor):
        def store(pos, v):
            s2[1][zs, k:k + 1, pos, 16 * c:16 * c + 16, :] = v
        e = block_sum(l, LA[1], [group[0][0]], [0, 1], [k], 16 * c, save, zs, za, anchor)
        operands(tie(e, anchor, 16).reshape(1, 2, 16, 128), group, st8, store)

    def unit26(l, c, k, save, st8, group, zs, za, anchor):
        i = group[0][0]
        f = block_sum(l, [(B11, 1), (B22, 1)], [i], [0, 1], [k], 16 * c, save, zs, za, anchor, False)
        e = tie(block_sum(l, [(B12, 1), (B21, 1)], [i], [0, 1], [k], 16 * c, save, zs, za, anchor), anchor)
        for J, v in enumerate((e + f, e - f)):
            r0 = xoff(0, J) + 16 * c
            xb[6][zs, i, 2 * J:2 * J + 2, k, r0:r0 + 16, :] = v.reshape(2, 16, 128)

    def unit3(l, p, kind, c, save, st8, group, zs, za, anchor):
        def store(pos, v):
            s3[(p, kind)][zs, :, pos, 16 * c:16 * c + 16, :] = v
        h, kk = group[0][0], [b[1] for b in group]
        ii, jj = {'35': ([0], [0, 1]), '47': ([0, 1], [1]), '26': ([0, 1], [0, 1])}[kind]
        src = (l, LA[p]) if p in LA else ('O', [((0, (2, 6).index(p)), 1)])
        n = 16 * len(kk)
        v = block_sum(*src, ii, jj, kk, h * Mq + 16 * c, save, zs, za, anchor)
        if kind == '26':
            e, f = tie(v, anchor, 16, 16) + v[32:48], v[0:16] + v[48:64]
            r0 = h * Mq + 16 * c
            s2[p][zs, kk[0], 0, r0:r0 + 16, :] = f.astype(bf16)
        else:
            e, f = tie(v, anchor, n - 16), v[n:]
        operands(jnp.concatenate([e + f, e - f], axis=0).reshape(2, len(kk), 16, 128), group, st8, store)

    GAPS = [w for pos in range(4) for w in [1] + [x for p in (2, 6, 3, 5, 1, 4, 7) for x in (
        [19] if p == 1 else [25] if pos < 3 else [13] + [19] * 6)]]

    def wtile(idx, n):
        if cfg.get('NOBC'):
            return w_ref[idx].reshape(16 * n, 128)
        return pltpu.bitcast(w_ref.bitcast(u32)[idx].reshape(8 * n, 128), bf16)

    def prep(l, u, anchors, zero, kb):
        mul = lambda v, s: v if s == 1.0 else v * s
        stack = lambda T: jnp.concatenate([T[q] for q in ORD], axis=0).reshape(7, 16, 128).astype(bf16)
        rows = pl.ds(16 * u, 16) if isinstance(u, int) else pl.ds(pl.multiple_of(16 * u, 16), 16)
        for k in range(2):
            if isinstance(l, int):
                wide = [w0_ref[phys(R, k), u].astype(f32) for R in range(4)]
                tile = lambda R, c: wide[R][:, c * 128:(c + 1) * 128]
            else:
                wide = [wtile((l - 1, slice(None), phys(R, k), u), 8).astype(f32) for R in range(4)]
                tile = lambda R, c: wide[R][c * 16:(c + 1) * 16]
            for n in range(2):
                anchor = next(anchors)
                blk = lambda R, C: mul(tile(R, phys(C, n)), scale(R, C, k, n))
                O = {(i, j): b_ops(blk(i, j), tie(blk(i, 2 + j), anchor, 0), blk(2 + i, j), blk(2 + i, 2 + j))
                     for i, j in BLOCKS}
                for p in (2, 6, 3, 5, 1, 4, 7):
                    o = [mul(O[b][p], 4.0 if p == 1 else 1.0) for b in BLOCKS]
                    T = b_ops(o[0], tie(o[1], next(anchors), 0), o[2], o[3], True)
                    if p == 1:
                        T[1] = T[1] * 2.0
                        t2[p][l, n, k, :, rows, :] = stack(T)
                        continue
                    t2[p][l, n, k, 0, rows, :] = (T[1] * 4.0).astype(bf16)
                    e0 = PRODS3.index((p, 5))
                    if (k, n) != (1, 1):
                        kb[zero, k * 2 + n, 16 * e0:16 * e0 + 96, :] = jnp.concatenate(
                            [T[q] for _, q in PRODS3[e0:e0 + 6]], axis=0)
                        continue
                    for e in range(e0, e0 + 6):
                        v = kb[0, 0:3, 16 * e:16 * e + 16, :]
                        T3 = b_ops(v[0], tie(v[1], next(anchors), 0), v[2], T[PRODS3[e][1]], True)
                        T3[1] = T3[1] * 2.0
                        t3_ref[l, e, :, rows, :] = stack(T3)

    outs = [(l, p) for l in range(L) for p in OUTER]
    G = len(outs)
    sched, start, use, vuse = [], [], [], []
    for g, (l, p) in enumerate(outs):
        start.append(len(use))
        for rd in rounds_of(p):
            n = NQ if isinstance(rd[1], str) else NC
            sched.append((g, rd, len(use), n))
            a, st_ = round_usage(p, rd, l == 0, l == L - 1, rd in DEFER.get(p, ()))
            a += extra.get((p, rd), 0)
            use += [max((2 * a + st_ + 2 + 16 / n) / 72, cfg['PORT'] * st_ / 8)] * n
            vuse += [st_ / 8] * n
    T = len(use)
    first = lambda g, kind: next(t0 for gg, rd, t0, _ in sched if gg == g and rd[0] == kind)
    jobs, late = [], []
    def add(lo, hi, alu, st_, ld_, scheme, kind, fn):
        w = alu / 64 + cfg['CS'] * (st_ + len(STAGES[scheme])) / 16 + cfg['CL'] * ld_ / 48
        jobs.append((lo, max(hi, lo), [w * f for _, f in STAGES[scheme]], st_ / 16 / w, scheme, kind, fn))
    for g, (l, p) in enumerate(outs):
        for gg, rd, t0, n_ in sched:
            if gg == g and rd in DEFER.get(p, ()):
                last = l == L - 1
                nops = sum(len(t.split()) + 1 + (l > 0) + 1.5 * last for _, t in OACT[p][1])
                islate = last and p == 6 and rd[0] == '26'
                due = {5: lambda: start[7 * l + 5] - 1, 7: lambda: start[g + 1] + cfg['EW7'],
                       6: lambda: T - cfg['TAIL'] - 1 if last else min(start[g + 1] + cfg['EW6'], first(g + 1, rd[0])) - 1}[p]()
                both = last and rd[0] == '26'
                step = cfg['FR'][(p == 6) + 2 * both]
                for r0 in range(0, Mq, step):
                    nr = min(step, Mq - r0)
                    for h, n in DONE[rd[1]]:
                        for leaves in [DONE[rd[0]]] if both else [[b] for b in DONE[rd[0]]]:
                            fn = (l, p, leaves, h, n, r0, nr)
                            nv = len(leaves) * nr // 8
                            add(0 if islate else t0 + n_, cfg['EW6'] - 1 if islate else due, nops * nv,
                                nv * len(OACT[p][1]) / (1 + both) - 1, 0.9 * nops * nv, 1, 'fin', fn)
                            if islate:
                                late.append(fn)
        if p in (3, 5):
            lo = start[7 * l - 2] + (cfg['EW7'] + 1 if l else -T)
        else:
            lo = start[7 * l] + cfg['EW6']
        hi = start[g] - LAG - 3
        save = SAVE.get(p) if l == 0 else None
        sv = save is not None
        if p == 1:
            for c, k in np.ndindex(NC, 2):
                add(lo, hi, 31 + 8 * sv, 7 + 8 * sv, 16, 2, l, functools.partial(unit1, l, c, k, save))
            continue
        nt = 2
        if p in (2, 6):
            mid = start[7 * l + 3] + cfg['MOFF']
            if p == 2:
                for c, k in np.ndindex(NC, 2):
                    add(lo, mid - 3, 40 + 8 * sv, 16 + 8 * sv, 32, 'O', l, functools.partial(unit26, l, c, k, save))
            lo, nt, save, sv = mid, 1, None, False
        for c in range(NQ):
            add(lo, hi if p in GUEST else first(g - 1, 'y') - LAG - 3, 32 * nt + 50 + 32 * sv, 18 + 32 * sv, 32 * nt,
                4, l, functools.partial(unit3, l, p, '26', c, save))
        for c in range(NQ):
            for kind in KINDS[:2]:
                add(lo, hi + (NC if g else 0), 16 * nt + 46, 14, 16 * nt, 3, l, functools.partial(unit3, l, p, kind, c, None))
    convs = [(R, Q, r) for R in range(4) for Q in range(4) for r in range(0, Mh, 32)]
    for x in convs:
        add(start[6], start[G - 2] - 2, 18, 7, 4, 1, 'conv', x)
    cap = [max(cfg['CAP'] - max(use[t], use[(t + 1) % T]), 0.0) * (t < T - cfg['TAIL']) for t in range(T)]
    when = spread_jobs(jobs, cap, [cfg['VK'] * (1 - vuse[(t + 1) % T]) for t in range(T)], cfg['TAIL'])
    plan = {}
    for t, _, ji, u in sorted((t % T, ts[0] % T, ji, u) for ji, ts in enumerate(when) for u, t in enumerate(ts)):
        plan.setdefault(t, []).append((jobs[ji][5], jobs[ji][6], STAGES[jobs[ji][4]][u][0]))
    assert cfg['EW6'] <= first(0, '26')
    carried = [job for ts, job in zip(when, jobs) if ts[0] < 0]

    def w_copy(l, c=None):
        if c is None:
            return pltpu.make_async_copy(w_ref.at[l - 1], w_ref.at[l - 1], sem.at[l])
        return pltpu.make_async_copy(w_hbm.at[l, :, :, :, pl.ds(c * 128, 128)], w_ref.at[l - 1, c], sem.at[l])

    def w0_copy(u):
        return pltpu.make_async_copy(w_hbm.at[0, :, u], w0_ref.at[:, u], sem.at[L + 6 + u])

    def in_copy(t, slot):
        return pltpu.make_async_copy(x_hbm.at[pl.ds(pl.multiple_of(t * TM, 32), TM)], xn2_ref.at[slot], sem.at[L + slot])

    def out_copy(t, slot, part):
        r0, nr = (0, TM) if part is None else ((0, 4 * Mq), (4 * Mq, Mq), (5 * Mq, Mq), (6 * Mq, 2 * Mq))[part]
        return pltpu.make_async_copy(o2_ref.at[slot, pl.ds(r0, nr)],
                                     o_hbm.at[pl.ds(pl.multiple_of(t * TM + r0, 16), nr)], sem.at[L + 4 + slot])

    xr_in = pltpu.make_async_copy(x_hbm.at[pl.ds(NMAIN * TM, R0)], xr_ref, sem.at[L + 2])
    xr_out = pltpu.make_async_copy(xr_ref, o_hbm.at[pl.ds(NMAIN * TM, R0)], sem.at[L + 2])
    b_in = pltpu.make_async_copy(b_hbm, b_ref, sem.at[L + 3])
    opaque = lambda i, s: jax.lax.shift_right_logical(i, s)
    mask = lambda zero: {n: jnp.broadcast_to(zero, (n, 128)) != 0 for n in (8, 16, 32)}

    def prologue():
        b_in.start()
        for u in range(8):
            w0_copy(u).start()
        xr_in.start()
        in_copy(0, 0).start()
        b_in.wait()
        for l in range(L):
            bf_ref[l] = b_ref[l:l + 1, :].astype(f32)

        def bias_tiles(l, carry):
            b = jnp.broadcast_to(bf_ref[l] + (l == 0).astype(f32), (8, D))
            for u in sites.values():
                terms = [b[:, e * 128:(e + 1) * 128] * float(cf) for e, cf in enumerate(bcoef[u]) if cf != 0.0]
                bt_ref[l, u] = functools.reduce(lambda x, y: x + y, terms or [jnp.zeros((8, 128), f32)])
            return carry
        jax.lax.fori_loop(0, L, bias_tiles, 0)
        if cfg.get('FAST'):
            return

        def slab(u, carry):
            w0_copy(u).wait()
            prep(0, u, iter(lambda: None, 0), opaque(u, 12), kb0)
            return opaque(u, 12)
        zero = jax.lax.fori_loop(0, cfg['NSLAB'], slab, 0)

        halves = lambda x: (x[:, :D // 2].astype(bf16), x[:, D // 2:].astype(bf16))

        def plain(l, xbf, x0f, x, j0, j1, gaps, free, never):
            passes = []
            for jt in range(j0, j1):
                cols = slice(jt * 128, (jt + 1) * 128)
                w = [w0_ref[b:b + 4, :, :, cols].reshape(D // 2, 128) if isinstance(l, int)
                     else wtile((l - 1, jt, slice(b, b + 4)), 32) for b in (0, 4)]
                ya = _dot(xbf[0], w[0]) + bf_ref[l, :, cols]
                passes += [ya, _dot(xbf[1], w[1]) + ya]
            xp_ref[0, :, j0 * 128:j1 * 128] = x0f * jnp.concatenate(passes[1::2], axis=1) + x
            for u in range(len(gaps)):
                ps, rr = divmod(sum(gaps[free:u]) * len(passes) * (R0 // 8) // sum(gaps[free:]), R0 // 8)
                yield None if u < free else (never, passes[ps][rr * 8:rr * 8 + 8, :])

        for l in range(1, L):
            for c in range(8):
                w_copy(l, c).start()
        in_copy(1, 1).start()
        for u in range(cfg['NSLAB'], 8):
            w0_copy(u).wait()
        xr_in.wait()
        jm = cfg['JM']
        x0f = xr_ref[:, :jm * 128].astype(f32)
        xp_ref[1, :, :jm * 128] = x0f
        anchors = plain(0, halves(xr_ref), x0f, x0f, 0, jm, (8 - cfg['NSLAB']) * GAPS, 2, mask(zero))
        for u in range(cfg['NSLAB'], 8):
            prep(0, u, anchors, zero, (kb0, kb1)[u % 2])
        in_copy(0, 0).wait()
        x0f = xr_ref[:, jm * 128:].astype(f32)
        xp_ref[1, :, jm * 128:] = x0f
        blank = [loc for j, n in BLOCKS for loc in [oloc(x, 1, j, n) for x in OSL]
                 + [f(3, 2 * J + j, n) for J in range(2) for f in (x0loc, functools.partial(xloc, L - 1))]]
        na = len(convs) + sum(len(j[2]) for j in carried) + 2 * len(blank) + 2
        anchors = plain(0, halves(xr_ref), x0f, x0f, jm, 8, [1] * na, 4, mask(zero))
        for x in convs[:len(convs) // 2]:
            conv(xn2_ref.at[0], *x, zero, next(anchors))
        for job in carried:
            st8 = {}
            for group, _ in STAGES[job[4]]:
                job[6](st8, group, zero, opaque(zero, 1), next(anchors))
        for x in convs[len(convs) // 2:]:
            conv(xn2_ref.at[0], *x, zero, next(anchors))
        for ref, idx, off in blank:
            for r0 in (off, off + Mq):
                ref[(0,) + idx + (slice(r0, r0 + Mq),)] = consts(next(anchors), [0.0] * NQ)

        def layer(l, carry):
            w_copy(l).wait()
            x, zero = xp_ref[0], opaque(l, 12)
            anchors = plain(l, halves(x), xp_ref[1], x, 0, 8, 8 * GAPS, 2, mask(zero))
            for u in range(8):
                prep(l, u, anchors, zero, (kb0, kb1)[u % 2])
            return carry

        jax.lax.fori_loop(1, L, layer, 0)
        xr_ref[...] = xp_ref[0].astype(bf16)
        xr_out.start()

    def main(tile, carry, only_late=False):
        zs, za = opaque(tile, 12), opaque(tile, 13)
        never = mask(zs)
        slot = tile % 2
        out = [o2_ref.at[1 - slot]]

        def rows(h, r0):
            lo, n = (0, Mh) if h is None else h if isinstance(h, tuple) else (h * Mq, Mq)
            return slice(r0 + lo, r0 + lo + n)

        def ld(loc, h):
            return loc[0][(0,) + loc[1] + (rows(h, loc[2]),)]

        def st(loc, v, h):
            loc[0][(zs,) + loc[1] + (rows(h, loc[2]),)] = v

        def operand(ref, idx, n):
            if cfg.get('NOBC'):
                return ref[idx + (slice(0, n),)]
            return pltpu.bitcast(ref.bitcast(u32)[idx + (slice(0, n // 2),)], bf16)

        def dot3(l, p, q, r):
            kind = next(x for x in KINDS if q in PAIR[x])
            return _dot(operand(s3[(p, kind)], (0, PAIR[kind].index(q), ORD.index(r)), Mq),
                        operand(t3_ref, (l, PRODS3.index((p, q)), ORD.index(r)), 128))

        def issue(l, p, rd):
            kind, n = rd
            if kind == 'x':
                return [dot3(l, p, q, 1) for q in (3, 5, 4, 7)]
            if kind == 'y':
                return [dot3(l, x, q, 1) for x in (p, GUEST[p]) for q in (2, 6)]
            if isinstance(n, str):
                return [dot3(l, p, int(q), int(r)) for q in kind for r in n]
            lhs = {q: [operand(s2[p], (0, k, pos2(p, q)), Mh) for k in range(2)] for q in map(int, kind)}
            return [_dot(lhs[q][k], operand(t2[p], (l, nn, k, pos2(p, q)), 128))
                    for q, nn in ([(1, 0), (1, 1)] if kind == '1' else [(int(q), n) for q in kind]) for k in range(2)]

        def biased(v, l, *site):
            if site not in sites:
                return v
            return (v.reshape(Mq // 8, 8, 128) + bt_ref[l, sites[site]]).reshape(Mq, 128)

        wait = {}
        def outer_act(l, p, i, j, n, d, h, part=None, last=lambda b, y: y):
            stores, finals = OACT[p]
            if part == 'park':
                stores, finals = stores[:1], []
            elif part == 'rest' or (p == 6 and (i, j) != B12 and (h, n) != B12):
                stores = stores[1:]
            cache = {'d': d}
            def comb(terms):
                for t in terms.split():
                    if t[1:] not in cache:
                        cache[t[1:]] = ld(oloc(t[1:], i, j, n), h)
                return lincomb([(int(t[0] + '1'), cache[t[1:]]) for t in terms.split()])
            fin = [(IJ, last(IJ, comb(terms))) for IJ, terms in finals]
            for name, v in [(name, comb(terms)) for name, terms in stores]:
                st(oloc(name, i, j, n), v, h)
            for (I, J), y in fin:
                R, C = 2 * I + i, 2 * J + j
                xn = ld(x0loc(R, C, n), h) * y
                if l > 0:
                    xn = xn + ld(xloc(l, R, C, n), h)
                if l < L - 1:
                    st(xloc(l + 1, R, C, n), xn, h)
                    continue
                s = scale(R, C, rows(h, 0).start // Mq, n)
                xn = xn if s == 1.0 else xn * (1.0 / s)
                c0 = phys(C, n) * 128
                if i == 0:
                    out[0][rows(h, R * Mh), c0:c0 + 128] = xn.astype(bf16)
                elif j == 1:
                    wait[J] = xn
                else:
                    out[0][rows(h, R * Mh), c0:c0 + 256] = jnp.concatenate([xn, wait.pop(J)], axis=1).astype(bf16)

        def inner_act(g, l, p, kind, n, h, P, Q, part=None):
            vloc = iloc(g, 'v', n) if p == 1 else oloc(OACT[p][0][0][0], 0, 1, n)
            if kind == '35':
                st(iloc(g, 's', n), Q + ld(iloc(g, 'm1', n), h), h)
                if p == 1:
                    st(vloc, P, h)
                outer_act(l, p, 0, 1, n, P, h, part)
            elif kind == '47':
                st(iloc(g, 'u', n), Q + ld(vloc, h), h)
                outer_act(l, p, 0, 0, n, P + ld(iloc(g, 's', n), h), h, part)
            else:
                outer_act(l, p, 1, 1, n, ld(iloc(g, 's', n), h) - Q, h, part)
                outer_act(l, p, 1, 0, n, P + ld(iloc(g, 'u', n), h), h, part)

        def consume(g, l, p, rd, res):
            kind, n = rd
            if n == '1':
                for u, (kd, x) in enumerate([('35', p), ('47', p)] if kind == 'x' else [('26', p), ('26', GUEST[p])]):
                    for al in range(2):
                        st(jloc(kd, '1', al, x != p), biased(res[2 * u + al], l, x, int(kd[al]), '1'), 0)
            elif isinstance(n, str):
                sm = [res[2 * al] + res[2 * al + 1] for al in range(2)]
                df = [res[2 * al] - res[2 * al + 1] for al in range(2)]
                J = lambda name, al: ld(jloc(kind, name, al, name == '1' and kind == '26' and p not in GUEST), 0)
                part = 'park' if rd in DEFER.get(p, ()) else None
                done = lambda h, nn, m: inner_act(g, l, p, kind, nn, h, m[0] + m[1], m[0] - m[1], part)
                if n == '35':
                    for al in range(2):
                        st(jloc(kind, 's', al), df[al] + J('1', al), 0)
                    done(0, 1, [biased(sm[al], l, p, int(kind[al]), 'v') for al in range(2)])
                elif n == '47':
                    for al in range(2):
                        st(jloc(kind, 'k', al), biased(df[al], l, p, int(kind[al]), 'k'), 0)
                    done(0, 0, [biased(sm[al] + J('s', al), l, p, int(kind[al]), 'm') for al in range(2)])
                else:
                    O = lambda i, j: ld(oloc(OACT[p][0][0][0], i, j, 1), 0)
                    m = [sm[al] + J('k', al) for al in range(2)]
                    P = m[0] + m[1] + O(*{'35': B12, '47': B11, '26': B21}[kind])
                    Q = m[0] - m[1] - (ld(iloc(g, 'm1', 1), 0) if kind == '35' else O(*{'47': B12, '26': B22}[kind]))
                    done(1, 1, [J('s', al) - df[al] for al in range(2)])
                    inner_act(g, l, p, kind, 0, 1, P, Q, part)
            else:
                m = []
                for al, (q, nn) in enumerate([(1, 0), (1, 1)] if kind == '1' else [(int(q), n) for q in kind]):
                    v = res[2 * al] + res[2 * al + 1]
                    if any((p, q, (h, nn)) in sites for h in range(2)):
                        v = jnp.concatenate([biased(v[h * Mq:(h + 1) * Mq], l, p, q, (h, nn)) for h in range(2)], axis=0)
                    m.append(v)
                if kind == '1':
                    for nn in range(2):
                        st(iloc(g, 'm1', nn), m[nn], None)
                else:
                    inner_act(g, l, p, kind, n, None, m[0] + m[1], m[0] - m[1])

        def finish(l, p, leaves, h, n, r0, nr, anchor):
            for i, j in leaves:
                d = ld(oloc(OACT[p][0][0][0], i, j, n), (h * Mq + r0, nr))
                last = lambda b, y: (y.reshape(nr // 8, 8, 128)
                                     + tie(bt_ref[l, sites[(b, (i, j), (h, n))]], anchor)).reshape(nr, 128)
                outer_act(l, p, i, j, n, d, (h * Mq + r0, nr), 'rest', last)

        if only_late:
            for x in late:
                finish(*x, None)
            out_copy(tile - 1, 1 - slot, 3).start()
            return carry
        state = {}
        count.clear()
        for g, rd, t0, n in sched:
            l, p = outs[g]
            if t0 == start[1]:
                pl.when(tile > 0)(lambda: out_copy(tile - 1, 1 - slot, 3).start())
                out[0] = o2_ref.at[slot]
            if t0 == first(G - 2, '35'):
                assert t0 > start[G - 2] + cfg['EW7']
                out_copy(tile, slot, 0).start()
            res = issue(l, p, rd)
            if t0 == first(G - 2, '35'):
                out[0][TM - 8:TM, 0:128] = res[0][0:8, :].astype(bf16)
            for t in range(t0, t0 + n):
                if t in plan:
                    r0 = 16 * (t - t0) + 8
                    anchor = (never, res[0 if isinstance(rd[1], str) else 1][r0:r0 + 8, :])
                for kind, fn, group in plan.get(t, []):
                    if kind == 'fin':
                        finish(*fn, anchor)
                    elif kind == 'conv':
                        conv(xn2_ref.at[1 - slot], *fn, zs, anchor)
                    else:
                        fn(state.setdefault(id(fn), {}), group, zs, za, anchor)
            if t0 == first(G - 1, '26'):
                out_copy(tile, slot, 1).start()
            if t0 + n == T:
                out_copy(tile, slot, 2).start()
            consume(g, l, p, rd, res)
        pl.when(tile + 3 < NMAIN)(lambda: in_copy(tile + 3, 1 - slot).start())
        pl.when(tile > 0)(lambda: out_copy(tile - 1, 1 - slot, None).wait())
        pl.when(tile + 2 < NMAIN)(lambda: in_copy(tile + 2, slot).wait())
        return carry

    prologue()
    in_copy(2, 0).start()
    in_copy(1, 1).wait()
    jax.lax.fori_loop(0, NMAIN, main, 0)
    main(jnp.int32(NMAIN), 0, True)
    xr_out.wait()
    out_copy(NMAIN - 1, (NMAIN - 1) % 2, None).wait()


def build(TM=640, **kw):
    def f(x0, ws, bs):
        B, D = x0.shape
        L = ws.shape[0]
        Mh = TM // 4
        nmain = (B - 1) // TM
        R0 = B - nmain * TM
        assert D == 1024 and L % 2 == 0 and L <= 8 and TM % 128 == 0 and R0 % 16 == 0 and nmain >= 3
        n3 = len(PRODS3)
        odd = lambda n: 16 * (n // 16 | 1)
        V = pltpu.VMEM
        scratch = ([V((1, 2, 2, 2, Mh + 40, 128), f32)] * 4 + [V((1, 2, 4, 2, Mh + 40, 128), f32)] * 7
                   + [V((1, Mh + 32, 128), f32)] * (16 + 56 + 20)
                   + [V((1, 2, 10 if p == 1 else 2, odd(Mh), 128), bf16) for p in range(1, 8)]
                   + [V((1, 2, 10, odd(Mh // 2), 128), bf16)] * (n3 // 2)
                   + [V((L, 2, 2, 7 if p == 1 else 1, 128, 128), bf16) for p in range(1, 8)]
                   + [V((L, n3, 7, 128, 128), bf16)] + [V((1, 4, 16 * n3 + 16, 128), f32)] * 2
                   + [V((L, 64, 8, 128), f32), V((8, 1, D), f32), V((2, TM, D), bf16), V((2, TM, D), bf16),
                      V((8, 8, 16, D), bf16), V((L - 1, 8, 8, 8, 16, 128), bf16), V((R0, D), bf16), V((2, R0, D), f32), V((L, D), bf16),
                      pltpu.SemaphoreType.DMA((L + 14,))])
        anyspec = pl.BlockSpec(memory_space=pl.ANY)
        return pl.pallas_call(
            functools.partial(_kernel, L=L, TM=TM, R0=R0, NMAIN=nmain, D=D, cfg=dict(CFG, **kw)),
            in_specs=[anyspec, anyspec, anyspec],
            out_specs=anyspec,
            out_shape=jax.ShapeDtypeStruct((B, D), x0.dtype),
            scratch_shapes=scratch,
            compiler_params=pltpu.CompilerParams(
                vmem_limit_bytes=120 * 1024 * 1024,
                internal_scratch_in_bytes=65536,
                disable_bounds_checks=True,
                disable_semaphore_checks=True,
            ),
        )(x0, ws.reshape(L, 8, 8, 16, D), bs)
    return f


@jax.jit
def pallas_standalone__dcn_v2_cross__recsys_kernel(x0, ws, bs):
    return build()(x0, ws, bs)
```

```python
import functools

import jax
import jax.numpy as jnp
import numpy as np
import jax.experimental.pallas as pl
import jax.experimental.pallas.tpu as pltpu

f32 = jnp.float32
bf16 = jnp.bfloat16
u32 = jnp.uint32

B11, B12, B21, B22 = BLOCKS = (0, 0), (0, 1), (1, 0), (1, 1)
LA = {1: [(B11, 1), (B22, 1)], 3: [(B11, 1), (B12, -1)], 5: [(B11, 1), (B12, 1)], 4: [(B12, 1), (B22, 1)],
      7: [(B12, 1), (B22, -1)]}
PC = {1: (1, 0, 0, 1), 2: (0, 0, 1, -1), 3: (1, 1, 1, 1), 4: (1, 0, 1, 0), 5: (-1, 1, 1, -1), 6: (0, 0, 1, 1),
      7: (1, 0, -1, 0)}
KINDS = ('35', '47', '26')
PAIR = {'35': (5, 3), '47': (4, 7), '26': (2, 6)}
ORD = (3, 5, 4, 7, 1, 2, 6)
OUTER = (3, 5, 1, 4, 7, 2, 6)
GUEST = {3: 5, 4: 7, 2: 6}
PRODS3 = [(p, q) for p in OUTER if p != 1 for kind in KINDS for q in PAIR[kind]]
GAMMA = 0.125
OACT = {
    3: ([('M3', '+d')], []),
    5: ([('M5', '+d')], [(B12, '+d +M3')]),
    1: ([('S', '+d +M3 -M5')], []),
    4: ([('M4', '+d')], []),
    7: ([('M7', '+d')], [(B11, '+d +S +M4')]),
    2: ([('M2', '+d')], []),
    6: ([('M6', '+d')], [(B22, '+d +S -M2'), (B21, '+d +M2 +M4 -M7 +M3 +M5')]),
}
OSL = {'M3': 0, 'M5': 1, 'S': 2, 'M4': 3, 'M7': 4, 'M2': 5, 'M6': 6}
ISL = {'m1': 0, 's': 1, 'v': 2, 'u': 3}
DEFER = {5: [('26', '26'), ('47', '26'), ('35', '26')], 7: [('26', '26'), ('47', '26'), ('35', '26')],
         6: [('26', '26'), ('47', '26'), ('35', '26'), ('26', '35'), ('26', '47')]}
DONE = {'35': [B12], '47': [B11], '26': [B22, B21]}
SAVE = {5: B12, 1: B11, 7: B22, 2: B21}
STAGES = {1: [(None, 1.0)], 2: [((B11, B12), .4), ((B21, B22), .6)], 'O': [((B11, B12), .5), ((B21, B22), .5)],
          3: [((B11, B12), .35), ((B22,), .37), ((B21,), .28)],
          4: [((B11,), .16), ((B12,), .26), ((B22,), .31), ((B21,), .27)]}
LAG = 8
CFG = dict(FR=(24, 16, 16, 8), CAP=0.92, PORT=0.9, CS=0.5, CL=0.3, VK=0.66, TAIL=3, EW7=12, EW6=40, MOFF=15, GE=12, NSLAB=6, JM=3)


def _dot(a, b):
    return jnp.dot(a, b, preferred_element_type=f32)


def scale(R, C, h, k):
    return 2.0 ** (R // 2 + R % 2 + h - C // 2 - C % 2 - k)


def phys(C, k):
    return 4 * (C // 2) + 2 * k + C % 2


def b_ops(b11, b12, b21, b22, final=False):
    r1 = b11 + b22
    if final:
        r1 = jax.lax.bitcast_convert_type((jax.lax.bitcast_convert_type(r1, jnp.int32) + 0x8000) & -0x10000, f32)
        b22 = r1 - b11
    g = b12 + b21
    return {1: r1, 2: b11 - b12, 3: b12 - b22, 4: g - r1, 5: b12 + b22, 6: b11 + b12, 7: g + r1}


def lincomb(terms):
    assert terms[0][0] == 1
    acc = terms[0][1]
    for s, v in terms[1:]:
        acc = acc + v if s == 1 else acc - v
    return acc


def rounds_of(p):
    if p == 1:
        return [('1', None)] + [(kind, n) for kind in KINDS for n in range(2)]
    minis = lambda kind: [(kind, r) for r in KINDS]
    return [('1', None), ('x', '1')] + minis('35') + minis('47') + [('y', '1')] * (p in GUEST) + minis('26')


def round_usage(p, rd, first, last, defer):
    stores, finals = OACT[p]
    kind, n = rd
    alu = sum(len(t.split()) - 1 for _, t in stores) + sum(len(t.split()) + (not first) + 2 * last for _, t in finals)
    nst = len(stores) + len(finals)
    if last and kind == '26':
        alu, nst = alu - 0.7 * len(finals), nst - 0.5 * len(finals)
    if defer:
        alu, nst = 0, 1
    elif p == 6 and kind != '35' and n != '35':
        nst -= 1
    if n == '1':
        a, st, m = 0, 4, 0
    elif isinstance(n, str):
        a, st, m = {'35': ((9, 3, 1), (16, 2, 2)), '47': ((10, 3, 1), (18, 2, 2)), '26': ((10, 2, 2), (18, 0, 4))}[kind][n == '26']
    else:
        a, st, m = {'1': (2, 2, 0), '35': (5, 2, 1), '47': (6, 1, 1), '26': (6, 0, 2)}[kind]
    return a + m * alu, st + m * nst


def bias_sites():
    cand = []
    for p in OUTER:
        for rd in rounds_of(p):
            kind, n = rd
            if n == '1':
                pq = [(p, q) for q in (3, 5, 4, 7)] if kind == 'x' else [(x, q) for x in (p, GUEST[p]) for q in (2, 6)]
                cand += [(p, rd, x + ('1',), (1, 0, 0, 1)) for x in pq]
            elif n in ('35', '47'):
                where = [('v', (0, 1, 1, 0))] if n == '35' else [('k', (0, 0, 1, 0)), ('m', (1, 0, 0, 0))]
                cand += [(p, rd, (p, int(q), w), pat) for q in kind for w, pat in where]
            elif n != '26':
                cand += [(p, rd, (p, int(q), (h, nn)), tuple(int(e == 2 * h + nn) for e in range(4)))
                         for q in kind for nn in ((0, 1) if kind == '1' else (n,)) for h in range(2)]
    unit = lambda b: tuple(int(x == b) for x in BLOCKS)
    sites = [(b, leaf, sub) for p in DEFER for rd in DEFER[p] for b, _ in OACT[p][1]
             for leaf in DONE[rd[0]] for sub in DONE[rd[1]]]
    rows = [np.kron(np.kron(unit(b), unit(leaf)), unit(sub)) for b, leaf, sub in sites]
    extra = {}
    def busy(c):
        a, st = round_usage(c[0], c[1], False, False, c[1] in DEFER.get(c[0], ()))
        return 2 * (a + extra.get(c[:2], 0)) + st + (5 if isinstance(c[1][1], str) else 3)
    while len(sites) < 64:
        c = min(cand, key=busy)
        cand.remove(c)
        row = np.kron(np.kron(PC[c[2][0]], PC[c[2][1]]), c[3])
        if np.linalg.matrix_rank(np.array(rows + [row])) > len(rows):
            rows.append(row)
            sites.append(c[2])
            extra[c[:2]] = extra.get(c[:2], 0) + (1 if isinstance(c[1][1], str) else 0.5)
    want = np.zeros((64, 8))
    for e, (I, J, i, j, h, n) in enumerate(np.ndindex(*(2,) * 6)):
        want[e, phys(2 * J + j, n)] = scale(2 * I + i, 2 * J + j, h, n) / GAMMA
    coef = np.round(np.linalg.solve(np.array(rows, float).T, want) * 4096) / 4096
    assert (np.array(rows).T @ coef == want).all()
    return {x: e for e, x in enumerate(sites) if coef[e].any() or isinstance(x[1], tuple)}, coef, extra


def yds(groups, cap):
    n = len(cap)
    speed, cls, gcls = [0.0] * n, [-1] * n, {}
    todo = list(groups)
    while todo:
        pre = [0.0]
        for t in range(n):
            pre.append(pre[-1] + (cap[t] if cls[t] < 0 else 0.0))
        best = None
        for a in sorted({g[0] for g in todo}):
            w = 0.0
            for g in sorted((g for g in todo if g[0] >= a), key=lambda g: g[1]):
                w += g[2]
                d = w / max(pre[g[1] + 1] - pre[a], 1e-9)
                if best is None or d > best[0]:
                    best = (d, a, g[1])
        d, a, b = best
        for t in range(a, b + 1):
            if cls[t] < 0:
                speed[t], cls[t] = d, len(gcls)
        gcls.update({g[:2]: len(gcls) for g in todo if g[0] >= a and g[1] <= b})
        todo = [g for g in todo if not (g[0] >= a and g[1] <= b)]
    return speed, cls, gcls


def spread_jobs(jobs, cap, vcap, tail):
    T = len(cap)
    cap3 = cap * 3
    all3 = [(j[0] + k * T, j[1] + k * T, ji, k) for k in range(3) for ji, j in enumerate(jobs) if j[0] + k * T >= 0]
    pend = {}
    for j in sorted(all3, key=lambda j: (j[1], j[3], j[2])):
        pend.setdefault(j[:2], []).append(j)
    left = {w: sum(sum(jobs[j[2]][2]) for j in q) for w, q in pend.items()}
    speed, cls, gcls = yds([w + (left[w],) for w in pend], cap3)
    cum = [0.0]
    for t in range(3 * T):
        cum.append(cum[-1] + speed[t] * cap3[t])
    when = [[] for _ in jobs]
    debt, vdebt, cur, done = 0.0, 0.0, None, 0

    def fits(j, t):
        need = max(debt, 0.0) + sum(jobs[j[2]][2]) + 1.0
        for w in pend:
            if w[1] >= j[1]:
                break
            if left[w] > 1e-9:
                need += left[w]
                if need > cum[w[1] + 1] - cum[t]:
                    return False
        return True

    for t in range(3 * T):
        if t % T == 0:
            debt, vdebt = min(debt, 0.0), -0.5
        while True:
            rdy = [q[0] for w, q in pend.items() if q and w[0] <= t and (gcls[w] == cls[t] or w[1] <= t)]
            j = cur
            if j is None:
                if not rdy:
                    debt = max(debt, 0.0)
                    break
                j = rdy[0]
                if j[1] > t:
                    j = (min if vdebt > 0 else max)([x for x in rdy if x is j or fits(x, t)], key=lambda x: jobs[x[2]][3])
                nst = len(jobs[j[2]][2])
                if nst > 1 and j[1] > t and (t + tail + 2 * nst) // T != t // T:
                    break
            must = j[1] <= t or (cur is not None and ((t + tail + 1) // T != t // T or (rdy and rdy[0][1] <= t)))
            if not must and (cap3[t] == 0.0 or debt > 0.5 * speed[t] * cap3[t]):
                break
            if cur is None:
                pend[j[:2]].pop(0)
                left[j[:2]] -= sum(jobs[j[2]][2])
                cur, done = j, 0
            debt += jobs[j[2]][2][done]
            vdebt += jobs[j[2]][2][done] * jobs[j[2]][3]
            if j[3] == 1:
                when[j[2]].append(t - T)
            done += 1
            if done == len(jobs[j[2]][2]):
                cur = None
        debt -= speed[t] * cap3[t]
        vdebt = min(max(vdebt - vcap[t % T], -0.5), 1.0)
    assert all(j[0] <= ts[0] and ts[-1] <= j[1] and (ts[0] < 0) == (ts[-1] < 0) for j, ts in zip(jobs, when))
    return when


def _kernel(x_hbm, w_hbm, b_hbm, o_hbm, *scratch, L, TM, R0, NMAIN, D, cfg):
    H, Mh, Mq = D // 4, TM // 4, TM // 8
    NC, NQ = Mh // 16, Mq // 16
    it = iter(scratch)
    take = lambda n: [next(it) for _ in range(n)]
    x0b, xb, ib, ob, jb = take(4), take(7), take(16), take(56), take(20)
    s2 = dict(zip(range(1, 8), take(7)))
    s3 = {(p, kind): next(it) for p in OUTER if p != 1 for kind in KINDS}
    t2 = dict(zip(range(1, 8), take(7)))
    t3_ref, kb0, kb1, bt_ref, bf_ref, xn2_ref, o2_ref, w0_ref, w_ref, xr_ref, xp_ref, b_ref, sem = it
    sites, bcoef, extra = bias_sites()
    pos2 = lambda p, q: ORD.index(q) if p == 1 else 0

    xset = lambda l: 6 if l == 'O' else 4 if l == 0 else (l % 2) * 2
    xoff = lambda I, J: 16 * ((I + J) % 2)
    xloc = lambda l, R, C, k: (xb[xset(l) + R // 2], (R % 2, C, k), xoff(R // 2, C // 2))
    x0loc = lambda R, C, k: (x0b[(R // 2) * 2 + C // 2], (R % 2, C % 2, k), 8 + xoff(R // 2, C // 2))
    iloc = lambda g, name, n: (ib[((g % 2) * 4 + ISL[name]) * 2 + n], (), 8 * ISL[name])
    oloc = lambda name, i, j, n: (ob[(OSL[name] * 4 + i * 2 + j) * 2 + n], (), 8 * ((OSL[name] + 2 * j) % 4))

    def jloc(kind, name, al, guest=False):
        u = ('1', 's', 'k').index(name)
        return jb[18 + al if guest else (KINDS.index(kind) * 3 + u) * 2 + al], (), 8 * ((3 * u + al) % 4)

    def tie(v, anchor, r=None, lo=0):
        if anchor is None:
            return v
        never, gate = anchor
        if r is None:
            n = v.shape[0]
            return jax.lax.select(never[n], gate if n == 8 else jnp.tile(gate, (n // 8, 1)), v)
        top = jax.lax.select(never[8], gate, v[r:r + 8])
        return jnp.concatenate(([v[lo:r]] if r > lo else []) + [top, v[r + 8:r + 16]], axis=0)

    def consts(anchor, ss):
        one = {s: tie(jnp.full((8, 128), s, f32), anchor) for s in set(ss)}
        return jnp.concatenate([one[s] for s in ss for _ in range(2)], axis=0)

    def conv(src, R, Q, r, zs, anchor):
        v = src[R * Mh + r:R * Mh + r + 32, Q * H:(Q + 1) * H].astype(f32)
        for j in range(2):
            C, k = 2 * (Q // 2) + j, Q % 2
            buf, idx, off = xloc(0, R, C, k)
            sv = consts(anchor, [scale(R, C, (r + u) // Mq, k) for u in (0, 16)])
            buf[(zs,) + idx + (slice(off + r, off + r + 32),)] = v[:, j * 128:(j + 1) * 128] * sv

    count = {}
    def block_sum(l, terms, ii, jj, kk, r, save, zs, za, anchor, gate=True):
        rng = lambda t: slice(t[0], t[-1] + 1)
        vals = []
        for u, ((I, J), s) in enumerate(terms):
            ref, r0 = xb[xset(l) + I], xoff(I, J) + r
            v = ref[za if u == 0 else 0, rng(ii), 2 * J + jj[0]:2 * J + jj[-1] + 1, rng(kk), r0:r0 + 16, :]
            if (I, J) == save:
                sv = consts(anchor, [GAMMA / scale(2 * I + i, 2 * J + j, r // Mq, k) for i in ii for j in jj for k in kk])
                x0b[I * 2 + J][zs, rng(ii), rng(jj), rng(kk), r0 + 8:r0 + 24, :] = v * sv.reshape(v.shape)
            if u == 0 and gate:
                count[xset(l)] = count.get(xset(l), -1) + 1
                if count[xset(l)] % cfg['GE'] == 0:
                    ref[0, 0, 0, 0, Mh + 24:Mh + 32, :] = count.get('prev', anchor)[1]
                count['prev'] = anchor
            vals.append((s, v))
        v = lincomb(vals)
        return v.reshape(v.size // 128, 128)

    def operands(a, group, st8, store):
        for u, b in enumerate(group):
            st8[b] = a if len(group) == 1 else a[:, u:u + 1]
        ops = {}
        if B12 in group:
            ops[3], ops[5] = st8[B11] - st8[B12], st8[B11] + st8[B12]
        if B22 in group:
            ops[4], ops[7] = st8[B12] + st8[B22], st8[B12] - st8[B22]
            ops[1] = st8['l1'] = st8[B11] + st8[B22]
        if B21 in group:
            g = st8[B12] + st8[B21]
            ops[2], ops[6] = g + st8['l1'], g - st8['l1']
        now = [q for q in ORD if q in ops]
        if now:
            u = ORD.index(now[0])
            store(slice(u, u + len(now)), jnp.concatenate([ops[q] for q in now], axis=1).astype(bf16))

    def unit1(l, c, k, save, st8, group, zs, za, anchor):
        def store(pos, v):
            s2[1][zs, k:k + 1, pos, 16 * c:16 * c + 16, :] = v
        e = block_sum(l, LA[1], [group[0][0]], [0, 1], [k], 16 * c, save, zs, za, anchor)
        operands(tie(e, anchor, 16).reshape(1, 2, 16, 128), group, st8, store)

    def unit26(l, c, k, save, st8, group, zs, za, anchor):
        i = group[0][0]
        f = block_sum(l, [(B11, 1), (B22, 1)], [i], [0, 1], [k], 16 * c, save, zs, za, anchor, False)
        e = tie(block_sum(l, [(B12, 1), (B21, 1)], [i], [0, 1], [k], 16 * c, save, zs, za, anchor), anchor)
        for J, v in enumerate((e + f, e - f)):
            r0 = xoff(0, J) + 16 * c
            xb[6][zs, i, 2 * J:2 * J + 2, k, r0:r0 + 16, :] = v.reshape(2, 16, 128)

    def unit3(l, p, kind, c, save, st8, group, zs, za, anchor):
        def store(pos, v):
            s3[(p, kind)][zs, :, pos, 16 * c:16 * c + 16, :] = v
        h, kk = group[0][0], [b[1] for b in group]
        ii, jj = {'35': ([0], [0, 1]), '47': ([0, 1], [1]), '26': ([0, 1], [0, 1])}[kind]
        src = (l, LA[p]) if p in LA else ('O', [((0, (2, 6).index(p)), 1)])
        n = 16 * len(kk)
        v = block_sum(*src, ii, jj, kk, h * Mq + 16 * c, save, zs, za, anchor)
        if kind == '26':
            e, f = tie(v, anchor, 16, 16) + v[32:48], v[0:16] + v[48:64]
            r0 = h * Mq + 16 * c
            s2[p][zs, kk[0], 0, r0:r0 + 16, :] = f.astype(bf16)
        else:
            e, f = tie(v, anchor, n - 16), v[n:]
        operands(jnp.concatenate([e + f, e - f], axis=0).reshape(2, len(kk), 16, 128), group, st8, store)

    GAPS = [w for pos in range(4) for w in [1] + [x for p in (2, 6, 3, 5, 1, 4, 7) for x in (
        [19] if p == 1 else [25] if pos < 3 else [13] + [19] * 6)]]

    def wtile(idx, n):
        if cfg.get('NOBC'):
            return w_ref[idx].reshape(16 * n, 128)
        return pltpu.bitcast(w_ref.at[idx].bitcast(u32)[...].reshape(8 * n, 128), bf16)

    def prep(l, u, anchors, zero, kb):
        mul = lambda v, s: v if s == 1.0 else v * s
        stack = lambda T: jnp.concatenate([T[q] for q in ORD], axis=0).reshape(7, 16, 128).astype(bf16)
        rows = pl.ds(16 * u, 16) if isinstance(u, int) else pl.ds(pl.multiple_of(16 * u, 16), 16)
        for k in range(2):
            if isinstance(l, int):
                wide = [w0_ref[phys(R, k), u].astype(f32) for R in range(4)]
                tile = lambda R, c: wide[R][:, c * 128:(c + 1) * 128]
            else:
                wide = [wtile((l - 1, slice(None), phys(R, k), u), 8).astype(f32) for R in range(4)]
                tile = lambda R, c: wide[R][c * 16:(c + 1) * 16]
            for n in range(2):
                anchor = next(anchors)
                blk = lambda R, C: mul(tile(R, phys(C, n)), scale(R, C, k, n))
                O = {(i, j): b_ops(blk(i, j), tie(blk(i, 2 + j), anchor, 0), blk(2 + i, j), blk(2 + i, 2 + j))
                     for i, j in BLOCKS}
                for p in (2, 6, 3, 5, 1, 4, 7):
                    o = [mul(O[b][p], 4.0 if p == 1 else 1.0) for b in BLOCKS]
                    T = b_ops(o[0], tie(o[1], next(anchors), 0), o[2], o[3], True)
                    if p == 1:
                        T[1] = T[1] * 2.0
                        t2[p][l, n, k, :, rows, :] = stack(T)
                        continue
                    t2[p][l, n, k, 0, rows, :] = (T[1] * 4.0).astype(bf16)
                    e0 = PRODS3.index((p, 5))
                    if (k, n) != (1, 1):
                        kb[zero, k * 2 + n, 16 * e0:16 * e0 + 96, :] = jnp.concatenate(
                            [T[q] for _, q in PRODS3[e0:e0 + 6]], axis=0)
                        continue
                    for e in range(e0, e0 + 6):
                        v = kb[0, 0:3, 16 * e:16 * e + 16, :]
                        T3 = b_ops(v[0], tie(v[1], next(anchors), 0), v[2], T[PRODS3[e][1]], True)
                        T3[1] = T3[1] * 2.0
                        t3_ref[l, e, :, rows, :] = stack(T3)

    outs = [(l, p) for l in range(L) for p in OUTER]
    G = len(outs)
    sched, start, use, vuse = [], [], [], []
    for g, (l, p) in enumerate(outs):
        start.append(len(use))
        for rd in rounds_of(p):
            n = NQ if isinstance(rd[1], str) else NC
            sched.append((g, rd, len(use), n))
            a, st_ = round_usage(p, rd, l == 0, l == L - 1, rd in DEFER.get(p, ()))
            a += extra.get((p, rd), 0)
            use += [max((2 * a + st_ + 2 + 16 / n) / 72, cfg['PORT'] * st_ / 8)] * n
            vuse += [st_ / 8] * n
    T = len(use)
    first = lambda g, kind: next(t0 for gg, rd, t0, _ in sched if gg == g and rd[0] == kind)
    jobs, late = [], []
    def add(lo, hi, alu, st_, ld_, scheme, kind, fn):
        w = alu / 64 + cfg['CS'] * (st_ + len(STAGES[scheme])) / 16 + cfg['CL'] * ld_ / 48
        jobs.append((lo, max(hi, lo), [w * f for _, f in STAGES[scheme]], st_ / 16 / w, scheme, kind, fn))
    for g, (l, p) in enumerate(outs):
        for gg, rd, t0, n_ in sched:
            if gg == g and rd in DEFER.get(p, ()):
                last = l == L - 1
                nops = sum(len(t.split()) + 1 + (l > 0) + 1.5 * last for _, t in OACT[p][1])
                islate = last and p == 6 and rd[0] == '26'
                due = {5: lambda: start[7 * l + 5] - 1, 7: lambda: start[g + 1] + cfg['EW7'],
                       6: lambda: T - cfg['TAIL'] - 1 if last else min(start[g + 1] + cfg['EW6'], first(g + 1, rd[0])) - 1}[p]()
                both = last and rd[0] == '26'
                step = cfg['FR'][(p == 6) + 2 * both]
                for r0 in range(0, Mq, step):
                    nr = min(step, Mq - r0)
                    for h, n in DONE[rd[1]]:
                        for leaves in [DONE[rd[0]]] if both else [[b] for b in DONE[rd[0]]]:
                            fn = (l, p, leaves, h, n, r0, nr)
                            nv = len(leaves) * nr // 8
                            add(0 if islate else t0 + n_, cfg['EW6'] - 1 if islate else due, nops * nv,
                                nv * len(OACT[p][1]) / (1 + both) - 1, 0.9 * nops * nv, 1, 'fin', fn)
                            if islate:
                                late.append(fn)
        if p in (3, 5):
            lo = start[7 * l - 2] + (cfg['EW7'] + 1 if l else -T)
        else:
            lo = start[7 * l] + cfg['EW6']
        hi = start[g] - LAG - 3
        save = SAVE.get(p) if l == 0 else None
        sv = save is not None
        if p == 1:
            for c, k in np.ndindex(NC, 2):
                add(lo, hi, 31 + 8 * sv, 7 + 8 * sv, 16, 2, l, functools.partial(unit1, l, c, k, save))
            continue
        nt = 2
        if p in (2, 6):
            mid = start[7 * l + 3] + cfg['MOFF']
            if p == 2:
                for c, k in np.ndindex(NC, 2):
                    add(lo, mid - 3, 40 + 8 * sv, 16 + 8 * sv, 32, 'O', l, functools.partial(unit26, l, c, k, save))
            lo, nt, save, sv = mid, 1, None, False
        for c in range(NQ):
            add(lo, hi if p in GUEST else first(g - 1, 'y') - LAG - 3, 32 * nt + 50 + 32 * sv, 18 + 32 * sv, 32 * nt,
                4, l, functools.partial(unit3, l, p, '26', c, save))
        for c in range(NQ):
            for kind in KINDS[:2]:
                add(lo, hi + (NC if g else 0), 16 * nt + 46, 14, 16 * nt, 3, l, functools.partial(unit3, l, p, kind, c, None))
    convs = [(R, Q, r) for R in range(4) for Q in range(4) for r in range(0, Mh, 32)]
    for x in convs:
        add(start[6], start[G - 2] - 2, 18, 7, 4, 1, 'conv', x)
    cap = [max(cfg['CAP'] - max(use[t], use[(t + 1) % T]), 0.0) * (t < T - cfg['TAIL']) for t in range(T)]
    when = spread_jobs(jobs, cap, [cfg['VK'] * (1 - vuse[(t + 1) % T]) for t in range(T)], cfg['TAIL'])
    plan = {}
    for t, _, ji, u in sorted((t % T, ts[0] % T, ji, u) for ji, ts in enumerate(when) for u, t in enumerate(ts)):
        plan.setdefault(t, []).append((jobs[ji][5], jobs[ji][6], STAGES[jobs[ji][4]][u][0]))
    assert cfg['EW6'] <= first(0, '26')
    carried = [job for ts, job in zip(when, jobs) if ts[0] < 0]

    def w_copy(l, c=None):
        if c is None:
            return pltpu.make_async_copy(w_ref.at[l - 1], w_ref.at[l - 1], sem.at[l])
        return pltpu.make_async_copy(w_hbm.at[l, :, :, :, pl.ds(c * 128, 128)], w_ref.at[l - 1, c], sem.at[l])

    def w0_copy(u):
        return pltpu.make_async_copy(w_hbm.at[0, :, u], w0_ref.at[:, u], sem.at[L + 6 + u])

    def in_copy(t, slot):
        return pltpu.make_async_copy(x_hbm.at[pl.ds(pl.multiple_of(t * TM, 32), TM)], xn2_ref.at[slot], sem.at[L + slot])

    def out_copy(t, slot, part):
        r0, nr = (0, TM) if part is None else ((0, 4 * Mq), (4 * Mq, Mq), (5 * Mq, Mq), (6 * Mq, 2 * Mq))[part]
        return pltpu.make_async_copy(o2_ref.at[slot, pl.ds(r0, nr)],
                                     o_hbm.at[pl.ds(pl.multiple_of(t * TM + r0, 16), nr)], sem.at[L + 4 + slot])

    xr_in = pltpu.make_async_copy(x_hbm.at[pl.ds(NMAIN * TM, R0)], xr_ref, sem.at[L + 2])
    xr_out = pltpu.make_async_copy(xr_ref, o_hbm.at[pl.ds(NMAIN * TM, R0)], sem.at[L + 2])
    b_in = pltpu.make_async_copy(b_hbm, b_ref, sem.at[L + 3])
    opaque = lambda i, s: jax.lax.shift_right_logical(i, s)
    mask = lambda zero: {n: jnp.broadcast_to(zero, (n, 128)) != 0 for n in (8, 16, 32)}

    def prologue():
        b_in.start()
        for u in range(8):
            w0_copy(u).start()
        xr_in.start()
        in_copy(0, 0).start()
        b_in.wait()
        for l in range(L):
            bf_ref[l] = b_ref[l:l + 1, :].astype(f32)

        def bias_tiles(l, carry):
            b = jnp.broadcast_to(bf_ref[l] + (l == 0).astype(f32), (8, D))
            for u in sites.values():
                terms = [b[:, e * 128:(e + 1) * 128] * float(cf) for e, cf in enumerate(bcoef[u]) if cf != 0.0]
                bt_ref[l, u] = functools.reduce(lambda x, y: x + y, terms or [jnp.zeros((8, 128), f32)])
            return carry
        jax.lax.fori_loop(0, L, bias_tiles, 0)
        if cfg.get('FAST'):
            return

        def slab(u, carry):
            w0_copy(u).wait()
            prep(0, u, iter(lambda: None, 0), opaque(u, 12), kb0)
            return opaque(u, 12)
        zero = jax.lax.fori_loop(0, cfg['NSLAB'], slab, 0)

        halves = lambda x: (x[:, :D // 2].astype(bf16), x[:, D // 2:].astype(bf16))

        def plain(l, xbf, x0f, x, j0, j1, gaps, free, never):
            passes = []
            for jt in range(j0, j1):
                cols = slice(jt * 128, (jt + 1) * 128)
                w = [w0_ref[b:b + 4, :, :, cols].reshape(D // 2, 128) if isinstance(l, int)
                     else wtile((l - 1, jt, slice(b, b + 4)), 32) for b in (0, 4)]
                ya = _dot(xbf[0], w[0]) + bf_ref[l, :, cols]
                passes += [ya, _dot(xbf[1], w[1]) + ya]
            xp_ref[0, :, j0 * 128:j1 * 128] = x0f * jnp.concatenate(passes[1::2], axis=1) + x
            for u in range(len(gaps)):
                ps, rr = divmod(sum(gaps[free:u]) * len(passes) * (R0 // 8) // sum(gaps[free:]), R0 // 8)
                yield None if u < free else (never, passes[ps][rr * 8:rr * 8 + 8, :])

        for l in range(1, L):
            for c in range(8):
                w_copy(l, c).start()
        in_copy(1, 1).start()
        for u in range(cfg['NSLAB'], 8):
            w0_copy(u).wait()
        xr_in.wait()
        jm = cfg['JM']
        x0f = xr_ref[:, :jm * 128].astype(f32)
        xp_ref[1, :, :jm * 128] = x0f
        anchors = plain(0, halves(xr_ref), x0f, x0f, 0, jm, (8 - cfg['NSLAB']) * GAPS, 2, mask(zero))
        for u in range(cfg['NSLAB'], 8):
            prep(0, u, anchors, zero, (kb0, kb1)[u % 2])
        in_copy(0, 0).wait()
        x0f = xr_ref[:, jm * 128:].astype(f32)
        xp_ref[1, :, jm * 128:] = x0f
        blank = [loc for j, n in BLOCKS for loc in [oloc(x, 1, j, n) for x in OSL]
                 + [f(3, 2 * J + j, n) for J in range(2) for f in (x0loc, functools.partial(xloc, L - 1))]]
        na = len(convs) + sum(len(j[2]) for j in carried) + 2 * len(blank) + 2
        anchors = plain(0, halves(xr_ref), x0f, x0f, jm, 8, [1] * na, 4, mask(zero))
        for x in convs[:len(convs) // 2]:
            conv(xn2_ref.at[0], *x, zero, next(anchors))
        for job in carried:
            st8 = {}
            for group, _ in STAGES[job[4]]:
                job[6](st8, group, zero, opaque(zero, 1), next(anchors))
        for x in convs[len(convs) // 2:]:
            conv(xn2_ref.at[0], *x, zero, next(anchors))
        for ref, idx, off in blank:
            for r0 in (off, off + Mq):
                ref[(0,) + idx + (slice(r0, r0 + Mq),)] = consts(next(anchors), [0.0] * NQ)

        def layer(l, carry):
            w_copy(l).wait()
            x, zero = xp_ref[0], opaque(l, 12)
            anchors = plain(l, halves(x), xp_ref[1], x, 0, 8, 8 * GAPS, 2, mask(zero))
            for u in range(8):
                prep(l, u, anchors, zero, (kb0, kb1)[u % 2])
            return carry

        jax.lax.fori_loop(1, L, layer, 0)
        xr_ref[...] = xp_ref[0].astype(bf16)
        xr_out.start()

    def main(tile, carry, only_late=False):
        zs, za = opaque(tile, 12), opaque(tile, 13)
        never = mask(zs)
        slot = tile % 2
        out = [o2_ref.at[1 - slot]]

        def rows(h, r0):
            lo, n = (0, Mh) if h is None else h if isinstance(h, tuple) else (h * Mq, Mq)
            return slice(r0 + lo, r0 + lo + n)

        def ld(loc, h, z=0):
            return loc[0][(z,) + loc[1] + (rows(h, loc[2]),)]

        def st(loc, v, h, z=zs):
            loc[0][(z,) + loc[1] + (rows(h, loc[2]),)] = v

        def operand(ref, idx, n):
            if cfg.get('NOBC'):
                return ref[idx + (slice(0, n),)]
            return pltpu.bitcast(ref.at[idx + (pl.ds(0, n),)].bitcast(u32)[...], bf16)

        def dot3(l, p, q, r):
            kind = next(x for x in KINDS if q in PAIR[x])
            return _dot(operand(s3[(p, kind)], (0, PAIR[kind].index(q), ORD.index(r)), Mq),
                        operand(t3_ref, (l, PRODS3.index((p, q)), ORD.index(r)), 128))

        def issue(l, p, rd):
            kind, n = rd
            if kind == 'x':
                return [dot3(l, p, q, 1) for q in (3, 5, 4, 7)]
            if kind == 'y':
                return [dot3(l, x, q, 1) for x in (p, GUEST[p]) for q in (2, 6)]
            if isinstance(n, str):
                return [dot3(l, p, int(q), int(r)) for q in kind for r in n]
            lhs = {q: [operand(s2[p], (0, k, pos2(p, q)), Mh) for k in range(2)] for q in map(int, kind)}
            return [_dot(lhs[q][k], operand(t2[p], (l, nn, k, pos2(p, q)), 128))
                    for q, nn in ([(1, 0), (1, 1)] if kind == '1' else [(int(q), n) for q in kind]) for k in range(2)]

        def biased(v, l, *site):
            if site not in sites:
                return v
            return (v.reshape(Mq // 8, 8, 128) + bt_ref[l, sites[site]]).reshape(Mq, 128)

        wait = {}
        def outer_act(l, p, i, j, n, d, h, part=None, last=lambda b, y: y):
            stores, finals = OACT[p]
            if part == 'park':
                stores, finals = stores[:1], []
            elif part == 'rest' or (p == 6 and (i, j) != B12 and (h, n) != B12):
                stores = stores[1:]
            cache = {'d': d}
            def comb(terms):
                for t in terms.split():
                    if t[1:] not in cache:
                        cache[t[1:]] = ld(oloc(t[1:], i, j, n), h)
                return lincomb([(int(t[0] + '1'), cache[t[1:]]) for t in terms.split()])
            fin = [(IJ, last(IJ, comb(terms))) for IJ, terms in finals]
            for name, v in [(name, comb(terms)) for name, terms in stores]:
                st(oloc(name, i, j, n), v, h, za if (h, n) == B22 else zs)
            for (I, J), y in fin:
                R, C = 2 * I + i, 2 * J + j
                xn = ld(x0loc(R, C, n), h) * y
                if l > 0:
                    xn = xn + ld(xloc(l, R, C, n), h)
                if l < L - 1:
                    st(xloc(l + 1, R, C, n), xn, h)
                    continue
                s = scale(R, C, rows(h, 0).start // Mq, n)
                xn = xn if s == 1.0 else xn * (1.0 / s)
                c0 = phys(C, n) * 128
                if i == 0:
                    out[0][rows(h, R * Mh), c0:c0 + 128] = xn.astype(bf16)
                elif j == 1:
                    wait[J] = xn
                else:
                    out[0][rows(h, R * Mh), c0:c0 + 256] = jnp.concatenate([xn, wait.pop(J)], axis=1).astype(bf16)

        def inner_act(g, l, p, kind, n, h, P, Q, part=None):
            vloc = iloc(g, 'v', n) if p == 1 else oloc(OACT[p][0][0][0], 0, 1, n)
            if kind == '35':
                st(iloc(g, 's', n), Q + ld(iloc(g, 'm1', n), h), h)
                if p == 1:
                    st(vloc, P, h)
                outer_act(l, p, 0, 1, n, P, h, part)
            elif kind == '47':
                st(iloc(g, 'u', n), Q + ld(vloc, h), h)
                outer_act(l, p, 0, 0, n, P + ld(iloc(g, 's', n), h), h, part)
            else:
                outer_act(l, p, 1, 1, n, ld(iloc(g, 's', n), h) - Q, h, part)
                outer_act(l, p, 1, 0, n, P + ld(iloc(g, 'u', n), h), h, part)

        def consume(g, l, p, rd, res):
            kind, n = rd
            if n == '1':
                for u, (kd, x) in enumerate([('35', p), ('47', p)] if kind == 'x' else [('26', p), ('26', GUEST[p])]):
                    for al in range(2):
                        st(jloc(kd, '1', al, x != p), biased(res[2 * u + al], l, x, int(kd[al]), '1'), 0)
            elif isinstance(n, str):
                sm = [res[2 * al] + res[2 * al + 1] for al in range(2)]
                df = [res[2 * al] - res[2 * al + 1] for al in range(2)]
                J = lambda name, al: ld(jloc(kind, name, al, name == '1' and kind == '26' and p not in GUEST), 0)
                part = 'park' if rd in DEFER.get(p, ()) else None
                done = lambda h, nn, m: inner_act(g, l, p, kind, nn, h, m[0] + m[1], m[0] - m[1], part)
                if n == '35':
                    for al in range(2):
                        st(jloc(kind, 's', al), df[al] + J('1', al), 0)
                    done(0, 1, [biased(sm[al], l, p, int(kind[al]), 'v') for al in range(2)])
                elif n == '47':
                    for al in range(2):
                        st(jloc(kind, 'k', al), biased(df[al], l, p, int(kind[al]), 'k'), 0)
                    done(0, 0, [biased(sm[al] + J('s', al), l, p, int(kind[al]), 'm') for al in range(2)])
                else:
                    O = lambda i, j: ld(oloc(OACT[p][0][0][0], i, j, 1), 0, za if (i, j) in DONE[kind] else 0)
                    m = [sm[al] + J('k', al) for al in range(2)]
                    P = m[0] + m[1] + O(*{'35': B12, '47': B11, '26': B21}[kind])
                    Q = m[0] - m[1] - (ld(iloc(g, 'm1', 1), 0) if kind == '35' else O(*{'47': B12, '26': B22}[kind]))
                    done(1, 1, [J('s', al) - df[al] for al in range(2)])
                    inner_act(g, l, p, kind, 0, 1, P, Q, part)
            else:
                m = []
                for al, (q, nn) in enumerate([(1, 0), (1, 1)] if kind == '1' else [(int(q), n) for q in kind]):
                    v = res[2 * al] + res[2 * al + 1]
                    if any((p, q, (h, nn)) in sites for h in range(2)):
                        v = jnp.concatenate([biased(v[h * Mq:(h + 1) * Mq], l, p, q, (h, nn)) for h in range(2)], axis=0)
                    m.append(v)
                if kind == '1':
                    for nn in range(2):
                        st(iloc(g, 'm1', nn), m[nn], None)
                else:
                    inner_act(g, l, p, kind, n, None, m[0] + m[1], m[0] - m[1])

        def finish(l, p, leaves, h, n, r0, nr, anchor):
            for i, j in leaves:
                d = ld(oloc(OACT[p][0][0][0], i, j, n), (h * Mq + r0, nr))
                last = lambda b, y: (y.reshape(nr // 8, 8, 128)
                                     + tie(bt_ref[l, sites[(b, (i, j), (h, n))]], anchor)).reshape(nr, 128)
                outer_act(l, p, i, j, n, d, (h * Mq + r0, nr), 'rest', last)

        if only_late:
            for x in late:
                finish(*x, None)
            out_copy(tile - 1, 1 - slot, 3).start()
            return carry
        state = {}
        count.clear()
        for g, rd, t0, n in sched:
            l, p = outs[g]
            if t0 == start[1]:
                pl.when(tile > 0)(lambda: out_copy(tile - 1, 1 - slot, 3).start())
                out[0] = o2_ref.at[slot]
            if t0 == first(G - 2, '35'):
                assert t0 > start[G - 2] + cfg['EW7']
                out_copy(tile, slot, 0).start()
            res = issue(l, p, rd)
            if t0 == first(G - 2, '35'):
                out[0][TM - 8:TM, 0:128] = res[0][0:8, :].astype(bf16)
            for t in range(t0, t0 + n):
                if t in plan:
                    r0 = 16 * (t - t0) + 8
                    anchor = (never, res[0 if isinstance(rd[1], str) else 1][r0:r0 + 8, :])
                for kind, fn, group in plan.get(t, []):
                    if kind == 'fin':
                        finish(*fn, anchor)
                    elif kind == 'conv':
                        conv(xn2_ref.at[1 - slot], *fn, zs, anchor)
                    else:
                        fn(state.setdefault(id(fn), {}), group, zs, za, anchor)
            if t0 == first(G - 1, '26'):
                out_copy(tile, slot, 1).start()
            if t0 + n == T:
                out_copy(tile, slot, 2).start()
            consume(g, l, p, rd, res)
        pl.when(tile + 3 < NMAIN)(lambda: in_copy(tile + 3, 1 - slot).start())
        pl.when(tile > 0)(lambda: out_copy(tile - 1, 1 - slot, None).wait())
        pl.when(tile + 2 < NMAIN)(lambda: in_copy(tile + 2, slot).wait())
        return carry

    prologue()
    in_copy(2, 0).start()
    in_copy(1, 1).wait()
    jax.lax.fori_loop(0, NMAIN, main, 0)
    main(jnp.int32(NMAIN), 0, True)
    xr_out.wait()
    out_copy(NMAIN - 1, (NMAIN - 1) % 2, None).wait()


def build(TM=640, **kw):
    def f(x0, ws, bs):
        B, D = x0.shape
        L = ws.shape[0]
        Mh = TM // 4
        nmain = (B - 1) // TM
        R0 = B - nmain * TM
        assert D == 1024 and L % 2 == 0 and L <= 8 and TM % 128 == 0 and R0 % 16 == 0 and nmain >= 3
        n3 = len(PRODS3)
        odd = lambda n: 16 * (n // 16 | 1)
        V = pltpu.VMEM
        scratch = ([V((1, 2, 2, 2, Mh + 40, 128), f32)] * 4 + [V((1, 2, 4, 2, Mh + 40, 128), f32)] * 7
                   + [V((1, Mh + 32, 128), f32)] * (16 + 56 + 20)
                   + [V((1, 2, 10 if p == 1 else 2, odd(Mh), 128), bf16) for p in range(1, 8)]
                   + [V((1, 2, 10, odd(Mh // 2), 128), bf16)] * (n3 // 2)
                   + [V((L, 2, 2, 7 if p == 1 else 1, 128, 128), bf16) for p in range(1, 8)]
                   + [V((L, n3, 7, 128, 128), bf16)] + [V((1, 4, 16 * n3 + 16, 128), f32)] * 2
                   + [V((L, 64, 8, 128), f32), V((8, 1, D), f32), V((2, TM, D), bf16), V((2, TM, D), bf16),
                      V((8, 8, 16, D), bf16), V((L - 1, 8, 8, 8, 16, 128), bf16), V((R0, D), bf16), V((2, R0, D), f32), V((L, D), bf16),
                      pltpu.SemaphoreType.DMA((L + 14,))])
        anyspec = pl.BlockSpec(memory_space=pl.ANY)
        return pl.pallas_call(
            functools.partial(_kernel, L=L, TM=TM, R0=R0, NMAIN=nmain, D=D, cfg=dict(CFG, **kw)),
            in_specs=[anyspec, anyspec, anyspec],
            out_specs=anyspec,
            out_shape=jax.ShapeDtypeStruct((B, D), x0.dtype),
            scratch_shapes=scratch,
            compiler_params=pltpu.CompilerParams(
                vmem_limit_bytes=120 * 1024 * 1024,
                internal_scratch_in_bytes=65536,
                disable_bounds_checks=True,
                disable_semaphore_checks=True,
            ),
        )(x0, ws.reshape(L, 8, 8, 16, D), bs)
    return f


@jax.jit
def pallas_standalone__dcn_v2_cross__recsys_kernel(x0, ws, bs):
    return build()(x0, ws, bs)
```
